```python
import jax
import jax.numpy as jnp

def _softmax(x, axis=-1):
    return jax.nn.softmax(x, axis=axis)
def _gelu(x):
    return jax.nn.gelu(x, approximate=True)
def _silu(x):
    return jax.nn.silu(x)
def _sigmoid(x):
    return jax.nn.sigmoid(x)
def _layernorm(x, axis=-1, eps=1e-5):
    m = jnp.mean(x, axis=axis, keepdims=True)
    v = jnp.var(x, axis=axis, keepdims=True)
    return (x - m) / jnp.sqrt(v + eps)
def _scatter_add(tgt, idx, src, axis=0):
    return tgt.at[idx].add(src)
def _segment_sum(src, seg, n):
    return jax.ops.segment_sum(src, seg, n)
class _Rng:
    def __init__(self, key):
        self._k = key
    def _next(self):
        self._k, sub = jax.random.split(self._k)
        return sub
    def normal(self, shape):
        return jax.random.normal(self._next(), shape, dtype=jnp.bfloat16)
    def randint(self, lo, hi, shape):
        return jax.random.randint(self._next(), shape, lo, hi, dtype=jnp.int32)
    def uniform(self, shape, lo=0.0, hi=1.0):
        return jax.random.uniform(self._next(), shape, jnp.bfloat16, lo, hi)
    def permutation(self, n):
        return jax.random.permutation(self._next(), n)


kernel_name = 'interleave_layers__sliding_local_dilated__glu_gated_geglu__prompt'

def setup_inputs():
    _rng = _Rng(jax.random.key(int.from_bytes(__import__("os").urandom(4), "little")))
    _w = (lambda a: (lambda t: t.astype(jnp.bfloat16) if jnp.issubdtype(t.dtype, jnp.floating) else t)(jnp.asarray(a)))
    def _A_setup():
        B, S, D = 1, 2048, 576
        return {
            "x": _w((lambda *s: _rng.normal(s) * 0.05)(B, S, D)),
            "wqkv": _w((lambda *s: _rng.normal(s) * 0.05)(D, 3 * D)),
            "wo": _w((lambda *s: _rng.normal(s) * 0.05)(D, D)),
        }
    _A_in = _A_setup()

    def _B_setup():
        B, S, Dm, Df = 1, 2048, 576, 4608
        return {
            "x": _w((lambda *s: _rng.normal(s) * 0.05)(B, S, Dm)),
            "w_gate": _w((lambda *s: _rng.normal(s) * 0.05)(Dm, Df) * (Dm ** -0.5)),
            "w_up": _w((lambda *s: _rng.normal(s) * 0.05)(Dm, Df) * (Dm ** -0.5)),
            "w_down": _w((lambda *s: _rng.normal(s) * 0.05)(Df, Dm) * (Df ** -0.5)),
        }
    _B_in = _B_setup()

    return {
        "A_x": _A_in["x"],
        "A_wqkv": _A_in["wqkv"],
        "A_wo": _A_in["wo"],
        "B_x": _B_in["x"],
        "B_w_gate": _B_in["w_gate"],
        "B_w_up": _B_in["w_up"],
        "B_w_down": _B_in["w_down"],
    }

def reference(A_x, A_wqkv, A_wo, B_x, B_w_gate, B_w_up, B_w_down):
    def _A_ref(x, wqkv, wo):
        B, S, D = x.shape
        H = 32; Dh = D // H
        W, dil = 8, 2
        qkv = (lambda x, *d: x.transpose(*d))((x @ wqkv).reshape(B, S, 3, H, Dh), 2, 0, 3, 1, 4)
        q, k, v = qkv[0], qkv[1], qkv[2]
        scale = Dh ** -0.5
        pos = jnp.arange(S)
        off = jnp.arange(W) * dil
        idx = pos[:, None] - off[None, :]
        mask = idx >= 0
        idx_c = jnp.where(mask, idx, 0).reshape(-1)
        kg = k[:, :, idx_c, :].reshape(B, H, S, W, Dh)
        vg = v[:, :, idx_c, :].reshape(B, H, S, W, Dh)
        logits = jnp.einsum("bhsd,bhswd->bhsw", q, kg) * scale
        logits = jnp.where(mask[None, None, :, :], logits, -1e9)
        attn = _softmax(logits, axis=-1)
        o = jnp.einsum("bhsw,bhswd->bhsd", attn, vg)
        return (lambda x, *d: x.transpose(*d))(o, 0, 2, 1, 3).reshape(B, S, D) @ wo

    def _B_ref(x, w_gate, w_up, w_down):
        g = jnp.einsum("bsd,df->bsf", x, w_gate)
        u = jnp.einsum("bsd,df->bsf", x, w_up)
        h = _gelu(g) * u
        return jnp.einsum("bsf,fd->bsd", h, w_down)

    x = A_x
    x = x + _A_ref(_layernorm(x, axis=-1), A_wqkv, A_wo)
    x = x + _B_ref(_layernorm(x, axis=-1), B_w_gate, B_w_up, B_w_down)
    x = x + _A_ref(_layernorm(x, axis=-1), A_wqkv, A_wo)
    x = x + _B_ref(_layernorm(x, axis=-1), B_w_gate, B_w_up, B_w_down)
    return x
```

```python
import functools
import math
import jax
import jax.numpy as jnp
from jax import lax
import jax.experimental.pallas as pl
import jax.experimental.pallas.tpu as pltpu

H = 32
DH = 18
W = 8
DIL = 2
HALO = 16
EPS = 1e-5
TB = 128
TM = 256
NH = 2
TF = 384
RB = 8
KP = 640
NQKV = 14 * 128
QKV_AT = 0
WO_AT = 4

f32 = jnp.float32
bf16 = jnp.bfloat16
NT = (((1,), (1,)), ((), ()))


def _ln_t(x):
    m = jnp.mean(x, axis=0, keepdims=True)
    xc = x - m
    v = jnp.mean(xc * xc, axis=0, keepdims=True)
    return xc * lax.rsqrt(v + EPS)


def _dst_row(sec, d):
    if sec == 0:
        return d * 32 if d < 16 else 1024 + (d - 16) * 32
    if sec == 1:
        return 512 + d * 32 if d < 16 else 13 * 128 + (d - 16) * 32
    return 9 * 128 + d * 32 if d < 16 else 1024 + 64 + (d - 16) * 32


def _kernel(x_ref, wqkv_hbm, wo_hbm, wg_hbm, wu_hbm, wd_hbm, o_ref,
            wqkv_raw, wo_raw, wqkvT, woT, wgu_v, wd_v, tmp, qkv_s, xres, xn_s, sems, *, D, DF, NB):
    s = pl.program_id(0)
    FH = DF // NH
    ncf = FH // TF
    nsteps = 2 * NB + NH

    def cp_qkv():
        return pltpu.make_async_copy(wqkv_hbm, wqkv_raw, sems.at[0])

    def cp_wo():
        return pltpu.make_async_copy(wo_hbm, wo_raw, sems.at[1])

    def ffn_copies(hf):
        cps = []
        for c in range(ncf):
            col = hf * FH + c * TF
            cps.append(pltpu.make_async_copy(wg_hbm.at[:, pl.ds(col, TF)], wgu_v.at[hf, c, :, pl.ds(0, TF)], sems.at[2 + hf]))
            cps.append(pltpu.make_async_copy(wu_hbm.at[:, pl.ds(col, TF)], wgu_v.at[hf, c, :, pl.ds(TF, TF)], sems.at[2 + hf]))
        cps.append(pltpu.make_async_copy(wd_hbm.at[:, pl.ds(hf * FH, FH)], wd_v.at[hf], sems.at[2 + hf]))
        return cps

    @pl.when(s == 0)
    def _():
        cp_qkv().start()
        cp_wo().start()
        for hf in range(NH):
            for cp in ffn_copies(hf):
                cp.start()
        qkv_s[:, pl.ds(TB, HALO), :] = jnp.zeros((14, HALO, 128), f32)
        zpad = jnp.zeros((KP - D, 128), f32)
        cp_qkv().wait()
        for j in range(14):
            wd_ = 128 if j < 13 else 64
            blk = wqkv_raw[:, j * 128:j * 128 + wd_].astype(f32)
            if wd_ < 128:
                blk = jnp.concatenate([blk, jnp.zeros((D, 128 - wd_), f32)], axis=1)
            bt = jnp.concatenate([blk, zpad], axis=0).T
            for t in range(5):
                tmp[t, pl.ds(j * 128, 128), :] = bt[:, t * 128:(t + 1) * 128]
        for sec in range(3):
            for d in range(DH):
                r = _dst_row(sec, d)
                for t in range(5):
                    wqkvT[pl.ds(r, 32), t * 128:(t + 1) * 128] = tmp[t, pl.ds(sec * D + d, 32, stride=DH), :].astype(bf16)
        wqkvT[pl.ds(13 * 128 + 64, 64), :] = jnp.zeros((64, KP), bf16)
        cp_wo().wait()
        for t in range(5):
            wd_ = 128 if t < 4 else 64
            blk = wo_raw[:, t * 128:t * 128 + wd_].astype(f32)
            if wd_ < 128:
                blk = jnp.concatenate([blk, jnp.zeros((D, 128 - wd_), f32)], axis=1)
            tmp[t, pl.ds(0, D), :] = blk
        for t in range(5):
            rows = [tmp[t, pl.ds(d, 32, stride=DH), :] for d in range(DH)]
            full = jnp.concatenate(rows[:16] + [zpad] + rows[16:], axis=0)
            ft = full.T
            n = 128 if t < 4 else 64
            woT[pl.ds(t * 128, n), :] = ft[:n].astype(bf16)

    QT = (0, 1, 2, 3, 8)
    KT = (4, 5, 6, 7, 13)
    VT = (9, 10, 11, 12, 8)
    scale = DH ** -0.5
    c2 = scale * math.log2(math.e)
    neg = -1e9 / scale
    k0 = math.sqrt(2.0 / math.pi)
    k1 = k0 * 0.044715

    def to_rows(xt):
        xp = jnp.concatenate([xt, jnp.zeros((KP - D, xt.shape[1]), f32)], axis=0)
        return xp.astype(bf16).T

    class A:
        pass

    def a_qkv(st):
        st.blk = s % NB
        st.x = jnp.where(s < NB, x_ref[...].astype(f32), xres[st.blk])
        xn = to_rows(_ln_t(st.x))
        qkv = lax.dot_general(xn, wqkvT[...], NT, preferred_element_type=f32)
        for t in range(4, 14):
            qkv_s[t, pl.ds(0, HALO), :] = qkv_s[t, pl.ds(TB, HALO), :]
        for t in range(14):
            qkv_s[t, pl.ds(HALO, TB), :] = qkv[:, t * 128:(t + 1) * 128]
        st.o_rows = []

    def a_rows(st, rs):
        for r in rs:
            r0 = r * RB
            q = [qkv_s[t, pl.ds(HALO + r0, RB), :] for t in QT]
            sc = []
            for w in range(W):
                off = HALO + r0 - DIL * w
                acc = None
                for j, t in enumerate(KT):
                    p = q[j] * qkv_s[t, pl.ds(off, RB), :]
                    acc = p if acc is None else acc + p
                acc = acc + pltpu.roll(acc, 64, 1)
                acc = acc + pltpu.roll(acc, 32, 1)
                if r0 - DIL * w < 0:
                    pos = st.blk * TB + r0 + lax.broadcasted_iota(jnp.int32, (RB, 128), 0)
                    acc = jnp.where(pos >= DIL * w, acc, neg)
                sc.append(acc)
            m = sc[0]
            for w in range(1, W):
                m = jnp.maximum(m, sc[w])
            e = [jnp.exp2((sc[w] - m) * c2) for w in range(W)]
            l = e[0]
            for w in range(1, W):
                l = l + e[w]
            rinv = 1.0 / l
            cols = []
            for j, t in enumerate(VT):
                acc = None
                for w in range(W):
                    off = HALO + r0 - DIL * w
                    p = e[w] * qkv_s[t, pl.ds(off, RB), :]
                    acc = p if acc is None else acc + p
                cols.append(acc * rinv)
            st.o_rows.append(jnp.concatenate(cols, axis=1))

    def a_wo(st):
        o = jnp.concatenate(st.o_rows, axis=0).astype(bf16)
        st.x1 = st.x + lax.dot_general(woT[...], o, NT, preferred_element_type=f32)
        st.xn2 = to_rows(_ln_t(st.x1))

    def a_store(st):
        xres[st.blk] = st.x1
        xn_s[(s // NH) % 2, s % NH] = st.xn2

    def f_init(st):
        f = s - NH
        j = f // NH
        st.hf = f % NH
        st.b0 = (j * NH) % NB
        st.xn = xn_s[j % 2].reshape(TM, KP)[:, :D]
        st.xin = jnp.concatenate([xres[st.b0 + k] for k in range(NH)], axis=1)
        st.acc = None
        st.h = {}

    def f_gu(st, c):
        gu = jnp.dot(st.xn, wgu_v[st.hf, c], preferred_element_type=f32)
        g = gu[:, :TF]
        u = gu[:, TF:]
        t = jnp.tanh(g * (k0 + k1 * (g * g)))
        gu2 = g * u
        st.h[c] = (gu2 + gu2 * t).astype(bf16)

    def f_d(st, c):
        p = lax.dot_general(wd_v[st.hf, :, c * TF:(c + 1) * TF], st.h.pop(c), NT, preferred_element_type=f32)
        st.acc = p if st.acc is None else st.acc + p

    def f_store(st):
        x2 = st.xin + 0.5 * st.acc
        for k in range(NH):
            xres[st.b0 + k] = x2[:, k * TB:(k + 1) * TB]
        o_ref[...] = x2.astype(o_ref.dtype)

    def run(do_a, do_f):
        a, f = A(), A()
        nr = TB // RB
        if not do_f:
            a_qkv(a); a_rows(a, range(nr)); a_wo(a); a_store(a)
            return
        f_init(f)
        rows_per = [[] for _ in range(ncf)]
        lo, hi = QKV_AT + 1, WO_AT
        slots = list(range(QKV_AT, WO_AT))
        for r in range(nr):
            rows_per[slots[r * len(slots) // nr]].append(r)
        for c in range(ncf):
            f_gu(f, c)
            if c > 0:
                f_d(f, c - 1)
            if do_a:
                if c == QKV_AT:
                    a_qkv(a)
                if c == WO_AT:
                    a_wo(a)
                a_rows(a, rows_per[c])
        f_d(f, ncf - 1)
        f_store(f)
        if do_a:
            a_store(a)

    for hf in range(NH):
        @pl.when(s == NH + hf)
        def _():
            for cp in ffn_copies(hf):
                cp.wait()

    @pl.when(s < NH)
    def _():
        run(True, False)

    @pl.when(jnp.logical_and(s >= NH, s < 2 * NB))
    def _():
        run(True, True)

    @pl.when(s >= 2 * NB)
    def _():
        run(False, True)


@jax.jit
def pallas_interleave_layers__sliding_local_dilated__glu_gated_geglu__prompt_kernel(
    A_x, A_wqkv, A_wo, B_x, B_w_gate, B_w_up, B_w_down):
    B, S, D = A_x.shape
    DF = B_w_gate.shape[1]
    NB = S // TB
    xT = A_x.reshape(S, D).T
    wdT = B_w_down.T
    FH = DF // NH
    ncf = FH // TF
    nsteps = 2 * NB + NH
    NP = S // TM
    hbm = pl.BlockSpec(memory_space=pltpu.HBM)
    outT = pl.pallas_call(
        functools.partial(_kernel, D=D, DF=DF, NB=NB),
        grid=(nsteps,),
        in_specs=[
            pl.BlockSpec((D, TB), lambda s: (0, jnp.minimum(s, NB - 1))),
            hbm, hbm, hbm, hbm, hbm,
        ],
        out_specs=pl.BlockSpec((D, TM), lambda s: (0, jnp.maximum((s - NH) // NH - NP, 0))),
        out_shape=jax.ShapeDtypeStruct((D, S), A_x.dtype),
        scratch_shapes=[
            pltpu.VMEM((D, 3 * D), bf16),
            pltpu.VMEM((D, D), bf16),
            pltpu.VMEM((NQKV, KP), bf16),
            pltpu.VMEM((D, KP), bf16),
            pltpu.VMEM((NH, ncf, D, 2 * TF), bf16),
            pltpu.VMEM((NH, D, FH), bf16),
            pltpu.VMEM((5, NQKV, 128), f32),
            pltpu.VMEM((14, HALO + TB, 128), f32),
            pltpu.VMEM((NB, D, TB), f32),
            pltpu.VMEM((2, NH, TB, KP), bf16),
            pltpu.SemaphoreType.DMA((2 + NH,)),
        ],
        compiler_params=pltpu.CompilerParams(
            dimension_semantics=("arbitrary",),
            vmem_limit_bytes=100 * 1024 * 1024,
        ),
    )(xT, A_wqkv, A_wo, B_w_gate, B_w_up, wdT)
    return outT.T.reshape(B, S, D)
```

```python
import functools
import math
import jax
import jax.numpy as jnp
from jax import lax
import jax.experimental.pallas as pl
import jax.experimental.pallas.tpu as pltpu

H = 32
DH = 18
W = 8
DIL = 2
HALO = 16
EPS = 1e-5
TB = 128
TM = 256
NH = 2
RB = 8
KP = 640
KH = 256
NQKV = 14 * 128
TC = 128
NSLOT = 8
DG = int(3)
ROWS_LO = int(0)
WO_AT = int(6)
DLAG = int(1)
LN1_AT = int(7)
SERIAL = int(1)
SERIAL_A = int(0)
NACC = int(4)
KPAIR = int(6)
CP = int(3)
QSPLIT = int(5)
XFIRST = 512
NPACE = int(4)
MODE_F = tuple(int(x) for x in '0,1,0'.split(','))
MODE_A = tuple(int(x) for x in '1,3,1'.split(','))
FENCE = int(1)
PR = 32
PW1 = float(1); PW2 = float(1); PW3 = float(1)
SOPS_EARLY = int(1)
CLIP = int(0)

f32 = jnp.float32
bf16 = jnp.bfloat16
u32 = jnp.uint32
NT = (((1,), (1,)), ((), ()))


def _pk(x):
    return pltpu.bitcast(x.astype(bf16), u32)


def _unpk(u, idx):
    return pltpu.unpack_elementwise(u, index=idx, packed_dtype=bf16, unpacked_dtype=f32)


def _pk2(even, odd):
    return pltpu.pack_elementwise([even, odd], packed_dtype=bf16).astype(u32)


def _up(x):
    return pltpu.bitcast(x, bf16)


def _dot(a, b):
    return jnp.dot(a, b, preferred_element_type=f32)


def _dot_nt(a, b):
    return lax.dot_general(a, b, NT, preferred_element_type=f32)


def _ln_stats(x):
    n = x.shape[0]
    c = x[0:1]
    s1 = [None] * NACC
    s2 = [None] * NACC
    for i in range(n // 8):
        d = x[i * 8:(i + 1) * 8] - c
        k = i % NACC
        s1[k] = d if s1[k] is None else s1[k] + d
        dd = d * d
        s2[k] = dd if s2[k] is None else s2[k] + dd
    while len(s1) > 1:
        s1 = [s1[i] + s1[i + 1] for i in range(0, len(s1), 2)]
        s2 = [s2[i] + s2[i + 1] for i in range(0, len(s2), 2)]
    m = jnp.sum(s1[0], axis=0, keepdims=True) * (1.0 / n)
    v = jnp.sum(s2[0], axis=0, keepdims=True) * (1.0 / n) - m * m
    v = jnp.maximum(v, 0.0)
    return c + m, lax.rsqrt(v + EPS)


def _tree(fn, xs):
    xs = list(xs)
    while len(xs) > 1:
        xs = [fn(xs[i], xs[i + 1]) for i in range(0, len(xs) - 1, 2)] + ([xs[-1]] if len(xs) % 2 else [])
    return xs[0]


def _lhs_ops(a11, a12, a21, a22):
    return (a11 + a22, a21 + a22, a11, a22, a11 + a12, a21 - a11, a12 - a22)


def _rhs_ops(b11, b12, b21, b22):
    return (b11 + b22, b11, b12 - b22, b21 - b11, b22, b11 + b12, b21 + b22)


def _dst_row(sec, d):
    if sec == 0:
        return d * 32 if d < 16 else 1024 + (d - 16) * 32
    if sec == 1:
        return 512 + d * 32 if d < 16 else 13 * 128 + (d - 16) * 32
    return 9 * 128 + d * 32 if d < 16 else 1024 + 64 + (d - 16) * 32


def _prep_plan(nchunk):
    plan = [[nchunk] * CP]
    nxt = 0
    for j in range(1, KPAIR):
        left_steps = KPAIR - 1 - j
        n = min(CP, nchunk - nxt)
        if j == 1:
            n = max(0, min(n, max(CP - 1, nchunk - nxt - left_steps * CP)))
        ids = list(range(nxt, nxt + n))
        nxt += n
        plan.append(ids + [nchunk] * (CP - n))
    return plan, nxt


def _kernel(x_hbm, wqkv_hbm, wo_hbm, wg_hbm, wu_hbm, wd_hbm, o_ref,
            xin, wqkv_raw, wo_raw, wqkvT, woT, raw, pw, tmp, qa, qb, xres, xn_f, xn1a, xn1b,
            s_scr, ar_scr, plan_s, sems, *, D, DF, NB):
    g = pl.program_id(0)
    FH = DF // NH
    NPC = FH // (2 * TC)
    NCH = NH * NPC
    NG = NPC // DG
    DHALF = D // 2
    K = 2 * KPAIR
    S = NB * TB
    plan, nprepped = _prep_plan(NCH)

    def cp_qkv():
        return pltpu.make_async_copy(wqkv_hbm, wqkv_raw, sems.at[0])

    def cp_wo():
        return pltpu.make_async_copy(wo_hbm, wo_raw, sems.at[1])

    def cp_x(k):
        lo, n = (0, XFIRST) if k == 0 else (XFIRST, S - XFIRST)
        return pltpu.make_async_copy(x_hbm.at[:, pl.ds(lo, n)], xin.at[:, pl.ds(lo, n)], sems.at[2 + k])

    def chunk_copies(c):
        return [pltpu.make_async_copy(w.at[:, pl.ds(c * 2 * TC, 2 * TC)], raw.at[c, m], sems.at[4 + c])
                for m, w in enumerate((wg_hbm, wu_hbm, wd_hbm))]

    R_WR = 7 * (KH // 2)
    R_SD = R_WR + (D - 2 * KH)
    R_END = R_SD + 4 * (DHALF // 2)

    def prep_pieces(c):
        def ld(m, r0, nr, col):
            u = pltpu.bitcast(raw[c, m, pl.ds(r0, nr), pl.ds(col, TC)], u32)
            return u, _unpk(u, 0), _unpk(u, 1)

        def ops(fn, blocks):
            ev = fn(*[b[1] for b in blocks])
            od = fn(*[b[2] for b in blocks])
            out = []
            for e, o in zip(ev, od):
                src = [b[0] for b in blocks if b[1] is e]
                out.append(src[0] if src else _pk2(e, o))
            return out

        def gu_piece(m, r):
            blocks = [ld(m, r, PR, 0), ld(m, r, PR, TC), ld(m, KH + r, PR, 0), ld(m, KH + r, PR, TC)]
            for i, t in enumerate(ops(_rhs_ops, blocks)):
                pw[c, pl.ds(i * (KH // 2) + r // 2, PR // 2), m * TC:(m + 1) * TC] = t

        def wr_piece():
            nrem = D - 2 * KH
            for m in range(2):
                for k in range(2):
                    pw[c, pl.ds(R_WR + k * (nrem // 2), nrem // 2), m * TC:(m + 1) * TC] = ld(m, 2 * KH, nrem, k * TC)[0]

        def d_piece(r):
            blocks = [ld(2, r, PR, 0), ld(2, r, PR, TC), ld(2, DHALF + r, PR, 0), ld(2, DHALF + r, PR, TC)]
            for i, t in enumerate(ops(_lhs_ops, blocks)):
                pw[c, pl.ds(R_SD + (i // 2) * (DHALF // 2) + r // 2, PR // 2), (i % 2) * TC:(i % 2 + 1) * TC] = t

        out = [functools.partial(gu_piece, m, r) for m in range(2) for r in range(0, KH, PR)]
        out.append(wr_piece)
        out += [functools.partial(d_piece, r) for r in range(0, DHALF, PR)]
        return out

    def prep_chunk(c):
        for piece in prep_pieces(c):
            piece()

    def pace_pw(v):
        pw[NCH, pl.ds(R_END, 8), 0:128] = pltpu.bitcast(v, u32)

    nr = TB // RB
    QT = (0, 1, 2, 3, 8)
    KT = (4, 5, 6, 7, 13)
    VT = (9, 10, 11, 12, 8)
    scale = DH ** -0.5
    c2e = scale * math.log2(math.e)
    neg = -1e9 * math.log2(math.e)
    k0 = math.sqrt(2.0 / math.pi)
    k1 = k0 * 0.044715
    zero8 = pl.multiple_of((g >> 20) * 8, 8)

    def x_convert(blk):
        x = xin[:, pl.ds(pl.multiple_of(blk * TB, TB), TB)].astype(f32)
        xres[blk] = x
        return x

    def a_ln1(blk, dst, from_input):
        x = x_convert(blk) if from_input else xres[blk]
        mean, rstd = _ln_stats(x)
        if not from_input:
            dst[pl.ds(0, 8), :] = jnp.zeros((8, KP), u32)
        xn = (xres[blk] - mean) * rstd
        xp = jnp.concatenate([xn, jnp.zeros((KP - D, TB), f32)], axis=0)
        dst[...] = pltpu.bitcast(xp.astype(bf16).T, u32)

    def a_qkv(src, qdst, qprev, t0=0, t1=14, cb=None):
        qkv = _dot_nt(_up(src[...]), _up(wqkvT[pl.ds(t0 * 64, (t1 - t0) * 64), :]))
        for t in range(max(t0, 4), t1):
            qdst[t, pl.ds(0, HALO), :] = qprev[t, pl.ds(TB, HALO), :]
        for t in range(t0, t1):
            qdst[t, pl.ds(HALO, TB), :] = qkv[:, (t - t0) * 128:(t - t0 + 1) * 128]
            if cb is not None:
                for k in range(NPACE):
                    rr = k * (TB // NPACE)
                    cb(qkv[rr:rr + 8, (t - t0) * 128:(t - t0 + 1) * 128])

    zvec = jnp.full((RB, 128), (g >> 20).astype(u32), u32)
    cbits = pltpu.bitcast(jnp.full((RB, 128), c2e, f32), u32)

    def tied_scale(deps):
        if not deps:
            return c2e
        acc = pltpu.bitcast(deps[0], u32)
        for dv in deps[1:]:
            acc = acc | pltpu.bitcast(dv, u32)
        return pltpu.bitcast(cbits | (acc & zvec), f32)

    def a_rows(q_s, blk, rs, mode, hist):
        lag_mid, lag_end, midkind = mode
        for r in rs:
            r0 = r * RB
            deps = []
            if lag_mid and r - lag_mid >= 0:
                deps.append(hist[('h' if midkind else 'm', r - lag_mid)])
            if lag_end and r - lag_end >= 0:
                deps += hist[('o', r - lag_end)]
            cs = tied_scale(deps)
            q = [q_s[t, pl.ds(HALO + r0, RB), :] * cs for t in QT]
            sc = []
            for w in range(W):
                off = HALO + r0 - DIL * w
                acc = None
                for j, t in enumerate(KT):
                    p = q[j] * q_s[t, pl.ds(off, RB), :]
                    acc = p if acc is None else acc + p
                acc = acc + pltpu.roll(acc, 64, 1)
                hist[('h', r)] = acc
                acc = acc + pltpu.roll(acc, 32, 1)
                if r0 - DIL * w < 0:
                    pos = blk * TB + r0 + lax.broadcasted_iota(jnp.int32, (RB, 128), 0)
                    acc = jnp.where(pos >= DIL * w, acc, neg)
                sc.append(acc)
            m = _tree(jnp.maximum, sc)
            hist[('m', r)] = m
            e = [jnp.exp2(sc[w] - m) for w in range(W)]
            l = _tree(jnp.add, e)
            rinv = pl.reciprocal(l, approx=True)
            rinv = rinv * (2.0 - l * rinv)
            outs = []
            for j, t in enumerate(VT):
                acc = None
                for w in range(W):
                    off = HALO + r0 - DIL * w
                    p = e[w] * q_s[t, pl.ds(off, RB), :]
                    acc = p if acc is None else acc + p
                o = acc * rinv
                st_off = r0 + zero8 if (j == 4 and r == nr - 1 and FENCE) else r0
                q_s[14 + j, pl.ds(st_off, RB), :] = o
                outs.append(o)
            hist[('o', r)] = outs

    def a_wo(q_s, blk, par):
        o = jnp.concatenate([q_s[14 + j, pl.ds(0, TB), :] for j in range(5)], axis=1).astype(bf16)
        x1 = xres[blk] + _dot_nt(_up(woT[...]), o)
        xres[blk] = x1
        mean, rstd = _ln_stats(x1)
        xn_f[par] = (xres[blk] - mean) * rstd

    def a_sops(slot):
        def blkf(which):
            tb, kh = which
            return xn_f[tb, pl.ds(kh * KH, KH), :]
        combos = (((0, 0), 1, (1, 1)), ((1, 0), 1, (1, 1)), ((0, 0), 0, None), ((1, 1), 0, None),
                  ((0, 0), 1, (0, 1)), ((1, 0), -1, (0, 0)), ((0, 1), -1, (1, 1)))
        for i, (u, sg, v) in enumerate(combos):
            t = blkf(u)
            if sg == 1:
                t = t + blkf(v)
            elif sg == -1:
                t = t - blkf(v)
            s_scr[slot, i] = pltpu.bitcast(t.astype(bf16).T, u32)
        rem = jnp.concatenate([xn_f[tb, pl.ds(2 * KH, D - 2 * KH), :] for tb in range(2)], axis=0)
        ar_scr[slot] = pltpu.bitcast(rem.astype(bf16).T, u32)

    class St:
        pass

    def f_init(st, f):
        j = f // NH
        st.c0 = (f % NH) * NPC
        st.b0 = (j * NH) % NB
        st.sb = j % NSLOT
        st.acc = [None] * 7
        st.t = {}

    def gelu_mul(c):
        gg = c[:, :TC]
        u = c[:, TC:]
        t = jnp.tanh(gg * (k0 + k1 * (gg * gg)))
        gu = gg * u
        return gu + gu * t

    def f_gu(st, p):
        c = st.c0 + p

        def M(i):
            return _dot(_up(s_scr[st.sb, i - 1]), _up(pw[c, pl.ds((i - 1) * (KH // 2), KH // 2), :]))
        rem = _up(ar_scr[st.sb])
        rt, rb = rem[:, :D - 2 * KH], rem[:, D - 2 * KH:]
        nrh = (D - 2 * KH) // 2
        w1 = _up(pw[c, pl.ds(R_WR, nrh), :])
        w2 = _up(pw[c, pl.ds(R_WR + nrh, nrh), :])
        m5 = M(5)
        m3 = M(3)
        h12 = gelu_mul(m3 + m5 + _dot(rt, w2))
        m4 = M(4)
        m2 = M(2)
        h21 = gelu_mul(m2 + m4 + _dot(rb, w1))
        m1 = M(1)
        h11 = gelu_mul(m1 + m4 - m5 + M(7) + _dot(rt, w1))
        h22 = gelu_mul(m1 - m2 + m3 + M(6) + _dot(rb, w2))
        st.t[p] = _rhs_ops(h11, h21, h12, h22)

    def f_d(st, gi):
        ps = range(gi * DG, (gi + 1) * DG)
        for i in range(7):
            a = jnp.concatenate([_up(pw[st.c0 + p, pl.ds(R_SD + (i // 2) * (DHALF // 2), DHALF // 2),
                                         (i % 2) * TC:(i % 2 + 1) * TC]) for p in ps], axis=1)
            t = jnp.concatenate([st.t[p][i] for p in ps], axis=1).astype(bf16)
            r = _dot_nt(a, t)
            st.acc[i] = r if st.acc[i] is None else st.acc[i] + r
        for p in ps:
            del st.t[p]

    def f_store(st):
        m1, m2, m3, m4, m5, m6, m7 = st.acc
        top = jnp.concatenate([m1 + m4 - m5 + m7, m2 + m4], axis=0)
        bot = jnp.concatenate([m3 + m5, m1 - m2 + m3 + m6], axis=0)
        for k, y in enumerate((top, bot)):
            x2 = xres[st.b0 + k] + 0.5 * y
            xres[st.b0 + k] = x2
            o_ref[:, k * TB:(k + 1) * TB] = x2.astype(o_ref.dtype)

    def run_f(f, a):
        st = St()
        hist = {}
        f_init(st, f)
        if a is not None:
            blk = a % NB
        rows_per = [[] for _ in range(NPC)]
        slots = list(range(ROWS_LO, WO_AT))
        for r in range(nr):
            rows_per[slots[r * len(slots) // nr]].append(r)
        done = 0
        for p in range(NPC):
            f_gu(st, p)
            while (done + 1) * DG + DLAG <= p + 1:
                f_d(st, done)
                done += 1
            if a is not None:
                if p == WO_AT:
                    a_wo(qa, blk, a % 2)
                if p == LN1_AT:
                    a_ln1((a + 1) % NB, xn1a, False)
                a_rows(qa, blk, rows_per[p], MODE_F, hist)
        if a is not None and SOPS_EARLY:
            a_sops((a // 2) % NSLOT)
        while done < NG:
            f_d(st, done)
            done += 1
        f_store(st)
        if a is not None:
            a_qkv(xn1a, qa, qa)
            if not SOPS_EARLY:
                a_sops((a // 2) % NSLOT)

    def run_aa(j):
        a = 2 * j
        b = a + 1
        pieces = []
        for k in range(CP):
            pieces += prep_pieces(plan_s[j * CP + k])
        wts = [PW1] * (14 * NPACE) + [PW3] * (13 * NPACE) + [0.0] * NPACE
        tot = sum(wts)
        state = dict(pt=0, done=0, cum=0.0)

        def cb(v):
            if not pieces:
                return
            state['cum'] += wts[state['pt']]
            state['pt'] += 1
            upto = int(round(len(pieces) * state['cum'] / tot))
            if upto > state['done'] or state['pt'] == 27 * NPACE + 1:
                pace_pw(v)
            for piece in pieces[state['done']:upto]:
                piece()
            state['done'] = upto

        a_rows(qa, a, range(nr), MODE_A, {})
        a_wo(qb, jnp.where(j == 0, NB, a - 1), 1)
        a_sops(jnp.where(j == 0, NSLOT, j - 1))
        a_ln1(a + 2, xn1a, True)
        a_qkv(xn1b, qb, qa, cb=cb)
        a_rows(qb, b, range(nr), MODE_A, {})
        a_wo(qa, a, 0)
        a_ln1(b + 2, xn1b, True)
        a_qkv(xn1a, qa, qb, cb=cb)
        assert state['done'] == len(pieces)

    @pl.when(g == 0)
    def _():
        cp_x(0).start()
        cp_qkv().start()
        for j in range(KPAIR):
            for k in range(CP):
                plan_s[j * CP + k] = plan[j][k]
        qb[:, pl.ds(TB, HALO), :] = jnp.zeros((19, HALO, 128), f32)
        zpad = jnp.zeros((KP - D, 128), f32)
        cp_x(0).wait()
        a_ln1(0, xn1a, True)
        a_ln1(1, xn1b, True)
        cp_qkv().wait()
        cp_wo().start()
        cp_x(1).start()
        for c in range(NCH):
            for cp in chunk_copies(c):
                cp.start()
        for j in range(14):
            wd_ = 128 if j < 13 else 64
            blk = wqkv_raw[:, j * 128:j * 128 + wd_].astype(f32)
            if wd_ < 128:
                blk = jnp.concatenate([blk, jnp.zeros((D, 128 - wd_), f32)], axis=1)
            bt = jnp.concatenate([blk, zpad], axis=0).T
            for t in range(5):
                tmp[t, pl.ds(j * 128, 128), :] = bt[:, t * 128:(t + 1) * 128]
        for sec in range(3):
            for d in range(DH):
                r = _dst_row(sec, d)
                for t in range(5):
                    wqkvT[pl.ds(r // 2, 16), t * 128:(t + 1) * 128] = _pk2(
                        tmp[t, pl.ds(sec * D + d, 16, stride=2 * DH), :],
                        tmp[t, pl.ds(sec * D + d + DH, 16, stride=2 * DH), :])
        wqkvT[pl.ds((13 * 128 + 64) // 2, 32), :] = jnp.zeros((32, KP), u32)
        cp_wo().wait()
        a_qkv(xn1a, qa, qb)
        for t in range(5):
            wd_ = 128 if t < 4 else 64
            blk = wo_raw[:, t * 128:t * 128 + wd_].astype(f32)
            if wd_ < 128:
                blk = jnp.concatenate([blk, jnp.zeros((D, 128 - wd_), f32)], axis=1)
            tmp[t, pl.ds(0, D), :] = blk
        for t in range(5):
            rows = [tmp[t, pl.ds(d, 32, stride=DH), :] for d in range(DH)]
            full = jnp.concatenate(rows[:16] + [zpad] + rows[16:], axis=0)
            ft = full.T
            n = 128 if t < 4 else 64
            woT[pl.ds(t * 64, n // 2), :] = _pk(ft[:n])

    for j in range(1, KPAIR):
        @pl.when(g == 1 + j)
        def _():
            if j == 1:
                cp_x(1).wait()
            for c in plan[j]:
                if c < NCH:
                    for cp in chunk_copies(c):
                        cp.wait()

    @pl.when(jnp.logical_and(g >= 1, g <= KPAIR))
    def _():
        run_aa(g - 1)

    @pl.when(g == KPAIR + 1)
    def _():
        a_wo(qb, K - 1, 1)
        a_sops(KPAIR - 1)
        for blk in range(K + 2, NB):
            x_convert(blk)

        def body(c, carry):
            for cp in chunk_copies(c):
                cp.wait()
            prep_chunk(c)
            return carry
        if nprepped < NCH:
            lax.fori_loop(nprepped, NCH, body, 0)

    f = g - (KPAIR + 1)

    @pl.when(jnp.logical_and(f >= 0, f < 2 * NB - K))
    def _():
        run_f(f, f + K)

    @pl.when(f >= 2 * NB - K)
    def _():
        run_f(f, None)


@jax.jit
def pallas_interleave_layers__sliding_local_dilated__glu_gated_geglu__prompt_kernel(
    A_x, A_wqkv, A_wo, B_x, B_w_gate, B_w_up, B_w_down):
    B, S, D = A_x.shape
    DF = B_w_gate.shape[1]
    NB = S // TB
    xT = A_x.reshape(S, D).T
    wdT = B_w_down.T
    NCH = DF // (2 * TC)
    nsteps = 1 + KPAIR + 2 * NB
    hbm = pl.BlockSpec(memory_space=pltpu.HBM)
    outT = pl.pallas_call(
        functools.partial(_kernel, D=D, DF=DF, NB=NB),
        grid=(nsteps,),
        in_specs=[hbm] * 6,
        out_specs=pl.BlockSpec((D, TM), lambda g: (0, jnp.maximum(g - (1 + KPAIR + NB), 0) // NH)),
        out_shape=jax.ShapeDtypeStruct((D, S), A_x.dtype),
        scratch_shapes=[
            pltpu.VMEM((D, S), bf16),
            pltpu.VMEM((D, 3 * D), bf16),
            pltpu.VMEM((D, D), bf16),
            pltpu.VMEM((NQKV // 2, KP), u32),
            pltpu.VMEM((D // 2, KP), u32),
            pltpu.VMEM((NCH + 1, 3, D, 2 * TC), bf16),
            pltpu.VMEM((NCH + 1, 7 * (KH // 2) + (D - 2 * KH) + D + 8, 2 * TC), u32),
            pltpu.VMEM((5, NQKV, 128), f32),
            pltpu.VMEM((19, HALO + TB, 128), f32),
            pltpu.VMEM((19, HALO + TB, 128), f32),
            pltpu.VMEM((NB + 1, D, TB), f32),
            pltpu.VMEM((2, D, TB), f32),
            pltpu.VMEM((TB // 2, KP), u32),
            pltpu.VMEM((TB // 2, KP), u32),
            pltpu.VMEM((NSLOT + 1, 7, TB // 2, KH), u32),
            pltpu.VMEM((NSLOT + 1, TB // 2, 128), u32),
            pltpu.SMEM((KPAIR * CP + 1,), jnp.int32),
            pltpu.SemaphoreType.DMA((4 + NCH,)),
        ],
        compiler_params=pltpu.CompilerParams(
            dimension_semantics=("arbitrary",),
            vmem_limit_bytes=110 * 1024 * 1024,
        ),
    )(xT, A_wqkv, A_wo, B_w_gate, B_w_up, wdT)
    return outT.T.reshape(B, S, D)
```

```python
import functools
import math
import jax
import jax.numpy as jnp
from jax import lax
import jax.experimental.pallas as pl
import jax.experimental.pallas.tpu as pltpu

H = 32
DH = 18
W = 8
DIL = 2
HALO = 16
EPS = 1e-5
TB = 128
TM = 256
NH = 2
RB = 8
KP = 640
KH = 256
KX = 192
KY = 64
V1_POS = ((7, 0), (0, 0), (1, 0), (2, 0), (3, 0), (5, 0), (4, 0))
V2_POS = ((7, KX), (0, KX), (2, KX), (1, KX), (3, KX), (6, 2 * KY), (6, 0))
NQKV = 14 * 128
TC = 128
NSLOT = 8
DG = int(3)
ROWS_LO = int(0)
WO_AT = int(6)
DLAG = int(1)
LN1_AT = int(7)
SERIAL = int(1)
SERIAL_A = int(0)
NACC = int(4)
KPAIR = int(6)
CP = int(3)
QSPLIT = int(5)
XFIRST = 512
NPACE = int(4)
MODE_F = tuple(int(x) for x in '0,1,0'.split(','))
MODE_A = tuple(int(x) for x in '1,3,1'.split(','))
FENCE = int(1)
PR = 32
PW1 = float(1); PW2 = float(1); PW3 = float(1)
SOPS_EARLY = int(1)
CLIP = int(0)

f32 = jnp.float32
bf16 = jnp.bfloat16
u32 = jnp.uint32
NT = (((1,), (1,)), ((), ()))


def _pk(x):
    return pltpu.bitcast(x.astype(bf16), u32)


def _unpk(u, idx):
    return pltpu.unpack_elementwise(u, index=idx, packed_dtype=bf16, unpacked_dtype=f32)


def _pk2(even, odd):
    return pltpu.pack_elementwise([even, odd], packed_dtype=bf16).astype(u32)


def _up(x):
    return pltpu.bitcast(x, bf16)


def _dot(a, b):
    return jnp.dot(a, b, preferred_element_type=f32)


def _dot_nt(a, b):
    return lax.dot_general(a, b, NT, preferred_element_type=f32)


def _ln_stats(x):
    n = x.shape[0]
    c = x[0:1]
    s1 = [None] * NACC
    s2 = [None] * NACC
    for i in range(n // 8):
        d = x[i * 8:(i + 1) * 8] - c
        k = i % NACC
        s1[k] = d if s1[k] is None else s1[k] + d
        dd = d * d
        s2[k] = dd if s2[k] is None else s2[k] + dd
    while len(s1) > 1:
        s1 = [s1[i] + s1[i + 1] for i in range(0, len(s1), 2)]
        s2 = [s2[i] + s2[i + 1] for i in range(0, len(s2), 2)]
    m = jnp.sum(s1[0], axis=0, keepdims=True) * (1.0 / n)
    v = jnp.sum(s2[0], axis=0, keepdims=True) * (1.0 / n) - m * m
    v = jnp.maximum(v, 0.0)
    return c + m, lax.rsqrt(v + EPS)


def _tree(fn, xs):
    xs = list(xs)
    while len(xs) > 1:
        xs = [fn(xs[i], xs[i + 1]) for i in range(0, len(xs) - 1, 2)] + ([xs[-1]] if len(xs) % 2 else [])
    return xs[0]


def _lhs_ops(a11, a12, a21, a22):
    return (a11 + a22, a21 + a22, a11, a22, a11 + a12, a21 - a11, a12 - a22)


def _rhs_ops(b11, b12, b21, b22):
    return (b11 + b22, b11, b12 - b22, b21 - b11, b22, b11 + b12, b21 + b22)


def _dst_row(sec, d):
    if sec == 0:
        return d * 32 if d < 16 else 1024 + (d - 16) * 32
    if sec == 1:
        return 512 + d * 32 if d < 16 else 13 * 128 + (d - 16) * 32
    return 9 * 128 + d * 32 if d < 16 else 1024 + 64 + (d - 16) * 32


def _prep_plan(nchunk):
    plan = [[nchunk] * CP]
    nxt = 0
    for j in range(1, KPAIR):
        left_steps = KPAIR - 1 - j
        n = min(CP, nchunk - nxt)
        if j == 1:
            n = max(0, min(n, max(CP - 1, nchunk - nxt - left_steps * CP)))
        ids = list(range(nxt, nxt + n))
        nxt += n
        plan.append(ids + [nchunk] * (CP - n))
    return plan, nxt


def _kernel(x_hbm, wqkv_hbm, wo_hbm, wg_hbm, wu_hbm, wd_hbm, o_ref,
            xin, wqkv_raw, wo_raw, wqkvT, woT, raw, pw, tmp, qa, qb, xres, xn_f, xn1a, xn1b,
            s_scr, plan_s, sems, *, D, DF, NB):
    g = pl.program_id(0)
    FH = DF // NH
    NPC = FH // (2 * TC)
    NCH = NH * NPC
    NG = NPC // DG
    DHALF = D // 2
    K = 2 * KPAIR
    S = NB * TB
    plan, nprepped = _prep_plan(NCH)

    def cp_qkv():
        return pltpu.make_async_copy(wqkv_hbm, wqkv_raw, sems.at[0])

    def cp_wo():
        return pltpu.make_async_copy(wo_hbm, wo_raw, sems.at[1])

    def cp_x(k):
        lo, n = (0, XFIRST) if k == 0 else (XFIRST, S - XFIRST)
        return pltpu.make_async_copy(x_hbm.at[:, pl.ds(lo, n)], xin.at[:, pl.ds(lo, n)], sems.at[2 + k])

    def chunk_copies(c):
        return [pltpu.make_async_copy(w.at[:, pl.ds(c * 2 * TC, 2 * TC)], raw.at[c, m], sems.at[4 + c])
                for m, w in enumerate((wg_hbm, wu_hbm, wd_hbm))]

    R_SD = 8 * (KH // 2)
    R_END = R_SD + 4 * (DHALF // 2)

    def prep_pieces(c):
        def ld(m, r0, nr, col):
            u = pltpu.bitcast(raw[c, m, pl.ds(r0, nr), pl.ds(col, TC)], u32)
            return u, _unpk(u, 0), _unpk(u, 1)

        def ops(fn, blocks):
            ev = fn(*[b[1] for b in blocks])
            od = fn(*[b[2] for b in blocks])
            out = []
            for e, o in zip(ev, od):
                src = [b[0] for b in blocks if b[1] is e]
                out.append(src[0] if src else _pk2(e, o))
            return out

        def put(m, slot, row, t):
            pw[c, pl.ds((slot * KH + row) // 2, t.shape[0]), m * TC:(m + 1) * TC] = t

        def gu1_piece(m, r):
            blocks = [ld(m, r, PR, 0), ld(m, r, PR, TC), ld(m, KX + r, PR, 0), ld(m, KX + r, PR, TC)]
            for (slot, row), t in zip(V1_POS, ops(_rhs_ops, blocks)):
                put(m, slot, row + r, t)

        def gu2_piece(m, r):
            kc, kd = 2 * KX + r, 2 * KX + KY + r
            blocks = [ld(m, kc, PR, TC), ld(m, kc, PR, 0), ld(m, kd, PR, TC), ld(m, kd, PR, 0)]
            for (slot, row), t in zip(V2_POS, ops(_rhs_ops, blocks)):
                put(m, slot, row + r, t)

        def wr_piece(m):
            r1 = ld(m, 2 * KH, KY, 0)[0]
            r2 = ld(m, 2 * KH, KY, TC)[0]
            put(m, 4, KX, r1)
            put(m, 6, 3 * KY, r1)
            put(m, 5, KX, r2)
            put(m, 6, KY, r2)

        def d_piece(r):
            blocks = [ld(2, r, PR, 0), ld(2, r, PR, TC), ld(2, DHALF + r, PR, 0), ld(2, DHALF + r, PR, TC)]
            for i, t in enumerate(ops(_lhs_ops, blocks)):
                pw[c, pl.ds(R_SD + (i // 2) * (DHALF // 2) + r // 2, PR // 2), (i % 2) * TC:(i % 2 + 1) * TC] = t

        out = []
        for m in range(2):
            out += [functools.partial(gu1_piece, m, r) for r in range(0, KX, PR)]
            out += [functools.partial(gu2_piece, m, r) for r in range(0, KY, PR)]
            out.append(functools.partial(wr_piece, m))
        out += [functools.partial(d_piece, r) for r in range(0, DHALF, PR)]
        return out

    def prep_chunk(c):
        for piece in prep_pieces(c):
            piece()

    def pace_pw(v):
        pw[NCH, pl.ds(R_END, 8), 0:128] = pltpu.bitcast(v, u32)

    nr = TB // RB
    QT = (0, 1, 2, 3, 8)
    KT = (4, 5, 6, 7, 13)
    VT = (9, 10, 11, 12, 8)
    scale = DH ** -0.5
    c2e = scale * math.log2(math.e)
    neg = -1e9 * math.log2(math.e)
    k0 = math.sqrt(2.0 / math.pi)
    k1 = k0 * 0.044715
    zero8 = pl.multiple_of((g >> 20) * 8, 8)

    def x_convert(blk):
        x = xin[:, pl.ds(pl.multiple_of(blk * TB, TB), TB)].astype(f32)
        xres[blk] = x
        return x

    def a_ln1(blk, dst, from_input):
        x = x_convert(blk) if from_input else xres[blk]
        mean, rstd = _ln_stats(x)
        if not from_input:
            dst[pl.ds(0, 8), :] = jnp.zeros((8, KP), u32)
        xn = (xres[blk] - mean) * rstd
        xp = jnp.concatenate([xn, jnp.zeros((KP - D, TB), f32)], axis=0)
        dst[...] = pltpu.bitcast(xp.astype(bf16).T, u32)

    def a_qkv(src, qdst, qprev, t0=0, t1=14, cb=None):
        qkv = _dot_nt(_up(src[...]), _up(wqkvT[pl.ds(t0 * 64, (t1 - t0) * 64), :]))
        for t in range(max(t0, 4), t1):
            qdst[t, pl.ds(0, HALO), :] = qprev[t, pl.ds(TB, HALO), :]
        for t in range(t0, t1):
            qdst[t, pl.ds(HALO, TB), :] = qkv[:, (t - t0) * 128:(t - t0 + 1) * 128]
            if cb is not None:
                for k in range(NPACE):
                    rr = k * (TB // NPACE)
                    cb(qkv[rr:rr + 8, (t - t0) * 128:(t - t0 + 1) * 128])

    zvec = jnp.full((RB, 128), (g >> 20).astype(u32), u32)
    cbits = pltpu.bitcast(jnp.full((RB, 128), c2e, f32), u32)

    def tied_scale(deps):
        if not deps:
            return c2e
        acc = pltpu.bitcast(deps[0], u32)
        for dv in deps[1:]:
            acc = acc | pltpu.bitcast(dv, u32)
        return pltpu.bitcast(cbits | (acc & zvec), f32)

    def a_rows(q_s, blk, rs, mode, hist):
        lag_mid, lag_end, midkind = mode
        for r in rs:
            r0 = r * RB
            deps = []
            if lag_mid and r - lag_mid >= 0:
                deps.append(hist[('h' if midkind else 'm', r - lag_mid)])
            if lag_end and r - lag_end >= 0:
                deps += hist[('o', r - lag_end)]
            cs = tied_scale(deps)
            q = [q_s[t, pl.ds(HALO + r0, RB), :] * cs for t in QT]
            sc = []
            for w in range(W):
                off = HALO + r0 - DIL * w
                acc = None
                for j, t in enumerate(KT):
                    p = q[j] * q_s[t, pl.ds(off, RB), :]
                    acc = p if acc is None else acc + p
                acc = acc + pltpu.roll(acc, 64, 1)
                hist[('h', r)] = acc
                acc = acc + pltpu.roll(acc, 32, 1)
                if r0 - DIL * w < 0:
                    pos = blk * TB + r0 + lax.broadcasted_iota(jnp.int32, (RB, 128), 0)
                    acc = jnp.where(pos >= DIL * w, acc, neg)
                sc.append(acc)
            m = _tree(jnp.maximum, sc)
            hist[('m', r)] = m
            e = [jnp.exp2(sc[w] - m) for w in range(W)]
            l = _tree(jnp.add, e)
            rinv = pl.reciprocal(l, approx=True)
            rinv = rinv * (2.0 - l * rinv)
            outs = []
            for j, t in enumerate(VT):
                acc = None
                for w in range(W):
                    off = HALO + r0 - DIL * w
                    p = e[w] * q_s[t, pl.ds(off, RB), :]
                    acc = p if acc is None else acc + p
                o = acc * rinv
                st_off = r0 + zero8 if (j == 4 and r == nr - 1 and FENCE) else r0
                q_s[14 + j, pl.ds(st_off, RB), :] = o
                outs.append(o)
            hist[('o', r)] = outs

    def a_wo(q_s, blk, par):
        o = jnp.concatenate([q_s[14 + j, pl.ds(0, TB), :] for j in range(5)], axis=1).astype(bf16)
        x1 = xres[blk] + _dot_nt(_up(woT[...]), o)
        xres[blk] = x1
        mean, rstd = _ln_stats(x1)
        xn_f[par] = (xres[blk] - mean) * rstd

    def a_sops(slot):
        def seg(tb, r0, n):
            return lambda: xn_f[tb, pl.ds(r0, n), :]
        A11, A12, A21, A22 = seg(0, 0, KX), seg(0, KX, KX), seg(1, 0, KX), seg(1, KX, KX)
        kc, kd = 2 * KX, 2 * KX + KY
        a11, a12, a21, a22 = seg(0, kc, KY), seg(0, kd, KY), seg(1, kc, KY), seg(1, kd, KY)
        rt, rb = seg(0, 2 * KH, KY), seg(1, 2 * KH, KY)
        parts = (
            lambda: (A21() + A22(), -(a21() + a22())),
            lambda: (A11(), a22()),
            lambda: (A22(), a11()),
            lambda: (A11() + A12(), -(a11() + a12())),
            lambda: (A12() - A22(), rt()),
            lambda: (A21() - A11(), rb()),
            lambda: (a12() - a22(), rt(), a21() - a11(), rb()),
            lambda: (A11() + A22(), a11() + a22()),
        )
        for i, fn in enumerate(parts):
            t = jnp.concatenate(fn(), axis=0)
            s_scr[slot, i] = pltpu.bitcast(t.astype(bf16).T, u32)

    class St:
        pass

    def f_init(st, f):
        j = f // NH
        st.c0 = (f % NH) * NPC
        st.b0 = (j * NH) % NB
        st.sb = j % NSLOT
        st.acc = [None] * 7
        st.t = {}

    def gelu_mul(c):
        gg = c[:, :TC]
        u = c[:, TC:]
        t = jnp.tanh(gg * (k0 + k1 * (gg * gg)))
        gu = gg * u
        return gu + gu * t

    def f_gu(st, p):
        c = st.c0 + p

        def Q(slot, k0_=0, k1_=KH):
            if k0_ % 128 == 0 and k1_ % 128 == 0:
                lhs = _up(s_scr[st.sb, slot, :, k0_:k1_])
            else:
                lhs = _up(s_scr[st.sb, slot])[:, k0_:k1_]
            return _dot(lhs, _up(pw[c, pl.ds((slot * KH + k0_) // 2, (k1_ - k0_) // 2), :]))
        q5 = Q(3)
        q3 = Q(1)
        q1b = Q(7, KX, KH)
        h12 = gelu_mul(q3 + q5 + q1b + Q(6, 0, 2 * KY))
        q4 = Q(2)
        q2 = Q(0)
        h21 = gelu_mul(q2 + q4 + q1b + Q(6, 2 * KY, KH))
        q1 = Q(7, 0, KX)
        h11 = gelu_mul(q1 + q4 - q5 + Q(4))
        h22 = gelu_mul(q1 - q2 + q3 + Q(5))
        st.t[p] = _rhs_ops(h11, h21, h12, h22)

    def f_d(st, gi):
        ps = range(gi * DG, (gi + 1) * DG)
        for i in range(7):
            a = jnp.concatenate([_up(pw[st.c0 + p, pl.ds(R_SD + (i // 2) * (DHALF // 2), DHALF // 2),
                                         (i % 2) * TC:(i % 2 + 1) * TC]) for p in ps], axis=1)
            t = jnp.concatenate([st.t[p][i] for p in ps], axis=1).astype(bf16)
            r = _dot_nt(a, t)
            st.acc[i] = r if st.acc[i] is None else st.acc[i] + r
        for p in ps:
            del st.t[p]

    def f_store(st):
        m1, m2, m3, m4, m5, m6, m7 = st.acc
        top = jnp.concatenate([m1 + m4 - m5 + m7, m2 + m4], axis=0)
        bot = jnp.concatenate([m3 + m5, m1 - m2 + m3 + m6], axis=0)
        for k, y in enumerate((top, bot)):
            x2 = xres[st.b0 + k] + 0.5 * y
            xres[st.b0 + k] = x2
            o_ref[:, k * TB:(k + 1) * TB] = x2.astype(o_ref.dtype)

    def run_f(f, a):
        st = St()
        hist = {}
        f_init(st, f)
        if a is not None:
            blk = a % NB
        rows_per = [[] for _ in range(NPC)]
        slots = list(range(ROWS_LO, WO_AT))
        for r in range(nr):
            rows_per[slots[r * len(slots) // nr]].append(r)
        done = 0
        for p in range(NPC):
            f_gu(st, p)
            while (done + 1) * DG + DLAG <= p + 1:
                f_d(st, done)
                done += 1
            if a is not None:
                if p == WO_AT:
                    a_wo(qa, blk, a % 2)
                if p == LN1_AT:
                    a_ln1((a + 1) % NB, xn1a, False)
                a_rows(qa, blk, rows_per[p], MODE_F, hist)
        if a is not None and SOPS_EARLY:
            a_sops((a // 2) % NSLOT)
        while done < NG:
            f_d(st, done)
            done += 1
        f_store(st)
        if a is not None:
            a_qkv(xn1a, qa, qa)
            if not SOPS_EARLY:
                a_sops((a // 2) % NSLOT)

    def run_aa(j):
        a = 2 * j
        b = a + 1
        pieces = []
        for k in range(CP):
            pieces += prep_pieces(plan_s[j * CP + k])
        wts = [PW1] * (14 * NPACE) + [PW3] * (13 * NPACE) + [0.0] * NPACE
        tot = sum(wts)
        state = dict(pt=0, done=0, cum=0.0)

        def cb(v):
            if not pieces:
                return
            state['cum'] += wts[state['pt']]
            state['pt'] += 1
            upto = int(round(len(pieces) * state['cum'] / tot))
            if upto > state['done'] or state['pt'] == 27 * NPACE + 1:
                pace_pw(v)
            for piece in pieces[state['done']:upto]:
                piece()
            state['done'] = upto

        a_rows(qa, a, range(nr), MODE_A, {})
        a_wo(qb, jnp.where(j == 0, NB, a - 1), 1)
        a_sops(jnp.where(j == 0, NSLOT, j - 1))
        a_ln1(a + 2, xn1a, True)
        a_qkv(xn1b, qb, qa, cb=cb)
        a_rows(qb, b, range(nr), MODE_A, {})
        a_wo(qa, a, 0)
        a_ln1(b + 2, xn1b, True)
        a_qkv(xn1a, qa, qb, cb=cb)
        assert state['done'] == len(pieces)

    @pl.when(g == 0)
    def _():
        cp_x(0).start()
        cp_qkv().start()
        for j in range(KPAIR):
            for k in range(CP):
                plan_s[j * CP + k] = plan[j][k]
        qb[:, pl.ds(TB, HALO), :] = jnp.zeros((19, HALO, 128), f32)
        zpad = jnp.zeros((KP - D, 128), f32)
        cp_x(0).wait()
        a_ln1(0, xn1a, True)
        a_ln1(1, xn1b, True)
        cp_qkv().wait()
        cp_wo().start()
        cp_x(1).start()
        for c in range(NCH):
            for cp in chunk_copies(c):
                cp.start()
        for j in range(14):
            wd_ = 128 if j < 13 else 64
            blk = wqkv_raw[:, j * 128:j * 128 + wd_].astype(f32)
            if wd_ < 128:
                blk = jnp.concatenate([blk, jnp.zeros((D, 128 - wd_), f32)], axis=1)
            bt = jnp.concatenate([blk, zpad], axis=0).T
            for t in range(5):
                tmp[t, pl.ds(j * 128, 128), :] = bt[:, t * 128:(t + 1) * 128]
        for sec in range(3):
            for d in range(DH):
                r = _dst_row(sec, d)
                for t in range(5):
                    wqkvT[pl.ds(r // 2, 16), t * 128:(t + 1) * 128] = _pk2(
                        tmp[t, pl.ds(sec * D + d, 16, stride=2 * DH), :],
                        tmp[t, pl.ds(sec * D + d + DH, 16, stride=2 * DH), :])
        wqkvT[pl.ds((13 * 128 + 64) // 2, 32), :] = jnp.zeros((32, KP), u32)
        cp_wo().wait()
        a_qkv(xn1a, qa, qb)
        for t in range(5):
            wd_ = 128 if t < 4 else 64
            blk = wo_raw[:, t * 128:t * 128 + wd_].astype(f32)
            if wd_ < 128:
                blk = jnp.concatenate([blk, jnp.zeros((D, 128 - wd_), f32)], axis=1)
            tmp[t, pl.ds(0, D), :] = blk
        for t in range(5):
            rows = [tmp[t, pl.ds(d, 32, stride=DH), :] for d in range(DH)]
            full = jnp.concatenate(rows[:16] + [zpad] + rows[16:], axis=0)
            ft = full.T
            n = 128 if t < 4 else 64
            woT[pl.ds(t * 64, n // 2), :] = _pk(ft[:n])

    for j in range(1, KPAIR):
        @pl.when(g == 1 + j)
        def _():
            if j == 1:
                cp_x(1).wait()
            for c in plan[j]:
                if c < NCH:
                    for cp in chunk_copies(c):
                        cp.wait()

    @pl.when(jnp.logical_and(g >= 1, g <= KPAIR))
    def _():
        run_aa(g - 1)

    @pl.when(g == KPAIR + 1)
    def _():
        a_wo(qb, K - 1, 1)
        a_sops(KPAIR - 1)
        for blk in range(K + 2, NB):
            x_convert(blk)

        def body(c, carry):
            for cp in chunk_copies(c):
                cp.wait()
            prep_chunk(c)
            return carry
        if nprepped < NCH:
            lax.fori_loop(nprepped, NCH, body, 0)

    f = g - (KPAIR + 1)

    @pl.when(jnp.logical_and(f >= 0, f < 2 * NB - K))
    def _():
        run_f(f, f + K)

    @pl.when(f >= 2 * NB - K)
    def _():
        run_f(f, None)


@jax.jit
def pallas_interleave_layers__sliding_local_dilated__glu_gated_geglu__prompt_kernel(
    A_x, A_wqkv, A_wo, B_x, B_w_gate, B_w_up, B_w_down):
    B, S, D = A_x.shape
    DF = B_w_gate.shape[1]
    NB = S // TB
    xT = A_x.reshape(S, D).T
    wdT = B_w_down.T
    NCH = DF // (2 * TC)
    nsteps = 1 + KPAIR + 2 * NB
    hbm = pl.BlockSpec(memory_space=pltpu.HBM)
    outT = pl.pallas_call(
        functools.partial(_kernel, D=D, DF=DF, NB=NB),
        grid=(nsteps,),
        in_specs=[hbm] * 6,
        out_specs=pl.BlockSpec((D, TM), lambda g: (0, jnp.maximum(g - (1 + KPAIR + NB), 0) // NH)),
        out_shape=jax.ShapeDtypeStruct((D, S), A_x.dtype),
        scratch_shapes=[
            pltpu.VMEM((D, S), bf16),
            pltpu.VMEM((D, 3 * D), bf16),
            pltpu.VMEM((D, D), bf16),
            pltpu.VMEM((NQKV // 2, KP), u32),
            pltpu.VMEM((D // 2, KP), u32),
            pltpu.VMEM((NCH + 1, 3, D, 2 * TC), bf16),
            pltpu.VMEM((NCH + 1, 8 * (KH // 2) + D + 8, 2 * TC), u32),
            pltpu.VMEM((5, NQKV, 128), f32),
            pltpu.VMEM((19, HALO + TB, 128), f32),
            pltpu.VMEM((19, HALO + TB, 128), f32),
            pltpu.VMEM((NB + 1, D, TB), f32),
            pltpu.VMEM((2, D, TB), f32),
            pltpu.VMEM((TB // 2, KP), u32),
            pltpu.VMEM((TB // 2, KP), u32),
            pltpu.VMEM((NSLOT + 1, 8, TB // 2, KH), u32),
            pltpu.SMEM((KPAIR * CP + 1,), jnp.int32),
            pltpu.SemaphoreType.DMA((4 + NCH,)),
        ],
        compiler_params=pltpu.CompilerParams(
            dimension_semantics=("arbitrary",),
            vmem_limit_bytes=110 * 1024 * 1024,
        ),
    )(xT, A_wqkv, A_wo, B_w_gate, B_w_up, wdT)
    return outT.T.reshape(B, S, D)
```

```python
import functools
import math
import jax
import jax.numpy as jnp
from jax import lax
import jax.experimental.pallas as pl
import jax.experimental.pallas.tpu as pltpu

H = 32
DH = 18
W = 8
DIL = 2
HALO = 16
EPS = 1e-5
TB = 128
TM = 256
NH = 2
RB = 8
KP = 640
KH = 256
KX = 192
KY = 64
V1_POS = ((7, 0), (0, 0), (1, 0), (2, 0), (3, 0), (5, 0), (4, 0))
V2_POS = ((7, KX), (0, KX), (2, KX), (1, KX), (3, KX), (6, 2 * KY), (6, 0))
NQKV = 14 * 128
TC = 128
NSLOT = 8
DG = int(3)
ROWS_LO = int(0)
WO_AT = int(6)
DLAG = int(1)
LN1_AT = int(7)
SERIAL = int(1)
SERIAL_A = int(0)
NACC = int(4)
KPAIR = int(6)
CP = int(3)
QSPLIT = int(5)
XFIRST = 512
DGROUPS = tuple(int(x) for x in '2,4,4,4,4'.split(','))
DGROUPS_F = tuple(int(x) for x in '3,3,3'.split(','))
DORD = tuple(int(x) for x in '0,1,2,3,4,5,6'.split(','))
QB_AT = int(3); WOA_AT = int(6); RB_AT = int(6)
LNA_AT = int(8); LNB_AT = int(10); WOB_AT = int(13)
NPACE = int(4)
MODE_F = tuple(int(x) for x in '0,1,0'.split(','))
MODE_A = tuple(int(x) for x in '1,3,1'.split(','))
FENCE = int(1)
PR = 32
PW1 = float(1); PW2 = float(1); PW3 = float(1)
SOPS_EARLY = int(1)
CLIP = int(0)

f32 = jnp.float32
bf16 = jnp.bfloat16
u32 = jnp.uint32
NT = (((1,), (1,)), ((), ()))


def _pk(x):
    return pltpu.bitcast(x.astype(bf16), u32)


def _unpk(u, idx):
    return pltpu.unpack_elementwise(u, index=idx, packed_dtype=bf16, unpacked_dtype=f32)


def _pk2(even, odd):
    return pltpu.pack_elementwise([even, odd], packed_dtype=bf16).astype(u32)


def _up(x):
    return pltpu.bitcast(x, bf16)


def _dot(a, b):
    return jnp.dot(a, b, preferred_element_type=f32)


def _dot_nt(a, b):
    return lax.dot_general(a, b, NT, preferred_element_type=f32)


def _ln_stats(x):
    n = x.shape[0]
    c = x[0:1]
    s1 = [None] * NACC
    s2 = [None] * NACC
    for i in range(n // 8):
        d = x[i * 8:(i + 1) * 8] - c
        k = i % NACC
        s1[k] = d if s1[k] is None else s1[k] + d
        dd = d * d
        s2[k] = dd if s2[k] is None else s2[k] + dd
    while len(s1) > 1:
        s1 = [s1[i] + s1[i + 1] for i in range(0, len(s1), 2)]
        s2 = [s2[i] + s2[i + 1] for i in range(0, len(s2), 2)]
    m = jnp.sum(s1[0], axis=0, keepdims=True) * (1.0 / n)
    v = jnp.sum(s2[0], axis=0, keepdims=True) * (1.0 / n) - m * m
    v = jnp.maximum(v, 0.0)
    return c + m, lax.rsqrt(v + EPS)


def _tree(fn, xs):
    xs = list(xs)
    while len(xs) > 1:
        xs = [fn(xs[i], xs[i + 1]) for i in range(0, len(xs) - 1, 2)] + ([xs[-1]] if len(xs) % 2 else [])
    return xs[0]


def _lhs_ops(a11, a12, a21, a22):
    return (a11 + a22, a21 + a22, a11, a22, a11 + a12, a21 - a11, a12 - a22)


def _rhs_ops(b11, b12, b21, b22):
    return (b11 + b22, b11, b12 - b22, b21 - b11, b22, b11 + b12, b21 + b22)


def _dst_row(sec, d):
    if sec == 0:
        return d * 32 if d < 16 else 1024 + (d - 16) * 32
    if sec == 1:
        return 512 + d * 32 if d < 16 else 13 * 128 + (d - 16) * 32
    return 9 * 128 + d * 32 if d < 16 else 1024 + 64 + (d - 16) * 32


def _prep_plan(nchunk):
    plan = [[nchunk] * CP]
    nxt = 0
    for j in range(1, KPAIR):
        left_steps = KPAIR - 1 - j
        n = min(CP, nchunk - nxt)
        if j == 1:
            n = max(0, min(n, max(CP - 1, nchunk - nxt - left_steps * CP)))
        ids = list(range(nxt, nxt + n))
        nxt += n
        plan.append(ids + [nchunk] * (CP - n))
    return plan, nxt


def _kernel(x_hbm, wqkv_hbm, wo_hbm, wg_hbm, wu_hbm, wd_hbm, o_ref,
            xin, wqkv_raw, wo_raw, wqkvT, woT, raw, pw, tmp, qa, qb, xres, xn_f, xn1a, xn1b,
            s_scr, plan_s, sems, *, D, DF, NB):
    g = pl.program_id(0)
    FH = DF // NH
    NPC = FH // (2 * TC)
    NCH = NH * NPC
    NG = NPC // DG
    DHALF = D // 2
    K = 2 * KPAIR
    S = NB * TB
    plan, nprepped = _prep_plan(NCH)

    def cp_qkv():
        return pltpu.make_async_copy(wqkv_hbm, wqkv_raw, sems.at[0])

    def cp_wo():
        return pltpu.make_async_copy(wo_hbm, wo_raw, sems.at[1])

    def cp_x(k):
        lo, n = (0, XFIRST) if k == 0 else (XFIRST, S - XFIRST)
        return pltpu.make_async_copy(x_hbm.at[:, pl.ds(lo, n)], xin.at[:, pl.ds(lo, n)], sems.at[2 + k])

    def chunk_copies(c):
        return [pltpu.make_async_copy(w.at[:, pl.ds(c * 2 * TC, 2 * TC)], raw.at[c, m], sems.at[4 + c])
                for m, w in enumerate((wg_hbm, wu_hbm, wd_hbm))]

    R_SD = 8 * (KH // 2)
    R_END = R_SD + 4 * (DHALF // 2)

    def prep_pieces(c):
        def ld(m, r0, nr, col):
            u = pltpu.bitcast(raw[c, m, pl.ds(r0, nr), pl.ds(col, TC)], u32)
            return u, _unpk(u, 0), _unpk(u, 1)

        def ops(fn, blocks):
            ev = fn(*[b[1] for b in blocks])
            od = fn(*[b[2] for b in blocks])
            out = []
            for e, o in zip(ev, od):
                src = [b[0] for b in blocks if b[1] is e]
                out.append(src[0] if src else _pk2(e, o))
            return out

        def put(m, slot, row, t):
            pw[c, pl.ds((slot * KH + row) // 2, t.shape[0]), m * TC:(m + 1) * TC] = t

        def gu1_piece(m, r):
            blocks = [ld(m, r, PR, 0), ld(m, r, PR, TC), ld(m, KX + r, PR, 0), ld(m, KX + r, PR, TC)]
            for (slot, row), t in zip(V1_POS, ops(_rhs_ops, blocks)):
                put(m, slot, row + r, t)

        def gu2_piece(m, r):
            kc, kd = 2 * KX + r, 2 * KX + KY + r
            blocks = [ld(m, kc, PR, TC), ld(m, kc, PR, 0), ld(m, kd, PR, TC), ld(m, kd, PR, 0)]
            for (slot, row), t in zip(V2_POS, ops(_rhs_ops, blocks)):
                put(m, slot, row + r, t)

        def wr_piece(m):
            r1 = ld(m, 2 * KH, KY, 0)[0]
            r2 = ld(m, 2 * KH, KY, TC)[0]
            put(m, 4, KX, r1)
            put(m, 6, 3 * KY, r1)
            put(m, 5, KX, r2)
            put(m, 6, KY, r2)

        def d_piece(r):
            blocks = [ld(2, r, PR, 0), ld(2, r, PR, TC), ld(2, DHALF + r, PR, 0), ld(2, DHALF + r, PR, TC)]
            for i, t in enumerate(ops(_lhs_ops, blocks)):
                pw[c, pl.ds(R_SD + (i // 2) * (DHALF // 2) + r // 2, PR // 2), (i % 2) * TC:(i % 2 + 1) * TC] = t

        out = []
        for m in range(2):
            out += [functools.partial(gu1_piece, m, r) for r in range(0, KX, PR)]
            out += [functools.partial(gu2_piece, m, r) for r in range(0, KY, PR)]
            out.append(functools.partial(wr_piece, m))
        out += [functools.partial(d_piece, r) for r in range(0, DHALF, PR)]
        return out

    def prep_chunk(c):
        for piece in prep_pieces(c):
            piece()

    def pace_pw(v):
        pw[NCH, pl.ds(R_END, 8), 0:128] = pltpu.bitcast(v, u32)

    nr = TB // RB
    QT = (0, 1, 2, 3, 8)
    KT = (4, 5, 6, 7, 13)
    VT = (9, 10, 11, 12, 8)
    scale = DH ** -0.5
    c2e = scale * math.log2(math.e)
    neg = -1e9 * math.log2(math.e)
    k0 = math.sqrt(2.0 / math.pi)
    k1 = k0 * 0.044715
    zero8 = pl.multiple_of((g >> 20) * 8, 8)

    def x_convert(blk):
        x = xin[:, pl.ds(pl.multiple_of(blk * TB, TB), TB)].astype(f32)
        xres[blk] = x
        return x

    def a_ln1(blk, dst, from_input):
        x = x_convert(blk) if from_input else xres[blk]
        mean, rstd = _ln_stats(x)
        if not from_input:
            dst[pl.ds(0, 8), :] = jnp.zeros((8, KP), u32)
        xn = (xres[blk] - mean) * rstd
        xp = jnp.concatenate([xn, jnp.zeros((KP - D, TB), f32)], axis=0)
        dst[...] = pltpu.bitcast(xp.astype(bf16).T, u32)

    def a_qkv(src, qdst, qprev, t0=0, t1=14, cb=None):
        qkv = _dot_nt(_up(src[...]), _up(wqkvT[pl.ds(t0 * 64, (t1 - t0) * 64), :]))
        for t in range(max(t0, 4), t1):
            qdst[t, pl.ds(0, HALO), :] = qprev[t, pl.ds(TB, HALO), :]
        for t in range(t0, t1):
            qdst[t, pl.ds(HALO, TB), :] = qkv[:, (t - t0) * 128:(t - t0 + 1) * 128]
            if cb is not None:
                for k in range(NPACE):
                    rr = k * (TB // NPACE)
                    cb(qkv[rr:rr + 8, (t - t0) * 128:(t - t0 + 1) * 128])

    zvec = jnp.full((RB, 128), (g >> 20).astype(u32), u32)
    cbits = pltpu.bitcast(jnp.full((RB, 128), c2e, f32), u32)

    def tied_scale(deps):
        if not deps:
            return c2e
        acc = pltpu.bitcast(deps[0], u32)
        for dv in deps[1:]:
            acc = acc | pltpu.bitcast(dv, u32)
        return pltpu.bitcast(cbits | (acc & zvec), f32)

    def a_rows(q_s, blk, rs, mode, hist):
        lag_mid, lag_end, midkind = mode
        for r in rs:
            r0 = r * RB
            deps = []
            if lag_mid and r - lag_mid >= 0:
                deps.append(hist[('h' if midkind else 'm', r - lag_mid)])
            if lag_end and r - lag_end >= 0:
                deps += hist[('o', r - lag_end)]
            cs = tied_scale(deps)
            q = [q_s[t, pl.ds(HALO + r0, RB), :] * cs for t in QT]
            sc = []
            for w in range(W):
                off = HALO + r0 - DIL * w
                acc = None
                for j, t in enumerate(KT):
                    p = q[j] * q_s[t, pl.ds(off, RB), :]
                    acc = p if acc is None else acc + p
                acc = acc + pltpu.roll(acc, 64, 1)
                hist[('h', r)] = acc
                acc = acc + pltpu.roll(acc, 32, 1)
                if r0 - DIL * w < 0:
                    pos = blk * TB + r0 + lax.broadcasted_iota(jnp.int32, (RB, 128), 0)
                    acc = jnp.where(pos >= DIL * w, acc, neg)
                sc.append(acc)
            m = _tree(jnp.maximum, sc)
            hist[('m', r)] = m
            e = [jnp.exp2(sc[w] - m) for w in range(W)]
            l = _tree(jnp.add, e)
            rinv = pl.reciprocal(l, approx=True)
            rinv = rinv * (2.0 - l * rinv)
            outs = []
            for j, t in enumerate(VT):
                acc = None
                for w in range(W):
                    off = HALO + r0 - DIL * w
                    p = e[w] * q_s[t, pl.ds(off, RB), :]
                    acc = p if acc is None else acc + p
                o = acc * rinv
                st_off = r0 + zero8 if (j == 4 and r == nr - 1 and FENCE) else r0
                q_s[14 + j, pl.ds(st_off, RB), :] = o
                outs.append(o)
            hist[('o', r)] = outs

    def a_wo(q_s, blk, par):
        o = jnp.concatenate([q_s[14 + j, pl.ds(0, TB), :] for j in range(5)], axis=1).astype(bf16)
        x1 = xres[blk] + _dot_nt(_up(woT[...]), o)
        xres[blk] = x1
        mean, rstd = _ln_stats(x1)
        xn_f[par] = (xres[blk] - mean) * rstd

    def a_sops(slot):
        def seg(tb, r0, n):
            return lambda: xn_f[tb, pl.ds(r0, n), :]
        A11, A12, A21, A22 = seg(0, 0, KX), seg(0, KX, KX), seg(1, 0, KX), seg(1, KX, KX)
        kc, kd = 2 * KX, 2 * KX + KY
        a11, a12, a21, a22 = seg(0, kc, KY), seg(0, kd, KY), seg(1, kc, KY), seg(1, kd, KY)
        rt, rb = seg(0, 2 * KH, KY), seg(1, 2 * KH, KY)
        parts = (
            lambda: (A21() + A22(), -(a21() + a22())),
            lambda: (A11(), a22()),
            lambda: (A22(), a11()),
            lambda: (A11() + A12(), -(a11() + a12())),
            lambda: (A12() - A22(), rt()),
            lambda: (A21() - A11(), rb()),
            lambda: (a12() - a22(), rt(), a21() - a11(), rb()),
            lambda: (A11() + A22(), a11() + a22()),
        )
        for i, fn in enumerate(parts):
            t = jnp.concatenate(fn(), axis=0)
            s_scr[slot, i] = pltpu.bitcast(t.astype(bf16).T, u32)

    class St:
        pass

    def f_init(st, j):
        st.c0 = 0
        st.b0 = (j * NH) % NB
        st.sb = j % NSLOT
        st.acc = [None] * 7
        st.t = {}

    def gelu_mul(c):
        gg = c[:, :TC]
        u = c[:, TC:]
        t = jnp.tanh(gg * (k0 + k1 * (gg * gg)))
        gu = gg * u
        return gu + gu * t

    def f_gu(st, p):
        c = st.c0 + p

        def Q(slot, k0_=0, k1_=KH):
            if k0_ % 128 == 0 and k1_ % 128 == 0:
                lhs = _up(s_scr[st.sb, slot, :, k0_:k1_])
            else:
                lhs = _up(s_scr[st.sb, slot])[:, k0_:k1_]
            return _dot(lhs, _up(pw[c, pl.ds((slot * KH + k0_) // 2, (k1_ - k0_) // 2), :]))
        q5 = Q(3)
        q3 = Q(1)
        q1b = Q(7, KX, KH)
        h12 = gelu_mul(q3 + q5 + q1b + Q(6, 0, 2 * KY))
        q4 = Q(2)
        q2 = Q(0)
        h21 = gelu_mul(q2 + q4 + q1b + Q(6, 2 * KY, KH))
        q1 = Q(7, 0, KX)
        h11 = gelu_mul(q1 + q4 - q5 + Q(4))
        h22 = gelu_mul(q1 - q2 + q3 + Q(5))
        st.t[p] = _rhs_ops(h11, h21, h12, h22)

    def f_d(st, ps):
        for i in DORD:
            a = jnp.concatenate([_up(pw[st.c0 + p, pl.ds(R_SD + (i // 2) * (DHALF // 2), DHALF // 2),
                                         (i % 2) * TC:(i % 2 + 1) * TC]) for p in ps], axis=1)
            t = jnp.concatenate([st.t[p][i] for p in ps], axis=1).astype(bf16)
            r = _dot_nt(a, t)
            st.acc[i] = r if st.acc[i] is None else st.acc[i] + r
        for p in ps:
            del st.t[p]

    def f_store(st):
        m1, m2, m3, m4, m5, m6, m7 = st.acc
        top = jnp.concatenate([m1 + m4 - m5 + m7, m2 + m4], axis=0)
        bot = jnp.concatenate([m3 + m5, m1 - m2 + m3 + m6], axis=0)
        for k, y in enumerate((top, bot)):
            x2 = xres[st.b0 + k] + 0.5 * y
            xres[st.b0 + k] = x2
            o_ref[:, k * TB:(k + 1) * TB] = x2.astype(o_ref.dtype)

    def run_pair(jf, ja):
        st = St()
        f_init(st, jf)
        groups = []
        p0 = 0
        for n in DGROUPS:
            groups.append(list(range(p0, p0 + n)))
            p0 += n
        assert p0 == NCH
        if ja is not None:
            a = (2 * ja) % NB
            b = a + 1
            a_rows(qa, a, range(nr), MODE_F, {})
        for p in range(NCH):
            f_gu(st, p)
            while groups and groups[0][-1] + DLAG <= p:
                f_d(st, groups.pop(0))
            if ja is not None:
                if p == QB_AT:
                    a_qkv(xn1b, qb, qa)
                if p == WOA_AT:
                    a_wo(qa, a, 0)
                if p == RB_AT:
                    a_rows(qb, b, range(nr), MODE_F, {})
                if p == LNA_AT:
                    a_ln1((a + 2) % NB, xn1a, False)
                if p == LNB_AT:
                    a_ln1((b + 2) % NB, xn1b, False)
                if p == WOB_AT:
                    a_wo(qb, b, 1)
        if ja is not None:
            a_sops(ja % NSLOT)
        while groups:
            f_d(st, groups.pop(0))
        f_store(st)
        if ja is not None:
            a_qkv(xn1a, qa, qb)

    def run_aa(j):
        a = 2 * j
        b = a + 1
        pieces = []
        for k in range(CP):
            pieces += prep_pieces(plan_s[j * CP + k])
        wts = [PW1] * (14 * NPACE) + [PW3] * (13 * NPACE) + [0.0] * NPACE
        tot = sum(wts)
        state = dict(pt=0, done=0, cum=0.0)

        def cb(v):
            if not pieces:
                return
            state['cum'] += wts[state['pt']]
            state['pt'] += 1
            upto = int(round(len(pieces) * state['cum'] / tot))
            if upto > state['done'] or state['pt'] == 27 * NPACE + 1:
                pace_pw(v)
            for piece in pieces[state['done']:upto]:
                piece()
            state['done'] = upto

        a_rows(qa, a, range(nr), MODE_A, {})
        a_wo(qb, jnp.where(j == 0, NB, a - 1), 1)
        a_sops(jnp.where(j == 0, NSLOT, j - 1))
        a_ln1(a + 2, xn1a, True)
        a_qkv(xn1b, qb, qa, cb=cb)
        a_rows(qb, b, range(nr), MODE_A, {})
        a_wo(qa, a, 0)
        a_ln1(b + 2, xn1b, True)
        a_qkv(xn1a, qa, qb, cb=cb)
        assert state['done'] == len(pieces)

    @pl.when(g == 0)
    def _():
        cp_x(0).start()
        cp_qkv().start()
        for j in range(KPAIR):
            for k in range(CP):
                plan_s[j * CP + k] = plan[j][k]
        qb[:, pl.ds(TB, HALO), :] = jnp.zeros((20, HALO, 128), f32)
        zpad = jnp.zeros((KP - D, 128), f32)
        cp_x(0).wait()
        a_ln1(0, xn1a, True)
        a_ln1(1, xn1b, True)
        cp_qkv().wait()
        cp_wo().start()
        cp_x(1).start()
        for c in range(NCH):
            for cp in chunk_copies(c):
                cp.start()
        for j in range(14):
            wd_ = 128 if j < 13 else 64
            blk = wqkv_raw[:, j * 128:j * 128 + wd_].astype(f32)
            if wd_ < 128:
                blk = jnp.concatenate([blk, jnp.zeros((D, 128 - wd_), f32)], axis=1)
            bt = jnp.concatenate([blk, zpad], axis=0).T
            for t in range(5):
                tmp[t, pl.ds(j * 128, 128), :] = bt[:, t * 128:(t + 1) * 128]
        for sec in range(3):
            for d in range(DH):
                r = _dst_row(sec, d)
                for t in range(5):
                    wqkvT[pl.ds(r // 2, 16), t * 128:(t + 1) * 128] = _pk2(
                        tmp[t, pl.ds(sec * D + d, 16, stride=2 * DH), :],
                        tmp[t, pl.ds(sec * D + d + DH, 16, stride=2 * DH), :])
        wqkvT[pl.ds((13 * 128 + 64) // 2, 32), :] = jnp.zeros((32, KP), u32)
        cp_wo().wait()
        a_qkv(xn1a, qa, qb)
        for t in range(5):
            wd_ = 128 if t < 4 else 64
            blk = wo_raw[:, t * 128:t * 128 + wd_].astype(f32)
            if wd_ < 128:
                blk = jnp.concatenate([blk, jnp.zeros((D, 128 - wd_), f32)], axis=1)
            tmp[t, pl.ds(0, D), :] = blk
        for t in range(5):
            rows = [tmp[t, pl.ds(d, 32, stride=DH), :] for d in range(DH)]
            full = jnp.concatenate(rows[:16] + [zpad] + rows[16:], axis=0)
            ft = full.T
            n = 128 if t < 4 else 64
            woT[pl.ds(t * 64, n // 2), :] = _pk(ft[:n])

    for j in range(1, KPAIR):
        @pl.when(g == 1 + j)
        def _():
            if j == 1:
                cp_x(1).wait()
            for c in plan[j]:
                if c < NCH:
                    for cp in chunk_copies(c):
                        cp.wait()

    @pl.when(jnp.logical_and(g >= 1, g <= KPAIR))
    def _():
        run_aa(g - 1)

    @pl.when(g == KPAIR + 1)
    def _():
        a_wo(qb, K - 1, 1)
        a_sops(KPAIR - 1)
        for blk in range(K + 2, NB):
            x_convert(blk)

        def body(c, carry):
            for cp in chunk_copies(c):
                cp.wait()
            prep_chunk(c)
            return carry
        if nprepped < NCH:
            lax.fori_loop(nprepped, NCH, body, 0)

    jf = g - (KPAIR + 1)

    @pl.when(jnp.logical_and(jf >= 0, jf < NB - KPAIR))
    def _():
        run_pair(jf, jf + KPAIR)

    @pl.when(jf >= NB - KPAIR)
    def _():
        def body(hf, carry):
            st = St()
            f_init(st, jf)
            st.c0 = hf * NPC
            groups = []
            p0 = 0
            for n in DGROUPS_F:
                groups.append(list(range(p0, p0 + n)))
                p0 += n
            for p in range(NPC):
                f_gu(st, p)
                while groups and groups[0][-1] + DLAG <= p:
                    f_d(st, groups.pop(0))
            while groups:
                f_d(st, groups.pop(0))
            f_store(st)
            return carry
        lax.fori_loop(0, NH, body, 0)


@jax.jit
def pallas_interleave_layers__sliding_local_dilated__glu_gated_geglu__prompt_kernel(
    A_x, A_wqkv, A_wo, B_x, B_w_gate, B_w_up, B_w_down):
    B, S, D = A_x.shape
    DF = B_w_gate.shape[1]
    NB = S // TB
    xT = A_x.reshape(S, D).T
    wdT = B_w_down.T
    NCH = DF // (2 * TC)
    nsteps = 1 + KPAIR + NB
    hbm = pl.BlockSpec(memory_space=pltpu.HBM)
    outT = pl.pallas_call(
        functools.partial(_kernel, D=D, DF=DF, NB=NB),
        grid=(nsteps,),
        in_specs=[hbm] * 6,
        out_specs=pl.BlockSpec((D, TM), lambda g: (0, jnp.maximum(g - (1 + KPAIR + NB // 2), 0))),
        out_shape=jax.ShapeDtypeStruct((D, S), A_x.dtype),
        scratch_shapes=[
            pltpu.VMEM((D, S), bf16),
            pltpu.VMEM((D, 3 * D), bf16),
            pltpu.VMEM((D, D), bf16),
            pltpu.VMEM((NQKV // 2, KP), u32),
            pltpu.VMEM((D // 2, KP), u32),
            pltpu.VMEM((NCH + 1, 3, D, 2 * TC), bf16),
            pltpu.VMEM((NCH + 1, 8 * (KH // 2) + D + 16, 2 * TC), u32),
            pltpu.VMEM((5, NQKV, 128), f32),
            pltpu.VMEM((20, HALO + TB, 128), f32),
            pltpu.VMEM((20, HALO + TB, 128), f32),
            pltpu.VMEM((NB + 1, D, TB), f32),
            pltpu.VMEM((2, D, TB), f32),
            pltpu.VMEM((TB // 2, KP), u32),
            pltpu.VMEM((TB // 2, KP), u32),
            pltpu.VMEM((NSLOT + 1, 8, TB // 2, KH), u32),
            pltpu.SMEM((KPAIR * CP + 1,), jnp.int32),
            pltpu.SemaphoreType.DMA((4 + NCH,)),
        ],
        compiler_params=pltpu.CompilerParams(
            dimension_semantics=("arbitrary",),
            vmem_limit_bytes=110 * 1024 * 1024,
        ),
    )(xT, A_wqkv, A_wo, B_w_gate, B_w_up, wdT)
    return outT.T.reshape(B, S, D)
```

```python
import functools
import math
import jax
import jax.numpy as jnp
from jax import lax
import jax.experimental.pallas as pl
import jax.experimental.pallas.tpu as pltpu

H = 32
DH = 18
W = 8
DIL = 2
HALO = 16
EPS = 1e-5
TB = 128
TM = 256
NH = 2
RB = 8
KP = 640
KH = 256
KX = 192
KY = 64
V1_POS = ((7, 0), (0, 0), (1, 0), (2, 0), (3, 0), (5, 0), (4, 0))
V2_POS = ((7, KX), (0, KX), (2, KX), (1, KX), (3, KX), (6, 2 * KY), (6, 0))
NQKV = 14 * 128
TC = 128
NSLOT = 8
DG = int(3)
ROWS_LO = int(0)
WO_AT = int(6)
DLAG = int(2)
LN1_AT = int(7)
SERIAL = int(1)
SERIAL_A = int(0)
NACC = int(4)
KPAIR = int(6)
CP = int(3)
QSPLIT = int(5)
XFIRST = 512
DGROUPS = tuple(int(x) for x in '4,4,4,4,2'.split(','))
DGROUPS_F = tuple(int(x) for x in '3,4,2'.split(','))
DORD = tuple(int(x) for x in '0,1,2,3,4,5,6'.split(','))
QB_AT = int(3); WOA_AT = int(6); RB_AT = int(6)
LNA_AT = int(8); LNB_AT = int(10); WOB_AT = int(13)
NPACE = int(4)
MODE_F = tuple(int(x) for x in '0,1,0,2,1'.split(','))
MODE_A = tuple(int(x) for x in '1,3,1,0,0'.split(','))
FENCE = int(1)
PR = 32
PW1 = float(1); PW2 = float(1); PW3 = float(1)
SOPS_EARLY = int(1)
CLIP = int(0)

f32 = jnp.float32
bf16 = jnp.bfloat16
u32 = jnp.uint32
NT = (((1,), (1,)), ((), ()))


def _pk(x):
    return pltpu.bitcast(x.astype(bf16), u32)


def _unpk(u, idx):
    return pltpu.unpack_elementwise(u, index=idx, packed_dtype=bf16, unpacked_dtype=f32)


def _pk2(even, odd):
    return pltpu.pack_elementwise([even, odd], packed_dtype=bf16).astype(u32)


def _up(x):
    return pltpu.bitcast(x, bf16)


def _dot(a, b):
    return jnp.dot(a, b, preferred_element_type=f32)


def _dot_nt(a, b):
    return lax.dot_general(a, b, NT, preferred_element_type=f32)


def _ln_stats(x):
    n = x.shape[0]
    c = x[0:1]
    s1 = [None] * NACC
    s2 = [None] * NACC
    for i in range(n // 8):
        d = x[i * 8:(i + 1) * 8] - c
        k = i % NACC
        s1[k] = d if s1[k] is None else s1[k] + d
        dd = d * d
        s2[k] = dd if s2[k] is None else s2[k] + dd
    while len(s1) > 1:
        s1 = [s1[i] + s1[i + 1] for i in range(0, len(s1), 2)]
        s2 = [s2[i] + s2[i + 1] for i in range(0, len(s2), 2)]
    m = jnp.sum(s1[0], axis=0, keepdims=True) * (1.0 / n)
    v = jnp.sum(s2[0], axis=0, keepdims=True) * (1.0 / n) - m * m
    v = jnp.maximum(v, 0.0)
    return c + m, lax.rsqrt(v + EPS)


def _tree(fn, xs):
    xs = list(xs)
    while len(xs) > 1:
        xs = [fn(xs[i], xs[i + 1]) for i in range(0, len(xs) - 1, 2)] + ([xs[-1]] if len(xs) % 2 else [])
    return xs[0]


def _lhs_ops(a11, a12, a21, a22):
    return (a11 + a22, a21 + a22, a11, a22, a11 + a12, a21 - a11, a12 - a22)


def _rhs_ops(b11, b12, b21, b22):
    return (b11 + b22, b11, b12 - b22, b21 - b11, b22, b11 + b12, b21 + b22)


def _dst_row(sec, d):
    if sec == 0:
        return d * 32 if d < 16 else 1024 + (d - 16) * 32
    if sec == 1:
        return 512 + d * 32 if d < 16 else 13 * 128 + (d - 16) * 32
    return 9 * 128 + d * 32 if d < 16 else 1024 + 64 + (d - 16) * 32


def _prep_plan(nchunk):
    plan = [[nchunk] * CP]
    nxt = 0
    for j in range(1, KPAIR):
        left_steps = KPAIR - 1 - j
        n = min(CP, nchunk - nxt)
        if j == 1:
            n = max(0, min(n, max(CP - 1, nchunk - nxt - left_steps * CP)))
        ids = list(range(nxt, nxt + n))
        nxt += n
        plan.append(ids + [nchunk] * (CP - n))
    return plan, nxt


def _kernel(x_hbm, wqkv_hbm, wo_hbm, wg_hbm, wu_hbm, wd_hbm, o_ref,
            xin, wqkv_raw, wo_raw, wqkvT, woT, raw, pw, tmp, qa, qb, xres, xn_f, xn1a, xn1b,
            s_scr, plan_s, sems, *, D, DF, NB):
    g = pl.program_id(0)
    FH = DF // NH
    NPC = FH // (2 * TC)
    NCH = NH * NPC
    NG = NPC // DG
    DHALF = D // 2
    K = 2 * KPAIR
    S = NB * TB
    plan, nprepped = _prep_plan(NCH)

    def cp_qkv():
        return pltpu.make_async_copy(wqkv_hbm, wqkv_raw, sems.at[0])

    def cp_wo():
        return pltpu.make_async_copy(wo_hbm, wo_raw, sems.at[1])

    def cp_x(k):
        lo, n = (0, XFIRST) if k == 0 else (XFIRST, S - XFIRST)
        return pltpu.make_async_copy(x_hbm.at[:, pl.ds(lo, n)], xin.at[:, pl.ds(lo, n)], sems.at[2 + k])

    def chunk_copies(c):
        return [pltpu.make_async_copy(w.at[:, pl.ds(c * 2 * TC, 2 * TC)], raw.at[c, m], sems.at[4 + c])
                for m, w in enumerate((wg_hbm, wu_hbm, wd_hbm))]

    R_SD = 8 * (KH // 2)
    R_END = R_SD + 4 * (DHALF // 2)

    def prep_pieces(c):
        def ld(m, r0, nr, col):
            u = pltpu.bitcast(raw[c, m, pl.ds(r0, nr), pl.ds(col, TC)], u32)
            return u, _unpk(u, 0), _unpk(u, 1)

        def ops(fn, blocks):
            ev = fn(*[b[1] for b in blocks])
            od = fn(*[b[2] for b in blocks])
            out = []
            for e, o in zip(ev, od):
                src = [b[0] for b in blocks if b[1] is e]
                out.append(src[0] if src else _pk2(e, o))
            return out

        def put(m, slot, row, t):
            pw[c, pl.ds((slot * KH + row) // 2, t.shape[0]), m * TC:(m + 1) * TC] = t

        def gu1_piece(m, r):
            blocks = [ld(m, r, PR, 0), ld(m, r, PR, TC), ld(m, KX + r, PR, 0), ld(m, KX + r, PR, TC)]
            for (slot, row), t in zip(V1_POS, ops(_rhs_ops, blocks)):
                put(m, slot, row + r, t)

        def gu2_piece(m, r):
            kc, kd = 2 * KX + r, 2 * KX + KY + r
            blocks = [ld(m, kc, PR, TC), ld(m, kc, PR, 0), ld(m, kd, PR, TC), ld(m, kd, PR, 0)]
            for (slot, row), t in zip(V2_POS, ops(_rhs_ops, blocks)):
                put(m, slot, row + r, t)

        def wr_piece(m):
            r1 = ld(m, 2 * KH, KY, 0)[0]
            r2 = ld(m, 2 * KH, KY, TC)[0]
            put(m, 4, KX, r1)
            put(m, 6, 3 * KY, r1)
            put(m, 5, KX, r2)
            put(m, 6, KY, r2)

        def d_piece(r):
            blocks = [ld(2, r, PR, 0), ld(2, r, PR, TC), ld(2, DHALF + r, PR, 0), ld(2, DHALF + r, PR, TC)]
            for i, t in enumerate(ops(_lhs_ops, blocks)):
                pw[c, pl.ds(R_SD + (i // 2) * (DHALF // 2) + r // 2, PR // 2), (i % 2) * TC:(i % 2 + 1) * TC] = t

        out = []
        for m in range(2):
            out += [functools.partial(gu1_piece, m, r) for r in range(0, KX, PR)]
            out += [functools.partial(gu2_piece, m, r) for r in range(0, KY, PR)]
            out.append(functools.partial(wr_piece, m))
        out += [functools.partial(d_piece, r) for r in range(0, DHALF, PR)]
        return out

    def prep_chunk(c):
        for piece in prep_pieces(c):
            piece()

    def pace_pw(v):
        pw[NCH, pl.ds(R_END, 8), 0:128] = pltpu.bitcast(v, u32)

    nr = TB // RB
    QT = (0, 1, 2, 3, 8)
    KT = (4, 5, 6, 7, 13)
    VT = (9, 10, 11, 12, 8)
    scale = DH ** -0.5
    c2e = scale * math.log2(math.e)
    neg = -1e9 * math.log2(math.e)
    k0 = math.sqrt(2.0 / math.pi)
    k1 = k0 * 0.044715
    zero8 = pl.multiple_of((g >> 20) * 8, 8)

    def x_convert(blk):
        x = xin[:, pl.ds(pl.multiple_of(blk * TB, TB), TB)].astype(f32)
        xres[blk] = x
        return x

    def a_ln1(blk, dst, from_input):
        x = x_convert(blk) if from_input else xres[blk]
        mean, rstd = _ln_stats(x)
        if not from_input:
            dst[pl.ds(0, 8), :] = jnp.zeros((8, KP), u32)
        xn = (xres[blk] - mean) * rstd
        xp = jnp.concatenate([xn, jnp.zeros((KP - D, TB), f32)], axis=0)
        dst[...] = pltpu.bitcast(xp.astype(bf16).T, u32)

    def a_qkv(src, qdst, qprev, t0=0, t1=14, cb=None):
        qkv = _dot_nt(_up(src[...]), _up(wqkvT[pl.ds(t0 * 64, (t1 - t0) * 64), :]))
        for t in range(max(t0, 4), t1):
            qdst[t, pl.ds(0, HALO), :] = qprev[t, pl.ds(TB, HALO), :]
        for t in range(t0, t1):
            qdst[t, pl.ds(HALO, TB), :] = qkv[:, (t - t0) * 128:(t - t0 + 1) * 128]
            if cb is not None:
                for k in range(NPACE):
                    rr = k * (TB // NPACE)
                    cb(qkv[rr:rr + 8, (t - t0) * 128:(t - t0 + 1) * 128])

    zvec = jnp.full((RB, 128), (g >> 20).astype(u32), u32)
    cbits = pltpu.bitcast(jnp.full((RB, 128), c2e, f32), u32)

    def tied_scale(deps):
        if not deps:
            return c2e
        acc = pltpu.bitcast(deps[0], u32)
        for dv in deps[1:]:
            acc = acc | pltpu.bitcast(dv, u32)
        return pltpu.bitcast(cbits | (acc & zvec), f32)

    def tie(x, dep):
        return pltpu.bitcast(pltpu.bitcast(x, u32) | (pltpu.bitcast(dep, u32) & zvec), f32)

    def a_rows(q_s, blk, rs, mode, hist):
        lag_mid, lag_end, midkind, fw, fv = mode
        for r in rs:
            r0 = r * RB
            deps = []
            if lag_mid and r - lag_mid >= 0:
                deps.append(hist[('h' if midkind else 'm', r - lag_mid)])
            if lag_end and r - lag_end >= 0:
                deps += hist[('o', r - lag_end)]
            cs = tied_scale(deps)
            q = [q_s[t, pl.ds(HALO + r0, RB), :] * cs for t in QT]
            sc = []
            q0 = q[0]
            prev = None
            for w in range(W):
                off = HALO + r0 - DIL * w
                acc = None
                if fw and w and w % fw == 0:
                    q0 = tie(q[0], prev)
                for j, t in enumerate(KT):
                    p = (q0 if j == 0 else q[j]) * q_s[t, pl.ds(off, RB), :]
                    acc = p if acc is None else acc + p
                prev = acc
                acc = acc + pltpu.roll(acc, 64, 1)
                hist[('h', r)] = acc
                acc = acc + pltpu.roll(acc, 32, 1)
                if r0 - DIL * w < 0:
                    pos = blk * TB + r0 + lax.broadcasted_iota(jnp.int32, (RB, 128), 0)
                    acc = jnp.where(pos >= DIL * w, acc, neg)
                sc.append(acc)
            m = _tree(jnp.maximum, sc)
            hist[('m', r)] = m
            e = [jnp.exp2(sc[w] - m) for w in range(W)]
            l = _tree(jnp.add, e)
            rinv = pl.reciprocal(l, approx=True)
            rinv = rinv * (2.0 - l * rinv)
            outs = []
            e0 = e[0]
            for j, t in enumerate(VT):
                if fv and j and j % fv == 0:
                    e0 = tie(e[0], acc)
                acc = None
                for w in range(W):
                    off = HALO + r0 - DIL * w
                    p = (e0 if w == 0 else e[w]) * q_s[t, pl.ds(off, RB), :]
                    acc = p if acc is None else acc + p
                o = acc * rinv
                st_off = r0 + zero8 if (j == 4 and r == nr - 1 and FENCE) else r0
                q_s[14 + j, pl.ds(st_off, RB), :] = o
                outs.append(o)
            hist[('o', r)] = outs[-1:] if fv == 1 else outs

    def a_wo(q_s, blk, par):
        o = jnp.concatenate([q_s[14 + j, pl.ds(0, TB), :] for j in range(5)], axis=1).astype(bf16)
        x1 = xres[blk] + _dot_nt(_up(woT[...]), o)
        xres[blk] = x1
        mean, rstd = _ln_stats(x1)
        xn_f[par] = (xres[blk] - mean) * rstd

    def a_sops(slot):
        def seg(tb, r0, n):
            return lambda: xn_f[tb, pl.ds(r0, n), :]
        A11, A12, A21, A22 = seg(0, 0, KX), seg(0, KX, KX), seg(1, 0, KX), seg(1, KX, KX)
        kc, kd = 2 * KX, 2 * KX + KY
        a11, a12, a21, a22 = seg(0, kc, KY), seg(0, kd, KY), seg(1, kc, KY), seg(1, kd, KY)
        rt, rb = seg(0, 2 * KH, KY), seg(1, 2 * KH, KY)
        parts = (
            lambda: (A21() + A22(), -(a21() + a22())),
            lambda: (A11(), a22()),
            lambda: (A22(), a11()),
            lambda: (A11() + A12(), -(a11() + a12())),
            lambda: (A12() - A22(), rt()),
            lambda: (A21() - A11(), rb()),
            lambda: (a12() - a22(), rt(), a21() - a11(), rb()),
            lambda: (A11() + A22(), a11() + a22()),
        )
        for i, fn in enumerate(parts):
            t = jnp.concatenate(fn(), axis=0)
            s_scr[slot, i] = pltpu.bitcast(t.astype(bf16).T, u32)

    class St:
        pass

    def f_init(st, j):
        st.c0 = 0
        st.b0 = (j * NH) % NB
        st.sb = j % NSLOT
        st.acc = [None] * 7
        st.t = {}

    def gelu_mul(c):
        gg = c[:, :TC]
        u = c[:, TC:]
        t = jnp.tanh(gg * (k0 + k1 * (gg * gg)))
        gu = gg * u
        return gu + gu * t

    def f_gu(st, p):
        c = st.c0 + p

        def Q(slot, k0_=0, k1_=KH):
            if k0_ % 128 == 0 and k1_ % 128 == 0:
                lhs = _up(s_scr[st.sb, slot, :, k0_:k1_])
            else:
                lhs = _up(s_scr[st.sb, slot])[:, k0_:k1_]
            return _dot(lhs, _up(pw[c, pl.ds((slot * KH + k0_) // 2, (k1_ - k0_) // 2), :]))
        q5 = Q(3)
        q3 = Q(1)
        q1b = Q(7, KX, KH)
        h12 = gelu_mul(q3 + q5 + q1b + Q(6, 0, 2 * KY))
        q4 = Q(2)
        q2 = Q(0)
        h21 = gelu_mul(q2 + q4 + q1b + Q(6, 2 * KY, KH))
        q1 = Q(7, 0, KX)
        h11 = gelu_mul(q1 + q4 - q5 + Q(4))
        h22 = gelu_mul(q1 - q2 + q3 + Q(5))
        st.t[p] = _rhs_ops(h11, h21, h12, h22)

    def f_d(st, ps):
        for i in DORD:
            a = jnp.concatenate([_up(pw[st.c0 + p, pl.ds(R_SD + (i // 2) * (DHALF // 2), DHALF // 2),
                                         (i % 2) * TC:(i % 2 + 1) * TC]) for p in ps], axis=1)
            t = jnp.concatenate([st.t[p][i] for p in ps], axis=1).astype(bf16)
            r = _dot_nt(a, t)
            st.acc[i] = r if st.acc[i] is None else st.acc[i] + r
        for p in ps:
            del st.t[p]

    def f_store(st):
        m1, m2, m3, m4, m5, m6, m7 = st.acc
        top = jnp.concatenate([m1 + m4 - m5 + m7, m2 + m4], axis=0)
        bot = jnp.concatenate([m3 + m5, m1 - m2 + m3 + m6], axis=0)
        for k, y in enumerate((top, bot)):
            x2 = xres[st.b0 + k] + 0.5 * y
            xres[st.b0 + k] = x2
            o_ref[:, k * TB:(k + 1) * TB] = x2.astype(o_ref.dtype)

    def run_pair(jf, ja):
        st = St()
        f_init(st, jf)
        groups = []
        p0 = 0
        for n in DGROUPS:
            groups.append(list(range(p0, p0 + n)))
            p0 += n
        assert p0 == NCH
        if ja is not None:
            a = (2 * ja) % NB
            b = a + 1
            a_rows(qa, a, range(nr), MODE_F, {})
        for p in range(NCH):
            f_gu(st, p)
            while groups and groups[0][-1] + DLAG <= p:
                f_d(st, groups.pop(0))
            if ja is not None:
                if p == QB_AT:
                    a_qkv(xn1b, qb, qa)
                if p == WOA_AT:
                    a_wo(qa, a, 0)
                if p == RB_AT:
                    a_rows(qb, b, range(nr), MODE_F, {})
                if p == LNA_AT:
                    a_ln1((a + 2) % NB, xn1a, False)
                if p == LNB_AT:
                    a_ln1((b + 2) % NB, xn1b, False)
                if p == WOB_AT:
                    a_wo(qb, b, 1)
        if ja is not None:
            a_sops(ja % NSLOT)
        while groups:
            f_d(st, groups.pop(0))
        f_store(st)
        if ja is not None:
            a_qkv(xn1a, qa, qb)

    def run_aa(j):
        a = 2 * j
        b = a + 1
        pieces = []
        for k in range(CP):
            pieces += prep_pieces(plan_s[j * CP + k])
        wts = [PW1] * (14 * NPACE) + [PW3] * (13 * NPACE) + [0.0] * NPACE
        tot = sum(wts)
        state = dict(pt=0, done=0, cum=0.0)

        def cb(v):
            if not pieces:
                return
            state['cum'] += wts[state['pt']]
            state['pt'] += 1
            upto = int(round(len(pieces) * state['cum'] / tot))
            if upto > state['done'] or state['pt'] == 27 * NPACE + 1:
                pace_pw(v)
            for piece in pieces[state['done']:upto]:
                piece()
            state['done'] = upto

        a_rows(qa, a, range(nr), MODE_A, {})
        a_wo(qb, jnp.where(j == 0, NB, a - 1), 1)
        a_sops(jnp.where(j == 0, NSLOT, j - 1))
        a_ln1(a + 2, xn1a, True)
        a_qkv(xn1b, qb, qa, cb=cb)
        a_rows(qb, b, range(nr), MODE_A, {})
        a_wo(qa, a, 0)
        a_ln1(b + 2, xn1b, True)
        a_qkv(xn1a, qa, qb, cb=cb)
        assert state['done'] == len(pieces)

    @pl.when(g == 0)
    def _():
        cp_x(0).start()
        cp_qkv().start()
        for j in range(KPAIR):
            for k in range(CP):
                plan_s[j * CP + k] = plan[j][k]
        qb[:, pl.ds(TB, HALO), :] = jnp.zeros((20, HALO, 128), f32)
        zpad = jnp.zeros((KP - D, 128), f32)
        cp_x(0).wait()
        a_ln1(0, xn1a, True)
        a_ln1(1, xn1b, True)
        cp_qkv().wait()
        cp_wo().start()
        cp_x(1).start()
        for c in range(NCH):
            for cp in chunk_copies(c):
                cp.start()
        for j in range(14):
            wd_ = 128 if j < 13 else 64
            blk = wqkv_raw[:, j * 128:j * 128 + wd_].astype(f32)
            if wd_ < 128:
                blk = jnp.concatenate([blk, jnp.zeros((D, 128 - wd_), f32)], axis=1)
            bt = jnp.concatenate([blk, zpad], axis=0).T
            for t in range(5):
                tmp[t, pl.ds(j * 128, 128), :] = bt[:, t * 128:(t + 1) * 128]
        for sec in range(3):
            for d in range(DH):
                r = _dst_row(sec, d)
                for t in range(5):
                    wqkvT[pl.ds(r // 2, 16), t * 128:(t + 1) * 128] = _pk2(
                        tmp[t, pl.ds(sec * D + d, 16, stride=2 * DH), :],
                        tmp[t, pl.ds(sec * D + d + DH, 16, stride=2 * DH), :])
        wqkvT[pl.ds((13 * 128 + 64) // 2, 32), :] = jnp.zeros((32, KP), u32)
        cp_wo().wait()
        a_qkv(xn1a, qa, qb)
        for t in range(5):
            wd_ = 128 if t < 4 else 64
            blk = wo_raw[:, t * 128:t * 128 + wd_].astype(f32)
            if wd_ < 128:
                blk = jnp.concatenate([blk, jnp.zeros((D, 128 - wd_), f32)], axis=1)
            tmp[t, pl.ds(0, D), :] = blk
        for t in range(5):
            rows = [tmp[t, pl.ds(d, 32, stride=DH), :] for d in range(DH)]
            full = jnp.concatenate(rows[:16] + [zpad] + rows[16:], axis=0)
            ft = full.T
            n = 128 if t < 4 else 64
            woT[pl.ds(t * 64, n // 2), :] = _pk(ft[:n])

    for j in range(1, KPAIR):
        @pl.when(g == 1 + j)
        def _():
            if j == 1:
                cp_x(1).wait()
            for c in plan[j]:
                if c < NCH:
                    for cp in chunk_copies(c):
                        cp.wait()

    @pl.when(jnp.logical_and(g >= 1, g <= KPAIR))
    def _():
        run_aa(g - 1)

    @pl.when(g == KPAIR + 1)
    def _():
        a_wo(qb, K - 1, 1)
        a_sops(KPAIR - 1)
        for blk in range(K + 2, NB):
            x_convert(blk)

        def body(c, carry):
            for cp in chunk_copies(c):
                cp.wait()
            prep_chunk(c)
            return carry
        if nprepped < NCH:
            lax.fori_loop(nprepped, NCH, body, 0)

    jf = g - (KPAIR + 1)

    @pl.when(jnp.logical_and(jf >= 0, jf < NB - KPAIR))
    def _():
        run_pair(jf, jf + KPAIR)

    @pl.when(jf >= NB - KPAIR)
    def _():
        def body(hf, carry):
            st = St()
            f_init(st, jf)
            st.c0 = hf * NPC
            groups = []
            p0 = 0
            for n in DGROUPS_F:
                groups.append(list(range(p0, p0 + n)))
                p0 += n
            for p in range(NPC):
                f_gu(st, p)
                while groups and groups[0][-1] + DLAG <= p:
                    f_d(st, groups.pop(0))
            while groups:
                f_d(st, groups.pop(0))
            f_store(st)
            return carry
        lax.fori_loop(0, NH, body, 0)


@jax.jit
def pallas_interleave_layers__sliding_local_dilated__glu_gated_geglu__prompt_kernel(
    A_x, A_wqkv, A_wo, B_x, B_w_gate, B_w_up, B_w_down):
    B, S, D = A_x.shape
    DF = B_w_gate.shape[1]
    NB = S // TB
    xT = A_x.reshape(S, D).T
    wdT = B_w_down.T
    NCH = DF // (2 * TC)
    nsteps = 1 + KPAIR + NB
    hbm = pl.BlockSpec(memory_space=pltpu.HBM)
    outT = pl.pallas_call(
        functools.partial(_kernel, D=D, DF=DF, NB=NB),
        grid=(nsteps,),
        in_specs=[hbm] * 6,
        out_specs=pl.BlockSpec((D, TM), lambda g: (0, jnp.maximum(g - (1 + KPAIR + NB // 2), 0))),
        out_shape=jax.ShapeDtypeStruct((D, S), A_x.dtype),
        scratch_shapes=[
            pltpu.VMEM((D, S), bf16),
            pltpu.VMEM((D, 3 * D), bf16),
            pltpu.VMEM((D, D), bf16),
            pltpu.VMEM((NQKV // 2, KP), u32),
            pltpu.VMEM((D // 2, KP), u32),
            pltpu.VMEM((NCH + 1, 3, D, 2 * TC), bf16),
            pltpu.VMEM((NCH + 1, 8 * (KH // 2) + D + 16, 2 * TC), u32),
            pltpu.VMEM((5, NQKV, 128), f32),
            pltpu.VMEM((20, HALO + TB, 128), f32),
            pltpu.VMEM((20, HALO + TB, 128), f32),
            pltpu.VMEM((NB + 1, D, TB), f32),
            pltpu.VMEM((2, D, TB), f32),
            pltpu.VMEM((TB // 2, KP), u32),
            pltpu.VMEM((TB // 2, KP), u32),
            pltpu.VMEM((NSLOT + 1, 8, TB // 2, KH), u32),
            pltpu.SMEM((KPAIR * CP + 1,), jnp.int32),
            pltpu.SemaphoreType.DMA((4 + NCH,)),
        ],
        compiler_params=pltpu.CompilerParams(
            dimension_semantics=("arbitrary",),
            vmem_limit_bytes=110 * 1024 * 1024,
        ),
    )(xT, A_wqkv, A_wo, B_w_gate, B_w_up, wdT)
    return outT.T.reshape(B, S, D)
```

```python
import functools
import math
import jax
import jax.numpy as jnp
from jax import lax
import jax.experimental.pallas as pl
import jax.experimental.pallas.tpu as pltpu

H = 32
DH = 18
W = 8
DIL = 2
HALO = 16
EPS = 1e-5
TB = 128
TM = 256
NH = 2
RB = 8
KP = 640
KH = 256
KX = 192
KY = 64
NQKV = 14 * 128
TC = 128
NSLOT = 8
DG = int(3)
ROWS_LO = int(0)
WO_AT = int(6)
DLAG = int(2)
LN1_AT = int(7)
SERIAL = int(1)
SERIAL_A = int(0)
LN_F = tuple(int(x) for x in '1,4'.split(','))
LN_A = tuple(int(x) for x in '2,8'.split(','))
KPAIR = int(6)
CP = int(3)
QSPLIT = int(5)
XFIRST = 512
DGROUPS = tuple(int(x) for x in '4,4,4,4,2'.split(','))
DGROUPS_F = tuple(int(x) for x in '3,4,2'.split(','))
DORD = tuple(int(x) for x in '0,1,2,3,4,5,6'.split(','))
QB_AT = int(6); WOA_AT = int(7)
LNA_AT = int(1); LNB_AT = int(3); WOB_AT = int(13)
QPR = 16
LND = tuple(int(x) for x in '3,8'.split(','))
WOSPLIT = int(1)
NPACE = int(4)
MODE_F = tuple(int(x) for x in '0,1,0,2,1'.split(','))
MODE_A = tuple(int(x) for x in '1,3,1,0,0'.split(','))
FENCE = int(1)
PR = 32
PW1 = float(1); PW2 = float(1); PW3 = float(1)
SOPS_EARLY = int(1)
CLIP = int(0)

f32 = jnp.float32
bf16 = jnp.bfloat16
u32 = jnp.uint32
NT = (((1,), (1,)), ((), ()))


def _pk(x):
    return pltpu.bitcast(x.astype(bf16), u32)


def _unpk(u, idx):
    return pltpu.unpack_elementwise(u, index=idx, packed_dtype=bf16, unpacked_dtype=f32)


def _pk2(even, odd):
    return pltpu.pack_elementwise([even, odd], packed_dtype=bf16).astype(u32)


def _up(x):
    return pltpu.bitcast(x, bf16)


def _dot(a, b):
    return jnp.dot(a, b, preferred_element_type=f32)


def _dot_nt(a, b):
    return lax.dot_general(a, b, NT, preferred_element_type=f32)


def _ln_stats(x, NACC, pin=None):
    n = x.shape[0]
    c = x[0:1] if pin is None else pin(x[0:8])[0:1]
    s1 = [None] * NACC
    s2 = [None] * NACC
    for i in range(n // 8):
        d = x[i * 8:(i + 1) * 8] - c
        k = i % NACC
        s1[k] = d if s1[k] is None else s1[k] + d
        dd = d * d
        s2[k] = dd if s2[k] is None else s2[k] + dd
    while len(s1) > 1:
        s1 = [s1[i] + s1[i + 1] for i in range(0, len(s1), 2)]
        s2 = [s2[i] + s2[i + 1] for i in range(0, len(s2), 2)]
    m = jnp.sum(s1[0], axis=0, keepdims=True) * (1.0 / n)
    v = jnp.sum(s2[0], axis=0, keepdims=True) * (1.0 / n) - m * m
    v = jnp.maximum(v, 0.0)
    return c + m, lax.rsqrt(v + EPS)


def _tree(fn, xs):
    xs = list(xs)
    while len(xs) > 1:
        xs = [fn(xs[i], xs[i + 1]) for i in range(0, len(xs) - 1, 2)] + ([xs[-1]] if len(xs) % 2 else [])
    return xs[0]


def _lhs_ops(a11, a12, a21, a22):
    return (a11 + a22, a21 + a22, a11, a22, a11 + a12, a21 - a11, a12 - a22)


def _rhs_ops(b11, b12, b21, b22):
    return (b11 + b22, b11, b12 - b22, b21 - b11, b22, b11 + b12, b21 + b22)


def _dst_row(sec, d):
    if sec == 0:
        return d * 32 if d < 16 else 1024 + (d - 16) * 32
    if sec == 1:
        return 512 + d * 32 if d < 16 else 13 * 128 + (d - 16) * 32
    return 9 * 128 + d * 32 if d < 16 else 1024 + 64 + (d - 16) * 32


def _prep_plan(nchunk):
    plan = [[nchunk] * CP]
    nxt = 0
    for j in range(1, KPAIR):
        left_steps = KPAIR - 1 - j
        n = min(CP, nchunk - nxt)
        if j == 1:
            n = max(0, min(n, max(CP - 1, nchunk - nxt - left_steps * CP)))
        ids = list(range(nxt, nxt + n))
        nxt += n
        plan.append(ids + [nchunk] * (CP - n))
    return plan, nxt


def _kernel(x_hbm, wqkv_hbm, wo_hbm, wg_hbm, wu_hbm, wd_hbm, o_ref,
            xin, wqkv_raw, wo_raw, wqkvT, woT, raw, pw, tmp, qa, qb, xres, xn_f, xn1a, xn1b,
            s_scr, wq_s, xn_g, sq_scr, plan_s, sems, *, D, DF, NB):
    g = pl.program_id(0)
    FH = DF // NH
    NPC = FH // (2 * TC)
    NCH = NH * NPC
    NG = NPC // DG
    DHALF = D // 2
    K = 2 * KPAIR
    S = NB * TB
    plan, nprepped = _prep_plan(NCH)

    def cp_qkv():
        return pltpu.make_async_copy(wqkv_hbm, wqkv_raw, sems.at[0])

    def cp_wo():
        return pltpu.make_async_copy(wo_hbm, wo_raw, sems.at[1])

    def cp_x(k):
        lo, n = (0, XFIRST) if k == 0 else (XFIRST, S - XFIRST)
        return pltpu.make_async_copy(x_hbm.at[:, pl.ds(lo, n)], xin.at[:, pl.ds(lo, n)], sems.at[2 + k])

    def chunk_copies(c):
        return [pltpu.make_async_copy(w.at[:, pl.ds(c * 2 * TC, 2 * TC)], raw.at[c, m], sems.at[4 + c])
                for m, w in enumerate((wg_hbm, wu_hbm, wd_hbm))]

    R_SD = 8 * (KH // 2)
    R_END = R_SD + 4 * (DHALF // 2)

    def prep_pieces(c):
        def ld(m, r0, nr, col):
            u = pltpu.bitcast(raw[c, m, pl.ds(r0, nr), pl.ds(col, TC)], u32)
            return u, _unpk(u, 0), _unpk(u, 1)

        def ops(fn, blocks):
            ev = fn(*[b[1] for b in blocks])
            od = fn(*[b[2] for b in blocks])
            out = []
            for e, o in zip(ev, od):
                src = [b[0] for b in blocks if b[1] is e]
                out.append(src[0] if src else _pk2(e, o))
            return out

        def put(m, slot, row, t):
            pw[c, pl.ds((slot * KH + row) // 2, t.shape[0]), m * TC:(m + 1) * TC] = t

        def gu_piece(m, r):
            x1, x2, y1, y2 = ld(m, r, PR, 0), ld(m, r, PR, TC), ld(m, KH + r, PR, 0), ld(m, KH + r, PR, TC)

            def add(u, v):
                return _pk2(u[1] + v[1], u[2] + v[2])

            def sub(u, v):
                return _pk2(u[1] - v[1], u[2] - v[2])
            put(m, 1, r, sub(x2, y2))
            put(m, 2, r, sub(y1, x1))
            if r < KX:
                put(m, 0, r, x1[0])
                put(m, 3, r, y2[0])
                put(m, 4, r, add(y1, y2))
                put(m, 5, r, add(x1, x2))
                put(m, 7, r, add(x1, y2))
            else:
                put(m, 0, r, x2[0])
                put(m, 3, r, y1[0])
                put(m, 6, KY + r - KX, add(y1, y2))
                put(m, 6, 3 * KY + r - KX, add(x1, x2))
                put(m, 7, r, add(x2, y1))

        def wr_piece(m):
            r1 = ld(m, 2 * KH, KY, 0)[0]
            r2 = ld(m, 2 * KH, KY, TC)[0]
            put(m, 4, KX, r1)
            put(m, 6, 2 * KY, r1)
            put(m, 5, KX, r2)
            put(m, 6, 0, r2)

        def d_piece(r):
            blocks = [ld(2, r, PR, 0), ld(2, r, PR, TC), ld(2, DHALF + r, PR, 0), ld(2, DHALF + r, PR, TC)]
            for i, t in enumerate(ops(_lhs_ops, blocks)):
                pw[c, pl.ds(R_SD + (i // 2) * (DHALF // 2) + r // 2, PR // 2), (i % 2) * TC:(i % 2 + 1) * TC] = t

        out = []
        for m in range(2):
            out += [functools.partial(gu_piece, m, r) for r in range(0, KH, PR)]
            out.append(functools.partial(wr_piece, m))
        out += [functools.partial(d_piece, r) for r in range(0, DHALF, PR)]
        return out

    def prep_chunk(c):
        for piece in prep_pieces(c):
            piece()

    def pace_pw(v):
        pw[NCH, pl.ds(R_END, 8), 0:128] = pltpu.bitcast(v, u32)

    nr = TB // RB
    QT = (0, 1, 2, 3, 8)
    KT = (4, 5, 6, 7, 13)
    VT = (9, 10, 11, 12, 8)
    scale = DH ** -0.5
    c2e = scale * math.log2(math.e)
    neg = -1e9 * math.log2(math.e)
    k0 = math.sqrt(2.0 / math.pi)
    k1 = k0 * 0.044715
    zero8 = pl.multiple_of((g >> 20) * 8, 8)

    zvec = jnp.full((RB, 128), (g >> 20).astype(u32), u32)

    def tie(x, dep):
        return pltpu.bitcast(pltpu.bitcast(x, u32) | (pltpu.bitcast(dep, u32) & zvec), f32)

    def normalize(blk, mean, rstd, link):
        if not link:
            return (xres[blk] - mean) * rstd
        rs = jnp.broadcast_to(rstd, (8, TB))
        mb = jnp.broadcast_to(mean, (8, TB))
        outs = []
        for i in range(D // 8):
            if i and i % link == 0:
                rs = tie(rs, outs[-1])
            outs.append((xres[blk, pl.ds(i * 8, 8), :] - mb) * rs)
        return jnp.concatenate(outs, axis=0)

    def x_convert(blk):
        x = xin[:, pl.ds(pl.multiple_of(blk * TB, TB), TB)].astype(f32)
        xres[blk] = x
        return x

    def a_ln1(blk, dst, from_input):
        x = x_convert(blk) if from_input else xres[blk]
        mean, rstd = _ln_stats(x, LN_A[0])
        if not from_input:
            dst[pl.ds(0, 8), :] = jnp.zeros((8, KP), u32)
        xn = (xres[blk] - mean) * rstd
        xp = jnp.concatenate([xn, jnp.zeros((KP - D, TB), f32)], axis=0)
        dst[...] = pltpu.bitcast(xp.astype(bf16).T, u32)

    def a_qkv(src, qdst, qprev, t0=0, t1=14, cb=None):
        qkv = _dot_nt(_up(src[...]), _up(wqkvT[pl.ds(t0 * 64, (t1 - t0) * 64), :]))
        for t in range(max(t0, 4), t1):
            qdst[t, pl.ds(0, HALO), :] = qprev[t, pl.ds(TB, HALO), :]
        for t in range(t0, t1):
            qdst[t, pl.ds(HALO, TB), :] = qkv[:, (t - t0) * 128:(t - t0 + 1) * 128]
            if cb is not None:
                for k in range(NPACE):
                    rr = k * (TB // NPACE)
                    cb(qkv[rr:rr + 8, (t - t0) * 128:(t - t0 + 1) * 128])

    cbits = pltpu.bitcast(jnp.full((RB, 128), c2e, f32), u32)

    def tied_scale(deps):
        if not deps:
            return c2e
        acc = pltpu.bitcast(deps[0], u32)
        for dv in deps[1:]:
            acc = acc | pltpu.bitcast(dv, u32)
        return pltpu.bitcast(cbits | (acc & zvec), f32)

    def a_rows(q_s, blk, rs, mode, hist):
        lag_mid, lag_end, midkind, fw, fv = mode
        for r in rs:
            r0 = r * RB
            deps = []
            if lag_mid and r - lag_mid >= 0:
                deps.append(hist[('h' if midkind else 'm', r - lag_mid)])
            if lag_end and r - lag_end >= 0:
                deps += hist[('o', r - lag_end)]
            cs = tied_scale(deps)
            q = [q_s[t, pl.ds(HALO + r0, RB), :] * cs for t in QT]
            sc = []
            q0 = q[0]
            prev = None
            for w in range(W):
                off = HALO + r0 - DIL * w
                acc = None
                if fw and w and w % fw == 0:
                    q0 = tie(q[0], prev)
                for j, t in enumerate(KT):
                    p = (q0 if j == 0 else q[j]) * q_s[t, pl.ds(off, RB), :]
                    acc = p if acc is None else acc + p
                prev = acc
                acc = acc + pltpu.roll(acc, 64, 1)
                hist[('h', r)] = acc
                acc = acc + pltpu.roll(acc, 32, 1)
                if r0 - DIL * w < 0:
                    pos = blk * TB + r0 + lax.broadcasted_iota(jnp.int32, (RB, 128), 0)
                    acc = jnp.where(pos >= DIL * w, acc, neg)
                sc.append(acc)
            m = _tree(jnp.maximum, sc)
            hist[('m', r)] = m
            e = [jnp.exp2(sc[w] - m) for w in range(W)]
            l = _tree(jnp.add, e)
            rinv = pl.reciprocal(l, approx=True)
            rinv = rinv * (2.0 - l * rinv)
            outs = []
            e0 = e[0]
            for j, t in enumerate(VT):
                if fv and j and j % fv == 0:
                    e0 = tie(e[0], acc)
                acc = None
                for w in range(W):
                    off = HALO + r0 - DIL * w
                    p = (e0 if w == 0 else e[w]) * q_s[t, pl.ds(off, RB), :]
                    acc = p if acc is None else acc + p
                o = acc * rinv
                st_off = r0 + zero8 if (j == 4 and r == nr - 1 and FENCE) else r0
                q_s[14 + j, pl.ds(st_off, RB), :] = o
                outs.append(o)
            hist[('o', r)] = outs[-1:] if fv == 1 else outs

    def a_wo(q_s, blk, par, ln):
        if WOSPLIT:
            o4 = q_s[18, pl.ds(0, TB), :].astype(bf16)
            rq = D // 8
            y = jnp.concatenate([_dot_nt(_up(woT[pl.ds(k * rq, rq), 512:640]), o4) for k in range(4)], axis=0)
            o = jnp.concatenate([q_s[14 + j, pl.ds(0, TB), :] for j in range(4)], axis=1).astype(bf16)
            x1 = _dot_nt(_up(woT[:, 0:512]), o) + (xres[blk] + y)
        else:
            o = jnp.concatenate([q_s[14 + j, pl.ds(0, TB), :] for j in range(5)], axis=1).astype(bf16)
            x1 = xres[blk] + _dot_nt(_up(woT[...]), o)
        xres[blk] = x1
        mean, rstd = _ln_stats(x1, ln[0])
        xn_f[par] = normalize(blk, mean, rstd, ln[1])

    def sops(src, put):
        def seg(tb, r0, n):
            return lambda: src[tb, pl.ds(r0, n), :]
        A11, A12, A21, A22 = seg(0, 0, KX), seg(0, KH, KX), seg(1, 0, KX), seg(1, KH, KX)
        a11, a12, a21, a22 = seg(0, KX, KY), seg(0, KH + KX, KY), seg(1, KX, KY), seg(1, KH + KX, KY)
        rt, rb = seg(0, 2 * KH, KY), seg(1, 2 * KH, KY)
        parts = (
            lambda: (A21() + A22(), -(a21() + a22())),
            lambda: (A11(), -a22()),
            lambda: (A22(), -a11()),
            lambda: (A11() + A12(), -(a11() + a12())),
            lambda: (A12() - A22(), rt()),
            lambda: (A21() - A11(), rb()),
            lambda: (rt(), a12() - a22(), rb(), a21() - a11()),
            lambda: (A11() + A22(), a11() + a22()),
        )
        for i, fn in enumerate(parts):
            t = jnp.concatenate(fn(), axis=0)
            put(i, pltpu.bitcast(t.astype(bf16).T, u32))

    def a_sops(slot):
        def put(i, v):
            s_scr[slot, i] = v
        sops(xn_f, put)

    NQH = NQKV // 4

    def q_prep_pieces():
        lo = lax.broadcasted_iota(jnp.int32, (QPR, 128), 1) < 64

        def piece(r):
            def ld(half, t):
                u = wqkvT[pl.ds(half * NQH + r, QPR), t * 128:(t + 1) * 128]
                return u, _unpk(u, 0), _unpk(u, 1)

            def add(u, v):
                return _pk2(u[1] + v[1], u[2] + v[2])

            def sub(u, v):
                return _pk2(u[1] - v[1], u[2] - v[2])

            def put(tile, v):
                wq_s[pl.ds(r, QPR), tile * 128:(tile + 1) * 128] = v
            r1, r2 = wqkvT[pl.ds(r, QPR), 512:640], wqkvT[pl.ds(NQH + r, QPR), 512:640]
            zero = jnp.zeros((QPR, 128), u32)
            for t in range(2):
                x1, x2, y1, y2 = ld(0, t), ld(1, t), ld(0, 2 + t), ld(1, 2 + t)
                put(2 + t, sub(x2, y2))
                put(4 + t, sub(y1, x1))
                sy, sx, d1 = add(y1, y2), add(x1, x2), add(x1, y2)
                if t == 0:
                    put(0, x1[0])
                    put(6, y2[0])
                    put(8, sy)
                    put(10, sx)
                    put(14, d1)
                else:
                    put(1, jnp.where(lo, x1[0], x2[0]))
                    put(7, jnp.where(lo, y2[0], y1[0]))
                    put(9, jnp.where(lo, sy, r1))
                    put(11, jnp.where(lo, sx, r2))
                    put(12, jnp.where(lo, r2, sy))
                    put(13, jnp.where(lo, r1, sx))
                    put(15, jnp.where(lo, d1, zero))
                    put(16, jnp.where(lo, zero, add(x2, y1)))
        return [functools.partial(piece, r) for r in range(0, NQH, QPR)]

    def a_ln1f(blk, par, dep=None):
        mean, rstd = _ln_stats(xres[blk], LN_F[0], None if dep is None else (lambda v: tie(v, dep)))
        xn_g[par, pl.ds(0, 8), :] = jnp.zeros((8, TB), f32)
        xn_g[par] = normalize(blk, mean, rstd, LN_F[1])

    def a_qsops():
        def put(i, v):
            sq_scr[i, pl.ds(zero8, TB // 2), :] = v
        sops(xn_g, put)

    def a_qkv2_halo(qtop, qbot):
        for t in range(4, 14):
            qtop[t, pl.ds(0, HALO), :] = qbot[t, pl.ds(TB, HALO), :]

    def a_qkv2(qtop, qbot, t0, nt):
        def Q(slot, l0, l1, w0):
            lhs = _up(sq_scr[slot, :, l0:l1])
            rhs = _up(wq_s[pl.ds(t0 * 64, nt * 64), w0 * 128:w0 * 128 + (l1 - l0)])
            return _dot_nt(lhs, rhs)

        def out(dst, tb, v):
            for k in range(nt):
                dst[tb + k, pl.ds(HALO, TB), :] = v[:, k * 128:(k + 1) * 128]
                if dst is qtop and tb + k >= 4:
                    qbot[tb + k, pl.ds(0, HALO), :] = v[TB - HALO:, k * 128:(k + 1) * 128]
        q5 = Q(3, 0, KH, 6)
        q3 = Q(1, 0, KH, 2)
        q1b = Q(7, 128, KH, 16)
        out(qtop, t0 + 7, q3 + q5 + q1b + Q(6, 0, 128, 12))
        q4 = Q(2, 0, KH, 4)
        q2 = Q(0, 0, KH, 0)
        out(qbot, t0, q2 + q4 + q1b + Q(6, 128, KH, 13))
        q1 = Q(7, 0, KH, 14)
        out(qtop, t0, q1 + q4 - q5 + Q(4, 0, KH, 8))
        out(qbot, t0 + 7, q1 - q2 + q3 + Q(5, 0, KH, 10))

    class St:
        pass

    def f_init(st, j):
        st.c0 = 0
        st.b0 = (j * NH) % NB
        st.sb = j % NSLOT
        st.acc = [None] * 7
        st.t = {}

    def gelu_mul(c):
        gg = c[:, :TC]
        u = c[:, TC:]
        t = jnp.tanh(gg * (k0 + k1 * (gg * gg)))
        gu = gg * u
        return gu + gu * t

    def f_gu(st, p):
        c = st.c0 + p

        def Q(slot, k0_=0, k1_=KH):
            if k0_ % 128 == 0 and k1_ % 128 == 0:
                lhs = _up(s_scr[st.sb, slot, :, k0_:k1_])
            else:
                lhs = _up(s_scr[st.sb, slot])[:, k0_:k1_]
            return _dot(lhs, _up(pw[c, pl.ds((slot * KH + k0_) // 2, (k1_ - k0_) // 2), :]))
        q5 = Q(3)
        q3 = Q(1)
        q1b = Q(7, KX, KH)
        h12 = gelu_mul(q3 + q5 + q1b + Q(6, 0, 2 * KY))
        q4 = Q(2)
        q2 = Q(0)
        h21 = gelu_mul(q2 + q4 + q1b + Q(6, 2 * KY, KH))
        q1 = Q(7, 0, KX)
        h11 = gelu_mul(q1 + q4 - q5 + Q(4))
        h22 = gelu_mul(q1 - q2 + q3 + Q(5))
        st.t[p] = _rhs_ops(h11, h21, h12, h22)

    def f_d(st, ps):
        for i in DORD:
            a = jnp.concatenate([_up(pw[st.c0 + p, pl.ds(R_SD + (i // 2) * (DHALF // 2), DHALF // 2),
                                         (i % 2) * TC:(i % 2 + 1) * TC]) for p in ps], axis=1)
            t = jnp.concatenate([st.t[p][i] for p in ps], axis=1).astype(bf16)
            r = _dot_nt(a, t)
            st.acc[i] = r if st.acc[i] is None else r + st.acc[i]
        for p in ps:
            del st.t[p]

    def f_store(st):
        m1, m2, m3, m4, m5, m6, m7 = st.acc
        top = jnp.concatenate([m1 + m4 - m5 + m7, m2 + m4], axis=0)
        bot = jnp.concatenate([m3 + m5, m1 - m2 + m3 + m6], axis=0)
        for k, y in enumerate((top, bot)):
            x2 = xres[st.b0 + k] + 0.5 * y
            xres[st.b0 + k] = x2
            o_ref[:, k * TB:(k + 1) * TB] = x2.astype(o_ref.dtype)

    def run_pair(jf, ja):
        st = St()
        f_init(st, jf)
        groups = []
        p0 = 0
        for n in DGROUPS:
            groups.append(list(range(p0, p0 + n)))
            p0 += n
        assert p0 == NCH
        if ja is not None:
            a = (2 * ja) % NB
            b = a + 1
            ha = {}
            a_rows(qa, a, range(nr), MODE_F, ha)
        for p in range(NCH):
            f_gu(st, p)
            while groups and groups[0][-1] + DLAG <= p:
                f_d(st, groups.pop(0))
            if ja is not None:
                if p == LNA_AT:
                    a_ln1f(b, 0, ha[('h', LND[0])] if LND[0] >= 0 else None)
                if p == LNB_AT:
                    a_ln1f((a + 2) % NB, 1, ha[('h', LND[1])] if LND[1] >= 0 else None)
                    a_qsops()
                if p == WOA_AT:
                    a_wo(qa, a, 0, LN_F)
                if p == QB_AT:
                    a_qkv2_halo(qb, qa)
                    for t0, nt in ((0, 2), (2, 2), (4, 2), (6, 1)):
                        a_qkv2(qb, qa, t0, nt)
                    a_rows(qb, b, range(nr), MODE_F, {})
                if p == WOB_AT:
                    a_wo(qb, b, 1, LN_F)
        if ja is not None:
            a_sops(ja % NSLOT)
        while groups:
            f_d(st, groups.pop(0))
        f_store(st)

    def run_aa(j):
        a = 2 * j
        b = a + 1
        pieces = []
        for k in range(CP):
            pieces += prep_pieces(plan_s[j * CP + k])
        wts = [PW1] * (14 * NPACE) + [PW3] * (13 * NPACE) + [0.0] * NPACE
        tot = sum(wts)
        state = dict(pt=0, done=0, cum=0.0)

        def cb(v):
            if not pieces:
                return
            state['cum'] += wts[state['pt']]
            state['pt'] += 1
            upto = int(round(len(pieces) * state['cum'] / tot))
            if upto > state['done'] or state['pt'] == 27 * NPACE + 1:
                pace_pw(v)
            for piece in pieces[state['done']:upto]:
                piece()
            state['done'] = upto

        a_rows(qa, a, range(nr), MODE_A, {})
        a_wo(qb, jnp.where(j == 0, NB, a - 1), 1, LN_A)
        a_sops(jnp.where(j == 0, NSLOT, j - 1))
        a_ln1(a + 2, xn1a, True)
        a_qkv(xn1b, qb, qa, cb=cb)
        a_rows(qb, b, range(nr), MODE_A, {})
        a_wo(qa, a, 0, LN_A)
        a_ln1(b + 2, xn1b, True)
        a_qkv(xn1a, qa, qb, cb=cb)
        assert state['done'] == len(pieces)

    @pl.when(g == 0)
    def _():
        cp_x(0).start()
        cp_qkv().start()
        for j in range(KPAIR):
            for k in range(CP):
                plan_s[j * CP + k] = plan[j][k]
        qb[:, pl.ds(TB, HALO), :] = jnp.zeros((20, HALO, 128), f32)
        zpad = jnp.zeros((KP - D, 128), f32)
        cp_x(0).wait()
        a_ln1(0, xn1a, True)
        a_ln1(1, xn1b, True)
        cp_qkv().wait()
        cp_wo().start()
        cp_x(1).start()
        for c in range(NCH):
            for cp in chunk_copies(c):
                cp.start()
        for j in range(14):
            wd_ = 128 if j < 13 else 64
            blk = wqkv_raw[:, j * 128:j * 128 + wd_].astype(f32)
            if wd_ < 128:
                blk = jnp.concatenate([blk, jnp.zeros((D, 128 - wd_), f32)], axis=1)
            bt = jnp.concatenate([blk, blk[2 * KH:]], axis=0).T
            for t in range(5):
                tmp[t, pl.ds(j * 128, 128), :] = bt[:, t * 128:(t + 1) * 128]
        for sec in range(3):
            for d in range(DH):
                r = _dst_row(sec, d)
                for t in range(5):
                    wqkvT[pl.ds(r // 2, 16), t * 128:(t + 1) * 128] = _pk2(
                        tmp[t, pl.ds(sec * D + d, 16, stride=2 * DH), :],
                        tmp[t, pl.ds(sec * D + d + DH, 16, stride=2 * DH), :])
        wqkvT[pl.ds((13 * 128 + 64) // 2, 32), :] = jnp.zeros((32, KP), u32)
        cp_wo().wait()
        a_qkv(xn1a, qa, qb)
        for t in range(5):
            wd_ = 128 if t < 4 else 64
            blk = wo_raw[:, t * 128:t * 128 + wd_].astype(f32)
            if wd_ < 128:
                blk = jnp.concatenate([blk, jnp.zeros((D, 128 - wd_), f32)], axis=1)
            tmp[t, pl.ds(0, D), :] = blk
        for t in range(5):
            rows = [tmp[t, pl.ds(d, 32, stride=DH), :] for d in range(DH)]
            full = jnp.concatenate(rows[:16] + [zpad] + rows[16:], axis=0)
            ft = full.T
            n = 128 if t < 4 else 64
            woT[pl.ds(t * 64, n // 2), :] = _pk(ft[:n])

    for j in range(1, KPAIR):
        @pl.when(g == 1 + j)
        def _():
            if j == 1:
                cp_x(1).wait()
            for c in plan[j]:
                if c < NCH:
                    for cp in chunk_copies(c):
                        cp.wait()

    @pl.when(jnp.logical_and(g >= 1, g <= KPAIR))
    def _():
        run_aa(g - 1)

    @pl.when(g == KPAIR + 1)
    def _():
        a_wo(qb, K - 1, 1, (4, 0))
        a_sops(KPAIR - 1)
        for piece in q_prep_pieces():
            piece()
        for blk in range(K + 2, NB):
            x_convert(blk)

        def body(c, carry):
            for cp in chunk_copies(c):
                cp.wait()
            prep_chunk(c)
            return carry
        if nprepped < NCH:
            lax.fori_loop(nprepped, NCH, body, 0)

    jf = g - (KPAIR + 1)

    @pl.when(jnp.logical_and(jf >= 0, jf < NB - KPAIR))
    def _():
        run_pair(jf, jf + KPAIR)

    @pl.when(jf >= NB - KPAIR)
    def _():
        def body(hf, carry):
            st = St()
            f_init(st, jf)
            st.c0 = hf * NPC
            groups = []
            p0 = 0
            for n in DGROUPS_F:
                groups.append(list(range(p0, p0 + n)))
                p0 += n
            for p in range(NPC):
                f_gu(st, p)
                while groups and groups[0][-1] + DLAG <= p:
                    f_d(st, groups.pop(0))
            while groups:
                f_d(st, groups.pop(0))
            f_store(st)
            return carry
        lax.fori_loop(0, NH, body, 0)


@jax.jit
def pallas_interleave_layers__sliding_local_dilated__glu_gated_geglu__prompt_kernel(
    A_x, A_wqkv, A_wo, B_x, B_w_gate, B_w_up, B_w_down):
    B, S, D = A_x.shape
    DF = B_w_gate.shape[1]
    NB = S // TB
    xT = A_x.reshape(S, D).T
    wdT = B_w_down.T
    NCH = DF // (2 * TC)
    nsteps = 1 + KPAIR + NB
    hbm = pl.BlockSpec(memory_space=pltpu.HBM)
    outT = pl.pallas_call(
        functools.partial(_kernel, D=D, DF=DF, NB=NB),
        grid=(nsteps,),
        in_specs=[hbm] * 6,
        out_specs=pl.BlockSpec((D, TM), lambda g: (0, jnp.maximum(g - (1 + KPAIR + NB // 2), 0))),
        out_shape=jax.ShapeDtypeStruct((D, S), A_x.dtype),
        scratch_shapes=[
            pltpu.VMEM((D, S), bf16),
            pltpu.VMEM((D, 3 * D), bf16),
            pltpu.VMEM((D, D), bf16),
            pltpu.VMEM((NQKV // 2, KP), u32),
            pltpu.VMEM((D // 2, KP), u32),
            pltpu.VMEM((NCH + 1, 3, D, 2 * TC), bf16),
            pltpu.VMEM((NCH + 1, 8 * (KH // 2) + D + 16, 2 * TC), u32),
            pltpu.VMEM((5, NQKV, 128), f32),
            pltpu.VMEM((20, HALO + TB, 128), f32),
            pltpu.VMEM((20, HALO + TB, 128), f32),
            pltpu.VMEM((NB + 1, D, TB), f32),
            pltpu.VMEM((2, D, TB), f32),
            pltpu.VMEM((TB // 2, KP), u32),
            pltpu.VMEM((TB // 2, KP), u32),
            pltpu.VMEM((NSLOT + 1, 8, TB // 2, KH), u32),
            pltpu.VMEM((NQKV // 4, 17 * 128), u32),
            pltpu.VMEM((2, D, TB), f32),
            pltpu.VMEM((8, TB // 2, KH), u32),
            pltpu.SMEM((KPAIR * CP + 1,), jnp.int32),
            pltpu.SemaphoreType.DMA((4 + NCH,)),
        ],
        compiler_params=pltpu.CompilerParams(
            dimension_semantics=("arbitrary",),
            vmem_limit_bytes=110 * 1024 * 1024,
        ),
    )(xT, A_wqkv, A_wo, B_w_gate, B_w_up, wdT)
    return outT.T.reshape(B, S, D)
```

```python
import functools
import math
import jax
import jax.numpy as jnp
from jax import lax
import jax.experimental.pallas as pl
import jax.experimental.pallas.tpu as pltpu

H = 32
DH = 18
W = 8
DIL = 2
HALO = 16
EPS = 1e-5
TB = 128
TM = 256
NH = 2
RB = 8
KP = 640
KH = 256
KX = 192
KY = 64
NQKV = 14 * 128
TC = 128
NSLOT = 8
DG = int(3)
ROWS_LO = int(0)
WO_AT = int(6)
DLAG = int(2)
LN1_AT = int(7)
SERIAL = int(1)
SERIAL_A = int(0)
LN_F = tuple(int(x) for x in '1,4'.split(','))
LN_A = tuple(int(x) for x in '2,8'.split(','))
KPAIR = int(6)
CP = int(3)
QSPLIT = int(5)
XFIRST = 512
DGROUPS = tuple(int(x) for x in '4,4,4,4,2'.split(','))
DGROUPS_F = tuple(int(x) for x in '3,4,2'.split(','))
DORD = tuple(int(x) for x in '0,1,2,3,4,5,6'.split(','))
QB_AT = int(6); WOA_AT = int(7)
LNA_AT = int(1); LNB_AT = int(3); WOB_AT = int(13)
QPR = 16
RESTAT = int(0)
TAILF = float(0.6)
LND = tuple(int(x) for x in '3,8'.split(','))
WOSPLIT = int(1)
NPACE = int(4)
MODE_F = tuple(int(x) for x in '0,1,0,2,1'.split(','))
MODE_A = tuple(int(x) for x in '1,3,1,0,0'.split(','))
FENCE = int(1)
PR = 32
PW1 = float(1); PW2 = float(1); PW3 = float(1)
SOPS_EARLY = int(1)
CLIP = int(0)

f32 = jnp.float32
bf16 = jnp.bfloat16
u32 = jnp.uint32
NT = (((1,), (1,)), ((), ()))


def _pk(x):
    return pltpu.bitcast(x.astype(bf16), u32)


def _unpk(u, idx):
    return pltpu.unpack_elementwise(u, index=idx, packed_dtype=bf16, unpacked_dtype=f32)


def _pk2(even, odd):
    return pltpu.pack_elementwise([even, odd], packed_dtype=bf16).astype(u32)


def _up(x):
    return pltpu.bitcast(x, bf16)


def _dot(a, b):
    return jnp.dot(a, b, preferred_element_type=f32)


def _dot_nt(a, b):
    return lax.dot_general(a, b, NT, preferred_element_type=f32)


def _ln_stats(x, NACC, pin=None):
    n = x.shape[0]
    c = x[0:1] if pin is None else pin(x[0:8])[0:1]
    s1 = [None] * NACC
    s2 = [None] * NACC
    for i in range(n // 8):
        d = x[i * 8:(i + 1) * 8] - c
        k = i % NACC
        s1[k] = d if s1[k] is None else s1[k] + d
        dd = d * d
        s2[k] = dd if s2[k] is None else s2[k] + dd
    while len(s1) > 1:
        s1 = [s1[i] + s1[i + 1] for i in range(0, len(s1), 2)]
        s2 = [s2[i] + s2[i + 1] for i in range(0, len(s2), 2)]
    m = jnp.sum(s1[0], axis=0, keepdims=True) * (1.0 / n)
    v = jnp.sum(s2[0], axis=0, keepdims=True) * (1.0 / n) - m * m
    v = jnp.maximum(v, 0.0)
    return c + m, lax.rsqrt(v + EPS)


def _tree(fn, xs):
    xs = list(xs)
    while len(xs) > 1:
        xs = [fn(xs[i], xs[i + 1]) for i in range(0, len(xs) - 1, 2)] + ([xs[-1]] if len(xs) % 2 else [])
    return xs[0]


def _lhs_ops(a11, a12, a21, a22):
    return (a11 + a22, a21 + a22, a11, a22, a11 + a12, a21 - a11, a12 - a22)


def _rhs_ops(b11, b12, b21, b22):
    return (b11 + b22, b11, b12 - b22, b21 - b11, b22, b11 + b12, b21 + b22)


def _dst_row(sec, d):
    if sec == 0:
        return d * 32 if d < 16 else 1024 + (d - 16) * 32
    if sec == 1:
        return 512 + d * 32 if d < 16 else 13 * 128 + (d - 16) * 32
    return 9 * 128 + d * 32 if d < 16 else 1024 + 64 + (d - 16) * 32


def _prep_plan(nchunk):
    plan = [[nchunk] * CP]
    nxt = 0
    for j in range(1, KPAIR):
        left_steps = KPAIR - 1 - j
        n = min(CP, nchunk - nxt)
        if j == 1:
            n = max(0, min(n, max(CP - 1, nchunk - nxt - left_steps * CP)))
        ids = list(range(nxt, nxt + n))
        nxt += n
        plan.append(ids + [nchunk] * (CP - n))
    return plan, nxt


def _kernel(x_hbm, wqkv_hbm, wo_hbm, wg_hbm, wu_hbm, wd_hbm, o_ref,
            xin, wqkv_raw, wo_raw, wqkvT, woT, raw, pw, tmp, qa, qb, xres, xn_f, xn1a, xn1b,
            s_scr, wq_s, xn_g, sq_scr, plan_s, sems, *, D, DF, NB):
    g = pl.program_id(0)
    FH = DF // NH
    NPC = FH // (2 * TC)
    NCH = NH * NPC
    NG = NPC // DG
    DHALF = D // 2
    K = 2 * KPAIR
    S = NB * TB
    plan, nprepped = _prep_plan(NCH)
    zero8 = pl.multiple_of((g >> 20) * 8, 8)

    QSEC = ((0, 5), (5, 9), (9, 14))
    XPC = ((0, 256), (256, 512), (512, 1024), (1024, 1536), (1536, S))

    def cp_qkv(sec):
        out = []
        for j in range(*QSEC[sec]):
            n = min(128, 3 * D - j * 128)
            out.append(pltpu.make_async_copy(wqkv_hbm.at[:, pl.ds(j * 128, n)], wqkv_raw.at[:, pl.ds(j * 128, n)],
                                             sems.at[sec]))
        return out

    def cp_wo():
        return pltpu.make_async_copy(wo_hbm, wo_raw, sems.at[3])

    def cp_x(k):
        lo, hi = XPC[k]
        return pltpu.make_async_copy(x_hbm.at[:, pl.ds(lo, hi - lo)], xin.at[:, pl.ds(lo, hi - lo)], sems.at[4 + k])

    def chunk_copies(c):
        return [pltpu.make_async_copy(w.at[:, pl.ds(c * 2 * TC, 2 * TC)], raw.at[c, m], sems.at[9 + c])
                for m, w in enumerate((wg_hbm, wu_hbm, wd_hbm))]

    R_SD = 8 * (KH // 2)
    R_END = R_SD + 4 * (DHALF // 2)

    def prep_pieces(c):
        def ld(m, r0, nr, col):
            u = pltpu.bitcast(raw[c, m, pl.ds(r0, nr), pl.ds(col, TC)], u32)
            return u, _unpk(u, 0), _unpk(u, 1)

        def ops(fn, blocks):
            ev = fn(*[b[1] for b in blocks])
            od = fn(*[b[2] for b in blocks])
            out = []
            for e, o in zip(ev, od):
                src = [b[0] for b in blocks if b[1] is e]
                out.append(src[0] if src else _pk2(e, o))
            return out

        def put(m, slot, row, t):
            pw[c, pl.ds((slot * KH + row) // 2, t.shape[0]), m * TC:(m + 1) * TC] = t

        def gu_piece(m, r):
            x1, x2, y1, y2 = ld(m, r, PR, 0), ld(m, r, PR, TC), ld(m, KH + r, PR, 0), ld(m, KH + r, PR, TC)

            def add(u, v):
                return _pk2(u[1] + v[1], u[2] + v[2])

            def sub(u, v):
                return _pk2(u[1] - v[1], u[2] - v[2])
            put(m, 1, r, sub(x2, y2))
            put(m, 2, r, sub(y1, x1))
            if r < KX:
                put(m, 0, r, x1[0])
                put(m, 3, r, y2[0])
                put(m, 4, r, add(y1, y2))
                put(m, 5, r, add(x1, x2))
                put(m, 7, r, add(x1, y2))
            else:
                put(m, 0, r, x2[0])
                put(m, 3, r, y1[0])
                put(m, 6, KY + r - KX, add(y1, y2))
                put(m, 6, 3 * KY + r - KX, add(x1, x2))
                put(m, 7, r, add(x2, y1))

        def wr_piece(m):
            r1 = ld(m, 2 * KH, KY, 0)[0]
            r2 = ld(m, 2 * KH, KY, TC)[0]
            put(m, 4, KX, r1)
            put(m, 6, 2 * KY, r1)
            put(m, 5, KX, r2)
            put(m, 6, 0, r2)

        def d_piece(r):
            blocks = [ld(2, r, PR, 0), ld(2, r, PR, TC), ld(2, DHALF + r, PR, 0), ld(2, DHALF + r, PR, TC)]
            for i, t in enumerate(ops(_lhs_ops, blocks)):
                pw[c, pl.ds(R_SD + (i // 2) * (DHALF // 2) + r // 2, PR // 2), (i % 2) * TC:(i % 2 + 1) * TC] = t

        out = []
        for m in range(2):
            out += [functools.partial(gu_piece, m, r) for r in range(0, KH, PR)]
            out.append(functools.partial(wr_piece, m))
        out += [functools.partial(d_piece, r) for r in range(0, DHALF, PR)]
        return out

    def prep_chunk(c):
        for piece in prep_pieces(c):
            piece()

    class Pacer:
        def __init__(self, pieces, pace, npts, idle=0):
            self.pieces, self.pace, self.n, self.pt, self.done = pieces, pace, npts - idle, 0, 0

        def __call__(self, v):
            self.pt += 1
            upto = min(len(self.pieces), int(round(len(self.pieces) * self.pt / self.n)))
            if upto > self.done or self.pt == self.n + 1:
                self.pace(v)
            for piece in self.pieces[self.done:upto]:
                piece()
            self.done = upto

    def pace_wq(v):
        wq_s[pl.ds(NQKV // 4 + zero8, 8), 0:128] = pltpu.bitcast(v, u32)

    def pace_pwz(v):
        pw[NCH, pl.ds(R_END + zero8, 8), 0:128] = pltpu.bitcast(v, u32)

    def pace_pw(v):
        pw[NCH, pl.ds(R_END, 8), 0:128] = pltpu.bitcast(v, u32)

    nr = TB // RB
    QT = (0, 1, 2, 3, 8)
    KT = (4, 5, 6, 7, 13)
    VT = (9, 10, 11, 12, 8)
    scale = DH ** -0.5
    c2e = scale * math.log2(math.e)
    neg = -1e9 * math.log2(math.e)
    k0 = math.sqrt(2.0 / math.pi)
    k1 = k0 * 0.044715

    zvec = jnp.full((RB, 128), (g >> 20).astype(u32), u32)

    def tie(x, dep):
        return pltpu.bitcast(pltpu.bitcast(x, u32) | (pltpu.bitcast(dep, u32) & zvec), f32)

    def normalize(blk, mean, rstd, link):
        if not link:
            return (xres[blk] - mean) * rstd
        rs = jnp.broadcast_to(rstd, (8, TB))
        mb = jnp.broadcast_to(mean, (8, TB))
        outs = []
        for i in range(D // 8):
            if i and i % link == 0:
                rs = tie(rs, outs[-1])
            outs.append((xres[blk, pl.ds(i * 8, 8), :] - mb) * rs)
        return jnp.concatenate(outs, axis=0)

    def x_convert(blk):
        x = xin[:, pl.ds(pl.multiple_of(blk * TB, TB), TB)].astype(f32)
        xres[blk] = x
        return x

    def a_ln1(blk, dst, from_input):
        x = x_convert(blk) if from_input else xres[blk]
        mean, rstd = _ln_stats(x, LN_A[0])
        if not from_input:
            dst[pl.ds(0, 8), :] = jnp.zeros((8, KP), u32)
        xn = (xres[blk] - mean) * rstd
        xp = jnp.concatenate([xn, jnp.zeros((KP - D, TB), f32)], axis=0)
        dst[...] = pltpu.bitcast(xp.astype(bf16).T, u32)

    def a_qkv(src, qdst, qprev, t0=0, t1=14, cb=None):
        qkv = _dot_nt(_up(src[...]), _up(wqkvT[pl.ds(t0 * 64, (t1 - t0) * 64), :]))
        for t in range(max(t0, 4), t1):
            qdst[t, pl.ds(0, HALO), :] = qprev[t, pl.ds(TB, HALO), :]
        for t in range(t0, t1):
            qdst[t, pl.ds(HALO, TB), :] = qkv[:, (t - t0) * 128:(t - t0 + 1) * 128]
            if cb is not None:
                for k in range(NPACE):
                    rr = k * (TB // NPACE)
                    cb(qkv[rr:rr + 8, (t - t0) * 128:(t - t0 + 1) * 128])

    cbits = pltpu.bitcast(jnp.full((RB, 128), c2e, f32), u32)

    def tied_scale(deps):
        if not deps:
            return c2e
        acc = pltpu.bitcast(deps[0], u32)
        for dv in deps[1:]:
            acc = acc | pltpu.bitcast(dv, u32)
        return pltpu.bitcast(cbits | (acc & zvec), f32)

    def a_rows(q_s, blk, rs, mode, hist):
        lag_mid, lag_end, midkind, fw, fv = mode
        for r in rs:
            r0 = r * RB
            deps = []
            if lag_mid and r - lag_mid >= 0:
                deps.append(hist[('h' if midkind else 'm', r - lag_mid)])
            if lag_end and r - lag_end >= 0:
                deps += hist[('o', r - lag_end)]
            cs = tied_scale(deps)
            q = [q_s[t, pl.ds(HALO + r0, RB), :] * cs for t in QT]
            sc = []
            q0 = q[0]
            prev = None
            for w in range(W):
                off = HALO + r0 - DIL * w
                acc = None
                if fw and w and w % fw == 0:
                    q0 = tie(q[0], prev)
                for j, t in enumerate(KT):
                    p = (q0 if j == 0 else q[j]) * q_s[t, pl.ds(off, RB), :]
                    acc = p if acc is None else acc + p
                prev = acc
                acc = acc + pltpu.roll(acc, 64, 1)
                hist[('h', r)] = acc
                acc = acc + pltpu.roll(acc, 32, 1)
                if r0 - DIL * w < 0:
                    pos = blk * TB + r0 + lax.broadcasted_iota(jnp.int32, (RB, 128), 0)
                    acc = jnp.where(pos >= DIL * w, acc, neg)
                sc.append(acc)
            m = _tree(jnp.maximum, sc)
            hist[('m', r)] = m
            e = [jnp.exp2(sc[w] - m) for w in range(W)]
            l = _tree(jnp.add, e)
            rinv = pl.reciprocal(l, approx=True)
            rinv = rinv * (2.0 - l * rinv)
            outs = []
            e0 = e[0]
            for j, t in enumerate(VT):
                if fv and j and j % fv == 0:
                    e0 = tie(e[0], acc)
                acc = None
                for w in range(W):
                    off = HALO + r0 - DIL * w
                    p = (e0 if w == 0 else e[w]) * q_s[t, pl.ds(off, RB), :]
                    acc = p if acc is None else acc + p
                o = acc * rinv
                st_off = r0 + zero8 if (j == 4 and r == nr - 1 and FENCE) else r0
                q_s[14 + j, pl.ds(st_off, RB), :] = o
                outs.append(o)
            hist[('o', r)] = outs[-1:] if fv == 1 else outs

    def a_wo(q_s, blk, par, ln, cb=None):
        if WOSPLIT:
            o4 = q_s[18, pl.ds(0, TB), :].astype(bf16)
            rq = D // 8
            y = jnp.concatenate([_dot_nt(_up(woT[pl.ds(k * rq, rq), 512:640]), o4) for k in range(4)], axis=0)
            o = jnp.concatenate([q_s[14 + j, pl.ds(0, TB), :] for j in range(4)], axis=1).astype(bf16)
            x1 = _dot_nt(_up(woT[:, 0:512]), o) + (xres[blk] + y)
        else:
            o = jnp.concatenate([q_s[14 + j, pl.ds(0, TB), :] for j in range(5)], axis=1).astype(bf16)
            x1 = xres[blk] + _dot_nt(_up(woT[...]), o)
        xres[blk] = x1
        if cb is not None:
            for i in range(0, D, 16):
                cb(x1[i:i + 8])
        mean, rstd = _ln_stats(x1, ln[0])
        xn_f[par] = normalize(blk, mean, rstd, ln[1])

    def sops(src, put):
        def seg(tb, r0, n):
            return lambda: src[tb, pl.ds(r0, n), :]
        A11, A12, A21, A22 = seg(0, 0, KX), seg(0, KH, KX), seg(1, 0, KX), seg(1, KH, KX)
        a11, a12, a21, a22 = seg(0, KX, KY), seg(0, KH + KX, KY), seg(1, KX, KY), seg(1, KH + KX, KY)
        rt, rb = seg(0, 2 * KH, KY), seg(1, 2 * KH, KY)
        parts = (
            lambda: (A21() + A22(), -(a21() + a22())),
            lambda: (A11(), -a22()),
            lambda: (A22(), -a11()),
            lambda: (A11() + A12(), -(a11() + a12())),
            lambda: (A12() - A22(), rt()),
            lambda: (A21() - A11(), rb()),
            lambda: (rt(), a12() - a22(), rb(), a21() - a11()),
            lambda: (A11() + A22(), a11() + a22()),
        )
        for i, fn in enumerate(parts):
            t = jnp.concatenate(fn(), axis=0)
            put(i, pltpu.bitcast(t.astype(bf16).T, u32))

    def a_sops(slot):
        def put(i, v):
            s_scr[slot, i] = v
        sops(xn_f, put)

    NQH = NQKV // 4

    def q_prep_pieces():
        lo = lax.broadcasted_iota(jnp.int32, (QPR, 128), 1) < 64

        def piece(r):
            def ld(half, t):
                u = wqkvT[pl.ds(half * NQH + r, QPR), t * 128:(t + 1) * 128]
                return u, _unpk(u, 0), _unpk(u, 1)

            def add(u, v):
                return _pk2(u[1] + v[1], u[2] + v[2])

            def sub(u, v):
                return _pk2(u[1] - v[1], u[2] - v[2])

            def put(tile, v):
                wq_s[pl.ds(r, QPR), tile * 128:(tile + 1) * 128] = v
            r1, r2 = wqkvT[pl.ds(r, QPR), 512:640], wqkvT[pl.ds(NQH + r, QPR), 512:640]
            zero = jnp.zeros((QPR, 128), u32)
            for t in range(2):
                x1, x2, y1, y2 = ld(0, t), ld(1, t), ld(0, 2 + t), ld(1, 2 + t)
                put(2 + t, sub(x2, y2))
                put(4 + t, sub(y1, x1))
                sy, sx, d1 = add(y1, y2), add(x1, x2), add(x1, y2)
                if t == 0:
                    put(0, x1[0])
                    put(6, y2[0])
                    put(8, sy)
                    put(10, sx)
                    put(14, d1)
                else:
                    put(1, jnp.where(lo, x1[0], x2[0]))
                    put(7, jnp.where(lo, y2[0], y1[0]))
                    put(9, jnp.where(lo, sy, r1))
                    put(11, jnp.where(lo, sx, r2))
                    put(12, jnp.where(lo, r2, sy))
                    put(13, jnp.where(lo, r1, sx))
                    put(15, jnp.where(lo, d1, zero))
                    put(16, jnp.where(lo, zero, add(x2, y1)))
        return [functools.partial(piece, r) for r in range(0, NQH, QPR)]

    def a_ln1f(blk, par, dep=None):
        mean, rstd = _ln_stats(xres[blk], LN_F[0], None if dep is None else (lambda v: tie(v, dep)))
        xn_g[par, pl.ds(0, 8), :] = jnp.zeros((8, TB), f32)
        xn_g[par] = normalize(blk, mean, rstd, LN_F[1])

    def a_qsops():
        def put(i, v):
            sq_scr[i, pl.ds(zero8, TB // 2), :] = v
        sops(xn_g, put)

    def a_qkv2_halo(qtop, qbot):
        for t in range(4, 14):
            qtop[t, pl.ds(0, HALO), :] = qbot[t, pl.ds(TB, HALO), :]

    def a_qkv2(qtop, qbot, t0, nt):
        def Q(slot, l0, l1, w0):
            lhs = _up(sq_scr[slot, :, l0:l1])
            rhs = _up(wq_s[pl.ds(t0 * 64, nt * 64), w0 * 128:w0 * 128 + (l1 - l0)])
            return _dot_nt(lhs, rhs)

        def out(dst, tb, v):
            for k in range(nt):
                dst[tb + k, pl.ds(HALO, TB), :] = v[:, k * 128:(k + 1) * 128]
                if dst is qtop and tb + k >= 4:
                    qbot[tb + k, pl.ds(0, HALO), :] = v[TB - HALO:, k * 128:(k + 1) * 128]
        q5 = Q(3, 0, KH, 6)
        q3 = Q(1, 0, KH, 2)
        q1b = Q(7, 128, KH, 16)
        out(qtop, t0 + 7, q3 + q5 + q1b + Q(6, 0, 128, 12))
        q4 = Q(2, 0, KH, 4)
        q2 = Q(0, 0, KH, 0)
        out(qbot, t0, q2 + q4 + q1b + Q(6, 128, KH, 13))
        q1 = Q(7, 0, KH, 14)
        out(qtop, t0, q1 + q4 - q5 + Q(4, 0, KH, 8))
        out(qbot, t0 + 7, q1 - q2 + q3 + Q(5, 0, KH, 10))

    class St:
        pass

    def f_init(st, j):
        st.c0 = 0
        st.b0 = (j * NH) % NB
        st.sb = j % NSLOT
        st.acc = [None] * 7
        st.t = {}

    def gelu_mul(c):
        gg = c[:, :TC]
        u = c[:, TC:]
        t = jnp.tanh(gg * (k0 + k1 * (gg * gg)))
        gu = gg * u
        return gu + gu * t

    def f_gu(st, p):
        c = st.c0 + p

        def Q(slot, k0_=0, k1_=KH):
            if k0_ % 128 == 0 and k1_ % 128 == 0:
                lhs = _up(s_scr[st.sb, slot, :, k0_:k1_])
            else:
                lhs = _up(s_scr[st.sb, slot])[:, k0_:k1_]
            return _dot(lhs, _up(pw[c, pl.ds((slot * KH + k0_) // 2, (k1_ - k0_) // 2), :]))
        q5 = Q(3)
        q3 = Q(1)
        q1b = Q(7, KX, KH)
        h12 = gelu_mul(q3 + q5 + q1b + Q(6, 0, 2 * KY))
        q4 = Q(2)
        q2 = Q(0)
        h21 = gelu_mul(q2 + q4 + q1b + Q(6, 2 * KY, KH))
        q1 = Q(7, 0, KX)
        h11 = gelu_mul(q1 + q4 - q5 + Q(4))
        h22 = gelu_mul(q1 - q2 + q3 + Q(5))
        st.t[p] = _rhs_ops(h11, h21, h12, h22)

    def f_d(st, ps):
        for i in DORD:
            a = jnp.concatenate([_up(pw[st.c0 + p, pl.ds(R_SD + (i // 2) * (DHALF // 2), DHALF // 2),
                                         (i % 2) * TC:(i % 2 + 1) * TC]) for p in ps], axis=1)
            t = jnp.concatenate([st.t[p][i] for p in ps], axis=1).astype(bf16)
            r = _dot_nt(a, t)
            st.acc[i] = r if st.acc[i] is None else r + st.acc[i]
        for p in ps:
            del st.t[p]

    def f_store(st):
        m1, m2, m3, m4, m5, m6, m7 = st.acc
        top = jnp.concatenate([m1 + m4 - m5 + m7, m2 + m4], axis=0)
        bot = jnp.concatenate([m3 + m5, m1 - m2 + m3 + m6], axis=0)
        for k, y in enumerate((top, bot)):
            x2 = xres[st.b0 + k] + 0.5 * y
            xres[st.b0 + k] = x2
            o_ref[:, k * TB:(k + 1) * TB] = x2.astype(o_ref.dtype)

    def run_pair(jf, ja):
        st = St()
        f_init(st, jf)
        groups = []
        p0 = 0
        for n in DGROUPS:
            groups.append(list(range(p0, p0 + n)))
            p0 += n
        assert p0 == NCH
        if ja is not None:
            a = (2 * ja) % NB
            b = a + 1
            ha = {}
            a_rows(qa, a, range(nr), MODE_F, ha)
        for p in range(NCH):
            f_gu(st, p)
            while groups and groups[0][-1] + DLAG <= p:
                f_d(st, groups.pop(0))
            if ja is not None:
                if p == LNA_AT:
                    a_ln1f(b, 0, ha[('h', LND[0])] if LND[0] >= 0 else None)
                if p == LNB_AT:
                    a_ln1f((a + 2) % NB, 1, ha[('h', LND[1])] if LND[1] >= 0 else None)
                    a_qsops()
                if p == WOA_AT:
                    a_wo(qa, a, 0, LN_F)
                if p == QB_AT:
                    a_qkv2_halo(qb, qa)
                    for t0, nt in ((0, 2), (2, 2), (4, 2), (6, 1)):
                        a_qkv2(qb, qa, t0, nt)
                    a_rows(qb, b, range(nr), MODE_F, {})
                if p == WOB_AT:
                    a_wo(qb, b, 1, LN_F)
        if ja is not None:
            a_sops(ja % NSLOT)
        while groups:
            f_d(st, groups.pop(0))
        f_store(st)

    def run_aa(j):
        a = 2 * j
        b = a + 1
        pieces = []
        for k in range(CP):
            pieces += prep_pieces(plan_s[j * CP + k])
        cb = Pacer(pieces, pace_pw, 28 * NPACE, NPACE)
        a_rows(qa, a, range(nr), MODE_A, {})
        a_wo(qb, jnp.where(j == 0, NB, a - 1), 1, LN_A)
        a_sops(jnp.where(j == 0, NSLOT, j - 1))
        a_ln1(a + 2, xn1a, True)
        a_qkv(xn1b, qb, qa, cb=cb)
        a_rows(qb, b, range(nr), MODE_A, {})
        a_wo(qa, a, 0, LN_A)
        a_ln1(b + 2, xn1b, True)
        a_qkv(xn1a, qa, qb, cb=cb)
        assert cb.done == len(pieces)

    def start_rest():
        cp_wo().start()
        cp_x(1).start()
        cp_x(2).start()
        for c in range(NCH):
            for cp in chunk_copies(c):
                cp.start()
            if c == 3:
                cp_x(3).start()
            if c == 9:
                cp_x(4).start()

    def qkv_section(sec):
        for cp in cp_qkv(sec):
            cp.wait()
        if sec == RESTAT:
            start_rest()
        for j in range(*QSEC[sec]):
            wd_ = min(128, 3 * D - j * 128)
            blk = wqkv_raw[:, j * 128:j * 128 + wd_].astype(f32)
            if wd_ < 128:
                blk = jnp.concatenate([blk, jnp.zeros((D, 128 - wd_), f32)], axis=1)
            bt = jnp.concatenate([blk, blk[2 * KH:]], axis=0).T
            for t in range(5):
                tmp[t, pl.ds(j * 128, 128), :] = bt[:, t * 128:(t + 1) * 128]
        for d in range(DH):
            r = _dst_row(sec, d)
            for t in range(5):
                wqkvT[pl.ds(r // 2, 16), t * 128:(t + 1) * 128] = _pk2(
                    tmp[t, pl.ds(sec * D + d, 16, stride=2 * DH), :],
                    tmp[t, pl.ds(sec * D + d + DH, 16, stride=2 * DH), :])

    @pl.when(g == 0)
    def _():
        cp_x(0).start()
        for sec in range(3):
            for cp in cp_qkv(sec):
                cp.start()
        if RESTAT < 0:
            start_rest()
        for j in range(KPAIR):
            for k in range(CP):
                plan_s[j * CP + k] = plan[j][k]
        qb[:, pl.ds(TB, HALO), :] = jnp.zeros((20, HALO, 128), f32)
        wqkvT[pl.ds((13 * 128 + 64) // 2, 32), :] = jnp.zeros((32, KP), u32)
        zpad = jnp.zeros((KP - D, 128), f32)
        cp_x(0).wait()
        a_ln1(0, xn1a, True)
        a_ln1(1, xn1b, True)
        qkv_section(0)
        a_qkv(xn1a, qa, qb, 0, 4)
        qkv_section(1)
        a_qkv(xn1a, qa, qb, 4, 8)
        qkv_section(2)
        cp_wo().wait()
        cb = Pacer(q_prep_pieces(), pace_wq, 6 * NPACE)
        a_qkv(xn1a, qa, qb, 8, 14, cb=cb)
        for t in range(5):
            wd_ = 128 if t < 4 else 64
            blk = wo_raw[:, t * 128:t * 128 + wd_].astype(f32)
            if wd_ < 128:
                blk = jnp.concatenate([blk, jnp.zeros((D, 128 - wd_), f32)], axis=1)
            tmp[t, pl.ds(0, D), :] = blk
        for t in range(5):
            rows = [tmp[t, pl.ds(d, 32, stride=DH), :] for d in range(DH)]
            full = jnp.concatenate(rows[:16] + [zpad] + rows[16:], axis=0)
            ft = full.T
            n = 128 if t < 4 else 64
            woT[pl.ds(t * 64, n // 2), :] = _pk(ft[:n])
        cp_x(1).wait()

    for j in range(1, KPAIR):
        @pl.when(g == 1 + j)
        def _():
            if j % 2 == 1:
                cp_x(2 + j // 2).wait()
            for c in plan[j]:
                if c < NCH:
                    for cp in chunk_copies(c):
                        cp.wait()

    @pl.when(jnp.logical_and(g >= 1, g <= KPAIR))
    def _():
        run_aa(g - 1)

    @pl.when(g == KPAIR + 1)
    def _():
        pieces = []
        for c in range(nprepped, NCH):
            for cp in chunk_copies(c):
                cp.wait()
            pieces += prep_pieces(c)
        n1 = int(len(pieces) * TAILF)
        cb = Pacer(pieces[:n1], pace_pwz, D // 16)
        a_wo(qb, K - 1, 1, (4, 0), cb=cb)

        cb2 = Pacer(pieces[n1:], pace_pwz, 8)

        def put(i, v):
            s_scr[KPAIR - 1, i] = v
            cb2(pltpu.bitcast(v[0:8, 0:128], f32))
        sops(xn_f, put)
        for blk in range(K + 2, NB):
            x_convert(blk)

    jf = g - (KPAIR + 1)

    @pl.when(jnp.logical_and(jf >= 0, jf < NB - KPAIR))
    def _():
        run_pair(jf, jf + KPAIR)

    @pl.when(jf >= NB - KPAIR)
    def _():
        def body(hf, carry):
            st = St()
            f_init(st, jf)
            st.c0 = hf * NPC
            groups = []
            p0 = 0
            for n in DGROUPS_F:
                groups.append(list(range(p0, p0 + n)))
                p0 += n
            for p in range(NPC):
                f_gu(st, p)
                while groups and groups[0][-1] + DLAG <= p:
                    f_d(st, groups.pop(0))
            while groups:
                f_d(st, groups.pop(0))
            f_store(st)
            return carry
        lax.fori_loop(0, NH, body, 0)


@jax.jit
def pallas_interleave_layers__sliding_local_dilated__glu_gated_geglu__prompt_kernel(
    A_x, A_wqkv, A_wo, B_x, B_w_gate, B_w_up, B_w_down):
    B, S, D = A_x.shape
    DF = B_w_gate.shape[1]
    NB = S // TB
    xT = A_x.reshape(S, D).T
    wdT = B_w_down.T
    NCH = DF // (2 * TC)
    nsteps = 1 + KPAIR + NB
    hbm = pl.BlockSpec(memory_space=pltpu.HBM)
    outT = pl.pallas_call(
        functools.partial(_kernel, D=D, DF=DF, NB=NB),
        grid=(nsteps,),
        in_specs=[hbm] * 6,
        out_specs=pl.BlockSpec((D, TM), lambda g: (0, jnp.maximum(g - (1 + KPAIR + NB // 2), 0))),
        out_shape=jax.ShapeDtypeStruct((D, S), A_x.dtype),
        scratch_shapes=[
            pltpu.VMEM((D, S), bf16),
            pltpu.VMEM((D, 3 * D), bf16),
            pltpu.VMEM((D, D), bf16),
            pltpu.VMEM((NQKV // 2, KP), u32),
            pltpu.VMEM((D // 2, KP), u32),
            pltpu.VMEM((NCH + 1, 3, D, 2 * TC), bf16),
            pltpu.VMEM((NCH + 1, 8 * (KH // 2) + D + 16, 2 * TC), u32),
            pltpu.VMEM((5, NQKV, 128), f32),
            pltpu.VMEM((20, HALO + TB, 128), f32),
            pltpu.VMEM((20, HALO + TB, 128), f32),
            pltpu.VMEM((NB + 1, D, TB), f32),
            pltpu.VMEM((2, D, TB), f32),
            pltpu.VMEM((TB // 2, KP), u32),
            pltpu.VMEM((TB // 2, KP), u32),
            pltpu.VMEM((NSLOT + 1, 8, TB // 2, KH), u32),
            pltpu.VMEM((NQKV // 4 + 32, 17 * 128), u32),
            pltpu.VMEM((2, D, TB), f32),
            pltpu.VMEM((8, TB // 2, KH), u32),
            pltpu.SMEM((KPAIR * CP + 1,), jnp.int32),
            pltpu.SemaphoreType.DMA((9 + NCH,)),
        ],
        compiler_params=pltpu.CompilerParams(
            dimension_semantics=("arbitrary",),
            vmem_limit_bytes=110 * 1024 * 1024,
        ),
    )(xT, A_wqkv, A_wo, B_w_gate, B_w_up, wdT)
    return outT.T.reshape(B, S, D)
```

```python
import functools
import math
import jax
import jax.numpy as jnp
from jax import lax
import jax.experimental.pallas as pl
import jax.experimental.pallas.tpu as pltpu

H = 32
DH = 18
W = 8
DIL = 2
HALO = 16
EPS = 1e-5
TB = 128
TM = 256
NH = 2
RB = 8
KP = 640
KH = 256
KX = 192
KY = 64
NQKV = 14 * 128
TC = 128
NSLOT = 8
DG = int(3)
ROWS_LO = int(0)
WO_AT = int(6)
DLAG = int(1)
LN1_AT = int(7)
SERIAL = int(1)
SERIAL_A = int(0)
LN_F = tuple(int(x) for x in '1,4'.split(','))
LN_A = tuple(int(x) for x in '2,8'.split(','))
KPAIR = int(6)
CP = int(3)
QSPLIT = int(5)
XFIRST = 512
DGROUPS = tuple(int(x) for x in '6,6,3,3'.split(','))
DGROUPS_F = tuple(int(x) for x in '3,3,3'.split(','))
DORD = tuple(int(x) for x in '0,1,2,3,6,7,8,9,12,14,13,10,11,4,5'.split(','))
QB_AT = int(7); WOA_AT = int(8)
LNA_AT = int(1); LNB_AT = int(3); WOB_AT = int(14)
QPR = 16
RBD = int(1)
DKEEP = int(2)
RESTAT = int(0)
TAILF = float(0.6)
LND = tuple(int(x) for x in '3,8'.split(','))
WOSPLIT = int(1)
NPACE = int(4)
MODE_F = tuple(int(x) for x in '0,1,0,2,1'.split(','))
MODE_A = tuple(int(x) for x in '1,3,1,0,0'.split(','))
FENCE = int(1)
PR = 32
PW1 = float(1); PW2 = float(1); PW3 = float(1)
SOPS_EARLY = int(1)
CLIP = int(0)

f32 = jnp.float32
bf16 = jnp.bfloat16
u32 = jnp.uint32
NT = (((1,), (1,)), ((), ()))


def _pk(x):
    return pltpu.bitcast(x.astype(bf16), u32)


def _unpk(u, idx):
    return pltpu.unpack_elementwise(u, index=idx, packed_dtype=bf16, unpacked_dtype=f32)


def _pk2(even, odd):
    return pltpu.pack_elementwise([even, odd], packed_dtype=bf16).astype(u32)


def _up(x):
    return pltpu.bitcast(x, bf16)


def _dot(a, b):
    return jnp.dot(a, b, preferred_element_type=f32)


def _dot_nt(a, b):
    return lax.dot_general(a, b, NT, preferred_element_type=f32)


def _ln_stats(x, NACC, pin=None):
    n = x.shape[0]
    c = x[0:1] if pin is None else pin(x[0:8])[0:1]
    s1 = [None] * NACC
    s2 = [None] * NACC
    for i in range(n // 8):
        d = x[i * 8:(i + 1) * 8] - c
        k = i % NACC
        s1[k] = d if s1[k] is None else s1[k] + d
        dd = d * d
        s2[k] = dd if s2[k] is None else s2[k] + dd
    while len(s1) > 1:
        s1 = [s1[i] + s1[i + 1] for i in range(0, len(s1), 2)]
        s2 = [s2[i] + s2[i + 1] for i in range(0, len(s2), 2)]
    m = jnp.sum(s1[0], axis=0, keepdims=True) * (1.0 / n)
    v = jnp.sum(s2[0], axis=0, keepdims=True) * (1.0 / n) - m * m
    v = jnp.maximum(v, 0.0)
    return c + m, lax.rsqrt(v + EPS)


def _tree(fn, xs):
    xs = list(xs)
    while len(xs) > 1:
        xs = [fn(xs[i], xs[i + 1]) for i in range(0, len(xs) - 1, 2)] + ([xs[-1]] if len(xs) % 2 else [])
    return xs[0]


def _lhs_ops(a11, a12, a21, a22):
    return (a11 + a22, a21 + a22, a11, a22, a11 + a12, a21 - a11, a12 - a22)


def _rhs_ops(b11, b12, b21, b22):
    return (b11 + b22, b11, b12 - b22, b21 - b11, b22, b11 + b12, b21 + b22)


_D_LHS = (
    ((0, 0, 1), (0, 2, -1), (1, 0, -1)), ((0, 0, 1), (0, 1, -1), (2, 0, -1)), ((1, 1, 1), (0, 1, -1), (1, 2, -1)),
    ((1, 1, 1), (1, 0, -1), (2, 1, -1)), ((2, 2, 1), (0, 2, -1), (2, 1, -1)), ((2, 2, 1), (1, 2, -1), (2, 0, -1)),
    ((0, 1, 1),), ((0, 1, 1), (1, 0, -1)), ((1, 0, 1),),
    ((0, 2, 1),), ((0, 2, 1), (2, 0, -1)), ((2, 0, 1),),
    ((1, 2, 1),), ((2, 1, 1), (1, 2, -1)), ((2, 1, 1),),
)
_D_OUT = {
    (0, 0): ((0, 1), (7, 1), (8, 1), (9, 1), (6, -1)),
    (0, 1): ((1, 1), (6, 1), (10, 1), (11, 1), (9, -1)),
    (1, 0): ((2, 1), (7, 1), (8, 1), (12, 1), (6, -1)),
    (1, 1): ((3, 1), (6, 1), (13, 1), (14, 1), (2, -1), (7, -1)),
    (2, 0): ((5, 1), (9, 1), (12, 1), (13, 1), (4, -1), (10, -1)),
    (2, 1): ((4, 1), (10, 1), (11, 1), (14, 1), (9, -1)),
}


def _d_rhs(b):
    s1 = b[1][0] + b[1][1]
    s2 = b[2][0] + b[2][1]
    t7 = b[0][1] + s1
    t10 = b[0][0] + s2
    return (b[0][0], b[0][1], b[1][0], s1, b[2][1], s2, b[0][1] + b[1][1], t7, b[0][0] + t7,
            b[0][0] + b[2][0], t10, b[0][1] + t10, b[1][0] + b[2][0], b[1][0] - b[2][1], b[1][1] + b[2][1])


def _signed_sum(terms):
    acc = None
    for v, sg in terms:
        if acc is None:
            assert sg == 1
            acc = v
        else:
            acc = acc + v if sg == 1 else acc - v
    return acc


def _dst_row(sec, d):
    if sec == 0:
        return d * 32 if d < 16 else 1024 + (d - 16) * 32
    if sec == 1:
        return 512 + d * 32 if d < 16 else 13 * 128 + (d - 16) * 32
    return 9 * 128 + d * 32 if d < 16 else 1024 + 64 + (d - 16) * 32


def _prep_plan(nchunk):
    plan = [[nchunk] * CP]
    nxt = 0
    for j in range(1, KPAIR):
        left_steps = KPAIR - 1 - j
        n = min(CP, nchunk - nxt)
        if j == 1:
            n = max(0, min(n, max(CP - 1, nchunk - nxt - left_steps * CP)))
        ids = list(range(nxt, nxt + n))
        nxt += n
        plan.append(ids + [nchunk] * (CP - n))
    return plan, nxt


def _kernel(x_hbm, wqkv_hbm, wo_hbm, wg_hbm, wu_hbm, wd_hbm, o_ref,
            xin, wqkv_raw, wo_raw, wqkvT, woT, raw, pw, tmp, qa, qb, xres, xn_f, xn1a, xn1b,
            s_scr, wq_s, xn_g, sq_scr, plan_s, sems, *, D, DF, NB):
    g = pl.program_id(0)
    FH = DF // NH
    NPC = FH // (2 * TC)
    NCH = NH * NPC
    NG = NPC // DG
    DHALF = D // 2
    K = 2 * KPAIR
    S = NB * TB
    plan, nprepped = _prep_plan(NCH)
    zero8 = pl.multiple_of((g >> 20) * 8, 8)

    QSEC = ((0, 5), (5, 9), (9, 14))
    XPC = ((0, 256), (256, 512), (512, 1024), (1024, 1536), (1536, S))

    def cp_qkv(sec):
        out = []
        for j in range(*QSEC[sec]):
            n = min(128, 3 * D - j * 128)
            out.append(pltpu.make_async_copy(wqkv_hbm.at[:, pl.ds(j * 128, n)], wqkv_raw.at[:, pl.ds(j * 128, n)],
                                             sems.at[sec]))
        return out

    def cp_wo():
        return pltpu.make_async_copy(wo_hbm, wo_raw, sems.at[3])

    def cp_x(k):
        lo, hi = XPC[k]
        return pltpu.make_async_copy(x_hbm.at[:, pl.ds(lo, hi - lo)], xin.at[:, pl.ds(lo, hi - lo)], sems.at[4 + k])

    def chunk_copies(c):
        return [pltpu.make_async_copy(w.at[:, pl.ds(c * 2 * TC, 2 * TC)], raw.at[c, m], sems.at[9 + c])
                for m, w in enumerate((wg_hbm, wu_hbm, wd_hbm))]

    R_SD = 8 * (KH // 2)
    D3 = D // 3
    R_END = R_SD + 5 * (D3 // 2)

    def prep_pieces(c):
        def ld(m, r0, nr, col):
            u = pltpu.bitcast(raw[c, m, pl.ds(r0, nr), pl.ds(col, TC)], u32)
            return u, _unpk(u, 0), _unpk(u, 1)

        def ops(fn, blocks):
            ev = fn(*[b[1] for b in blocks])
            od = fn(*[b[2] for b in blocks])
            out = []
            for e, o in zip(ev, od):
                src = [b[0] for b in blocks if b[1] is e]
                out.append(src[0] if src else _pk2(e, o))
            return out

        def put(m, slot, row, t):
            pw[c, pl.ds((slot * KH + row) // 2, t.shape[0]), m * TC:(m + 1) * TC] = t

        def gu_piece(m, r):
            x1, x2, y1, y2 = ld(m, r, PR, 0), ld(m, r, PR, TC), ld(m, KH + r, PR, 0), ld(m, KH + r, PR, TC)

            def add(u, v):
                return _pk2(u[1] + v[1], u[2] + v[2])

            def sub(u, v):
                return _pk2(u[1] - v[1], u[2] - v[2])
            put(m, 1, r, sub(x2, y2))
            put(m, 2, r, sub(y1, x1))
            if r < KX:
                put(m, 0, r, x1[0])
                put(m, 3, r, y2[0])
                put(m, 4, r, add(y1, y2))
                put(m, 5, r, add(x1, x2))
                put(m, 7, r, add(x1, y2))
            else:
                put(m, 0, r, x2[0])
                put(m, 3, r, y1[0])
                put(m, 6, KY + r - KX, add(y1, y2))
                put(m, 6, 3 * KY + r - KX, add(x1, x2))
                put(m, 7, r, add(x2, y1))

        def wr_piece(m):
            r1 = ld(m, 2 * KH, KY, 0)[0]
            r2 = ld(m, 2 * KH, KY, TC)[0]
            put(m, 4, KX, r1)
            put(m, 6, 2 * KY, r1)
            put(m, 5, KX, r2)
            put(m, 6, 0, r2)

        out = []
        for m in range(2):
            out += [functools.partial(gu_piece, m, r) for r in range(0, KH, PR)]
            out.append(functools.partial(wr_piece, m))
        return out

    def prep_group(cs):
        def d_piece(r, lt):
            blk = {}
            for i in range(3):
                for j in range(3):
                    u = pltpu.bitcast(raw[cs[j], 2, pl.ds(i * D3 + r, 16), pl.ds(lt * TC, TC)], u32)
                    blk[i, j] = (u, _unpk(u, 0), _unpk(u, 1))
            for k, terms in enumerate(_D_LHS):
                if len(terms) == 1:
                    t = blk[terms[0][:2]][0]
                else:
                    t = _pk2(_signed_sum([(blk[i, j][1], sg) for i, j, sg in terms]),
                             _signed_sum([(blk[i, j][2], sg) for i, j, sg in terms]))
                pw[cs[k // 5], pl.ds(R_SD + (k % 5) * (D3 // 2) + r // 2, 8), lt * TC:(lt + 1) * TC] = t
        out = []
        for c in cs:
            out += prep_pieces(c)
        out += [functools.partial(d_piece, r, lt) for r in range(0, D3, 16) for lt in range(2)]
        return out

    class Pacer:
        def __init__(self, pieces, pace, npts, idle=0):
            self.pieces, self.pace, self.n, self.pt, self.done = pieces, pace, npts - idle, 0, 0

        def __call__(self, v):
            self.pt += 1
            upto = min(len(self.pieces), int(round(len(self.pieces) * self.pt / self.n)))
            if upto > self.done or self.pt == self.n + 1:
                self.pace(v)
            for piece in self.pieces[self.done:upto]:
                piece()
            self.done = upto

    def pace_wq(v):
        wq_s[pl.ds(NQKV // 4 + zero8, 8), 0:128] = pltpu.bitcast(v, u32)

    def pace_pwz(v):
        pw[NCH, pl.ds(R_END + zero8, 8), 0:128] = pltpu.bitcast(v, u32)

    def pace_pw(v):
        pw[NCH, pl.ds(R_END, 8), 0:128] = pltpu.bitcast(v, u32)

    nr = TB // RB
    QT = (0, 1, 2, 3, 8)
    KT = (4, 5, 6, 7, 13)
    VT = (9, 10, 11, 12, 8)
    scale = DH ** -0.5
    c2e = scale * math.log2(math.e)
    neg = -1e9 * math.log2(math.e)
    k0 = math.sqrt(2.0 / math.pi)
    k1 = k0 * 0.044715

    zvec = jnp.full((RB, 128), (g >> 20).astype(u32), u32)

    def tie(x, dep):
        return pltpu.bitcast(pltpu.bitcast(x, u32) | (pltpu.bitcast(dep, u32) & zvec), f32)

    def normalize(blk, mean, rstd, link):
        if not link:
            return (xres[blk] - mean) * rstd
        rs = jnp.broadcast_to(rstd, (8, TB))
        mb = jnp.broadcast_to(mean, (8, TB))
        outs = []
        for i in range(D // 8):
            if i and i % link == 0:
                rs = tie(rs, outs[-1])
            outs.append((xres[blk, pl.ds(i * 8, 8), :] - mb) * rs)
        return jnp.concatenate(outs, axis=0)

    def x_convert(blk):
        x = xin[:, pl.ds(pl.multiple_of(blk * TB, TB), TB)].astype(f32)
        xres[blk] = x
        return x

    def a_ln1(blk, dst, from_input):
        x = x_convert(blk) if from_input else xres[blk]
        mean, rstd = _ln_stats(x, LN_A[0])
        if not from_input:
            dst[pl.ds(0, 8), :] = jnp.zeros((8, KP), u32)
        xn = (xres[blk] - mean) * rstd
        xp = jnp.concatenate([xn, jnp.zeros((KP - D, TB), f32)], axis=0)
        dst[...] = pltpu.bitcast(xp.astype(bf16).T, u32)

    def a_qkv(src, qdst, qprev, t0=0, t1=14, cb=None):
        qkv = _dot_nt(_up(src[...]), _up(wqkvT[pl.ds(t0 * 64, (t1 - t0) * 64), :]))
        for t in range(max(t0, 4), t1):
            qdst[t, pl.ds(0, HALO), :] = qprev[t, pl.ds(TB, HALO), :]
        for t in range(t0, t1):
            qdst[t, pl.ds(HALO, TB), :] = qkv[:, (t - t0) * 128:(t - t0 + 1) * 128]
            if cb is not None:
                for k in range(NPACE):
                    rr = k * (TB // NPACE)
                    cb(qkv[rr:rr + 8, (t - t0) * 128:(t - t0 + 1) * 128])

    cbits = pltpu.bitcast(jnp.full((RB, 128), c2e, f32), u32)

    def tied_scale(deps):
        if not deps:
            return c2e
        acc = pltpu.bitcast(deps[0], u32)
        for dv in deps[1:]:
            acc = acc | pltpu.bitcast(dv, u32)
        return pltpu.bitcast(cbits | (acc & zvec), f32)

    def a_rows(q_s, blk, rs, mode, hist, start=None):
        lag_mid, lag_end, midkind, fw, fv = mode
        for r in rs:
            r0 = r * RB
            deps = [start] if (start is not None and r == 0) else []
            if lag_mid and r - lag_mid >= 0:
                deps.append(hist[('h' if midkind else 'm', r - lag_mid)])
            if lag_end and r - lag_end >= 0:
                deps += hist[('o', r - lag_end)]
            cs = tied_scale(deps)
            q = [q_s[t, pl.ds(HALO + r0, RB), :] * cs for t in QT]
            sc = []
            q0 = q[0]
            prev = None
            for w in range(W):
                off = HALO + r0 - DIL * w
                acc = None
                if fw and w and w % fw == 0:
                    q0 = tie(q[0], prev)
                for j, t in enumerate(KT):
                    p = (q0 if j == 0 else q[j]) * q_s[t, pl.ds(off, RB), :]
                    acc = p if acc is None else acc + p
                prev = acc
                acc = acc + pltpu.roll(acc, 64, 1)
                hist[('h', r)] = acc
                acc = acc + pltpu.roll(acc, 32, 1)
                if r0 - DIL * w < 0:
                    pos = blk * TB + r0 + lax.broadcasted_iota(jnp.int32, (RB, 128), 0)
                    acc = jnp.where(pos >= DIL * w, acc, neg)
                sc.append(acc)
            m = _tree(jnp.maximum, sc)
            hist[('m', r)] = m
            e = [jnp.exp2(sc[w] - m) for w in range(W)]
            l = _tree(jnp.add, e)
            rinv = pl.reciprocal(l, approx=True)
            rinv = rinv * (2.0 - l * rinv)
            outs = []
            e0 = e[0]
            for j, t in enumerate(VT):
                if fv and j and j % fv == 0:
                    e0 = tie(e[0], acc)
                acc = None
                for w in range(W):
                    off = HALO + r0 - DIL * w
                    p = (e0 if w == 0 else e[w]) * q_s[t, pl.ds(off, RB), :]
                    acc = p if acc is None else acc + p
                o = acc * rinv
                st_off = r0 + zero8 if (j == 4 and r == nr - 1 and FENCE) else r0
                q_s[14 + j, pl.ds(st_off, RB), :] = o
                outs.append(o)
            hist[('o', r)] = outs[-1:] if fv == 1 else outs

    def a_wo(q_s, blk, par, ln, cb=None):
        if WOSPLIT:
            o4 = q_s[18, pl.ds(0, TB), :].astype(bf16)
            rq = D // 8
            y = jnp.concatenate([_dot_nt(_up(woT[pl.ds(k * rq, rq), 512:640]), o4) for k in range(4)], axis=0)
            o = jnp.concatenate([q_s[14 + j, pl.ds(0, TB), :] for j in range(4)], axis=1).astype(bf16)
            x1 = _dot_nt(_up(woT[:, 0:512]), o) + (xres[blk] + y)
        else:
            o = jnp.concatenate([q_s[14 + j, pl.ds(0, TB), :] for j in range(5)], axis=1).astype(bf16)
            x1 = xres[blk] + _dot_nt(_up(woT[...]), o)
        xres[blk] = x1
        if cb is not None:
            for i in range(0, D, 16):
                cb(x1[i:i + 8])
        mean, rstd = _ln_stats(x1, ln[0])
        xn_f[par] = normalize(blk, mean, rstd, ln[1])

    def sops(src, put):
        def seg(tb, r0, n):
            return lambda: src[tb, pl.ds(r0, n), :]
        A11, A12, A21, A22 = seg(0, 0, KX), seg(0, KH, KX), seg(1, 0, KX), seg(1, KH, KX)
        a11, a12, a21, a22 = seg(0, KX, KY), seg(0, KH + KX, KY), seg(1, KX, KY), seg(1, KH + KX, KY)
        rt, rb = seg(0, 2 * KH, KY), seg(1, 2 * KH, KY)
        parts = (
            lambda: (A21() + A22(), -(a21() + a22())),
            lambda: (A11(), -a22()),
            lambda: (A22(), -a11()),
            lambda: (A11() + A12(), -(a11() + a12())),
            lambda: (A12() - A22(), rt()),
            lambda: (A21() - A11(), rb()),
            lambda: (rt(), a12() - a22(), rb(), a21() - a11()),
            lambda: (A11() + A22(), a11() + a22()),
        )
        for i, fn in enumerate(parts):
            t = jnp.concatenate(fn(), axis=0)
            put(i, pltpu.bitcast(t.astype(bf16).T, u32))

    def a_sops(slot):
        def put(i, v):
            s_scr[slot, i] = v
        sops(xn_f, put)

    NQH = NQKV // 4

    def q_prep_pieces():
        lo = lax.broadcasted_iota(jnp.int32, (QPR, 128), 1) < 64

        def piece(r):
            def ld(half, t):
                u = wqkvT[pl.ds(half * NQH + r, QPR), t * 128:(t + 1) * 128]
                return u, _unpk(u, 0), _unpk(u, 1)

            def add(u, v):
                return _pk2(u[1] + v[1], u[2] + v[2])

            def sub(u, v):
                return _pk2(u[1] - v[1], u[2] - v[2])

            def put(tile, v):
                wq_s[pl.ds(r, QPR), tile * 128:(tile + 1) * 128] = v
            r1, r2 = wqkvT[pl.ds(r, QPR), 512:640], wqkvT[pl.ds(NQH + r, QPR), 512:640]
            zero = jnp.zeros((QPR, 128), u32)
            for t in range(2):
                x1, x2, y1, y2 = ld(0, t), ld(1, t), ld(0, 2 + t), ld(1, 2 + t)
                put(2 + t, sub(x2, y2))
                put(4 + t, sub(y1, x1))
                sy, sx, d1 = add(y1, y2), add(x1, x2), add(x1, y2)
                if t == 0:
                    put(0, x1[0])
                    put(6, y2[0])
                    put(8, sy)
                    put(10, sx)
                    put(14, d1)
                else:
                    put(1, jnp.where(lo, x1[0], x2[0]))
                    put(7, jnp.where(lo, y2[0], y1[0]))
                    put(9, jnp.where(lo, sy, r1))
                    put(11, jnp.where(lo, sx, r2))
                    put(12, jnp.where(lo, r2, sy))
                    put(13, jnp.where(lo, r1, sx))
                    put(15, jnp.where(lo, d1, zero))
                    put(16, jnp.where(lo, zero, add(x2, y1)))
        return [functools.partial(piece, r) for r in range(0, NQH, QPR)]

    def a_ln1f(blk, par, dep=None):
        mean, rstd = _ln_stats(xres[blk], LN_F[0], None if dep is None else (lambda v: tie(v, dep)))
        xn_g[par, pl.ds(0, 8), :] = jnp.zeros((8, TB), f32)
        xn_g[par] = normalize(blk, mean, rstd, LN_F[1])

    def a_qsops():
        def put(i, v):
            sq_scr[i, pl.ds(zero8, TB // 2), :] = v
        sops(xn_g, put)

    def a_qkv2_halo(qtop, qbot):
        for t in range(4, 14):
            qtop[t, pl.ds(0, HALO), :] = qbot[t, pl.ds(TB, HALO), :]

    def a_qkv2(qtop, qbot, t0, nt):
        def Q(slot, l0, l1, w0):
            lhs = _up(sq_scr[slot, :, l0:l1])
            rhs = _up(wq_s[pl.ds(t0 * 64, nt * 64), w0 * 128:w0 * 128 + (l1 - l0)])
            return _dot_nt(lhs, rhs)

        def out(dst, tb, v):
            for k in range(nt):
                dst[tb + k, pl.ds(HALO, TB), :] = v[:, k * 128:(k + 1) * 128]
                if dst is qtop and tb + k >= 4:
                    qbot[tb + k, pl.ds(0, HALO), :] = v[TB - HALO:, k * 128:(k + 1) * 128]
        q5 = Q(3, 0, KH, 6)
        q3 = Q(1, 0, KH, 2)
        q1b = Q(7, 128, KH, 16)
        out(qtop, t0 + 7, q3 + q5 + q1b + Q(6, 0, 128, 12))
        q4 = Q(2, 0, KH, 4)
        q2 = Q(0, 0, KH, 0)
        out(qbot, t0, q2 + q4 + q1b + Q(6, 128, KH, 13))
        q1 = Q(7, 0, KH, 14)
        out(qtop, t0, q1 + q4 - q5 + Q(4, 0, KH, 8))
        out(qbot, t0 + 7, q1 - q2 + q3 + Q(5, 0, KH, 10))

    class St:
        pass

    def f_init(st, j):
        st.c0 = 0
        st.b0 = (j * NH) % NB
        st.sb = j % NSLOT
        st.acc = [None] * 15
        st.t = {}

    def gelu_mul(c):
        gg = c[:, :TC]
        u = c[:, TC:]
        t = jnp.tanh(gg * (k0 + k1 * (gg * gg)))
        gu = gg * u
        return gu + gu * t

    def f_gu(st, p):
        c = st.c0 + p

        def Q(slot, k0_=0, k1_=KH):
            if k0_ % 128 == 0 and k1_ % 128 == 0:
                lhs = _up(s_scr[st.sb, slot, :, k0_:k1_])
            else:
                lhs = _up(s_scr[st.sb, slot])[:, k0_:k1_]
            return _dot(lhs, _up(pw[c, pl.ds((slot * KH + k0_) // 2, (k1_ - k0_) // 2), :]))
        q5 = Q(3)
        q3 = Q(1)
        q1b = Q(7, KX, KH)
        h12 = gelu_mul(q3 + q5 + q1b + Q(6, 0, 2 * KY))
        st.first = q3[0:8, 0:128]
        q4 = Q(2)
        q2 = Q(0)
        h21 = gelu_mul(q2 + q4 + q1b + Q(6, 2 * KY, KH))
        q1 = Q(7, 0, KX)
        h11 = gelu_mul(q1 + q4 - q5 + Q(4))
        h22 = gelu_mul(q1 - q2 + q3 + Q(5))
        st.t[p] = (jnp.concatenate([h11, h12], axis=1), jnp.concatenate([h21, h22], axis=1))

    def f_d(st, ps):
        sgs = [ps[k:k + 3] for k in range(0, len(ps), 3)]
        rhs = [_d_rhs([st.t.pop(p) for p in sg]) for sg in sgs]
        for i in DORD:
            a = jnp.concatenate([_up(pw[st.c0 + sg[i // 5], pl.ds(R_SD + (i % 5) * (D3 // 2), D3 // 2), :])
                                 for sg in sgs], axis=1)
            t = jnp.concatenate([r[i] for r in rhs], axis=1).astype(bf16)
            r = _dot_nt(a, t)
            st.acc[i] = r if st.acc[i] is None else r + st.acc[i]

    def f_store(st):
        for k in range(NH):
            y = jnp.concatenate([_signed_sum([(st.acc[n], sg) for n, sg in _D_OUT[i, k]]) for i in range(3)], axis=0)
            x2 = xres[st.b0 + k] + 0.5 * y
            xres[st.b0 + k] = x2
            o_ref[:, k * TB:(k + 1) * TB] = x2.astype(o_ref.dtype)

    def run_pair(jf, ja):
        st = St()
        f_init(st, jf)
        groups = []
        p0 = 0
        for n in DGROUPS:
            groups.append(list(range(p0, p0 + n)))
            p0 += n
        assert p0 == NCH
        if ja is not None:
            a = (2 * ja) % NB
            b = a + 1
            ha = {}
            a_rows(qa, a, range(nr), MODE_F, ha)
        for p in range(NCH):
            f_gu(st, p)
            while groups and len(groups) > DKEEP and groups[0][-1] + DLAG <= p:
                f_d(st, groups.pop(0))
            if ja is not None:
                if p == LNA_AT:
                    a_ln1f(b, 0, ha[('h', LND[0])] if LND[0] >= 0 else None)
                if p == LNB_AT:
                    a_ln1f((a + 2) % NB, 1, ha[('h', LND[1])] if LND[1] >= 0 else None)
                    a_qsops()
                if p == WOA_AT:
                    a_wo(qa, a, 0, LN_F)
                if p == QB_AT:
                    a_qkv2_halo(qb, qa)
                    for t0, nt in ((0, 2), (2, 2), (4, 2), (6, 1)):
                        a_qkv2(qb, qa, t0, nt)
                    if not RBD:
                        a_rows(qb, b, range(nr), MODE_F, {})
                if RBD and p == QB_AT + RBD:
                    a_rows(qb, b, range(nr), MODE_F, {}, st.first)
                if p == WOB_AT:
                    a_wo(qb, b, 1, LN_F)
        if ja is not None:
            a_sops(ja % NSLOT)
        while groups:
            f_d(st, groups.pop(0))
        f_store(st)

    def run_aa(j):
        a = 2 * j
        b = a + 1
        pieces = prep_group([plan_s[j * CP + k] for k in range(CP)])
        cb = Pacer(pieces, pace_pw, 28 * NPACE, NPACE)
        a_rows(qa, a, range(nr), MODE_A, {})
        a_wo(qb, jnp.where(j == 0, NB, a - 1), 1, LN_A)
        a_sops(jnp.where(j == 0, NSLOT, j - 1))
        a_ln1(a + 2, xn1a, True)
        a_qkv(xn1b, qb, qa, cb=cb)
        a_rows(qb, b, range(nr), MODE_A, {})
        a_wo(qa, a, 0, LN_A)
        a_ln1(b + 2, xn1b, True)
        a_qkv(xn1a, qa, qb, cb=cb)
        assert cb.done == len(pieces)

    def start_rest():
        cp_wo().start()
        cp_x(1).start()
        cp_x(2).start()
        for c in range(NCH):
            for cp in chunk_copies(c):
                cp.start()
            if c == 3:
                cp_x(3).start()
            if c == 9:
                cp_x(4).start()

    def qkv_section(sec):
        for cp in cp_qkv(sec):
            cp.wait()
        if sec == RESTAT:
            start_rest()
        for j in range(*QSEC[sec]):
            wd_ = min(128, 3 * D - j * 128)
            blk = wqkv_raw[:, j * 128:j * 128 + wd_].astype(f32)
            if wd_ < 128:
                blk = jnp.concatenate([blk, jnp.zeros((D, 128 - wd_), f32)], axis=1)
            bt = jnp.concatenate([blk, blk[2 * KH:]], axis=0).T
            for t in range(5):
                tmp[t, pl.ds(j * 128, 128), :] = bt[:, t * 128:(t + 1) * 128]
        for d in range(DH):
            r = _dst_row(sec, d)
            for t in range(5):
                wqkvT[pl.ds(r // 2, 16), t * 128:(t + 1) * 128] = _pk2(
                    tmp[t, pl.ds(sec * D + d, 16, stride=2 * DH), :],
                    tmp[t, pl.ds(sec * D + d + DH, 16, stride=2 * DH), :])

    @pl.when(g == 0)
    def _():
        cp_x(0).start()
        for sec in range(3):
            for cp in cp_qkv(sec):
                cp.start()
        if RESTAT < 0:
            start_rest()
        for j in range(KPAIR):
            for k in range(CP):
                plan_s[j * CP + k] = plan[j][k]
        qb[:, pl.ds(TB, HALO), :] = jnp.zeros((20, HALO, 128), f32)
        wqkvT[pl.ds((13 * 128 + 64) // 2, 32), :] = jnp.zeros((32, KP), u32)
        zpad = jnp.zeros((KP - D, 128), f32)
        cp_x(0).wait()
        a_ln1(0, xn1a, True)
        a_ln1(1, xn1b, True)
        qkv_section(0)
        a_qkv(xn1a, qa, qb, 0, 4)
        qkv_section(1)
        a_qkv(xn1a, qa, qb, 4, 8)
        qkv_section(2)
        cp_wo().wait()
        cb = Pacer(q_prep_pieces(), pace_wq, 6 * NPACE)
        a_qkv(xn1a, qa, qb, 8, 14, cb=cb)
        for t in range(5):
            wd_ = 128 if t < 4 else 64
            blk = wo_raw[:, t * 128:t * 128 + wd_].astype(f32)
            if wd_ < 128:
                blk = jnp.concatenate([blk, jnp.zeros((D, 128 - wd_), f32)], axis=1)
            tmp[t, pl.ds(0, D), :] = blk
        for t in range(5):
            rows = [tmp[t, pl.ds(d, 32, stride=DH), :] for d in range(DH)]
            full = jnp.concatenate(rows[:16] + [zpad] + rows[16:], axis=0)
            ft = full.T
            n = 128 if t < 4 else 64
            woT[pl.ds(t * 64, n // 2), :] = _pk(ft[:n])
        cp_x(1).wait()

    for j in range(1, KPAIR):
        @pl.when(g == 1 + j)
        def _():
            if j % 2 == 1:
                cp_x(2 + j // 2).wait()
            for c in plan[j]:
                if c < NCH:
                    for cp in chunk_copies(c):
                        cp.wait()

    @pl.when(jnp.logical_and(g >= 1, g <= KPAIR))
    def _():
        run_aa(g - 1)

    @pl.when(g == KPAIR + 1)
    def _():
        pieces = []
        for c in range(nprepped, NCH):
            for cp in chunk_copies(c):
                cp.wait()
        for c in range(nprepped, NCH, 3):
            pieces += prep_group([c, c + 1, c + 2])
        n1 = int(len(pieces) * TAILF)
        cb = Pacer(pieces[:n1], pace_pwz, D // 16)
        a_wo(qb, K - 1, 1, (4, 0), cb=cb)

        cb2 = Pacer(pieces[n1:], pace_pwz, 8)

        def put(i, v):
            s_scr[KPAIR - 1, i] = v
            cb2(pltpu.bitcast(v[0:8, 0:128], f32))
        sops(xn_f, put)
        for blk in range(K + 2, NB):
            x_convert(blk)

    jf = g - (KPAIR + 1)

    @pl.when(jnp.logical_and(jf >= 0, jf < NB - KPAIR))
    def _():
        run_pair(jf, jf + KPAIR)

    @pl.when(jf >= NB - KPAIR)
    def _():
        def body(hf, carry):
            st = St()
            f_init(st, jf)
            st.c0 = hf * NPC
            groups = []
            p0 = 0
            for n in DGROUPS_F:
                groups.append(list(range(p0, p0 + n)))
                p0 += n
            for p in range(NPC):
                f_gu(st, p)
                while groups and len(groups) > DKEEP and groups[0][-1] + DLAG <= p:
                    f_d(st, groups.pop(0))
            while groups:
                f_d(st, groups.pop(0))
            f_store(st)
            return carry
        lax.fori_loop(0, NH, body, 0)


@jax.jit
def pallas_interleave_layers__sliding_local_dilated__glu_gated_geglu__prompt_kernel(
    A_x, A_wqkv, A_wo, B_x, B_w_gate, B_w_up, B_w_down):
    B, S, D = A_x.shape
    DF = B_w_gate.shape[1]
    NB = S // TB
    xT = A_x.reshape(S, D).T
    wdT = B_w_down.T
    NCH = DF // (2 * TC)
    nsteps = 1 + KPAIR + NB
    hbm = pl.BlockSpec(memory_space=pltpu.HBM)
    outT = pl.pallas_call(
        functools.partial(_kernel, D=D, DF=DF, NB=NB),
        grid=(nsteps,),
        in_specs=[hbm] * 6,
        out_specs=pl.BlockSpec((D, TM), lambda g: (0, jnp.maximum(g - (1 + KPAIR + NB // 2), 0))),
        out_shape=jax.ShapeDtypeStruct((D, S), A_x.dtype),
        scratch_shapes=[
            pltpu.VMEM((D, S), bf16),
            pltpu.VMEM((D, 3 * D), bf16),
            pltpu.VMEM((D, D), bf16),
            pltpu.VMEM((NQKV // 2, KP), u32),
            pltpu.VMEM((D // 2, KP), u32),
            pltpu.VMEM((NCH + 1, 3, D, 2 * TC), bf16),
            pltpu.VMEM((NCH + 1, 8 * (KH // 2) + 5 * (D // 6) + 16, 2 * TC), u32),
            pltpu.VMEM((5, NQKV, 128), f32),
            pltpu.VMEM((20, HALO + TB, 128), f32),
            pltpu.VMEM((20, HALO + TB, 128), f32),
            pltpu.VMEM((NB + 1, D, TB), f32),
            pltpu.VMEM((2, D, TB), f32),
            pltpu.VMEM((TB // 2, KP), u32),
            pltpu.VMEM((TB // 2, KP), u32),
            pltpu.VMEM((NSLOT + 1, 8, TB // 2, KH), u32),
            pltpu.VMEM((NQKV // 4 + 32, 17 * 128), u32),
            pltpu.VMEM((2, D, TB), f32),
            pltpu.VMEM((8, TB // 2, KH), u32),
            pltpu.SMEM((KPAIR * CP + 1,), jnp.int32),
            pltpu.SemaphoreType.DMA((9 + NCH,)),
        ],
        compiler_params=pltpu.CompilerParams(
            dimension_semantics=("arbitrary",),
            vmem_limit_bytes=110 * 1024 * 1024,
        ),
    )(xT, A_wqkv, A_wo, B_w_gate, B_w_up, wdT)
    return outT.T.reshape(B, S, D)
```

```python
import functools
import math
import jax
import jax.numpy as jnp
from jax import lax
import jax.experimental.pallas as pl
import jax.experimental.pallas.tpu as pltpu

H = 32
DH = 18
W = 8
DIL = 2
HALO = 16
EPS = 1e-5
TB = 128
TM = 256
NH = 2
RB = 8
KP = 640
KH = 256
KX = 192
KY = 64
NQKV = 14 * 128
TC = 128
CW = 3 * TC
NSLOT = 8
DG = int(3)
ROWS_LO = int(0)
WO_AT = int(6)
DLAG = int(1)
LN1_AT = int(7)
SERIAL = int(1)
SERIAL_A = int(0)
LN_F = tuple(int(x) for x in '1,4'.split(','))
LN_A = tuple(int(x) for x in '2,8'.split(','))
KPAIR = int(6)
CP = int(2)
QSPLIT = int(5)
XFIRST = 512
DGROUPS = tuple(int(x) for x in '4,4,2,2'.split(','))
DGROUPS_F = tuple(int(x) for x in '2,2,2'.split(','))
DORD = tuple(int(x) for x in '2,3,12,4,5,13,14,0,9,10,1,6,7,8,11'.split(','))
QB_AT = int(4); WOA_AT = int(5)
LNA_AT = int(0); LNB_AT = int(2); WOB_AT = int(9)
QPR = 16
RBD = int(1)
DKEEP = int(2)
RESTAT = int(0)
TAILF = float(0.6)
LND = tuple(int(x) for x in '3,8'.split(','))
WOSPLIT = int(1)
NPACE = int(4)
MODE_F = tuple(int(x) for x in '0,1,0,2,1'.split(','))
MODE_A = tuple(int(x) for x in '1,3,1,0,0'.split(','))
FENCE = int(1)
PR = 32
PW1 = float(1); PW2 = float(1); PW3 = float(1)
SOPS_EARLY = int(1)
CLIP = int(0)

f32 = jnp.float32
bf16 = jnp.bfloat16
u32 = jnp.uint32
NT = (((1,), (1,)), ((), ()))


def _pk(x):
    return pltpu.bitcast(x.astype(bf16), u32)


def _unpk(u, idx):
    return pltpu.unpack_elementwise(u, index=idx, packed_dtype=bf16, unpacked_dtype=f32)


def _pk2(even, odd):
    return pltpu.pack_elementwise([even, odd], packed_dtype=bf16).astype(u32)


def _up(x):
    return pltpu.bitcast(x, bf16)


def _dot(a, b):
    return jnp.dot(a, b, preferred_element_type=f32)


def _dot_nt(a, b):
    return lax.dot_general(a, b, NT, preferred_element_type=f32)


def _ln_stats(x, NACC, pin=None):
    n = x.shape[0]
    c = x[0:1] if pin is None else pin(x[0:8])[0:1]
    s1 = [None] * NACC
    s2 = [None] * NACC
    for i in range(n // 8):
        d = x[i * 8:(i + 1) * 8] - c
        k = i % NACC
        s1[k] = d if s1[k] is None else s1[k] + d
        dd = d * d
        s2[k] = dd if s2[k] is None else s2[k] + dd
    while len(s1) > 1:
        s1 = [s1[i] + s1[i + 1] for i in range(0, len(s1), 2)]
        s2 = [s2[i] + s2[i + 1] for i in range(0, len(s2), 2)]
    m = jnp.sum(s1[0], axis=0, keepdims=True) * (1.0 / n)
    v = jnp.sum(s2[0], axis=0, keepdims=True) * (1.0 / n) - m * m
    v = jnp.maximum(v, 0.0)
    return c + m, lax.rsqrt(v + EPS)


def _tree(fn, xs):
    xs = list(xs)
    while len(xs) > 1:
        xs = [fn(xs[i], xs[i + 1]) for i in range(0, len(xs) - 1, 2)] + ([xs[-1]] if len(xs) % 2 else [])
    return xs[0]


def _lhs_ops(a11, a12, a21, a22):
    return (a11 + a22, a21 + a22, a11, a22, a11 + a12, a21 - a11, a12 - a22)


def _rhs_ops(b11, b12, b21, b22):
    return (b11 + b22, b11, b12 - b22, b21 - b11, b22, b11 + b12, b21 + b22)


_D_LHS = (
    ((0, 0, 1), (0, 2, -1), (1, 0, -1)), ((0, 0, 1), (0, 1, -1), (2, 0, -1)), ((1, 1, 1), (0, 1, -1), (1, 2, -1)),
    ((1, 1, 1), (1, 0, -1), (2, 1, -1)), ((2, 2, 1), (0, 2, -1), (2, 1, -1)), ((2, 2, 1), (1, 2, -1), (2, 0, -1)),
    ((0, 1, 1),), ((0, 1, 1), (1, 0, -1)), ((1, 0, 1),),
    ((0, 2, 1),), ((0, 2, 1), (2, 0, -1)), ((2, 0, 1),),
    ((1, 2, 1),), ((2, 1, 1), (1, 2, -1)), ((2, 1, 1),),
)
_D_OUT = {
    (0, 0): ((0, 1), (7, 1), (8, 1), (9, 1), (6, -1)),
    (0, 1): ((1, 1), (6, 1), (10, 1), (11, 1), (9, -1)),
    (1, 0): ((2, 1), (7, 1), (8, 1), (12, 1), (6, -1)),
    (1, 1): ((3, 1), (6, 1), (13, 1), (14, 1), (2, -1), (7, -1)),
    (2, 0): ((5, 1), (9, 1), (12, 1), (13, 1), (4, -1), (10, -1)),
    (2, 1): ((4, 1), (10, 1), (11, 1), (14, 1), (9, -1)),
}


def _d_rhs(b):
    s1 = b[1][0] + b[1][1]
    s2 = b[2][0] + b[2][1]
    t7 = b[0][1] + s1
    t10 = b[0][0] + s2
    return (b[0][0], b[0][1], b[1][0], s1, b[2][1], s2, b[0][1] + b[1][1], t7, b[0][0] + t7,
            b[0][0] + b[2][0], t10, b[0][1] + t10, b[1][0] + b[2][0], b[1][0] - b[2][1], b[1][1] + b[2][1])


def _signed_sum(terms):
    acc = None
    for v, sg in terms:
        if acc is None:
            assert sg == 1
            acc = v
        else:
            acc = acc + v if sg == 1 else acc - v
    return acc


def _dst_row(sec, d):
    if sec == 0:
        return d * 32 if d < 16 else 1024 + (d - 16) * 32
    if sec == 1:
        return 512 + d * 32 if d < 16 else 13 * 128 + (d - 16) * 32
    return 9 * 128 + d * 32 if d < 16 else 1024 + 64 + (d - 16) * 32


def _prep_plan(nchunk):
    plan = [[nchunk] * CP]
    nxt = 0
    for j in range(1, KPAIR):
        left_steps = KPAIR - 1 - j
        n = min(CP, nchunk - nxt)
        if j == 1:
            n = max(0, min(n, max(CP - 1, nchunk - nxt - left_steps * CP)))
        ids = list(range(nxt, nxt + n))
        nxt += n
        plan.append(ids + [nchunk] * (CP - n))
    return plan, nxt


def _kernel(x_hbm, wqkv_hbm, wo_hbm, wg_hbm, wu_hbm, wd_hbm, o_ref,
            xin, wqkv_raw, wo_raw, wqkvT, woT, raw, pw, tmp, qa, qb, xres, xn_f, xn1a, xn1b,
            s_scr, wq_s, xn_g, sq_scr, plan_s, sems, *, D, DF, NB):
    g = pl.program_id(0)
    NCH = DF // CW
    NPC = NCH // NH
    K = 2 * KPAIR
    S = NB * TB
    plan, nprepped = _prep_plan(NCH)
    zero8 = pl.multiple_of((g >> 20) * 8, 8)

    QSEC = ((0, 5), (5, 9), (9, 14))
    XPC = ((0, 256), (256, 512), (512, 1024), (1024, 1536), (1536, S))

    def cp_qkv(sec):
        out = []
        for j in range(*QSEC[sec]):
            n = min(128, 3 * D - j * 128)
            out.append(pltpu.make_async_copy(wqkv_hbm.at[:, pl.ds(j * 128, n)], wqkv_raw.at[:, pl.ds(j * 128, n)],
                                             sems.at[sec]))
        return out

    def cp_wo():
        return pltpu.make_async_copy(wo_hbm, wo_raw, sems.at[3])

    def cp_x(k):
        lo, hi = XPC[k]
        return pltpu.make_async_copy(x_hbm.at[:, pl.ds(lo, hi - lo)], xin.at[:, pl.ds(lo, hi - lo)], sems.at[4 + k])

    def chunk_copies(c):
        return [pltpu.make_async_copy(w.at[:, pl.ds(c * CW, CW)], raw.at[c, m], sems.at[9 + c])
                for m, w in enumerate((wg_hbm, wu_hbm, wd_hbm))]

    D3 = D // 3
    KR = D - 3 * TC
    R_TR = 15 * (TC // 2)
    R_SD = R_TR + 3 * (KR // 2)
    R_END = R_SD + 8 * (D3 // 2)

    def prep_pieces(c):
        def hk_piece(m, r):
            rb = D3 if m == 2 else TC
            blk = {}
            for i in range(3):
                for j in range(3):
                    u = pltpu.bitcast(raw[c, m, pl.ds(i * rb + r, 16), pl.ds(j * TC, TC)], u32)
                    blk[i, j] = (u, _unpk(u, 0), _unpk(u, 1))
            for k, terms in enumerate(_D_LHS):
                if len(terms) == 1:
                    t = blk[terms[0][:2]][0]
                else:
                    t = _pk2(_signed_sum([(blk[i, j][1], sg) for i, j, sg in terms]),
                             _signed_sum([(blk[i, j][2], sg) for i, j, sg in terms]))
                if m == 2:
                    pw[c, pl.ds(R_SD + (k // 2) * (D3 // 2) + r // 2, 8), (k % 2) * TC:(k % 2 + 1) * TC] = t
                else:
                    pw[c, pl.ds(k * (TC // 2) + r // 2, 8), m * TC:(m + 1) * TC] = t

        def rem_piece(m, j):
            pw[c, pl.ds(R_TR + j * (KR // 2), KR // 2), m * TC:(m + 1) * TC] = pltpu.bitcast(
                raw[c, m, pl.ds(3 * TC, KR), pl.ds(j * TC, TC)], u32)

        out = []
        for m in range(2):
            out += [functools.partial(hk_piece, m, r) for r in range(0, TC, 16)]
            out += [functools.partial(rem_piece, m, j) for j in range(3)]
        out += [functools.partial(hk_piece, 2, r) for r in range(0, D3, 16)]
        return out

    def prep_group(cs):
        out = []
        for c in cs:
            out += prep_pieces(c)
        return out

    class Pacer:
        def __init__(self, pieces, pace, npts, idle=0):
            self.pieces, self.pace, self.n, self.pt, self.done = pieces, pace, npts - idle, 0, 0

        def __call__(self, v):
            self.pt += 1
            upto = min(len(self.pieces), int(round(len(self.pieces) * self.pt / self.n)))
            if upto > self.done or self.pt == self.n + 1:
                self.pace(v)
            for piece in self.pieces[self.done:upto]:
                piece()
            self.done = upto

    def pace_wq(v):
        wq_s[pl.ds(NQKV // 4 + zero8, 8), 0:128] = pltpu.bitcast(v, u32)

    def pace_pwz(v):
        pw[NCH, pl.ds(R_END + zero8, 8), 0:128] = pltpu.bitcast(v, u32)

    def pace_pw(v):
        pw[NCH, pl.ds(R_END, 8), 0:128] = pltpu.bitcast(v, u32)

    nr = TB // RB
    QT = (0, 1, 2, 3, 8)
    KT = (4, 5, 6, 7, 13)
    VT = (9, 10, 11, 12, 8)
    scale = DH ** -0.5
    c2e = scale * math.log2(math.e)
    neg = -1e9 * math.log2(math.e)
    k0 = math.sqrt(2.0 / math.pi)
    k1 = k0 * 0.044715

    zvec = jnp.full((RB, 128), (g >> 20).astype(u32), u32)

    def tie(x, dep):
        return pltpu.bitcast(pltpu.bitcast(x, u32) | (pltpu.bitcast(dep, u32) & zvec), f32)

    def normalize(blk, mean, rstd, link):
        if not link:
            return (xres[blk] - mean) * rstd
        rs = jnp.broadcast_to(rstd, (8, TB))
        mb = jnp.broadcast_to(mean, (8, TB))
        outs = []
        for i in range(D // 8):
            if i and i % link == 0:
                rs = tie(rs, outs[-1])
            outs.append((xres[blk, pl.ds(i * 8, 8), :] - mb) * rs)
        return jnp.concatenate(outs, axis=0)

    def x_convert(blk):
        x = xin[:, pl.ds(pl.multiple_of(blk * TB, TB), TB)].astype(f32)
        xres[blk] = x
        return x

    def a_ln1(blk, dst, from_input):
        x = x_convert(blk) if from_input else xres[blk]
        mean, rstd = _ln_stats(x, LN_A[0])
        if not from_input:
            dst[pl.ds(0, 8), :] = jnp.zeros((8, KP), u32)
        xn = (xres[blk] - mean) * rstd
        xp = jnp.concatenate([xn, jnp.zeros((KP - D, TB), f32)], axis=0)
        dst[...] = pltpu.bitcast(xp.astype(bf16).T, u32)

    def a_qkv(src, qdst, qprev, t0=0, t1=14, cb=None):
        qkv = _dot_nt(_up(src[...]), _up(wqkvT[pl.ds(t0 * 64, (t1 - t0) * 64), :]))
        for t in range(max(t0, 4), t1):
            qdst[t, pl.ds(0, HALO), :] = qprev[t, pl.ds(TB, HALO), :]
        for t in range(t0, t1):
            qdst[t, pl.ds(HALO, TB), :] = qkv[:, (t - t0) * 128:(t - t0 + 1) * 128]
            if cb is not None:
                for k in range(NPACE):
                    rr = k * (TB // NPACE)
                    cb(qkv[rr:rr + 8, (t - t0) * 128:(t - t0 + 1) * 128])

    cbits = pltpu.bitcast(jnp.full((RB, 128), c2e, f32), u32)

    def tied_scale(deps):
        if not deps:
            return c2e
        acc = pltpu.bitcast(deps[0], u32)
        for dv in deps[1:]:
            acc = acc | pltpu.bitcast(dv, u32)
        return pltpu.bitcast(cbits | (acc & zvec), f32)

    def a_rows(q_s, blk, rs, mode, hist, start=None):
        lag_mid, lag_end, midkind, fw, fv = mode
        for r in rs:
            r0 = r * RB
            deps = [start] if (start is not None and r == 0) else []
            if lag_mid and r - lag_mid >= 0:
                deps.append(hist[('h' if midkind else 'm', r - lag_mid)])
            if lag_end and r - lag_end >= 0:
                deps += hist[('o', r - lag_end)]
            cs = tied_scale(deps)
            q = [q_s[t, pl.ds(HALO + r0, RB), :] * cs for t in QT]
            sc = []
            q0 = q[0]
            prev = None
            for w in range(W):
                off = HALO + r0 - DIL * w
                acc = None
                if fw and w and w % fw == 0:
                    q0 = tie(q[0], prev)
                for j, t in enumerate(KT):
                    p = (q0 if j == 0 else q[j]) * q_s[t, pl.ds(off, RB), :]
                    acc = p if acc is None else acc + p
                prev = acc
                acc = acc + pltpu.roll(acc, 64, 1)
                hist[('h', r)] = acc
                acc = acc + pltpu.roll(acc, 32, 1)
                if r0 - DIL * w < 0:
                    pos = blk * TB + r0 + lax.broadcasted_iota(jnp.int32, (RB, 128), 0)
                    acc = jnp.where(pos >= DIL * w, acc, neg)
                sc.append(acc)
            m = _tree(jnp.maximum, sc)
            hist[('m', r)] = m
            e = [jnp.exp2(sc[w] - m) for w in range(W)]
            l = _tree(jnp.add, e)
            rinv = pl.reciprocal(l, approx=True)
            rinv = rinv * (2.0 - l * rinv)
            outs = []
            e0 = e[0]
            for j, t in enumerate(VT):
                if fv and j and j % fv == 0:
                    e0 = tie(e[0], acc)
                acc = None
                for w in range(W):
                    off = HALO + r0 - DIL * w
                    p = (e0 if w == 0 else e[w]) * q_s[t, pl.ds(off, RB), :]
                    acc = p if acc is None else acc + p
                o = acc * rinv
                st_off = r0 + zero8 if (j == 4 and r == nr - 1 and FENCE) else r0
                q_s[14 + j, pl.ds(st_off, RB), :] = o
                outs.append(o)
            hist[('o', r)] = outs[-1:] if fv == 1 else outs

    def a_wo(q_s, blk, par, ln, cb=None):
        if WOSPLIT:
            o4 = q_s[18, pl.ds(0, TB), :].astype(bf16)
            rq = D // 8
            y = jnp.concatenate([_dot_nt(_up(woT[pl.ds(k * rq, rq), 512:640]), o4) for k in range(4)], axis=0)
            o = jnp.concatenate([q_s[14 + j, pl.ds(0, TB), :] for j in range(4)], axis=1).astype(bf16)
            x1 = _dot_nt(_up(woT[:, 0:512]), o) + (xres[blk] + y)
        else:
            o = jnp.concatenate([q_s[14 + j, pl.ds(0, TB), :] for j in range(5)], axis=1).astype(bf16)
            x1 = xres[blk] + _dot_nt(_up(woT[...]), o)
        xres[blk] = x1
        if cb is not None:
            for i in range(0, D, 16):
                cb(x1[i:i + 8])
        mean, rstd = _ln_stats(x1, ln[0])
        xn_f[par] = normalize(blk, mean, rstd, ln[1])

    def sops(src, put):
        def seg(tb, r0, n):
            return lambda: src[tb, pl.ds(r0, n), :]
        A11, A12, A21, A22 = seg(0, 0, KX), seg(0, KH, KX), seg(1, 0, KX), seg(1, KH, KX)
        a11, a12, a21, a22 = seg(0, KX, KY), seg(0, KH + KX, KY), seg(1, KX, KY), seg(1, KH + KX, KY)
        rt, rb = seg(0, 2 * KH, KY), seg(1, 2 * KH, KY)
        parts = (
            lambda: (A21() + A22(), -(a21() + a22())),
            lambda: (A11(), -a22()),
            lambda: (A22(), -a11()),
            lambda: (A11() + A12(), -(a11() + a12())),
            lambda: (A12() - A22(), rt()),
            lambda: (A21() - A11(), rb()),
            lambda: (rt(), a12() - a22(), rb(), a21() - a11()),
            lambda: (A11() + A22(), a11() + a22()),
        )
        for i, fn in enumerate(parts):
            t = jnp.concatenate(fn(), axis=0)
            put(i, pltpu.bitcast(t.astype(bf16).T, u32))

    def sops15(put):
        def X(t, r0, n):
            return xn_f[t, pl.ds(r0, n), :]
        for n in range(15):
            terms = [(i, t, sg) for (i, t), lst in _D_OUT.items() for k, sg in lst if k == n]
            terms.sort(key=lambda z: -z[2])
            v = _signed_sum([(X(t, i * TC, TC), sg) for i, t, sg in terms])
            put(n, pltpu.bitcast(v.astype(bf16).T, u32))
        k1, k2, k3 = 3 * TC, 3 * TC + KY, 3 * TC + 2 * KY
        trick = ((lambda: (X(0, k1, KY), X(0, k2, KY) - X(1, k2, KY))),
                 (lambda: (X(1, k1, KY), X(1, k3, KY) - X(0, k3, KY))),
                 (lambda: (X(1, k2, KY), X(0, k3, KY))))
        for n, fn in enumerate(trick):
            put(15 + n, pltpu.bitcast(jnp.concatenate(fn(), axis=0).astype(bf16).T, u32))

    def a_sops(slot):
        def put(i, v):
            s_scr[slot, i] = v
        sops15(put)

    NQH = NQKV // 4

    def q_prep_pieces():
        lo = lax.broadcasted_iota(jnp.int32, (QPR, 128), 1) < 64

        def piece(r):
            def ld(half, t):
                u = wqkvT[pl.ds(half * NQH + r, QPR), t * 128:(t + 1) * 128]
                return u, _unpk(u, 0), _unpk(u, 1)

            def add(u, v):
                return _pk2(u[1] + v[1], u[2] + v[2])

            def sub(u, v):
                return _pk2(u[1] - v[1], u[2] - v[2])

            def put(tile, v):
                wq_s[pl.ds(r, QPR), tile * 128:(tile + 1) * 128] = v
            r1, r2 = wqkvT[pl.ds(r, QPR), 512:640], wqkvT[pl.ds(NQH + r, QPR), 512:640]
            zero = jnp.zeros((QPR, 128), u32)
            for t in range(2):
                x1, x2, y1, y2 = ld(0, t), ld(1, t), ld(0, 2 + t), ld(1, 2 + t)
                put(2 + t, sub(x2, y2))
                put(4 + t, sub(y1, x1))
                sy, sx, d1 = add(y1, y2), add(x1, x2), add(x1, y2)
                if t == 0:
                    put(0, x1[0])
                    put(6, y2[0])
                    put(8, sy)
                    put(10, sx)
                    put(14, d1)
                else:
                    put(1, jnp.where(lo, x1[0], x2[0]))
                    put(7, jnp.where(lo, y2[0], y1[0]))
                    put(9, jnp.where(lo, sy, r1))
                    put(11, jnp.where(lo, sx, r2))
                    put(12, jnp.where(lo, r2, sy))
                    put(13, jnp.where(lo, r1, sx))
                    put(15, jnp.where(lo, d1, zero))
                    put(16, jnp.where(lo, zero, add(x2, y1)))
        return [functools.partial(piece, r) for r in range(0, NQH, QPR)]

    def a_ln1f(blk, par, dep=None):
        mean, rstd = _ln_stats(xres[blk], LN_F[0], None if dep is None else (lambda v: tie(v, dep)))
        xn_g[par, pl.ds(0, 8), :] = jnp.zeros((8, TB), f32)
        xn_g[par] = normalize(blk, mean, rstd, LN_F[1])

    def a_qsops():
        def put(i, v):
            sq_scr[i, pl.ds(zero8, TB // 2), :] = v
        sops(xn_g, put)

    def a_qkv2_halo(qtop, qbot):
        for t in range(4, 14):
            qtop[t, pl.ds(0, HALO), :] = qbot[t, pl.ds(TB, HALO), :]

    def a_qkv2(qtop, qbot, t0, nt):
        def Q(slot, l0, l1, w0):
            lhs = _up(sq_scr[slot, :, l0:l1])
            rhs = _up(wq_s[pl.ds(t0 * 64, nt * 64), w0 * 128:w0 * 128 + (l1 - l0)])
            return _dot_nt(lhs, rhs)

        def out(dst, tb, v):
            for k in range(nt):
                dst[tb + k, pl.ds(HALO, TB), :] = v[:, k * 128:(k + 1) * 128]
                if dst is qtop and tb + k >= 4:
                    qbot[tb + k, pl.ds(0, HALO), :] = v[TB - HALO:, k * 128:(k + 1) * 128]
        q5 = Q(3, 0, KH, 6)
        q3 = Q(1, 0, KH, 2)
        q1b = Q(7, 128, KH, 16)
        out(qtop, t0 + 7, q3 + q5 + q1b + Q(6, 0, 128, 12))
        q4 = Q(2, 0, KH, 4)
        q2 = Q(0, 0, KH, 0)
        out(qbot, t0, q2 + q4 + q1b + Q(6, 128, KH, 13))
        q1 = Q(7, 0, KH, 14)
        out(qtop, t0, q1 + q4 - q5 + Q(4, 0, KH, 8))
        out(qbot, t0 + 7, q1 - q2 + q3 + Q(5, 0, KH, 10))

    class St:
        pass

    def f_init(st, j):
        st.c0 = 0
        st.b0 = (j * NH) % NB
        st.sb = j % NSLOT
        st.acc = [None] * 15
        st.t = {}

    def gelu_mul(c):
        gg = c[:, :TC]
        u = c[:, TC:]
        t = jnp.tanh(gg * (k0 + k1 * (gg * gg)))
        gu = gg * u
        return gu + gu * t

    def f_gu(st, p):
        c = st.c0 + p
        hk = KY // 2

        def L(n):
            return s_scr[st.sb, n]

        def R(n):
            return pw[c, pl.ds(n * (TC // 2), TC // 2), :]

        def RT(j, kind):
            r0 = R_TR + j * (KR // 2)
            if kind == 1:
                return jnp.concatenate([pw[c, pl.ds(r0, hk), :], pw[c, pl.ds(r0 + 2 * hk, hk), :]], axis=0)
            return pw[c, pl.ds(r0 + (hk if kind == 2 else 0), 2 * hk), :]

        def P(n):
            return _dot(_up(L(n)), _up(R(n)))

        def T(j, kind):
            return _dot(_up(L(15 + kind)), _up(RT(j, kind)))

        def PT(n, j, kind):
            return _dot(_up(jnp.concatenate([L(n), L(15 + kind)], axis=1)),
                        _up(jnp.concatenate([R(n), RT(j, kind)], axis=0)))
        p8 = P(8)
        t7 = P(7) + p8
        st.first = t7[0:8, 0:128]
        s1 = PT(3, 1, 2) + t7
        p6 = P(6)
        p14 = P(14)
        h11 = gelu_mul(T(1, 1) + (p6 + p14 + s1))
        p12 = P(12)
        p13 = P(13)
        h10 = gelu_mul(PT(2, 1, 0) + (p12 + p13 + s1))
        p11 = P(11)
        t10 = P(10) + p11
        s2 = PT(5, 2, 2) + t10
        p9 = P(9)
        h20 = gelu_mul(T(2, 0) + (p9 + p12 + s2))
        h21 = gelu_mul(PT(4, 2, 1) + (p14 - p13 + s2))
        w0 = T(0, 2)
        h00 = gelu_mul(PT(0, 0, 0) + (p8 + p9 + t10 + w0))
        h01 = gelu_mul(PT(1, 0, 1) + (p6 + p11 + t7 + w0))
        st.t[p] = ((h00, h01), (h10, h11), (h20, h21))

    def f_d(st, ps):
        rhs = [_d_rhs(st.t.pop(p)) for p in ps]
        for i in DORD:
            a = jnp.concatenate([_up(pw[st.c0 + p, pl.ds(R_SD + (i // 2) * (D3 // 2), D3 // 2),
                                        (i % 2) * TC:(i % 2 + 1) * TC]) for p in ps], axis=1)
            t = jnp.concatenate([r[i] for r in rhs], axis=1).astype(bf16)
            r = _dot_nt(a, t)
            st.acc[i] = r if st.acc[i] is None else r + st.acc[i]

    def f_store(st):
        for k in range(NH):
            y = jnp.concatenate([_signed_sum([(st.acc[n], sg) for n, sg in _D_OUT[i, k]]) for i in range(3)], axis=0)
            x2 = xres[st.b0 + k] + 0.5 * y
            xres[st.b0 + k] = x2
            o_ref[:, k * TB:(k + 1) * TB] = x2.astype(o_ref.dtype)

    def run_pair(jf, ja):
        st = St()
        f_init(st, jf)
        groups = []
        p0 = 0
        for n in DGROUPS:
            groups.append(list(range(p0, p0 + n)))
            p0 += n
        assert p0 == NCH
        if ja is not None:
            a = (2 * ja) % NB
            b = a + 1
            ha = {}
            a_rows(qa, a, range(nr), MODE_F, ha)
        for p in range(NCH):
            f_gu(st, p)
            while groups and len(groups) > DKEEP and groups[0][-1] + DLAG <= p:
                f_d(st, groups.pop(0))
            if ja is not None:
                if p == LNA_AT:
                    a_ln1f(b, 0, ha[('h', LND[0])] if LND[0] >= 0 else None)
                if p == LNB_AT:
                    a_ln1f((a + 2) % NB, 1, ha[('h', LND[1])] if LND[1] >= 0 else None)
                    a_qsops()
                if p == WOA_AT:
                    a_wo(qa, a, 0, LN_F)
                if p == QB_AT:
                    a_qkv2_halo(qb, qa)
                    for t0, nt in ((0, 2), (2, 2), (4, 2), (6, 1)):
                        a_qkv2(qb, qa, t0, nt)
                    if not RBD:
                        a_rows(qb, b, range(nr), MODE_F, {})
                if RBD and p == QB_AT + RBD:
                    a_rows(qb, b, range(nr), MODE_F, {}, st.first)
                if p == WOB_AT:
                    a_wo(qb, b, 1, LN_F)
        if ja is not None:
            a_sops(ja % NSLOT)
        while groups:
            f_d(st, groups.pop(0))
        f_store(st)

    def run_aa(j):
        a = 2 * j
        b = a + 1
        pieces = prep_group([plan_s[j * CP + k] for k in range(CP)])
        cb = Pacer(pieces, pace_pw, 28 * NPACE, NPACE)
        a_rows(qa, a, range(nr), MODE_A, {})
        a_wo(qb, jnp.where(j == 0, NB, a - 1), 1, LN_A)
        a_sops(jnp.where(j == 0, NSLOT, j - 1))
        a_ln1(a + 2, xn1a, True)
        a_qkv(xn1b, qb, qa, cb=cb)
        a_rows(qb, b, range(nr), MODE_A, {})
        a_wo(qa, a, 0, LN_A)
        a_ln1(b + 2, xn1b, True)
        a_qkv(xn1a, qa, qb, cb=cb)
        assert cb.done == len(pieces)

    def start_rest():
        cp_wo().start()
        cp_x(1).start()
        cp_x(2).start()
        for c in range(NCH):
            for cp in chunk_copies(c):
                cp.start()
            if c == 2:
                cp_x(3).start()
            if c == 6:
                cp_x(4).start()

    def qkv_section(sec):
        for cp in cp_qkv(sec):
            cp.wait()
        if sec == RESTAT:
            start_rest()
        for j in range(*QSEC[sec]):
            wd_ = min(128, 3 * D - j * 128)
            blk = wqkv_raw[:, j * 128:j * 128 + wd_].astype(f32)
            if wd_ < 128:
                blk = jnp.concatenate([blk, jnp.zeros((D, 128 - wd_), f32)], axis=1)
            bt = jnp.concatenate([blk, blk[2 * KH:]], axis=0).T
            for t in range(5):
                tmp[t, pl.ds(j * 128, 128), :] = bt[:, t * 128:(t + 1) * 128]
        for d in range(DH):
            r = _dst_row(sec, d)
            for t in range(5):
                wqkvT[pl.ds(r // 2, 16), t * 128:(t + 1) * 128] = _pk2(
                    tmp[t, pl.ds(sec * D + d, 16, stride=2 * DH), :],
                    tmp[t, pl.ds(sec * D + d + DH, 16, stride=2 * DH), :])

    @pl.when(g == 0)
    def _():
        cp_x(0).start()
        for sec in range(3):
            for cp in cp_qkv(sec):
                cp.start()
        if RESTAT < 0:
            start_rest()
        for j in range(KPAIR):
            for k in range(CP):
                plan_s[j * CP + k] = plan[j][k]
        qb[:, pl.ds(TB, HALO), :] = jnp.zeros((20, HALO, 128), f32)
        wqkvT[pl.ds((13 * 128 + 64) // 2, 32), :] = jnp.zeros((32, KP), u32)
        zpad = jnp.zeros((KP - D, 128), f32)
        cp_x(0).wait()
        a_ln1(0, xn1a, True)
        a_ln1(1, xn1b, True)
        qkv_section(0)
        a_qkv(xn1a, qa, qb, 0, 4)
        qkv_section(1)
        a_qkv(xn1a, qa, qb, 4, 8)
        qkv_section(2)
        cp_wo().wait()
        cb = Pacer(q_prep_pieces(), pace_wq, 6 * NPACE)
        a_qkv(xn1a, qa, qb, 8, 14, cb=cb)
        for t in range(5):
            wd_ = 128 if t < 4 else 64
            blk = wo_raw[:, t * 128:t * 128 + wd_].astype(f32)
            if wd_ < 128:
                blk = jnp.concatenate([blk, jnp.zeros((D, 128 - wd_), f32)], axis=1)
            tmp[t, pl.ds(0, D), :] = blk
        for t in range(5):
            rows = [tmp[t, pl.ds(d, 32, stride=DH), :] for d in range(DH)]
            full = jnp.concatenate(rows[:16] + [zpad] + rows[16:], axis=0)
            ft = full.T
            n = 128 if t < 4 else 64
            woT[pl.ds(t * 64, n // 2), :] = _pk(ft[:n])
        cp_x(1).wait()

    for j in range(1, KPAIR):
        @pl.when(g == 1 + j)
        def _():
            if j % 2 == 1:
                cp_x(2 + j // 2).wait()
            for c in plan[j]:
                if c < NCH:
                    for cp in chunk_copies(c):
                        cp.wait()

    @pl.when(jnp.logical_and(g >= 1, g <= KPAIR))
    def _():
        run_aa(g - 1)

    @pl.when(g == KPAIR + 1)
    def _():
        pieces = []
        for c in range(nprepped, NCH):
            for cp in chunk_copies(c):
                cp.wait()
        pieces += prep_group(range(nprepped, NCH))
        n1 = int(len(pieces) * TAILF)
        cb = Pacer(pieces[:n1], pace_pwz, D // 16)
        a_wo(qb, K - 1, 1, (4, 0), cb=cb)

        cb2 = Pacer(pieces[n1:], pace_pwz, 18)

        def put(i, v):
            s_scr[KPAIR - 1, i] = v
            cb2(pltpu.bitcast(v[0:8, 0:128], f32))
        sops15(put)
        for blk in range(K + 2, NB):
            x_convert(blk)

    jf = g - (KPAIR + 1)

    @pl.when(jnp.logical_and(jf >= 0, jf < NB - KPAIR))
    def _():
        run_pair(jf, jf + KPAIR)

    @pl.when(jf >= NB - KPAIR)
    def _():
        def body(hf, carry):
            st = St()
            f_init(st, jf)
            st.c0 = hf * NPC
            groups = []
            p0 = 0
            for n in DGROUPS_F:
                groups.append(list(range(p0, p0 + n)))
                p0 += n
            for p in range(NPC):
                f_gu(st, p)
                while groups and len(groups) > DKEEP and groups[0][-1] + DLAG <= p:
                    f_d(st, groups.pop(0))
            while groups:
                f_d(st, groups.pop(0))
            f_store(st)
            return carry
        lax.fori_loop(0, NH, body, 0)


@jax.jit
def pallas_interleave_layers__sliding_local_dilated__glu_gated_geglu__prompt_kernel(
    A_x, A_wqkv, A_wo, B_x, B_w_gate, B_w_up, B_w_down):
    B, S, D = A_x.shape
    DF = B_w_gate.shape[1]
    NB = S // TB
    xT = A_x.reshape(S, D).T
    wdT = B_w_down.T
    NCH = DF // CW
    nsteps = 1 + KPAIR + NB
    hbm = pl.BlockSpec(memory_space=pltpu.HBM)
    outT = pl.pallas_call(
        functools.partial(_kernel, D=D, DF=DF, NB=NB),
        grid=(nsteps,),
        in_specs=[hbm] * 6,
        out_specs=pl.BlockSpec((D, TM), lambda g: (0, jnp.maximum(g - (1 + KPAIR + NB // 2), 0))),
        out_shape=jax.ShapeDtypeStruct((D, S), A_x.dtype),
        scratch_shapes=[
            pltpu.VMEM((D, S), bf16),
            pltpu.VMEM((D, 3 * D), bf16),
            pltpu.VMEM((D, D), bf16),
            pltpu.VMEM((NQKV // 2, KP), u32),
            pltpu.VMEM((D // 2, KP), u32),
            pltpu.VMEM((NCH + 1, 3, D, CW), bf16),
            pltpu.VMEM((NCH + 1, 15 * (TC // 2) + 3 * (D - CW) // 2 + 8 * (D // 6) + 16, 2 * TC), u32),
            pltpu.VMEM((5, NQKV, 128), f32),
            pltpu.VMEM((20, HALO + TB, 128), f32),
            pltpu.VMEM((20, HALO + TB, 128), f32),
            pltpu.VMEM((NB + 1, D, TB), f32),
            pltpu.VMEM((2, D, TB), f32),
            pltpu.VMEM((TB // 2, KP), u32),
            pltpu.VMEM((TB // 2, KP), u32),
            pltpu.VMEM((NSLOT + 1, 18, TB // 2, TC), u32),
            pltpu.VMEM((NQKV // 4 + 32, 17 * 128), u32),
            pltpu.VMEM((2, D, TB), f32),
            pltpu.VMEM((8, TB // 2, KH), u32),
            pltpu.SMEM((KPAIR * CP + 1,), jnp.int32),
            pltpu.SemaphoreType.DMA((9 + NCH,)),
        ],
        compiler_params=pltpu.CompilerParams(
            dimension_semantics=("arbitrary",),
            vmem_limit_bytes=110 * 1024 * 1024,
        ),
    )(xT, A_wqkv, A_wo, B_w_gate, B_w_up, wdT)
    return outT.T.reshape(B, S, D)
```

```python
import functools
import math
import jax
import jax.numpy as jnp
from jax import lax
import jax.experimental.pallas as pl
import jax.experimental.pallas.tpu as pltpu

H = 32
DH = 18
W = 8
DIL = 2
HALO = 16
EPS = 1e-5
TB = 128
TM = 256
NH = 2
RB = 8
KP = 640
KH = 256
KX = 192
KY = 64
NQKV = 14 * 128
TC = 128
CW = 3 * TC
NSLOT = 8
DG = int(3)
ROWS_LO = int(0)
WO_AT = int(6)
DLAG = int(1)
LN1_AT = int(7)
SERIAL = int(1)
SERIAL_A = int(0)
LN_F = tuple(int(x) for x in '2,4'.split(','))
LN_A = tuple(int(x) for x in '2,8'.split(','))
KPAIR = int(6)
CP = int(2)
QSPLIT = int(5)
XFIRST = 512
DGROUPS = tuple(int(x) for x in '4,4,2,2'.split(','))
DGROUPS_F = tuple(int(x) for x in '2,2,2'.split(','))
DORD = tuple(int(x) for x in '2,3,12,4,5,13,14,0,9,10,1,6,7,8,11'.split(','))
QB_AT = int(4); WOA_AT = int(-1)
LNA_AT = int(0); LNB_AT = int(2); WOB_AT = int(11)
QPR = 16
XNG = int(1); XNF = int(0)
SCRIPT = 'G,G,la+1400,G,lb+300,D2,G,G,G,ra+1400,G,D4,Q,WA,Q,Q,Q,G,G,G,rb+1400,G,D4,G,WB,S,D2'.split(',')
SDEAD = int(11)
QSP = int(1)
WOA_IN = int(1)
RA_T0 = int(7600); RA_PER = int(600); RB_T0 = int(6100); RB_PER = int(600)
LNA_T = int(2200); LNB_T = int(4500)
ONLY = ''
RA_AT = int(-1)
RBD = int(1)
DKEEP = int(2)
RESTAT = int(0)
TAILF = float(0.6)
LND = tuple(int(x) for x in '3,8'.split(','))
WOSPLIT = int(1)
NPACE = int(4)
MODE_F = tuple(int(x) for x in '1,3,1,0,0'.split(','))
MODE_A = tuple(int(x) for x in '1,3,1,0,0'.split(','))
FENCE = int(0)
PR = 32
PW1 = float(1); PW2 = float(1); PW3 = float(1)
SOPS_EARLY = int(1)
CLIP = int(0)

f32 = jnp.float32
bf16 = jnp.bfloat16
u32 = jnp.uint32
NT = (((1,), (1,)), ((), ()))


def _pk(x):
    return pltpu.bitcast(x.astype(bf16), u32)


def _unpk(u, idx):
    return pltpu.unpack_elementwise(u, index=idx, packed_dtype=bf16, unpacked_dtype=f32)


def _pk2(even, odd):
    return pltpu.pack_elementwise([even, odd], packed_dtype=bf16).astype(u32)


def _up(x):
    return pltpu.bitcast(x, bf16)


def _dot(a, b):
    return jnp.dot(a, b, preferred_element_type=f32)


def _dot_nt(a, b):
    return lax.dot_general(a, b, NT, preferred_element_type=f32)


def _ln_stats(x, NACC, pin=None):
    n = x.shape[0]
    c = x[0:1] if pin is None else pin(x[0:8])[0:1]
    s1 = [None] * NACC
    s2 = [None] * NACC
    for i in range(n // 8):
        d = x[i * 8:(i + 1) * 8] - c
        k = i % NACC
        s1[k] = d if s1[k] is None else s1[k] + d
        dd = d * d
        s2[k] = dd if s2[k] is None else s2[k] + dd
    while len(s1) > 1:
        s1 = [s1[i] + s1[i + 1] for i in range(0, len(s1), 2)]
        s2 = [s2[i] + s2[i + 1] for i in range(0, len(s2), 2)]
    m = jnp.sum(s1[0], axis=0, keepdims=True) * (1.0 / n)
    v = jnp.sum(s2[0], axis=0, keepdims=True) * (1.0 / n) - m * m
    v = jnp.maximum(v, 0.0)
    return c + m, lax.rsqrt(v + EPS)


def _tree(fn, xs):
    xs = list(xs)
    while len(xs) > 1:
        xs = [fn(xs[i], xs[i + 1]) for i in range(0, len(xs) - 1, 2)] + ([xs[-1]] if len(xs) % 2 else [])
    return xs[0]


def _lhs_ops(a11, a12, a21, a22):
    return (a11 + a22, a21 + a22, a11, a22, a11 + a12, a21 - a11, a12 - a22)


def _rhs_ops(b11, b12, b21, b22):
    return (b11 + b22, b11, b12 - b22, b21 - b11, b22, b11 + b12, b21 + b22)


_D_LHS = (
    ((0, 0, 1), (0, 2, -1), (1, 0, -1)), ((0, 0, 1), (0, 1, -1), (2, 0, -1)), ((1, 1, 1), (0, 1, -1), (1, 2, -1)),
    ((1, 1, 1), (1, 0, -1), (2, 1, -1)), ((2, 2, 1), (0, 2, -1), (2, 1, -1)), ((2, 2, 1), (1, 2, -1), (2, 0, -1)),
    ((0, 1, 1),), ((0, 1, 1), (1, 0, -1)), ((1, 0, 1),),
    ((0, 2, 1),), ((0, 2, 1), (2, 0, -1)), ((2, 0, 1),),
    ((1, 2, 1),), ((2, 1, 1), (1, 2, -1)), ((2, 1, 1),),
)
_D_OUT = {
    (0, 0): ((0, 1), (7, 1), (8, 1), (9, 1), (6, -1)),
    (0, 1): ((1, 1), (6, 1), (10, 1), (11, 1), (9, -1)),
    (1, 0): ((2, 1), (7, 1), (8, 1), (12, 1), (6, -1)),
    (1, 1): ((3, 1), (6, 1), (13, 1), (14, 1), (2, -1), (7, -1)),
    (2, 0): ((5, 1), (9, 1), (12, 1), (13, 1), (4, -1), (10, -1)),
    (2, 1): ((4, 1), (10, 1), (11, 1), (14, 1), (9, -1)),
}


def _d_rhs(b):
    s1 = b[1][0] + b[1][1]
    s2 = b[2][0] + b[2][1]
    t7 = b[0][1] + s1
    t10 = b[0][0] + s2
    return (b[0][0], b[0][1], b[1][0], s1, b[2][1], s2, b[0][1] + b[1][1], t7, b[0][0] + t7,
            b[0][0] + b[2][0], t10, b[0][1] + t10, b[1][0] + b[2][0], b[1][0] - b[2][1], b[1][1] + b[2][1])


def _signed_sum(terms):
    acc = None
    for v, sg in terms:
        if acc is None:
            assert sg == 1
            acc = v
        else:
            acc = acc + v if sg == 1 else acc - v
    return acc


def _dst_row(sec, d):
    if sec == 0:
        return d * 32 if d < 16 else 1024 + (d - 16) * 32
    if sec == 1:
        return 512 + d * 32 if d < 16 else 13 * 128 + (d - 16) * 32
    return 9 * 128 + d * 32 if d < 16 else 1024 + 64 + (d - 16) * 32


def _prep_plan(nchunk):
    plan = [[nchunk] * CP]
    nxt = 0
    for j in range(1, KPAIR):
        left_steps = KPAIR - 1 - j
        n = min(CP, nchunk - nxt)
        if j == 1:
            n = max(0, min(n, max(CP - 1, nchunk - nxt - left_steps * CP)))
        ids = list(range(nxt, nxt + n))
        nxt += n
        plan.append(ids + [nchunk] * (CP - n))
    return plan, nxt


def _kernel(x_hbm, wqkv_hbm, wo_hbm, wg_hbm, wu_hbm, wd_hbm, o_ref,
            xin, wqkv_raw, wo_raw, wqkvT, woT, raw, pw, tmp, qa, qb, xres, xn_f, xn1a, xn1b,
            s_scr, wq_s, xn_g, sq_scr, plan_s, sems, *, D, DF, NB):
    g = pl.program_id(0)
    NCH = DF // CW
    NPC = NCH // NH
    K = 2 * KPAIR
    S = NB * TB
    plan, nprepped = _prep_plan(NCH)
    zero8 = pl.multiple_of((g >> 20) * 8, 8)

    QSEC = ((0, 5), (5, 9), (9, 14))
    XPC = ((0, 256), (256, 512), (512, 1024), (1024, 1536), (1536, S))

    def cp_qkv(sec):
        out = []
        for j in range(*QSEC[sec]):
            n = min(128, 3 * D - j * 128)
            out.append(pltpu.make_async_copy(wqkv_hbm.at[:, pl.ds(j * 128, n)], wqkv_raw.at[:, pl.ds(j * 128, n)],
                                             sems.at[sec]))
        return out

    def cp_wo():
        return pltpu.make_async_copy(wo_hbm, wo_raw, sems.at[3])

    def cp_x(k):
        lo, hi = XPC[k]
        return pltpu.make_async_copy(x_hbm.at[:, pl.ds(lo, hi - lo)], xin.at[:, pl.ds(lo, hi - lo)], sems.at[4 + k])

    def chunk_copies(c):
        return [pltpu.make_async_copy(w.at[:, pl.ds(c * CW, CW)], raw.at[c, m], sems.at[9 + c])
                for m, w in enumerate((wg_hbm, wu_hbm, wd_hbm))]

    D3 = D // 3
    KR = D - 3 * TC
    R_TR = 15 * (TC // 2)
    R_SD = R_TR + 3 * (KR // 2)
    R_END = R_SD + 8 * (D3 // 2)

    def prep_pieces(c):
        def hk_piece(m, r):
            rb = D3 if m == 2 else TC
            blk = {}
            for i in range(3):
                for j in range(3):
                    u = pltpu.bitcast(raw[c, m, pl.ds(i * rb + r, 16), pl.ds(j * TC, TC)], u32)
                    blk[i, j] = (u, _unpk(u, 0), _unpk(u, 1))
            for k, terms in enumerate(_D_LHS):
                if len(terms) == 1:
                    t = blk[terms[0][:2]][0]
                else:
                    t = _pk2(_signed_sum([(blk[i, j][1], sg) for i, j, sg in terms]),
                             _signed_sum([(blk[i, j][2], sg) for i, j, sg in terms]))
                if m == 2:
                    pw[c, pl.ds(R_SD + (k // 2) * (D3 // 2) + r // 2, 8), (k % 2) * TC:(k % 2 + 1) * TC] = t
                else:
                    pw[c, pl.ds(k * (TC // 2) + r // 2, 8), m * TC:(m + 1) * TC] = t

        def rem_piece(m, j):
            pw[c, pl.ds(R_TR + j * (KR // 2), KR // 2), m * TC:(m + 1) * TC] = pltpu.bitcast(
                raw[c, m, pl.ds(3 * TC, KR), pl.ds(j * TC, TC)], u32)

        out = []
        for m in range(2):
            out += [functools.partial(hk_piece, m, r) for r in range(0, TC, 16)]
            out += [functools.partial(rem_piece, m, j) for j in range(3)]
        out += [functools.partial(hk_piece, 2, r) for r in range(0, D3, 16)]
        return out

    def prep_group(cs):
        out = []
        for c in cs:
            out += prep_pieces(c)
        return out

    class Pacer:
        def __init__(self, pieces, pace, npts, idle=0):
            self.pieces, self.pace, self.n, self.pt, self.done = pieces, pace, npts - idle, 0, 0

        def __call__(self, v):
            self.pt += 1
            upto = min(len(self.pieces), int(round(len(self.pieces) * self.pt / self.n)))
            if upto > self.done or self.pt == self.n + 1:
                self.pace(v)
            for piece in self.pieces[self.done:upto]:
                piece()
            self.done = upto

    def pace_wq(v):
        wq_s[pl.ds(NQKV // 4 + zero8, 8), 0:128] = pltpu.bitcast(v, u32)

    def pace_pwz(v):
        pw[NCH, pl.ds(R_END + zero8, 8), 0:128] = pltpu.bitcast(v, u32)

    def pace_pw(v):
        pw[NCH, pl.ds(R_END, 8), 0:128] = pltpu.bitcast(v, u32)

    nr = TB // RB
    QT = (0, 1, 2, 3, 8)
    KT = (4, 5, 6, 7, 13)
    VT = (9, 10, 11, 12, 8)
    scale = DH ** -0.5
    c2e = scale * math.log2(math.e)
    neg = -1e9 * math.log2(math.e)
    k0 = math.sqrt(2.0 / math.pi)
    k1 = k0 * 0.044715

    zvec = jnp.full((RB, 128), (g >> 20).astype(u32), u32)

    def tie(x, dep):
        return pltpu.bitcast(pltpu.bitcast(x, u32) | (pltpu.bitcast(dep, u32) & zvec), f32)

    def normalize(blk, mean, rstd, link):
        if not link:
            return (xres[blk] - mean) * rstd
        rs = jnp.broadcast_to(rstd, (8, TB))
        mb = jnp.broadcast_to(mean, (8, TB))
        outs = []
        for i in range(D // 8):
            if i and i % link == 0:
                rs = tie(rs, outs[-1])
            outs.append((xres[blk, pl.ds(i * 8, 8), :] - mb) * rs)
        return jnp.concatenate(outs, axis=0)

    def x_convert(blk):
        x = xin[:, pl.ds(pl.multiple_of(blk * TB, TB), TB)].astype(f32)
        xres[blk] = x
        return x

    def a_ln1(blk, dst, from_input):
        x = x_convert(blk) if from_input else xres[blk]
        mean, rstd = _ln_stats(x, LN_A[0])
        if not from_input:
            dst[pl.ds(0, 8), :] = jnp.zeros((8, KP), u32)
        xn = (xres[blk] - mean) * rstd
        xp = jnp.concatenate([xn, jnp.zeros((KP - D, TB), f32)], axis=0)
        dst[...] = pltpu.bitcast(xp.astype(bf16).T, u32)

    def a_qkv(src, qdst, qprev, t0=0, t1=14, cb=None):
        qkv = _dot_nt(_up(src[...]), _up(wqkvT[pl.ds(t0 * 64, (t1 - t0) * 64), :]))
        for t in range(max(t0, 4), t1):
            qdst[t, pl.ds(0, HALO), :] = qprev[t, pl.ds(TB, HALO), :]
        for t in range(t0, t1):
            qdst[t, pl.ds(HALO, TB), :] = qkv[:, (t - t0) * 128:(t - t0 + 1) * 128]
            if cb is not None:
                for k in range(NPACE):
                    rr = k * (TB // NPACE)
                    cb(qkv[rr:rr + 8, (t - t0) * 128:(t - t0 + 1) * 128])

    cbits = pltpu.bitcast(jnp.full((RB, 128), c2e, f32), u32)

    def tied_scale(deps):
        if not deps:
            return c2e
        acc = pltpu.bitcast(deps[0], u32)
        for dv in deps[1:]:
            acc = acc | pltpu.bitcast(dv, u32)
        return pltpu.bitcast(cbits | (acc & zvec), f32)

    def a_rows(q_s, blk, rs, mode, hist, start=None, sink=False):
        lag_mid, lag_end, midkind, fw, fv = mode
        for r in rs:
            r0 = r * RB
            deps = [start] if (start is not None and r == rs[0]) else []
            if lag_mid and r - lag_mid >= 0:
                deps.append(hist[('h' if midkind else 'm', r - lag_mid)])
            if lag_end and r - lag_end >= 0:
                deps += hist[('o', r - lag_end)]
            cs = tied_scale(deps)
            q = [q_s[t, pl.ds(HALO + r0, RB), :] * cs for t in QT]
            sc = []
            q0 = q[0]
            prev = None
            for w in range(W):
                off = HALO + r0 - DIL * w
                acc = None
                if fw and w and w % fw == 0:
                    q0 = tie(q[0], prev)
                for j, t in enumerate(KT):
                    p = (q0 if j == 0 else q[j]) * q_s[t, pl.ds(off, RB), :]
                    acc = p if acc is None else acc + p
                prev = acc
                acc = acc + pltpu.roll(acc, 64, 1)
                hist[('h', r)] = acc
                acc = acc + pltpu.roll(acc, 32, 1)
                if r0 - DIL * w < 0:
                    pos = blk * TB + r0 + lax.broadcasted_iota(jnp.int32, (RB, 128), 0)
                    acc = jnp.where(pos >= DIL * w, acc, neg)
                sc.append(acc)
            m = _tree(jnp.maximum, sc)
            hist[('m', r)] = m
            e = [jnp.exp2(sc[w] - m) for w in range(W)]
            l = _tree(jnp.add, e)
            rinv = pl.reciprocal(l, approx=True)
            rinv = rinv * (2.0 - l * rinv)
            outs = []
            e0 = e[0]
            for j, t in enumerate(VT):
                if fv and j and j % fv == 0:
                    e0 = tie(e[0], acc)
                acc = None
                for w in range(W):
                    off = HALO + r0 - DIL * w
                    p = (e0 if w == 0 else e[w]) * q_s[t, pl.ds(off, RB), :]
                    acc = p if acc is None else acc + p
                o = acc * rinv
                st_off = r0 + zero8 if (j == 4 and r == nr - 1 and FENCE and not sink) else r0
                q_s[14 + j, pl.ds(st_off, RB), :] = o
                outs.append(o)
            hist[('o', r)] = outs[-1:] if fv == 1 else outs
            if sink:
                q_s[19, pl.ds(r0, RB), :] = outs[-1]

    def a_wo(q_s, blk, par, ln, cb=None):
        if WOSPLIT:
            o4 = q_s[18, pl.ds(0, TB), :].astype(bf16)
            rq = D // 8
            y = jnp.concatenate([_dot_nt(_up(woT[pl.ds(k * rq, rq), 512:640]), o4) for k in range(4)], axis=0)
            o = jnp.concatenate([q_s[14 + j, pl.ds(0, TB), :] for j in range(4)], axis=1).astype(bf16)
            x1 = _dot_nt(_up(woT[:, 0:512]), o) + (xres[blk] + y)
        else:
            o = jnp.concatenate([q_s[14 + j, pl.ds(0, TB), :] for j in range(5)], axis=1).astype(bf16)
            x1 = xres[blk] + _dot_nt(_up(woT[...]), o)
        xres[blk] = x1
        if cb is not None:
            for i in range(0, D, 16):
                cb(x1[i:i + 8])
        mean, rstd = _ln_stats(x1, ln[0])
        xn_f[par, pl.ds(zero8 if XNF else 0, D), :] = normalize(blk, mean, rstd, ln[1])

    def sops(src, put):
        def seg(tb, r0, n):
            return lambda: src[tb, pl.ds(r0, n), :]
        A11, A12, A21, A22 = seg(0, 0, KX), seg(0, KH, KX), seg(1, 0, KX), seg(1, KH, KX)
        a11, a12, a21, a22 = seg(0, KX, KY), seg(0, KH + KX, KY), seg(1, KX, KY), seg(1, KH + KX, KY)
        rt, rb = seg(0, 2 * KH, KY), seg(1, 2 * KH, KY)
        parts = (
            lambda: (A21() + A22(), -(a21() + a22())),
            lambda: (A11(), -a22()),
            lambda: (A22(), -a11()),
            lambda: (A11() + A12(), -(a11() + a12())),
            lambda: (A12() - A22(), rt()),
            lambda: (A21() - A11(), rb()),
            lambda: (rt(), a12() - a22(), rb(), a21() - a11()),
            lambda: (A11() + A22(), a11() + a22()),
        )
        for i, fn in enumerate(parts):
            t = jnp.concatenate(fn(), axis=0)
            put(i, pltpu.bitcast(t.astype(bf16).T, u32))

    def sops15(put):
        def X(t, r0, n):
            return xn_f[t, pl.ds(r0, n), :]
        for n in range(15):
            terms = [(i, t, sg) for (i, t), lst in _D_OUT.items() for k, sg in lst if k == n]
            terms.sort(key=lambda z: -z[2])
            v = _signed_sum([(X(t, i * TC, TC), sg) for i, t, sg in terms])
            put(n, pltpu.bitcast(v.astype(bf16).T, u32))
        k1, k2, k3 = 3 * TC, 3 * TC + KY, 3 * TC + 2 * KY
        trick = ((lambda: (X(0, k1, KY), X(0, k2, KY) - X(1, k2, KY))),
                 (lambda: (X(1, k1, KY), X(1, k3, KY) - X(0, k3, KY))),
                 (lambda: (X(1, k2, KY), X(0, k3, KY))))
        for n, fn in enumerate(trick):
            put(15 + n, pltpu.bitcast(jnp.concatenate(fn(), axis=0).astype(bf16).T, u32))

    def a_sops(slot):
        def put(i, v):
            s_scr[slot, i] = v
        sops15(put)

    NQH = NQKV // 4

    def q_prep_pieces():
        lo = lax.broadcasted_iota(jnp.int32, (QPR, 128), 1) < 64

        def piece(r):
            def ld(half, t):
                u = wqkvT[pl.ds(half * NQH + r, QPR), t * 128:(t + 1) * 128]
                return u, _unpk(u, 0), _unpk(u, 1)

            def add(u, v):
                return _pk2(u[1] + v[1], u[2] + v[2])

            def sub(u, v):
                return _pk2(u[1] - v[1], u[2] - v[2])

            def put(tile, v):
                wq_s[pl.ds(r, QPR), tile * 128:(tile + 1) * 128] = v
            r1, r2 = wqkvT[pl.ds(r, QPR), 512:640], wqkvT[pl.ds(NQH + r, QPR), 512:640]
            zero = jnp.zeros((QPR, 128), u32)
            for t in range(2):
                x1, x2, y1, y2 = ld(0, t), ld(1, t), ld(0, 2 + t), ld(1, 2 + t)
                put(2 + t, sub(x2, y2))
                put(4 + t, sub(y1, x1))
                sy, sx, d1 = add(y1, y2), add(x1, x2), add(x1, y2)
                if t == 0:
                    put(0, x1[0])
                    put(6, y2[0])
                    put(8, sy)
                    put(10, sx)
                    put(14, d1)
                else:
                    put(1, jnp.where(lo, x1[0], x2[0]))
                    put(7, jnp.where(lo, y2[0], y1[0]))
                    put(9, jnp.where(lo, sy, r1))
                    put(11, jnp.where(lo, sx, r2))
                    put(12, jnp.where(lo, r2, sy))
                    put(13, jnp.where(lo, r1, sx))
                    put(15, jnp.where(lo, d1, zero))
                    put(16, jnp.where(lo, zero, add(x2, y1)))
        return [functools.partial(piece, r) for r in range(0, NQH, QPR)]

    def a_ln1f(blk, par, dep=None):
        mean, rstd = _ln_stats(xres[blk], LN_F[0], None if dep is None else (lambda v: tie(v, dep)))
        xn_g[par, pl.ds(0, 8), :] = jnp.zeros((8, TB), f32)
        xn_g[par, pl.ds(zero8 if XNG else 0, D), :] = normalize(blk, mean, rstd, LN_F[1])

    def a_qsops():
        def put(i, v):
            sq_scr[i, pl.ds(zero8, TB // 2), :] = v
        sops(xn_g, put)

    def a_qkv2_halo(qtop, qbot):
        for t in range(4, 14):
            qtop[t, pl.ds(0, HALO), :] = qbot[t, pl.ds(TB, HALO), :]

    def a_qkv2(qtop, qbot, t0, nt):
        def Q(slot, l0, l1, w0):
            lhs = _up(sq_scr[slot, :, l0:l1])
            rhs = _up(wq_s[pl.ds(t0 * 64, nt * 64), w0 * 128:w0 * 128 + (l1 - l0)])
            if QSP and nt == 1 and l1 - l0 == 128:
                return jnp.concatenate([_dot_nt(_up(sq_scr[slot, pl.ds(k * 16, 16), l0:l1]), rhs) for k in range(4)],
                                       axis=0)
            return _dot_nt(lhs, rhs)

        def out(dst, tb, v):
            for k in range(nt):
                dst[tb + k, pl.ds(HALO, TB), :] = v[:, k * 128:(k + 1) * 128]
                if dst is qtop and tb + k >= 4:
                    qbot[tb + k, pl.ds(0, HALO), :] = v[TB - HALO:, k * 128:(k + 1) * 128]
        q5 = Q(3, 0, KH, 6)
        q3 = Q(1, 0, KH, 2)
        q1b = Q(7, 128, KH, 16)
        out(qtop, t0 + 7, q3 + q5 + q1b + Q(6, 0, 128, 12))
        q4 = Q(2, 0, KH, 4)
        q2 = Q(0, 0, KH, 0)
        out(qbot, t0, q2 + q4 + q1b + Q(6, 128, KH, 13))
        q1 = Q(7, 0, KH, 14)
        out(qtop, t0, q1 + q4 - q5 + Q(4, 0, KH, 8))
        out(qbot, t0 + 7, q1 - q2 + q3 + Q(5, 0, KH, 10))

    class St:
        pass

    class Timeline:
        def __init__(self):
            self.t = 0
            self.jobs = []

        def add(self, when, fn):
            self.jobs.append((when, fn))
            self.jobs.sort(key=lambda z: z[0])

        def tick(self, dur, v):
            self.t += dur
            if self.jobs and self.jobs[0][0] <= self.t:
                self.jobs.pop(0)[1](v[0:8, 0:128])

        def flush(self, upto=None):
            assert not [j for j in self.jobs if upto is None or j[0] < upto], (self.t, [j[0] for j in self.jobs])

    def f_init(st, j):
        st.c0 = 0
        st.b0 = (j * NH) % NB
        st.sb = j % NSLOT
        st.acc = [None] * 15
        st.tl = Timeline()
        st.sdep = None
        st.t = {}

    def gelu_mul(c):
        gg = c[:, :TC]
        u = c[:, TC:]
        t = jnp.tanh(gg * (k0 + k1 * (gg * gg)))
        gu = gg * u
        return gu + gu * t

    def f_gu(st, p):
        c = st.c0 + p
        hk = KY // 2

        def L(n):
            return s_scr[st.sb, n]

        def R(n):
            return pw[c, pl.ds(n * (TC // 2), TC // 2), :]

        def RT(j, kind):
            r0 = R_TR + j * (KR // 2)
            if kind == 1:
                return jnp.concatenate([pw[c, pl.ds(r0, hk), :], pw[c, pl.ds(r0 + 2 * hk, hk), :]], axis=0)
            return pw[c, pl.ds(r0 + (hk if kind == 2 else 0), 2 * hk), :]

        def P(n):
            return _dot(_up(L(n)), _up(R(n)))

        def T(j, kind):
            return _dot(_up(L(15 + kind)), _up(RT(j, kind)))

        def PT(n, j, kind):
            return _dot(_up(jnp.concatenate([L(n), L(15 + kind)], axis=1)),
                        _up(jnp.concatenate([R(n), RT(j, kind)], axis=0)))
        tk = st.tl.tick
        p8 = P(8)
        t7 = P(7) + p8
        st.first = t7[0:8, 0:128]
        tk(128, t7)
        s1 = PT(3, 1, 2) + t7
        tk(128, s1)
        p6 = P(6)
        p14 = P(14)
        tk(128, p14)
        h11 = gelu_mul(T(1, 1) + (p6 + p14 + s1))
        p12 = P(12)
        tk(128, p12)
        p13 = P(13)
        h10 = gelu_mul(PT(2, 1, 0) + (p12 + p13 + s1))
        tk(192, h10)
        p11 = P(11)
        t10 = P(10) + p11
        tk(128, t10)
        s2 = PT(5, 2, 2) + t10
        tk(128, s2)
        p9 = P(9)
        h20 = gelu_mul(T(2, 0) + (p9 + p12 + s2))
        tk(128, h20)
        h21 = gelu_mul(PT(4, 2, 1) + (p14 - p13 + s2))
        w0 = T(0, 2)
        tk(192, w0)
        h00 = gelu_mul(PT(0, 0, 0) + (p8 + p9 + t10 + w0))
        tk(128, h00)
        h01 = gelu_mul(PT(1, 0, 1) + (p6 + p11 + t7 + w0))
        tk(128, h01)
        st.t[p] = ((h00, h01), (h10, h11), (h20, h21))

    def f_d(st, ps):
        rhs = [_d_rhs(st.t.pop(p)) for p in ps]
        for pos, i in enumerate(DORD):
            au = [pw[st.c0 + p, pl.ds(R_SD + (i // 2) * (D3 // 2), D3 // 2), (i % 2) * TC:(i % 2 + 1) * TC] for p in ps]
            if st.sdep is not None and pos == SDEAD:
                probe = s_scr[st.sdep, 17, pl.ds(zero8, 8), :]
                au[0] = jnp.concatenate([au[0][0:8] | (probe & zvec), au[0][8:]], axis=0)
                st.sdep = None
            a = jnp.concatenate([_up(v) for v in au], axis=1)
            t = jnp.concatenate([r[i] for r in rhs], axis=1).astype(bf16)
            r = _dot_nt(a, t)
            st.acc[i] = r if st.acc[i] is None else r + st.acc[i]
            st.tl.tick(48 * len(ps), st.acc[i])

    def f_store(st):
        for k in range(NH):
            y = jnp.concatenate([_signed_sum([(st.acc[n], sg) for n, sg in _D_OUT[i, k]]) for i in range(3)], axis=0)
            x2 = xres[st.b0 + k] + 0.5 * y
            xres[st.b0 + k] = x2
            o_ref[:, k * TB:(k + 1) * TB] = x2.astype(o_ref.dtype)

    def run_pair(jf, ja):
        st = St()
        f_init(st, jf)
        a = (2 * ja) % NB
        b = a + 1
        tl = st.tl

        def lnb(dep):
            a_ln1f((a + 2) % NB, 1, dep)
            a_qsops()
        jobs = {
            'ra': lambda dep: a_rows(qa, a, range(nr), MODE_F, {}, dep),
            'rb': lambda dep: a_rows(qb, b, range(nr), MODE_F, {}, dep),
            'la': lambda dep: a_ln1f(b, 0, dep),
            'lb': lnb,
        }
        qchunks = [(0, 2), (2, 2), (4, 2), (6, 1)]
        pg = pd = 0
        for tok in SCRIPT:
            if tok == 'G':
                f_gu(st, pg)
                pg += 1
            elif tok[0] == 'D':
                n = int(tok[1:])
                f_d(st, list(range(pd, pd + n)))
                pd += n
            elif tok == 'Q':
                if len(qchunks) == 4:
                    tl.flush()
                    a_qkv2_halo(qb, qa)
                t0, nt = qchunks.pop(0)
                a_qkv2(qb, qa, t0, nt)
                tl.t += 544 * nt
            elif tok == 'WA':
                tl.flush()
                a_wo(qa, a, 0, LN_F)
                tl.t += 720
            elif tok == 'WB':
                tl.flush()
                a_wo(qb, b, 1, LN_F)
                tl.t += 720
            elif tok == 'S':
                a_sops(ja % NSLOT)
                st.sdep = (ja % NSLOT) if SDEAD >= 0 else None
            else:
                name, _, dt = tok.partition('+')
                tl.add(tl.t + int(dt or 0), jobs[name])
        assert pg == NCH and pd == NCH and not qchunks
        tl.flush()
        f_store(st)

    def run_aa(j):
        a = 2 * j
        b = a + 1
        pieces = prep_group([plan_s[j * CP + k] for k in range(CP)])
        cb = Pacer(pieces, pace_pw, 28 * NPACE, NPACE)
        a_rows(qa, a, range(nr), MODE_A, {})
        a_wo(qb, jnp.where(j == 0, NB, a - 1), 1, LN_A)
        a_sops(jnp.where(j == 0, NSLOT, j - 1))
        a_ln1(a + 2, xn1a, True)
        a_qkv(xn1b, qb, qa, cb=cb)
        a_rows(qb, b, range(nr), MODE_A, {})
        a_wo(qa, a, 0, LN_A)
        a_ln1(b + 2, xn1b, True)
        a_qkv(xn1a, qa, qb, cb=cb)
        assert cb.done == len(pieces)

    def start_rest():
        cp_wo().start()
        cp_x(1).start()
        cp_x(2).start()
        for c in range(NCH):
            for cp in chunk_copies(c):
                cp.start()
            if c == 2:
                cp_x(3).start()
            if c == 6:
                cp_x(4).start()

    def qkv_section(sec):
        for cp in cp_qkv(sec):
            cp.wait()
        if sec == RESTAT:
            start_rest()
        for j in range(*QSEC[sec]):
            wd_ = min(128, 3 * D - j * 128)
            blk = wqkv_raw[:, j * 128:j * 128 + wd_].astype(f32)
            if wd_ < 128:
                blk = jnp.concatenate([blk, jnp.zeros((D, 128 - wd_), f32)], axis=1)
            bt = jnp.concatenate([blk, blk[2 * KH:]], axis=0).T
            for t in range(5):
                tmp[t, pl.ds(j * 128, 128), :] = bt[:, t * 128:(t + 1) * 128]
        for d in range(DH):
            r = _dst_row(sec, d)
            for t in range(5):
                wqkvT[pl.ds(r // 2, 16), t * 128:(t + 1) * 128] = _pk2(
                    tmp[t, pl.ds(sec * D + d, 16, stride=2 * DH), :],
                    tmp[t, pl.ds(sec * D + d + DH, 16, stride=2 * DH), :])

    @pl.when(g == 0)
    def _():
        if ONLY:
            return
        cp_x(0).start()
        for sec in range(3):
            for cp in cp_qkv(sec):
                cp.start()
        if RESTAT < 0:
            start_rest()
        for j in range(KPAIR):
            for k in range(CP):
                plan_s[j * CP + k] = plan[j][k]
        qb[:, pl.ds(TB, HALO), :] = jnp.zeros((20, HALO, 128), f32)
        wqkvT[pl.ds((13 * 128 + 64) // 2, 32), :] = jnp.zeros((32, KP), u32)
        zpad = jnp.zeros((KP - D, 128), f32)
        cp_x(0).wait()
        a_ln1(0, xn1a, True)
        a_ln1(1, xn1b, True)
        qkv_section(0)
        a_qkv(xn1a, qa, qb, 0, 4)
        qkv_section(1)
        a_qkv(xn1a, qa, qb, 4, 8)
        qkv_section(2)
        cp_wo().wait()
        cb = Pacer(q_prep_pieces(), pace_wq, 6 * NPACE)
        a_qkv(xn1a, qa, qb, 8, 14, cb=cb)
        for t in range(5):
            wd_ = 128 if t < 4 else 64
            blk = wo_raw[:, t * 128:t * 128 + wd_].astype(f32)
            if wd_ < 128:
                blk = jnp.concatenate([blk, jnp.zeros((D, 128 - wd_), f32)], axis=1)
            tmp[t, pl.ds(0, D), :] = blk
        for t in range(5):
            rows = [tmp[t, pl.ds(d, 32, stride=DH), :] for d in range(DH)]
            full = jnp.concatenate(rows[:16] + [zpad] + rows[16:], axis=0)
            ft = full.T
            n = 128 if t < 4 else 64
            woT[pl.ds(t * 64, n // 2), :] = _pk(ft[:n])
        cp_x(1).wait()

    for j in range(1, KPAIR):
        @pl.when(g == 1 + j)
        def _():
            if j % 2 == 1:
                cp_x(2 + j // 2).wait()
            for c in plan[j]:
                if c < NCH:
                    for cp in chunk_copies(c):
                        cp.wait()

    @pl.when(jnp.logical_and(g >= 1, g <= KPAIR))
    def _():
        if ONLY in ('', 'aa'):
            run_aa(g - 1)

    @pl.when(g == KPAIR + 1)
    def _():
        if ONLY:
            return
        pieces = []
        for c in range(nprepped, NCH):
            for cp in chunk_copies(c):
                cp.wait()
        pieces += prep_group(range(nprepped, NCH))
        n1 = int(len(pieces) * TAILF)
        cb = Pacer(pieces[:n1], pace_pwz, D // 16)
        a_wo(qb, K - 1, 1, (4, 0), cb=cb)

        cb2 = Pacer(pieces[n1:], pace_pwz, 18)

        def put(i, v):
            s_scr[KPAIR - 1, i] = v
            cb2(pltpu.bitcast(v[0:8, 0:128], f32))
        sops15(put)
        for blk in range(K + 2, NB):
            x_convert(blk)

    jf = g - (KPAIR + 1)

    @pl.when(jnp.logical_and(jf >= 0, jf < NB - KPAIR))
    def _():
        if ONLY in ('', 'pair'):
            run_pair(jf, jf + KPAIR)

    @pl.when(jf >= NB - KPAIR)
    def _():
        def body(hf, carry):
            st = St()
            f_init(st, jf)
            st.c0 = hf * NPC
            groups = []
            p0 = 0
            for n in DGROUPS_F:
                groups.append(list(range(p0, p0 + n)))
                p0 += n
            for p in range(NPC):
                f_gu(st, p)
                while groups and len(groups) > DKEEP and groups[0][-1] + DLAG <= p:
                    f_d(st, groups.pop(0))
            while groups:
                f_d(st, groups.pop(0))
            f_store(st)
            return carry
        if ONLY in ('', 'f'):
            lax.fori_loop(0, NH, body, 0)


@jax.jit
def pallas_interleave_layers__sliding_local_dilated__glu_gated_geglu__prompt_kernel(
    A_x, A_wqkv, A_wo, B_x, B_w_gate, B_w_up, B_w_down):
    B, S, D = A_x.shape
    DF = B_w_gate.shape[1]
    NB = S // TB
    xT = A_x.reshape(S, D).T
    wdT = B_w_down.T
    NCH = DF // CW
    nsteps = 1 + KPAIR + NB
    hbm = pl.BlockSpec(memory_space=pltpu.HBM)
    outT = pl.pallas_call(
        functools.partial(_kernel, D=D, DF=DF, NB=NB),
        grid=(nsteps,),
        in_specs=[hbm] * 6,
        out_specs=pl.BlockSpec((D, TM), lambda g: (0, jnp.maximum(g - (1 + KPAIR + NB // 2), 0))),
        out_shape=jax.ShapeDtypeStruct((D, S), A_x.dtype),
        scratch_shapes=[
            pltpu.VMEM((D, S), bf16),
            pltpu.VMEM((D, 3 * D), bf16),
            pltpu.VMEM((D, D), bf16),
            pltpu.VMEM((NQKV // 2, KP), u32),
            pltpu.VMEM((D // 2, KP), u32),
            pltpu.VMEM((NCH + 1, 3, D, CW), bf16),
            pltpu.VMEM((NCH + 1, 15 * (TC // 2) + 3 * (D - CW) // 2 + 8 * (D // 6) + 16, 2 * TC), u32),
            pltpu.VMEM((5, NQKV, 128), f32),
            pltpu.VMEM((20, HALO + TB, 128), f32),
            pltpu.VMEM((20, HALO + TB, 128), f32),
            pltpu.VMEM((NB + 1, D, TB), f32),
            pltpu.VMEM((2, D, TB), f32),
            pltpu.VMEM((TB // 2, KP), u32),
            pltpu.VMEM((TB // 2, KP), u32),
            pltpu.VMEM((NSLOT + 1, 18, TB // 2, TC), u32),
            pltpu.VMEM((NQKV // 4 + 32, 17 * 128), u32),
            pltpu.VMEM((2, D, TB), f32),
            pltpu.VMEM((8, TB // 2, KH), u32),
            pltpu.SMEM((KPAIR * CP + 1,), jnp.int32),
            pltpu.SemaphoreType.DMA((9 + NCH,)),
        ],
        compiler_params=pltpu.CompilerParams(
            dimension_semantics=("arbitrary",),
            vmem_limit_bytes=110 * 1024 * 1024,
        ),
    )(xT, A_wqkv, A_wo, B_w_gate, B_w_up, wdT)
    return outT.T.reshape(B, S, D)
```

```python
import functools
import math
import jax
import jax.numpy as jnp
from jax import lax
import jax.experimental.pallas as pl
import jax.experimental.pallas.tpu as pltpu

H = 32
DH = 18
W = 8
DIL = 2
HALO = 16
EPS = 1e-5
TB = 128
RB = 8
TC = 128
CW = 3 * TC
KY = 64
ONLY = ''
LN_P = tuple(int(x) for x in '1,2'.split(','))
CFG_Q1 = tuple(int(x) for x in '1,4,60,560'.split(','))
CFG_Q2 = tuple(int(x) for x in '1,2,60,560'.split(','))
QP0 = int(200); QP1 = int(3360); QTK = int(4)
MODE_P = tuple(int(x) for x in '1,3'.split(','))
MODE_A = tuple(int(x) for x in '1,3'.split(','))
SCRIPT = 'G,G,G,G,ra+1540,G,D4,X,G,G,G,rb+1540,G,D4,X,G,G,Y+1200,G,W,S,D4'.split(',')
SCRIPT_F = 'G,G,G,D2,G,G,G,D2,D2'.split(',')
DORD = tuple(int(x) for x in '2,3,12,4,5,13,14,0,9,10,1,6,7,8,11'.split(','))
SDEAD = int(11)
PLAN = tuple(int(x) for x in '0,0,2,2,2,1,2,2'.split(','))
CP = 2
CFG_QA = tuple(int(x) for x in '1,4,60,560'.split(','))
QA_T = tuple(int(x) for x in '10,100'.split(','))
QA_DEAD = int(10)
QPAD = int(40)
LNSER = int(0); XNF = int(0)
WORD = tuple(int(x) for x in '6,7,8,9,0,10,11,1,2,12,13,14,3,4,5'.split(','))
A0_AFTER = int(1)

f32 = jnp.float32
bf16 = jnp.bfloat16
u32 = jnp.uint32
NT = (((1,), (1,)), ((), ()))


def _unpk(u, idx):
    return pltpu.unpack_elementwise(u, index=idx, packed_dtype=bf16, unpacked_dtype=f32)


def _pk2(even, odd):
    return pltpu.pack_elementwise([even, odd], packed_dtype=bf16).astype(u32)


def _up(x):
    return pltpu.bitcast(x, bf16)


def _dot(a, b):
    return jnp.dot(a, b, preferred_element_type=f32)


def _dot_nt(a, b):
    return lax.dot_general(a, b, NT, preferred_element_type=f32)


def _tree(fn, xs):
    xs = list(xs)
    while len(xs) > 1:
        xs = [fn(xs[i], xs[i + 1]) for i in range(0, len(xs) - 1, 2)] + ([xs[-1]] if len(xs) % 2 else [])
    return xs[0]


def _ln_stats(x, nacc, pin=None):
    n = x.shape[0]
    c = x[0:1] if pin is None else pin(x[0:8])[0:1]
    s1 = [None] * nacc
    s2 = [None] * nacc
    for i in range(n // 8):
        d = x[i * 8:(i + 1) * 8] - c
        k = i % nacc
        s1[k] = d if s1[k] is None else s1[k] + d
        dd = d * d
        s2[k] = dd if s2[k] is None else s2[k] + dd
    m = jnp.sum(_tree(jnp.add, s1), axis=0, keepdims=True) * (1.0 / n)
    v = jnp.sum(_tree(jnp.add, s2), axis=0, keepdims=True) * (1.0 / n) - m * m
    v = jnp.maximum(v, 0.0)
    return c + m, lax.rsqrt(v + EPS)


_HK_A = (
    ((0, 0, 1), (0, 2, -1), (1, 0, -1)), ((0, 0, 1), (0, 1, -1), (2, 0, -1)), ((1, 1, 1), (0, 1, -1), (1, 2, -1)),
    ((1, 1, 1), (1, 0, -1), (2, 1, -1)), ((2, 2, 1), (0, 2, -1), (2, 1, -1)), ((2, 2, 1), (1, 2, -1), (2, 0, -1)),
    ((0, 1, 1),), ((0, 1, 1), (1, 0, -1)), ((1, 0, 1),),
    ((0, 2, 1),), ((0, 2, 1), (2, 0, -1)), ((2, 0, 1),),
    ((1, 2, 1),), ((2, 1, 1), (1, 2, -1)), ((2, 1, 1),),
)
_HK_C = {
    (0, 0): ((0, 1), (7, 1), (8, 1), (9, 1), (6, -1)),
    (0, 1): ((1, 1), (6, 1), (10, 1), (11, 1), (9, -1)),
    (1, 0): ((2, 1), (7, 1), (8, 1), (12, 1), (6, -1)),
    (1, 1): ((3, 1), (6, 1), (13, 1), (14, 1), (2, -1), (7, -1)),
    (2, 0): ((5, 1), (9, 1), (12, 1), (13, 1), (4, -1), (10, -1)),
    (2, 1): ((4, 1), (10, 1), (11, 1), (14, 1), (9, -1)),
}


def _hk_b(b):
    s1 = b[1][0] + b[1][1]
    s2 = b[2][0] + b[2][1]
    t7 = b[0][1] + s1
    t10 = b[0][0] + s2
    return (b[0][0], b[0][1], b[1][0], s1, b[2][1], s2, b[0][1] + b[1][1], t7, b[0][0] + t7,
            b[0][0] + b[2][0], t10, b[0][1] + t10, b[1][0] + b[2][0], b[1][0] - b[2][1], b[1][1] + b[2][1])


def _ssum(terms):
    terms = sorted([t for t in terms if t[0] is not None], key=lambda z: -z[1])
    if not terms:
        return None
    acc = terms[0][0] if terms[0][1] == 1 else -terms[0][0]
    for v, sg in terms[1:]:
        acc = acc + v if sg == 1 else acc - v
    return acc


class _Timeline:
    def __init__(self):
        self.t = 0
        self.jobs = []

    def add(self, when, fn):
        self.jobs.append((when, len(self.jobs), fn))
        self.jobs.sort(key=lambda z: z[:2])

    def tick(self, dur, v, n=1):
        for k in range(n):
            self.t += dur // n
            r = k * (v.shape[0] // n)
            while self.jobs and self.jobs[0][0] <= self.t:
                self.jobs.pop(0)[2](v[r:r + 8, 0:128])


def _kernel(x_hbm, wqkv_hbm, wo_hbm, wg_hbm, wu_hbm, wd_hbm, o_ref,
            xin, wqkv_raw, wo_raw, tmp, wq, woT, wo2, raw, pw, qall, o_s, xres, xn_f, xn_g, s_scr, sq_scr,
            plan_s, sems, *, D, DF, S):
    g = pl.program_id(0)
    NB = S // TB
    NP = NB // 2
    NCH = DF // CW
    NPC = NCH // 2
    D3 = D // 3
    DHALF = D // 2
    KR = D - 3 * TC
    nr = TB // RB
    zero8 = pl.multiple_of((g >> 20) * 8, 8)
    zvec = jnp.full((8, 128), (g >> 20).astype(u32), u32)

    def tie(x, dep):
        return pltpu.bitcast(pltpu.bitcast(x, u32) | (pltpu.bitcast(dep, u32) & zvec), f32)

    QSEC = ((0, 5), (5, 9), (9, 14))

    def cp_qkv(sec):
        out = []
        for j in range(*QSEC[sec]):
            n = min(128, 3 * D - j * 128)
            out.append(pltpu.make_async_copy(wqkv_hbm.at[:, pl.ds(j * 128, n)], wqkv_raw.at[:, pl.ds(j * 128, n)],
                                             sems.at[sec]))
        return out

    def cp_wo():
        return pltpu.make_async_copy(wo_hbm, wo_raw, sems.at[3])

    def cp_x(k):
        return pltpu.make_async_copy(x_hbm.at[:, pl.ds(k * 2 * TB, 2 * TB)], xin.at[k], sems.at[4 + k])

    def cp_chunk(c):
        return [pltpu.make_async_copy(w.at[:, pl.ds(c * CW, CW)], raw.at[c, m], sems.at[4 + NP + c])
                for m, w in enumerate((wg_hbm, wu_hbm, wd_hbm))]

    R_TR = 15 * (TC // 2)
    R_SD = R_TR + 3 * (KR // 2)
    R_END = R_SD + 8 * (D3 // 2)

    def hk_a_ops(load):
        blk = {}
        for i in range(3):
            for j in range(3):
                u = load(i, j)
                blk[i, j] = (u, _unpk(u, 0), _unpk(u, 1))
        out = []
        for terms in _HK_A:
            if len(terms) == 1:
                out.append(blk[terms[0][:2]][0])
            else:
                out.append(_pk2(_ssum([(blk[i, j][1], sg) for i, j, sg in terms]),
                                _ssum([(blk[i, j][2], sg) for i, j, sg in terms])))
        return out

    def prep_pieces(c):
        def hk_piece(m, r):
            rb = D3 if m == 2 else TC
            ops = hk_a_ops(lambda i, j: pltpu.bitcast(raw[c, m, pl.ds(i * rb + r, 16), pl.ds(j * TC, TC)], u32))
            for k, t in enumerate(ops):
                if m == 2:
                    pw[c, pl.ds(R_SD + (k // 2) * (D3 // 2) + r // 2, 8), (k % 2) * TC:(k % 2 + 1) * TC] = t
                else:
                    pw[c, pl.ds(k * (TC // 2) + r // 2, 8), m * TC:(m + 1) * TC] = t

        def rem_piece(m, j):
            pw[c, pl.ds(R_TR + j * (KR // 2), KR // 2), m * TC:(m + 1) * TC] = pltpu.bitcast(
                raw[c, m, pl.ds(3 * TC, KR), pl.ds(j * TC, TC)], u32)

        out = []
        for m in range(2):
            out += [functools.partial(hk_piece, m, r) for r in range(0, TC, 16)]
            out += [functools.partial(rem_piece, m, j) for j in range(3)]
        out += [functools.partial(hk_piece, 2, r) for r in range(0, D3, 16)]
        return out

    def transpose_qkv(sec):
        for j in range(*QSEC[sec]):
            wd_ = min(128, 3 * D - j * 128)
            blk = wqkv_raw[:, j * 128:j * 128 + wd_].astype(f32)
            if wd_ < 128:
                blk = jnp.concatenate([blk, jnp.zeros((D, 128 - wd_), f32)], axis=1)
            bt = jnp.concatenate([blk, blk[D - KY:]], axis=0).T
            for t in range(5):
                tmp[t, pl.ds(j * 128, 128), :] = bt[:, t * 128:(t + 1) * 128]

    def build_wq():
        lo = lax.broadcasted_iota(jnp.int32, (16, 128), 1) < KY

        def group(secs, d, row):
            def ld(sec, t, par):
                return None if sec is None else tmp[t, pl.ds(sec * D + d + par * DH, 16, stride=2 * DH), :]
            blk = {(i, j): (ld(secs[j], i, 0), ld(secs[j], i, 1)) for i in range(3) for j in range(3)}
            for n, terms in enumerate(_HK_A):
                if secs[2] is None and n in (4, 5, 9, 12):
                    continue
                ev = _ssum([(blk[i, j][0], sg) for i, j, sg in terms])
                od = _ssum([(blk[i, j][1], sg) for i, j, sg in terms])
                wq[n, pl.ds(row, 16), :] = _pk2(ev, od)
            for j in range(3 if secs[2] is not None else 2):
                t3 = _pk2(ld(secs[j], 3, 0), ld(secs[j], 3, 1))
                t4 = _pk2(ld(secs[j], 4, 0), ld(secs[j], 4, 1))
                wq[15 + 3 * j, pl.ds(row, 16), :] = t3
                wq[16 + 3 * j, pl.ds(row, 16), :] = jnp.where(lo, t3, t4)
                wq[17 + 3 * j, pl.ds(row, 16), :] = jnp.where(lo, t4, t3)
        for d in range(16):
            group((0, 1, 2), d, d * 16)
        for d in range(16, DH):
            group((2, 1, None), d, d * 16)
            group((2, 0, None), d, (d + 2) * 16)

    def build_wo():
        for t in range(5):
            wd_ = min(128, D - t * 128)
            blk = wo_raw[:, t * 128:t * 128 + wd_].astype(f32)
            if wd_ < 128:
                blk = jnp.concatenate([blk, jnp.zeros((D, 128 - wd_), f32)], axis=1)
            tmp[t, pl.ds(0, D), :] = blk
        for t in range(5):
            rows = [tmp[t, pl.ds(d, 32, stride=DH), :] for d in range(DH)]
            ft = jnp.concatenate(rows + rows[16:], axis=0).T
            n = min(128, D - t * 128)
            woT[pl.ds(t * 64, n // 2), :] = pltpu.bitcast(ft[:n].astype(bf16), u32)
        for r in range(0, D3 // 2, 8):
            ops = hk_a_ops(lambda i, j: woT[pl.ds(i * (D3 // 2) + r, 8), j * TC:(j + 1) * TC])
            for k, t in enumerate(ops):
                wo2[pl.ds(k * (D3 // 2) + r, 8), :] = t
        lo = lax.broadcasted_iota(jnp.int32, (8, 128), 1) < KY
        hh = DHALF // 2
        for r in range(0, hh, 8):
            a3, a4 = woT[pl.ds(r, 8), 384:512], woT[pl.ds(r, 8), 512:640]
            b3, b4 = woT[pl.ds(hh + r, 8), 384:512], woT[pl.ds(hh + r, 8), 512:640]

            def dif(u, v):
                return _pk2(_unpk(u, 0) - _unpk(v, 0), _unpk(u, 1) - _unpk(v, 1))
            base = 15 * (D3 // 2)
            wo2[pl.ds(base + r, 8), :] = jnp.where(lo, a3, dif(a3, b3))
            wo2[pl.ds(base + hh + r, 8), :] = jnp.where(lo, b3, dif(b4, a4))
            wo2[pl.ds(base + 2 * hh + r, 8), :] = jnp.where(lo, a4, b3)

    def normalize(blk, mean, rstd, link):
        if not link:
            return (xres[blk] - mean) * rstd
        rs = jnp.broadcast_to(rstd, (8, TB))
        mb = jnp.broadcast_to(mean, (8, TB))
        outs = []
        for i in range(D // 8):
            if i and i % link == 0:
                rs = tie(rs, outs[-1])
            outs.append((xres[blk, pl.ds(i * 8, 8), :] - mb) * rs)
        return jnp.concatenate(outs, axis=0)

    def left_ops(src, put):
        def X(t, r0, n):
            return src[t, pl.ds(r0, n), :]
        for n in range(15):
            v = _ssum([(X(t, i * TC, TC), sg) for (i, t), lst in _HK_C.items() for k, sg in lst if k == n])
            put(n, pltpu.bitcast(v.astype(bf16).T, u32))
        k1, k2, k3 = 3 * TC, 3 * TC + KY, 3 * TC + 2 * KY
        trick = ((lambda: (X(0, k1, KY), X(0, k2, KY) - X(1, k2, KY))),
                 (lambda: (X(1, k1, KY), X(1, k3, KY) - X(0, k3, KY))),
                 (lambda: (X(0, k3, KY), X(1, k2, KY))))
        for n, fn in enumerate(trick):
            put(15 + n, pltpu.bitcast(jnp.concatenate(fn(), axis=0).astype(bf16).T, u32))

    def ln1(pr, par, src, ln, dep=None):
        blk = 2 * pr + par
        if src == 'res':
            x = xres[blk]
        else:
            x = xin[pr, :, par * TB:(par + 1) * TB].astype(f32)
            if src != 'in':
                x = jnp.where(src[0], x, xres[blk])
            xres[blk] = x
        mean, rstd = _ln_stats(x, ln[0], None if dep is None else (lambda v: tie(v, dep)))
        if src == 'res':
            xn_g[par, pl.ds(0, 8), :] = jnp.zeros((8, TB), f32)
        xn_g[par, pl.ds(zero8, D), :] = normalize(blk, mean, rstd, ln[1])

    def q_left():
        def put(i, v):
            sq_scr[i] = v
        left_ops(xn_g, put)

    def hk_outputs(P, T, PT, tk, emit, two_cols=False):
        p8 = P(8)
        t7 = P(7) + p8
        tk(2, t7)
        s1 = PT(3, 1, 2) + t7
        tk(2, s1)
        p6 = P(6)
        p14 = P(14)
        tk(2, p14)
        emit(1, 1, T(1, 1) + (p6 + p14 + s1), 1)
        p13 = P(13)
        if two_cols:
            emit(1, 0, PT(2, 1, 0) + (p13 + s1), 3)
        else:
            p12 = P(12)
            tk(2, p12)
            emit(1, 0, PT(2, 1, 0) + (p12 + p13 + s1), 2)
        p11 = P(11)
        t10 = P(10) + p11
        tk(2, t10)
        if not two_cols:
            s2 = PT(5, 2, 2) + t10
            tk(2, s2)
            p9 = P(9)
            emit(2, 0, T(2, 0) + (p9 + p12 + s2), 2)
            emit(2, 1, PT(4, 2, 1) + (p14 - p13 + s2), 2)
        w0 = T(0, 2)
        emit(0, 0, PT(0, 0, 0) + ((p8 + t10 + w0) if two_cols else (p8 + p9 + t10 + w0)), 3)
        emit(0, 1, PT(1, 0, 1) + (p6 + p11 + t7 + w0), 2)

    QT = (0, 1, 2, 3)
    KT = (4, 5, 6, 7, 13)
    VT = (8, 9, 10, 11, 12)
    c2e = DH ** -0.5 * math.log2(math.e)
    neg = -1e9 * math.log2(math.e)

    def q_step(pr, cs, src, cfg, rows=False):
        clock = _Timeline()
        if rows:
            base, nx = pr * (2 * TB), pr + 1
            clock.add(QA_T[0], functools.partial(a_rows, 0, 0, MODE_A))
            clock.add(QA_T[1], functools.partial(a_rows, 1, 1, MODE_A))
        else:
            base = pl.multiple_of(pr * (2 * TB), 2 * TB)
            nx = jnp.minimum(pr + 1, NP - 1)
        ln_q, la_t, lb_t = cfg[:2], cfg[2], cfg[3]
        pieces = []
        for c in cs:
            pieces += prep_pieces(c)

        def paced(piece, dep):
            pw[NCH, pl.ds(R_END, 8), 0:128] = pltpu.bitcast(dep, u32)
            piece()
        for k, piece in enumerate(pieces):
            clock.add(QP0 + k * (QP1 - QP0) // len(pieces), functools.partial(paced, piece))
        clock.add(la_t, lambda dep: ln1(nx, 0, src, ln_q, dep))
        clock.add(lb_t, lambda dep: ln1(nx, 1, src, ln_q, dep))
        for r0, nt, tiles in ((0, 2, (0, 4, 8)), (TC, 2, (2, 6, 10)), (2 * TC, 1, (12, 13))):
            def R(k):
                return wq[k, pl.ds(r0, nt * 64), :]

            def P(k):
                lhs = sq_scr[k]
                if rows and nt == 1 and k == QA_DEAD:
                    probe = pltpu.bitcast(o_s[0, pl.ds(zero8, 8), :], u32)
                    lhs = jnp.concatenate([lhs[0:8] | (probe & zvec), lhs[8:]], axis=0)
                return _dot_nt(_up(lhs), _up(R(k)))

            def T(j, kind):
                return _dot_nt(_up(sq_scr[15 + kind]), _up(R(15 + 3 * j + kind)))

            def PT(k, j, kind):
                return _dot_nt(_up(jnp.concatenate([sq_scr[k], sq_scr[15 + kind]], axis=1)),
                               _up(jnp.concatenate([R(k), R(15 + 3 * j + kind)], axis=1)))

            def tk(np_, v):
                clock.tick(32 * nt * np_, v, QTK)

            def emit(col, half, v, np_):
                for k in range(nt):
                    qall[tiles[col] + k, pl.ds(base + (HALO + half * TB), TB), :] = v[:, k * 128:(k + 1) * 128]
                tk(np_, v)
            hk_outputs(P, T, PT, tk, emit, two_cols=(nt == 1))
        assert not clock.jobs
        q_left()

    def a_rows(blk, par, mode, start=None):
        lag_mid, lag_end = mode
        base = blk * TB if isinstance(blk, int) else pl.multiple_of(blk * TB, TB)
        cbits = pltpu.bitcast(jnp.full((RB, 128), c2e, f32), u32)
        lo = lax.broadcasted_iota(jnp.int32, (RB, 128), 1) < KY
        mid, fin = {}, {}
        for r in range(nr):
            r0 = r * RB
            deps = [start] if (start is not None and r == 0) else []
            if lag_mid and r >= lag_mid:
                deps.append(mid[r - lag_mid])
            if lag_end and r >= lag_end:
                deps += fin[r - lag_end]
            if deps:
                acc = _tree(jnp.bitwise_or, [pltpu.bitcast(v, u32) for v in deps])
                cs = pltpu.bitcast(cbits | (acc & zvec), f32)
            else:
                cs = c2e

            def ld(t, w):
                return qall[t, pl.ds(base + (HALO + r0 - DIL * w), RB), :]
            q = [ld(t, 0) * cs for t in QT] + [jnp.where(lo, pltpu.roll(ld(13, 0), KY, 1), 0.0) * cs]
            sc = []
            for w in range(W):
                acc = None
                for j, t in enumerate(KT):
                    p = q[j] * ld(t, w)
                    acc = p if acc is None else acc + p
                acc = acc + pltpu.roll(acc, 64, 1)
                mid[r] = acc
                acc = acc + pltpu.roll(acc, 32, 1)
                if r0 - DIL * w < 0:
                    pos = blk * TB + r0 + lax.broadcasted_iota(jnp.int32, (RB, 128), 0)
                    acc = jnp.where(pos >= DIL * w, acc, neg)
                sc.append(acc)
            m = _tree(jnp.maximum, sc)
            e = [jnp.exp2(sc[w] - m) for w in range(W)]
            l = _tree(jnp.add, e)
            rinv = pl.reciprocal(l, approx=True)
            rinv = rinv * (2.0 - l * rinv)
            fin[r] = []
            for j, t in enumerate(VT):
                acc = None
                for w in range(W):
                    p = e[w] * ld(t, w)
                    acc = p if acc is None else acc + p
                o = acc * rinv
                o_s[par * 5 + j, pl.ds(r0, RB), :] = o
                fin[r].append(o)

    def a_wo(blk0, ln, off):
        lo = lax.broadcasted_iota(jnp.int32, (TB, 128), 1) < KY
        hh = DHALF // 2
        base = 15 * (D3 // 2)

        def O(t, j):
            return o_s[t * 5 + j, pl.ds(off, TB), :]

        def rem(t):
            o3, o4 = O(t, 3), O(t, 4)
            rhs = (o3, jnp.where(lo, o3, o4), jnp.where(lo, o4, o3))
            u, v, w_ = [_dot_nt(_up(wo2[pl.ds(base + k * hh, hh), :]), rhs[k].astype(bf16)) for k in range(3)]
            return xres[blk0 + t] + jnp.concatenate([u + w_, v + w_], axis=0)
        rhs = _hk_b([[O(t, j) for t in range(2)] for j in range(3)])
        prod = [None] * 15
        rems = []
        for pos, k in enumerate(WORD):
            if pos in (0, 2):
                rems.append(rem(len(rems)))
            prod[k] = _dot_nt(_up(wo2[pl.ds(k * (D3 // 2), D3 // 2), :]), rhs[k].astype(bf16))
        for t in range(2):
            y = jnp.concatenate([_ssum([(prod[k], sg) for k, sg in _HK_C[i, t]]) for i in range(3)], axis=0)
            x1 = y + rems[t]
            xres[blk0 + t] = x1
            mean, rstd = _ln_stats(x1, ln[0], (lambda v: tie(v, prev)) if (t and LNSER and ln[1]) else None)
            xn = normalize(blk0 + t, mean, rstd, ln[1])
            prev = xn[0:8]
            xn_f[t, pl.ds(zero8 if XNF else 0, D), :] = xn

    def a_left(slot):
        def put(i, v):
            s_scr[slot, i] = v
        left_ops(xn_f, put)

    k0 = math.sqrt(2.0 / math.pi)
    k1 = k0 * 0.044715

    def ffn(j, c0, script):
        clock = _Timeline()
        sb = j % 2
        b0 = (2 * j) % NB
        an = (2 * j + 2) % NB
        acc = [None] * 15
        hs = {}
        state = dict(sdep=False, odep=False)
        hk = KY // 2

        def gu(p):
            c = c0 + p

            def R(n):
                return pw[c, pl.ds(n * (TC // 2), TC // 2), :]

            def RT(jc, kind):
                r0 = R_TR + jc * (KR // 2)
                a_, b_ = ((0, 1), (0, 2), (2, 1))[kind]
                return jnp.concatenate([pw[c, pl.ds(r0 + a_ * hk, hk), :], pw[c, pl.ds(r0 + b_ * hk, hk), :]], axis=0)

            def P(n):
                lhs = s_scr[sb, n]
                if state['odep']:
                    probe = pltpu.bitcast(o_s[0, pl.ds(zero8, 8), :], u32)
                    lhs = jnp.concatenate([lhs[0:8] | (probe & zvec), lhs[8:]], axis=0)
                    state['odep'] = False
                return _dot(_up(lhs), _up(R(n)))

            def T(jc, kind):
                return _dot(_up(s_scr[sb, 15 + kind]), _up(RT(jc, kind)))

            def PT(n, jc, kind):
                return _dot(_up(jnp.concatenate([s_scr[sb, n], s_scr[sb, 15 + kind]], axis=1)),
                            _up(jnp.concatenate([R(n), RT(jc, kind)], axis=0)))
            h = [[None, None] for _ in range(3)]

            def emit(col, half, v, np_):
                gg = v[:, :TC]
                gu_ = gg * v[:, TC:]
                h[col][half] = gu_ + gu_ * jnp.tanh(gg * (k0 + k1 * (gg * gg)))
                clock.tick(64 * np_, h[col][half])
            hk_outputs(P, T, PT, lambda np_, v: clock.tick(64 * np_, v), emit)
            hs[p] = h

        def down(ps):
            rhs = [_hk_b(hs.pop(p)) for p in ps]
            for pos, i in enumerate(DORD):
                au = [pw[c0 + p, pl.ds(R_SD + (i // 2) * (D3 // 2), D3 // 2), (i % 2) * TC:(i % 2 + 1) * TC]
                      for p in ps]
                if state['sdep'] and pos == SDEAD:
                    probe = s_scr[1 - sb, 17, pl.ds(zero8, 8), :]
                    au[0] = jnp.concatenate([au[0][0:8] | (probe & zvec), au[0][8:]], axis=0)
                    state['sdep'] = False
                r = _dot_nt(jnp.concatenate([_up(v) for v in au], axis=1),
                            jnp.concatenate([r_[i] for r_ in rhs], axis=1).astype(bf16))
                acc[i] = r if acc[i] is None else r + acc[i]
                clock.tick(48 * len(ps), acc[i])

        pg = pd = 0
        for tok in script:
            if tok == 'G':
                gu(pg)
                pg += 1
            elif tok[0] == 'D':
                down(list(range(pd, pd + int(tok[1:]))))
                pd += int(tok[1:])
            elif tok == 'W':
                assert not clock.jobs
                a_wo(an, LN_P, zero8)
                clock.t += 1152
            elif tok[0] == 'Y':
                def hold(dep):
                    o_s[10, pl.ds(0, 8), :] = dep
                clock.add(clock.t + int(tok[2:]), hold)
            elif tok == 'X':
                state['odep'] = True
            elif tok == 'S':
                a_left(1 - sb)
                state['sdep'] = SDEAD >= 0
            else:
                par = 0 if tok[1] == 'a' else 1
                clock.add(clock.t + int(tok[3:] or 0), functools.partial(a_rows, an + par, par, MODE_P))
        assert pg == pd and not clock.jobs
        for t in range(2):
            y = jnp.concatenate([_ssum([(acc[k], sg) for k, sg in _HK_C[i, t]]) for i in range(3)], axis=0)
            x2 = xres[b0 + t] + 0.5 * y
            xres[b0 + t] = x2
            o_ref[:, t * TB:(t + 1) * TB] = x2.astype(o_ref.dtype)

    plan = []
    nxt = 0
    for n_ in PLAN:
        plan.append(list(range(nxt, nxt + n_)))
        nxt += n_
    G_P0 = 1 + NP
    G_L = G_P0 + NP - 1

    @pl.when(g == 0)
    def _():
        if ONLY not in ('', 'pro'):
            return
        cp_x(0).start()
        for sec in range(3):
            for cp in cp_qkv(sec):
                cp.start()
        for n_ in range(NP):
            for k in range(CP):
                plan_s[n_ * CP + k] = plan[n_][k] if k < len(plan[n_]) else NCH
        qall[:, pl.ds(0, HALO), :] = jnp.zeros((16, HALO, 128), f32)
        cp_x(0).wait()

    @pl.when(jnp.logical_or(g == 0, g == G_L))
    def _():
        if ONLY not in ('', 'pro'):
            return
        ln1(0, 0, (g == 0,), (4, 0))
        ln1(0, 1, (g == 0,), (4, 0))
        q_left()

    @pl.when(g == 0)
    def _():
        if ONLY not in ('', 'pro'):
            return
        for sec in range(3):
            for cp in cp_qkv(sec):
                cp.wait()
            if sec == 0:
                cp_x(1).start()
                cp_x(2).start()
                cp_wo().start()
                for c in range(NCH):
                    for cp in cp_chunk(c):
                        cp.start()
                    if 3 + c < NP:
                        cp_x(3 + c).start()
            transpose_qkv(sec)
        build_wq()

    for n_ in range(NP):
        @pl.when(g == 1 + n_)
        def _():
            if n_ + 1 < NP:
                cp_x(n_ + 1).wait()
            for c in plan[n_]:
                for cp in cp_chunk(c):
                    cp.wait()

    @pl.when(jnp.logical_and(jnp.logical_and(g >= 1, g < G_P0), g != 2))
    def _():
        if ONLY in ('', 'q'):
            q_step(g - 1, [plan_s[(g - 1) * CP + k] for k in range(CP)], 'in', CFG_Q1)

    @pl.when(g == 2)
    def _():
        if ONLY in ('', 'a'):
            q_step(1, [], 'in', CFG_QA, rows=True)

    @pl.when(jnp.logical_and(g >= G_L, g < G_L + NP))
    def _():
        if ONLY in ('', 'q'):
            q_step(g - G_L, [], 'res', CFG_Q2)

    if ONLY in ('q', 'a', 'pro'):
        @pl.when(g == G_L + NP)
        def _():
            o_ref[0:16, 0:128] = (qall[g % 16, pl.ds(zero8, 16), :] + xres[g % 16, pl.ds(zero8, 16), :]
                                  + pltpu.bitcast(pw[g % 8, pl.ds(zero8, 16), 0:128] | s_scr[g % 2, g % 8, pl.ds(zero8, 16), :]
                                                  | wo2[pl.ds(zero8, 16), :] | wq[g % 8, pl.ds(zero8, 16), :] | sq_scr[g % 8, pl.ds(zero8, 16), :], f32)).astype(bf16)

    @pl.when(g == 1 + A0_AFTER)
    def _():
        if ONLY in ('', 'a'):
            cp_wo().wait()
            build_wo()
            a_wo(0, (4, 0), 0)
            a_left(0)

    @pl.when(g == G_P0)
    def _():
        def body(c, carry):
            for cp in cp_chunk(c):
                cp.wait()
            for piece in prep_pieces(c):
                piece()
            return carry
        if nxt < NCH and not ONLY:
            lax.fori_loop(nxt, NCH, body, 0)

    @pl.when(jnp.logical_and(g >= G_P0, g < G_P0 + 2 * NP - 1))
    def _():
        if ONLY in ('', 'p'):
            ffn(g - G_P0, 0, SCRIPT)

    @pl.when(g == G_P0 + 2 * NP - 1)
    def _():
        def body(hf, carry):
            ffn(2 * NP - 1, hf * NPC, SCRIPT_F)
            return carry
        if ONLY in ('', 'f'):
            lax.fori_loop(0, 2, body, 0)


@jax.jit
def pallas_interleave_layers__sliding_local_dilated__glu_gated_geglu__prompt_kernel(
    A_x, A_wqkv, A_wo, B_x, B_w_gate, B_w_up, B_w_down):
    B, S, D = A_x.shape
    DF = B_w_gate.shape[1]
    NB = S // TB
    NP = NB // 2
    NCH = DF // CW
    xT = A_x.reshape(S, D).T
    wdT = B_w_down.T
    hbm = pl.BlockSpec(memory_space=pltpu.HBM)
    outT = pl.pallas_call(
        functools.partial(_kernel, D=D, DF=DF, S=S),
        grid=(1 + 3 * NP,),
        in_specs=[hbm] * 6,
        out_specs=pl.BlockSpec((D, 2 * TB), lambda g: (0, jnp.maximum(g - (1 + 2 * NP), 0))),
        out_shape=jax.ShapeDtypeStruct((D, S), A_x.dtype),
        scratch_shapes=[
            pltpu.VMEM((NP, D, 2 * TB), bf16),
            pltpu.VMEM((D, 3 * D), bf16),
            pltpu.VMEM((D, D), bf16),
            pltpu.VMEM((5, 14 * 128, 128), f32),
            pltpu.VMEM((24, 320, 128), u32),
            pltpu.VMEM((D // 2, 640), u32),
            pltpu.VMEM((15 * (D // 6) + 3 * (D // 4) + 16, 128), u32),
            pltpu.VMEM((NCH + 1, 3, D, CW), bf16),
            pltpu.VMEM((NCH + 1, 15 * (TC // 2) + 3 * (D - CW) // 2 + 8 * (D // 6) + 16, 2 * TC), u32),
            pltpu.VMEM((16, S + QPAD, 128), f32),
            pltpu.VMEM((11, TB, 128), f32),
            pltpu.VMEM((NB, D, TB), f32),
            pltpu.VMEM((2, D, TB), f32),
            pltpu.VMEM((2, D, TB), f32),
            pltpu.VMEM((2, 18, TB // 2, TC), u32),
            pltpu.VMEM((18, TB // 2, TC), u32),
            pltpu.SMEM((NP * CP,), jnp.int32),
            pltpu.SemaphoreType.DMA((4 + NP + NCH,)),
        ],
        compiler_params=pltpu.CompilerParams(
            dimension_semantics=("arbitrary",),
            vmem_limit_bytes=110 * 1024 * 1024,
        ),
    )(xT, A_wqkv, A_wo, B_w_gate, B_w_up, wdT)
    return outT.T.reshape(B, S, D)
```

```python
import functools
import math
import jax
import jax.numpy as jnp
from jax import lax
import jax.experimental.pallas as pl
import jax.experimental.pallas.tpu as pltpu

H = 32
DH = 18
W = 8
DIL = 2
HALO = 16
EPS = 1e-5
TB = 128
RB = 8
TC = 128
CW = 3 * TC
KY = 64
ONLY = ''
LN_P = tuple(int(x) for x in '1,2'.split(','))
CFG_Q1 = tuple(int(x) for x in '1,2,1500,2500'.split(','))
CFG_Q2 = tuple(int(x) for x in '1,2,60,560'.split(','))
QP0 = int(200); QP1 = int(4000); QTK = int(16)
MODE_P = tuple(int(x) for x in '1,3'.split(','))
MODE_A = tuple(int(x) for x in '1,3'.split(','))
SCRIPT = 'G,G,G,G,ra+1540,G,D4,X,G,G,G,rb+1540,G,D4,X,G,G,Y+1200,G,W,S,D4'.split(',')
SCRIPT_F = 'G,G,G,D2,G,G,G,D2,D2'.split(',')
DORD = tuple(int(x) for x in '2,3,12,4,5,13,14,0,9,10,1,6,7,8,11'.split(','))
SDEAD = int(11)
PLAN = tuple(int(x) for x in '0,0,2,2,2,1,2,2'.split(','))
CP = 2
CFG_QA = tuple(int(x) for x in '1,2,200,500'.split(','))
QA_T = tuple(int(x) for x in '100,800'.split(','))
QA_DEAD = tuple(int(x) for x in '1,1'.split(','))
QPAD = int(40)
LNSER = int(0); XNF = int(0)
WORD = tuple(int(x) for x in '6,7,8,9,0,10,11,1,2,12,13,14,3,4,5'.split(','))
A0_AFTER = int(1)

f32 = jnp.float32
bf16 = jnp.bfloat16
u32 = jnp.uint32
NT = (((1,), (1,)), ((), ()))


def _unpk(u, idx):
    return pltpu.unpack_elementwise(u, index=idx, packed_dtype=bf16, unpacked_dtype=f32)


def _pk2(even, odd):
    return pltpu.pack_elementwise([even, odd], packed_dtype=bf16).astype(u32)


def _up(x):
    return pltpu.bitcast(x, bf16)


def _dot(a, b):
    return jnp.dot(a, b, preferred_element_type=f32)


def _dot_nt(a, b):
    return lax.dot_general(a, b, NT, preferred_element_type=f32)


def _tree(fn, xs):
    xs = list(xs)
    while len(xs) > 1:
        xs = [fn(xs[i], xs[i + 1]) for i in range(0, len(xs) - 1, 2)] + ([xs[-1]] if len(xs) % 2 else [])
    return xs[0]


def _ln_stats(x, nacc, pin=None):
    n = x.shape[0]
    c = x[0:1] if pin is None else pin(x[0:8])[0:1]
    s1 = [None] * nacc
    s2 = [None] * nacc
    for i in range(n // 8):
        d = x[i * 8:(i + 1) * 8] - c
        k = i % nacc
        s1[k] = d if s1[k] is None else s1[k] + d
        dd = d * d
        s2[k] = dd if s2[k] is None else s2[k] + dd
    m = jnp.sum(_tree(jnp.add, s1), axis=0, keepdims=True) * (1.0 / n)
    v = jnp.sum(_tree(jnp.add, s2), axis=0, keepdims=True) * (1.0 / n) - m * m
    v = jnp.maximum(v, 0.0)
    return c + m, lax.rsqrt(v + EPS)


_HK_A = (
    ((0, 0, 1), (0, 2, -1), (1, 0, -1)), ((0, 0, 1), (0, 1, -1), (2, 0, -1)), ((1, 1, 1), (0, 1, -1), (1, 2, -1)),
    ((1, 1, 1), (1, 0, -1), (2, 1, -1)), ((2, 2, 1), (0, 2, -1), (2, 1, -1)), ((2, 2, 1), (1, 2, -1), (2, 0, -1)),
    ((0, 1, 1),), ((0, 1, 1), (1, 0, -1)), ((1, 0, 1),),
    ((0, 2, 1),), ((0, 2, 1), (2, 0, -1)), ((2, 0, 1),),
    ((1, 2, 1),), ((2, 1, 1), (1, 2, -1)), ((2, 1, 1),),
)
_HK_C = {
    (0, 0): ((0, 1), (7, 1), (8, 1), (9, 1), (6, -1)),
    (0, 1): ((1, 1), (6, 1), (10, 1), (11, 1), (9, -1)),
    (1, 0): ((2, 1), (7, 1), (8, 1), (12, 1), (6, -1)),
    (1, 1): ((3, 1), (6, 1), (13, 1), (14, 1), (2, -1), (7, -1)),
    (2, 0): ((5, 1), (9, 1), (12, 1), (13, 1), (4, -1), (10, -1)),
    (2, 1): ((4, 1), (10, 1), (11, 1), (14, 1), (9, -1)),
}


def _hk_b(b):
    s1 = b[1][0] + b[1][1]
    s2 = b[2][0] + b[2][1]
    t7 = b[0][1] + s1
    t10 = b[0][0] + s2
    return (b[0][0], b[0][1], b[1][0], s1, b[2][1], s2, b[0][1] + b[1][1], t7, b[0][0] + t7,
            b[0][0] + b[2][0], t10, b[0][1] + t10, b[1][0] + b[2][0], b[1][0] - b[2][1], b[1][1] + b[2][1])


def _ssum(terms):
    terms = sorted([t for t in terms if t[0] is not None], key=lambda z: -z[1])
    if not terms:
        return None
    acc = terms[0][0] if terms[0][1] == 1 else -terms[0][0]
    for v, sg in terms[1:]:
        acc = acc + v if sg == 1 else acc - v
    return acc


class _Timeline:
    def __init__(self):
        self.t = 0
        self.jobs = []

    def add(self, when, fn):
        self.jobs.append((when, len(self.jobs), fn))
        self.jobs.sort(key=lambda z: z[:2])

    def tick(self, dur, v, n=1, seq=1):
        per = max(n // seq, 1)
        for k in range(n):
            self.t += dur // n
            r = (k % per) * (v.shape[0] // per)
            c = (k // per) * 128
            while self.jobs and self.jobs[0][0] <= self.t:
                self.jobs.pop(0)[2](v[r:r + 8, c:c + 128])


def _kernel(x_hbm, wqkv_hbm, wo_hbm, wg_hbm, wu_hbm, wd_hbm, o_ref,
            xin, wqkv_raw, wo_raw, tmp, wq, woT, wo2, raw, pw, qall, o_s, xres, xn_f, xn_g, s_scr, sq_scr,
            plan_s, sems, *, D, DF, S):
    g = pl.program_id(0)
    NB = S // TB
    NP = NB // 2
    NCH = DF // CW
    NPC = NCH // 2
    D3 = D // 3
    DHALF = D // 2
    KR = D - 3 * TC
    nr = TB // RB
    zero8 = pl.multiple_of((g >> 20) * 8, 8)
    zvec = jnp.full((8, 128), (g >> 20).astype(u32), u32)

    def tie(x, dep):
        return pltpu.bitcast(pltpu.bitcast(x, u32) | (pltpu.bitcast(dep, u32) & zvec), f32)

    QSEC = ((0, 5), (5, 9), (9, 14))

    def cp_qkv(sec):
        out = []
        for j in range(*QSEC[sec]):
            n = min(128, 3 * D - j * 128)
            out.append(pltpu.make_async_copy(wqkv_hbm.at[:, pl.ds(j * 128, n)], wqkv_raw.at[:, pl.ds(j * 128, n)],
                                             sems.at[sec]))
        return out

    def cp_wo():
        return pltpu.make_async_copy(wo_hbm, wo_raw, sems.at[3])

    def cp_x(k):
        return pltpu.make_async_copy(x_hbm.at[:, pl.ds(k * 2 * TB, 2 * TB)], xin.at[k], sems.at[4 + k])

    def cp_chunk(c):
        return [pltpu.make_async_copy(w.at[:, pl.ds(c * CW, CW)], raw.at[c, m], sems.at[4 + NP + c])
                for m, w in enumerate((wg_hbm, wu_hbm, wd_hbm))]

    R_TR = 15 * (TC // 2)
    R_SD = R_TR + 3 * (KR // 2)
    R_END = R_SD + 8 * (D3 // 2)

    def hk_a_ops(load):
        blk = {}
        for i in range(3):
            for j in range(3):
                u = load(i, j)
                blk[i, j] = (u, _unpk(u, 0), _unpk(u, 1))
        out = []
        for terms in _HK_A:
            if len(terms) == 1:
                out.append(blk[terms[0][:2]][0])
            else:
                out.append(_pk2(_ssum([(blk[i, j][1], sg) for i, j, sg in terms]),
                                _ssum([(blk[i, j][2], sg) for i, j, sg in terms])))
        return out

    def prep_pieces(c):
        def hk_piece(m, r):
            rb = D3 if m == 2 else TC
            ops = hk_a_ops(lambda i, j: pltpu.bitcast(raw[c, m, pl.ds(i * rb + r, 16), pl.ds(j * TC, TC)], u32))
            for k, t in enumerate(ops):
                if m == 2:
                    pw[c, pl.ds(R_SD + (k // 2) * (D3 // 2) + r // 2, 8), (k % 2) * TC:(k % 2 + 1) * TC] = t
                else:
                    pw[c, pl.ds(k * (TC // 2) + r // 2, 8), m * TC:(m + 1) * TC] = t

        def rem_piece(m, j):
            pw[c, pl.ds(R_TR + j * (KR // 2), KR // 2), m * TC:(m + 1) * TC] = pltpu.bitcast(
                raw[c, m, pl.ds(3 * TC, KR), pl.ds(j * TC, TC)], u32)

        out = []
        for m in range(2):
            out += [functools.partial(hk_piece, m, r) for r in range(0, TC, 16)]
            out += [functools.partial(rem_piece, m, j) for j in range(3)]
        out += [functools.partial(hk_piece, 2, r) for r in range(0, D3, 16)]
        return out

    def transpose_qkv(sec):
        for j in range(*QSEC[sec]):
            wd_ = min(128, 3 * D - j * 128)
            blk = wqkv_raw[:, j * 128:j * 128 + wd_].astype(f32)
            if wd_ < 128:
                blk = jnp.concatenate([blk, jnp.zeros((D, 128 - wd_), f32)], axis=1)
            bt = jnp.concatenate([blk, blk[D - KY:]], axis=0).T
            for t in range(5):
                tmp[t, pl.ds(j * 128, 128), :] = bt[:, t * 128:(t + 1) * 128]

    def wq_slot(i, j):
        return 24 + i if i == j else [n for n, t in enumerate(_HK_A) if t == ((i, j, 1),)][0]

    def build_wq():
        lo = lax.broadcasted_iota(jnp.int32, (16, 128), 1) < KY

        def group(secs, d, row):
            for j, sec in enumerate(secs):
                tt = [_pk2(tmp[t, pl.ds(sec * D + d, 16, stride=2 * DH), :],
                           tmp[t, pl.ds(sec * D + d + DH, 16, stride=2 * DH), :]) for t in range(5)]
                for i in range(3):
                    wq[wq_slot(i, j), pl.ds(row, 16), :] = tt[i]
                wq[15 + 3 * j, pl.ds(row, 16), :] = tt[3]
                wq[16 + 3 * j, pl.ds(row, 16), :] = jnp.where(lo, tt[3], tt[4])
                wq[17 + 3 * j, pl.ds(row, 16), :] = jnp.where(lo, tt[4], tt[3])
        for d in range(16):
            group((0, 1, 2), d, d * 16)
        for d in range(16, DH):
            group((2, 1), d, d * 16)
            group((2, 0), d, (d + 2) * 16)

    def build_wq_sums(rs):
        for r in rs:
            ncol = 3 if r < 256 else 2
            blk = {}
            for i in range(3):
                for j in range(ncol):
                    u = wq[wq_slot(i, j), pl.ds(r, 8), :]
                    blk[i, j] = (_unpk(u, 0), _unpk(u, 1))
            for n, terms in enumerate(_HK_A):
                if len(terms) == 1 or (ncol == 2 and n in (4, 5)):
                    continue
                wq[n, pl.ds(r, 8), :] = _pk2(*[_ssum([(blk[i, j][p_], sg) for i, j, sg in terms if j < ncol])
                                               for p_ in range(2)])

    def build_wo():
        for t in range(5):
            wd_ = min(128, D - t * 128)
            blk = wo_raw[:, t * 128:t * 128 + wd_].astype(f32)
            if wd_ < 128:
                blk = jnp.concatenate([blk, jnp.zeros((D, 128 - wd_), f32)], axis=1)
            tmp[t, pl.ds(0, D), :] = blk
        for t in range(5):
            rows = [tmp[t, pl.ds(d, 32, stride=DH), :] for d in range(DH)]
            ft = jnp.concatenate(rows + rows[16:], axis=0).T
            n = min(128, D - t * 128)
            woT[pl.ds(t * 64, n // 2), :] = pltpu.bitcast(ft[:n].astype(bf16), u32)
        for r in range(0, D3 // 2, 8):
            ops = hk_a_ops(lambda i, j: woT[pl.ds(i * (D3 // 2) + r, 8), j * TC:(j + 1) * TC])
            for k, t in enumerate(ops):
                wo2[pl.ds(k * (D3 // 2) + r, 8), :] = t
        lo = lax.broadcasted_iota(jnp.int32, (8, 128), 1) < KY
        hh = DHALF // 2
        for r in range(0, hh, 8):
            a3, a4 = woT[pl.ds(r, 8), 384:512], woT[pl.ds(r, 8), 512:640]
            b3, b4 = woT[pl.ds(hh + r, 8), 384:512], woT[pl.ds(hh + r, 8), 512:640]

            def dif(u, v):
                return _pk2(_unpk(u, 0) - _unpk(v, 0), _unpk(u, 1) - _unpk(v, 1))
            base = 15 * (D3 // 2)
            wo2[pl.ds(base + r, 8), :] = jnp.where(lo, a3, dif(a3, b3))
            wo2[pl.ds(base + hh + r, 8), :] = jnp.where(lo, b3, dif(b4, a4))
            wo2[pl.ds(base + 2 * hh + r, 8), :] = jnp.where(lo, a4, b3)

    def normalize(blk, mean, rstd, link):
        if not link:
            return (xres[blk] - mean) * rstd
        rs = jnp.broadcast_to(rstd, (8, TB))
        mb = jnp.broadcast_to(mean, (8, TB))
        outs = []
        for i in range(D // 8):
            if i and i % link == 0:
                rs = tie(rs, outs[-1])
            outs.append((xres[blk, pl.ds(i * 8, 8), :] - mb) * rs)
        return jnp.concatenate(outs, axis=0)

    def left_ops(src, put, plain=False):
        def X(t, r0, n):
            return src[t, pl.ds(r0, n), :]
        for n in range(6 if plain else 15):
            if plain:
                v = X(n // 3, (n % 3) * TC, TC)
            else:
                v = _ssum([(X(t, i * TC, TC), sg) for (i, t), lst in _HK_C.items() for k, sg in lst if k == n])
            put(n, pltpu.bitcast(v.astype(bf16).T, u32))
        k1, k2, k3 = 3 * TC, 3 * TC + KY, 3 * TC + 2 * KY
        trick = ((lambda: (X(0, k1, KY), X(0, k2, KY) - X(1, k2, KY))),
                 (lambda: (X(1, k1, KY), X(1, k3, KY) - X(0, k3, KY))),
                 (lambda: (X(0, k3, KY), X(1, k2, KY))))
        for n, fn in enumerate(trick):
            put(15 + n, pltpu.bitcast(jnp.concatenate(fn(), axis=0).astype(bf16).T, u32))

    def ln1(pr, par, src, ln, dep=None):
        blk = 2 * pr + par
        if src == 'res':
            x = xres[blk]
        else:
            x = xin[pr, :, par * TB:(par + 1) * TB].astype(f32)
            xres[blk] = x
        mean, rstd = _ln_stats(x, ln[0], None if dep is None else (lambda v: tie(v, dep)))
        if src == 'res':
            xn_g[par, pl.ds(0, 8), :] = jnp.zeros((8, TB), f32)
        xn_g[par, pl.ds(zero8, D), :] = normalize(blk, mean, rstd, ln[1])

    def q_left(plain):
        def put(i, v):
            sq_scr[i] = v
        left_ops(xn_g, put, plain)

    def hk_outputs(P, T, PT, tk, emit, two_cols=False):
        p8 = P(8)
        t7 = P(7) + p8
        tk(2, t7)
        s1 = PT(3, 1, 2) + t7
        tk(2, s1)
        p6 = P(6)
        p14 = P(14)
        tk(2, p14)
        emit(1, 1, T(1, 1) + (p6 + p14 + s1), 1)
        p13 = P(13)
        if two_cols:
            emit(1, 0, PT(2, 1, 0) + (p13 + s1), 3)
        else:
            p12 = P(12)
            tk(2, p12)
            emit(1, 0, PT(2, 1, 0) + (p12 + p13 + s1), 2)
        p11 = P(11)
        t10 = P(10) + p11
        tk(2, t10)
        if not two_cols:
            s2 = PT(5, 2, 2) + t10
            tk(2, s2)
            p9 = P(9)
            emit(2, 0, T(2, 0) + (p9 + p12 + s2), 2)
            emit(2, 1, PT(4, 2, 1) + (p14 - p13 + s2), 2)
        w0 = T(0, 2)
        emit(0, 0, PT(0, 0, 0) + ((p8 + t10 + w0) if two_cols else (p8 + p9 + t10 + w0)), 3)
        emit(0, 1, PT(1, 0, 1) + (p6 + p11 + t7 + w0), 2)

    QT = (0, 1, 2, 3)
    KT = (4, 5, 6, 7, 13)
    VT = (8, 9, 10, 11, 12)
    c2e = DH ** -0.5 * math.log2(math.e)
    neg = -1e9 * math.log2(math.e)

    def q_step(pr, cs, src, cfg, rows=False):
        clock = _Timeline()
        if rows:
            base, nx = pr * (2 * TB), pr + 1
            clock.add(QA_T[0], functools.partial(a_rows, 0, 0, MODE_A))
            clock.add(QA_T[1], functools.partial(a_rows, 1, 1, MODE_A))
        else:
            base = pl.multiple_of(pr * (2 * TB), 2 * TB)
            nx = jnp.minimum(pr + 1, NP - 1)
        ln_q, la_t, lb_t = cfg[:2], cfg[2], cfg[3]
        pieces = []
        for c in cs:
            pieces += prep_pieces(c)

        def paced(piece, dep):
            pw[NCH, pl.ds(R_END, 8), 0:128] = pltpu.bitcast(dep, u32)
            piece()
        for k, piece in enumerate(pieces):
            clock.add(QP0 + k * (QP1 - QP0) // len(pieces), functools.partial(paced, piece))
        clock.add(la_t, lambda dep: ln1(nx, 0, src, ln_q, dep))
        clock.add(lb_t, lambda dep: ln1(nx, 1, src, ln_q, dep))
        for r0, nt, tiles in ((0, 2, (0, 4, 8)), (TC, 2, (2, 6, 10)), (2 * TC, 1, (12, 13))):
            def R(k):
                return wq[k, pl.ds(r0, nt * 64), :]

            def P(k):
                return _dot_nt(_up(sq_scr[k]), _up(R(k)))

            def T(j, kind):
                return _dot_nt(_up(sq_scr[15 + kind]), _up(R(15 + 3 * j + kind)))

            def PT(k, j, kind):
                return _dot_nt(_up(jnp.concatenate([sq_scr[k], sq_scr[15 + kind]], axis=1)),
                               _up(jnp.concatenate([R(k), R(15 + 3 * j + kind)], axis=1)))

            def tk(np_, v):
                clock.tick(32 * nt * np_, v, QTK if src == 'in' else 4, nt if src == 'in' else 1)

            def emit(col, half, v, np_):
                for k in range(nt):
                    qall[tiles[col] + k, pl.ds(base + (HALO + half * TB), TB), :] = v[:, k * 128:(k + 1) * 128]
                tk(np_, v)
            if src == 'res':
                hk_outputs(P, T, PT, tk, emit, two_cols=(nt == 1))
                continue
            for j in range(len(tiles)):
                both = T(j, 2)
                for t in range(2):
                    lhs = [sq_scr[3 * t + i] for i in range(3)] + [sq_scr[15 + t]]
                    if rows and nt == 1 and (j, t) == QA_DEAD:
                        probe = pltpu.bitcast(o_s[0, pl.ds(zero8, 8), :], u32)
                        lhs[0] = jnp.concatenate([lhs[0][0:8] | (probe & zvec), lhs[0][8:]], axis=0)
                    rhs = [R(wq_slot(i, j)) for i in range(3)] + [R(15 + 3 * j + t)]
                    emit(j, t, _dot_nt(_up(jnp.concatenate(lhs, axis=1)), _up(jnp.concatenate(rhs, axis=1))) + both,
                         5 - t)
        assert not clock.jobs
        q_left(src == 'in')

    def a_rows(blk, par, mode, start=None):
        lag_mid, lag_end = mode
        base = blk * TB if isinstance(blk, int) else pl.multiple_of(blk * TB, TB)
        cbits = pltpu.bitcast(jnp.full((RB, 128), c2e, f32), u32)
        lo = lax.broadcasted_iota(jnp.int32, (RB, 128), 1) < KY
        mid, fin = {}, {}
        for r in range(nr):
            r0 = r * RB
            deps = [start] if (start is not None and r == 0) else []
            if lag_mid and r >= lag_mid:
                deps.append(mid[r - lag_mid])
            if lag_end and r >= lag_end:
                deps += fin[r - lag_end]
            if deps:
                acc = _tree(jnp.bitwise_or, [pltpu.bitcast(v, u32) for v in deps])
                cs = pltpu.bitcast(cbits | (acc & zvec), f32)
            else:
                cs = c2e

            def ld(t, w):
                return qall[t, pl.ds(base + (HALO + r0 - DIL * w), RB), :]
            q = [ld(t, 0) * cs for t in QT] + [jnp.where(lo, pltpu.roll(ld(13, 0), KY, 1), 0.0) * cs]
            sc = []
            for w in range(W):
                acc = None
                for j, t in enumerate(KT):
                    p = q[j] * ld(t, w)
                    acc = p if acc is None else acc + p
                acc = acc + pltpu.roll(acc, 64, 1)
                mid[r] = acc
                acc = acc + pltpu.roll(acc, 32, 1)
                if r0 - DIL * w < 0:
                    pos = blk * TB + r0 + lax.broadcasted_iota(jnp.int32, (RB, 128), 0)
                    acc = jnp.where(pos >= DIL * w, acc, neg)
                sc.append(acc)
            m = _tree(jnp.maximum, sc)
            e = [jnp.exp2(sc[w] - m) for w in range(W)]
            l = _tree(jnp.add, e)
            rinv = pl.reciprocal(l, approx=True)
            rinv = rinv * (2.0 - l * rinv)
            fin[r] = []
            for j, t in enumerate(VT):
                acc = None
                for w in range(W):
                    p = e[w] * ld(t, w)
                    acc = p if acc is None else acc + p
                o = acc * rinv
                o_s[par * 5 + j, pl.ds(r0, RB), :] = o
                fin[r].append(o)

    def a_wo(blk0, ln, off, cb=None):
        lo = lax.broadcasted_iota(jnp.int32, (TB, 128), 1) < KY
        hh = DHALF // 2
        base = 15 * (D3 // 2)

        def O(t, j):
            return o_s[t * 5 + j, pl.ds(off, TB), :]

        def rem(t):
            o3, o4 = O(t, 3), O(t, 4)
            rhs = (o3, jnp.where(lo, o3, o4), jnp.where(lo, o4, o3))
            u, v, w_ = [_dot_nt(_up(wo2[pl.ds(base + k * hh, hh), :]), rhs[k].astype(bf16)) for k in range(3)]
            return xres[blk0 + t] + jnp.concatenate([u + w_, v + w_], axis=0)
        rhs = _hk_b([[O(t, j) for t in range(2)] for j in range(3)])
        prod = [None] * 15
        rems = []
        for pos, k in enumerate(WORD):
            if pos in (0, 2):
                rems.append(rem(len(rems)))
            prod[k] = _dot_nt(_up(wo2[pl.ds(k * (D3 // 2), D3 // 2), :]), rhs[k].astype(bf16))
            if cb is not None:
                cb(pos, prod[k])
        for t in range(2):
            y = jnp.concatenate([_ssum([(prod[k], sg) for k, sg in _HK_C[i, t]]) for i in range(3)], axis=0)
            x1 = y + rems[t]
            xres[blk0 + t] = x1
            mean, rstd = _ln_stats(x1, ln[0], (lambda v: tie(v, prev)) if (t and LNSER and ln[1]) else None)
            xn = normalize(blk0 + t, mean, rstd, ln[1])
            prev = xn[0:8]
            xn_f[t, pl.ds(zero8 if XNF else 0, D), :] = xn

    def a_left(slot):
        def put(i, v):
            s_scr[slot, i] = v
        left_ops(xn_f, put)

    k0 = math.sqrt(2.0 / math.pi)
    k1 = k0 * 0.044715

    def ffn(j, c0, script):
        clock = _Timeline()
        sb = j % 2
        b0 = (2 * j) % NB
        an = (2 * j + 2) % NB
        acc = [None] * 15
        hs = {}
        state = dict(sdep=False, odep=False)
        hk = KY // 2

        def gu(p):
            c = c0 + p

            def R(n):
                return pw[c, pl.ds(n * (TC // 2), TC // 2), :]

            def RT(jc, kind):
                r0 = R_TR + jc * (KR // 2)
                a_, b_ = ((0, 1), (0, 2), (2, 1))[kind]
                return jnp.concatenate([pw[c, pl.ds(r0 + a_ * hk, hk), :], pw[c, pl.ds(r0 + b_ * hk, hk), :]], axis=0)

            def P(n):
                lhs = s_scr[sb, n]
                if state['odep']:
                    probe = pltpu.bitcast(o_s[0, pl.ds(zero8, 8), :], u32)
                    lhs = jnp.concatenate([lhs[0:8] | (probe & zvec), lhs[8:]], axis=0)
                    state['odep'] = False
                return _dot(_up(lhs), _up(R(n)))

            def T(jc, kind):
                return _dot(_up(s_scr[sb, 15 + kind]), _up(RT(jc, kind)))

            def PT(n, jc, kind):
                return _dot(_up(jnp.concatenate([s_scr[sb, n], s_scr[sb, 15 + kind]], axis=1)),
                            _up(jnp.concatenate([R(n), RT(jc, kind)], axis=0)))
            h = [[None, None] for _ in range(3)]

            def emit(col, half, v, np_):
                gg = v[:, :TC]
                gu_ = gg * v[:, TC:]
                h[col][half] = gu_ + gu_ * jnp.tanh(gg * (k0 + k1 * (gg * gg)))
                clock.tick(64 * np_, h[col][half])
            hk_outputs(P, T, PT, lambda np_, v: clock.tick(64 * np_, v), emit)
            hs[p] = h

        def down(ps):
            rhs = [_hk_b(hs.pop(p)) for p in ps]
            for pos, i in enumerate(DORD):
                au = [pw[c0 + p, pl.ds(R_SD + (i // 2) * (D3 // 2), D3 // 2), (i % 2) * TC:(i % 2 + 1) * TC]
                      for p in ps]
                if state['sdep'] and pos == SDEAD:
                    probe = s_scr[1 - sb, 17, pl.ds(zero8, 8), :]
                    au[0] = jnp.concatenate([au[0][0:8] | (probe & zvec), au[0][8:]], axis=0)
                    state['sdep'] = False
                r = _dot_nt(jnp.concatenate([_up(v) for v in au], axis=1),
                            jnp.concatenate([r_[i] for r_ in rhs], axis=1).astype(bf16))
                acc[i] = r if acc[i] is None else r + acc[i]
                clock.tick(48 * len(ps), acc[i])

        pg = pd = 0
        for tok in script:
            if tok == 'G':
                gu(pg)
                pg += 1
            elif tok[0] == 'D':
                down(list(range(pd, pd + int(tok[1:]))))
                pd += int(tok[1:])
            elif tok == 'W':
                assert not clock.jobs
                a_wo(an, LN_P, zero8)
                clock.t += 1152
            elif tok[0] == 'Y':
                def hold(dep):
                    o_s[10, pl.ds(0, 8), :] = dep
                clock.add(clock.t + int(tok[2:]), hold)
            elif tok == 'X':
                state['odep'] = True
            elif tok == 'S':
                a_left(1 - sb)
                state['sdep'] = SDEAD >= 0
            else:
                par = 0 if tok[1] == 'a' else 1
                clock.add(clock.t + int(tok[3:] or 0), functools.partial(a_rows, an + par, par, MODE_P))
        assert pg == pd and not clock.jobs
        for t in range(2):
            y = jnp.concatenate([_ssum([(acc[k], sg) for k, sg in _HK_C[i, t]]) for i in range(3)], axis=0)
            x2 = xres[b0 + t] + 0.5 * y
            xres[b0 + t] = x2
            o_ref[:, t * TB:(t + 1) * TB] = x2.astype(o_ref.dtype)

    plan = []
    nxt = 0
    for n_ in PLAN:
        plan.append(list(range(nxt, nxt + n_)))
        nxt += n_
    G_P0 = 1 + NP
    G_L = G_P0 + NP - 1

    @pl.when(g == 0)
    def _():
        if ONLY not in ('', 'pro'):
            return
        cp_x(0).start()
        for sec in range(3):
            for cp in cp_qkv(sec):
                cp.start()
        for n_ in range(NP):
            for k in range(CP):
                plan_s[n_ * CP + k] = plan[n_][k] if k < len(plan[n_]) else NCH
        qall[:, pl.ds(0, HALO), :] = jnp.zeros((16, HALO, 128), f32)
        cp_x(0).wait()
        ln1(0, 0, 'in', (4, 0))
        ln1(0, 1, 'in', (4, 0))
        q_left(True)
        for sec in range(3):
            for cp in cp_qkv(sec):
                cp.wait()
            if sec == 0:
                cp_x(1).start()
                cp_x(2).start()
                cp_wo().start()
                for c in range(NCH):
                    for cp in cp_chunk(c):
                        cp.start()
                    if 3 + c < NP:
                        cp_x(3 + c).start()
            transpose_qkv(sec)
        build_wq()

    @pl.when(g == G_L)
    def _():
        if ONLY not in ('', 'pro'):
            return
        ln1(0, 0, 'res', (4, 0))
        ln1(0, 1, 'res', (4, 0))
        q_left(False)

    for n_ in range(NP):
        @pl.when(g == 1 + n_)
        def _():
            if n_ + 1 < NP:
                cp_x(n_ + 1).wait()
            for c in plan[n_]:
                for cp in cp_chunk(c):
                    cp.wait()

    @pl.when(jnp.logical_and(jnp.logical_and(g >= 1, g < G_P0), g != 2))
    def _():
        if ONLY in ('', 'q'):
            q_step(g - 1, [plan_s[(g - 1) * CP + k] for k in range(CP)], 'in', CFG_Q1)

    @pl.when(g == 2)
    def _():
        if ONLY in ('', 'a'):
            q_step(1, [], 'in', CFG_QA, rows=True)

    @pl.when(jnp.logical_and(g >= G_L, g < G_L + NP))
    def _():
        if ONLY in ('', 'q'):
            q_step(g - G_L, [], 'res', CFG_Q2)

    if ONLY in ('q', 'a', 'pro'):
        @pl.when(g == G_L + NP)
        def _():
            o_ref[0:16, 0:128] = (qall[g % 16, pl.ds(zero8, 16), :] + xres[g % 16, pl.ds(zero8, 16), :]
                                  + pltpu.bitcast(pw[g % 8, pl.ds(zero8, 16), 0:128] | s_scr[g % 2, g % 8, pl.ds(zero8, 16), :]
                                                  | wo2[pl.ds(zero8, 16), :] | wq[g % 8, pl.ds(zero8, 16), :] | sq_scr[g % 8, pl.ds(zero8, 16), :], f32)).astype(bf16)

    @pl.when(g == 1 + A0_AFTER)
    def _():
        if ONLY in ('', 'a'):
            cp_wo().wait()
            build_wo()

            def cb(pos, v):
                if pos % 4 == 2 or pos == 0:
                    for k in range(8):
                        wq[27, pl.ds(zero8, 8), :] = pltpu.bitcast(v[k * 24:k * 24 + 8], u32)
                        build_wq_sums([todo.pop(0)])
            todo = list(range(0, 320, 8))
            a_wo(0, (4, 0), 0, cb)
            assert not todo
            a_left(0)

    @pl.when(g == G_P0)
    def _():
        def body(c, carry):
            for cp in cp_chunk(c):
                cp.wait()
            for piece in prep_pieces(c):
                piece()
            return carry
        if nxt < NCH and not ONLY:
            lax.fori_loop(nxt, NCH, body, 0)

    @pl.when(jnp.logical_and(g >= G_P0, g < G_P0 + 2 * NP - 1))
    def _():
        if ONLY in ('', 'p'):
            ffn(g - G_P0, 0, SCRIPT)

    @pl.when(g == G_P0 + 2 * NP - 1)
    def _():
        def body(hf, carry):
            ffn(2 * NP - 1, hf * NPC, SCRIPT_F)
            return carry
        if ONLY in ('', 'f'):
            lax.fori_loop(0, 2, body, 0)


@jax.jit
def pallas_interleave_layers__sliding_local_dilated__glu_gated_geglu__prompt_kernel(
    A_x, A_wqkv, A_wo, B_x, B_w_gate, B_w_up, B_w_down):
    B, S, D = A_x.shape
    DF = B_w_gate.shape[1]
    NB = S // TB
    NP = NB // 2
    NCH = DF // CW
    xT = A_x.reshape(S, D).T
    wdT = B_w_down.T
    hbm = pl.BlockSpec(memory_space=pltpu.HBM)
    outT = pl.pallas_call(
        functools.partial(_kernel, D=D, DF=DF, S=S),
        grid=(1 + 3 * NP,),
        in_specs=[hbm] * 6,
        out_specs=pl.BlockSpec((D, 2 * TB), lambda g: (0, jnp.maximum(g - (1 + 2 * NP), 0))),
        out_shape=jax.ShapeDtypeStruct((D, S), A_x.dtype),
        scratch_shapes=[
            pltpu.VMEM((NP, D, 2 * TB), bf16),
            pltpu.VMEM((D, 3 * D), bf16),
            pltpu.VMEM((D, D), bf16),
            pltpu.VMEM((5, 14 * 128, 128), f32),
            pltpu.VMEM((28, 320, 128), u32),
            pltpu.VMEM((D // 2, 640), u32),
            pltpu.VMEM((15 * (D // 6) + 3 * (D // 4) + 16, 128), u32),
            pltpu.VMEM((NCH + 1, 3, D, CW), bf16),
            pltpu.VMEM((NCH + 1, 15 * (TC // 2) + 3 * (D - CW) // 2 + 8 * (D // 6) + 16, 2 * TC), u32),
            pltpu.VMEM((16, S + QPAD, 128), f32),
            pltpu.VMEM((11, TB, 128), f32),
            pltpu.VMEM((NB, D, TB), f32),
            pltpu.VMEM((2, D, TB), f32),
            pltpu.VMEM((2, D, TB), f32),
            pltpu.VMEM((2, 18, TB // 2, TC), u32),
            pltpu.VMEM((18, TB // 2, TC), u32),
            pltpu.SMEM((NP * CP,), jnp.int32),
            pltpu.SemaphoreType.DMA((4 + NP + NCH,)),
        ],
        compiler_params=pltpu.CompilerParams(
            dimension_semantics=("arbitrary",),
            vmem_limit_bytes=110 * 1024 * 1024,
        ),
    )(xT, A_wqkv, A_wo, B_w_gate, B_w_up, wdT)
    return outT.T.reshape(B, S, D)
```

```python
import functools
import math
import jax
import jax.numpy as jnp
from jax import lax
import jax.experimental.pallas as pl
import jax.experimental.pallas.tpu as pltpu

H = 32
DH = 18
W = 8
DIL = 2
HALO = 16
EPS = 1e-5
TB = 128
RB = 8
TC = 128
CW = 3 * TC
KY = 64
ONLY = ''
LN_P = tuple(int(x) for x in '1,2'.split(','))
CFG_Q1 = tuple(int(x) for x in '1,2,1500,2500'.split(','))
CFG_Q2 = tuple(int(x) for x in '1,2,60,560'.split(','))
QP0 = int(200); QP1 = int(4000); QTK = int(16)
MODE_P = tuple(int(x) for x in '1,3'.split(','))
MODE_A = tuple(int(x) for x in '1,3'.split(','))
SCRIPT = 'G,G,G,G,ra+1540,G,D4,X,G,G,G,rb+1540,G,D4,X,G,G,Y+1200,G,W,S,D4'.split(',')
SCRIPT_F = 'G,G,G,D2,G,G,G,D2,D2'.split(',')
DORD = tuple(int(x) for x in '2,3,12,4,5,13,14,0,9,10,1,6,7,8,11'.split(','))
SDEAD = int(11)
PLAN = tuple(int(x) for x in '0,0,2,2,2,1,2,2'.split(','))
CP = 2
CFG_QA = tuple(int(x) for x in '1,2,200,500'.split(','))
QA_T = tuple(int(x) for x in '100,800'.split(','))
QA_DEAD = tuple(int(x) for x in '1,1'.split(','))
QPAD = int(40)
LNSER = int(0); XNF = int(0)
WORD = tuple(int(x) for x in '6,7,8,9,0,10,11,1,2,12,13,14,3,4,5'.split(','))
NOCHK = int(0)

f32 = jnp.float32
bf16 = jnp.bfloat16
u32 = jnp.uint32
NT = (((1,), (1,)), ((), ()))


def _unpk(u, idx):
    return pltpu.unpack_elementwise(u, index=idx, packed_dtype=bf16, unpacked_dtype=f32)


def _pk2(even, odd):
    return pltpu.pack_elementwise([even, odd], packed_dtype=bf16).astype(u32)


def _up(x):
    return pltpu.bitcast(x, bf16)


def _dot(a, b):
    return jnp.dot(a, b, preferred_element_type=f32)


def _dot_nt(a, b):
    return lax.dot_general(a, b, NT, preferred_element_type=f32)


def _tree(fn, xs):
    xs = list(xs)
    while len(xs) > 1:
        xs = [fn(xs[i], xs[i + 1]) for i in range(0, len(xs) - 1, 2)] + ([xs[-1]] if len(xs) % 2 else [])
    return xs[0]


def _ln_stats(x, nacc, pin=None):
    n = x.shape[0]
    c = x[0:1] if pin is None else pin(x[0:8])[0:1]
    s1 = [None] * nacc
    s2 = [None] * nacc
    for i in range(n // 8):
        d = x[i * 8:(i + 1) * 8] - c
        k = i % nacc
        s1[k] = d if s1[k] is None else s1[k] + d
        dd = d * d
        s2[k] = dd if s2[k] is None else s2[k] + dd
    m = jnp.sum(_tree(jnp.add, s1), axis=0, keepdims=True) * (1.0 / n)
    v = jnp.sum(_tree(jnp.add, s2), axis=0, keepdims=True) * (1.0 / n) - m * m
    v = jnp.maximum(v, 0.0)
    return c + m, lax.rsqrt(v + EPS)


_HK_A = (
    ((0, 0, 1), (0, 2, -1), (1, 0, -1)), ((0, 0, 1), (0, 1, -1), (2, 0, -1)), ((1, 1, 1), (0, 1, -1), (1, 2, -1)),
    ((1, 1, 1), (1, 0, -1), (2, 1, -1)), ((2, 2, 1), (0, 2, -1), (2, 1, -1)), ((2, 2, 1), (1, 2, -1), (2, 0, -1)),
    ((0, 1, 1),), ((0, 1, 1), (1, 0, -1)), ((1, 0, 1),),
    ((0, 2, 1),), ((0, 2, 1), (2, 0, -1)), ((2, 0, 1),),
    ((1, 2, 1),), ((2, 1, 1), (1, 2, -1)), ((2, 1, 1),),
)
_HK_C = {
    (0, 0): ((0, 1), (7, 1), (8, 1), (9, 1), (6, -1)),
    (0, 1): ((1, 1), (6, 1), (10, 1), (11, 1), (9, -1)),
    (1, 0): ((2, 1), (7, 1), (8, 1), (12, 1), (6, -1)),
    (1, 1): ((3, 1), (6, 1), (13, 1), (14, 1), (2, -1), (7, -1)),
    (2, 0): ((5, 1), (9, 1), (12, 1), (13, 1), (4, -1), (10, -1)),
    (2, 1): ((4, 1), (10, 1), (11, 1), (14, 1), (9, -1)),
}


def _hk_b(b):
    s1 = b[1][0] + b[1][1]
    s2 = b[2][0] + b[2][1]
    t7 = b[0][1] + s1
    t10 = b[0][0] + s2
    return (b[0][0], b[0][1], b[1][0], s1, b[2][1], s2, b[0][1] + b[1][1], t7, b[0][0] + t7,
            b[0][0] + b[2][0], t10, b[0][1] + t10, b[1][0] + b[2][0], b[1][0] - b[2][1], b[1][1] + b[2][1])


def _ssum(terms):
    terms = sorted([t for t in terms if t[0] is not None], key=lambda z: -z[1])
    if not terms:
        return None
    acc = terms[0][0] if terms[0][1] == 1 else -terms[0][0]
    for v, sg in terms[1:]:
        acc = acc + v if sg == 1 else acc - v
    return acc


class _Timeline:
    def __init__(self):
        self.t = 0
        self.jobs = []

    def add(self, when, fn):
        self.jobs.append((when, len(self.jobs), fn))
        self.jobs.sort(key=lambda z: z[:2])

    def tick(self, dur, v, n=1, seq=1):
        per = max(n // seq, 1)
        for k in range(n):
            self.t += dur // n
            r = (k % per) * (v.shape[0] // per)
            c = (k // per) * 128
            while self.jobs and self.jobs[0][0] <= self.t:
                self.jobs.pop(0)[2](v[r:r + 8, c:c + 128])


def _kernel(x_hbm, wqkv_hbm, wo_hbm, wg_hbm, wu_hbm, wd_hbm, o_ref,
            xin, wqkv_raw, wo_raw, tmp, wq, woT, wo2, raw, pw, qall, o_s, xres, xn_f, xn_g, s_scr, sq_scr,
            plan_s, sems, *, D, DF, S):
    g = pl.program_id(0)
    NB = S // TB
    NP = NB // 2
    NCH = DF // CW
    NPC = NCH // 2
    D3 = D // 3
    DHALF = D // 2
    KR = D - 3 * TC
    nr = TB // RB
    zero8 = pl.multiple_of((g >> 20) * 8, 8)
    zvec = jnp.full((8, 128), (g >> 20).astype(u32), u32)

    def tie(x, dep):
        return pltpu.bitcast(pltpu.bitcast(x, u32) | (pltpu.bitcast(dep, u32) & zvec), f32)

    QSEC = ((0, 5), (5, 9), (9, 14))

    def cp_qkv(sec):
        out = []
        for j in range(*QSEC[sec]):
            n = min(128, 3 * D - j * 128)
            out.append(pltpu.make_async_copy(wqkv_hbm.at[:, pl.ds(j * 128, n)], wqkv_raw.at[:, pl.ds(j * 128, n)],
                                             sems.at[sec]))
        return out

    def cp_wo():
        return pltpu.make_async_copy(wo_hbm, wo_raw, sems.at[3])

    def cp_x(k):
        return pltpu.make_async_copy(x_hbm.at[:, pl.ds(k * 2 * TB, 2 * TB)], xin.at[k], sems.at[4 + k])

    def cp_chunk(c):
        return [pltpu.make_async_copy(w.at[:, pl.ds(c * CW, CW)], raw.at[c, m], sems.at[4 + NP + c])
                for m, w in enumerate((wg_hbm, wu_hbm, wd_hbm))]

    R_TR = 15 * (TC // 2)
    R_SD = R_TR + 3 * (KR // 2)
    R_END = R_SD + 8 * (D3 // 2)

    def hk_a_ops(load):
        blk = {}
        for i in range(3):
            for j in range(3):
                u = load(i, j)
                blk[i, j] = (u, _unpk(u, 0), _unpk(u, 1))
        out = []
        for terms in _HK_A:
            if len(terms) == 1:
                out.append(blk[terms[0][:2]][0])
            else:
                out.append(_pk2(_ssum([(blk[i, j][1], sg) for i, j, sg in terms]),
                                _ssum([(blk[i, j][2], sg) for i, j, sg in terms])))
        return out

    def prep_pieces(c):
        def hk_piece(m, r):
            rb = D3 if m == 2 else TC
            ops = hk_a_ops(lambda i, j: pltpu.bitcast(raw[c, m, pl.ds(i * rb + r, 16), pl.ds(j * TC, TC)], u32))
            for k, t in enumerate(ops):
                if m == 2:
                    pw[c, pl.ds(R_SD + (k // 2) * (D3 // 2) + r // 2, 8), (k % 2) * TC:(k % 2 + 1) * TC] = t
                else:
                    pw[c, pl.ds(k * (TC // 2) + r // 2, 8), m * TC:(m + 1) * TC] = t

        def rem_piece(m, j):
            pw[c, pl.ds(R_TR + j * (KR // 2), KR // 2), m * TC:(m + 1) * TC] = pltpu.bitcast(
                raw[c, m, pl.ds(3 * TC, KR), pl.ds(j * TC, TC)], u32)

        out = []
        for m in range(2):
            out += [functools.partial(hk_piece, m, r) for r in range(0, TC, 16)]
            out += [functools.partial(rem_piece, m, j) for j in range(3)]
        out += [functools.partial(hk_piece, 2, r) for r in range(0, D3, 16)]
        return out

    def transpose_qkv(sec):
        for j in range(*QSEC[sec]):
            wd_ = min(128, 3 * D - j * 128)
            blk = wqkv_raw[:, j * 128:j * 128 + wd_].astype(f32)
            if wd_ < 128:
                blk = jnp.concatenate([blk, jnp.zeros((D, 128 - wd_), f32)], axis=1)
            bt = jnp.concatenate([blk, blk[D - KY:]], axis=0).T
            for t in range(5):
                tmp[t, pl.ds(j * 128, 128), :] = bt[:, t * 128:(t + 1) * 128]

    def wq_slot(i, j):
        return 24 + i if i == j else [n for n, t in enumerate(_HK_A) if t == ((i, j, 1),)][0]

    def build_wq(sec):
        lo = lax.broadcasted_iota(jnp.int32, (16, 128), 1) < KY
        for d in range(DH):
            tt = [_pk2(tmp[t, pl.ds(sec * D + d, 16, stride=2 * DH), :],
                       tmp[t, pl.ds(sec * D + d + DH, 16, stride=2 * DH), :]) for t in range(5)]
            ops = tt[:4] + [jnp.where(lo, tt[3], tt[4]), jnp.where(lo, tt[4], tt[3])]
            if d < 16:
                dst = [(sec, d * 16)]
            else:
                dst = ([(1, (d + 2) * 16)], [(1, d * 16)], [(0, d * 16), (0, (d + 2) * 16)])[sec]
            for j, row in dst:
                for k, v in enumerate(ops):
                    wq[wq_slot(k, j) if k < 3 else 12 + 3 * j + k, pl.ds(row, 16), :] = v

    def build_wq_sums(rs):
        for r in rs:
            ncol = 3 if r < 256 else 2
            blk = {}
            for i in range(3):
                for j in range(ncol):
                    u = wq[wq_slot(i, j), pl.ds(r, 8), :]
                    blk[i, j] = (_unpk(u, 0), _unpk(u, 1))
            for n, terms in enumerate(_HK_A):
                if len(terms) == 1 or (ncol == 2 and n in (4, 5)):
                    continue
                wq[n, pl.ds(r, 8), :] = _pk2(*[_ssum([(blk[i, j][p_], sg) for i, j, sg in terms if j < ncol])
                                               for p_ in range(2)])

    def build_wo():
        for t in range(5):
            wd_ = min(128, D - t * 128)
            blk = wo_raw[:, t * 128:t * 128 + wd_].astype(f32)
            if wd_ < 128:
                blk = jnp.concatenate([blk, jnp.zeros((D, 128 - wd_), f32)], axis=1)
            tmp[t, pl.ds(0, D), :] = blk
        for t in range(5):
            rows = [tmp[t, pl.ds(d, 32, stride=DH), :] for d in range(DH)]
            ft = jnp.concatenate(rows + rows[16:], axis=0).T
            n = min(128, D - t * 128)
            woT[pl.ds(t * 64, n // 2), :] = pltpu.bitcast(ft[:n].astype(bf16), u32)
        for r in range(0, D3 // 2, 8):
            ops = hk_a_ops(lambda i, j: woT[pl.ds(i * (D3 // 2) + r, 8), j * TC:(j + 1) * TC])
            for k, t in enumerate(ops):
                wo2[pl.ds(k * (D3 // 2) + r, 8), :] = t
        lo = lax.broadcasted_iota(jnp.int32, (8, 128), 1) < KY
        hh = DHALF // 2
        for r in range(0, hh, 8):
            a3, a4 = woT[pl.ds(r, 8), 384:512], woT[pl.ds(r, 8), 512:640]
            b3, b4 = woT[pl.ds(hh + r, 8), 384:512], woT[pl.ds(hh + r, 8), 512:640]

            def dif(u, v):
                return _pk2(_unpk(u, 0) - _unpk(v, 0), _unpk(u, 1) - _unpk(v, 1))
            base = 15 * (D3 // 2)
            wo2[pl.ds(base + r, 8), :] = jnp.where(lo, a3, dif(a3, b3))
            wo2[pl.ds(base + hh + r, 8), :] = jnp.where(lo, b3, dif(b4, a4))
            wo2[pl.ds(base + 2 * hh + r, 8), :] = jnp.where(lo, a4, b3)

    def normalize(blk, mean, rstd, link):
        if not link:
            return (xres[blk] - mean) * rstd
        rs = jnp.broadcast_to(rstd, (8, TB))
        mb = jnp.broadcast_to(mean, (8, TB))
        outs = []
        for i in range(D // 8):
            if i and i % link == 0:
                rs = tie(rs, outs[-1])
            outs.append((xres[blk, pl.ds(i * 8, 8), :] - mb) * rs)
        return jnp.concatenate(outs, axis=0)

    def left_ops(src, put, plain=False):
        def X(t, r0, n):
            return src[t, pl.ds(r0, n), :]
        for n in range(6 if plain else 15):
            if plain:
                v = X(n // 3, (n % 3) * TC, TC)
            else:
                v = _ssum([(X(t, i * TC, TC), sg) for (i, t), lst in _HK_C.items() for k, sg in lst if k == n])
            put(n, pltpu.bitcast(v.astype(bf16).T, u32))
        k1, k2, k3 = 3 * TC, 3 * TC + KY, 3 * TC + 2 * KY
        trick = ((lambda: (X(0, k1, KY), X(0, k2, KY) - X(1, k2, KY))),
                 (lambda: (X(1, k1, KY), X(1, k3, KY) - X(0, k3, KY))),
                 (lambda: (X(0, k3, KY), X(1, k2, KY))))
        for n, fn in enumerate(trick):
            put(15 + n, pltpu.bitcast(jnp.concatenate(fn(), axis=0).astype(bf16).T, u32))

    def ln1(pr, par, src, ln, dep=None):
        blk = 2 * pr + par
        if src == 'res':
            x = xres[blk]
        else:
            x = xin[pr, :, par * TB:(par + 1) * TB].astype(f32)
            xres[blk] = x
        mean, rstd = _ln_stats(x, ln[0], None if dep is None else (lambda v: tie(v, dep)))
        if src == 'res':
            xn_g[par, pl.ds(0, 8), :] = jnp.zeros((8, TB), f32)
        xn_g[par, pl.ds(zero8, D), :] = normalize(blk, mean, rstd, ln[1])

    def q_left(plain):
        def put(i, v):
            sq_scr[i] = v
        left_ops(xn_g, put, plain)

    def hk_outputs(P, T, PT, tk, emit, two_cols=False):
        p8 = P(8)
        t7 = P(7) + p8
        tk(2, t7)
        s1 = PT(3, 1, 2) + t7
        tk(2, s1)
        p6 = P(6)
        p14 = P(14)
        tk(2, p14)
        emit(1, 1, T(1, 1) + (p6 + p14 + s1), 1)
        p13 = P(13)
        if two_cols:
            emit(1, 0, PT(2, 1, 0) + (p13 + s1), 3)
        else:
            p12 = P(12)
            tk(2, p12)
            emit(1, 0, PT(2, 1, 0) + (p12 + p13 + s1), 2)
        p11 = P(11)
        t10 = P(10) + p11
        tk(2, t10)
        if not two_cols:
            s2 = PT(5, 2, 2) + t10
            tk(2, s2)
            p9 = P(9)
            emit(2, 0, T(2, 0) + (p9 + p12 + s2), 2)
            emit(2, 1, PT(4, 2, 1) + (p14 - p13 + s2), 2)
        w0 = T(0, 2)
        emit(0, 0, PT(0, 0, 0) + ((p8 + t10 + w0) if two_cols else (p8 + p9 + t10 + w0)), 3)
        emit(0, 1, PT(1, 0, 1) + (p6 + p11 + t7 + w0), 2)

    QT = (0, 1, 2, 3)
    KT = (4, 5, 6, 7, 13)
    VT = (8, 9, 10, 11, 12)
    c2e = DH ** -0.5 * math.log2(math.e)
    neg = -1e9 * math.log2(math.e)

    def q_step(pr, cs, src, cfg, rows=False):
        clock = _Timeline()
        if rows:
            base, nx = pr * (2 * TB), pr + 1
            clock.add(QA_T[0], functools.partial(a_rows, 0, 0, MODE_A))
            clock.add(QA_T[1], functools.partial(a_rows, 1, 1, MODE_A))
        else:
            base = pl.multiple_of(pr * (2 * TB), 2 * TB)
            nx = jnp.minimum(pr + 1, NP - 1)
        ln_q, la_t, lb_t = cfg[:2], cfg[2], cfg[3]
        pieces = []
        for c in cs:
            pieces += prep_pieces(c)

        def paced(piece, dep):
            pw[NCH, pl.ds(R_END, 8), 0:128] = pltpu.bitcast(dep, u32)
            piece()
        for k, piece in enumerate(pieces):
            clock.add(QP0 + k * (QP1 - QP0) // len(pieces), functools.partial(paced, piece))
        clock.add(la_t, lambda dep: ln1(nx, 0, src, ln_q, dep))
        clock.add(lb_t, lambda dep: ln1(nx, 1, src, ln_q, dep))
        for r0, nt, tiles in ((0, 2, (0, 4, 8)), (TC, 2, (2, 6, 10)), (2 * TC, 1, (12, 13))):
            def R(k):
                return wq[k, pl.ds(r0, nt * 64), :]

            def P(k):
                return _dot_nt(_up(sq_scr[k]), _up(R(k)))

            def T(j, kind):
                return _dot_nt(_up(sq_scr[15 + kind]), _up(R(15 + 3 * j + kind)))

            def PT(k, j, kind):
                return _dot_nt(_up(jnp.concatenate([sq_scr[k], sq_scr[15 + kind]], axis=1)),
                               _up(jnp.concatenate([R(k), R(15 + 3 * j + kind)], axis=1)))

            def tk(np_, v):
                clock.tick(32 * nt * np_, v, QTK if src == 'in' else 4, nt if src == 'in' else 1)

            def emit(col, half, v, np_):
                for k in range(nt):
                    qall[tiles[col] + k, pl.ds(base + (HALO + half * TB), TB), :] = v[:, k * 128:(k + 1) * 128]
                tk(np_, v)
            if src == 'res':
                hk_outputs(P, T, PT, tk, emit, two_cols=(nt == 1))
                continue
            for j in range(len(tiles)):
                both = T(j, 2)
                for t in range(2):
                    lhs = [sq_scr[3 * t + i] for i in range(3)] + [sq_scr[15 + t]]
                    if rows and nt == 1 and (j, t) == QA_DEAD:
                        probe = pltpu.bitcast(o_s[0, pl.ds(zero8, 8), :], u32)
                        lhs[0] = jnp.concatenate([lhs[0][0:8] | (probe & zvec), lhs[0][8:]], axis=0)
                    rhs = [R(wq_slot(i, j)) for i in range(3)] + [R(15 + 3 * j + t)]
                    emit(j, t, _dot_nt(_up(jnp.concatenate(lhs, axis=1)), _up(jnp.concatenate(rhs, axis=1))) + both,
                         5 - t)
        assert not clock.jobs
        q_left(src == 'in')

    def a_rows(blk, par, mode, start=None):
        lag_mid, lag_end = mode
        base = blk * TB if isinstance(blk, int) else pl.multiple_of(blk * TB, TB)
        cbits = pltpu.bitcast(jnp.full((RB, 128), c2e, f32), u32)
        lo = lax.broadcasted_iota(jnp.int32, (RB, 128), 1) < KY
        mid, fin = {}, {}
        for r in range(nr):
            r0 = r * RB
            deps = [start] if (start is not None and r == 0) else []
            if lag_mid and r >= lag_mid:
                deps.append(mid[r - lag_mid])
            if lag_end and r >= lag_end:
                deps += fin[r - lag_end]
            if deps:
                acc = _tree(jnp.bitwise_or, [pltpu.bitcast(v, u32) for v in deps])
                cs = pltpu.bitcast(cbits | (acc & zvec), f32)
            else:
                cs = c2e

            def ld(t, w):
                return qall[t, pl.ds(base + (HALO + r0 - DIL * w), RB), :]
            q = [ld(t, 0) * cs for t in QT] + [jnp.where(lo, pltpu.roll(ld(13, 0), KY, 1), 0.0) * cs]
            sc = []
            for w in range(W):
                acc = None
                for j, t in enumerate(KT):
                    p = q[j] * ld(t, w)
                    acc = p if acc is None else acc + p
                acc = acc + pltpu.roll(acc, 64, 1)
                mid[r] = acc
                acc = acc + pltpu.roll(acc, 32, 1)
                if r0 - DIL * w < 0:
                    pos = blk * TB + r0 + lax.broadcasted_iota(jnp.int32, (RB, 128), 0)
                    acc = jnp.where(pos >= DIL * w, acc, neg)
                sc.append(acc)
            m = _tree(jnp.maximum, sc)
            e = [jnp.exp2(sc[w] - m) for w in range(W)]
            l = _tree(jnp.add, e)
            rinv = pl.reciprocal(l, approx=True)
            rinv = rinv * (2.0 - l * rinv)
            fin[r] = []
            for j, t in enumerate(VT):
                acc = None
                for w in range(W):
                    p = e[w] * ld(t, w)
                    acc = p if acc is None else acc + p
                o = acc * rinv
                o_s[par * 5 + j, pl.ds(r0, RB), :] = o
                fin[r].append(o)

    def a_wo(blk0, ln, off, cb=None):
        lo = lax.broadcasted_iota(jnp.int32, (TB, 128), 1) < KY
        hh = DHALF // 2
        base = 15 * (D3 // 2)

        def O(t, j):
            return o_s[t * 5 + j, pl.ds(off, TB), :]

        def rem(t):
            o3, o4 = O(t, 3), O(t, 4)
            rhs = (o3, jnp.where(lo, o3, o4), jnp.where(lo, o4, o3))
            u, v, w_ = [_dot_nt(_up(wo2[pl.ds(base + k * hh, hh), :]), rhs[k].astype(bf16)) for k in range(3)]
            return xres[blk0 + t] + jnp.concatenate([u + w_, v + w_], axis=0)
        rhs = _hk_b([[O(t, j) for t in range(2)] for j in range(3)])
        prod = [None] * 15
        rems = []
        for pos, k in enumerate(WORD):
            if pos in (0, 2):
                rems.append(rem(len(rems)))
            prod[k] = _dot_nt(_up(wo2[pl.ds(k * (D3 // 2), D3 // 2), :]), rhs[k].astype(bf16))
            if cb is not None:
                cb(pos, prod[k])
        for t in range(2):
            y = jnp.concatenate([_ssum([(prod[k], sg) for k, sg in _HK_C[i, t]]) for i in range(3)], axis=0)
            x1 = y + rems[t]
            xres[blk0 + t] = x1
            mean, rstd = _ln_stats(x1, ln[0], (lambda v: tie(v, prev)) if (t and LNSER and ln[1]) else None)
            xn = normalize(blk0 + t, mean, rstd, ln[1])
            prev = xn[0:8]
            xn_f[t, pl.ds(zero8 if XNF else 0, D), :] = xn

    def a_left(slot):
        def put(i, v):
            s_scr[slot, i] = v
        left_ops(xn_f, put)

    k0 = math.sqrt(2.0 / math.pi)
    k1 = k0 * 0.044715

    def ffn(j, c0, script):
        clock = _Timeline()
        sb = j % 2
        b0 = (2 * j) % NB
        an = (2 * j + 2) % NB
        acc = [None] * 15
        hs = {}
        state = dict(sdep=False, odep=False)
        hk = KY // 2

        def gu(p):
            c = c0 + p

            def R(n):
                return pw[c, pl.ds(n * (TC // 2), TC // 2), :]

            def RT(jc, kind):
                r0 = R_TR + jc * (KR // 2)
                a_, b_ = ((0, 1), (0, 2), (2, 1))[kind]
                return jnp.concatenate([pw[c, pl.ds(r0 + a_ * hk, hk), :], pw[c, pl.ds(r0 + b_ * hk, hk), :]], axis=0)

            def P(n):
                lhs = s_scr[sb, n]
                if state['odep']:
                    probe = pltpu.bitcast(o_s[0, pl.ds(zero8, 8), :], u32)
                    lhs = jnp.concatenate([lhs[0:8] | (probe & zvec), lhs[8:]], axis=0)
                    state['odep'] = False
                return _dot(_up(lhs), _up(R(n)))

            def T(jc, kind):
                return _dot(_up(s_scr[sb, 15 + kind]), _up(RT(jc, kind)))

            def PT(n, jc, kind):
                return _dot(_up(jnp.concatenate([s_scr[sb, n], s_scr[sb, 15 + kind]], axis=1)),
                            _up(jnp.concatenate([R(n), RT(jc, kind)], axis=0)))
            h = [[None, None] for _ in range(3)]

            def emit(col, half, v, np_):
                gg = v[:, :TC]
                gu_ = gg * v[:, TC:]
                h[col][half] = gu_ + gu_ * jnp.tanh(gg * (k0 + k1 * (gg * gg)))
                clock.tick(64 * np_, h[col][half])
            hk_outputs(P, T, PT, lambda np_, v: clock.tick(64 * np_, v), emit)
            hs[p] = h

        def down(ps):
            rhs = [_hk_b(hs.pop(p)) for p in ps]
            for pos, i in enumerate(DORD):
                au = [pw[c0 + p, pl.ds(R_SD + (i // 2) * (D3 // 2), D3 // 2), (i % 2) * TC:(i % 2 + 1) * TC]
                      for p in ps]
                if state['sdep'] and pos == SDEAD:
                    probe = s_scr[1 - sb, 17, pl.ds(zero8, 8), :]
                    au[0] = jnp.concatenate([au[0][0:8] | (probe & zvec), au[0][8:]], axis=0)
                    state['sdep'] = False
                r = _dot_nt(jnp.concatenate([_up(v) for v in au], axis=1),
                            jnp.concatenate([r_[i] for r_ in rhs], axis=1).astype(bf16))
                acc[i] = r if acc[i] is None else r + acc[i]
                clock.tick(48 * len(ps), acc[i])

        pg = pd = 0
        for tok in script:
            if tok == 'G':
                gu(pg)
                pg += 1
            elif tok[0] == 'D':
                down(list(range(pd, pd + int(tok[1:]))))
                pd += int(tok[1:])
            elif tok == 'W':
                assert not clock.jobs
                a_wo(an, LN_P, zero8)
                clock.t += 1152
            elif tok[0] == 'Y':
                def hold(dep):
                    o_s[10, pl.ds(0, 8), :] = dep
                clock.add(clock.t + int(tok[2:]), hold)
            elif tok == 'X':
                state['odep'] = True
            elif tok == 'S':
                a_left(1 - sb)
                state['sdep'] = SDEAD >= 0
            else:
                par = 0 if tok[1] == 'a' else 1
                clock.add(clock.t + int(tok[3:] or 0), functools.partial(a_rows, an + par, par, MODE_P))
        assert pg == pd and not clock.jobs
        for t in range(2):
            y = jnp.concatenate([_ssum([(acc[k], sg) for k, sg in _HK_C[i, t]]) for i in range(3)], axis=0)
            x2 = xres[b0 + t] + 0.5 * y
            xres[b0 + t] = x2
            o_ref[:, t * TB:(t + 1) * TB] = x2.astype(o_ref.dtype)

    plan = []
    nxt = 0
    for n_ in PLAN:
        plan.append(list(range(nxt, nxt + n_)))
        nxt += n_

    def prologue():
        cp_x(0).start()
        for sec in range(3):
            for cp in cp_qkv(sec):
                cp.start()
        for n_ in range(NP):
            for k in range(CP):
                plan_s[n_ * CP + k] = plan[n_][k] if k < len(plan[n_]) else NCH
        qall[:, pl.ds(0, HALO), :] = jnp.zeros((16, HALO, 128), f32)
        cp_x(0).wait()
        ln1(0, 0, 'in', (4, 0))
        ln1(0, 1, 'in', (4, 0))
        q_left(True)
        for sec in range(3):
            for cp in cp_qkv(sec):
                cp.wait()
            if sec == 0:
                cp_x(1).start()
                cp_x(2).start()
                cp_wo().start()
                for c in range(NCH):
                    for cp in cp_chunk(c):
                        cp.start()
                    if 3 + c < NP:
                        cp_x(3 + c).start()
            transpose_qkv(sec)
            build_wq(sec)

    def first_attention():
        q_step(1, [], 'in', CFG_QA, rows=True)
        cp_wo().wait()
        build_wo()

        def cb(pos, v):
            if pos % 4 == 2 or pos == 0:
                for k in range(8):
                    wq[27, pl.ds(zero8, 8), :] = pltpu.bitcast(v[k * 24:k * 24 + 8], u32)
                    build_wq_sums([todo.pop(0)])
        todo = list(range(0, 320, 8))
        a_wo(0, (4, 0), 0, cb)
        assert not todo
        a_left(0)

    def startup_step(n, carry):
        for n_ in range(NP):
            @pl.when(n == n_)
            def _():
                if n_ + 1 < NP:
                    cp_x(n_ + 1).wait()
                for c in plan[n_]:
                    for cp in cp_chunk(c):
                        cp.wait()

        @pl.when(n != 1)
        def _():
            if ONLY in ('', 'q'):
                q_step(n, [plan_s[n * CP + k] for k in range(CP)], 'in', CFG_Q1)

        @pl.when(n == 1)
        def _():
            if ONLY in ('', 'a'):
                first_attention()
        return carry

    @pl.when(g == 0)
    def _():
        if ONLY in ('', 'pro'):
            prologue()
        if ONLY in ('', 'q', 'a'):
            lax.fori_loop(0, NP, startup_step, 0)
        if not ONLY:
            for c in range(nxt, NCH):
                for cp in cp_chunk(c):
                    cp.wait()
                for piece in prep_pieces(c):
                    piece()

    @pl.when(jnp.logical_and(g >= NP - 1, g < 2 * NP - 1))
    def _():
        @pl.when(g == NP - 1)
        def _():
            if ONLY in ('', 'pro'):
                ln1(0, 0, 'res', (4, 0))
                ln1(0, 1, 'res', (4, 0))
                q_left(False)
        if ONLY in ('', 'q'):
            q_step(g - (NP - 1), [], 'res', CFG_Q2)

    if ONLY in ('q', 'a', 'pro'):
        @pl.when(g == 2 * NP - 1)
        def _():
            o_ref[0:16, 0:128] = (qall[g % 16, pl.ds(zero8, 16), :] + xres[g % 16, pl.ds(zero8, 16), :]
                                  + pltpu.bitcast(pw[g % 8, pl.ds(zero8, 16), 0:128] | s_scr[g % 2, g % 8, pl.ds(zero8, 16), :]
                                                  | wo2[pl.ds(zero8, 16), :] | wq[g % 8, pl.ds(zero8, 16), :] | sq_scr[g % 8, pl.ds(zero8, 16), :], f32)).astype(bf16)

    @pl.when(g < 2 * NP - 1)
    def _():
        if ONLY in ('', 'p'):
            ffn(g, 0, SCRIPT)

    @pl.when(g == 2 * NP - 1)
    def _():
        def body(hf, carry):
            ffn(2 * NP - 1, hf * NPC, SCRIPT_F)
            return carry
        if ONLY in ('', 'f'):
            lax.fori_loop(0, 2, body, 0)


@jax.jit
def pallas_interleave_layers__sliding_local_dilated__glu_gated_geglu__prompt_kernel(
    A_x, A_wqkv, A_wo, B_x, B_w_gate, B_w_up, B_w_down):
    B, S, D = A_x.shape
    DF = B_w_gate.shape[1]
    NB = S // TB
    NP = NB // 2
    NCH = DF // CW
    xT = A_x.reshape(S, D).T
    wdT = B_w_down.T
    hbm = pl.BlockSpec(memory_space=pltpu.HBM)
    outT = pl.pallas_call(
        functools.partial(_kernel, D=D, DF=DF, S=S),
        grid=(2 * NP,),
        in_specs=[hbm] * 6,
        out_specs=pl.BlockSpec((D, 2 * TB), lambda g: (0, jnp.maximum(g - NP, 0))),
        out_shape=jax.ShapeDtypeStruct((D, S), A_x.dtype),
        scratch_shapes=[
            pltpu.VMEM((NP, D, 2 * TB), bf16),
            pltpu.VMEM((D, 3 * D), bf16),
            pltpu.VMEM((D, D), bf16),
            pltpu.VMEM((5, 14 * 128, 128), f32),
            pltpu.VMEM((28, 320, 128), u32),
            pltpu.VMEM((D // 2, 640), u32),
            pltpu.VMEM((15 * (D // 6) + 3 * (D // 4) + 16, 128), u32),
            pltpu.VMEM((NCH + 1, 3, D, CW), bf16),
            pltpu.VMEM((NCH + 1, 15 * (TC // 2) + 3 * (D - CW) // 2 + 8 * (D // 6) + 16, 2 * TC), u32),
            pltpu.VMEM((16, S + QPAD, 128), f32),
            pltpu.VMEM((11, TB, 128), f32),
            pltpu.VMEM((NB, D, TB), f32),
            pltpu.VMEM((2, D, TB), f32),
            pltpu.VMEM((2, D, TB), f32),
            pltpu.VMEM((2, 18, TB // 2, TC), u32),
            pltpu.VMEM((18, TB // 2, TC), u32),
            pltpu.SMEM((NP * CP,), jnp.int32),
            pltpu.SemaphoreType.DMA((4 + NP + NCH,)),
        ],
        compiler_params=pltpu.CompilerParams(
            dimension_semantics=("arbitrary",),
            vmem_limit_bytes=110 * 1024 * 1024,
            disable_bounds_checks=bool(NOCHK),
            disable_semaphore_checks=bool(NOCHK),
        ),
    )(xT, A_wqkv, A_wo, B_w_gate, B_w_up, wdT)
    return outT.T.reshape(B, S, D)
```

```python
import functools
import math
import jax
import jax.numpy as jnp
from jax import lax
import jax.experimental.pallas as pl
import jax.experimental.pallas.tpu as pltpu

H = 32
DH = 18
W = 8
DIL = 2
HALO = 16
EPS = 1e-5
TB = 128
RB = 8
TC = 128
CW = 3 * TC
KY = 64
ONLY = ''
LN_P = tuple(int(x) for x in '1,2'.split(','))
CFG_Q1 = tuple(int(x) for x in '1,2,1500,2500'.split(','))
CFG_Q2 = tuple(int(x) for x in '1,2,60,560'.split(','))
QP0 = int(200); QP1 = int(4000); QTK = int(16)
MODE_P = tuple(int(x) for x in '1,3'.split(','))
MODE_A = tuple(int(x) for x in '1,3'.split(','))
SCRIPT = 'G,G,G,G,ra+1600,G,D4,X,G,G,G,rb+1700,G,D4,G,X,G,Y0+1400,G,W,n0+100,n1+388,l0+1162,l1+1312,D4'.split(',')
SCRIPT_F = 'G,G,G,D2,G,G,G,D2,D2'.split(',')
DORD = tuple(int(x) for x in '2,3,12,4,5,13,14,0,9,10,1,6,7,8,11'.split(','))
SDEAD = int(13)
PLAN = tuple(int(x) for x in '0,0,2,2,2,1,2,2'.split(','))
CP = 2
CFG_QA = tuple(int(x) for x in '1,2,200,500'.split(','))
QA_T = tuple(int(x) for x in '100,800'.split(','))
QA_DEAD = tuple(int(x) for x in '1,1'.split(','))
QPAD = int(40)
LNJ = tuple(int(x) for x in '4,4,72,48'.split(','))
DTK = int(8)
XNF = int(1); XNL = int(1); NLEFT = int(2)
YSPLIT = tuple(int(x) for x in '0,21'.split(','))
WORD = tuple(int(x) for x in '6,7,8,9,0,10,11,1,2,12,13,14,3,4,5'.split(','))
NOCHK = int(1)

f32 = jnp.float32
bf16 = jnp.bfloat16
u32 = jnp.uint32
NT = (((1,), (1,)), ((), ()))


def _unpk(u, idx):
    return pltpu.unpack_elementwise(u, index=idx, packed_dtype=bf16, unpacked_dtype=f32)


def _pk2(even, odd):
    return pltpu.pack_elementwise([even, odd], packed_dtype=bf16).astype(u32)


def _up(x):
    return pltpu.bitcast(x, bf16)


def _dot(a, b):
    return jnp.dot(a, b, preferred_element_type=f32)


def _dot_nt(a, b):
    return lax.dot_general(a, b, NT, preferred_element_type=f32)


def _tree(fn, xs):
    xs = list(xs)
    while len(xs) > 1:
        xs = [fn(xs[i], xs[i + 1]) for i in range(0, len(xs) - 1, 2)] + ([xs[-1]] if len(xs) % 2 else [])
    return xs[0]


def _ln_stats(x, nacc, pin=None):
    n = x.shape[0]
    c = x[0:1] if pin is None else pin(x[0:8])[0:1]
    s1 = [None] * nacc
    s2 = [None] * nacc
    for i in range(n // 8):
        d = x[i * 8:(i + 1) * 8] - c
        k = i % nacc
        s1[k] = d if s1[k] is None else s1[k] + d
        dd = d * d
        s2[k] = dd if s2[k] is None else s2[k] + dd
    m = jnp.sum(_tree(jnp.add, s1), axis=0, keepdims=True) * (1.0 / n)
    v = jnp.sum(_tree(jnp.add, s2), axis=0, keepdims=True) * (1.0 / n) - m * m
    v = jnp.maximum(v, 0.0)
    return c + m, lax.rsqrt(v + EPS)


_HK_A = (
    ((0, 0, 1), (0, 2, -1), (1, 0, -1)), ((0, 0, 1), (0, 1, -1), (2, 0, -1)), ((1, 1, 1), (0, 1, -1), (1, 2, -1)),
    ((1, 1, 1), (1, 0, -1), (2, 1, -1)), ((2, 2, 1), (0, 2, -1), (2, 1, -1)), ((2, 2, 1), (1, 2, -1), (2, 0, -1)),
    ((0, 1, 1),), ((0, 1, 1), (1, 0, -1)), ((1, 0, 1),),
    ((0, 2, 1),), ((0, 2, 1), (2, 0, -1)), ((2, 0, 1),),
    ((1, 2, 1),), ((2, 1, 1), (1, 2, -1)), ((2, 1, 1),),
)
_HK_C = {
    (0, 0): ((0, 1), (7, 1), (8, 1), (9, 1), (6, -1)),
    (0, 1): ((1, 1), (6, 1), (10, 1), (11, 1), (9, -1)),
    (1, 0): ((2, 1), (7, 1), (8, 1), (12, 1), (6, -1)),
    (1, 1): ((3, 1), (6, 1), (13, 1), (14, 1), (2, -1), (7, -1)),
    (2, 0): ((5, 1), (9, 1), (12, 1), (13, 1), (4, -1), (10, -1)),
    (2, 1): ((4, 1), (10, 1), (11, 1), (14, 1), (9, -1)),
}


def _hk_b(b):
    s1 = b[1][0] + b[1][1]
    s2 = b[2][0] + b[2][1]
    t7 = b[0][1] + s1
    t10 = b[0][0] + s2
    return (b[0][0], b[0][1], b[1][0], s1, b[2][1], s2, b[0][1] + b[1][1], t7, b[0][0] + t7,
            b[0][0] + b[2][0], t10, b[0][1] + t10, b[1][0] + b[2][0], b[1][0] - b[2][1], b[1][1] + b[2][1])


def _ssum(terms):
    terms = sorted([t for t in terms if t[0] is not None], key=lambda z: -z[1])
    if not terms:
        return None
    acc = terms[0][0] if terms[0][1] == 1 else -terms[0][0]
    for v, sg in terms[1:]:
        acc = acc + v if sg == 1 else acc - v
    return acc


class _Timeline:
    def __init__(self):
        self.t = 0
        self.jobs = []

    def add(self, when, fn):
        self.jobs.append((when, len(self.jobs), fn))
        self.jobs.sort(key=lambda z: z[:2])

    def tick(self, dur, v, n=1, seq=1):
        per = max(n // seq, 1)
        for k in range(n):
            self.t += dur // n
            r = (k % per) * (v.shape[0] // per)
            c = (k // per) * 128
            while self.jobs and self.jobs[0][0] <= self.t:
                self.jobs.pop(0)[2](v[r:r + 8, c:c + 128])


def _kernel(x_hbm, wqkv_hbm, wo_hbm, wg_hbm, wu_hbm, wd_hbm, o_ref,
            xin, wqkv_raw, wo_raw, tmp, wq, woT, wo2, raw, pw, qall, o_s, xres, xn_f, xn_g, s_scr, sq_scr,
            plan_s, sems, *, D, DF, S):
    g = pl.program_id(0)
    NB = S // TB
    NP = NB // 2
    NCH = DF // CW
    NPC = NCH // 2
    D3 = D // 3
    DHALF = D // 2
    KR = D - 3 * TC
    nr = TB // RB
    hh = DHALF // 2
    zero8 = pl.multiple_of((g >> 20) * 8, 8)
    zvec = jnp.full((8, 128), (g >> 20).astype(u32), u32)

    def tie(x, dep):
        return pltpu.bitcast(pltpu.bitcast(x, u32) | (pltpu.bitcast(dep, u32) & zvec), f32)

    QSEC = ((0, 5), (5, 9), (9, 14))

    def cp_qkv(sec):
        out = []
        for j in range(*QSEC[sec]):
            n = min(128, 3 * D - j * 128)
            out.append(pltpu.make_async_copy(wqkv_hbm.at[:, pl.ds(j * 128, n)], wqkv_raw.at[:, pl.ds(j * 128, n)],
                                             sems.at[sec]))
        return out

    def cp_wo():
        return pltpu.make_async_copy(wo_hbm, wo_raw, sems.at[3])

    def cp_x(k):
        return pltpu.make_async_copy(x_hbm.at[:, pl.ds(k * 2 * TB, 2 * TB)], xin.at[k], sems.at[4 + k])

    def cp_chunk(c):
        return [pltpu.make_async_copy(w.at[:, pl.ds(c * CW, CW)], raw.at[c, m], sems.at[4 + NP + c])
                for m, w in enumerate((wg_hbm, wu_hbm, wd_hbm))]

    R_TR = 15 * (TC // 2)
    R_SD = R_TR + 3 * (KR // 2)
    R_END = R_SD + 8 * (D3 // 2)

    def hk_a_ops(load):
        blk = {}
        for i in range(3):
            for j in range(3):
                u = load(i, j)
                blk[i, j] = (u, _unpk(u, 0), _unpk(u, 1))
        out = []
        for terms in _HK_A:
            if len(terms) == 1:
                out.append(blk[terms[0][:2]][0])
            else:
                out.append(_pk2(_ssum([(blk[i, j][1], sg) for i, j, sg in terms]),
                                _ssum([(blk[i, j][2], sg) for i, j, sg in terms])))
        return out

    def prep_pieces(c):
        def hk_piece(m, r):
            rb = D3 if m == 2 else TC
            ops = hk_a_ops(lambda i, j: pltpu.bitcast(raw[c, m, pl.ds(i * rb + r, 16), pl.ds(j * TC, TC)], u32))
            for k, t in enumerate(ops):
                if m == 2:
                    pw[c, pl.ds(R_SD + (k // 2) * (D3 // 2) + r // 2, 8), (k % 2) * TC:(k % 2 + 1) * TC] = t
                else:
                    pw[c, pl.ds(k * (TC // 2) + r // 2, 8), m * TC:(m + 1) * TC] = t

        def rem_piece(m, j):
            pw[c, pl.ds(R_TR + j * (KR // 2), KR // 2), m * TC:(m + 1) * TC] = pltpu.bitcast(
                raw[c, m, pl.ds(3 * TC, KR), pl.ds(j * TC, TC)], u32)

        out = []
        for m in range(2):
            out += [functools.partial(hk_piece, m, r) for r in range(0, TC, 16)]
            out += [functools.partial(rem_piece, m, j) for j in range(3)]
        out += [functools.partial(hk_piece, 2, r) for r in range(0, D3, 16)]
        return out

    def transpose_qkv(sec):
        for j in range(*QSEC[sec]):
            wd_ = min(128, 3 * D - j * 128)
            blk = wqkv_raw[:, j * 128:j * 128 + wd_].astype(f32)
            if wd_ < 128:
                blk = jnp.concatenate([blk, jnp.zeros((D, 128 - wd_), f32)], axis=1)
            bt = jnp.concatenate([blk, blk[D - KY:]], axis=0).T
            for t in range(5):
                tmp[t, pl.ds(j * 128, 128), :] = bt[:, t * 128:(t + 1) * 128]

    def wq_slot(i, j):
        return 24 + i if i == j else [n for n, t in enumerate(_HK_A) if t == ((i, j, 1),)][0]

    def build_wq(sec):
        lo = lax.broadcasted_iota(jnp.int32, (16, 128), 1) < KY
        for d in range(DH):
            tt = [_pk2(tmp[t, pl.ds(sec * D + d, 16, stride=2 * DH), :],
                       tmp[t, pl.ds(sec * D + d + DH, 16, stride=2 * DH), :]) for t in range(5)]
            ops = tt[:4] + [jnp.where(lo, tt[3], tt[4]), jnp.where(lo, tt[4], tt[3])]
            if d < 16:
                dst = [(sec, d * 16)]
            else:
                dst = ([(1, (d + 2) * 16)], [(1, d * 16)], [(0, d * 16), (0, (d + 2) * 16)])[sec]
            for j, row in dst:
                for k, v in enumerate(ops):
                    wq[wq_slot(k, j) if k < 3 else 12 + 3 * j + k, pl.ds(row, 16), :] = v

    def build_wq_sums(rs):
        for r in rs:
            ncol = 3 if r < 256 else 2
            blk = {}
            for i in range(3):
                for j in range(ncol):
                    u = wq[wq_slot(i, j), pl.ds(r, 8), :]
                    blk[i, j] = (_unpk(u, 0), _unpk(u, 1))
            for n, terms in enumerate(_HK_A):
                if len(terms) == 1 or (ncol == 2 and n in (4, 5)):
                    continue
                wq[n, pl.ds(r, 8), :] = _pk2(*[_ssum([(blk[i, j][p_], sg) for i, j, sg in terms if j < ncol])
                                               for p_ in range(2)])

    def build_wo():
        for t in range(5):
            wd_ = min(128, D - t * 128)
            blk = wo_raw[:, t * 128:t * 128 + wd_].astype(f32)
            if wd_ < 128:
                blk = jnp.concatenate([blk, jnp.zeros((D, 128 - wd_), f32)], axis=1)
            tmp[t, pl.ds(0, D), :] = blk
        for t in range(5):
            rows = [tmp[t, pl.ds(d, 32, stride=DH), :] for d in range(DH)]
            ft = jnp.concatenate(rows + rows[16:], axis=0).T
            n = min(128, D - t * 128)
            woT[pl.ds(t * 64, n // 2), :] = pltpu.bitcast(ft[:n].astype(bf16), u32)
        for r in range(0, D3 // 2, 8):
            ops = hk_a_ops(lambda i, j: woT[pl.ds(i * (D3 // 2) + r, 8), j * TC:(j + 1) * TC])
            for k, t in enumerate(ops):
                wo2[pl.ds(k * (D3 // 2) + r, 8), :] = t
        lo = lax.broadcasted_iota(jnp.int32, (8, 128), 1) < KY
        for r in range(0, hh, 8):
            a3, a4 = woT[pl.ds(r, 8), 384:512], woT[pl.ds(r, 8), 512:640]
            b3, b4 = woT[pl.ds(hh + r, 8), 384:512], woT[pl.ds(hh + r, 8), 512:640]

            def dif(u, v):
                return _pk2(_unpk(u, 0) - _unpk(v, 0), _unpk(u, 1) - _unpk(v, 1))
            base = 15 * (D3 // 2)
            wo2[pl.ds(base + r, 8), :] = jnp.where(lo, a3, dif(a3, b3))
            wo2[pl.ds(base + hh + r, 8), :] = jnp.where(lo, b3, dif(b4, a4))
            wo2[pl.ds(base + 2 * hh + r, 8), :] = jnp.where(lo, a4, b3)

    def normalize(blk, mean, rstd, link):
        if not link:
            return (xres[blk] - mean) * rstd
        rs = jnp.broadcast_to(rstd, (8, TB))
        mb = jnp.broadcast_to(mean, (8, TB))
        outs = []
        for i in range(D // 8):
            if i and i % link == 0:
                rs = tie(rs, outs[-1])
            outs.append((xres[blk, pl.ds(i * 8, 8), :] - mb) * rs)
        return jnp.concatenate(outs, axis=0)

    def left_ops(src, put, plain=False, which=None, dep=None):
        def X(t, r0, n):
            return src[t, pl.ds(r0, n), :]
        k1, k2, k3 = 3 * TC, 3 * TC + KY, 3 * TC + 2 * KY
        for n in (list(range(6 if plain else 15)) + [15, 16, 17]) if which is None else which:
            if n == 15:
                v = jnp.concatenate([X(0, k1, KY), X(0, k2, KY) - X(1, k2, KY)], axis=0)
            elif n == 16:
                v = jnp.concatenate([X(1, k1, KY), X(1, k3, KY) - X(0, k3, KY)], axis=0)
            elif n == 17:
                v = jnp.concatenate([X(0, k3, KY), X(1, k2, KY)], axis=0)
            elif plain:
                v = X(n // 3, (n % 3) * TC, TC)
            else:
                v = _ssum([(X(t, i * TC, TC), sg) for (i, t), lst in _HK_C.items() for k, sg in lst if k == n])
            if dep is not None:
                v = jnp.concatenate([tie(v[0:8], dep), v[8:]], axis=0)
            put(n, pltpu.bitcast(v.astype(bf16).T, u32))

    def ln1(pr, par, src, ln, dep=None):
        blk = 2 * pr + par
        if src == 'res':
            x = xres[blk]
        else:
            x = xin[pr, :, par * TB:(par + 1) * TB].astype(f32)
            xres[blk] = x
        mean, rstd = _ln_stats(x, ln[0], None if dep is None else (lambda v: tie(v, dep)))
        if src == 'res':
            xn_g[par, pl.ds(0, 8), :] = jnp.zeros((8, TB), f32)
        xn_g[par, pl.ds(zero8, D), :] = normalize(blk, mean, rstd, ln[1])

    def q_left(plain):
        def put(i, v):
            sq_scr[i] = v
        left_ops(xn_g, put, plain)

    def hk_outputs(P, T, PT, tk, emit, two_cols=False):
        p8 = P(8)
        t7 = P(7) + p8
        tk(2, t7)
        s1 = PT(3, 1, 2) + t7
        tk(2, s1)
        p6 = P(6)
        p14 = P(14)
        tk(2, p14)
        emit(1, 1, T(1, 1) + (p6 + p14 + s1), 1)
        p13 = P(13)
        if two_cols:
            emit(1, 0, PT(2, 1, 0) + (p13 + s1), 3)
        else:
            p12 = P(12)
            tk(2, p12)
            emit(1, 0, PT(2, 1, 0) + (p12 + p13 + s1), 2)
        p11 = P(11)
        t10 = P(10) + p11
        tk(2, t10)
        if not two_cols:
            s2 = PT(5, 2, 2) + t10
            tk(2, s2)
            p9 = P(9)
            emit(2, 0, T(2, 0) + (p9 + p12 + s2), 2)
            emit(2, 1, PT(4, 2, 1) + (p14 - p13 + s2), 2)
        w0 = T(0, 2)
        emit(0, 0, PT(0, 0, 0) + ((p8 + t10 + w0) if two_cols else (p8 + p9 + t10 + w0)), 3)
        emit(0, 1, PT(1, 0, 1) + (p6 + p11 + t7 + w0), 2)

    QT = (0, 1, 2, 3)
    KT = (4, 5, 6, 7, 13)
    VT = (8, 9, 10, 11, 12)
    c2e = DH ** -0.5 * math.log2(math.e)
    neg = -1e9 * math.log2(math.e)

    def q_step(pr, cs, src, cfg, rows=False):
        clock = _Timeline()
        if rows:
            base, nx = pr * (2 * TB), pr + 1
            clock.add(QA_T[0], functools.partial(a_rows, 0, 0, MODE_A))
            clock.add(QA_T[1], functools.partial(a_rows, 1, 1, MODE_A))
        else:
            base = pl.multiple_of(pr * (2 * TB), 2 * TB)
            nx = jnp.minimum(pr + 1, NP - 1)
        ln_q, la_t, lb_t = cfg[:2], cfg[2], cfg[3]
        pieces = []
        for c in cs:
            pieces += prep_pieces(c)

        def paced(piece, dep):
            pw[NCH, pl.ds(R_END, 8), 0:128] = pltpu.bitcast(dep, u32)
            piece()
        for k, piece in enumerate(pieces):
            clock.add(QP0 + k * (QP1 - QP0) // len(pieces), functools.partial(paced, piece))
        clock.add(la_t, lambda dep: ln1(nx, 0, src, ln_q, dep))
        clock.add(lb_t, lambda dep: ln1(nx, 1, src, ln_q, dep))
        for r0, nt, tiles in ((0, 2, (0, 4, 8)), (TC, 2, (2, 6, 10)), (2 * TC, 1, (12, 13))):
            def R(k):
                return wq[k, pl.ds(r0, nt * 64), :]

            def P(k):
                return _dot_nt(_up(sq_scr[k]), _up(R(k)))

            def T(j, kind):
                return _dot_nt(_up(sq_scr[15 + kind]), _up(R(15 + 3 * j + kind)))

            def PT(k, j, kind):
                return _dot_nt(_up(jnp.concatenate([sq_scr[k], sq_scr[15 + kind]], axis=1)),
                               _up(jnp.concatenate([R(k), R(15 + 3 * j + kind)], axis=1)))

            def tk(np_, v):
                clock.tick(32 * nt * np_, v, QTK if src == 'in' else 4, nt if src == 'in' else 1)

            def emit(col, half, v, np_):
                for k in range(nt):
                    qall[tiles[col] + k, pl.ds(base + (HALO + half * TB), TB), :] = v[:, k * 128:(k + 1) * 128]
                tk(np_, v)
            if src == 'res':
                hk_outputs(P, T, PT, tk, emit, two_cols=(nt == 1))
                continue
            for j in range(len(tiles)):
                both = T(j, 2)
                for t in range(2):
                    lhs = [sq_scr[3 * t + i] for i in range(3)] + [sq_scr[15 + t]]
                    if rows and nt == 1 and (j, t) == QA_DEAD:
                        probe = pltpu.bitcast(o_s[0, pl.ds(zero8, 8), :], u32)
                        lhs[0] = jnp.concatenate([lhs[0][0:8] | (probe & zvec), lhs[0][8:]], axis=0)
                    rhs = [R(wq_slot(i, j)) for i in range(3)] + [R(15 + 3 * j + t)]
                    emit(j, t, _dot_nt(_up(jnp.concatenate(lhs, axis=1)), _up(jnp.concatenate(rhs, axis=1))) + both,
                         5 - t)
        assert not clock.jobs
        q_left(src == 'in')

    def a_rows(blk, par, mode, start=None):
        lag_mid, lag_end = mode
        base = blk * TB if isinstance(blk, int) else pl.multiple_of(blk * TB, TB)
        cbits = pltpu.bitcast(jnp.full((RB, 128), c2e, f32), u32)
        lo = lax.broadcasted_iota(jnp.int32, (RB, 128), 1) < KY
        mid, fin = {}, {}
        for r in range(nr):
            r0 = r * RB
            deps = [start] if (start is not None and r == 0) else []
            if lag_mid and r >= lag_mid:
                deps.append(mid[r - lag_mid])
            if lag_end and r >= lag_end:
                deps += fin[r - lag_end]
            if deps:
                acc = _tree(jnp.bitwise_or, [pltpu.bitcast(v, u32) for v in deps])
                cs = pltpu.bitcast(cbits | (acc & zvec), f32)
            else:
                cs = c2e

            def ld(t, w):
                return qall[t, pl.ds(base + (HALO + r0 - DIL * w), RB), :]
            q = [ld(t, 0) * cs for t in QT] + [jnp.where(lo, pltpu.roll(ld(13, 0), KY, 1), 0.0) * cs]
            sc = []
            for w in range(W):
                acc = None
                for j, t in enumerate(KT):
                    p = q[j] * ld(t, w)
                    acc = p if acc is None else acc + p
                acc = acc + pltpu.roll(acc, 64, 1)
                mid[r] = acc
                acc = acc + pltpu.roll(acc, 32, 1)
                if r0 - DIL * w < 0:
                    pos = blk * TB + r0 + lax.broadcasted_iota(jnp.int32, (RB, 128), 0)
                    acc = jnp.where(pos >= DIL * w, acc, neg)
                sc.append(acc)
            m = _tree(jnp.maximum, sc)
            e = [jnp.exp2(sc[w] - m) for w in range(W)]
            l = _tree(jnp.add, e)
            rinv = pl.reciprocal(l, approx=True)
            rinv = rinv * (2.0 - l * rinv)
            fin[r] = []
            for j, t in enumerate(VT):
                acc = None
                for w in range(W):
                    p = e[w] * ld(t, w)
                    acc = p if acc is None else acc + p
                o = acc * rinv
                o_s[par * 5 + j, pl.ds(r0, RB), :] = o
                fin[r].append(o)

    wo_seq = []
    for pos, k in enumerate(WORD):
        if pos in (0, 2):
            wo_seq += [('r', pos // 2, k_) for k_ in range(3)]
        wo_seq.append(('p', k))

    def wo_rhs(items, off, rhs):
        lo = lax.broadcasted_iota(jnp.int32, (TB, 128), 1) < KY

        def O(t, j):
            return o_s[t * 5 + j, pl.ds(off, TB), :]
        hkb = _hk_b([[O(t, j) for t in range(2)] for j in range(3)])
        for it in items:
            if it[0] == 'p':
                v = hkb[it[1]]
            else:
                o3, o4 = O(it[1], 3), O(it[1], 4)
                v = (o3, jnp.where(lo, o3, o4), jnp.where(lo, o4, o3))[it[2]]
            rhs[it] = v.astype(bf16)

    def wo_mm(blk0, rhs, cb=None):
        res = {}
        for pos, it in enumerate(wo_seq):
            if it[0] == 'p':
                lhs = wo2[pl.ds(it[1] * (D3 // 2), D3 // 2), :]
            else:
                lhs = wo2[pl.ds(15 * (D3 // 2) + it[2] * hh, hh), :]
            res[it] = _dot_nt(_up(lhs), rhs[it])
            if cb is not None:
                cb(pos, res[it])
        for t in range(2):
            both = res['r', t, 2]
            rem = xres[blk0 + t] + jnp.concatenate([res['r', t, 0] + both, res['r', t, 1] + both], axis=0)
            y = jnp.concatenate([_ssum([(res['p', k], sg) for k, sg in _HK_C[i, t]]) for i in range(3)], axis=0)
            xres[blk0 + t] = y + rem

    def ln2(blk, par, ln, dep=None):
        mean, rstd = _ln_stats(xres[blk, pl.ds(zero8 if XNL else 0, D), :], ln[0],
                               None if dep is None else (lambda v: tie(v, dep)))
        xn_f[par, pl.ds(0, 8), :] = jnp.zeros((8, TB), f32)
        xn_f[par, pl.ds(zero8 if XNF else 0, D), :] = normalize(blk, mean, rstd, ln[1])

    def ln_jobs(blk, dst, par, np1, np2):
        st = dict(s1=[], s2=[])
        nv = D // 8

        def stats(k, dep):
            if k == 0:
                st['c'] = jnp.broadcast_to(xres[blk, pl.ds(zero8, 8), :][0:1], (8, TB))
            c = tie(st['c'], dep)
            ds = [xres[blk, pl.ds(zero8 + i * 8, 8), :] - c for i in range(k * nv // np1, (k + 1) * nv // np1)]
            st['s1'].append(_tree(jnp.add, ds))
            st['s2'].append(_tree(jnp.add, [d * d for d in ds]))

        def norm(k, dep):
            if k == 0:
                m = jnp.sum(_tree(jnp.add, st['s1']), axis=0, keepdims=True) * (1.0 / D)
                v = jnp.sum(_tree(jnp.add, st['s2']), axis=0, keepdims=True) * (1.0 / D) - m * m
                st['mean'] = st['c'] + m
                st['rstd'] = jnp.broadcast_to(lax.rsqrt(jnp.maximum(v, 0.0) + EPS), (8, TB))
            mean = tie(st['mean'], dep)
            for i in range(k * nv // np2, (k + 1) * nv // np2):
                dst[par, pl.ds(zero8 + i * 8, 8), :] = (xres[blk, pl.ds(i * 8, 8), :] - mean) * st['rstd']
        return [functools.partial(stats, k) for k in range(np1)], [functools.partial(norm, k) for k in range(np2)]

    def a_left(slot, which=None, dep=None):
        def put(i, v):
            s_scr[slot, i] = v
        left_ops(xn_f, put, which=which, dep=dep)

    k0 = math.sqrt(2.0 / math.pi)
    k1 = k0 * 0.044715

    def ffn(j, c0, script):
        clock = _Timeline()
        sb = j % 2
        b0 = (2 * j) % NB
        an = (2 * j + 2) % NB
        acc = [None] * 15
        hs = {}
        wrhs = {}
        state = dict(sdep=False, odep=False)
        hk = KY // 2

        def gu(p):
            c = c0 + p

            def R(n):
                return pw[c, pl.ds(n * (TC // 2), TC // 2), :]

            def RT(jc, kind):
                r0 = R_TR + jc * (KR // 2)
                a_, b_ = ((0, 1), (0, 2), (2, 1))[kind]
                return jnp.concatenate([pw[c, pl.ds(r0 + a_ * hk, hk), :], pw[c, pl.ds(r0 + b_ * hk, hk), :]], axis=0)

            def P(n):
                lhs = s_scr[sb, n]
                if state['odep']:
                    probe = pltpu.bitcast(o_s[0, pl.ds(zero8, 8), :], u32)
                    lhs = jnp.concatenate([lhs[0:8] | (probe & zvec), lhs[8:]], axis=0)
                    state['odep'] = False
                return _dot(_up(lhs), _up(R(n)))

            def T(jc, kind):
                return _dot(_up(s_scr[sb, 15 + kind]), _up(RT(jc, kind)))

            def PT(n, jc, kind):
                return _dot(_up(jnp.concatenate([s_scr[sb, n], s_scr[sb, 15 + kind]], axis=1)),
                            _up(jnp.concatenate([R(n), RT(jc, kind)], axis=0)))
            h = [[None, None] for _ in range(3)]

            def emit(col, half, v, np_):
                gg = v[:, :TC]
                gu_ = gg * v[:, TC:]
                h[col][half] = gu_ + gu_ * jnp.tanh(gg * (k0 + k1 * (gg * gg)))
                clock.tick(64 * np_, h[col][half])
            hk_outputs(P, T, PT, lambda np_, v: clock.tick(64 * np_, v), emit)
            hs[p] = h

        def down(ps):
            rhs = [_hk_b(hs.pop(p)) for p in ps]
            for pos, i in enumerate(DORD):
                au = [pw[c0 + p, pl.ds(R_SD + (i // 2) * (D3 // 2), D3 // 2), (i % 2) * TC:(i % 2 + 1) * TC]
                      for p in ps]
                if state['sdep'] and pos >= SDEAD:
                    probe = s_scr[1 - sb, 17, pl.ds(zero8, 8), :]
                    au[0] = jnp.concatenate([au[0][0:8] | (probe & zvec), au[0][8:]], axis=0)
                    state['sdep'] = False
                r = _dot_nt(jnp.concatenate([_up(v) for v in au], axis=1),
                            jnp.concatenate([r_[i] for r_ in rhs], axis=1).astype(bf16))
                acc[i] = r if acc[i] is None else r + acc[i]
                clock.tick(48 * len(ps), acc[i], DTK)

        pg = pd = 0
        for tok in script:
            if tok == 'G':
                gu(pg)
                pg += 1
            elif tok[0] == 'D':
                down(list(range(pd, pd + int(tok[1:]))))
                pd += int(tok[1:])
            elif tok == 'W':
                assert not clock.jobs
                wo_mm(an, wrhs)
                clock.t += 1152
            elif tok[0] == 'Y':
                def hold(items, dep):
                    o_s[10, pl.ds(0, 8), :] = dep
                    wo_rhs(items, zero8, wrhs)
                lo_, hi_ = YSPLIT[int(tok[1])], YSPLIT[int(tok[1]) + 1]
                clock.add(clock.t + int(tok[3:]), functools.partial(hold, wo_seq[lo_:hi_]))
            elif tok == 'X':
                state['odep'] = True
            elif tok[0] == 'n':
                j1, j2 = ln_jobs(an + int(tok[1]), xn_f, int(tok[1]), LNJ[0], LNJ[1])
                t_ = clock.t + int(tok[3:])
                for job in j1:
                    clock.add(t_, job)
                    t_ += LNJ[2]
                t_ += LNJ[3]
                for job in j2:
                    clock.add(t_, job)
                    t_ += LNJ[2]
            elif tok[0] == 'l':
                def left(which, last, dep):
                    a_left(1 - sb, which, dep)
                    state['sdep'] = last and SDEAD >= 0
                k_ = int(tok[1])
                clock.add(clock.t + int(tok[3:]),
                          functools.partial(left, list(range(k_ * 18 // NLEFT, (k_ + 1) * 18 // NLEFT)), k_ == NLEFT - 1))
            else:
                par = 0 if tok[1] == 'a' else 1
                clock.add(clock.t + int(tok[3:] or 0), functools.partial(a_rows, an + par, par, MODE_P))
        assert pg == pd and not clock.jobs
        for t in range(2):
            y = jnp.concatenate([_ssum([(acc[k], sg) for k, sg in _HK_C[i, t]]) for i in range(3)], axis=0)
            x2 = xres[b0 + t] + 0.5 * y
            xres[b0 + t] = x2
            o_ref[:, t * TB:(t + 1) * TB] = x2.astype(o_ref.dtype)

    plan = []
    nxt = 0
    for n_ in PLAN:
        plan.append(list(range(nxt, nxt + n_)))
        nxt += n_

    def prologue():
        cp_x(0).start()
        for sec in range(3):
            for cp in cp_qkv(sec):
                cp.start()
        for n_ in range(NP):
            for k in range(CP):
                plan_s[n_ * CP + k] = plan[n_][k] if k < len(plan[n_]) else NCH
        qall[:, pl.ds(0, HALO), :] = jnp.zeros((16, HALO, 128), f32)
        cp_x(0).wait()
        ln1(0, 0, 'in', (4, 0))
        ln1(0, 1, 'in', (4, 0))
        q_left(True)
        for sec in range(3):
            for cp in cp_qkv(sec):
                cp.wait()
            if sec == 0:
                cp_x(1).start()
                cp_x(2).start()
                cp_wo().start()
                for c in range(NCH):
                    for cp in cp_chunk(c):
                        cp.start()
                    if 3 + c < NP:
                        cp_x(3 + c).start()
            transpose_qkv(sec)
            build_wq(sec)

    def first_attention():
        q_step(1, [], 'in', CFG_QA, rows=True)
        cp_wo().wait()
        build_wo()

        def cb(pos, v):
            if pos in (3, 8, 12, 16, 20):
                for k in range(8):
                    wq[27, pl.ds(zero8, 8), :] = pltpu.bitcast(v[k * 24:k * 24 + 8], u32)
                    build_wq_sums([todo.pop(0)])
        todo = list(range(0, 320, 8))
        rhs = {}
        wo_rhs(wo_seq, 0, rhs)
        wo_mm(0, rhs, cb)
        assert not todo
        ln2(0, 0, (4, 0))
        ln2(1, 1, (4, 0))
        a_left(0)

    def startup_step(n, carry):
        for n_ in range(NP):
            @pl.when(n == n_)
            def _():
                if n_ + 1 < NP:
                    cp_x(n_ + 1).wait()
                for c in plan[n_]:
                    for cp in cp_chunk(c):
                        cp.wait()

        @pl.when(n != 1)
        def _():
            if ONLY in ('', 'q'):
                q_step(n, [plan_s[n * CP + k] for k in range(CP)], 'in', CFG_Q1)

        @pl.when(n == 1)
        def _():
            if ONLY in ('', 'a'):
                first_attention()
        return carry

    @pl.when(g == 0)
    def _():
        if ONLY in ('', 'pro'):
            prologue()
        if ONLY in ('', 'q', 'a'):
            lax.fori_loop(0, NP, startup_step, 0)
        if not ONLY:
            for c in range(nxt, NCH):
                for cp in cp_chunk(c):
                    cp.wait()
                for piece in prep_pieces(c):
                    piece()

    @pl.when(jnp.logical_and(g >= NP - 1, g < 2 * NP - 1))
    def _():
        @pl.when(g == NP - 1)
        def _():
            if ONLY in ('', 'pro'):
                ln1(0, 0, 'res', (4, 0))
                ln1(0, 1, 'res', (4, 0))
                q_left(False)
        if ONLY in ('', 'q'):
            q_step(g - (NP - 1), [], 'res', CFG_Q2)

    if ONLY in ('q', 'a', 'pro'):
        @pl.when(g == 2 * NP - 1)
        def _():
            o_ref[0:16, 0:128] = (qall[g % 16, pl.ds(zero8, 16), :] + xres[g % 16, pl.ds(zero8, 16), :]
                                  + pltpu.bitcast(pw[g % 8, pl.ds(zero8, 16), 0:128] | s_scr[g % 2, g % 8, pl.ds(zero8, 16), :]
                                                  | wo2[pl.ds(zero8, 16), :] | wq[g % 8, pl.ds(zero8, 16), :] | sq_scr[g % 8, pl.ds(zero8, 16), :], f32)).astype(bf16)

    @pl.when(g < 2 * NP - 1)
    def _():
        if ONLY in ('', 'p'):
            ffn(g, 0, SCRIPT)

    @pl.when(g == 2 * NP - 1)
    def _():
        def body(hf, carry):
            ffn(2 * NP - 1, hf * NPC, SCRIPT_F)
            return carry
        if ONLY in ('', 'f'):
            lax.fori_loop(0, 2, body, 0)


@jax.jit
def pallas_interleave_layers__sliding_local_dilated__glu_gated_geglu__prompt_kernel(
    A_x, A_wqkv, A_wo, B_x, B_w_gate, B_w_up, B_w_down):
    B, S, D = A_x.shape
    DF = B_w_gate.shape[1]
    NB = S // TB
    NP = NB // 2
    NCH = DF // CW
    xT = A_x.reshape(S, D).T
    wdT = B_w_down.T
    hbm = pl.BlockSpec(memory_space=pltpu.HBM)
    outT = pl.pallas_call(
        functools.partial(_kernel, D=D, DF=DF, S=S),
        grid=(2 * NP,),
        in_specs=[hbm] * 6,
        out_specs=pl.BlockSpec((D, 2 * TB), lambda g: (0, jnp.maximum(g - NP, 0))),
        out_shape=jax.ShapeDtypeStruct((D, S), A_x.dtype),
        scratch_shapes=[
            pltpu.VMEM((NP, D, 2 * TB), bf16),
            pltpu.VMEM((D, 3 * D), bf16),
            pltpu.VMEM((D, D), bf16),
            pltpu.VMEM((5, 14 * 128, 128), f32),
            pltpu.VMEM((28, 320, 128), u32),
            pltpu.VMEM((D // 2, 640), u32),
            pltpu.VMEM((15 * (D // 6) + 3 * (D // 4) + 16, 128), u32),
            pltpu.VMEM((NCH + 1, 3, D, CW), bf16),
            pltpu.VMEM((NCH + 1, 15 * (TC // 2) + 3 * (D - CW) // 2 + 8 * (D // 6) + 16, 2 * TC), u32),
            pltpu.VMEM((16, S + QPAD, 128), f32),
            pltpu.VMEM((11, TB, 128), f32),
            pltpu.VMEM((NB, D, TB), f32),
            pltpu.VMEM((2, D, TB), f32),
            pltpu.VMEM((2, D, TB), f32),
            pltpu.VMEM((2, 18, TB // 2, TC), u32),
            pltpu.VMEM((18, TB // 2, TC), u32),
            pltpu.SMEM((NP * CP,), jnp.int32),
            pltpu.SemaphoreType.DMA((4 + NP + NCH,)),
        ],
        compiler_params=pltpu.CompilerParams(
            dimension_semantics=("arbitrary",),
            vmem_limit_bytes=110 * 1024 * 1024,
            disable_bounds_checks=bool(NOCHK),
            disable_semaphore_checks=bool(NOCHK),
        ),
    )(xT, A_wqkv, A_wo, B_w_gate, B_w_up, wdT)
    return outT.T.reshape(B, S, D)
```

```python
import functools
import math
import jax
import jax.numpy as jnp
from jax import lax
import jax.experimental.pallas as pl
import jax.experimental.pallas.tpu as pltpu

H = 32
DH = 18
W = 8
DIL = 2
HALO = 16
EPS = 1e-5
TB = 128
RB = 8
TC = 128
CW = 6 * TC
KY = 64
ONLY = ''
LN_P = tuple(int(x) for x in '1,2'.split(','))
CFG_Q1 = tuple(int(x) for x in '1,2,1500,2500'.split(','))
CFG_Q2 = tuple(int(x) for x in '1,2,60,560'.split(','))
QP0 = int(200); QP1 = int(4000); QTK = int(16)
MODE_P = tuple(int(x) for x in '1,3'.split(','))
MODE_A = tuple(int(x) for x in '1,3'.split(','))
SCRIPT = 'G,G,G,G,ra+30,D4,X,G,G,G,rb+1100,G,D4,W,n0+1500,n1+2364,l+3328+600,G,G,G,G,c+200+120,D4'.split(',')
SCRIPT_F = 'G,G,G,G,D2,G,G,D2,D2'.split(',')
DORD = tuple(int(x) for x in '1,6,0,9,10,4,11,5,14,7,2,8,3,12,13'.split(','))
GU_LAG = int(2); D_LAG = int(3)
CP = 3
JDL = int(400); LDL = int(1000); GTK = int(2)
PLAG = int(5); DADV = int(1)
UFIRST = int(0); USCR = int(0)
CFG_QA = tuple(int(x) for x in '1,2,200,500'.split(','))
QA_T = tuple(int(x) for x in '100,800'.split(','))
QA_DEAD = tuple(int(x) for x in '1,1'.split(','))
QPAD = int(40)
LNJ = tuple(int(x) for x in '8,8,48,96'.split(','))
DTK = int(8)
XNF = int(1); XNL = int(1); NLEFT = int(3)
YSPLIT = tuple(int(x) for x in '0,21'.split(','))
WORD = tuple(int(x) for x in '0,1,2,6,7,8,9,10,11,12,13,14,3,4,5'.split(','))
NOCHK = int(1)

f32 = jnp.float32
bf16 = jnp.bfloat16
u32 = jnp.uint32
NT = (((1,), (1,)), ((), ()))


def _unpk(u, idx):
    return pltpu.unpack_elementwise(u, index=idx, packed_dtype=bf16, unpacked_dtype=f32)


def _pk2(even, odd):
    return pltpu.pack_elementwise([even, odd], packed_dtype=bf16).astype(u32)


def _up(x):
    return pltpu.bitcast(x, bf16)


def _dot(a, b):
    return jnp.dot(a, b, preferred_element_type=f32)


def _dot_nt(a, b):
    return lax.dot_general(a, b, NT, preferred_element_type=f32)


def _tree(fn, xs):
    xs = list(xs)
    while len(xs) > 1:
        xs = [fn(xs[i], xs[i + 1]) for i in range(0, len(xs) - 1, 2)] + ([xs[-1]] if len(xs) % 2 else [])
    return xs[0]


def _ln_stats(x, nacc, pin=None):
    n = x.shape[0]
    c = x[0:1] if pin is None else pin(x[0:8])[0:1]
    s1 = [None] * nacc
    s2 = [None] * nacc
    for i in range(n // 8):
        d = x[i * 8:(i + 1) * 8] - c
        k = i % nacc
        s1[k] = d if s1[k] is None else s1[k] + d
        dd = d * d
        s2[k] = dd if s2[k] is None else s2[k] + dd
    m = jnp.sum(_tree(jnp.add, s1), axis=0, keepdims=True) * (1.0 / n)
    v = jnp.sum(_tree(jnp.add, s2), axis=0, keepdims=True) * (1.0 / n) - m * m
    v = jnp.maximum(v, 0.0)
    return c + m, lax.rsqrt(v + EPS)


_HK_A = (
    ((0, 0, 1), (0, 2, -1), (1, 0, -1)), ((0, 0, 1), (0, 1, -1), (2, 0, -1)), ((1, 1, 1), (0, 1, -1), (1, 2, -1)),
    ((1, 1, 1), (1, 0, -1), (2, 1, -1)), ((2, 2, 1), (0, 2, -1), (2, 1, -1)), ((2, 2, 1), (1, 2, -1), (2, 0, -1)),
    ((0, 1, 1),), ((0, 1, 1), (1, 0, -1)), ((1, 0, 1),),
    ((0, 2, 1),), ((0, 2, 1), (2, 0, -1)), ((2, 0, 1),),
    ((1, 2, 1),), ((2, 1, 1), (1, 2, -1)), ((2, 1, 1),),
)
_HK_C = {
    (0, 0): ((0, 1), (7, 1), (8, 1), (9, 1), (6, -1)),
    (0, 1): ((1, 1), (6, 1), (10, 1), (11, 1), (9, -1)),
    (1, 0): ((2, 1), (7, 1), (8, 1), (12, 1), (6, -1)),
    (1, 1): ((3, 1), (6, 1), (13, 1), (14, 1), (2, -1), (7, -1)),
    (2, 0): ((5, 1), (9, 1), (12, 1), (13, 1), (4, -1), (10, -1)),
    (2, 1): ((4, 1), (10, 1), (11, 1), (14, 1), (9, -1)),
}


_HK_B = (((0, 0, 1),), ((0, 1, 1),), ((1, 0, 1),), ((1, 0, 1), (1, 1, 1)), ((2, 1, 1),), ((2, 0, 1), (2, 1, 1)),
         ((0, 1, 1), (1, 1, 1)), ((0, 1, 1), (1, 0, 1), (1, 1, 1)), ((0, 0, 1), (0, 1, 1), (1, 0, 1), (1, 1, 1)),
         ((0, 0, 1), (2, 0, 1)), ((0, 0, 1), (2, 0, 1), (2, 1, 1)), ((0, 0, 1), (0, 1, 1), (2, 0, 1), (2, 1, 1)),
         ((1, 0, 1), (2, 0, 1)), ((1, 0, 1), (2, 1, -1)), ((1, 1, 1), (2, 1, 1)))


def _hk_b(b):
    s1 = b[1][0] + b[1][1]
    s2 = b[2][0] + b[2][1]
    t7 = b[0][1] + s1
    t10 = b[0][0] + s2
    return (b[0][0], b[0][1], b[1][0], s1, b[2][1], s2, b[0][1] + b[1][1], t7, b[0][0] + t7,
            b[0][0] + b[2][0], t10, b[0][1] + t10, b[1][0] + b[2][0], b[1][0] - b[2][1], b[1][1] + b[2][1])


def _ssum(terms):
    terms = sorted([t for t in terms if t[0] is not None], key=lambda z: -z[1])
    if not terms:
        return None
    acc = terms[0][0] if terms[0][1] == 1 else -terms[0][0]
    for v, sg in terms[1:]:
        acc = acc + v if sg == 1 else acc - v
    return acc


GU_ORD = tuple(int(x) for x in '8,6,7,11,3,1,10,14,9,5,0,13,12,4,2'.split(','))
GU_POST = {
    8: ((), ('p8', None), None),
    7: ((('p8', 1),), (None, 't7'), None),
    3: ((('t7', 1),), (None, 's1'), None),
    6: ((), ('p6', None), None),
    14: ((('p6', 1), ('s1', 1)), ('p14', None), (1, 1)),
    12: ((('p9', 1), ('s2', 1)), ('p12', None), (2, 0)),
    13: ((), ('p13', None), None),
    2: ((('p12', 1), ('p13', 1), ('s1', 1)), (None, None), (1, 0)),
    11: ((), ('p11', None), None),
    10: ((('p11', 1),), (None, 't10'), None),
    5: ((('t10', 1),), (None, 's2'), None),
    9: ((), ('p9', None), None),
    4: ((('p14', 1), ('s2', 1), ('p13', -1)), (None, None), (2, 1)),
    0: ((('p8', 1), ('p9', 1), ('t10', 1)), (None, None), (0, 0)),
    1: ((('p6', 1), ('p11', 1), ('t7', 1)), (None, None), (0, 1)),
}
PSLOT = {k: i for i, k in enumerate(('p8', 't7', 's1', 'p6', 'p14', 'p12', 'p13', 'p11', 't10', 's2', 'p9'))}


class _Timeline:
    def __init__(self):
        self.t = 0
        self.jobs = []

    def add(self, when, fn):
        self.jobs.append((when, len(self.jobs), fn))
        self.jobs.sort(key=lambda z: z[:2])

    def tick(self, dur, v, n=1, seq=1):
        per = max(n // seq, 1)
        for k in range(n):
            self.t += dur // n
            r = (k % per) * (v.shape[0] // per)
            c = (k // per) * 128
            while self.jobs and self.jobs[0][0] <= self.t:
                self.jobs.pop(0)[2](v[r:r + 8, c:c + 128])


def _kernel(x_hbm, wqkv_hbm, wo_hbm, wg_hbm, wu_hbm, wd_hbm, o_ref,
            xin, wqkv_raw, wo_raw, tmp, wq, woT, wo2, raw, pw, qall, o_s, xres, xn_f, xn_g, s_scr, st_s, sq_scr,
            plan_s, sems, *p_s, D, DF, S):
    g = pl.program_id(0)
    NB = S // TB
    NP = NB // 2
    NCH = DF // CW
    NPC = NCH // 2
    D3 = D // 3
    DHALF = D // 2
    nr = TB // RB
    hh = DHALF // 2
    zero8 = pl.multiple_of((g >> 20) * 8, 8)
    zvec = jnp.full((8, 128), (g >> 20).astype(u32), u32)
    zeros = [pl.multiple_of((g >> (8 + k)) * 8, 8) for k in range(21)]

    def tie(x, dep):
        return pltpu.bitcast(pltpu.bitcast(x, u32) | (pltpu.bitcast(dep, u32) & zvec), f32)

    QSEC = ((0, 5), (5, 9), (9, 14))

    def cp_qkv(sec):
        out = []
        for j in range(*QSEC[sec]):
            n = min(128, 3 * D - j * 128)
            out.append(pltpu.make_async_copy(wqkv_hbm.at[:, pl.ds(j * 128, n)], wqkv_raw.at[:, pl.ds(j * 128, n)],
                                             sems.at[sec]))
        return out

    def cp_wo():
        return pltpu.make_async_copy(wo_hbm, wo_raw, sems.at[3])

    def cp_x(k):
        return pltpu.make_async_copy(x_hbm.at[:, pl.ds(k * 2 * TB, 2 * TB)], xin.at[k], sems.at[4 + k])

    def cp_unit(c, m):
        return pltpu.make_async_copy((wg_hbm, wu_hbm, wd_hbm)[m].at[:, pl.ds(c * CW, CW)], raw.at[c, m],
                                     sems.at[4 + NP + 3 * c + m])

    R_SD = 45 * (TC // 2)
    R_END = R_SD + 15 * (D3 // 2)

    def hk_a_ops(load, minus=None):
        blk = {}
        for i in range(3):
            for j in range(3):
                u = load(i, j)
                if minus is None:
                    blk[i, j] = (u, _unpk(u, 0), _unpk(u, 1))
                else:
                    v = minus(i, j)
                    blk[i, j] = (None, _unpk(u, 0) - _unpk(v, 0), _unpk(u, 1) - _unpk(v, 1))
        out = []
        for terms in _HK_A:
            if len(terms) == 1 and minus is None:
                out.append(blk[terms[0][:2]][0])
            else:
                out.append(_pk2(_ssum([(blk[i, j][1], sg) for i, j, sg in terms]),
                                _ssum([(blk[i, j][2], sg) for i, j, sg in terms])))
        return out

    def prep_pieces(c, m):
        def ld(r, cs):
            return lambda i, j: pltpu.bitcast(raw[c, m, pl.ds(i * D3 + r, 16), pl.ds((3 * cs + j) * TC, TC)], u32)

        def gu_piece(q, r, cs, neg, kind, half):
            ops = hk_a_ops(ld(q * KY + r, cs), None if neg is None else ld(q * KY + r, neg))
            for k, t in enumerate(ops):
                pw[c, pl.ds((3 * k + kind) * (TC // 2) + (half * KY + r) // 2, 8), m * TC:(m + 1) * TC] = t

        def d_piece(r, cs):
            for k, t in enumerate(hk_a_ops(ld(r, cs))):
                pw[c, pl.ds(R_SD + k * (D3 // 2) + r // 2, 8), cs * TC:(cs + 1) * TC] = t
        if m == 2:
            return [functools.partial(d_piece, r, cs) for r in range(0, D3, 16) for cs in range(2)]
        spec = ((0, 0, None, 0, 0), (1, 0, 1, 0, 1), (0, 1, None, 1, 0), (2, 1, 0, 1, 1),
                (2, 0, None, 2, 0), (1, 1, None, 2, 1))
        return [functools.partial(gu_piece, q, r, cs, neg, kind, half)
                for r in range(0, KY, 16) for q, cs, neg, kind, half in spec]

    def transpose_qkv(sec):
        for j in range(*QSEC[sec]):
            wd_ = min(128, 3 * D - j * 128)
            blk = wqkv_raw[:, j * 128:j * 128 + wd_].astype(f32)
            if wd_ < 128:
                blk = jnp.concatenate([blk, jnp.zeros((D, 128 - wd_), f32)], axis=1)
            bt = jnp.concatenate([blk, blk[D - KY:]], axis=0).T
            for t in range(5):
                tmp[t, pl.ds(j * 128, 128), :] = bt[:, t * 128:(t + 1) * 128]

    def wq_slot(i, j):
        return 24 + i if i == j else [n for n, t in enumerate(_HK_A) if t == ((i, j, 1),)][0]

    def build_wq(sec):
        lo = lax.broadcasted_iota(jnp.int32, (16, 128), 1) < KY
        for d in range(DH):
            tt = [_pk2(tmp[t, pl.ds(sec * D + d, 16, stride=2 * DH), :],
                       tmp[t, pl.ds(sec * D + d + DH, 16, stride=2 * DH), :]) for t in range(5)]
            ops = tt[:4] + [jnp.where(lo, tt[3], tt[4]), jnp.where(lo, tt[4], tt[3])]
            if d < 16:
                dst = [(sec, d * 16)]
            else:
                dst = ([(1, (d + 2) * 16)], [(1, d * 16)], [(0, d * 16), (0, (d + 2) * 16)])[sec]
            for j, row in dst:
                for k, v in enumerate(ops):
                    wq[wq_slot(k, j) if k < 3 else 12 + 3 * j + k, pl.ds(row, 16), :] = v

    def build_wq_sums(rs):
        for r in rs:
            ncol = 3 if r < 256 else 2
            blk = {}
            for i in range(3):
                for j in range(ncol):
                    u = wq[wq_slot(i, j), pl.ds(r, 8), :]
                    blk[i, j] = (_unpk(u, 0), _unpk(u, 1))
            for n, terms in enumerate(_HK_A):
                if len(terms) == 1 or (ncol == 2 and n in (4, 5)):
                    continue
                wq[n, pl.ds(r, 8), :] = _pk2(*[_ssum([(blk[i, j][p_], sg) for i, j, sg in terms if j < ncol])
                                               for p_ in range(2)])

    def build_wo():
        for t in range(5):
            wd_ = min(128, D - t * 128)
            blk = wo_raw[:, t * 128:t * 128 + wd_].astype(f32)
            if wd_ < 128:
                blk = jnp.concatenate([blk, jnp.zeros((D, 128 - wd_), f32)], axis=1)
            tmp[t, pl.ds(0, D), :] = blk
        for t in range(5):
            rows = [tmp[t, pl.ds(d, 32, stride=DH), :] for d in range(DH)]
            ft = jnp.concatenate(rows + rows[16:], axis=0).T
            n = min(128, D - t * 128)
            woT[pl.ds(t * 64, n // 2), :] = pltpu.bitcast(ft[:n].astype(bf16), u32)
        for r in range(0, D3 // 2, 8):
            ops = hk_a_ops(lambda i, j: woT[pl.ds(i * (D3 // 2) + r, 8), j * TC:(j + 1) * TC])
            for k, t in enumerate(ops):
                wo2[pl.ds(k * (D3 // 2) + r, 8), :] = t
        lo = lax.broadcasted_iota(jnp.int32, (8, 128), 1) < KY
        for r in range(0, hh, 8):
            a3, a4 = woT[pl.ds(r, 8), 384:512], woT[pl.ds(r, 8), 512:640]
            b3, b4 = woT[pl.ds(hh + r, 8), 384:512], woT[pl.ds(hh + r, 8), 512:640]

            def dif(u, v):
                return _pk2(_unpk(u, 0) - _unpk(v, 0), _unpk(u, 1) - _unpk(v, 1))
            base = 15 * (D3 // 2)
            wo2[pl.ds(base + r, 8), :] = jnp.where(lo, a3, dif(a3, b3))
            wo2[pl.ds(base + hh + r, 8), :] = jnp.where(lo, b3, dif(b4, a4))
            wo2[pl.ds(base + 2 * hh + r, 8), :] = jnp.where(lo, a4, b3)

    def normalize(blk, mean, rstd, link):
        if not link:
            return (xres[blk] - mean) * rstd
        rs = jnp.broadcast_to(rstd, (8, TB))
        mb = jnp.broadcast_to(mean, (8, TB))
        outs = []
        for i in range(D // 8):
            if i and i % link == 0:
                rs = tie(rs, outs[-1])
            outs.append((xres[blk, pl.ds(i * 8, 8), :] - mb) * rs)
        return jnp.concatenate(outs, axis=0)

    def left_ops(src, put, plain=False, which=None, dep=None):
        def X(t, r0, n):
            return src[t, pl.ds(r0, n), :]
        k1, k2, k3 = 3 * TC, 3 * TC + KY, 3 * TC + 2 * KY
        for n in (list(range(6 if plain else 15)) + [15, 16, 17]) if which is None else which:
            if n == 15:
                v = jnp.concatenate([X(0, k1, KY), X(0, k2, KY) - X(1, k2, KY)], axis=0)
            elif n == 16:
                v = jnp.concatenate([X(1, k1, KY), X(1, k3, KY) - X(0, k3, KY)], axis=0)
            elif n == 17:
                v = jnp.concatenate([X(0, k3, KY), X(1, k2, KY)], axis=0)
            elif plain:
                v = X(n // 3, (n % 3) * TC, TC)
            else:
                v = _ssum([(X(t, i * TC, TC), sg) for (i, t), lst in _HK_C.items() for k, sg in lst if k == n])
            if dep is not None:
                v = jnp.concatenate([tie(v[0:8], dep), v[8:]], axis=0)
            put(n, pltpu.bitcast(v.astype(bf16).T, u32))

    def ln1(pr, par, src, ln, dep=None):
        blk = 2 * pr + par
        if src == 'res':
            x = xres[blk]
        else:
            x = xin[pr, :, par * TB:(par + 1) * TB].astype(f32)
            xres[blk] = x
        mean, rstd = _ln_stats(x, ln[0], None if dep is None else (lambda v: tie(v, dep)))
        if src == 'res':
            xn_g[par, pl.ds(0, 8), :] = jnp.zeros((8, TB), f32)
        xn_g[par, pl.ds(zero8, D), :] = normalize(blk, mean, rstd, ln[1])

    def q_left(plain):
        def put(i, v):
            sq_scr[i] = v
        left_ops(xn_g, put, plain)

    def hk_outputs(P, T, PT, tk, emit, two_cols=False):
        p8 = P(8)
        t7 = P(7) + p8
        tk(2, t7)
        s1 = PT(3, 1, 2) + t7
        tk(2, s1)
        p6 = P(6)
        p14 = P(14)
        tk(2, p14)
        emit(1, 1, T(1, 1) + (p6 + p14 + s1), 1)
        p13 = P(13)
        if two_cols:
            emit(1, 0, PT(2, 1, 0) + (p13 + s1), 3)
        else:
            p12 = P(12)
            tk(2, p12)
            emit(1, 0, PT(2, 1, 0) + (p12 + p13 + s1), 2)
        p11 = P(11)
        t10 = P(10) + p11
        tk(2, t10)
        if not two_cols:
            s2 = PT(5, 2, 2) + t10
            tk(2, s2)
            p9 = P(9)
            emit(2, 0, T(2, 0) + (p9 + p12 + s2), 2)
            emit(2, 1, PT(4, 2, 1) + (p14 - p13 + s2), 2)
        w0 = T(0, 2)
        emit(0, 0, PT(0, 0, 0) + ((p8 + t10 + w0) if two_cols else (p8 + p9 + t10 + w0)), 3)
        emit(0, 1, PT(1, 0, 1) + (p6 + p11 + t7 + w0), 2)

    QT = (0, 1, 2, 3)
    KT = (4, 5, 6, 7, 13)
    VT = (8, 9, 10, 11, 12)
    c2e = DH ** -0.5 * math.log2(math.e)
    neg = -1e9 * math.log2(math.e)

    def q_step(pr, cs, src, cfg, rows=False):
        clock = _Timeline()
        if rows:
            base, nx = pr * (2 * TB), pr + 1
            clock.add(QA_T[0], functools.partial(a_rows, 0, 0, MODE_A))
            clock.add(QA_T[1], functools.partial(a_rows, 1, 1, MODE_A))
        else:
            base = pl.multiple_of(pr * (2 * TB), 2 * TB)
            nx = jnp.minimum(pr + 1, NP - 1)
        ln_q, la_t, lb_t = cfg[:2], cfg[2], cfg[3]
        pieces = []
        for m, c in enumerate(cs):
            pieces += prep_pieces(c, m)

        def paced(piece, dep):
            pw[NCH, pl.ds(R_END, 8), 0:128] = pltpu.bitcast(dep, u32)
            piece()
        for k, piece in enumerate(pieces):
            clock.add(QP0 + k * (QP1 - QP0) // len(pieces), functools.partial(paced, piece))
        clock.add(la_t, lambda dep: ln1(nx, 0, src, ln_q, dep))
        clock.add(lb_t, lambda dep: ln1(nx, 1, src, ln_q, dep))
        for r0, nt, tiles in ((0, 2, (0, 4, 8)), (TC, 2, (2, 6, 10)), (2 * TC, 1, (12, 13))):
            def R(k):
                return wq[k, pl.ds(r0, nt * 64), :]

            def P(k):
                return _dot_nt(_up(sq_scr[k]), _up(R(k)))

            def T(j, kind):
                return _dot_nt(_up(sq_scr[15 + kind]), _up(R(15 + 3 * j + kind)))

            def PT(k, j, kind):
                return _dot_nt(_up(jnp.concatenate([sq_scr[k], sq_scr[15 + kind]], axis=1)),
                               _up(jnp.concatenate([R(k), R(15 + 3 * j + kind)], axis=1)))

            def tk(np_, v):
                clock.tick(32 * nt * np_, v, QTK if src == 'in' else 4, nt if src == 'in' else 1)

            def emit(col, half, v, np_):
                for k in range(nt):
                    qall[tiles[col] + k, pl.ds(base + (HALO + half * TB), TB), :] = v[:, k * 128:(k + 1) * 128]
                tk(np_, v)
            if src == 'res':
                hk_outputs(P, T, PT, tk, emit, two_cols=(nt == 1))
                continue
            for j in range(len(tiles)):
                both = T(j, 2)
                for t in range(2):
                    lhs = [sq_scr[3 * t + i] for i in range(3)] + [sq_scr[15 + t]]
                    if rows and nt == 1 and (j, t) == QA_DEAD:
                        probe = pltpu.bitcast(o_s[0, pl.ds(zero8, 8), :], u32)
                        lhs[0] = jnp.concatenate([lhs[0][0:8] | (probe & zvec), lhs[0][8:]], axis=0)
                    rhs = [R(wq_slot(i, j)) for i in range(3)] + [R(15 + 3 * j + t)]
                    emit(j, t, _dot_nt(_up(jnp.concatenate(lhs, axis=1)), _up(jnp.concatenate(rhs, axis=1))) + both,
                         5 - t)
        assert not clock.jobs
        q_left(src == 'in')

    def a_rows(blk, par, mode, start=None):
        lag_mid, lag_end = mode[:2]
        fw, fv = mode[2:] if len(mode) > 2 else (0, 0)
        base = blk * TB if isinstance(blk, int) else pl.multiple_of(blk * TB, TB)
        cbits = pltpu.bitcast(jnp.full((RB, 128), c2e, f32), u32)
        lo = lax.broadcasted_iota(jnp.int32, (RB, 128), 1) < KY
        mid, fin = {}, {}
        for r in range(nr):
            r0 = r * RB
            deps = [start] if (start is not None and r == 0) else []
            if lag_mid and r >= lag_mid:
                deps.append(mid[r - lag_mid])
            if lag_end and r >= lag_end:
                deps += fin[r - lag_end]
            if deps:
                acc = _tree(jnp.bitwise_or, [pltpu.bitcast(v, u32) for v in deps])
                cs = pltpu.bitcast(cbits | (acc & zvec), f32)
            else:
                cs = c2e

            def ld(t, w):
                return qall[t, pl.ds(base + (HALO + r0 - DIL * w), RB), :]
            q = [ld(t, 0) * cs for t in QT] + [jnp.where(lo, pltpu.roll(ld(13, 0), KY, 1), 0.0) * cs]
            sc = []
            for w in range(W):
                q0 = tie(q[0], prev) if (fw and w and w % fw == 0) else (q[0] if w == 0 else q0)
                acc = None
                for j, t in enumerate(KT):
                    p = (q0 if j == 0 else q[j]) * ld(t, w)
                    acc = p if acc is None else acc + p
                prev = acc
                acc = acc + pltpu.roll(acc, 64, 1)
                mid[r] = acc
                acc = acc + pltpu.roll(acc, 32, 1)
                if r0 - DIL * w < 0:
                    pos = blk * TB + r0 + lax.broadcasted_iota(jnp.int32, (RB, 128), 0)
                    acc = jnp.where(pos >= DIL * w, acc, neg)
                sc.append(acc)
            m = _tree(jnp.maximum, sc)
            e = [jnp.exp2(sc[w] - m) for w in range(W)]
            l = _tree(jnp.add, e)
            rinv = pl.reciprocal(l, approx=True)
            rinv = rinv * (2.0 - l * rinv)
            fin[r] = []
            for j, t in enumerate(VT):
                e0 = tie(e[0], acc) if (fv and j and j % fv == 0) else (e[0] if j == 0 else e0)
                acc = None
                for w in range(W):
                    p = (e0 if w == 0 else e[w]) * ld(t, w)
                    acc = p if acc is None else acc + p
                o = acc * rinv
                o_s[par * 5 + j, pl.ds(r0, RB), :] = o
                fin[r] = [o] if fv == 1 else fin[r] + [o]

    wo_seq = []
    for pos, k in enumerate(WORD):
        if pos in (0, 2):
            wo_seq += [('r', pos // 2, k_) for k_ in range(3)]
        wo_seq.append(('p', k))

    def wo_rhs(items, off, rhs):
        lo = lax.broadcasted_iota(jnp.int32, (TB, 128), 1) < KY

        for it in items:
            z = zeros[wo_seq.index(it)] if off is None else off

            def O(t, j):
                return o_s[t * 5 + j, pl.ds(z, TB), :]
            if it[0] == 'p':
                v = _ssum([(O(t, j), sg) for j, t, sg in _HK_B[it[1]]])
            elif it[2] == 0:
                v = O(it[1], 3)
            else:
                v = jnp.where(lo, O(it[1], 2 + it[2]), O(it[1], 5 - it[2]))
            rhs[it] = v.astype(bf16)

    def wo_mm(blk0, rhs, cb=None):
        res = {}
        for pos, it in enumerate(wo_seq):
            if it[0] == 'p':
                lhs = wo2[pl.ds(it[1] * (D3 // 2), D3 // 2), :]
            else:
                lhs = wo2[pl.ds(15 * (D3 // 2) + it[2] * hh, hh), :]
            res[it] = _dot_nt(_up(lhs), rhs[it])
            if cb is not None:
                cb(pos, res[it])
        for t in range(2):
            both = res['r', t, 2]
            rem = xres[blk0 + t] + jnp.concatenate([res['r', t, 0] + both, res['r', t, 1] + both], axis=0)
            y = jnp.concatenate([_ssum([(res['p', k], sg) for k, sg in _HK_C[i, t]]) for i in range(3)], axis=0)
            xres[blk0 + t] = y + rem

    def ln2(blk, par, ln, dep=None):
        mean, rstd = _ln_stats(xres[blk, pl.ds(zero8 if XNL else 0, D), :], ln[0],
                               None if dep is None else (lambda v: tie(v, dep)))
        xn_f[par, pl.ds(0, 8), :] = jnp.zeros((8, TB), f32)
        xn_f[par, pl.ds(zero8 if XNF else 0, D), :] = normalize(blk, mean, rstd, ln[1])

    def ln_jobs(blk, dst, par, np1, np2):
        st = dict(s1=[], s2=[])
        nv = D // 8

        def stats(k, dep):
            if k == 0:
                st['c'] = jnp.broadcast_to(xres[blk, pl.ds(zero8, 8), :][0:1], (8, TB))
            c = tie(st['c'], dep)
            ds = [xres[blk, pl.ds(zero8 + i * 8, 8), :] - c for i in range(k * nv // np1, (k + 1) * nv // np1)]
            st['s1'].append(_tree(jnp.add, ds))
            st['s2'].append(_tree(jnp.add, [d * d for d in ds]))
            a_, b_ = st['s1'][-1], st['s2'][-1]
            return lambda: pltpu.bitcast(a_, u32) | pltpu.bitcast(b_, u32)

        def norm(k, dep):
            if k == 0:
                m = jnp.sum(_tree(jnp.add, st['s1']), axis=0, keepdims=True) * (1.0 / D)
                v = jnp.sum(_tree(jnp.add, st['s2']), axis=0, keepdims=True) * (1.0 / D) - m * m
                st['mean'] = st['c'] + m
                st['rstd'] = jnp.broadcast_to(lax.rsqrt(jnp.maximum(v, 0.0) + EPS), (8, TB))
            mean = tie(st['mean'], dep)
            for i in range(k * nv // np2, (k + 1) * nv // np2):
                dst[par, pl.ds(i * 8, 8), :] = (xres[blk, pl.ds(i * 8, 8), :] - mean) * st['rstd']
            return lambda: pltpu.bitcast(dst[par, pl.ds(zero8, 8), :], u32)
        return [functools.partial(stats, k) for k in range(np1)], [functools.partial(norm, k) for k in range(np2)]

    def a_left(which=range(15), dep=None):
        for n in which:
            v = _ssum([(xn_f[t, pl.ds(zeros[n] + i * D3, D3), :], sg)
                       for (i, t), lst in _HK_C.items() for k, sg in lst if k == n])
            if dep is not None:
                v = jnp.concatenate([tie(v[0:8], dep), v[8:2 * KY], tie(v[2 * KY:2 * KY + 8], dep), v[2 * KY + 8:]],
                                    axis=0)
            st_s[2 * n] = pltpu.bitcast(v[:2 * KY].astype(bf16).T, u32)
            st_s[2 * n + 1] = pltpu.bitcast(jnp.concatenate([v[2 * KY:], v[2 * KY:]], axis=0).astype(bf16).T, u32)

    def a_arrange(which=range(15), dep=None):
        lo = lax.broadcasted_iota(jnp.int32, (TB // 2, 128), 1) < KY
        if dep is not None:
            st_s[30, pl.ds(0, 8), :] = pltpu.bitcast(dep, u32)
        for n in which:
            t1 = st_s[2 * n, pl.ds(zero8, TB // 2), :]
            t2 = st_s[2 * n + 1, pl.ds(zero8, TB // 2), :]
            s_scr[3 * n] = t1
            s_scr[3 * n + 1] = jnp.where(lo, t1, t2)
            s_scr[3 * n + 2] = jnp.where(lo, t2, t1)

    k0 = math.sqrt(2.0 / math.pi)
    k1 = k0 * 0.044715

    def ffn(j, c0, script):
        clock = _Timeline()
        b0 = (2 * j) % NB
        an = (2 * j + 2) % NB
        acc = [None] * 15
        hs = {}
        wrhs = {}
        state = dict(odep=False, norm=0, left=set())

        pend = []
        fresh = []

        def advance(keep):
            while len(pend) > keep:
                pend.pop(0)()

        def probe_of(ref_val):
            return pltpu.bitcast(ref_val, u32) & zvec

        def take_probe():
            pr = _tree(jnp.bitwise_or, [k() if callable(k) else pltpu.bitcast(p_s[k][pl.ds(zero8, 8), 0:128], u32)
                                        for k in fresh]) & zvec
            del fresh[:]
            return pr

        def with_deadline(job, delay):
            def run(dep):
                val = job(dep)()
                clock.add(clock.t + delay, lambda _: fresh.append(lambda: val))
            return run

        def gu(p):
            c, second = c0 + p // 2, p % 2
            m = 1 - second if UFIRST else second
            h = hs.setdefault(p // 2, [[None, None] for _ in range(3)])

            def mm(n, kind, probe=None):
                lhs = s_scr[3 * n + kind]
                if state['odep']:
                    pr = probe_of(o_s[0, pl.ds(zero8, 8), :])
                    probe = pr if probe is None else probe | pr
                    state['odep'] = False
                if probe is not None:
                    lhs = jnp.concatenate([lhs[0:8] | probe, lhs[8:]], axis=0)
                return _dot(_up(lhs), _up(pw[c, pl.ds((3 * n + kind) * (TC // 2), TC // 2), m * TC:(m + 1) * TC]))

            def get(name):
                return p_s[PSLOT[name]][pl.ds(zero8, TB), :]

            def post(n, v):
                adds, keep, emits = GU_POST[n]
                if keep[0] is not None:
                    p_s[PSLOT[keep[0]]][...] = v
                    fresh.append(PSLOT[keep[0]])
                w_ = v
                for name, sg in adds:
                    w_ = w_ + get(name) if sg == 1 else w_ - get(name)
                if keep[1] is not None:
                    p_s[PSLOT[keep[1]]][...] = w_
                    fresh.append(PSLOT[keep[1]])
                if emits is not None:
                    col, half = emits
                    if m == 0:
                        w_ = w_ + w_ * jnp.tanh(w_ * (k0 + k1 * (w_ * w_)))
                    if second:
                        k_ = 17 + 6 * ((p // 2) % 2) + 2 * col + half
                        p_s[k_][...] = w_ * p_s[11 + 2 * col + half][pl.ds(zero8, TB), :]
                        fresh.append(k_)
                        h[col][half] = k_
                    else:
                        p_s[11 + 2 * col + half][...] = w_
                        fresh.append(11 + 2 * col + half)
            for n in GU_ORD:
                both = mm(n, 2, take_probe() if fresh else None)
                v = jnp.concatenate([mm(n, 0) + both, mm(n, 1) + both], axis=1)
                pend.append(functools.partial(post, n, v))
                advance(PLAG)
                clock.tick(96, both, GTK)

        def down(ps):
            cs = ps[::2]
            hsl = [hs.pop(p // 2) for p in cs]
            for pos, i in enumerate(DORD):
                while any(h_[j_][t_] is None for h_ in hsl for j_, t_, _ in _HK_B[i]):
                    advance(len(pend) - 1)
                au = []
                for p in cs:
                    au += [pw[c0 + p // 2, pl.ds(R_SD + i * (D3 // 2), D3 // 2), k * TC:(k + 1) * TC] for k in range(2)]
                if fresh:
                    au[0] = jnp.concatenate([au[0][0:8] | take_probe(), au[0][8:]], axis=0)
                r = _dot_nt(jnp.concatenate([_up(v) for v in au], axis=1),
                            jnp.concatenate([_ssum([(p_s[h_[j_][t_]][pl.ds(zeros[i], TB), :], sg) for j_, t_, sg in _HK_B[i]])
                                             for h_ in hsl], axis=1).astype(bf16))
                acc[i] = r if acc[i] is None else r + acc[i]
                advance(max(len(pend) - DADV, 0))
                clock.tick(48 * len(ps), acc[i], DTK)

        pg = pd = 0
        for tok in script:
            if tok == 'G':
                gu(pg)
                pg += 1
            elif tok[0] == 'D':
                down(list(range(pd, pd + int(tok[1:]))))
                pd += int(tok[1:])
            elif tok == 'W':
                assert not clock.jobs
                advance(0)
                if not wrhs:
                    wo_rhs(wo_seq, None, wrhs)
                wo_mm(an, wrhs)
                clock.t += 1152
            elif tok[0] == 'Y':
                def hold(items, dep):
                    o_s[10, pl.ds(0, 8), :] = dep
                    wo_rhs(items, None, wrhs)
                lo_, hi_ = YSPLIT[int(tok[1])], YSPLIT[int(tok[1]) + 1]
                clock.add(clock.t + int(tok[3:]), functools.partial(hold, wo_seq[lo_:hi_]))
            elif tok == 'X':
                state['odep'] = True
            elif tok[0] == 'n':
                j1, j2 = ln_jobs(an + int(tok[1]), xn_f, int(tok[1]), LNJ[0], LNJ[1])
                t_ = clock.t + int(tok[3:])
                for job in j1:
                    clock.add(t_, with_deadline(job, JDL))
                    t_ += LNJ[2]
                t_ += LNJ[3]
                for job in j2:
                    def counted(job_, dep):
                        state['norm'] += 1
                        return job_(dep)
                    clock.add(t_, with_deadline(functools.partial(counted, job), JDL))
                    t_ += LNJ[2]
            elif tok[0] == 'l':
                _, t0_, dt_ = tok.split('+')

                def left(which, dep):
                    assert state['norm'] == 2 * LNJ[1]
                    state['left'].update(which)
                    a_left(which, dep)
                    return lambda: st_s[0, pl.ds(zero8, 8), :]
                for k_ in range(NLEFT):
                    clock.add(clock.t + int(t0_) + k_ * int(dt_), with_deadline(
                        functools.partial(left, list(range(k_ * 15 // NLEFT, (k_ + 1) * 15 // NLEFT))), LDL))
            elif tok[0] == 'c':
                _, t0_, dt_ = tok.split('+')
                for k_ in range(15):
                    def arrange(k__, dep):
                        assert k__ in state['left'] and pg == 2 * NCH
                        a_arrange([k__], dep)
                    clock.add(clock.t + int(t0_) + k_ * int(dt_), functools.partial(arrange, k_))
            else:
                par = 0 if tok[1] == 'a' else 1
                clock.add(clock.t + int(tok[3:] or 0), functools.partial(a_rows, an + par, par, MODE_P))
        assert pg == pd and not [j_ for j_ in clock.jobs if j_[2].__class__ is functools.partial or j_[2].__name__ == 'run']
        for t in range(2):
            y = jnp.concatenate([_ssum([(acc[k], sg) for k, sg in _HK_C[i, t]]) for i in range(3)], axis=0)
            x2 = xres[b0 + t] + 0.5 * y
            xres[b0 + t] = x2
            o_ref[:, t * TB:(t + 1) * TB] = x2.astype(o_ref.dtype)

    plan = [[n_ - lag if 0 <= n_ - lag < NCH else NCH for lag in (GU_LAG, GU_LAG, D_LAG)] for n_ in range(NP)]
    rest = [(c, m) for c in range(NCH) for m in range(3) if c not in [p_[m] for p_ in plan]]
    order = [(p_[m], m) for p_ in plan for m in range(3) if p_[m] < NCH] + rest

    def prologue():
        cp_x(0).start()
        for sec in range(3):
            for cp in cp_qkv(sec):
                cp.start()
        for n_ in range(NP):
            for k in range(CP):
                plan_s[n_ * CP + k] = plan[n_][k]
        qall[:, pl.ds(0, HALO), :] = jnp.zeros((16, HALO, 128), f32)
        cp_x(0).wait()
        ln1(0, 0, 'in', (4, 0))
        ln1(0, 1, 'in', (4, 0))
        q_left(True)
        for sec in range(3):
            for cp in cp_qkv(sec):
                cp.wait()
            if sec == 0:
                cp_x(1).start()
                cp_x(2).start()
                cp_wo().start()
                for k, (c, m) in enumerate(order):
                    cp_unit(c, m).start()
                    if k % 2 == 0 and 3 + k // 2 < NP:
                        cp_x(3 + k // 2).start()
            transpose_qkv(sec)
            build_wq(sec)

    def first_attention():
        q_step(1, [], 'in', CFG_QA, rows=True)
        cp_wo().wait()
        build_wo()

        def cb(pos, v):
            if pos in (3, 8, 12, 16, 20):
                for k in range(8):
                    wq[27, pl.ds(zero8, 8), :] = pltpu.bitcast(v[k * 24:k * 24 + 8], u32)
                    build_wq_sums([todo.pop(0)])
        todo = list(range(0, 320, 8))
        rhs = {}
        wo_rhs(wo_seq, 0, rhs)
        wo_mm(0, rhs, cb)
        assert not todo
        ln2(0, 0, (4, 0))
        ln2(1, 1, (4, 0))
        a_left()
        a_arrange()

    def startup_step(n, carry):
        for n_ in range(NP):
            @pl.when(n == n_)
            def _():
                if n_ + 1 < NP:
                    cp_x(n_ + 1).wait()
                for m, c in enumerate(plan[n_]):
                    if c < NCH:
                        cp_unit(c, m).wait()

        @pl.when(n != 1)
        def _():
            if ONLY in ('', 'q'):
                q_step(n, [plan_s[n * CP + k] for k in range(CP)], 'in', CFG_Q1)

        @pl.when(n == 1)
        def _():
            if ONLY in ('', 'a'):
                first_attention()
        return carry

    @pl.when(g == 0)
    def _():
        if ONLY in ('', 'pro'):
            prologue()
        if ONLY in ('', 'q', 'a'):
            lax.fori_loop(0, NP, startup_step, 0)
        if not ONLY:
            for c, m in rest:
                cp_unit(c, m).wait()
                for piece in prep_pieces(c, m):
                    piece()

    @pl.when(jnp.logical_and(g >= NP - 1, g < 2 * NP - 1))
    def _():
        @pl.when(g == NP - 1)
        def _():
            if ONLY in ('', 'pro'):
                ln1(0, 0, 'res', (4, 0))
                ln1(0, 1, 'res', (4, 0))
                q_left(False)
        if ONLY in ('', 'q'):
            q_step(g - (NP - 1), [], 'res', CFG_Q2)

    if ONLY in ('q', 'a', 'pro'):
        @pl.when(g == 2 * NP - 1)
        def _():
            o_ref[0:16, 0:128] = (qall[g % 16, pl.ds(zero8, 16), :] + xres[g % 16, pl.ds(zero8, 16), :]
                                  + pltpu.bitcast(pw[g % 4, pl.ds(zero8, 16), 0:128] | s_scr[g % 8, pl.ds(zero8, 16), :]
                                                  | wo2[pl.ds(zero8, 16), :] | wq[g % 8, pl.ds(zero8, 16), :] | sq_scr[g % 8, pl.ds(zero8, 16), :], f32)).astype(bf16)

    @pl.when(g < 2 * NP - 1)
    def _():
        if ONLY in ('', 'p'):
            ffn(g, 0, SCRIPT)

    @pl.when(g == 2 * NP - 1)
    def _():
        def body(hf, carry):
            ffn(2 * NP - 1, hf * NPC, SCRIPT_F)
            return carry
        if ONLY in ('', 'f'):
            lax.fori_loop(0, 2, body, 0)


@jax.jit
def pallas_interleave_layers__sliding_local_dilated__glu_gated_geglu__prompt_kernel(
    A_x, A_wqkv, A_wo, B_x, B_w_gate, B_w_up, B_w_down):
    B, S, D = A_x.shape
    DF = B_w_gate.shape[1]
    NB = S // TB
    NP = NB // 2
    NCH = DF // CW
    xT = A_x.reshape(S, D).T
    wdT = B_w_down.T
    hbm = pl.BlockSpec(memory_space=pltpu.HBM)
    outT = pl.pallas_call(
        functools.partial(_kernel, D=D, DF=DF, S=S),
        grid=(2 * NP,),
        in_specs=[hbm] * 6,
        out_specs=pl.BlockSpec((D, 2 * TB), lambda g: (0, jnp.maximum(g - NP, 0))),
        out_shape=jax.ShapeDtypeStruct((D, S), A_x.dtype),
        scratch_shapes=[
            pltpu.VMEM((NP, D, 2 * TB), bf16),
            pltpu.VMEM((D, 3 * D), bf16),
            pltpu.VMEM((D, D), bf16),
            pltpu.VMEM((5, 14 * 128, 128), f32),
            pltpu.VMEM((28, 320, 128), u32),
            pltpu.VMEM((D // 2, 640), u32),
            pltpu.VMEM((15 * (D // 6) + 3 * (D // 4) + 16, 128), u32),
            pltpu.VMEM((NCH + 1, 3, D, CW), bf16),
            pltpu.VMEM((NCH + 1, 45 * (TC // 2) + 15 * (D // 6) + 16, 2 * TC), u32),
            pltpu.VMEM((16, S + QPAD, 128), f32),
            pltpu.VMEM((11, TB, 128), f32),
            pltpu.VMEM((NB, D, TB), f32),
            pltpu.VMEM((2, D, TB), f32),
            pltpu.VMEM((2, D, TB), f32),
            pltpu.VMEM((45, TB // 2, TC), u32),
            pltpu.VMEM((31, TB // 2, TC), u32),
            pltpu.VMEM((18, TB // 2, TC), u32),
            pltpu.SMEM((NP * CP,), jnp.int32),
            pltpu.SemaphoreType.DMA((4 + NP + 3 * NCH,)),
        ] + [pltpu.VMEM((TB, 2 * TC), f32)] * 29,
        compiler_params=pltpu.CompilerParams(
            dimension_semantics=("arbitrary",),
            vmem_limit_bytes=110 * 1024 * 1024,
            disable_bounds_checks=bool(NOCHK),
            disable_semaphore_checks=bool(NOCHK),
        ),
    )(xT, A_wqkv, A_wo, B_w_gate, B_w_up, wdT)
    return outT.T.reshape(B, S, D)
```

```python
import functools
import math
import jax
import jax.numpy as jnp
from jax import lax
import jax.experimental.pallas as pl
import jax.experimental.pallas.tpu as pltpu

H = 32
DH = 18
W = 8
DIL = 2
HALO = 16
EPS = 1e-5
TB = 128
RB = 8
TC = 128
CW = 6 * TC
KY = 64
ONLY = ''
LN_P = tuple(int(x) for x in '1,2'.split(','))
CFG_Q1 = tuple(int(x) for x in '1,2,1500,2500'.split(','))
CFG_Q2 = tuple(int(x) for x in '1,2,60,560'.split(','))
QP0 = int(200); QP1 = int(4000); QTK = int(16)
MODE_P = tuple(int(x) for x in '1,3'.split(','))
MODE_A = tuple(int(x) for x in '1,3'.split(','))
SCRIPT = 'R1+50+400,G,R5+0+290,G,G,R10+0+350,G,D4,G,R5+0+290,G,G,R11+0+250,G,D4,W,n0+1500,n1+2124,l+3424+500,G,G,G,G,c+200+96,D4'.split(',')
SCRIPT_F = 'G,G,G,G,D2,G,G,D2,D2'.split(',')
DORD = tuple(int(x) for x in '1,6,0,9,10,4,11,5,14,7,2,8,3,12,13'.split(','))
GU_LAG = int(2); D_LAG = int(2)
CP = 3
RG = tuple(int(x) for x in '2,1,48,420'.split(','))
RDL = int(700)
ZM = int(8)
JDL = int(250); LDL = int(600); GTK = int(2)
PLAG = int(4); DADV = int(1)
UFIRST = int(0); USCR = int(0)
CFG_QA = tuple(int(x) for x in '1,2,200,500'.split(','))
QA_T = tuple(int(x) for x in '100,800'.split(','))
QA_DEAD = tuple(int(x) for x in '1,1'.split(','))
QPAD = int(40)
LNJ = tuple(int(x) for x in '12,12,48,48'.split(','))
DTK = int(8)
XNF = int(1); XNL = int(1); NLEFT = int(3)
YSPLIT = tuple(int(x) for x in '0,21'.split(','))
WORD = tuple(int(x) for x in '0,1,2,6,7,8,9,10,11,12,13,14,3,4,5'.split(','))
NOCHK = int(1)

f32 = jnp.float32
bf16 = jnp.bfloat16
u32 = jnp.uint32
NT = (((1,), (1,)), ((), ()))


def _unpk(u, idx):
    return pltpu.unpack_elementwise(u, index=idx, packed_dtype=bf16, unpacked_dtype=f32)


def _pk2(even, odd):
    return pltpu.pack_elementwise([even, odd], packed_dtype=bf16).astype(u32)


def _up(x):
    return pltpu.bitcast(x, bf16)


def _dot(a, b):
    return jnp.dot(a, b, preferred_element_type=f32)


def _dot_nt(a, b):
    return lax.dot_general(a, b, NT, preferred_element_type=f32)


def _tree(fn, xs):
    xs = list(xs)
    while len(xs) > 1:
        xs = [fn(xs[i], xs[i + 1]) for i in range(0, len(xs) - 1, 2)] + ([xs[-1]] if len(xs) % 2 else [])
    return xs[0]


def _ln_stats(x, nacc, pin=None):
    n = x.shape[0]
    c = x[0:1] if pin is None else pin(x[0:8])[0:1]
    s1 = [None] * nacc
    s2 = [None] * nacc
    for i in range(n // 8):
        d = x[i * 8:(i + 1) * 8] - c
        k = i % nacc
        s1[k] = d if s1[k] is None else s1[k] + d
        dd = d * d
        s2[k] = dd if s2[k] is None else s2[k] + dd
    m = jnp.sum(_tree(jnp.add, s1), axis=0, keepdims=True) * (1.0 / n)
    v = jnp.sum(_tree(jnp.add, s2), axis=0, keepdims=True) * (1.0 / n) - m * m
    v = jnp.maximum(v, 0.0)
    return c + m, lax.rsqrt(v + EPS)


_HK_A = (
    ((0, 0, 1), (0, 2, -1), (1, 0, -1)), ((0, 0, 1), (0, 1, -1), (2, 0, -1)), ((1, 1, 1), (0, 1, -1), (1, 2, -1)),
    ((1, 1, 1), (1, 0, -1), (2, 1, -1)), ((2, 2, 1), (0, 2, -1), (2, 1, -1)), ((2, 2, 1), (1, 2, -1), (2, 0, -1)),
    ((0, 1, 1),), ((0, 1, 1), (1, 0, -1)), ((1, 0, 1),),
    ((0, 2, 1),), ((0, 2, 1), (2, 0, -1)), ((2, 0, 1),),
    ((1, 2, 1),), ((2, 1, 1), (1, 2, -1)), ((2, 1, 1),),
)
_HK_C = {
    (0, 0): ((0, 1), (7, 1), (8, 1), (9, 1), (6, -1)),
    (0, 1): ((1, 1), (6, 1), (10, 1), (11, 1), (9, -1)),
    (1, 0): ((2, 1), (7, 1), (8, 1), (12, 1), (6, -1)),
    (1, 1): ((3, 1), (6, 1), (13, 1), (14, 1), (2, -1), (7, -1)),
    (2, 0): ((5, 1), (9, 1), (12, 1), (13, 1), (4, -1), (10, -1)),
    (2, 1): ((4, 1), (10, 1), (11, 1), (14, 1), (9, -1)),
}


_HK_B = (((0, 0, 1),), ((0, 1, 1),), ((1, 0, 1),), ((1, 0, 1), (1, 1, 1)), ((2, 1, 1),), ((2, 0, 1), (2, 1, 1)),
         ((0, 1, 1), (1, 1, 1)), ((0, 1, 1), (1, 0, 1), (1, 1, 1)), ((0, 0, 1), (0, 1, 1), (1, 0, 1), (1, 1, 1)),
         ((0, 0, 1), (2, 0, 1)), ((0, 0, 1), (2, 0, 1), (2, 1, 1)), ((0, 0, 1), (0, 1, 1), (2, 0, 1), (2, 1, 1)),
         ((1, 0, 1), (2, 0, 1)), ((1, 0, 1), (2, 1, -1)), ((1, 1, 1), (2, 1, 1)))


def _hk_b(b):
    s1 = b[1][0] + b[1][1]
    s2 = b[2][0] + b[2][1]
    t7 = b[0][1] + s1
    t10 = b[0][0] + s2
    return (b[0][0], b[0][1], b[1][0], s1, b[2][1], s2, b[0][1] + b[1][1], t7, b[0][0] + t7,
            b[0][0] + b[2][0], t10, b[0][1] + t10, b[1][0] + b[2][0], b[1][0] - b[2][1], b[1][1] + b[2][1])


def _ssum(terms):
    terms = sorted([t for t in terms if t[0] is not None], key=lambda z: -z[1])
    if not terms:
        return None
    acc = terms[0][0] if terms[0][1] == 1 else -terms[0][0]
    for v, sg in terms[1:]:
        acc = acc + v if sg == 1 else acc - v
    return acc


GU_ORD = tuple(int(x) for x in '8,6,7,11,3,1,10,14,9,5,0,13,12,4,2'.split(','))
GU_POST = {
    8: ((), ('p8', None), None),
    7: ((('p8', 1),), (None, 't7'), None),
    3: ((('t7', 1),), (None, 's1'), None),
    6: ((), ('p6', None), None),
    14: ((('p6', 1), ('s1', 1)), ('p14', None), (1, 1)),
    12: ((('p9', 1), ('s2', 1)), ('p12', None), (2, 0)),
    13: ((), ('p13', None), None),
    2: ((('p12', 1), ('p13', 1), ('s1', 1)), (None, None), (1, 0)),
    11: ((), ('p11', None), None),
    10: ((('p11', 1),), (None, 't10'), None),
    5: ((('t10', 1),), (None, 's2'), None),
    9: ((), ('p9', None), None),
    4: ((('p14', 1), ('s2', 1), ('p13', -1)), (None, None), (2, 1)),
    0: ((('p8', 1), ('p9', 1), ('t10', 1)), (None, None), (0, 0)),
    1: ((('p6', 1), ('p11', 1), ('t7', 1)), (None, None), (0, 1)),
}
PSLOT = {k: i for i, k in enumerate(('p8', 't7', 's1', 'p6', 'p14', 'p12', 'p13', 'p11', 't10', 's2', 'p9'))}


class _Timeline:
    def __init__(self):
        self.t = 0
        self.jobs = []

    def add(self, when, fn):
        self.jobs.append((when, len(self.jobs), fn))
        self.jobs.sort(key=lambda z: z[:2])

    def tick(self, dur, v, n=1, seq=1):
        per = max(n // seq, 1)
        for k in range(n):
            self.t += dur // n
            r = (k % per) * (v.shape[0] // per)
            c = (k // per) * 128
            while self.jobs and self.jobs[0][0] <= self.t:
                self.jobs.pop(0)[2](v[r:r + 8, c:c + 128])


def _kernel(x_hbm, wqkv_hbm, wo_hbm, wg_hbm, wu_hbm, wd_hbm, o_ref,
            xin, wqkv_raw, wo_raw, tmp, wq, woT, wo2, raw, pw, qall, o_s, xres, xn_f, xn_g, s_scr, st_s, sq_scr,
            plan_s, sems, *p_s, D, DF, S):
    g = pl.program_id(0)
    NB = S // TB
    NP = NB // 2
    NCH = DF // CW
    NPC = NCH // 2
    D3 = D // 3
    DHALF = D // 2
    nr = TB // RB
    hh = DHALF // 2
    zero8 = pl.multiple_of((g >> 20) * ZM, ZM)
    zvec = jnp.full((8, 128), (g >> 20).astype(u32), u32)

    def zero(k):
        return pl.multiple_of((g >> (8 + k)) * ZM, ZM)

    def tie(x, dep):
        return pltpu.bitcast(pltpu.bitcast(x, u32) | (pltpu.bitcast(dep, u32) & zvec), f32)

    QSEC = ((0, 5), (5, 9), (9, 14))

    def cp_qkv(sec):
        out = []
        for j in range(*QSEC[sec]):
            n = min(128, 3 * D - j * 128)
            out.append(pltpu.make_async_copy(wqkv_hbm.at[:, pl.ds(j * 128, n)], wqkv_raw.at[:, pl.ds(j * 128, n)],
                                             sems.at[sec]))
        return out

    def cp_wo():
        return pltpu.make_async_copy(wo_hbm, wo_raw, sems.at[3])

    def cp_x(k):
        return pltpu.make_async_copy(x_hbm.at[:, pl.ds(k * 2 * TB, 2 * TB)], xin.at[k], sems.at[4 + k])

    def cp_unit(c, m):
        return pltpu.make_async_copy((wg_hbm, wu_hbm, wd_hbm)[m].at[:, pl.ds(c * CW, CW)], raw.at[c, m],
                                     sems.at[4 + NP + 3 * c + m])

    R_SD = 45 * (TC // 2)
    R_END = R_SD + 15 * (D3 // 2)

    def hk_a_ops(load, minus=None):
        blk = {}
        for i in range(3):
            for j in range(3):
                u = load(i, j)
                if minus is None:
                    blk[i, j] = (u, _unpk(u, 0), _unpk(u, 1))
                else:
                    v = minus(i, j)
                    blk[i, j] = (None, _unpk(u, 0) - _unpk(v, 0), _unpk(u, 1) - _unpk(v, 1))
        out = []
        for terms in _HK_A:
            if len(terms) == 1 and minus is None:
                out.append(blk[terms[0][:2]][0])
            else:
                out.append(_pk2(_ssum([(blk[i, j][1], sg) for i, j, sg in terms]),
                                _ssum([(blk[i, j][2], sg) for i, j, sg in terms])))
        return out

    def prep_pieces(c, m):
        def ld(r, cs):
            return lambda i, j: pltpu.bitcast(raw[c, m, pl.ds(i * D3 + r, 16), pl.ds((3 * cs + j) * TC, TC)], u32)

        def gu_piece(q, r, cs, neg, kind, half):
            ops = hk_a_ops(ld(q * KY + r, cs), None if neg is None else ld(q * KY + r, neg))
            for k, t in enumerate(ops):
                pw[c, pl.ds((3 * k + kind) * (TC // 2) + (half * KY + r) // 2, 8), m * TC:(m + 1) * TC] = t

        def d_piece(r, cs):
            for k, t in enumerate(hk_a_ops(ld(r, cs))):
                pw[c, pl.ds(R_SD + k * (D3 // 2) + r // 2, 8), cs * TC:(cs + 1) * TC] = t
        if m == 2:
            return [functools.partial(d_piece, r, cs) for r in range(0, D3, 16) for cs in range(2)]
        spec = ((0, 0, None, 0, 0), (1, 0, 1, 0, 1), (0, 1, None, 1, 0), (2, 1, 0, 1, 1),
                (2, 0, None, 2, 0), (1, 1, None, 2, 1))
        return [functools.partial(gu_piece, q, r, cs, neg, kind, half)
                for r in range(0, KY, 16) for q, cs, neg, kind, half in spec]

    def transpose_qkv(sec):
        for j in range(*QSEC[sec]):
            wd_ = min(128, 3 * D - j * 128)
            blk = wqkv_raw[:, j * 128:j * 128 + wd_].astype(f32)
            if wd_ < 128:
                blk = jnp.concatenate([blk, jnp.zeros((D, 128 - wd_), f32)], axis=1)
            bt = jnp.concatenate([blk, blk[D - KY:]], axis=0).T
            for t in range(5):
                tmp[t, pl.ds(j * 128, 128), :] = bt[:, t * 128:(t + 1) * 128]

    def wq_slot(i, j):
        return 24 + i if i == j else [n for n, t in enumerate(_HK_A) if t == ((i, j, 1),)][0]

    def build_wq(sec):
        lo = lax.broadcasted_iota(jnp.int32, (16, 128), 1) < KY
        for d in range(DH):
            tt = [_pk2(tmp[t, pl.ds(sec * D + d, 16, stride=2 * DH), :],
                       tmp[t, pl.ds(sec * D + d + DH, 16, stride=2 * DH), :]) for t in range(5)]
            ops = tt[:4] + [jnp.where(lo, tt[3], tt[4]), jnp.where(lo, tt[4], tt[3])]
            if d < 16:
                dst = [(sec, d * 16)]
            else:
                dst = ([(1, (d + 2) * 16)], [(1, d * 16)], [(0, d * 16), (0, (d + 2) * 16)])[sec]
            for j, row in dst:
                for k, v in enumerate(ops):
                    wq[wq_slot(k, j) if k < 3 else 12 + 3 * j + k, pl.ds(row, 16), :] = v

    def build_wq_sums(rs):
        for r in rs:
            ncol = 3 if r < 256 else 2
            blk = {}
            for i in range(3):
                for j in range(ncol):
                    u = wq[wq_slot(i, j), pl.ds(r, 8), :]
                    blk[i, j] = (_unpk(u, 0), _unpk(u, 1))
            for n, terms in enumerate(_HK_A):
                if len(terms) == 1 or (ncol == 2 and n in (4, 5)):
                    continue
                wq[n, pl.ds(r, 8), :] = _pk2(*[_ssum([(blk[i, j][p_], sg) for i, j, sg in terms if j < ncol])
                                               for p_ in range(2)])

    def build_wo():
        for t in range(5):
            wd_ = min(128, D - t * 128)
            blk = wo_raw[:, t * 128:t * 128 + wd_].astype(f32)
            if wd_ < 128:
                blk = jnp.concatenate([blk, jnp.zeros((D, 128 - wd_), f32)], axis=1)
            tmp[t, pl.ds(0, D), :] = blk
        for t in range(5):
            rows = [tmp[t, pl.ds(d, 32, stride=DH), :] for d in range(DH)]
            ft = jnp.concatenate(rows + rows[16:], axis=0).T
            n = min(128, D - t * 128)
            woT[pl.ds(t * 64, n // 2), :] = pltpu.bitcast(ft[:n].astype(bf16), u32)
        for r in range(0, D3 // 2, 8):
            ops = hk_a_ops(lambda i, j: woT[pl.ds(i * (D3 // 2) + r, 8), j * TC:(j + 1) * TC])
            for k, t in enumerate(ops):
                wo2[pl.ds(k * (D3 // 2) + r, 8), :] = t
        lo = lax.broadcasted_iota(jnp.int32, (8, 128), 1) < KY
        for r in range(0, hh, 8):
            a3, a4 = woT[pl.ds(r, 8), 384:512], woT[pl.ds(r, 8), 512:640]
            b3, b4 = woT[pl.ds(hh + r, 8), 384:512], woT[pl.ds(hh + r, 8), 512:640]

            def dif(u, v):
                return _pk2(_unpk(u, 0) - _unpk(v, 0), _unpk(u, 1) - _unpk(v, 1))
            base = 15 * (D3 // 2)
            wo2[pl.ds(base + r, 8), :] = jnp.where(lo, a3, dif(a3, b3))
            wo2[pl.ds(base + hh + r, 8), :] = jnp.where(lo, b3, dif(b4, a4))
            wo2[pl.ds(base + 2 * hh + r, 8), :] = jnp.where(lo, a4, b3)

    def normalize(blk, mean, rstd, link):
        if not link:
            return (xres[blk] - mean) * rstd
        rs = jnp.broadcast_to(rstd, (8, TB))
        mb = jnp.broadcast_to(mean, (8, TB))
        outs = []
        for i in range(D // 8):
            if i and i % link == 0:
                rs = tie(rs, outs[-1])
            outs.append((xres[blk, pl.ds(i * 8, 8), :] - mb) * rs)
        return jnp.concatenate(outs, axis=0)

    def left_ops(src, put, plain=False, which=None, dep=None):
        def X(t, r0, n):
            return src[t, pl.ds(r0, n), :]
        k1, k2, k3 = 3 * TC, 3 * TC + KY, 3 * TC + 2 * KY
        for n in (list(range(6 if plain else 15)) + [15, 16, 17]) if which is None else which:
            if n == 15:
                v = jnp.concatenate([X(0, k1, KY), X(0, k2, KY) - X(1, k2, KY)], axis=0)
            elif n == 16:
                v = jnp.concatenate([X(1, k1, KY), X(1, k3, KY) - X(0, k3, KY)], axis=0)
            elif n == 17:
                v = jnp.concatenate([X(0, k3, KY), X(1, k2, KY)], axis=0)
            elif plain:
                v = X(n // 3, (n % 3) * TC, TC)
            else:
                v = _ssum([(X(t, i * TC, TC), sg) for (i, t), lst in _HK_C.items() for k, sg in lst if k == n])
            if dep is not None:
                v = jnp.concatenate([tie(v[0:8], dep), v[8:]], axis=0)
            put(n, pltpu.bitcast(v.astype(bf16).T, u32))

    def ln1(pr, par, src, ln, dep=None):
        blk = 2 * pr + par
        if src == 'res':
            x = xres[blk]
        else:
            x = xin[pr, :, par * TB:(par + 1) * TB].astype(f32)
            xres[blk] = x
        mean, rstd = _ln_stats(x, ln[0], None if dep is None else (lambda v: tie(v, dep)))
        if src == 'res':
            xn_g[par, pl.ds(0, 8), :] = jnp.zeros((8, TB), f32)
        xn_g[par, pl.ds(zero8, D), :] = normalize(blk, mean, rstd, ln[1])

    def q_left(plain):
        def put(i, v):
            sq_scr[i] = v
        left_ops(xn_g, put, plain)

    def hk_outputs(P, T, PT, tk, emit, two_cols=False):
        p8 = P(8)
        t7 = P(7) + p8
        tk(2, t7)
        s1 = PT(3, 1, 2) + t7
        tk(2, s1)
        p6 = P(6)
        p14 = P(14)
        tk(2, p14)
        emit(1, 1, T(1, 1) + (p6 + p14 + s1), 1)
        p13 = P(13)
        if two_cols:
            emit(1, 0, PT(2, 1, 0) + (p13 + s1), 3)
        else:
            p12 = P(12)
            tk(2, p12)
            emit(1, 0, PT(2, 1, 0) + (p12 + p13 + s1), 2)
        p11 = P(11)
        t10 = P(10) + p11
        tk(2, t10)
        if not two_cols:
            s2 = PT(5, 2, 2) + t10
            tk(2, s2)
            p9 = P(9)
            emit(2, 0, T(2, 0) + (p9 + p12 + s2), 2)
            emit(2, 1, PT(4, 2, 1) + (p14 - p13 + s2), 2)
        w0 = T(0, 2)
        emit(0, 0, PT(0, 0, 0) + ((p8 + t10 + w0) if two_cols else (p8 + p9 + t10 + w0)), 3)
        emit(0, 1, PT(1, 0, 1) + (p6 + p11 + t7 + w0), 2)

    QT = (0, 1, 2, 3)
    KT = (4, 5, 6, 7, 13)
    VT = (8, 9, 10, 11, 12)
    c2e = DH ** -0.5 * math.log2(math.e)
    neg = -1e9 * math.log2(math.e)

    def q_step(pr, cs, src, cfg, rows=False):
        clock = _Timeline()
        if rows:
            base, nx = pr * (2 * TB), pr + 1
            clock.add(QA_T[0], functools.partial(a_rows, 0, 0, MODE_A))
            clock.add(QA_T[1], functools.partial(a_rows, 1, 1, MODE_A))
        else:
            base = pl.multiple_of(pr * (2 * TB), 2 * TB)
            nx = jnp.minimum(pr + 1, NP - 1)
        ln_q, la_t, lb_t = cfg[:2], cfg[2], cfg[3]
        pieces = []
        for m, c in enumerate(cs):
            pieces += prep_pieces(c, m)

        def paced(piece, dep):
            pw[NCH, pl.ds(R_END, 8), 0:128] = pltpu.bitcast(dep, u32)
            piece()
        for k, piece in enumerate(pieces):
            clock.add(QP0 + k * (QP1 - QP0) // len(pieces), functools.partial(paced, piece))
        clock.add(la_t, lambda dep: ln1(nx, 0, src, ln_q, dep))
        clock.add(lb_t, lambda dep: ln1(nx, 1, src, ln_q, dep))
        for r0, nt, tiles in ((0, 2, (0, 4, 8)), (TC, 2, (2, 6, 10)), (2 * TC, 1, (12, 13))):
            def R(k):
                return wq[k, pl.ds(r0, nt * 64), :]

            def P(k):
                return _dot_nt(_up(sq_scr[k]), _up(R(k)))

            def T(j, kind):
                return _dot_nt(_up(sq_scr[15 + kind]), _up(R(15 + 3 * j + kind)))

            def PT(k, j, kind):
                return _dot_nt(_up(jnp.concatenate([sq_scr[k], sq_scr[15 + kind]], axis=1)),
                               _up(jnp.concatenate([R(k), R(15 + 3 * j + kind)], axis=1)))

            def tk(np_, v):
                clock.tick(32 * nt * np_, v, QTK if src == 'in' else 4, nt if src == 'in' else 1)

            def emit(col, half, v, np_):
                for k in range(nt):
                    qall[tiles[col] + k, pl.ds(base + (HALO + half * TB), TB), :] = v[:, k * 128:(k + 1) * 128]
                tk(np_, v)
            if src == 'res':
                hk_outputs(P, T, PT, tk, emit, two_cols=(nt == 1))
                continue
            for j in range(len(tiles)):
                both = T(j, 2)
                for t in range(2):
                    lhs = [sq_scr[3 * t + i] for i in range(3)] + [sq_scr[15 + t]]
                    if rows and nt == 1 and (j, t) == QA_DEAD:
                        probe = pltpu.bitcast(o_s[0, pl.ds(zero8, 8), :], u32)
                        lhs[0] = jnp.concatenate([lhs[0][0:8] | (probe & zvec), lhs[0][8:]], axis=0)
                    rhs = [R(wq_slot(i, j)) for i in range(3)] + [R(15 + 3 * j + t)]
                    emit(j, t, _dot_nt(_up(jnp.concatenate(lhs, axis=1)), _up(jnp.concatenate(rhs, axis=1))) + both,
                         5 - t)
        assert not clock.jobs
        q_left(src == 'in')

    def a_rows(blk, par, mode, start=None, rs=None):
        lag_mid, lag_end = mode[:2]
        fw, fv = mode[2:] if len(mode) > 2 else (0, 0)
        base = blk * TB if isinstance(blk, int) else pl.multiple_of(blk * TB, TB)
        cbits = pltpu.bitcast(jnp.full((RB, 128), c2e, f32), u32)
        lo = lax.broadcasted_iota(jnp.int32, (RB, 128), 1) < KY
        mid, fin = {}, {}
        rs = range(nr) if rs is None else rs
        for r in rs:
            r0 = r * RB
            deps = [start] if (start is not None and r == rs[0]) else []
            if lag_mid and r >= lag_mid:
                deps.append(mid[r - lag_mid])
            if lag_end and r >= lag_end:
                deps += fin[r - lag_end]
            if deps:
                acc = _tree(jnp.bitwise_or, [pltpu.bitcast(v, u32) for v in deps])
                cs = pltpu.bitcast(cbits | (acc & zvec), f32)
            else:
                cs = c2e

            def ld(t, w):
                return qall[t, pl.ds(base + (HALO + r0 - DIL * w), RB), :]
            q = [ld(t, 0) * cs for t in QT] + [jnp.where(lo, pltpu.roll(ld(13, 0), KY, 1), 0.0) * cs]
            sc = []
            for w in range(W):
                q0 = tie(q[0], prev) if (fw and w and w % fw == 0) else (q[0] if w == 0 else q0)
                acc = None
                for j, t in enumerate(KT):
                    p = (q0 if j == 0 else q[j]) * ld(t, w)
                    acc = p if acc is None else acc + p
                prev = acc
                acc = acc + pltpu.roll(acc, 64, 1)
                mid[r] = acc
                acc = acc + pltpu.roll(acc, 32, 1)
                if r0 - DIL * w < 0:
                    pos = blk * TB + r0 + lax.broadcasted_iota(jnp.int32, (RB, 128), 0)
                    acc = jnp.where(pos >= DIL * w, acc, neg)
                sc.append(acc)
            m = _tree(jnp.maximum, sc)
            e = [jnp.exp2(sc[w] - m) for w in range(W)]
            l = _tree(jnp.add, e)
            rinv = pl.reciprocal(l, approx=True)
            rinv = rinv * (2.0 - l * rinv)
            fin[r] = []
            for j, t in enumerate(VT):
                e0 = tie(e[0], acc) if (fv and j and j % fv == 0) else (e[0] if j == 0 else e0)
                acc = None
                for w in range(W):
                    p = (e0 if w == 0 else e[w]) * ld(t, w)
                    acc = p if acc is None else acc + p
                o = acc * rinv
                o_s[par * 5 + j, pl.ds(r0, RB), :] = o
                fin[r] = [o] if fv == 1 else fin[r] + [o]
        return lambda: _tree(jnp.bitwise_or, [pltpu.bitcast(v, u32) for v in fin[rs[-1]]])

    def row_group(blk, par, r, nw, nv):
        base = pl.multiple_of(blk * TB, TB)
        lo = lax.broadcasted_iota(jnp.int32, (RB, 128), 1) < KY
        r0 = r * RB

        def ld(t, w):
            return qall[t, pl.ds(base + (HALO + r0 - DIL * w), RB), :]
        dep = yield
        cs = tie(jnp.full((RB, 128), c2e, f32), dep)
        q = [ld(t, 0) * cs for t in QT] + [jnp.where(lo, pltpu.roll(ld(13, 0), KY, 1), 0.0) * cs]
        sc = []
        for w in range(W):
            if w and w % nw == 0:
                dep = yield
                q = [tie(q[0], dep)] + q[1:]
            acc = None
            for j, t in enumerate(KT):
                p = q[j] * ld(t, w)
                acc = p if acc is None else acc + p
            acc = acc + pltpu.roll(acc, 64, 1)
            acc = acc + pltpu.roll(acc, 32, 1)
            if r0 - DIL * w < 0:
                pos = blk * TB + r0 + lax.broadcasted_iota(jnp.int32, (RB, 128), 0)
                acc = jnp.where(pos >= DIL * w, acc, neg)
            sc.append(acc)
        m = _tree(jnp.maximum, sc)
        e = [jnp.exp2(sc[w] - m) for w in range(W)]
        l = _tree(jnp.add, e)
        rinv = pl.reciprocal(l, approx=True)
        rinv = rinv * (2.0 - l * rinv)
        outs = []
        for j, t in enumerate(VT):
            if j and j % nv == 0:
                dep = yield _tree(jnp.bitwise_or, [pltpu.bitcast(v, u32) for v in outs])
                outs = []
                e = [tie(e[0], dep)] + e[1:]
            acc = None
            for w in range(W):
                p = e[w] * ld(t, w)
                acc = p if acc is None else acc + p
            o = acc * rinv
            o_s[par * 5 + j, pl.ds(r0, RB), :] = o
            outs.append(o)
        yield _tree(jnp.bitwise_or, [pltpu.bitcast(v, u32) for v in outs])

    wo_seq = []
    for pos, k in enumerate(WORD):
        if pos in (0, 2):
            wo_seq += [('r', pos // 2, k_) for k_ in range(3)]
        wo_seq.append(('p', k))

    def wo_rhs(items, off, rhs):
        lo = lax.broadcasted_iota(jnp.int32, (TB, 128), 1) < KY

        for it in items:
            z = zero(wo_seq.index(it)) if off is None else off

            def O(t, j):
                return o_s[t * 5 + j, pl.ds(z, TB), :]
            if it[0] == 'p':
                v = _ssum([(O(t, j), sg) for j, t, sg in _HK_B[it[1]]])
            elif it[2] == 0:
                v = O(it[1], 3)
            else:
                v = jnp.where(lo, O(it[1], 2 + it[2]), O(it[1], 5 - it[2]))
            rhs[it] = v.astype(bf16)

    def wo_mm(blk0, rhs, cb=None):
        res = {}
        for pos, it in enumerate(wo_seq):
            if it[0] == 'p':
                lhs = wo2[pl.ds(it[1] * (D3 // 2), D3 // 2), :]
            else:
                lhs = wo2[pl.ds(15 * (D3 // 2) + it[2] * hh, hh), :]
            res[it] = _dot_nt(_up(lhs), rhs[it])
            if cb is not None:
                cb(pos, res[it])
        for t in range(2):
            both = res['r', t, 2]
            rem = xres[blk0 + t] + jnp.concatenate([res['r', t, 0] + both, res['r', t, 1] + both], axis=0)
            y = jnp.concatenate([_ssum([(res['p', k], sg) for k, sg in _HK_C[i, t]]) for i in range(3)], axis=0)
            xres[blk0 + t] = y + rem

    def ln2(blk, par, ln, dep=None):
        mean, rstd = _ln_stats(xres[blk, pl.ds(zero8 if XNL else 0, D), :], ln[0],
                               None if dep is None else (lambda v: tie(v, dep)))
        xn_f[par, pl.ds(0, 8), :] = jnp.zeros((8, TB), f32)
        xn_f[par, pl.ds(zero8 if XNF else 0, D), :] = normalize(blk, mean, rstd, ln[1])

    def ln_jobs(blk, dst, par, np1, np2):
        st = dict(s1=[], s2=[])
        nv = D // 8

        def stats(k, dep):
            if k == 0:
                st['c'] = jnp.broadcast_to(xres[blk, pl.ds(zero8, 8), :][0:1], (8, TB))
            c = tie(st['c'], dep)
            ds = [xres[blk, pl.ds(zero8 + i * 8, 8), :] - c for i in range(k * nv // np1, (k + 1) * nv // np1)]
            st['s1'].append(_tree(jnp.add, ds))
            st['s2'].append(_tree(jnp.add, [d * d for d in ds]))
            a_, b_ = st['s1'][-1], st['s2'][-1]
            return lambda: pltpu.bitcast(a_, u32) | pltpu.bitcast(b_, u32)

        def norm(k, dep):
            if k == 0:
                m = jnp.sum(_tree(jnp.add, st['s1']), axis=0, keepdims=True) * (1.0 / D)
                v = jnp.sum(_tree(jnp.add, st['s2']), axis=0, keepdims=True) * (1.0 / D) - m * m
                st['mean'] = st['c'] + m
                st['rstd'] = jnp.broadcast_to(lax.rsqrt(jnp.maximum(v, 0.0) + EPS), (8, TB))
            mean = tie(st['mean'], dep)
            for i in range(k * nv // np2, (k + 1) * nv // np2):
                dst[par, pl.ds(i * 8, 8), :] = (xres[blk, pl.ds(i * 8, 8), :] - mean) * st['rstd']
            return lambda: pltpu.bitcast(dst[par, pl.ds(zero8, 8), :], u32)
        return [functools.partial(stats, k) for k in range(np1)], [functools.partial(norm, k) for k in range(np2)]

    def a_left(which=range(15), dep=None):
        for n in which:
            v = _ssum([(xn_f[t, pl.ds(zero(n) + i * D3, D3), :], sg)
                       for (i, t), lst in _HK_C.items() for k, sg in lst if k == n])
            if dep is not None:
                v = jnp.concatenate([tie(v[0:8], dep), v[8:2 * KY], tie(v[2 * KY:2 * KY + 8], dep), v[2 * KY + 8:]],
                                    axis=0)
            st_s[2 * n] = pltpu.bitcast(v[:2 * KY].astype(bf16).T, u32)
            st_s[2 * n + 1] = pltpu.bitcast(jnp.concatenate([v[2 * KY:], v[2 * KY:]], axis=0).astype(bf16).T, u32)

    def a_arrange(which=range(15), dep=None):
        lo = lax.broadcasted_iota(jnp.int32, (TB // 2, 128), 1) < KY
        if dep is not None:
            st_s[30, pl.ds(0, 8), :] = pltpu.bitcast(dep, u32)
        for n in which:
            t1 = st_s[2 * n, pl.ds(zero8, TB // 2), :]
            t2 = st_s[2 * n + 1, pl.ds(zero8, TB // 2), :]
            s_scr[3 * n] = t1
            s_scr[3 * n + 1] = jnp.where(lo, t1, t2)
            s_scr[3 * n + 2] = jnp.where(lo, t2, t1)

    k0 = math.sqrt(2.0 / math.pi)
    k1 = k0 * 0.044715

    def ffn(j, c0, script):
        clock = _Timeline()
        b0 = (2 * j) % NB
        an = (2 * j + 2) % NB
        acc = [None] * 15
        hs = {}
        wrhs = {}
        state = dict(odep=False, rows=0, norm=0, left=set())

        pend = []
        fresh = []

        def advance(keep):
            while len(pend) > keep:
                pend.pop(0)()

        def probe_of(ref_val):
            return pltpu.bitcast(ref_val, u32) & zvec

        def take_probe():
            pr = _tree(jnp.bitwise_or, [k() if callable(k) else pltpu.bitcast(p_s[k][pl.ds(zero8, 8), 0:128], u32)
                                        for k in fresh]) & zvec
            del fresh[:]
            return pr

        def with_deadline(job, delay):
            def run(dep):
                val = job(dep)()
                clock.add(clock.t + delay, lambda _: fresh.append(lambda: val))
            return run

        def gu(p):
            c, second = c0 + p // 2, p % 2
            m = 1 - second if UFIRST else second
            h = hs.setdefault(p // 2, [[None, None] for _ in range(3)])

            def mm(n, kind, probe=None):
                lhs = s_scr[3 * n + kind]
                if state['odep']:
                    pr = probe_of(o_s[0, pl.ds(zero8, 8), :])
                    probe = pr if probe is None else probe | pr
                    state['odep'] = False
                if probe is not None:
                    lhs = jnp.concatenate([lhs[0:8] | probe, lhs[8:]], axis=0)
                return _dot(_up(lhs), _up(pw[c, pl.ds((3 * n + kind) * (TC // 2), TC // 2), m * TC:(m + 1) * TC]))

            def get(name):
                return p_s[PSLOT[name]][pl.ds(zero8, TB), :]

            def post(n, v):
                adds, keep, emits = GU_POST[n]
                if keep[0] is not None:
                    p_s[PSLOT[keep[0]]][...] = v
                    fresh.append(PSLOT[keep[0]])
                w_ = v
                for name, sg in adds:
                    w_ = w_ + get(name) if sg == 1 else w_ - get(name)
                if keep[1] is not None:
                    p_s[PSLOT[keep[1]]][...] = w_
                    fresh.append(PSLOT[keep[1]])
                if emits is not None:
                    col, half = emits
                    if m == 0:
                        w_ = w_ + w_ * jnp.tanh(w_ * (k0 + k1 * (w_ * w_)))
                    if second:
                        k_ = 17 + 6 * ((p // 2) % 2) + 2 * col + half
                        p_s[k_][...] = w_ * p_s[11 + 2 * col + half][pl.ds(zero8, TB), :]
                        fresh.append(k_)
                        h[col][half] = k_
                    else:
                        p_s[11 + 2 * col + half][...] = w_
                        fresh.append(11 + 2 * col + half)
            for n in GU_ORD:
                both = mm(n, 2, take_probe() if fresh else None)
                v = jnp.concatenate([mm(n, 0) + both, mm(n, 1) + both], axis=1)
                pend.append(functools.partial(post, n, v))
                advance(PLAG)
                clock.tick(96, both, GTK)

        def down(ps):
            cs = ps[::2]
            hsl = [hs.pop(p // 2) for p in cs]
            for pos, i in enumerate(DORD):
                while any(h_[j_][t_] is None for h_ in hsl for j_, t_, _ in _HK_B[i]):
                    advance(len(pend) - 1)
                au = []
                for p in cs:
                    au += [pw[c0 + p // 2, pl.ds(R_SD + i * (D3 // 2), D3 // 2), k * TC:(k + 1) * TC] for k in range(2)]
                if fresh:
                    au[0] = jnp.concatenate([au[0][0:8] | take_probe(), au[0][8:]], axis=0)
                r = _dot_nt(jnp.concatenate([_up(v) for v in au], axis=1),
                            jnp.concatenate([_ssum([(p_s[h_[j_][t_]][pl.ds(zero(i), TB), :], sg) for j_, t_, sg in _HK_B[i]])
                                             for h_ in hsl], axis=1).astype(bf16))
                acc[i] = r if acc[i] is None else r + acc[i]
                advance(max(len(pend) - DADV, 0))
                clock.tick(48 * len(ps), acc[i], DTK)

        pg = pd = 0
        for tok in script:
            if tok == 'G':
                gu(pg)
                pg += 1
            elif tok[0] == 'D':
                down(list(range(pd, pd + int(tok[1:]))))
                pd += int(tok[1:])
            elif tok == 'W':
                assert not [j_ for j_ in clock.jobs if j_[2].__class__ is functools.partial or j_[2].__name__ == 'run']
                assert state['rows'] in (0, 2 * nr)
                advance(0)
                if not wrhs:
                    wo_rhs(wo_seq, None, wrhs)
                wo_mm(an, wrhs)
                clock.t += 1152
            elif tok[0] == 'Y':
                def hold(items, dep):
                    o_s[10, pl.ds(0, 8), :] = dep
                    wo_rhs(items, None, wrhs)
                lo_, hi_ = YSPLIT[int(tok[1])], YSPLIT[int(tok[1]) + 1]
                clock.add(clock.t + int(tok[3:]), functools.partial(hold, wo_seq[lo_:hi_]))
            elif tok == 'X':
                state['odep'] = True
            elif tok[0] == 'n':
                j1, j2 = ln_jobs(an + int(tok[1]), xn_f, int(tok[1]), LNJ[0], LNJ[1])
                t_ = clock.t + int(tok[3:])
                for job in j1:
                    clock.add(t_, with_deadline(job, JDL))
                    t_ += LNJ[2]
                t_ += LNJ[3]
                for job in j2:
                    def counted(job_, dep):
                        state['norm'] += 1
                        return job_(dep)
                    clock.add(t_, with_deadline(functools.partial(counted, job), JDL))
                    t_ += LNJ[2]
            elif tok[0] == 'l':
                _, t0_, dt_ = tok.split('+')

                def left(which, dep):
                    assert state['norm'] == 2 * LNJ[1]
                    state['left'].update(which)
                    a_left(which, dep)
                    return lambda: st_s[0, pl.ds(zero8, 8), :]
                for k_ in range(NLEFT):
                    clock.add(clock.t + int(t0_) + k_ * int(dt_), with_deadline(
                        functools.partial(left, list(range(k_ * 15 // NLEFT, (k_ + 1) * 15 // NLEFT))), LDL))
            elif tok[0] == 'c':
                _, t0_, dt_ = tok.split('+')
                for k_ in range(15):
                    def arrange(k__, dep):
                        assert k__ in state['left'] and pg == 2 * NCH
                        a_arrange([k__], dep)
                    clock.add(clock.t + int(t0_) + k_ * int(dt_), functools.partial(arrange, k_))
            elif tok[0] == 'R':
                n_, t0_, dt_ = tok[1:].split('+')
                for k_ in range(int(n_)):
                    par, r_ = divmod(state['rows'], nr)
                    state['rows'] += 1
                    gen = row_group(an + par, par, r_, RG[0], RG[1])
                    next(gen)

                    def stage(gen_, delay, dep):
                        val = gen_.send(dep)
                        if val is not None:
                            clock.add(clock.t + delay, lambda _: fresh.append(lambda: val))
                    t_ = clock.t + int(t0_) + k_ * int(dt_)
                    n1_, n2_ = -(-W // RG[0]), -(-5 // RG[1])
                    for s_ in range(n1_):
                        clock.add(t_ + s_ * RG[2], functools.partial(stage, gen, RDL))
                    for s_ in range(n2_ - 1):
                        clock.add(t_ + (n1_ - 1) * RG[2] + RG[3] + s_ * RG[2], functools.partial(stage, gen, JDL))
            else:
                par = 0 if tok[1] == 'a' else 1
                clock.add(clock.t + int(tok[3:] or 0), functools.partial(a_rows, an + par, par, MODE_P))
        assert pg == pd and not [j_ for j_ in clock.jobs if j_[2].__class__ is functools.partial or j_[2].__name__ == 'run']
        for t in range(2):
            y = jnp.concatenate([_ssum([(acc[k], sg) for k, sg in _HK_C[i, t]]) for i in range(3)], axis=0)
            x2 = xres[b0 + t] + 0.5 * y
            xres[b0 + t] = x2
            o_ref[:, t * TB:(t + 1) * TB] = x2.astype(o_ref.dtype)

    plan = [[n_ - lag if 0 <= n_ - lag < NCH else NCH for lag in (GU_LAG, GU_LAG, D_LAG)] for n_ in range(NP)]
    rest = [(c, m) for c in range(NCH) for m in range(3) if c not in [p_[m] for p_ in plan]]
    order = [(p_[m], m) for p_ in plan for m in range(3) if p_[m] < NCH] + rest

    def prologue():
        cp_x(0).start()
        for sec in range(3):
            for cp in cp_qkv(sec):
                cp.start()
        for n_ in range(NP):
            for k in range(CP):
                plan_s[n_ * CP + k] = plan[n_][k]
        qall[:, pl.ds(0, HALO), :] = jnp.zeros((16, HALO, 128), f32)
        cp_x(0).wait()
        ln1(0, 0, 'in', (4, 0))
        ln1(0, 1, 'in', (4, 0))
        q_left(True)
        for sec in range(3):
            for cp in cp_qkv(sec):
                cp.wait()
            if sec == 0:
                cp_x(1).start()
                cp_x(2).start()
                cp_wo().start()
                for k, (c, m) in enumerate(order):
                    cp_unit(c, m).start()
                    if k % 2 == 0 and 3 + k // 2 < NP:
                        cp_x(3 + k // 2).start()
            transpose_qkv(sec)
            build_wq(sec)

    def first_attention():
        q_step(1, [], 'in', CFG_QA, rows=True)
        cp_wo().wait()
        build_wo()

        def cb(pos, v):
            if pos in (3, 8, 12, 16, 20):
                for k in range(8):
                    wq[27, pl.ds(zero8, 8), :] = pltpu.bitcast(v[k * 24:k * 24 + 8], u32)
                    build_wq_sums([todo.pop(0)])
        todo = list(range(0, 320, 8))
        rhs = {}
        wo_rhs(wo_seq, 0, rhs)
        wo_mm(0, rhs, cb)
        assert not todo
        ln2(0, 0, (4, 0))
        ln2(1, 1, (4, 0))
        a_left()
        a_arrange()

    def startup_step(n, carry):
        for n_ in range(NP):
            @pl.when(n == n_)
            def _():
                if n_ + 1 < NP:
                    cp_x(n_ + 1).wait()
                for m, c in enumerate(plan[n_]):
                    if c < NCH:
                        cp_unit(c, m).wait()

        @pl.when(n != 1)
        def _():
            if ONLY in ('', 'q'):
                q_step(n, [plan_s[n * CP + k] for k in range(CP)], 'in', CFG_Q1)

        @pl.when(n == 1)
        def _():
            if ONLY in ('', 'a'):
                first_attention()
        return carry

    @pl.when(g == 0)
    def _():
        if ONLY in ('', 'pro'):
            prologue()
        if ONLY in ('', 'q', 'a'):
            lax.fori_loop(0, NP, startup_step, 0)
        if not ONLY:
            for c, m in rest:
                cp_unit(c, m).wait()
                for piece in prep_pieces(c, m):
                    piece()

    @pl.when(jnp.logical_and(g >= NP - 1, g < 2 * NP - 1))
    def _():
        @pl.when(g == NP - 1)
        def _():
            if ONLY in ('', 'pro'):
                ln1(0, 0, 'res', (4, 0))
                ln1(0, 1, 'res', (4, 0))
                q_left(False)
        if ONLY in ('', 'q'):
            q_step(g - (NP - 1), [], 'res', CFG_Q2)

    if ONLY in ('q', 'a', 'pro'):
        @pl.when(g == 2 * NP - 1)
        def _():
            o_ref[0:16, 0:128] = (qall[g % 16, pl.ds(zero8, 16), :] + xres[g % 16, pl.ds(zero8, 16), :]
                                  + pltpu.bitcast(pw[g % 4, pl.ds(zero8, 16), 0:128] | s_scr[g % 8, pl.ds(zero8, 16), :]
                                                  | wo2[pl.ds(zero8, 16), :] | wq[g % 8, pl.ds(zero8, 16), :] | sq_scr[g % 8, pl.ds(zero8, 16), :], f32)).astype(bf16)

    @pl.when(g < 2 * NP - 1)
    def _():
        if ONLY in ('', 'p'):
            ffn(g, 0, SCRIPT)

    @pl.when(g == 2 * NP - 1)
    def _():
        def body(hf, carry):
            ffn(2 * NP - 1, hf * NPC, SCRIPT_F)
            return carry
        if ONLY in ('', 'f'):
            lax.fori_loop(0, 2, body, 0)


@jax.jit
def pallas_interleave_layers__sliding_local_dilated__glu_gated_geglu__prompt_kernel(
    A_x, A_wqkv, A_wo, B_x, B_w_gate, B_w_up, B_w_down):
    B, S, D = A_x.shape
    DF = B_w_gate.shape[1]
    NB = S // TB
    NP = NB // 2
    NCH = DF // CW
    xT = A_x.reshape(S, D).T
    wdT = B_w_down.T
    hbm = pl.BlockSpec(memory_space=pltpu.HBM)
    outT = pl.pallas_call(
        functools.partial(_kernel, D=D, DF=DF, S=S),
        grid=(2 * NP,),
        in_specs=[hbm] * 6,
        out_specs=pl.BlockSpec((D, 2 * TB), lambda g: (0, jnp.maximum(g - NP, 0))),
        out_shape=jax.ShapeDtypeStruct((D, S), A_x.dtype),
        scratch_shapes=[
            pltpu.VMEM((NP, D, 2 * TB), bf16),
            pltpu.VMEM((D, 3 * D), bf16),
            pltpu.VMEM((D, D), bf16),
            pltpu.VMEM((5, 14 * 128, 128), f32),
            pltpu.VMEM((28, 320, 128), u32),
            pltpu.VMEM((D // 2, 640), u32),
            pltpu.VMEM((15 * (D // 6) + 3 * (D // 4) + 16, 128), u32),
            pltpu.VMEM((NCH + 1, 3, D, CW), bf16),
            pltpu.VMEM((NCH + 1, 45 * (TC // 2) + 15 * (D // 6) + 16, 2 * TC), u32),
            pltpu.VMEM((16, S + QPAD, 128), f32),
            pltpu.VMEM((11, TB, 128), f32),
            pltpu.VMEM((NB, D, TB), f32),
            pltpu.VMEM((2, D, TB), f32),
            pltpu.VMEM((2, D, TB), f32),
            pltpu.VMEM((45, TB // 2, TC), u32),
            pltpu.VMEM((31, TB // 2, TC), u32),
            pltpu.VMEM((18, TB // 2, TC), u32),
            pltpu.SMEM((NP * CP,), jnp.int32),
            pltpu.SemaphoreType.DMA((4 + NP + 3 * NCH,)),
        ] + [pltpu.VMEM((TB, 2 * TC), f32)] * 29,
        compiler_params=pltpu.CompilerParams(
            dimension_semantics=("arbitrary",),
            vmem_limit_bytes=110 * 1024 * 1024,
            disable_bounds_checks=bool(NOCHK),
            disable_semaphore_checks=bool(NOCHK),
        ),
    )(xT, A_wqkv, A_wo, B_w_gate, B_w_up, wdT)
    return outT.T.reshape(B, S, D)
```

```python
import functools
import math
import jax
import jax.numpy as jnp
from jax import lax
import jax.experimental.pallas as pl
import jax.experimental.pallas.tpu as pltpu

H = 32
DH = 18
W = 8
DIL = 2
HALO = 16
EPS = 1e-5
TB = 128
RB = 8
TC = 128
CW = 6 * TC
WQR = 320
KY = 64
ONLY = ''
LN_P = tuple(int(x) for x in '1,2'.split(','))
CFG_Q1 = tuple(int(x) for x in '1,2,1500,2500'.split(','))
CFG_Q2 = tuple(int(x) for x in '1,2,60,560'.split(','))
QP0 = int(200); QP1 = int(4000); QTK = int(16)
MODE_P = tuple(int(x) for x in '1,3'.split(','))
MODE_A = tuple(int(x) for x in '1,3'.split(','))
SCRIPT = 'R1+50+400,G,R5+0+290,G,G,R10+0+350,G,D4,G,R5+0+290,G,G,R11+0+250,G,D4,W,n0+1500,n1+2124,l+3424+500,G,G,G,G,c+200+96,D4'.split(',')
SCRIPT_F = 'G,G,G,G,D2,G,G,D2,D2'.split(',')
DORD = tuple(int(x) for x in '1,6,0,9,10,4,11,5,14,7,2,8,3,12,13'.split(','))
LAGS = tuple(int(x) for x in '0,0,0'.split(','))
USPLIT = int(1)
CFG_Q0 = tuple(int(x) for x in '1,2,1500,2500'.split(','))
RG = tuple(int(x) for x in '2,1,48,420'.split(','))
RDL = int(700)
ZM = int(8)
JDL = int(250); LDL = int(600); GTK = int(2)
PLAG = int(4); DADV = int(1)
UFIRST = int(0); USCR = int(0)
CFG_QA = tuple(int(x) for x in '1,2,200,500'.split(','))
QA_T = tuple(int(x) for x in '100,800'.split(','))
QA_DEAD = tuple(int(x) for x in '1,1'.split(','))
QPAD = int(40)
LNJ = tuple(int(x) for x in '12,12,48,48'.split(','))
DTK = int(8)
XNF = int(1); XNL = int(1); NLEFT = int(3)
YSPLIT = tuple(int(x) for x in '0,21'.split(','))
WORD = tuple(int(x) for x in '0,1,2,6,7,8,9,10,11,12,13,14,3,4,5'.split(','))
NOCHK = int(1)

f32 = jnp.float32
bf16 = jnp.bfloat16
u32 = jnp.uint32
NT = (((1,), (1,)), ((), ()))


def _al(i, n):
    return i if isinstance(i, int) else pl.multiple_of(i, n)


def _lt(k):
    return slice(k * 128, (k + 1) * 128)


def _pk(x):
    return pltpu.bitcast(x.astype(bf16), u32)


def _up(x):
    return pltpu.bitcast(x, bf16)


def _dot(a, b):
    return jnp.dot(a, b, preferred_element_type=f32)


def _dot_nt(a, b):
    return lax.dot_general(a, b, NT, preferred_element_type=f32)


def _tree(fn, xs):
    xs = list(xs)
    while len(xs) > 1:
        xs = [fn(xs[i], xs[i + 1]) for i in range(0, len(xs) - 1, 2)] + ([xs[-1]] if len(xs) % 2 else [])
    return xs[0]


def _ln_stats(x, nacc, pin=None):
    n = x.shape[0]
    c = x[0:1] if pin is None else pin(x[0:8])[0:1]
    s1 = [None] * nacc
    s2 = [None] * nacc
    for i in range(n // 8):
        d = x[i * 8:(i + 1) * 8] - c
        k = i % nacc
        s1[k] = d if s1[k] is None else s1[k] + d
        dd = d * d
        s2[k] = dd if s2[k] is None else s2[k] + dd
    m = jnp.sum(_tree(jnp.add, s1), axis=0, keepdims=True) * (1.0 / n)
    v = jnp.sum(_tree(jnp.add, s2), axis=0, keepdims=True) * (1.0 / n) - m * m
    v = jnp.maximum(v, 0.0)
    return c + m, lax.rsqrt(v + EPS)


_HK_A = (
    ((0, 0, 1), (0, 2, -1), (1, 0, -1)), ((0, 0, 1), (0, 1, -1), (2, 0, -1)), ((1, 1, 1), (0, 1, -1), (1, 2, -1)),
    ((1, 1, 1), (1, 0, -1), (2, 1, -1)), ((2, 2, 1), (0, 2, -1), (2, 1, -1)), ((2, 2, 1), (1, 2, -1), (2, 0, -1)),
    ((0, 1, 1),), ((0, 1, 1), (1, 0, -1)), ((1, 0, 1),),
    ((0, 2, 1),), ((0, 2, 1), (2, 0, -1)), ((2, 0, 1),),
    ((1, 2, 1),), ((2, 1, 1), (1, 2, -1)), ((2, 1, 1),),
)
_HK_C = {
    (0, 0): ((0, 1), (7, 1), (8, 1), (9, 1), (6, -1)),
    (0, 1): ((1, 1), (6, 1), (10, 1), (11, 1), (9, -1)),
    (1, 0): ((2, 1), (7, 1), (8, 1), (12, 1), (6, -1)),
    (1, 1): ((3, 1), (6, 1), (13, 1), (14, 1), (2, -1), (7, -1)),
    (2, 0): ((5, 1), (9, 1), (12, 1), (13, 1), (4, -1), (10, -1)),
    (2, 1): ((4, 1), (10, 1), (11, 1), (14, 1), (9, -1)),
}


_HK_B = (((0, 0, 1),), ((0, 1, 1),), ((1, 0, 1),), ((1, 0, 1), (1, 1, 1)), ((2, 1, 1),), ((2, 0, 1), (2, 1, 1)),
         ((0, 1, 1), (1, 1, 1)), ((0, 1, 1), (1, 0, 1), (1, 1, 1)), ((0, 0, 1), (0, 1, 1), (1, 0, 1), (1, 1, 1)),
         ((0, 0, 1), (2, 0, 1)), ((0, 0, 1), (2, 0, 1), (2, 1, 1)), ((0, 0, 1), (0, 1, 1), (2, 0, 1), (2, 1, 1)),
         ((1, 0, 1), (2, 0, 1)), ((1, 0, 1), (2, 1, -1)), ((1, 1, 1), (2, 1, 1)))


def _hk_b(b):
    s1 = b[1][0] + b[1][1]
    s2 = b[2][0] + b[2][1]
    t7 = b[0][1] + s1
    t10 = b[0][0] + s2
    return (b[0][0], b[0][1], b[1][0], s1, b[2][1], s2, b[0][1] + b[1][1], t7, b[0][0] + t7,
            b[0][0] + b[2][0], t10, b[0][1] + t10, b[1][0] + b[2][0], b[1][0] - b[2][1], b[1][1] + b[2][1])


def _ssum(terms):
    terms = sorted([t for t in terms if t[0] is not None], key=lambda z: -z[1])
    if not terms:
        return None
    acc = terms[0][0] if terms[0][1] == 1 else -terms[0][0]
    for v, sg in terms[1:]:
        acc = acc + v if sg == 1 else acc - v
    return acc


GU_ORD = tuple(int(x) for x in '8,6,7,11,3,1,10,14,9,5,0,13,12,4,2'.split(','))
GU_POST = {
    8: ((), ('p8', None), None),
    7: ((('p8', 1),), (None, 't7'), None),
    3: ((('t7', 1),), (None, 's1'), None),
    6: ((), ('p6', None), None),
    14: ((('p6', 1), ('s1', 1)), ('p14', None), (1, 1)),
    12: ((('p9', 1), ('s2', 1)), ('p12', None), (2, 0)),
    13: ((), ('p13', None), None),
    2: ((('p12', 1), ('p13', 1), ('s1', 1)), (None, None), (1, 0)),
    11: ((), ('p11', None), None),
    10: ((('p11', 1),), (None, 't10'), None),
    5: ((('t10', 1),), (None, 's2'), None),
    9: ((), ('p9', None), None),
    4: ((('p14', 1), ('s2', 1), ('p13', -1)), (None, None), (2, 1)),
    0: ((('p8', 1), ('p9', 1), ('t10', 1)), (None, None), (0, 0)),
    1: ((('p6', 1), ('p11', 1), ('t7', 1)), (None, None), (0, 1)),
}
PSLOT = {k: i for i, k in enumerate(('p8', 't7', 's1', 'p6', 'p14', 'p12', 'p13', 'p11', 't10', 's2', 'p9'))}


class _Timeline:
    def __init__(self):
        self.t = 0
        self.jobs = []

    def add(self, when, fn):
        self.jobs.append((when, len(self.jobs), fn))
        self.jobs.sort(key=lambda z: z[:2])

    def tick(self, dur, v, n=1, seq=1):
        per = max(n // seq, 1)
        for k in range(n):
            self.t += dur // n
            r = (k % per) * (v.shape[0] // per)
            c = (k // per) * 128
            while self.jobs and self.jobs[0][0] <= self.t:
                self.jobs.pop(0)[2](v[r:r + 8, c:c + 128])


def _kernel(x_hbm, wqkv_hbm, wo_hbm, wg_hbm, wu_hbm, wd_hbm, o_ref,
            xin, wqkv_raw, wo_raw, tmp, wq, woT, wo2, raw, pw, qall, o_s, xres, xn_f, xn_g, s_scr, st_s, sq_scr,
            sems, *p_s, D, DF, S):
    g = pl.program_id(0)
    NB = S // TB
    NP = NB // 2
    NCH = DF // CW
    NPC = NCH // 2
    D3 = D // 3
    DHALF = D // 2
    nr = TB // RB
    hh = DHALF // 2
    zero8 = pl.multiple_of((g >> 20) * ZM, ZM)
    zvec = jnp.full((8, 128), (g >> 20).astype(u32), u32)

    def zero(k):
        return pl.multiple_of((g >> (8 + k)) * ZM, ZM)

    def tie(x, dep):
        return pltpu.bitcast(pltpu.bitcast(x, u32) | (pltpu.bitcast(dep, u32) & zvec), f32)

    QSEC = ((0, 5), (5, 9), (9, 14))

    def cp_qkv(sec):
        out = []
        for j in range(*QSEC[sec]):
            n = min(128, 3 * D - j * 128)
            out.append(pltpu.make_async_copy(wqkv_hbm.at[:, pl.ds(j * 128, n)], wqkv_raw.at[:, pl.ds(j * 128, n)],
                                             sems.at[sec]))
        return out

    def cp_wo():
        return pltpu.make_async_copy(wo_hbm, wo_raw, sems.at[3])

    def cp_x(k):
        return pltpu.make_async_copy(x_hbm.at[:, pl.ds(_al(k * 2 * TB, 128), 2 * TB)], xin.at[k], sems.at[4 + k])

    class Unit:
        def __init__(self, c, m):
            src = (wg_hbm, wu_hbm, wd_hbm)[m]
            n = D // USPLIT
            self.cps = [pltpu.make_async_copy(src.at[pl.ds(k * n, n), pl.ds(_al(c * CW, 128), CW)],
                                              raw.at[c, m, pl.ds(k * n, n), :], sems.at[4 + NP + 3 * c + m])
                        for k in range(USPLIT)]

        def start(self):
            for cp in self.cps:
                cp.start()

        def wait(self):
            for cp in self.cps:
                cp.wait()
    cp_unit = Unit

    R_SD = 45 * (TC // 2)
    R_END = R_SD + 15 * (D3 // 2)

    def hk_a_ops(load, minus=None):
        blk = {}
        for i in range(3):
            for j in range(3):
                blk[i, j] = load(i, j).astype(f32)
                if minus is not None:
                    blk[i, j] = blk[i, j] - minus(i, j).astype(f32)
        return [_pk(_ssum([(blk[i, j], sg) for i, j, sg in terms])) for terms in _HK_A]

    def prep_pieces(c, m):
        def ld(r, cs):
            return lambda i, j: raw[c, m, pl.ds(i * D3 + r, 16), pl.ds((3 * cs + j) * TC, TC)]

        def gu_piece(q, r, cs, neg, kind, half):
            ops = hk_a_ops(ld(q * KY + r, cs), None if neg is None else ld(q * KY + r, neg))
            for k, t in enumerate(ops):
                pw.at[c][pl.ds((3 * k + kind) * (TC // 2) + (half * KY + r) // 2, 8), m * TC:(m + 1) * TC] = t

        def d_piece(r, cs):
            for k, t in enumerate(hk_a_ops(ld(r, cs))):
                pw.at[c][pl.ds(R_SD + k * (D3 // 2) + r // 2, 8), cs * TC:(cs + 1) * TC] = t
        if m == 2:
            return [functools.partial(d_piece, r, cs) for r in range(0, D3, 16) for cs in range(2)]
        spec = ((0, 0, None, 0, 0), (1, 0, 1, 0, 1), (0, 1, None, 1, 0), (2, 1, 0, 1, 1),
                (2, 0, None, 2, 0), (1, 1, None, 2, 1))
        return [functools.partial(gu_piece, q, r, cs, neg, kind, half)
                for r in range(0, KY, 16) for q, cs, neg, kind, half in spec]

    def transpose_qkv(sec):
        for j in range(*QSEC[sec]):
            wd_ = min(128, 3 * D - j * 128)
            blk = wqkv_raw[:, j * 128:j * 128 + wd_].astype(f32)
            if wd_ < 128:
                blk = jnp.concatenate([blk, jnp.zeros((D, 128 - wd_), f32)], axis=1)
            bt = jnp.concatenate([blk, blk[D - KY:]], axis=0).T
            for t in range(5):
                tmp[t, pl.ds(j * 128, 128), :] = bt[:, t * 128:(t + 1) * 128]

    def wq_slot(i, j):
        return 24 + i if i == j else [n for n, t in enumerate(_HK_A) if t == ((i, j, 1),)][0]

    def build_wq(sec):
        lo = lax.broadcasted_iota(jnp.int32, (32, 128), 1) < KY
        for d in range(DH):
            tt = [tmp[t, pl.ds(sec * D + d, 32, stride=DH), :] for t in range(5)]
            ops = tt[:4] + [jnp.where(lo, tt[3], tt[4]), jnp.where(lo, tt[4], tt[3])]
            if d < 16:
                dst = [(sec, d * 16)]
            else:
                dst = ([(1, (d + 2) * 16)], [(1, d * 16)], [(0, d * 16), (0, (d + 2) * 16)])[sec]
            for j, row in dst:
                for k, v in enumerate(ops):
                    wq[pl.ds(row, 16), _lt(wq_slot(k, j) if k < 3 else 12 + 3 * j + k)] = _pk(v)

    def wq_sums(r, dep):
        ncol = 3 if r < 256 else 2
        pin = pltpu.bitcast(dep, u32) & zvec
        blk = {(i, j): _up(wq[pl.ds(r, 8), _lt(wq_slot(i, j))] | pin).astype(f32) for i in range(3) for j in range(ncol)}
        for n, terms in enumerate(_HK_A):
            if len(terms) > 1 and not (ncol == 2 and n in (4, 5)):
                wq[pl.ds(r, 8), _lt(n)] = _pk(_ssum([(blk[i, j], sg) for i, j, sg in terms if j < ncol]))

    def build_wo():
        for t in range(5):
            wd_ = min(128, D - t * 128)
            blk = wo_raw[:, t * 128:t * 128 + wd_].astype(f32)
            if wd_ < 128:
                blk = jnp.concatenate([blk, jnp.zeros((D, 128 - wd_), f32)], axis=1)
            tmp[t, pl.ds(0, D), :] = blk
        for t in range(5):
            rows = [tmp[t, pl.ds(d, 32, stride=DH), :] for d in range(DH)]
            ft = jnp.concatenate(rows + rows[16:], axis=0).T
            n = min(128, D - t * 128)
            woT[pl.ds(t * 64, n // 2), :] = _pk(ft[:n])
        for r in range(0, D3 // 2, 8):
            ops = hk_a_ops(lambda i, j: _up(woT[pl.ds(i * (D3 // 2) + r, 8), j * TC:(j + 1) * TC]))
            for k, t in enumerate(ops):
                wo2[pl.ds(r, 8), _lt(k)] = t
        lo = lax.broadcasted_iota(jnp.int32, (16, 128), 1) < KY
        for r in range(0, hh, 8):
            a3, a4, b3, b4 = [_up(woT[pl.ds(r0 + r, 8), c0:c0 + 128]).astype(f32)
                              for r0 in (0, hh) for c0 in (384, 512)]
            wo2[pl.ds(r, 8), _lt(15)] = _pk(jnp.where(lo, a3, a3 - b3))
            wo2[pl.ds(r, 8), _lt(16)] = _pk(jnp.where(lo, b3, b4 - a4))
            wo2[pl.ds(r, 8), _lt(17)] = _pk(jnp.where(lo, a4, b3))

    def normalize(blk, mean, rstd, link):
        if not link:
            return (xres[blk] - mean) * rstd
        rs = jnp.broadcast_to(rstd, (8, TB))
        mb = jnp.broadcast_to(mean, (8, TB))
        outs = []
        for i in range(D // 8):
            if i and i % link == 0:
                rs = tie(rs, outs[-1])
            outs.append((xres[blk, pl.ds(i * 8, 8), :] - mb) * rs)
        return jnp.concatenate(outs, axis=0)

    def left_ops(src, put, plain=False, which=None, dep=None):
        def X(t, r0, n):
            return src[t, pl.ds(r0, n), :]
        k1, k2, k3 = 3 * TC, 3 * TC + KY, 3 * TC + 2 * KY
        for n in (list(range(6 if plain else 15)) + [15, 16, 17]) if which is None else which:
            if n == 15:
                v = jnp.concatenate([X(0, k1, KY), X(0, k2, KY) - X(1, k2, KY)], axis=0)
            elif n == 16:
                v = jnp.concatenate([X(1, k1, KY), X(1, k3, KY) - X(0, k3, KY)], axis=0)
            elif n == 17:
                v = jnp.concatenate([X(0, k3, KY), X(1, k2, KY)], axis=0)
            elif plain:
                v = X(n // 3, (n % 3) * TC, TC)
            else:
                v = _ssum([(X(t, i * TC, TC), sg) for (i, t), lst in _HK_C.items() for k, sg in lst if k == n])
            if dep is not None:
                v = jnp.concatenate([tie(v[0:8], dep), v[8:]], axis=0)
            put(n, pltpu.bitcast(v.astype(bf16).T, u32))

    def ln1(pr, par, src, ln, dep=None):
        blk = 2 * pr + par
        if src == 'res':
            x = xres[blk]
        else:
            x = xin[pr, :, par * TB:(par + 1) * TB].astype(f32)
            xres[blk] = x
        mean, rstd = _ln_stats(x, ln[0], None if dep is None else (lambda v: tie(v, dep)))
        if src == 'res':
            xn_g[par, pl.ds(0, 8), :] = jnp.zeros((8, TB), f32)
        xn_g[par, pl.ds(zero8, D), :] = normalize(blk, mean, rstd, ln[1])

    def q_left(plain):
        def put(i, v):
            sq_scr[i] = v
        left_ops(xn_g, put, plain)

    def hk_outputs(P, T, PT, tk, emit, two_cols=False):
        p8 = P(8)
        t7 = P(7) + p8
        tk(2, t7)
        s1 = PT(3, 1, 2) + t7
        tk(2, s1)
        p6 = P(6)
        p14 = P(14)
        tk(2, p14)
        emit(1, 1, T(1, 1) + (p6 + p14 + s1), 1)
        p13 = P(13)
        if two_cols:
            emit(1, 0, PT(2, 1, 0) + (p13 + s1), 3)
        else:
            p12 = P(12)
            tk(2, p12)
            emit(1, 0, PT(2, 1, 0) + (p12 + p13 + s1), 2)
        p11 = P(11)
        t10 = P(10) + p11
        tk(2, t10)
        if not two_cols:
            s2 = PT(5, 2, 2) + t10
            tk(2, s2)
            p9 = P(9)
            emit(2, 0, T(2, 0) + (p9 + p12 + s2), 2)
            emit(2, 1, PT(4, 2, 1) + (p14 - p13 + s2), 2)
        w0 = T(0, 2)
        emit(0, 0, PT(0, 0, 0) + ((p8 + t10 + w0) if two_cols else (p8 + p9 + t10 + w0)), 3)
        emit(0, 1, PT(1, 0, 1) + (p6 + p11 + t7 + w0), 2)

    QT = (0, 1, 2, 3)
    KT = (4, 5, 6, 7, 13)
    VT = (8, 9, 10, 11, 12)
    c2e = DH ** -0.5 * math.log2(math.e)
    neg = -1e9 * math.log2(math.e)

    def q_step(pr, chunk, src, cfg, rows=False, sums=False):
        clock = _Timeline()
        if sums:
            base, nx = 0, 1
            for k in range(40):
                clock.add(200 + k * 90, functools.partial(wq_sums, 8 * k))
        elif rows:
            base, nx = pr * (2 * TB), pr + 1
            clock.add(QA_T[0], functools.partial(a_rows, 0, 0, MODE_A))
            clock.add(QA_T[1], functools.partial(a_rows, 1, 1, MODE_A))
        else:
            base = pl.multiple_of(pr * (2 * TB), 2 * TB)
            nx = jnp.minimum(pr + 1, NP - 1)
        ln_q, la_t, lb_t = cfg[:2], cfg[2], cfg[3]
        pieces = []
        if chunk is not None:
            for m in range(3):
                pieces += prep_pieces(jnp.maximum(chunk - LAGS[m], 0) if LAGS[m] else chunk, m)

        def paced(piece, dep):
            pw[0, pl.ds(R_END, 8), 0:128] = pltpu.bitcast(dep, u32)
            piece()
        for k, piece in enumerate(pieces):
            clock.add(QP0 + k * (QP1 - QP0) // len(pieces), functools.partial(paced, piece))
        clock.add(la_t, lambda dep: ln1(nx, 0, src, ln_q, dep))
        clock.add(lb_t, lambda dep: ln1(nx, 1, src, ln_q, dep))
        for r0, nt, tiles in ((0, 2, (0, 4, 8)), (TC, 2, (2, 6, 10)), (2 * TC, 1, (12, 13))):
            def R(k):
                return wq[pl.ds(r0, nt * 64), _lt(k)]

            def P(k):
                return _dot_nt(_up(sq_scr[k]), _up(R(k)))

            def T(j, kind):
                return _dot_nt(_up(sq_scr[15 + kind]), _up(R(15 + 3 * j + kind)))

            def PT(k, j, kind):
                return _dot_nt(_up(jnp.concatenate([sq_scr[k], sq_scr[15 + kind]], axis=1)),
                               _up(jnp.concatenate([R(k), R(15 + 3 * j + kind)], axis=1)))

            def tk(np_, v):
                clock.tick(32 * nt * np_, v, QTK if src == 'in' else 4, nt if src == 'in' else 1)

            def emit(col, half, v, np_):
                for k in range(nt):
                    qall[tiles[col] + k, pl.ds(base + (HALO + half * TB), TB), :] = v[:, k * 128:(k + 1) * 128]
                tk(np_, v)
            if src == 'res':
                hk_outputs(P, T, PT, tk, emit, two_cols=(nt == 1))
                continue
            for j in range(len(tiles)):
                both = T(j, 2)
                for t in range(2):
                    lhs = [sq_scr[3 * t + i] for i in range(3)] + [sq_scr[15 + t]]
                    if rows and nt == 1 and (j, t) == QA_DEAD:
                        probe = pltpu.bitcast(o_s[0, pl.ds(zero8, 8), :], u32)
                        lhs[0] = jnp.concatenate([lhs[0][0:8] | (probe & zvec), lhs[0][8:]], axis=0)
                    rhs = [R(wq_slot(i, j)) for i in range(3)] + [R(15 + 3 * j + t)]
                    emit(j, t, _dot_nt(_up(jnp.concatenate(lhs, axis=1)), _up(jnp.concatenate(rhs, axis=1))) + both,
                         5 - t)
        assert not clock.jobs
        q_left(src == 'in')

    def a_rows(blk, par, mode, start=None, rs=None):
        lag_mid, lag_end = mode[:2]
        fw, fv = mode[2:] if len(mode) > 2 else (0, 0)
        base = blk * TB if isinstance(blk, int) else pl.multiple_of(blk * TB, TB)
        cbits = pltpu.bitcast(jnp.full((RB, 128), c2e, f32), u32)
        lo = lax.broadcasted_iota(jnp.int32, (RB, 128), 1) < KY
        mid, fin = {}, {}
        rs = range(nr) if rs is None else rs
        for r in rs:
            r0 = r * RB
            deps = [start] if (start is not None and r == rs[0]) else []
            if lag_mid and r >= lag_mid:
                deps.append(mid[r - lag_mid])
            if lag_end and r >= lag_end:
                deps += fin[r - lag_end]
            if deps:
                acc = _tree(jnp.bitwise_or, [pltpu.bitcast(v, u32) for v in deps])
                cs = pltpu.bitcast(cbits | (acc & zvec), f32)
            else:
                cs = c2e

            def ld(t, w):
                return qall[t, pl.ds(base + (HALO + r0 - DIL * w), RB), :]
            q = [ld(t, 0) * cs for t in QT] + [jnp.where(lo, pltpu.roll(ld(13, 0), KY, 1), 0.0) * cs]
            sc = []
            for w in range(W):
                q0 = tie(q[0], prev) if (fw and w and w % fw == 0) else (q[0] if w == 0 else q0)
                acc = None
                for j, t in enumerate(KT):
                    p = (q0 if j == 0 else q[j]) * ld(t, w)
                    acc = p if acc is None else acc + p
                prev = acc
                acc = acc + pltpu.roll(acc, 64, 1)
                mid[r] = acc
                acc = acc + pltpu.roll(acc, 32, 1)
                if r0 - DIL * w < 0:
                    pos = blk * TB + r0 + lax.broadcasted_iota(jnp.int32, (RB, 128), 0)
                    acc = jnp.where(pos >= DIL * w, acc, neg)
                sc.append(acc)
            m = _tree(jnp.maximum, sc)
            e = [jnp.exp2(sc[w] - m) for w in range(W)]
            l = _tree(jnp.add, e)
            rinv = pl.reciprocal(l, approx=True)
            rinv = rinv * (2.0 - l * rinv)
            fin[r] = []
            for j, t in enumerate(VT):
                e0 = tie(e[0], acc) if (fv and j and j % fv == 0) else (e[0] if j == 0 else e0)
                acc = None
                for w in range(W):
                    p = (e0 if w == 0 else e[w]) * ld(t, w)
                    acc = p if acc is None else acc + p
                o = acc * rinv
                o_s[par * 5 + j, pl.ds(r0, RB), :] = o
                fin[r] = [o] if fv == 1 else fin[r] + [o]
        return lambda: _tree(jnp.bitwise_or, [pltpu.bitcast(v, u32) for v in fin[rs[-1]]])

    def row_group(blk, par, r, nw, nv):
        base = pl.multiple_of(blk * TB, TB)
        lo = lax.broadcasted_iota(jnp.int32, (RB, 128), 1) < KY
        r0 = r * RB

        def ld(t, w):
            return qall[t, pl.ds(base + (HALO + r0 - DIL * w), RB), :]
        dep = yield
        cs = tie(jnp.full((RB, 128), c2e, f32), dep)
        q = [ld(t, 0) * cs for t in QT] + [jnp.where(lo, pltpu.roll(ld(13, 0), KY, 1), 0.0) * cs]
        sc = []
        for w in range(W):
            if w and w % nw == 0:
                dep = yield
                q = [tie(q[0], dep)] + q[1:]
            acc = None
            for j, t in enumerate(KT):
                p = q[j] * ld(t, w)
                acc = p if acc is None else acc + p
            acc = acc + pltpu.roll(acc, 64, 1)
            acc = acc + pltpu.roll(acc, 32, 1)
            if r0 - DIL * w < 0:
                pos = blk * TB + r0 + lax.broadcasted_iota(jnp.int32, (RB, 128), 0)
                acc = jnp.where(pos >= DIL * w, acc, neg)
            sc.append(acc)
        m = _tree(jnp.maximum, sc)
        e = [jnp.exp2(sc[w] - m) for w in range(W)]
        l = _tree(jnp.add, e)
        rinv = pl.reciprocal(l, approx=True)
        rinv = rinv * (2.0 - l * rinv)
        outs = []
        for j, t in enumerate(VT):
            if j and j % nv == 0:
                dep = yield _tree(jnp.bitwise_or, [pltpu.bitcast(v, u32) for v in outs])
                outs = []
                e = [tie(e[0], dep)] + e[1:]
            acc = None
            for w in range(W):
                p = e[w] * ld(t, w)
                acc = p if acc is None else acc + p
            o = acc * rinv
            o_s[par * 5 + j, pl.ds(r0, RB), :] = o
            outs.append(o)
        yield _tree(jnp.bitwise_or, [pltpu.bitcast(v, u32) for v in outs])

    wo_seq = []
    for pos, k in enumerate(WORD):
        if pos in (0, 2):
            wo_seq += [('r', pos // 2, k_) for k_ in range(3)]
        wo_seq.append(('p', k))

    def wo_rhs(items, off, rhs):
        lo = lax.broadcasted_iota(jnp.int32, (TB, 128), 1) < KY

        for it in items:
            z = zero(wo_seq.index(it)) if off is None else off

            def O(t, j):
                return o_s[t * 5 + j, pl.ds(z, TB), :]
            if it[0] == 'p':
                v = _ssum([(O(t, j), sg) for j, t, sg in _HK_B[it[1]]])
            elif it[2] == 0:
                v = O(it[1], 3)
            else:
                v = jnp.where(lo, O(it[1], 2 + it[2]), O(it[1], 5 - it[2]))
            rhs[it] = v.astype(bf16)

    def wo_mm(blk0, rhs):
        res = {}
        for it in wo_seq:
            if it[0] == 'p':
                lhs = wo2[pl.ds(0, D3 // 2), _lt(it[1])]
            else:
                lhs = wo2[:, _lt(15 + it[2])]
            res[it] = _dot_nt(_up(lhs), rhs[it])
        for t in range(2):
            both = res['r', t, 2]
            rem = xres[blk0 + t] + jnp.concatenate([res['r', t, 0] + both, res['r', t, 1] + both], axis=0)
            y = jnp.concatenate([_ssum([(res['p', k], sg) for k, sg in _HK_C[i, t]]) for i in range(3)], axis=0)
            xres[blk0 + t] = y + rem

    def ln2(blk, par, ln, dep=None):
        mean, rstd = _ln_stats(xres[blk, pl.ds(zero8 if XNL else 0, D), :], ln[0],
                               None if dep is None else (lambda v: tie(v, dep)))
        xn_f[par, pl.ds(0, 8), :] = jnp.zeros((8, TB), f32)
        xn_f[par, pl.ds(zero8 if XNF else 0, D), :] = normalize(blk, mean, rstd, ln[1])

    def ln_jobs(blk, dst, par, np1, np2):
        st = dict(s1=[], s2=[])
        nv = D // 8

        def stats(k, dep):
            if k == 0:
                st['c'] = jnp.broadcast_to(xres[blk, pl.ds(zero8, 8), :][0:1], (8, TB))
            c = tie(st['c'], dep)
            ds = [xres[blk, pl.ds(zero8 + i * 8, 8), :] - c for i in range(k * nv // np1, (k + 1) * nv // np1)]
            st['s1'].append(_tree(jnp.add, ds))
            st['s2'].append(_tree(jnp.add, [d * d for d in ds]))
            a_, b_ = st['s1'][-1], st['s2'][-1]
            return lambda: pltpu.bitcast(a_, u32) | pltpu.bitcast(b_, u32)

        def norm(k, dep):
            if k == 0:
                m = jnp.sum(_tree(jnp.add, st['s1']), axis=0, keepdims=True) * (1.0 / D)
                v = jnp.sum(_tree(jnp.add, st['s2']), axis=0, keepdims=True) * (1.0 / D) - m * m
                st['mean'] = st['c'] + m
                st['rstd'] = jnp.broadcast_to(lax.rsqrt(jnp.maximum(v, 0.0) + EPS), (8, TB))
            mean = tie(st['mean'], dep)
            for i in range(k * nv // np2, (k + 1) * nv // np2):
                dst[par, pl.ds(i * 8, 8), :] = (xres[blk, pl.ds(i * 8, 8), :] - mean) * st['rstd']
            return lambda: pltpu.bitcast(dst[par, pl.ds(zero8, 8), :], u32)
        return [functools.partial(stats, k) for k in range(np1)], [functools.partial(norm, k) for k in range(np2)]

    def a_left(which=range(15), dep=None):
        for n in which:
            v = _ssum([(xn_f[t, pl.ds(zero(n) + i * D3, D3), :], sg)
                       for (i, t), lst in _HK_C.items() for k, sg in lst if k == n])
            if dep is not None:
                v = jnp.concatenate([tie(v[0:8], dep), v[8:2 * KY], tie(v[2 * KY:2 * KY + 8], dep), v[2 * KY + 8:]],
                                    axis=0)
            st_s[2 * n] = pltpu.bitcast(v[:2 * KY].astype(bf16).T, u32)
            st_s[2 * n + 1] = pltpu.bitcast(jnp.concatenate([v[2 * KY:], v[2 * KY:]], axis=0).astype(bf16).T, u32)

    def a_arrange(which=range(15), dep=None):
        lo = lax.broadcasted_iota(jnp.int32, (TB // 2, 128), 1) < KY
        if dep is not None:
            st_s[30, pl.ds(0, 8), :] = pltpu.bitcast(dep, u32)
        for n in which:
            t1 = st_s[2 * n, pl.ds(zero8, TB // 2), :]
            t2 = st_s[2 * n + 1, pl.ds(zero8, TB // 2), :]
            s_scr[3 * n] = t1
            s_scr[3 * n + 1] = jnp.where(lo, t1, t2)
            s_scr[3 * n + 2] = jnp.where(lo, t2, t1)

    k0 = math.sqrt(2.0 / math.pi)
    k1 = k0 * 0.044715

    def ffn(j, c0, script):
        clock = _Timeline()
        b0 = (2 * j) % NB
        an = (2 * j + 2) % NB
        acc = [None] * 15
        hs = {}
        wrhs = {}
        state = dict(odep=False, rows=0, norm=0, left=set())

        pend = []
        fresh = []

        def advance(keep):
            while len(pend) > keep:
                pend.pop(0)()

        def probe_of(ref_val):
            return pltpu.bitcast(ref_val, u32) & zvec

        def take_probe():
            pr = _tree(jnp.bitwise_or, [k() if callable(k) else pltpu.bitcast(p_s[k][pl.ds(zero8, 8), 0:128], u32)
                                        for k in fresh]) & zvec
            del fresh[:]
            return pr

        def with_deadline(job, delay):
            def run(dep):
                val = job(dep)()
                clock.add(clock.t + delay, lambda _: fresh.append(lambda: val))
            return run

        def gu(p):
            c, second = c0 + p // 2, p % 2
            m = 1 - second if UFIRST else second
            h = hs.setdefault(p // 2, [[None, None] for _ in range(3)])

            def mm(n, kind, probe=None):
                lhs = s_scr[3 * n + kind]
                if state['odep']:
                    pr = probe_of(o_s[0, pl.ds(zero8, 8), :])
                    probe = pr if probe is None else probe | pr
                    state['odep'] = False
                if probe is not None:
                    lhs = jnp.concatenate([lhs[0:8] | probe, lhs[8:]], axis=0)
                return _dot(_up(lhs), _up(pw[c, pl.ds((3 * n + kind) * (TC // 2), TC // 2), m * TC:(m + 1) * TC]))

            def get(name):
                return p_s[PSLOT[name]][pl.ds(zero8, TB), :]

            def post(n, v):
                adds, keep, emits = GU_POST[n]
                if keep[0] is not None:
                    p_s[PSLOT[keep[0]]][...] = v
                    fresh.append(PSLOT[keep[0]])
                w_ = v
                for name, sg in adds:
                    w_ = w_ + get(name) if sg == 1 else w_ - get(name)
                if keep[1] is not None:
                    p_s[PSLOT[keep[1]]][...] = w_
                    fresh.append(PSLOT[keep[1]])
                if emits is not None:
                    col, half = emits
                    if m == 0:
                        w_ = w_ + w_ * jnp.tanh(w_ * (k0 + k1 * (w_ * w_)))
                    if second:
                        k_ = 17 + 6 * ((p // 2) % 2) + 2 * col + half
                        p_s[k_][...] = w_ * p_s[11 + 2 * col + half][pl.ds(zero8, TB), :]
                        fresh.append(k_)
                        h[col][half] = k_
                    else:
                        p_s[11 + 2 * col + half][...] = w_
                        fresh.append(11 + 2 * col + half)
            for n in GU_ORD:
                both = mm(n, 2, take_probe() if fresh else None)
                v = jnp.concatenate([mm(n, 0) + both, mm(n, 1) + both], axis=1)
                pend.append(functools.partial(post, n, v))
                advance(PLAG)
                clock.tick(96, both, GTK)

        def down(ps):
            cs = ps[::2]
            hsl = [hs.pop(p // 2) for p in cs]
            for pos, i in enumerate(DORD):
                while any(h_[j_][t_] is None for h_ in hsl for j_, t_, _ in _HK_B[i]):
                    advance(len(pend) - 1)
                au = []
                for p in cs:
                    au += [pw[c0 + p // 2, pl.ds(R_SD + i * (D3 // 2), D3 // 2), k * TC:(k + 1) * TC] for k in range(2)]
                if fresh:
                    au[0] = jnp.concatenate([au[0][0:8] | take_probe(), au[0][8:]], axis=0)
                r = _dot_nt(jnp.concatenate([_up(v) for v in au], axis=1),
                            jnp.concatenate([_ssum([(p_s[h_[j_][t_]][pl.ds(zero(i), TB), :], sg) for j_, t_, sg in _HK_B[i]])
                                             for h_ in hsl], axis=1).astype(bf16))
                acc[i] = r if acc[i] is None else r + acc[i]
                advance(max(len(pend) - DADV, 0))
                clock.tick(48 * len(ps), acc[i], DTK)

        pg = pd = 0
        for tok in script:
            if tok == 'G':
                gu(pg)
                pg += 1
            elif tok[0] == 'D':
                down(list(range(pd, pd + int(tok[1:]))))
                pd += int(tok[1:])
            elif tok == 'W':
                assert not [j_ for j_ in clock.jobs if j_[2].__class__ is functools.partial or j_[2].__name__ == 'run']
                assert state['rows'] in (0, 2 * nr)
                advance(0)
                if not wrhs:
                    wo_rhs(wo_seq, None, wrhs)
                wo_mm(an, wrhs)
                clock.t += 1152
            elif tok[0] == 'Y':
                def hold(items, dep):
                    o_s[10, pl.ds(0, 8), :] = dep
                    wo_rhs(items, None, wrhs)
                lo_, hi_ = YSPLIT[int(tok[1])], YSPLIT[int(tok[1]) + 1]
                clock.add(clock.t + int(tok[3:]), functools.partial(hold, wo_seq[lo_:hi_]))
            elif tok == 'X':
                state['odep'] = True
            elif tok[0] == 'n':
                j1, j2 = ln_jobs(an + int(tok[1]), xn_f, int(tok[1]), LNJ[0], LNJ[1])
                t_ = clock.t + int(tok[3:])
                for job in j1:
                    clock.add(t_, with_deadline(job, JDL))
                    t_ += LNJ[2]
                t_ += LNJ[3]
                for job in j2:
                    def counted(job_, dep):
                        state['norm'] += 1
                        return job_(dep)
                    clock.add(t_, with_deadline(functools.partial(counted, job), JDL))
                    t_ += LNJ[2]
            elif tok[0] == 'l':
                _, t0_, dt_ = tok.split('+')

                def left(which, dep):
                    assert state['norm'] == 2 * LNJ[1]
                    state['left'].update(which)
                    a_left(which, dep)
                    return lambda: st_s[0, pl.ds(zero8, 8), :]
                for k_ in range(NLEFT):
                    clock.add(clock.t + int(t0_) + k_ * int(dt_), with_deadline(
                        functools.partial(left, list(range(k_ * 15 // NLEFT, (k_ + 1) * 15 // NLEFT))), LDL))
            elif tok[0] == 'c':
                _, t0_, dt_ = tok.split('+')
                for k_ in range(15):
                    def arrange(k__, dep):
                        assert k__ in state['left'] and pg == 2 * NCH
                        a_arrange([k__], dep)
                    clock.add(clock.t + int(t0_) + k_ * int(dt_), functools.partial(arrange, k_))
            elif tok[0] == 'R':
                n_, t0_, dt_ = tok[1:].split('+')
                for k_ in range(int(n_)):
                    par, r_ = divmod(state['rows'], nr)
                    state['rows'] += 1
                    gen = row_group(an + par, par, r_, RG[0], RG[1])
                    next(gen)

                    def stage(gen_, delay, dep):
                        val = gen_.send(dep)
                        if val is not None:
                            clock.add(clock.t + delay, lambda _: fresh.append(lambda: val))
                    t_ = clock.t + int(t0_) + k_ * int(dt_)
                    n1_, n2_ = -(-W // RG[0]), -(-5 // RG[1])
                    for s_ in range(n1_):
                        clock.add(t_ + s_ * RG[2], functools.partial(stage, gen, RDL))
                    for s_ in range(n2_ - 1):
                        clock.add(t_ + (n1_ - 1) * RG[2] + RG[3] + s_ * RG[2], functools.partial(stage, gen, JDL))
            else:
                par = 0 if tok[1] == 'a' else 1
                clock.add(clock.t + int(tok[3:] or 0), functools.partial(a_rows, an + par, par, MODE_P))
        assert pg == pd and not [j_ for j_ in clock.jobs if j_[2].__class__ is functools.partial or j_[2].__name__ == 'run']
        for t in range(2):
            y = jnp.concatenate([_ssum([(acc[k], sg) for k, sg in _HK_C[i, t]]) for i in range(3)], axis=0)
            x2 = xres[b0 + t] + 0.5 * y
            xres[b0 + t] = x2
            o_ref[:, t * TB:(t + 1) * TB] = x2.astype(o_ref.dtype)

    assert NCH == NP - 2

    late = [(c, m) for c in range(NCH) for m in range(3) if c >= NCH - LAGS[m]]

    def prologue():
        cp_x(0).start()
        for sec in range(3):
            for cp in cp_qkv(sec):
                cp.start()
        qall[:, pl.ds(0, HALO), :] = jnp.zeros((16, HALO, 128), f32)
        cp_x(0).wait()
        ln1(0, 0, 'in', (4, 0))
        ln1(0, 1, 'in', (4, 0))
        q_left(True)
        for sec in range(3):
            for cp in cp_qkv(sec):
                cp.wait()
            if sec == 0:
                cp_x(1).start()
                cp_x(2).start()
                cp_wo().start()
                for c in range(NCH):
                    if 3 + c < NP:
                        cp_x(3 + c).start()
                    for m in range(3):
                        if c == 0 or c > LAGS[m]:
                            cp_unit(max(c - LAGS[m], 0), m).start()
                for c, m in late:
                    cp_unit(c, m).start()
            transpose_qkv(sec)
            build_wq(sec)

    def first_attention():
        cp_x(2).wait()
        q_step(1, None, 'in', CFG_QA, rows=True)
        cp_wo().wait()
        build_wo()
        rhs = {}
        wo_rhs(wo_seq, 0, rhs)
        wo_mm(0, rhs)
        ln2(0, 0, (4, 0))
        ln2(1, 1, (4, 0))
        a_left()
        a_arrange()

    def startup_step(c, carry):
        @pl.when(c + 3 < NP)
        def _():
            cp_x(c + 3).wait()
        for m in range(3):
            if LAGS[m]:
                @pl.when(jnp.logical_or(c == 0, c > LAGS[m]))
                def _():
                    cp_unit(jnp.maximum(c - LAGS[m], 0), m).wait()
            else:
                cp_unit(c, m).wait()
        q_step(c + 2, c, 'in', CFG_Q1)
        return carry

    @pl.when(g == 0)
    def _():
        if ONLY in ('', 'pro'):
            prologue()
            cp_x(1).wait()
            q_step(0, None, 'in', CFG_Q0, sums=True)
        if ONLY in ('', 'a'):
            first_attention()
        if ONLY in ('', 'q'):
            lax.fori_loop(0, NCH, startup_step, 0)
        if not ONLY:
            for c, m in late:
                cp_unit(c, m).wait()
                for piece in prep_pieces(c, m):
                    piece()

    @pl.when(jnp.logical_and(g >= NP - 1, g < 2 * NP - 1))
    def _():
        @pl.when(g == NP - 1)
        def _():
            if ONLY in ('', 'pro'):
                ln1(0, 0, 'res', (4, 0))
                ln1(0, 1, 'res', (4, 0))
                q_left(False)
        if ONLY in ('', 'q'):
            q_step(g - (NP - 1), None, 'res', CFG_Q2)

    if ONLY in ('q', 'a', 'pro'):
        @pl.when(g == 2 * NP - 1)
        def _():
            o_ref[0:16, 0:128] = (qall[g % 16, pl.ds(zero8, 16), :] + xres[g % 16, pl.ds(zero8, 16), :]
                                  + pltpu.bitcast(pw[g % 4, pl.ds(zero8, 16), 0:128] | s_scr[g % 8, pl.ds(zero8, 16), :]
                                                  | wo2[pl.ds(zero8, 16), 0:128] | wq[pl.ds(zero8, 16), 0:128] | sq_scr[g % 8, pl.ds(zero8, 16), :], f32)).astype(bf16)

    @pl.when(g < 2 * NP - 1)
    def _():
        if ONLY in ('', 'p'):
            ffn(g, 0, SCRIPT)

    @pl.when(g == 2 * NP - 1)
    def _():
        def body(hf, carry):
            ffn(2 * NP - 1, hf * NPC, SCRIPT_F)
            return carry
        if ONLY in ('', 'f'):
            lax.fori_loop(0, 2, body, 0)


@jax.jit
def pallas_interleave_layers__sliding_local_dilated__glu_gated_geglu__prompt_kernel(
    A_x, A_wqkv, A_wo, B_x, B_w_gate, B_w_up, B_w_down):
    B, S, D = A_x.shape
    DF = B_w_gate.shape[1]
    NB = S // TB
    NP = NB // 2
    NCH = DF // CW
    xT = A_x.reshape(S, D).T
    wdT = B_w_down.T
    hbm = pl.BlockSpec(memory_space=pltpu.HBM)
    outT = pl.pallas_call(
        functools.partial(_kernel, D=D, DF=DF, S=S),
        grid=(2 * NP,),
        in_specs=[hbm] * 6,
        out_specs=pl.BlockSpec((D, 2 * TB), lambda g: (0, jnp.maximum(g - NP, 0))),
        out_shape=jax.ShapeDtypeStruct((D, S), A_x.dtype),
        scratch_shapes=[
            pltpu.VMEM((NP, D, 2 * TB), bf16),
            pltpu.VMEM((D, 3 * D), bf16),
            pltpu.VMEM((D, D), bf16),
            pltpu.VMEM((5, 14 * 128, 128), f32),
            pltpu.VMEM((WQR, 27 * 128), u32),
            pltpu.VMEM((D // 2, 640), u32),
            pltpu.VMEM((D // 4, 18 * 128), u32),
            pltpu.VMEM((NCH, 3, D, CW), bf16),
            pltpu.VMEM((NCH, 45 * (TC // 2) + 15 * (D // 6) + 16, 2 * TC), u32),
            pltpu.VMEM((16, S + QPAD, 128), f32),
            pltpu.VMEM((11, TB, 128), f32),
            pltpu.VMEM((NB, D, TB), f32),
            pltpu.VMEM((2, D, TB), f32),
            pltpu.VMEM((2, D, TB), f32),
            pltpu.VMEM((45, TB // 2, TC), u32),
            pltpu.VMEM((31, TB // 2, TC), u32),
            pltpu.VMEM((18, TB // 2, TC), u32),
            pltpu.SemaphoreType.DMA((4 + NP + 3 * NCH,)),
        ] + [pltpu.VMEM((TB, 2 * TC), f32)] * 29,
        compiler_params=pltpu.CompilerParams(
            dimension_semantics=("arbitrary",),
            vmem_limit_bytes=110 * 1024 * 1024,
            disable_bounds_checks=bool(NOCHK),
            disable_semaphore_checks=bool(NOCHK),
        ),
    )(xT, A_wqkv, A_wo, B_w_gate, B_w_up, wdT)
    return outT.T.reshape(B, S, D)
```

```python
import functools
import math
import jax
import jax.numpy as jnp
from jax import lax
import jax.experimental.pallas as pl
import jax.experimental.pallas.tpu as pltpu

H = 32
DH = 18
W = 8
DIL = 2
HALO = 16
EPS = 1e-5
TB = 128
RB = 8
TC = 128
CW = 6 * TC
WQR = 320
KY = 64
ONLY = ''
LN_P = tuple(int(x) for x in '1,2'.split(','))
CFG_Q1 = tuple(int(x) for x in '300,1428,9,9,48,64,300'.split(','))
CFG_Q2 = tuple(int(x) for x in '1,2,60,560'.split(','))
QP0 = int(30); QP1 = int(3850); QTK = int(8)
SCRIPT = 'R1+50+400,G,R5+0+290,G,G,R10+0+350,G,D4,G,R5+0+290,G,G,R11+0+250,G,D4,W,n0+1500,n1+2124,l+3424+500,G,G,G,G,c+200+96,D4'.split(',')
SCRIPT_F = 'G,G,G,G,D2,G,G,D2,D2'.split(',')
DORD = tuple(int(x) for x in '1,6,0,9,10,4,11,5,14,7,2,8,3,12,13'.split(','))
LAGS = tuple(int(x) for x in '0,0,1'.split(','))
USPLIT = int(1)
W0DYN = int(0)
CFG_Q0 = tuple(int(x) for x in '300,1428,9,9,48,64,300'.split(','))
RG = tuple(int(x) for x in '2,1,48,420'.split(','))
RDL = int(700)
ZM = int(8)
JDL = int(250); LDL = int(600); GTK = int(2)
PLAG = int(4); DADV = int(1)
UFIRST = int(0); USCR = int(0)
CFG_QA = tuple(int(x) for x in '300,748,6,6,32,64,350'.split(','))
QA_T = tuple(int(x) for x in '300,1000,4,3850'.split(','))
QPAD = int(40)
LNJ = tuple(int(x) for x in '12,12,48,48'.split(','))
DTK = int(8)
XNF = int(0); XNL = int(0); NLEFT = int(3)
WORD = tuple(int(x) for x in '0,1,2,6,7,8,9,10,11,12,13,14,3,4,5'.split(','))
NOCHK = int(1)

f32 = jnp.float32
bf16 = jnp.bfloat16
u32 = jnp.uint32
NT = (((1,), (1,)), ((), ()))


def _al(i, n):
    return i if isinstance(i, int) else pl.multiple_of(i, n)


def _lt(k):
    return slice(k * 128, (k + 1) * 128)


def _pk(x):
    return pltpu.bitcast(x.astype(bf16), u32)


def _up(x):
    return pltpu.bitcast(x, bf16)


def _dot(a, b):
    return jnp.dot(a, b, preferred_element_type=f32)


def _dot_nt(a, b):
    return lax.dot_general(a, b, NT, preferred_element_type=f32)


def _tree(fn, xs):
    xs = list(xs)
    while len(xs) > 1:
        xs = [fn(xs[i], xs[i + 1]) for i in range(0, len(xs) - 1, 2)] + ([xs[-1]] if len(xs) % 2 else [])
    return xs[0]


def _ln_stats(x, nacc, pin=None):
    n = x.shape[0]
    c = x[0:1] if pin is None else pin(x[0:8])[0:1]
    s1 = [None] * nacc
    s2 = [None] * nacc
    for i in range(n // 8):
        d = x[i * 8:(i + 1) * 8] - c
        k = i % nacc
        s1[k] = d if s1[k] is None else s1[k] + d
        dd = d * d
        s2[k] = dd if s2[k] is None else s2[k] + dd
    m = jnp.sum(_tree(jnp.add, s1), axis=0, keepdims=True) * (1.0 / n)
    v = jnp.sum(_tree(jnp.add, s2), axis=0, keepdims=True) * (1.0 / n) - m * m
    v = jnp.maximum(v, 0.0)
    return c + m, lax.rsqrt(v + EPS)


_HK_A = (
    ((0, 0, 1), (0, 2, -1), (1, 0, -1)), ((0, 0, 1), (0, 1, -1), (2, 0, -1)), ((1, 1, 1), (0, 1, -1), (1, 2, -1)),
    ((1, 1, 1), (1, 0, -1), (2, 1, -1)), ((2, 2, 1), (0, 2, -1), (2, 1, -1)), ((2, 2, 1), (1, 2, -1), (2, 0, -1)),
    ((0, 1, 1),), ((0, 1, 1), (1, 0, -1)), ((1, 0, 1),),
    ((0, 2, 1),), ((0, 2, 1), (2, 0, -1)), ((2, 0, 1),),
    ((1, 2, 1),), ((2, 1, 1), (1, 2, -1)), ((2, 1, 1),),
)
_HK_C = {
    (0, 0): ((0, 1), (7, 1), (8, 1), (9, 1), (6, -1)),
    (0, 1): ((1, 1), (6, 1), (10, 1), (11, 1), (9, -1)),
    (1, 0): ((2, 1), (7, 1), (8, 1), (12, 1), (6, -1)),
    (1, 1): ((3, 1), (6, 1), (13, 1), (14, 1), (2, -1), (7, -1)),
    (2, 0): ((5, 1), (9, 1), (12, 1), (13, 1), (4, -1), (10, -1)),
    (2, 1): ((4, 1), (10, 1), (11, 1), (14, 1), (9, -1)),
}


_HK_B = (((0, 0, 1),), ((0, 1, 1),), ((1, 0, 1),), ((1, 0, 1), (1, 1, 1)), ((2, 1, 1),), ((2, 0, 1), (2, 1, 1)),
         ((0, 1, 1), (1, 1, 1)), ((0, 1, 1), (1, 0, 1), (1, 1, 1)), ((0, 0, 1), (0, 1, 1), (1, 0, 1), (1, 1, 1)),
         ((0, 0, 1), (2, 0, 1)), ((0, 0, 1), (2, 0, 1), (2, 1, 1)), ((0, 0, 1), (0, 1, 1), (2, 0, 1), (2, 1, 1)),
         ((1, 0, 1), (2, 0, 1)), ((1, 0, 1), (2, 1, -1)), ((1, 1, 1), (2, 1, 1)))


def _hk_b(b):
    s1 = b[1][0] + b[1][1]
    s2 = b[2][0] + b[2][1]
    t7 = b[0][1] + s1
    t10 = b[0][0] + s2
    return (b[0][0], b[0][1], b[1][0], s1, b[2][1], s2, b[0][1] + b[1][1], t7, b[0][0] + t7,
            b[0][0] + b[2][0], t10, b[0][1] + t10, b[1][0] + b[2][0], b[1][0] - b[2][1], b[1][1] + b[2][1])


def _ssum(terms):
    terms = sorted([t for t in terms if t[0] is not None], key=lambda z: -z[1])
    if not terms:
        return None
    acc = terms[0][0] if terms[0][1] == 1 else -terms[0][0]
    for v, sg in terms[1:]:
        acc = acc + v if sg == 1 else acc - v
    return acc


GU_ORD = tuple(int(x) for x in '8,6,7,11,3,1,10,14,9,5,0,13,12,4,2'.split(','))
GU_POST = {
    8: ((), ('p8', None), None),
    7: ((('p8', 1),), (None, 't7'), None),
    3: ((('t7', 1),), (None, 's1'), None),
    6: ((), ('p6', None), None),
    14: ((('p6', 1), ('s1', 1)), ('p14', None), (1, 1)),
    12: ((('p9', 1), ('s2', 1)), ('p12', None), (2, 0)),
    13: ((), ('p13', None), None),
    2: ((('p12', 1), ('p13', 1), ('s1', 1)), (None, None), (1, 0)),
    11: ((), ('p11', None), None),
    10: ((('p11', 1),), (None, 't10'), None),
    5: ((('t10', 1),), (None, 's2'), None),
    9: ((), ('p9', None), None),
    4: ((('p14', 1), ('s2', 1), ('p13', -1)), (None, None), (2, 1)),
    0: ((('p8', 1), ('p9', 1), ('t10', 1)), (None, None), (0, 0)),
    1: ((('p6', 1), ('p11', 1), ('t7', 1)), (None, None), (0, 1)),
}
PSLOT = {k: i for i, k in enumerate(('p8', 't7', 's1', 'p6', 'p14', 'p12', 'p13', 'p11', 't10', 's2', 'p9'))}


class _Timeline:
    def __init__(self):
        self.t = 0
        self.jobs = []
        self.due = []

    def add(self, when, fn):
        self.jobs.append((when, len(self.jobs), fn))
        self.jobs.sort(key=lambda z: z[:2])

    def add_due(self, when, job, delay):
        def run(dep):
            val = job(dep)
            if val is not None:
                self.add(self.t + delay, lambda _: self.due.append(lambda: val))
        self.add(when, run)

    def pending(self):
        return [j for j in self.jobs if getattr(j[2], '__name__', '') != '<lambda>']

    def tick(self, dur, v, n=1, seq=1):
        per = max(n // seq, 1)
        for k in range(n):
            self.t += dur // n
            r = (k % per) * (v.shape[0] // per)
            c = (k // per) * 128
            while self.jobs and self.jobs[0][0] <= self.t:
                self.jobs.pop(0)[2](v[r:r + 8, c:c + 128])


def _kernel(x_hbm, wqkv_hbm, wo_hbm, wg_hbm, wu_hbm, wd_hbm, o_ref,
            xin, wqkv_raw, wo_raw, tmp, wq, woT, wo2, raw, pw, qall, o_s, xres, xn_f, xn_g, s_scr, st_s, sq_scr,
            sems, *p_s, D, DF, S):
    g = pl.program_id(0)
    NB = S // TB
    NP = NB // 2
    NCH = DF // CW
    NPC = NCH // 2
    D3 = D // 3
    DHALF = D // 2
    nr = TB // RB
    hh = DHALF // 2
    zero8 = pl.multiple_of((g >> 20) * ZM, ZM)
    zvec = jnp.full((8, 128), (g >> 20).astype(u32), u32)

    def zero(k):
        return pl.multiple_of((g >> (8 + k)) * ZM, ZM)

    def tie(x, dep):
        return pltpu.bitcast(pltpu.bitcast(x, u32) | (pltpu.bitcast(dep, u32) & zvec), f32)

    def gate(lhs, clock):
        if not clock.due:
            return lhs
        pr = _tree(jnp.bitwise_or, [k() for k in clock.due]) & zvec
        del clock.due[:]
        return jnp.concatenate([lhs[0:8] | pr, lhs[8:]], axis=0)

    QSEC = ((0, 5), (5, 9), (9, 14))

    def cp_qkv(sec):
        out = []
        for j in range(*QSEC[sec]):
            n = min(128, 3 * D - j * 128)
            out.append(pltpu.make_async_copy(wqkv_hbm.at[:, pl.ds(j * 128, n)], wqkv_raw.at[:, pl.ds(j * 128, n)],
                                             sems.at[sec]))
        return out

    def cp_wo():
        return pltpu.make_async_copy(wo_hbm, wo_raw, sems.at[3])

    def cp_x(k):
        return pltpu.make_async_copy(x_hbm.at[:, pl.ds(_al(k * 2 * TB, 128), 2 * TB)], xin.at[k], sems.at[4 + k])

    class Unit:
        def __init__(self, c, m):
            src = (wg_hbm, wu_hbm, wd_hbm)[m]
            n = D // USPLIT
            self.cps = [pltpu.make_async_copy(src.at[pl.ds(k * n, n), pl.ds(_al(c * CW, 128), CW)],
                                              raw.at[c, m, pl.ds(k * n, n), :], sems.at[4 + NP + 3 * c + m])
                        for k in range(USPLIT)]

        def start(self):
            for cp in self.cps:
                cp.start()

        def wait(self):
            for cp in self.cps:
                cp.wait()
    cp_unit = Unit

    R_SD = 45 * (TC // 2)
    R_END = R_SD + 15 * (D3 // 2)

    def hk_a_ops(load, minus=None):
        blk = {}
        for i in range(3):
            for j in range(3):
                blk[i, j] = load(i, j).astype(f32)
                if minus is not None:
                    blk[i, j] = blk[i, j] - minus(i, j).astype(f32)
        return [_pk(_ssum([(blk[i, j], sg) for i, j, sg in terms])) for terms in _HK_A]

    def prep_pieces(c, m):
        def ld(r, cs):
            return lambda i, j: raw[c, m, pl.ds(i * D3 + r, 16), pl.ds((3 * cs + j) * TC, TC)]

        def gu_piece(q, r, cs, neg, kind, half):
            ops = hk_a_ops(ld(q * KY + r, cs), None if neg is None else ld(q * KY + r, neg))
            for k, t in enumerate(ops):
                pw.at[c][pl.ds((3 * k + kind) * (TC // 2) + (half * KY + r) // 2, 8), m * TC:(m + 1) * TC] = t

        def d_piece(r, cs):
            for k, t in enumerate(hk_a_ops(ld(r, cs))):
                pw.at[c][pl.ds(R_SD + k * (D3 // 2) + r // 2, 8), cs * TC:(cs + 1) * TC] = t
        if m == 2:
            return [functools.partial(d_piece, r, cs) for r in range(0, D3, 16) for cs in range(2)]
        spec = ((0, 0, None, 0, 0), (1, 0, 1, 0, 1), (0, 1, None, 1, 0), (2, 1, 0, 1, 1),
                (2, 0, None, 2, 0), (1, 1, None, 2, 1))
        return [functools.partial(gu_piece, q, r, cs, neg, kind, half)
                for r in range(0, KY, 16) for q, cs, neg, kind, half in spec]

    def transpose_qkv(sec):
        for j in range(*QSEC[sec]):
            wd_ = min(128, 3 * D - j * 128)
            blk = wqkv_raw[:, j * 128:j * 128 + wd_].astype(f32)
            if wd_ < 128:
                blk = jnp.concatenate([blk, jnp.zeros((D, 128 - wd_), f32)], axis=1)
            bt = jnp.concatenate([blk, blk[D - KY:]], axis=0).T
            for t in range(5):
                tmp[t, pl.ds(j * 128, 128), :] = bt[:, t * 128:(t + 1) * 128]

    def wq_slot(i, j):
        return 24 + i if i == j else [n for n, t in enumerate(_HK_A) if t == ((i, j, 1),)][0]

    def build_wq(sec):
        lo = lax.broadcasted_iota(jnp.int32, (32, 128), 1) < KY
        for d in range(DH):
            tt = [tmp[t, pl.ds(sec * D + d, 32, stride=DH), :] for t in range(5)]
            ops = tt[:4] + [jnp.where(lo, tt[3], tt[4]), jnp.where(lo, tt[4], tt[3])]
            if d < 16:
                dst = [(sec, d * 16)]
            else:
                dst = ([(1, (d + 2) * 16)], [(1, d * 16)], [(0, d * 16), (0, (d + 2) * 16)])[sec]
            for j, row in dst:
                for k, v in enumerate(ops):
                    wq[pl.ds(row, 16), _lt(wq_slot(k, j) if k < 3 else 12 + 3 * j + k)] = _pk(v)

    def wq_sums(r, dep):
        ncol = 3 if r < 256 else 2
        pin = pltpu.bitcast(dep, u32) & zvec
        blk = {(i, j): _up(wq[pl.ds(r, 8), _lt(wq_slot(i, j))] | pin).astype(f32) for i in range(3) for j in range(ncol)}
        for n, terms in enumerate(_HK_A):
            if len(terms) > 1 and not (ncol == 2 and n in (4, 5)):
                wq[pl.ds(r, 8), _lt(n)] = _pk(_ssum([(blk[i, j], sg) for i, j, sg in terms if j < ncol]))

    def build_wo():
        for t in range(5):
            wd_ = min(128, D - t * 128)
            blk = wo_raw[:, t * 128:t * 128 + wd_].astype(f32)
            if wd_ < 128:
                blk = jnp.concatenate([blk, jnp.zeros((D, 128 - wd_), f32)], axis=1)
            tmp[t, pl.ds(0, D), :] = blk
        for t in range(5):
            rows = [tmp[t, pl.ds(d, 32, stride=DH), :] for d in range(DH)]
            ft = jnp.concatenate(rows + rows[16:], axis=0).T
            n = min(128, D - t * 128)
            woT[pl.ds(t * 64, n // 2), :] = _pk(ft[:n])
        for r in range(0, D3 // 2, 8):
            ops = hk_a_ops(lambda i, j: _up(woT[pl.ds(i * (D3 // 2) + r, 8), j * TC:(j + 1) * TC]))
            for k, t in enumerate(ops):
                wo2[pl.ds(r, 8), _lt(k)] = t
        lo = lax.broadcasted_iota(jnp.int32, (16, 128), 1) < KY
        for r in range(0, hh, 8):
            a3, a4, b3, b4 = [_up(woT[pl.ds(r0 + r, 8), c0:c0 + 128]).astype(f32)
                              for r0 in (0, hh) for c0 in (384, 512)]
            wo2[pl.ds(r, 8), _lt(15)] = _pk(jnp.where(lo, a3, a3 - b3))
            wo2[pl.ds(r, 8), _lt(16)] = _pk(jnp.where(lo, b3, b4 - a4))
            wo2[pl.ds(r, 8), _lt(17)] = _pk(jnp.where(lo, a4, b3))

    def normalize(blk, mean, rstd, link):
        if not link:
            return (xres[blk] - mean) * rstd
        rs = jnp.broadcast_to(rstd, (8, TB))
        mb = jnp.broadcast_to(mean, (8, TB))
        outs = []
        for i in range(D // 8):
            if i and i % link == 0:
                rs = tie(rs, outs[-1])
            outs.append((xres[blk, pl.ds(i * 8, 8), :] - mb) * rs)
        return jnp.concatenate(outs, axis=0)

    def left_ops(src, put, plain=False, which=None, dep=None):
        def X(t, r0, n):
            return src[t, pl.ds((zero8 if plain else 0) + r0, n), :]
        k1, k2, k3 = 3 * TC, 3 * TC + KY, 3 * TC + 2 * KY
        for n in (list(range(6 if plain else 15)) + [15, 16, 17]) if which is None else which:
            if n == 15:
                v = jnp.concatenate([X(0, k1, KY), X(0, k2, KY) - X(1, k2, KY)], axis=0)
            elif n == 16:
                v = jnp.concatenate([X(1, k1, KY), X(1, k3, KY) - X(0, k3, KY)], axis=0)
            elif n == 17:
                v = jnp.concatenate([X(0, k3, KY), X(1, k2, KY)], axis=0)
            elif plain:
                v = X(n // 3, (n % 3) * TC, TC)
            else:
                v = _ssum([(X(t, i * TC, TC), sg) for (i, t), lst in _HK_C.items() for k, sg in lst if k == n])
            if dep is not None:
                v = jnp.concatenate([tie(v[0:8], dep), v[8:]], axis=0)
            put(n, pltpu.bitcast(v.astype(bf16).T, u32))

    def ln1(pr, par, src, ln, dep=None):
        blk = 2 * pr + par
        if src == 'res':
            x = xres[blk]
        else:
            x = xin[pr, :, par * TB:(par + 1) * TB].astype(f32)
            xres[blk] = x
        mean, rstd = _ln_stats(x, ln[0], None if dep is None else (lambda v: tie(v, dep)))
        if src == 'res':
            xn_g[par, pl.ds(0, 8), :] = jnp.zeros((8, TB), f32)
        xn_g[par, pl.ds(zero8, D), :] = normalize(blk, mean, rstd, ln[1])

    def add_ln(clock, t0, cfg, blk, dst, par, inp=None):
        np1, np2, step, gap, delay = cfg
        st = dict(s1=[], s2=[], left=np2)
        nv = D // 16

        def load(i):
            if inp is None:
                return xres[blk, pl.ds(zero8 + i * 16, 16), :]
            x = inp(i).astype(f32)
            xres[blk, pl.ds(i * 16, 16), :] = x
            return x

        def stats(k, dep):
            xs = []
            for i in range(k * nv // np1, (k + 1) * nv // np1):
                x = load(i)
                xs += [x[0:8], x[8:16]]
            if k == 0:
                st['c'] = jnp.broadcast_to(xs[0][0:1], (8, TB))
            c = tie(st['c'], dep)
            ds = [x - c for x in xs]
            st['s1'].append(_tree(jnp.add, ds))
            st['s2'].append(_tree(jnp.add, [d * d for d in ds]))
            return pltpu.bitcast(st['s1'][-1], u32) | pltpu.bitcast(st['s2'][-1], u32)

        def norm(k, dep):
            if k == 0:
                m = jnp.sum(_tree(jnp.add, st['s1']), axis=0, keepdims=True) * (1.0 / D)
                v = jnp.sum(_tree(jnp.add, st['s2']), axis=0, keepdims=True) * (1.0 / D) - m * m
                st['mean'] = st['c'] + m
                st['rstd'] = jnp.broadcast_to(lax.rsqrt(jnp.maximum(v, 0.0) + EPS), (8, TB))
            mean = tie(st['mean'], dep)
            off = 0 if inp is None else zero8
            for i in range(k * 2 * nv // np2, (k + 1) * 2 * nv // np2):
                dst[par, pl.ds(i * 8, 8), :] = (xres[blk, pl.ds(off + i * 8, 8), :] - mean) * st['rstd']
            st['left'] -= 1
            return pltpu.bitcast(dst[par, pl.ds(zero8, 8), :], u32)
        for k in range(np1):
            clock.add_due(t0 + k * step, functools.partial(stats, k), delay)
        for k in range(np2):
            clock.add_due(t0 + np1 * step + gap + k * step, functools.partial(norm, k), delay)
        return st

    def q_left(plain):
        def put(i, v):
            sq_scr[i] = v
        left_ops(xn_g, put, plain)

    def hk_outputs(P, T, PT, tk, emit, two_cols=False):
        p8 = P(8)
        t7 = P(7) + p8
        tk(2, t7)
        s1 = PT(3, 1, 2) + t7
        tk(2, s1)
        p6 = P(6)
        p14 = P(14)
        tk(2, p14)
        emit(1, 1, T(1, 1) + (p6 + p14 + s1), 1)
        p13 = P(13)
        if two_cols:
            emit(1, 0, PT(2, 1, 0) + (p13 + s1), 3)
        else:
            p12 = P(12)
            tk(2, p12)
            emit(1, 0, PT(2, 1, 0) + (p12 + p13 + s1), 2)
        p11 = P(11)
        t10 = P(10) + p11
        tk(2, t10)
        if not two_cols:
            s2 = PT(5, 2, 2) + t10
            tk(2, s2)
            p9 = P(9)
            emit(2, 0, T(2, 0) + (p9 + p12 + s2), 2)
            emit(2, 1, PT(4, 2, 1) + (p14 - p13 + s2), 2)
        w0 = T(0, 2)
        emit(0, 0, PT(0, 0, 0) + ((p8 + t10 + w0) if two_cols else (p8 + p9 + t10 + w0)), 3)
        emit(0, 1, PT(1, 0, 1) + (p6 + p11 + t7 + w0), 2)

    QT = (0, 1, 2, 3)
    KT = (4, 5, 6, 7, 13)
    VT = (8, 9, 10, 11, 12)
    c2e = DH ** -0.5 * math.log2(math.e)
    neg = -1e9 * math.log2(math.e)

    def q_step(pr, chunk, src, cfg, rows=False, sums=False):
        clock = _Timeline()
        if sums:
            base, nx = 0, 1
            for k in range(40):
                clock.add(200 + k * 90, functools.partial(wq_sums, 8 * k))
        elif rows:
            base, nx = pr * (2 * TB), pr + 1
            for k in range(2):
                clock.add_due(QA_T[k], functools.partial(row_chain, k, QA_T[2]), QA_T[3] - QA_T[k])
        else:
            base = pl.multiple_of(pr * (2 * TB), 2 * TB)
            nx = jnp.minimum(pr + 1, NP - 1)
        pieces = []
        if chunk is not None:
            for m in range(3):
                pieces += prep_pieces(jnp.maximum(chunk - LAGS[m], 0) if LAGS[m] else chunk, m)

        def paced(piece, dep):
            pw[0, pl.ds(R_END, 8), 0:128] = pltpu.bitcast(dep, u32)
            piece()
        for k, piece in enumerate(pieces):
            clock.add(QP0 + k * (QP1 - QP0) // len(pieces), functools.partial(paced, piece))
        if src == 'in':
            for par in range(2):
                add_ln(clock, cfg[par], cfg[2:], 2 * nx + par, xn_g, par,
                       functools.partial(lambda par_, i: xin[nx, pl.ds(i * 16, 16), par_ * TB:(par_ + 1) * TB], par))
        else:
            clock.add(cfg[2], functools.partial(ln1, nx, 0, src, cfg[:2]))
            clock.add(cfg[3], functools.partial(ln1, nx, 1, src, cfg[:2]))
        for r0, nt, tiles in ((0, 2, (0, 4, 8)), (TC, 2, (2, 6, 10)), (2 * TC, 1, (12, 13))):
            def R(k):
                return wq[pl.ds(r0, nt * 64), _lt(k)]

            def P(k):
                return _dot_nt(_up(sq_scr[k]), _up(R(k)))

            def T(j, kind):
                return _dot_nt(_up(sq_scr[15 + kind]), _up(R(15 + 3 * j + kind)))

            def PT(k, j, kind):
                return _dot_nt(_up(jnp.concatenate([sq_scr[k], sq_scr[15 + kind]], axis=1)),
                               _up(jnp.concatenate([R(k), R(15 + 3 * j + kind)], axis=1)))

            def tk(np_, v):
                clock.tick(32 * nt * np_, v, 4)

            def emit(col, half, v, np_):
                for k in range(nt):
                    qall[tiles[col] + k, pl.ds(base + (HALO + half * TB), TB), :] = v[:, k * 128:(k + 1) * 128]
                tk(np_, v)
            if src == 'res':
                hk_outputs(P, T, PT, tk, emit, two_cols=(nt == 1))
                continue
            for j in range(len(tiles)):
                both = T(j, 2)
                clock.t += 32 * nt
                for t in range(2):
                    for k in range(nt):
                        lhs = [sq_scr[3 * t + i] for i in range(3)] + [sq_scr[15 + t]]
                        lhs[0] = gate(lhs[0], clock)
                        rhs = [wq[pl.ds(r0 + k * 64, 64), _lt(n)]
                               for n in [wq_slot(i, j) for i in range(3)] + [15 + 3 * j + t]]
                        v = _dot_nt(_up(jnp.concatenate(lhs, axis=1)), _up(jnp.concatenate(rhs, axis=1))) + both[:, _lt(k)]
                        qall[tiles[j] + k, pl.ds(base + (HALO + t * TB), TB), :] = v
                        clock.tick(128, v, QTK)
        assert not clock.pending()
        q_left(src == 'in')

    def row_group(blk, par, r, nw, nv, mids=None):
        base = _al(blk * TB, TB)
        lo = lax.broadcasted_iota(jnp.int32, (RB, 128), 1) < KY
        r0 = r * RB

        def ld(t, w):
            return qall[t, pl.ds(base + (HALO + r0 - DIL * w), RB), :]
        dep = yield
        cs = tie(jnp.full((RB, 128), c2e, f32), dep)
        q = [ld(t, 0) * cs for t in QT] + [jnp.where(lo, pltpu.roll(ld(13, 0), KY, 1), 0.0) * cs]
        sc = []
        for w in range(W):
            if w and w % nw == 0:
                dep = yield
                q = [tie(q[0], dep)] + q[1:]
            acc = None
            for j, t in enumerate(KT):
                p = q[j] * ld(t, w)
                acc = p if acc is None else acc + p
            acc = acc + pltpu.roll(acc, 64, 1)
            if mids is not None:
                mids[r] = pltpu.bitcast(acc, u32)
            acc = acc + pltpu.roll(acc, 32, 1)
            if r0 - DIL * w < 0:
                pos = blk * TB + r0 + lax.broadcasted_iota(jnp.int32, (RB, 128), 0)
                acc = jnp.where(pos >= DIL * w, acc, neg)
            sc.append(acc)
        m = _tree(jnp.maximum, sc)
        e = [jnp.exp2(sc[w] - m) for w in range(W)]
        l = _tree(jnp.add, e)
        rinv = pl.reciprocal(l, approx=True)
        rinv = rinv * (2.0 - l * rinv)
        outs = []
        for j, t in enumerate(VT):
            if j and j % nv == 0:
                dep = yield _tree(jnp.bitwise_or, [pltpu.bitcast(v, u32) for v in outs])
                outs = []
                e = [tie(e[0], dep)] + e[1:]
            acc = None
            for w in range(W):
                p = e[w] * ld(t, w)
                acc = p if acc is None else acc + p
            o = acc * rinv
            o_s[par * 5 + j, pl.ds(r0, RB), :] = o
            outs.append(o)
        yield _tree(jnp.bitwise_or, [pltpu.bitcast(v, u32) for v in outs])

    def add_rows(clock, t0, blk, par, r, cfg):
        nw, nv, step, gap, d1, d2 = cfg
        gen = row_group(blk, par, r, nw, nv)
        next(gen)
        n1, n2 = -(-W // nw), -(-5 // nv)
        for k in range(n1):
            clock.add_due(t0 + k * step, gen.send, d1)
        for k in range(n2 - 1):
            clock.add_due(t0 + (n1 - 1) * step + gap + k * step, gen.send, d2)

    def row_chain(blk, lag, dep):
        mids, fins = {}, {}
        for r in range(nr):
            gen = row_group(blk, blk, r, W, 5, mids)
            next(gen)
            if r:
                dep = pltpu.bitcast(mids[r - 1] | fins[r - lag] if r >= lag else mids[r - 1], f32)
            fins[r] = gen.send(dep)
        return _tree(jnp.bitwise_or, [fins[r] for r in range(nr - lag, nr)])

    wo_seq = []
    for pos, k in enumerate(WORD):
        if pos in (0, 2):
            wo_seq += [('r', pos // 2, k_) for k_ in range(3)]
        wo_seq.append(('p', k))

    def wo_rhs(off):
        lo = lax.broadcasted_iota(jnp.int32, (TB, 128), 1) < KY

        rhs = {}
        for it in wo_seq:
            z = zero(wo_seq.index(it)) if off is None else off

            def O(t, j):
                return o_s[t * 5 + j, pl.ds(z, TB), :]
            if it[0] == 'p':
                v = _ssum([(O(t, j), sg) for j, t, sg in _HK_B[it[1]]])
            elif it[2] == 0:
                v = O(it[1], 3)
            else:
                v = jnp.where(lo, O(it[1], 2 + it[2]), O(it[1], 5 - it[2]))
            rhs[it] = v.astype(bf16)
        return rhs

    def wo_mm(blk0, rhs):
        res = {}
        for it in wo_seq:
            if it[0] == 'p':
                lhs = wo2[pl.ds(0, D3 // 2), _lt(it[1])]
            else:
                lhs = wo2[:, _lt(15 + it[2])]
            res[it] = _dot_nt(_up(lhs), rhs[it])
        for t in range(2):
            both = res['r', t, 2]
            rem = xres[blk0 + t] + jnp.concatenate([res['r', t, 0] + both, res['r', t, 1] + both], axis=0)
            y = jnp.concatenate([_ssum([(res['p', k], sg) for k, sg in _HK_C[i, t]]) for i in range(3)], axis=0)
            xres[blk0 + t] = y + rem

    def ln2(blk, par, ln, dep=None):
        mean, rstd = _ln_stats(xres[blk, pl.ds(zero8 if XNL else 0, D), :], ln[0],
                               None if dep is None else (lambda v: tie(v, dep)))
        xn_f[par, pl.ds(0, 8), :] = jnp.zeros((8, TB), f32)
        xn_f[par, pl.ds(zero8 if XNF else 0, D), :] = normalize(blk, mean, rstd, ln[1])

    def a_left(which=range(15), dep=None):
        for n in which:
            v = _ssum([(xn_f[t, pl.ds(zero(n) + i * D3, D3), :], sg)
                       for (i, t), lst in _HK_C.items() for k, sg in lst if k == n])
            if dep is not None:
                v = jnp.concatenate([tie(v[0:8], dep), v[8:2 * KY], tie(v[2 * KY:2 * KY + 8], dep), v[2 * KY + 8:]],
                                    axis=0)
            t1 = pltpu.bitcast(v[:2 * KY].astype(bf16).T, u32)
            t2 = pltpu.bitcast(jnp.concatenate([v[2 * KY:], v[2 * KY:]], axis=0).astype(bf16).T, u32)
            if dep is None:
                arrange(n, t1, t2)
            else:
                st_s[2 * n] = t1
                st_s[2 * n + 1] = t2

    def arrange(n, t1, t2):
        lo = lax.broadcasted_iota(jnp.int32, (TB // 2, 128), 1) < KY
        s_scr[3 * n] = t1
        s_scr[3 * n + 1] = jnp.where(lo, t1, t2)
        s_scr[3 * n + 2] = jnp.where(lo, t2, t1)

    def a_arrange(n, dep):
        st_s[30, pl.ds(0, 8), :] = pltpu.bitcast(dep, u32)
        arrange(n, st_s[2 * n, pl.ds(zero8, TB // 2), :], st_s[2 * n + 1, pl.ds(zero8, TB // 2), :])

    k0 = math.sqrt(2.0 / math.pi)
    k1 = k0 * 0.044715

    def ffn(j, c0, script):
        clock = _Timeline()
        b0 = (2 * j) % NB
        an = (2 * j + 2) % NB
        acc = [None] * 15
        hs = {}
        lns, staged, nrows = [], set(), 0

        pend = []

        def advance(keep):
            while len(pend) > keep:
                pend.pop(0)()

        def written(k):
            clock.due.append(lambda: pltpu.bitcast(p_s[k][pl.ds(zero8, 8), 0:128], u32))

        def gu(p):
            c, second = c0 + p // 2, p % 2
            m = 1 - second if UFIRST else second
            h = hs.setdefault(p // 2, [[None, None] for _ in range(3)])

            def mm(n, kind):
                lhs = gate(s_scr[3 * n + kind], clock)
                return _dot(_up(lhs), _up(pw[c, pl.ds((3 * n + kind) * (TC // 2), TC // 2), m * TC:(m + 1) * TC]))

            def get(name):
                return p_s[PSLOT[name]][pl.ds(zero8, TB), :]

            def post(n, v):
                adds, keep, emits = GU_POST[n]
                if keep[0] is not None:
                    p_s[PSLOT[keep[0]]][...] = v
                    written(PSLOT[keep[0]])
                w_ = v
                for name, sg in adds:
                    w_ = w_ + get(name) if sg == 1 else w_ - get(name)
                if keep[1] is not None:
                    p_s[PSLOT[keep[1]]][...] = w_
                    written(PSLOT[keep[1]])
                if emits is not None:
                    col, half = emits
                    if m == 0:
                        w_ = w_ + w_ * jnp.tanh(w_ * (k0 + k1 * (w_ * w_)))
                    if second:
                        k_ = 17 + 6 * ((p // 2) % 2) + 2 * col + half
                        p_s[k_][...] = w_ * p_s[11 + 2 * col + half][pl.ds(zero8, TB), :]
                        written(k_)
                        h[col][half] = k_
                    else:
                        p_s[11 + 2 * col + half][...] = w_
                        written(11 + 2 * col + half)
            for n in GU_ORD:
                both = mm(n, 2)
                v = jnp.concatenate([mm(n, 0) + both, mm(n, 1) + both], axis=1)
                pend.append(functools.partial(post, n, v))
                advance(PLAG)
                clock.tick(96, both, GTK)

        def down(ps):
            cs = ps[::2]
            hsl = [hs.pop(p // 2) for p in cs]
            for pos, i in enumerate(DORD):
                while any(h_[j_][t_] is None for h_ in hsl for j_, t_, _ in _HK_B[i]):
                    advance(len(pend) - 1)
                au = []
                for p in cs:
                    au += [pw[c0 + p // 2, pl.ds(R_SD + i * (D3 // 2), D3 // 2), k * TC:(k + 1) * TC] for k in range(2)]
                au[0] = gate(au[0], clock)
                r = _dot_nt(jnp.concatenate([_up(v) for v in au], axis=1),
                            jnp.concatenate([_ssum([(p_s[h_[j_][t_]][pl.ds(zero(i), TB), :], sg) for j_, t_, sg in _HK_B[i]])
                                             for h_ in hsl], axis=1).astype(bf16))
                acc[i] = r if acc[i] is None else r + acc[i]
                advance(max(len(pend) - DADV, 0))
                clock.tick(48 * len(ps), acc[i], DTK)

        pg = pd = 0
        for tok in script:
            if tok == 'G':
                gu(pg)
                pg += 1
            elif tok[0] == 'D':
                down(list(range(pd, pd + int(tok[1:]))))
                pd += int(tok[1:])
            elif tok == 'W':
                assert not clock.pending() and nrows == 2 * nr
                advance(0)
                wo_mm(an, wo_rhs(None))
                clock.t += 1152
            elif tok[0] == 'n':
                lns.append(add_ln(clock, clock.t + int(tok[3:]), LNJ + (JDL,), an + int(tok[1]), xn_f, int(tok[1])))
            elif tok[0] == 'l':
                _, t0, dt = tok.split('+')

                def left(which, dep):
                    assert len(lns) == 2 and not any(st['left'] for st in lns)
                    staged.update(which)
                    a_left(which, dep)
                    return st_s[0, pl.ds(zero8, 8), :]
                for k in range(NLEFT):
                    clock.add_due(clock.t + int(t0) + k * int(dt),
                                  functools.partial(left, range(k * 15 // NLEFT, (k + 1) * 15 // NLEFT)), LDL)
            elif tok[0] == 'c':
                _, t0, dt = tok.split('+')
                assert pg == 2 * NCH

                def place(k, dep):
                    assert k in staged
                    a_arrange(k, dep)
                for k in range(15):
                    clock.add(clock.t + int(t0) + k * int(dt), functools.partial(place, k))
            else:
                n, t0, dt = tok[1:].split('+')
                for k in range(int(n)):
                    add_rows(clock, clock.t + int(t0) + k * int(dt), an + nrows // nr, nrows // nr, nrows % nr,
                             RG + (RDL, JDL))
                    nrows += 1
        assert pg == pd and not clock.pending()
        for t in range(2):
            y = jnp.concatenate([_ssum([(acc[k], sg) for k, sg in _HK_C[i, t]]) for i in range(3)], axis=0)
            x2 = xres[b0 + t] + 0.5 * y
            xres[b0 + t] = x2
            o_ref[:, t * TB:(t + 1) * TB] = x2.astype(o_ref.dtype)

    assert NCH == NP - 2

    late = [(c, m) for c in range(NCH) for m in range(3) if c >= NCH - LAGS[m]]

    def prologue():
        cp_x(0).start()
        for sec in range(3):
            for cp in cp_qkv(sec):
                cp.start()
        qall[:, pl.ds(0, HALO), :] = jnp.zeros((16, HALO, 128), f32)
        cp_x(0).wait()
        ln1(0, 0, 'in', (4, 0))
        ln1(0, 1, 'in', (4, 0))
        q_left(True)
        for sec in range(3):
            for cp in cp_qkv(sec):
                cp.wait()
            if sec == 0:
                cp_x(1).start()
                cp_x(2).start()
                cp_wo().start()
                for c in range(NCH):
                    if 3 + c < NP:
                        cp_x(3 + c).start()
                    for m in range(3):
                        if c == 0 or c > LAGS[m]:
                            cp_unit(max(c - LAGS[m], 0), m).start()
                for c, m in late:
                    cp_unit(c, m).start()
            transpose_qkv(sec)
            build_wq(sec)

    def first_attention():
        cp_x(2).wait()
        q_step(1, None, 'in', CFG_QA, rows=True)
        cp_wo().wait()
        build_wo()
        wo_mm(0, wo_rhs(None if W0DYN else 0))
        ln2(0, 0, (4, 0))
        ln2(1, 1, (4, 0))
        a_left()

    def startup_step(c, carry):
        @pl.when(c + 3 < NP)
        def _():
            cp_x(c + 3).wait()
        for m in range(3):
            if LAGS[m]:
                @pl.when(jnp.logical_or(c == 0, c > LAGS[m]))
                def _():
                    cp_unit(jnp.maximum(c - LAGS[m], 0), m).wait()
            else:
                cp_unit(c, m).wait()
        q_step(c + 2, c, 'in', CFG_Q1)
        return carry

    @pl.when(g == 0)
    def _():
        if ONLY in ('', 'pro'):
            prologue()
            cp_x(1).wait()
            q_step(0, None, 'in', CFG_Q0, sums=True)
        if ONLY in ('', 'a'):
            first_attention()
        if ONLY in ('', 'q'):
            lax.fori_loop(0, NCH, startup_step, 0)
        if not ONLY:
            for c, m in late:
                cp_unit(c, m).wait()
                for piece in prep_pieces(c, m):
                    piece()

    @pl.when(jnp.logical_and(g >= NP - 1, g < 2 * NP - 1))
    def _():
        @pl.when(g == NP - 1)
        def _():
            if ONLY in ('', 'pro'):
                ln1(0, 0, 'res', (4, 0))
                ln1(0, 1, 'res', (4, 0))
                q_left(False)
        if ONLY in ('', 'q'):
            q_step(g - (NP - 1), None, 'res', CFG_Q2)

    if ONLY in ('q', 'a', 'pro'):
        @pl.when(g == 2 * NP - 1)
        def _():
            o_ref[0:16, 0:128] = (qall[g % 16, pl.ds(zero8, 16), :] + xres[g % 16, pl.ds(zero8, 16), :]
                                  + pltpu.bitcast(pw[g % 4, pl.ds(zero8, 16), 0:128] | s_scr[g % 8, pl.ds(zero8, 16), :]
                                                  | wo2[pl.ds(zero8, 16), 0:128] | wq[pl.ds(zero8, 16), 0:128] | sq_scr[g % 8, pl.ds(zero8, 16), :], f32)).astype(bf16)

    @pl.when(g < 2 * NP - 1)
    def _():
        if ONLY in ('', 'p'):
            ffn(g, 0, SCRIPT)

    @pl.when(g == 2 * NP - 1)
    def _():
        def body(hf, carry):
            ffn(2 * NP - 1, hf * NPC, SCRIPT_F)
            return carry
        if ONLY in ('', 'f'):
            lax.fori_loop(0, 2, body, 0)


@jax.jit
def pallas_interleave_layers__sliding_local_dilated__glu_gated_geglu__prompt_kernel(
    A_x, A_wqkv, A_wo, B_x, B_w_gate, B_w_up, B_w_down):
    B, S, D = A_x.shape
    DF = B_w_gate.shape[1]
    NB = S // TB
    NP = NB // 2
    NCH = DF // CW
    xT = A_x.reshape(S, D).T
    wdT = B_w_down.T
    hbm = pl.BlockSpec(memory_space=pltpu.HBM)
    outT = pl.pallas_call(
        functools.partial(_kernel, D=D, DF=DF, S=S),
        grid=(2 * NP,),
        in_specs=[hbm] * 6,
        out_specs=pl.BlockSpec((D, 2 * TB), lambda g: (0, jnp.maximum(g - NP, 0))),
        out_shape=jax.ShapeDtypeStruct((D, S), A_x.dtype),
        scratch_shapes=[
            pltpu.VMEM((NP, D, 2 * TB), bf16),
            pltpu.VMEM((D, 3 * D), bf16),
            pltpu.VMEM((D, D), bf16),
            pltpu.VMEM((5, 14 * 128, 128), f32),
            pltpu.VMEM((WQR, 27 * 128), u32),
            pltpu.VMEM((D // 2, 640), u32),
            pltpu.VMEM((D // 4, 18 * 128), u32),
            pltpu.VMEM((NCH, 3, D, CW), bf16),
            pltpu.VMEM((NCH, 45 * (TC // 2) + 15 * (D // 6) + 16, 2 * TC), u32),
            pltpu.VMEM((16, S + QPAD, 128), f32),
            pltpu.VMEM((11, TB, 128), f32),
            pltpu.VMEM((NB, D, TB), f32),
            pltpu.VMEM((2, D, TB), f32),
            pltpu.VMEM((2, D, TB), f32),
            pltpu.VMEM((45, TB // 2, TC), u32),
            pltpu.VMEM((31, TB // 2, TC), u32),
            pltpu.VMEM((18, TB // 2, TC), u32),
            pltpu.SemaphoreType.DMA((4 + NP + 3 * NCH,)),
        ] + [pltpu.VMEM((TB, 2 * TC), f32)] * 29,
        compiler_params=pltpu.CompilerParams(
            dimension_semantics=("arbitrary",),
            vmem_limit_bytes=110 * 1024 * 1024,
            disable_bounds_checks=bool(NOCHK),
            disable_semaphore_checks=bool(NOCHK),
        ),
    )(xT, A_wqkv, A_wo, B_w_gate, B_w_up, wdT)
    return outT.T.reshape(B, S, D)
```

```python
import functools
import math
import jax
import jax.numpy as jnp
from jax import lax
import jax.experimental.pallas as pl
import jax.experimental.pallas.tpu as pltpu

H = 32
DH = 18
W = 8
DIL = 2
HALO = 16
EPS = 1e-5
TB = 128
RB = 8
TC = 128
CW = 6 * TC
WQR = 320
KY = 64
ONLY = ''
LN_P = tuple(int(x) for x in '1,2'.split(','))
CFG_Q1 = tuple(int(x) for x in '300,1428,9,9,48,64,300'.split(','))
CFG_Q2 = tuple(int(x) for x in '1,2,60,560'.split(','))
QP0 = int(30); QP1 = int(3850); QTK = int(8)
SCRIPT = 'R1+50+400,G,R5+0+290,G,G,R10+0+350,G,D4,G,R5+0+290,G,G,R11+0+250,G,D4,W,n0+1500,n1+2124,l+3424+500,G,G,G,G,c+200+96,D4'.split(',')
SCRIPT_F = 'G,G,G,G,D2,G,G,D2,D2'.split(',')
DORD = tuple(int(x) for x in '1,6,0,9,10,4,11,5,14,7,2,8,3,12,13'.split(','))
LAGS = tuple(int(x) for x in '0,0,1'.split(','))
USPLIT = int(1)
W0DYN = int(0)
CFG_Q0 = tuple(int(x) for x in '300,1428,9,9,48,64,300'.split(','))
RG = tuple(int(x) for x in '2,1,48,420'.split(','))
RDL = int(700)
ZM = int(8)
JDL = int(250); LDL = int(600); GTK = int(2)
PLAG = int(4); DADV = int(1)
UFIRST = int(0); USCR = int(0)
CFG_QA = tuple(int(x) for x in '300,748,6,6,32,64,350'.split(','))
QA_T = tuple(int(x) for x in '300,1000,4,3850'.split(','))
QPAD = int(40)
LNJ = tuple(int(x) for x in '12,12,48,48'.split(','))
DTK = int(8)
XNF = int(0); XNL = int(0); NLEFT = int(3)
WORD = tuple(int(x) for x in '0,1,2,6,7,8,9,10,11,12,13,14,3,4,5'.split(','))
NOCHK = int(1)

f32 = jnp.float32
bf16 = jnp.bfloat16
u32 = jnp.uint32
NT = (((1,), (1,)), ((), ()))


def _al(i, n):
    return i if isinstance(i, int) else pl.multiple_of(i, n)


def _lt(k):
    return slice(k * 128, (k + 1) * 128)


def _pk(x):
    return pltpu.bitcast(x.astype(bf16), u32)


def _up(x):
    return pltpu.bitcast(x, bf16)


def _dot(a, b):
    return jnp.dot(a, b, preferred_element_type=f32)


def _dot_nt(a, b):
    return lax.dot_general(a, b, NT, preferred_element_type=f32)


def _tree(fn, xs):
    xs = list(xs)
    while len(xs) > 1:
        xs = [fn(xs[i], xs[i + 1]) for i in range(0, len(xs) - 1, 2)] + ([xs[-1]] if len(xs) % 2 else [])
    return xs[0]


def _ln_stats(x, nacc, pin=None):
    n = x.shape[0]
    c = x[0:1] if pin is None else pin(x[0:8])[0:1]
    s1 = [None] * nacc
    s2 = [None] * nacc
    for i in range(n // 8):
        d = x[i * 8:(i + 1) * 8] - c
        k = i % nacc
        s1[k] = d if s1[k] is None else s1[k] + d
        dd = d * d
        s2[k] = dd if s2[k] is None else s2[k] + dd
    m = jnp.sum(_tree(jnp.add, s1), axis=0, keepdims=True) * (1.0 / n)
    v = jnp.sum(_tree(jnp.add, s2), axis=0, keepdims=True) * (1.0 / n) - m * m
    v = jnp.maximum(v, 0.0)
    return c + m, lax.rsqrt(v + EPS)


_HK_A = (
    ((0, 0, 1), (0, 2, -1), (1, 0, -1)), ((0, 0, 1), (0, 1, -1), (2, 0, -1)), ((1, 1, 1), (0, 1, -1), (1, 2, -1)),
    ((1, 1, 1), (1, 0, -1), (2, 1, -1)), ((2, 2, 1), (0, 2, -1), (2, 1, -1)), ((2, 2, 1), (1, 2, -1), (2, 0, -1)),
    ((0, 1, 1),), ((0, 1, 1), (1, 0, -1)), ((1, 0, 1),),
    ((0, 2, 1),), ((0, 2, 1), (2, 0, -1)), ((2, 0, 1),),
    ((1, 2, 1),), ((2, 1, 1), (1, 2, -1)), ((2, 1, 1),),
)
_HK_C = {
    (0, 0): ((0, 1), (7, 1), (8, 1), (9, 1), (6, -1)),
    (0, 1): ((1, 1), (6, 1), (10, 1), (11, 1), (9, -1)),
    (1, 0): ((2, 1), (7, 1), (8, 1), (12, 1), (6, -1)),
    (1, 1): ((3, 1), (6, 1), (13, 1), (14, 1), (2, -1), (7, -1)),
    (2, 0): ((5, 1), (9, 1), (12, 1), (13, 1), (4, -1), (10, -1)),
    (2, 1): ((4, 1), (10, 1), (11, 1), (14, 1), (9, -1)),
}


_HK_B = (((0, 0, 1),), ((0, 1, 1),), ((1, 0, 1),), ((1, 0, 1), (1, 1, 1)), ((2, 1, 1),), ((2, 0, 1), (2, 1, 1)),
         ((0, 1, 1), (1, 1, 1)), ((0, 1, 1), (1, 0, 1), (1, 1, 1)), ((0, 0, 1), (0, 1, 1), (1, 0, 1), (1, 1, 1)),
         ((0, 0, 1), (2, 0, 1)), ((0, 0, 1), (2, 0, 1), (2, 1, 1)), ((0, 0, 1), (0, 1, 1), (2, 0, 1), (2, 1, 1)),
         ((1, 0, 1), (2, 0, 1)), ((1, 0, 1), (2, 1, -1)), ((1, 1, 1), (2, 1, 1)))


def _hk_b(b):
    s1 = b[1][0] + b[1][1]
    s2 = b[2][0] + b[2][1]
    t7 = b[0][1] + s1
    t10 = b[0][0] + s2
    return (b[0][0], b[0][1], b[1][0], s1, b[2][1], s2, b[0][1] + b[1][1], t7, b[0][0] + t7,
            b[0][0] + b[2][0], t10, b[0][1] + t10, b[1][0] + b[2][0], b[1][0] - b[2][1], b[1][1] + b[2][1])


def _ssum(terms):
    terms = sorted([t for t in terms if t[0] is not None], key=lambda z: -z[1])
    if not terms:
        return None
    acc = terms[0][0] if terms[0][1] == 1 else -terms[0][0]
    for v, sg in terms[1:]:
        acc = acc + v if sg == 1 else acc - v
    return acc


GU_ORD = tuple(int(x) for x in '8,6,7,11,3,1,10,14,9,5,0,13,12,4,2'.split(','))
GU_POST = {
    8: ((), ('p8', None), None),
    7: ((('p8', 1),), (None, 't7'), None),
    3: ((('t7', 1),), (None, 's1'), None),
    6: ((), ('p6', None), None),
    14: ((('p6', 1), ('s1', 1)), ('p14', None), (1, 1)),
    12: ((('p9', 1), ('s2', 1)), ('p12', None), (2, 0)),
    13: ((), ('p13', None), None),
    2: ((('p12', 1), ('p13', 1), ('s1', 1)), (None, None), (1, 0)),
    11: ((), ('p11', None), None),
    10: ((('p11', 1),), (None, 't10'), None),
    5: ((('t10', 1),), (None, 's2'), None),
    9: ((), ('p9', None), None),
    4: ((('p14', 1), ('s2', 1), ('p13', -1)), (None, None), (2, 1)),
    0: ((('p8', 1), ('p9', 1), ('t10', 1)), (None, None), (0, 0)),
    1: ((('p6', 1), ('p11', 1), ('t7', 1)), (None, None), (0, 1)),
}
PSLOT = {k: i for i, k in enumerate(('p8', 't7', 's1', 'p6', 'p14', 'p12', 'p13', 'p11', 't10', 's2', 'p9'))}


class _Timeline:
    def __init__(self):
        self.t = 0
        self.jobs = []
        self.due = []

    def add(self, when, fn):
        self.jobs.append((when, len(self.jobs), fn))
        self.jobs.sort(key=lambda z: z[:2])

    def add_due(self, when, job, delay):
        def run(dep):
            val = job(dep)
            if val is not None:
                self.add(self.t + delay, lambda _: self.due.append(lambda: val))
        self.add(when, run)

    def pending(self):
        return [j for j in self.jobs if getattr(j[2], '__name__', '') != '<lambda>']

    def tick(self, dur, v, n=1, seq=1):
        per = max(n // seq, 1)
        for k in range(n):
            self.t += dur // n
            r = (k % per) * (v.shape[0] // per)
            c = (k // per) * 128
            while self.jobs and self.jobs[0][0] <= self.t:
                self.jobs.pop(0)[2](v[r:r + 8, c:c + 128])


def _step(g, last, x_hbm, wqkv_hbm, wo_hbm, wg_hbm, wu_hbm, wd_hbm, o_hbm,
            xin, wqkv_raw, wo_raw, tmp, wq, woT, wo2, raw, pw, qall, o_s, xres, xn_f, xn_g, s_scr, st_s, sq_scr,
            sems, *p_s, D, DF, S):
    NB = S // TB
    NP = NB // 2
    NCH = DF // CW
    NPC = NCH // 2
    D3 = D // 3
    DHALF = D // 2
    nr = TB // RB
    hh = DHALF // 2
    zero8 = pl.multiple_of((g >> 20) * ZM, ZM)
    zvec = jnp.full((8, 128), (g >> 20).astype(u32), u32)

    def zero(k):
        return pl.multiple_of((g >> (8 + k)) * ZM, ZM)

    def tie(x, dep):
        return pltpu.bitcast(pltpu.bitcast(x, u32) | (pltpu.bitcast(dep, u32) & zvec), f32)

    def gate(lhs, clock):
        if not clock.due:
            return lhs
        pr = _tree(jnp.bitwise_or, [k() for k in clock.due]) & zvec
        del clock.due[:]
        return jnp.concatenate([lhs[0:8] | pr, lhs[8:]], axis=0)

    QSEC = ((0, 5), (5, 9), (9, 14))

    def cp_qkv(sec):
        out = []
        for j in range(*QSEC[sec]):
            n = min(128, 3 * D - j * 128)
            out.append(pltpu.make_async_copy(wqkv_hbm.at[:, pl.ds(j * 128, n)], wqkv_raw.at[:, pl.ds(j * 128, n)],
                                             sems.at[sec]))
        return out

    def cp_wo():
        return pltpu.make_async_copy(wo_hbm, wo_raw, sems.at[3])

    def cp_x(k):
        return pltpu.make_async_copy(x_hbm.at[:, pl.ds(_al(k * 2 * TB, 128), 2 * TB)], xin.at[k], sems.at[4 + k])

    class Unit:
        def __init__(self, c, m):
            src = (wg_hbm, wu_hbm, wd_hbm)[m]
            n = D // USPLIT
            self.cps = [pltpu.make_async_copy(src.at[pl.ds(k * n, n), pl.ds(_al(c * CW, 128), CW)],
                                              raw.at[c, m, pl.ds(k * n, n), :], sems.at[4 + NP + 3 * c + m])
                        for k in range(USPLIT)]

        def start(self):
            for cp in self.cps:
                cp.start()

        def wait(self):
            for cp in self.cps:
                cp.wait()
    cp_unit = Unit

    R_SD = 45 * (TC // 2)
    R_END = R_SD + 15 * (D3 // 2)

    def hk_a_ops(load, minus=None):
        blk = {}
        for i in range(3):
            for j in range(3):
                blk[i, j] = load(i, j).astype(f32)
                if minus is not None:
                    blk[i, j] = blk[i, j] - minus(i, j).astype(f32)
        return [_pk(_ssum([(blk[i, j], sg) for i, j, sg in terms])) for terms in _HK_A]

    def prep_pieces(c, m):
        def ld(r, cs):
            return lambda i, j: raw[c, m, pl.ds(i * D3 + r, 16), pl.ds((3 * cs + j) * TC, TC)]

        def gu_piece(q, r, cs, neg, kind, half):
            ops = hk_a_ops(ld(q * KY + r, cs), None if neg is None else ld(q * KY + r, neg))
            for k, t in enumerate(ops):
                pw.at[c][pl.ds((3 * k + kind) * (TC // 2) + (half * KY + r) // 2, 8), m * TC:(m + 1) * TC] = t

        def d_piece(r, cs):
            for k, t in enumerate(hk_a_ops(ld(r, cs))):
                pw.at[c][pl.ds(R_SD + k * (D3 // 2) + r // 2, 8), cs * TC:(cs + 1) * TC] = t
        if m == 2:
            return [functools.partial(d_piece, r, cs) for r in range(0, D3, 16) for cs in range(2)]
        spec = ((0, 0, None, 0, 0), (1, 0, 1, 0, 1), (0, 1, None, 1, 0), (2, 1, 0, 1, 1),
                (2, 0, None, 2, 0), (1, 1, None, 2, 1))
        return [functools.partial(gu_piece, q, r, cs, neg, kind, half)
                for r in range(0, KY, 16) for q, cs, neg, kind, half in spec]

    def transpose_qkv(sec):
        for j in range(*QSEC[sec]):
            wd_ = min(128, 3 * D - j * 128)
            blk = wqkv_raw[:, j * 128:j * 128 + wd_].astype(f32)
            if wd_ < 128:
                blk = jnp.concatenate([blk, jnp.zeros((D, 128 - wd_), f32)], axis=1)
            bt = jnp.concatenate([blk, blk[D - KY:]], axis=0).T
            for t in range(5):
                tmp[t, pl.ds(j * 128, 128), :] = bt[:, t * 128:(t + 1) * 128]

    def wq_slot(i, j):
        return 24 + i if i == j else [n for n, t in enumerate(_HK_A) if t == ((i, j, 1),)][0]

    def build_wq(sec):
        lo = lax.broadcasted_iota(jnp.int32, (32, 128), 1) < KY
        for d in range(DH):
            tt = [tmp[t, pl.ds(sec * D + d, 32, stride=DH), :] for t in range(5)]
            ops = tt[:4] + [jnp.where(lo, tt[3], tt[4]), jnp.where(lo, tt[4], tt[3])]
            if d < 16:
                dst = [(sec, d * 16)]
            else:
                dst = ([(1, (d + 2) * 16)], [(1, d * 16)], [(0, d * 16), (0, (d + 2) * 16)])[sec]
            for j, row in dst:
                for k, v in enumerate(ops):
                    wq[pl.ds(row, 16), _lt(wq_slot(k, j) if k < 3 else 12 + 3 * j + k)] = _pk(v)

    def wq_sums(r, dep):
        ncol = 3 if r < 256 else 2
        pin = pltpu.bitcast(dep, u32) & zvec
        blk = {(i, j): _up(wq[pl.ds(r, 8), _lt(wq_slot(i, j))] | pin).astype(f32) for i in range(3) for j in range(ncol)}
        for n, terms in enumerate(_HK_A):
            if len(terms) > 1 and not (ncol == 2 and n in (4, 5)):
                wq[pl.ds(r, 8), _lt(n)] = _pk(_ssum([(blk[i, j], sg) for i, j, sg in terms if j < ncol]))

    def build_wo():
        for t in range(5):
            wd_ = min(128, D - t * 128)
            blk = wo_raw[:, t * 128:t * 128 + wd_].astype(f32)
            if wd_ < 128:
                blk = jnp.concatenate([blk, jnp.zeros((D, 128 - wd_), f32)], axis=1)
            tmp[t, pl.ds(0, D), :] = blk
        for t in range(5):
            rows = [tmp[t, pl.ds(d, 32, stride=DH), :] for d in range(DH)]
            ft = jnp.concatenate(rows + rows[16:], axis=0).T
            n = min(128, D - t * 128)
            woT[pl.ds(t * 64, n // 2), :] = _pk(ft[:n])
        for r in range(0, D3 // 2, 8):
            ops = hk_a_ops(lambda i, j: _up(woT[pl.ds(i * (D3 // 2) + r, 8), j * TC:(j + 1) * TC]))
            for k, t in enumerate(ops):
                wo2[pl.ds(r, 8), _lt(k)] = t
        lo = lax.broadcasted_iota(jnp.int32, (16, 128), 1) < KY
        for r in range(0, hh, 8):
            a3, a4, b3, b4 = [_up(woT[pl.ds(r0 + r, 8), c0:c0 + 128]).astype(f32)
                              for r0 in (0, hh) for c0 in (384, 512)]
            wo2[pl.ds(r, 8), _lt(15)] = _pk(jnp.where(lo, a3, a3 - b3))
            wo2[pl.ds(r, 8), _lt(16)] = _pk(jnp.where(lo, b3, b4 - a4))
            wo2[pl.ds(r, 8), _lt(17)] = _pk(jnp.where(lo, a4, b3))

    def normalize(blk, mean, rstd, link):
        if not link:
            return (xres[blk] - mean) * rstd
        rs = jnp.broadcast_to(rstd, (8, TB))
        mb = jnp.broadcast_to(mean, (8, TB))
        outs = []
        for i in range(D // 8):
            if i and i % link == 0:
                rs = tie(rs, outs[-1])
            outs.append((xres[blk, pl.ds(i * 8, 8), :] - mb) * rs)
        return jnp.concatenate(outs, axis=0)

    def left_ops(src, put, plain=False, which=None, dep=None):
        def X(t, r0, n):
            return src[t, pl.ds((zero8 if plain else 0) + r0, n), :]
        k1, k2, k3 = 3 * TC, 3 * TC + KY, 3 * TC + 2 * KY
        for n in (list(range(6 if plain else 15)) + [15, 16, 17]) if which is None else which:
            if n == 15:
                v = jnp.concatenate([X(0, k1, KY), X(0, k2, KY) - X(1, k2, KY)], axis=0)
            elif n == 16:
                v = jnp.concatenate([X(1, k1, KY), X(1, k3, KY) - X(0, k3, KY)], axis=0)
            elif n == 17:
                v = jnp.concatenate([X(0, k3, KY), X(1, k2, KY)], axis=0)
            elif plain:
                v = X(n // 3, (n % 3) * TC, TC)
            else:
                v = _ssum([(X(t, i * TC, TC), sg) for (i, t), lst in _HK_C.items() for k, sg in lst if k == n])
            if dep is not None:
                v = jnp.concatenate([tie(v[0:8], dep), v[8:]], axis=0)
            put(n, pltpu.bitcast(v.astype(bf16).T, u32))

    def ln1(pr, par, src, ln, dep=None):
        blk = 2 * pr + par
        if src == 'res':
            x = xres[blk]
        else:
            x = xin[pr, :, par * TB:(par + 1) * TB].astype(f32)
            xres[blk] = x
        mean, rstd = _ln_stats(x, ln[0], None if dep is None else (lambda v: tie(v, dep)))
        if src == 'res':
            xn_g[par, pl.ds(0, 8), :] = jnp.zeros((8, TB), f32)
        xn_g[par, pl.ds(zero8, D), :] = normalize(blk, mean, rstd, ln[1])

    def add_ln(clock, t0, cfg, blk, dst, par, inp=None):
        np1, np2, step, gap, delay = cfg
        st = dict(s1=[], s2=[], left=np2)
        nv = D // 16

        def load(i):
            if inp is None:
                return xres[blk, pl.ds(zero8 + i * 16, 16), :]
            x = inp(i).astype(f32)
            xres[blk, pl.ds(i * 16, 16), :] = x
            return x

        def stats(k, dep):
            xs = []
            for i in range(k * nv // np1, (k + 1) * nv // np1):
                x = load(i)
                xs += [x[0:8], x[8:16]]
            if k == 0:
                st['c'] = jnp.broadcast_to(xs[0][0:1], (8, TB))
            c = tie(st['c'], dep)
            ds = [x - c for x in xs]
            st['s1'].append(_tree(jnp.add, ds))
            st['s2'].append(_tree(jnp.add, [d * d for d in ds]))
            return pltpu.bitcast(st['s1'][-1], u32) | pltpu.bitcast(st['s2'][-1], u32)

        def norm(k, dep):
            if k == 0:
                m = jnp.sum(_tree(jnp.add, st['s1']), axis=0, keepdims=True) * (1.0 / D)
                v = jnp.sum(_tree(jnp.add, st['s2']), axis=0, keepdims=True) * (1.0 / D) - m * m
                st['mean'] = st['c'] + m
                st['rstd'] = jnp.broadcast_to(lax.rsqrt(jnp.maximum(v, 0.0) + EPS), (8, TB))
            mean = tie(st['mean'], dep)
            off = 0 if inp is None else zero8
            for i in range(k * 2 * nv // np2, (k + 1) * 2 * nv // np2):
                dst[par, pl.ds(i * 8, 8), :] = (xres[blk, pl.ds(off + i * 8, 8), :] - mean) * st['rstd']
            st['left'] -= 1
            return pltpu.bitcast(dst[par, pl.ds(zero8, 8), :], u32)
        for k in range(np1):
            clock.add_due(t0 + k * step, functools.partial(stats, k), delay)
        for k in range(np2):
            clock.add_due(t0 + np1 * step + gap + k * step, functools.partial(norm, k), delay)
        return st

    def q_left(plain):
        def put(i, v):
            sq_scr[i] = v
        left_ops(xn_g, put, plain)

    def hk_outputs(P, T, PT, tk, emit, two_cols=False):
        p8 = P(8)
        t7 = P(7) + p8
        tk(2, t7)
        s1 = PT(3, 1, 2) + t7
        tk(2, s1)
        p6 = P(6)
        p14 = P(14)
        tk(2, p14)
        emit(1, 1, T(1, 1) + (p6 + p14 + s1), 1)
        p13 = P(13)
        if two_cols:
            emit(1, 0, PT(2, 1, 0) + (p13 + s1), 3)
        else:
            p12 = P(12)
            tk(2, p12)
            emit(1, 0, PT(2, 1, 0) + (p12 + p13 + s1), 2)
        p11 = P(11)
        t10 = P(10) + p11
        tk(2, t10)
        if not two_cols:
            s2 = PT(5, 2, 2) + t10
            tk(2, s2)
            p9 = P(9)
            emit(2, 0, T(2, 0) + (p9 + p12 + s2), 2)
            emit(2, 1, PT(4, 2, 1) + (p14 - p13 + s2), 2)
        w0 = T(0, 2)
        emit(0, 0, PT(0, 0, 0) + ((p8 + t10 + w0) if two_cols else (p8 + p9 + t10 + w0)), 3)
        emit(0, 1, PT(1, 0, 1) + (p6 + p11 + t7 + w0), 2)

    QT = (0, 1, 2, 3)
    KT = (4, 5, 6, 7, 13)
    VT = (8, 9, 10, 11, 12)
    c2e = DH ** -0.5 * math.log2(math.e)
    neg = -1e9 * math.log2(math.e)

    def q_step(pr, chunk, src, cfg, rows=False, sums=False):
        clock = _Timeline()
        if sums:
            base, nx = 0, 1
            for k in range(40):
                clock.add(200 + k * 90, functools.partial(wq_sums, 8 * k))
        elif rows:
            base, nx = pr * (2 * TB), pr + 1
            for k in range(2):
                clock.add_due(QA_T[k], functools.partial(row_chain, k, QA_T[2]), QA_T[3] - QA_T[k])
        else:
            base = pl.multiple_of(pr * (2 * TB), 2 * TB)
            nx = jnp.minimum(pr + 1, NP - 1)
        pieces = []
        if chunk is not None:
            for m in range(3):
                pieces += prep_pieces(jnp.maximum(chunk - LAGS[m], 0) if LAGS[m] else chunk, m)

        def paced(piece, dep):
            pw[0, pl.ds(R_END, 8), 0:128] = pltpu.bitcast(dep, u32)
            piece()
        for k, piece in enumerate(pieces):
            clock.add(QP0 + k * (QP1 - QP0) // len(pieces), functools.partial(paced, piece))
        if src == 'in':
            for par in range(2):
                add_ln(clock, cfg[par], cfg[2:], 2 * nx + par, xn_g, par,
                       functools.partial(lambda par_, i: xin[nx, pl.ds(i * 16, 16), par_ * TB:(par_ + 1) * TB], par))
        else:
            clock.add(cfg[2], functools.partial(ln1, nx, 0, src, cfg[:2]))
            clock.add(cfg[3], functools.partial(ln1, nx, 1, src, cfg[:2]))
        for r0, nt, tiles in ((0, 2, (0, 4, 8)), (TC, 2, (2, 6, 10)), (2 * TC, 1, (12, 13))):
            def R(k):
                return wq[pl.ds(r0, nt * 64), _lt(k)]

            def P(k):
                return _dot_nt(_up(sq_scr[k]), _up(R(k)))

            def T(j, kind):
                return _dot_nt(_up(sq_scr[15 + kind]), _up(R(15 + 3 * j + kind)))

            def PT(k, j, kind):
                return _dot_nt(_up(jnp.concatenate([sq_scr[k], sq_scr[15 + kind]], axis=1)),
                               _up(jnp.concatenate([R(k), R(15 + 3 * j + kind)], axis=1)))

            def tk(np_, v):
                clock.tick(32 * nt * np_, v, 4)

            def emit(col, half, v, np_):
                for k in range(nt):
                    qall[tiles[col] + k, pl.ds(base + (HALO + half * TB), TB), :] = v[:, k * 128:(k + 1) * 128]
                tk(np_, v)
            if src == 'res':
                hk_outputs(P, T, PT, tk, emit, two_cols=(nt == 1))
                continue
            for j in range(len(tiles)):
                both = T(j, 2)
                clock.t += 32 * nt
                for t in range(2):
                    for k in range(nt):
                        lhs = [sq_scr[3 * t + i] for i in range(3)] + [sq_scr[15 + t]]
                        lhs[0] = gate(lhs[0], clock)
                        rhs = [wq[pl.ds(r0 + k * 64, 64), _lt(n)]
                               for n in [wq_slot(i, j) for i in range(3)] + [15 + 3 * j + t]]
                        v = _dot_nt(_up(jnp.concatenate(lhs, axis=1)), _up(jnp.concatenate(rhs, axis=1))) + both[:, _lt(k)]
                        qall[tiles[j] + k, pl.ds(base + (HALO + t * TB), TB), :] = v
                        clock.tick(128, v, QTK)
        assert not clock.pending()
        q_left(src == 'in')

    def row_group(blk, par, r, nw, nv, mids=None):
        base = _al(blk * TB, TB)
        lo = lax.broadcasted_iota(jnp.int32, (RB, 128), 1) < KY
        r0 = r * RB

        def ld(t, w):
            return qall[t, pl.ds(base + (HALO + r0 - DIL * w), RB), :]
        dep = yield
        cs = tie(jnp.full((RB, 128), c2e, f32), dep)
        q = [ld(t, 0) * cs for t in QT] + [jnp.where(lo, pltpu.roll(ld(13, 0), KY, 1), 0.0) * cs]
        sc = []
        for w in range(W):
            if w and w % nw == 0:
                dep = yield
                q = [tie(q[0], dep)] + q[1:]
            acc = None
            for j, t in enumerate(KT):
                p = q[j] * ld(t, w)
                acc = p if acc is None else acc + p
            acc = acc + pltpu.roll(acc, 64, 1)
            if mids is not None:
                mids[r] = pltpu.bitcast(acc, u32)
            acc = acc + pltpu.roll(acc, 32, 1)
            if r0 - DIL * w < 0:
                pos = blk * TB + r0 + lax.broadcasted_iota(jnp.int32, (RB, 128), 0)
                acc = jnp.where(pos >= DIL * w, acc, neg)
            sc.append(acc)
        m = _tree(jnp.maximum, sc)
        e = [jnp.exp2(sc[w] - m) for w in range(W)]
        l = _tree(jnp.add, e)
        rinv = pl.reciprocal(l, approx=True)
        rinv = rinv * (2.0 - l * rinv)
        outs = []
        for j, t in enumerate(VT):
            if j and j % nv == 0:
                dep = yield _tree(jnp.bitwise_or, [pltpu.bitcast(v, u32) for v in outs])
                outs = []
                e = [tie(e[0], dep)] + e[1:]
            acc = None
            for w in range(W):
                p = e[w] * ld(t, w)
                acc = p if acc is None else acc + p
            o = acc * rinv
            o_s[par * 5 + j, pl.ds(r0, RB), :] = o
            outs.append(o)
        yield _tree(jnp.bitwise_or, [pltpu.bitcast(v, u32) for v in outs])

    def add_rows(clock, t0, blk, par, r, cfg):
        nw, nv, step, gap, d1, d2 = cfg
        gen = row_group(blk, par, r, nw, nv)
        next(gen)
        n1, n2 = -(-W // nw), -(-5 // nv)
        for k in range(n1):
            clock.add_due(t0 + k * step, gen.send, d1)
        for k in range(n2 - 1):
            clock.add_due(t0 + (n1 - 1) * step + gap + k * step, gen.send, d2)

    def row_chain(blk, lag, dep):
        mids, fins = {}, {}
        for r in range(nr):
            gen = row_group(blk, blk, r, W, 5, mids)
            next(gen)
            if r:
                dep = pltpu.bitcast(mids[r - 1] | fins[r - lag] if r >= lag else mids[r - 1], f32)
            fins[r] = gen.send(dep)
        return _tree(jnp.bitwise_or, [fins[r] for r in range(nr - lag, nr)])

    wo_seq = []
    for pos, k in enumerate(WORD):
        if pos in (0, 2):
            wo_seq += [('r', pos // 2, k_) for k_ in range(3)]
        wo_seq.append(('p', k))

    def wo_rhs(off):
        lo = lax.broadcasted_iota(jnp.int32, (TB, 128), 1) < KY

        rhs = {}
        for it in wo_seq:
            z = zero(wo_seq.index(it)) if off is None else off

            def O(t, j):
                return o_s[t * 5 + j, pl.ds(z, TB), :]
            if it[0] == 'p':
                v = _ssum([(O(t, j), sg) for j, t, sg in _HK_B[it[1]]])
            elif it[2] == 0:
                v = O(it[1], 3)
            else:
                v = jnp.where(lo, O(it[1], 2 + it[2]), O(it[1], 5 - it[2]))
            rhs[it] = v.astype(bf16)
        return rhs

    def wo_mm(blk0, rhs):
        res = {}
        for it in wo_seq:
            if it[0] == 'p':
                lhs = wo2[pl.ds(0, D3 // 2), _lt(it[1])]
            else:
                lhs = wo2[:, _lt(15 + it[2])]
            res[it] = _dot_nt(_up(lhs), rhs[it])
        for t in range(2):
            both = res['r', t, 2]
            rem = xres[blk0 + t] + jnp.concatenate([res['r', t, 0] + both, res['r', t, 1] + both], axis=0)
            y = jnp.concatenate([_ssum([(res['p', k], sg) for k, sg in _HK_C[i, t]]) for i in range(3)], axis=0)
            xres[blk0 + t] = y + rem

    def ln2(blk, par, ln, dep=None):
        mean, rstd = _ln_stats(xres[blk, pl.ds(zero8 if XNL else 0, D), :], ln[0],
                               None if dep is None else (lambda v: tie(v, dep)))
        xn_f[par, pl.ds(0, 8), :] = jnp.zeros((8, TB), f32)
        xn_f[par, pl.ds(zero8 if XNF else 0, D), :] = normalize(blk, mean, rstd, ln[1])

    def a_left(which=range(15), dep=None):
        for n in which:
            v = _ssum([(xn_f[t, pl.ds(zero(n) + i * D3, D3), :], sg)
                       for (i, t), lst in _HK_C.items() for k, sg in lst if k == n])
            if dep is not None:
                v = jnp.concatenate([tie(v[0:8], dep), v[8:2 * KY], tie(v[2 * KY:2 * KY + 8], dep), v[2 * KY + 8:]],
                                    axis=0)
            t1 = pltpu.bitcast(v[:2 * KY].astype(bf16).T, u32)
            t2 = pltpu.bitcast(jnp.concatenate([v[2 * KY:], v[2 * KY:]], axis=0).astype(bf16).T, u32)
            if dep is None:
                arrange(n, t1, t2)
            else:
                st_s[2 * n] = t1
                st_s[2 * n + 1] = t2

    def arrange(n, t1, t2):
        lo = lax.broadcasted_iota(jnp.int32, (TB // 2, 128), 1) < KY
        s_scr[3 * n] = t1
        s_scr[3 * n + 1] = jnp.where(lo, t1, t2)
        s_scr[3 * n + 2] = jnp.where(lo, t2, t1)

    def a_arrange(n, dep):
        st_s[30, pl.ds(0, 8), :] = pltpu.bitcast(dep, u32)
        arrange(n, st_s[2 * n, pl.ds(zero8, TB // 2), :], st_s[2 * n + 1, pl.ds(zero8, TB // 2), :])

    k0 = math.sqrt(2.0 / math.pi)
    k1 = k0 * 0.044715

    def ffn(j, c0, script):
        clock = _Timeline()
        b0 = (2 * j) % NB
        an = (2 * j + 2) % NB
        acc = [None] * 15
        hs = {}
        lns, staged, nrows = [], set(), 0

        pend = []

        def advance(keep):
            while len(pend) > keep:
                pend.pop(0)()

        def written(k):
            clock.due.append(lambda: pltpu.bitcast(p_s[k][pl.ds(zero8, 8), 0:128], u32))

        def gu(p):
            c, second = c0 + p // 2, p % 2
            m = 1 - second if UFIRST else second
            h = hs.setdefault(p // 2, [[None, None] for _ in range(3)])

            def mm(n, kind):
                lhs = gate(s_scr[3 * n + kind], clock)
                return _dot(_up(lhs), _up(pw[c, pl.ds((3 * n + kind) * (TC // 2), TC // 2), m * TC:(m + 1) * TC]))

            def get(name):
                return p_s[PSLOT[name]][pl.ds(zero8, TB), :]

            def post(n, v):
                adds, keep, emits = GU_POST[n]
                if keep[0] is not None:
                    p_s[PSLOT[keep[0]]][...] = v
                    written(PSLOT[keep[0]])
                w_ = v
                for name, sg in adds:
                    w_ = w_ + get(name) if sg == 1 else w_ - get(name)
                if keep[1] is not None:
                    p_s[PSLOT[keep[1]]][...] = w_
                    written(PSLOT[keep[1]])
                if emits is not None:
                    col, half = emits
                    if m == 0:
                        w_ = w_ + w_ * jnp.tanh(w_ * (k0 + k1 * (w_ * w_)))
                    if second:
                        k_ = 17 + 6 * ((p // 2) % 2) + 2 * col + half
                        p_s[k_][...] = w_ * p_s[11 + 2 * col + half][pl.ds(zero8, TB), :]
                        written(k_)
                        h[col][half] = k_
                    else:
                        p_s[11 + 2 * col + half][...] = w_
                        written(11 + 2 * col + half)
            for n in GU_ORD:
                both = mm(n, 2)
                v = jnp.concatenate([mm(n, 0) + both, mm(n, 1) + both], axis=1)
                pend.append(functools.partial(post, n, v))
                advance(PLAG)
                clock.tick(96, both, GTK)

        def down(ps):
            cs = ps[::2]
            hsl = [hs.pop(p // 2) for p in cs]
            for pos, i in enumerate(DORD):
                while any(h_[j_][t_] is None for h_ in hsl for j_, t_, _ in _HK_B[i]):
                    advance(len(pend) - 1)
                au = []
                for p in cs:
                    au += [pw[c0 + p // 2, pl.ds(R_SD + i * (D3 // 2), D3 // 2), k * TC:(k + 1) * TC] for k in range(2)]
                au[0] = gate(au[0], clock)
                r = _dot_nt(jnp.concatenate([_up(v) for v in au], axis=1),
                            jnp.concatenate([_ssum([(p_s[h_[j_][t_]][pl.ds(zero(i), TB), :], sg) for j_, t_, sg in _HK_B[i]])
                                             for h_ in hsl], axis=1).astype(bf16))
                acc[i] = r if acc[i] is None else r + acc[i]
                advance(max(len(pend) - DADV, 0))
                clock.tick(48 * len(ps), acc[i], DTK)

        pg = pd = 0
        for tok in script:
            if tok == 'G':
                gu(pg)
                pg += 1
            elif tok[0] == 'D':
                down(list(range(pd, pd + int(tok[1:]))))
                pd += int(tok[1:])
            elif tok == 'W':
                assert not clock.pending() and nrows == 2 * nr
                advance(0)
                wo_mm(an, wo_rhs(None))
                clock.t += 1152
            elif tok[0] == 'n':
                lns.append(add_ln(clock, clock.t + int(tok[3:]), LNJ + (JDL,), an + int(tok[1]), xn_f, int(tok[1])))
            elif tok[0] == 'l':
                _, t0, dt = tok.split('+')

                def left(which, dep):
                    assert len(lns) == 2 and not any(st['left'] for st in lns)
                    staged.update(which)
                    a_left(which, dep)
                    return st_s[0, pl.ds(zero8, 8), :]
                for k in range(NLEFT):
                    clock.add_due(clock.t + int(t0) + k * int(dt),
                                  functools.partial(left, range(k * 15 // NLEFT, (k + 1) * 15 // NLEFT)), LDL)
            elif tok[0] == 'c':
                _, t0, dt = tok.split('+')
                assert pg == 2 * NCH

                def place(k, dep):
                    assert k in staged
                    a_arrange(k, dep)
                for k in range(15):
                    clock.add(clock.t + int(t0) + k * int(dt), functools.partial(place, k))
            else:
                n, t0, dt = tok[1:].split('+')
                for k in range(int(n)):
                    add_rows(clock, clock.t + int(t0) + k * int(dt), an + nrows // nr, nrows // nr, nrows % nr,
                             RG + (RDL, JDL))
                    nrows += 1
        assert pg == pd and not clock.pending()
        for t in range(2):
            y = jnp.concatenate([_ssum([(acc[k], sg) for k, sg in _HK_C[i, t]]) for i in range(3)], axis=0)
            x2 = xres[b0 + t] + 0.5 * y
            xres[b0 + t] = x2
            xin[j % NP, :, t * TB:(t + 1) * TB] = x2.astype(bf16)

    if last:
        if ONLY in ('', 'f'):
            ffn(2 * NP - 1, g * NPC, SCRIPT_F)
        return
    assert NCH == NP - 2

    late = [(c, m) for c in range(NCH) for m in range(3) if c >= NCH - LAGS[m]]

    def prologue():
        cp_x(0).start()
        for sec in range(3):
            for cp in cp_qkv(sec):
                cp.start()
        qall[:, pl.ds(0, HALO), :] = jnp.zeros((16, HALO, 128), f32)
        cp_x(0).wait()
        ln1(0, 0, 'in', (4, 0))
        ln1(0, 1, 'in', (4, 0))
        q_left(True)
        for sec in range(3):
            for cp in cp_qkv(sec):
                cp.wait()
            if sec == 0:
                cp_x(1).start()
                cp_x(2).start()
                cp_wo().start()
                for c in range(NCH):
                    if 3 + c < NP:
                        cp_x(3 + c).start()
                    for m in range(3):
                        if c == 0 or c > LAGS[m]:
                            cp_unit(max(c - LAGS[m], 0), m).start()
                for c, m in late:
                    cp_unit(c, m).start()
            transpose_qkv(sec)
            build_wq(sec)

    def first_attention():
        cp_x(2).wait()
        q_step(1, None, 'in', CFG_QA, rows=True)
        cp_wo().wait()
        build_wo()
        wo_mm(0, wo_rhs(None if W0DYN else 0))
        ln2(0, 0, (4, 0))
        ln2(1, 1, (4, 0))
        a_left()

    def startup_step(c, carry):
        @pl.when(c + 3 < NP)
        def _():
            cp_x(c + 3).wait()
        for m in range(3):
            if LAGS[m]:
                @pl.when(jnp.logical_or(c == 0, c > LAGS[m]))
                def _():
                    cp_unit(jnp.maximum(c - LAGS[m], 0), m).wait()
            else:
                cp_unit(c, m).wait()
        q_step(c + 2, c, 'in', CFG_Q1)
        return carry

    @pl.when(g == 0)
    def _():
        if ONLY in ('', 'pro'):
            prologue()
            cp_x(1).wait()
            q_step(0, None, 'in', CFG_Q0, sums=True)
        if ONLY in ('', 'a'):
            first_attention()
        if ONLY in ('', 'q'):
            lax.fori_loop(0, NCH, startup_step, 0)
        if not ONLY:
            for c, m in late:
                cp_unit(c, m).wait()
                for piece in prep_pieces(c, m):
                    piece()

    @pl.when(g >= NP - 1)
    def _():
        @pl.when(g == NP - 1)
        def _():
            if ONLY in ('', 'pro'):
                ln1(0, 0, 'res', (4, 0))
                ln1(0, 1, 'res', (4, 0))
                q_left(False)
        if ONLY in ('', 'q'):
            q_step(g - (NP - 1), None, 'res', CFG_Q2)

    if ONLY in ('q', 'a', 'pro'):
        @pl.when(g == 2 * NP - 2)
        def _():
            xin[0, 0:16, 0:128] = (qall[g % 16, pl.ds(zero8, 16), :] + xres[g % 16, pl.ds(zero8, 16), :]
                                  + pltpu.bitcast(pw[g % 4, pl.ds(zero8, 16), 0:128] | s_scr[g % 8, pl.ds(zero8, 16), :]
                                                  | wo2[pl.ds(zero8, 16), 0:128] | wq[pl.ds(zero8, 16), 0:128] | sq_scr[g % 8, pl.ds(zero8, 16), :], f32)).astype(bf16)

    if ONLY in ('', 'p'):
        ffn(g, 0, SCRIPT)

    @pl.when(g >= NP)
    def _():
        _cp_out(g - NP, o_hbm, xin, sems).start()


def _cp_out(k, o_hbm, xin, sems):
    return pltpu.make_async_copy(xin.at[k], o_hbm.at[:, pl.ds(_al(k * 2 * TB, 128), 2 * TB)], sems.at[4 + k])


def _kernel(*refs, D, DF, S):
    def body(last, g, carry):
        _step(g, last, *refs, D=D, DF=DF, S=S)
        return carry
    NP = S // (2 * TB)
    lax.fori_loop(0, 2 * NP - 1, functools.partial(body, False), 0)
    lax.fori_loop(0, 2, functools.partial(body, True), 0)
    o_hbm, xin, sems = refs[6], refs[7], refs[24]
    _cp_out(NP - 1, o_hbm, xin, sems).start()
    for k in range(NP):
        _cp_out(k, o_hbm, xin, sems).wait()


@jax.jit
def pallas_interleave_layers__sliding_local_dilated__glu_gated_geglu__prompt_kernel(
    A_x, A_wqkv, A_wo, B_x, B_w_gate, B_w_up, B_w_down):
    B, S, D = A_x.shape
    DF = B_w_gate.shape[1]
    NB = S // TB
    NP = NB // 2
    NCH = DF // CW
    xT = A_x.reshape(S, D).T
    wdT = B_w_down.T
    hbm = pl.BlockSpec(memory_space=pltpu.HBM)
    outT = pl.pallas_call(
        functools.partial(_kernel, D=D, DF=DF, S=S),
        in_specs=[hbm] * 6,
        out_specs=hbm,
        out_shape=jax.ShapeDtypeStruct((D, S), A_x.dtype),
        scratch_shapes=[
            pltpu.VMEM((NP, D, 2 * TB), bf16),
            pltpu.VMEM((D, 3 * D), bf16),
            pltpu.VMEM((D, D), bf16),
            pltpu.VMEM((5, 14 * 128, 128), f32),
            pltpu.VMEM((WQR, 27 * 128), u32),
            pltpu.VMEM((D // 2, 640), u32),
            pltpu.VMEM((D // 4, 18 * 128), u32),
            pltpu.VMEM((NCH, 3, D, CW), bf16),
            pltpu.VMEM((NCH, 45 * (TC // 2) + 15 * (D // 6) + 16, 2 * TC), u32),
            pltpu.VMEM((16, S + QPAD, 128), f32),
            pltpu.VMEM((11, TB, 128), f32),
            pltpu.VMEM((NB, D, TB), f32),
            pltpu.VMEM((2, D, TB), f32),
            pltpu.VMEM((2, D, TB), f32),
            pltpu.VMEM((45, TB // 2, TC), u32),
            pltpu.VMEM((31, TB // 2, TC), u32),
            pltpu.VMEM((18, TB // 2, TC), u32),
            pltpu.SemaphoreType.DMA((4 + NP + 3 * NCH,)),
        ] + [pltpu.VMEM((TB, 2 * TC), f32)] * 29,
        compiler_params=pltpu.CompilerParams(
            vmem_limit_bytes=110 * 1024 * 1024,
            disable_bounds_checks=bool(NOCHK),
            disable_semaphore_checks=bool(NOCHK),
        ),
    )(xT, A_wqkv, A_wo, B_w_gate, B_w_up, wdT)
    return outT.T.reshape(B, S, D)
```

```python
import functools
import math
import jax
import jax.numpy as jnp
from jax import lax
import jax.experimental.pallas as pl
import jax.experimental.pallas.tpu as pltpu

H = 32
DH = 18
W = 8
DIL = 2
HALO = 16
EPS = 1e-5
TB = 128
RB = 8
TC = 128
CW = 6 * TC
WQR = 320
KY = 64
ONLY = ''
LN_P = tuple(int(x) for x in '1,2'.split(','))
CFG_Q1 = tuple(int(x) for x in '40,1456,9,9,64,64,300'.split(','))
DORD_F = tuple(int(x) for x in '1,6,0,9,10,4,11,5,14,7,2,8,3,12,13'.split(','))
QSPL = [((0, 2),), ((1, 1),), ()][int(0)]
QSPL0 = [((0, 2), (1, 2)), ()][int(0)]
TLN = int(3)
NQL = int(9)
QP0 = int(100); QP1 = int(3850); QTK = int(8)
SCRIPT = 'm0+50,m1+2900,k+8700+100,G,R6+50+240,G,G,R10+50+350,G,D4,G,R6+50+240,G,G,R10+50+280,G,D4,W,n0+1600,n1+2152,l+4300+180,G,G,G,G,c+400+96,D4'.split(',')
SCRIPT_F = 'G,G,G,G,D2,G,G,D2,D2'.split(',')
DORD = tuple(int(x) for x in '1,6,0,9,10,11,4,14,5,7,8,12,13,2,3'.split(','))
LAGS = tuple(int(x) for x in '0,0,2'.split(','))
USPLIT = int(1)
W0DYN = int(0)
CFG_Q0 = tuple(int(x) for x in '40,1816,18,18,48,48,350'.split(','))
RG = tuple(int(x) for x in '1,1,48,460'.split(','))
RDL = int(650)
ZM = int(8)
JDL = int(250); LDL = int(500); GTK = int(4)
PLAG = int(5); DADV = int(2)
UFIRST = int(0); USCR = int(0)
CFG_QA = tuple(int(x) for x in '300,748,6,6,32,64,350'.split(','))
QA_T = tuple(int(x) for x in '300,1000,4,3850'.split(','))
QPAD = int(40)
LNJ = tuple(int(x) for x in '12,9,48,48'.split(','))
DTK = int(4)
XNF = int(0); XNL = int(0); NLEFT = int(5)
WORD = tuple(int(x) for x in '0,1,2,6,7,8,9,10,11,12,13,14,3,4,5'.split(','))
NOCHK = int(1)

f32 = jnp.float32
bf16 = jnp.bfloat16
u32 = jnp.uint32
NT = (((1,), (1,)), ((), ()))


def _al(i, n):
    return i if isinstance(i, int) else pl.multiple_of(i, n)


def _lt(k):
    return slice(k * 128, (k + 1) * 128)


def _pk(x):
    return pltpu.bitcast(x.astype(bf16), u32)


def _up(x):
    return pltpu.bitcast(x, bf16)


def _dot(a, b):
    return jnp.dot(a, b, preferred_element_type=f32)


def _dot_nt(a, b):
    return lax.dot_general(a, b, NT, preferred_element_type=f32)


def _tree(fn, xs):
    xs = list(xs)
    while len(xs) > 1:
        xs = [fn(xs[i], xs[i + 1]) for i in range(0, len(xs) - 1, 2)] + ([xs[-1]] if len(xs) % 2 else [])
    return xs[0]


def _ln_stats(x, nacc, pin=None):
    n = x.shape[0]
    c = x[0:1] if pin is None else pin(x[0:8])[0:1]
    s1 = [None] * nacc
    s2 = [None] * nacc
    for i in range(n // 8):
        d = x[i * 8:(i + 1) * 8] - c
        k = i % nacc
        s1[k] = d if s1[k] is None else s1[k] + d
        dd = d * d
        s2[k] = dd if s2[k] is None else s2[k] + dd
    m = jnp.sum(_tree(jnp.add, s1), axis=0, keepdims=True) * (1.0 / n)
    v = jnp.sum(_tree(jnp.add, s2), axis=0, keepdims=True) * (1.0 / n) - m * m
    v = jnp.maximum(v, 0.0)
    return c + m, lax.rsqrt(v + EPS)


_HK_A = (
    ((0, 0, 1), (0, 2, -1), (1, 0, -1)), ((0, 0, 1), (0, 1, -1), (2, 0, -1)), ((1, 1, 1), (0, 1, -1), (1, 2, -1)),
    ((1, 1, 1), (1, 0, -1), (2, 1, -1)), ((2, 2, 1), (0, 2, -1), (2, 1, -1)), ((2, 2, 1), (1, 2, -1), (2, 0, -1)),
    ((0, 1, 1),), ((0, 1, 1), (1, 0, -1)), ((1, 0, 1),),
    ((0, 2, 1),), ((0, 2, 1), (2, 0, -1)), ((2, 0, 1),),
    ((1, 2, 1),), ((2, 1, 1), (1, 2, -1)), ((2, 1, 1),),
)
_HK_C = {
    (0, 0): ((0, 1), (7, 1), (8, 1), (9, 1), (6, -1)),
    (0, 1): ((1, 1), (6, 1), (10, 1), (11, 1), (9, -1)),
    (1, 0): ((2, 1), (7, 1), (8, 1), (12, 1), (6, -1)),
    (1, 1): ((3, 1), (6, 1), (13, 1), (14, 1), (2, -1), (7, -1)),
    (2, 0): ((5, 1), (9, 1), (12, 1), (13, 1), (4, -1), (10, -1)),
    (2, 1): ((4, 1), (10, 1), (11, 1), (14, 1), (9, -1)),
}


_HK_B = (((0, 0, 1),), ((0, 1, 1),), ((1, 0, 1),), ((1, 0, 1), (1, 1, 1)), ((2, 1, 1),), ((2, 0, 1), (2, 1, 1)),
         ((0, 1, 1), (1, 1, 1)), ((0, 1, 1), (1, 0, 1), (1, 1, 1)), ((0, 0, 1), (0, 1, 1), (1, 0, 1), (1, 1, 1)),
         ((0, 0, 1), (2, 0, 1)), ((0, 0, 1), (2, 0, 1), (2, 1, 1)), ((0, 0, 1), (0, 1, 1), (2, 0, 1), (2, 1, 1)),
         ((1, 0, 1), (2, 0, 1)), ((1, 0, 1), (2, 1, -1)), ((1, 1, 1), (2, 1, 1)))


def _hk_b(b):
    s1 = b[1][0] + b[1][1]
    s2 = b[2][0] + b[2][1]
    t7 = b[0][1] + s1
    t10 = b[0][0] + s2
    return (b[0][0], b[0][1], b[1][0], s1, b[2][1], s2, b[0][1] + b[1][1], t7, b[0][0] + t7,
            b[0][0] + b[2][0], t10, b[0][1] + t10, b[1][0] + b[2][0], b[1][0] - b[2][1], b[1][1] + b[2][1])


def _ssum(terms):
    terms = sorted([t for t in terms if t[0] is not None], key=lambda z: -z[1])
    if not terms:
        return None
    acc = terms[0][0] if terms[0][1] == 1 else -terms[0][0]
    for v, sg in terms[1:]:
        acc = acc + v if sg == 1 else acc - v
    return acc


GU_ORD = tuple(int(x) for x in '8,6,7,11,3,1,10,14,9,5,0,13,12,4,2'.split(','))
GU_POST = {
    8: ((), ('p8', None), None),
    7: ((('p8', 1),), (None, 't7'), None),
    3: ((('t7', 1),), (None, 's1'), None),
    6: ((), ('p6', None), None),
    14: ((('p6', 1), ('s1', 1)), ('p14', None), (1, 1)),
    12: ((('p9', 1), ('s2', 1)), ('p12', None), (2, 0)),
    13: ((), ('p13', None), None),
    2: ((('p12', 1), ('p13', 1), ('s1', 1)), (None, None), (1, 0)),
    11: ((), ('p11', None), None),
    10: ((('p11', 1),), (None, 't10'), None),
    5: ((('t10', 1),), (None, 's2'), None),
    9: ((), ('p9', None), None),
    4: ((('p14', 1), ('s2', 1), ('p13', -1)), (None, None), (2, 1)),
    0: ((('p8', 1), ('p9', 1), ('t10', 1)), (None, None), (0, 0)),
    1: ((('p6', 1), ('p11', 1), ('t7', 1)), (None, None), (0, 1)),
}
PSLOT = {k: i for i, k in enumerate(('p8', 't7', 's1', 'p6', 'p14', 'p12', 'p13', 'p11', 't10', 's2', 'p9'))}


class _Timeline:
    def __init__(self):
        self.t = 0
        self.jobs = []
        self.due = []

    def add(self, when, fn):
        self.jobs.append((when, len(self.jobs), fn))
        self.jobs.sort(key=lambda z: z[:2])

    def add_due(self, when, job, delay):
        def run(dep):
            val = job(dep)
            if val is not None:
                self.add(self.t + delay, lambda _: self.due.append(lambda: val))
        self.add(when, run)

    def pending(self):
        return [j for j in self.jobs if getattr(j[2], '__name__', '') != '<lambda>']

    def tick(self, dur, v, n=1, seq=1):
        per = max(n // seq, 1)
        for k in range(n):
            self.t += dur // n
            r = (k % per) * (v.shape[0] // per)
            c = (k // per) * 128
            while self.jobs and self.jobs[0][0] <= self.t:
                self.jobs.pop(0)[2](v[r:r + 8, c:c + 128])


def _step(g, last, x_hbm, wqkv_hbm, wo_hbm, wg_hbm, wu_hbm, wd_hbm, o_hbm,
            xin, wqkv_raw, wo_raw, tmp, wq, woT, wo2, raw, pw, qall, o_s, xres, xn_f, xn_g, s_scr, st_s, sq_scr,
            sems, *p_s, D, DF, S):
    NB = S // TB
    NP = NB // 2
    NCH = DF // CW
    NPC = NCH // 2
    D3 = D // 3
    DHALF = D // 2
    nr = TB // RB
    hh = DHALF // 2
    zero8 = pl.multiple_of((g >> 20) * ZM, ZM)
    zvec = jnp.full((8, 128), (g >> 20).astype(u32), u32)

    def zero(k):
        return pl.multiple_of((g >> (8 + k)) * ZM, ZM)

    def tie(x, dep):
        return pltpu.bitcast(pltpu.bitcast(x, u32) | (pltpu.bitcast(dep, u32) & zvec), f32)

    def gate(lhs, clock):
        if not clock.due:
            return lhs
        pr = _tree(jnp.bitwise_or, [k() for k in clock.due]) & zvec
        del clock.due[:]
        return jnp.concatenate([lhs[0:8] | pr, lhs[8:]], axis=0)

    QSEC = ((0, 5), (5, 9), (9, 14))

    def cp_qkv(sec):
        out = []
        for j in range(*QSEC[sec]):
            n = min(128, 3 * D - j * 128)
            out.append(pltpu.make_async_copy(wqkv_hbm.at[:, pl.ds(j * 128, n)], wqkv_raw.at[:, pl.ds(j * 128, n)],
                                             sems.at[sec]))
        return out

    def cp_wo():
        return pltpu.make_async_copy(wo_hbm, wo_raw, sems.at[3])

    def cp_x(k):
        return pltpu.make_async_copy(x_hbm.at[:, pl.ds(_al(k * 2 * TB, 128), 2 * TB)], xin.at[k], sems.at[4 + k])

    class Unit:
        def __init__(self, c, m):
            src = (wg_hbm, wu_hbm, wd_hbm)[m]
            n = D // USPLIT
            self.cps = [pltpu.make_async_copy(src.at[pl.ds(k * n, n), pl.ds(_al(c * CW, 128), CW)],
                                              raw.at[c, m, pl.ds(k * n, n), :], sems.at[4 + NP + 3 * c + m])
                        for k in range(USPLIT)]

        def start(self):
            for cp in self.cps:
                cp.start()

        def wait(self):
            for cp in self.cps:
                cp.wait()
    cp_unit = Unit

    R_SD = 45 * (TC // 2)
    R_END = R_SD + 15 * (D3 // 2)

    def hk_a_ops(load, minus=None):
        blk = {}
        for i in range(3):
            for j in range(3):
                blk[i, j] = load(i, j).astype(f32)
                if minus is not None:
                    blk[i, j] = blk[i, j] - minus(i, j).astype(f32)
        return [_pk(_ssum([(blk[i, j], sg) for i, j, sg in terms])) for terms in _HK_A]

    def prep_pieces(c, m):
        def ld(r, cs):
            return lambda i, j: raw[c, m, pl.ds(i * D3 + r, 16), pl.ds((3 * cs + j) * TC, TC)]

        def gu_piece(q, r, cs, neg, kind, half):
            ops = hk_a_ops(ld(q * KY + r, cs), None if neg is None else ld(q * KY + r, neg))
            for k, t in enumerate(ops):
                pw.at[c][pl.ds((3 * k + kind) * (TC // 2) + (half * KY + r) // 2, 8), m * TC:(m + 1) * TC] = t

        def d_piece(r, cs):
            for k, t in enumerate(hk_a_ops(ld(r, cs))):
                pw.at[c][pl.ds(R_SD + k * (D3 // 2) + r // 2, 8), cs * TC:(cs + 1) * TC] = t
        if m == 2:
            return [functools.partial(d_piece, r, cs) for r in range(0, D3, 16) for cs in range(2)]
        spec = ((0, 0, None, 0, 0), (1, 0, 1, 0, 1), (0, 1, None, 1, 0), (2, 1, 0, 1, 1),
                (2, 0, None, 2, 0), (1, 1, None, 2, 1))
        return [functools.partial(gu_piece, q, r, cs, neg, kind, half)
                for r in range(0, KY, 16) for q, cs, neg, kind, half in spec]

    def transpose_qkv(sec):
        for j in range(*QSEC[sec]):
            wd_ = min(128, 3 * D - j * 128)
            blk = wqkv_raw[:, j * 128:j * 128 + wd_].astype(f32)
            if wd_ < 128:
                blk = jnp.concatenate([blk, jnp.zeros((D, 128 - wd_), f32)], axis=1)
            bt = jnp.concatenate([blk, blk[D - KY:]], axis=0).T
            for t in range(5):
                tmp[t, pl.ds(j * 128, 128), :] = bt[:, t * 128:(t + 1) * 128]

    def wq_slot(i, j):
        return 24 + i if i == j else [n for n, t in enumerate(_HK_A) if t == ((i, j, 1),)][0]

    def build_wq(sec):
        lo = lax.broadcasted_iota(jnp.int32, (32, 128), 1) < KY
        for d in range(DH):
            tt = [tmp[t, pl.ds(sec * D + d, 32, stride=DH), :] for t in range(5)]
            ops = tt[:4] + [jnp.where(lo, tt[3], tt[4]), jnp.where(lo, tt[4], tt[3])]
            if d < 16:
                dst = [(sec, d * 16)]
            else:
                dst = ([(1, (d + 2) * 16)], [(1, d * 16)], [(0, d * 16), (0, (d + 2) * 16)])[sec]
            for j, row in dst:
                for k, v in enumerate(ops):
                    wq[pl.ds(row, 16), _lt(wq_slot(k, j) if k < 3 else 12 + 3 * j + k)] = _pk(v)

    def wq_sums(r, dep):
        ncol = 3 if r < 256 else 2
        pin = pltpu.bitcast(dep, u32) & zvec
        blk = {(i, j): _up(wq[pl.ds(r, 8), _lt(wq_slot(i, j))] | pin).astype(f32) for i in range(3) for j in range(ncol)}
        for n, terms in enumerate(_HK_A):
            if len(terms) > 1 and not (ncol == 2 and n in (4, 5)):
                wq[pl.ds(r, 8), _lt(n)] = _pk(_ssum([(blk[i, j], sg) for i, j, sg in terms if j < ncol]))

    def build_wo():
        for t in range(5):
            wd_ = min(128, D - t * 128)
            blk = wo_raw[:, t * 128:t * 128 + wd_].astype(f32)
            if wd_ < 128:
                blk = jnp.concatenate([blk, jnp.zeros((D, 128 - wd_), f32)], axis=1)
            tmp[t, pl.ds(0, D), :] = blk
        for t in range(5):
            rows = [tmp[t, pl.ds(d, 32, stride=DH), :] for d in range(DH)]
            ft = jnp.concatenate(rows + rows[16:], axis=0).T
            n = min(128, D - t * 128)
            woT[pl.ds(t * 64, n // 2), :] = _pk(ft[:n])
        for r in range(0, D3 // 2, 8):
            ops = hk_a_ops(lambda i, j: _up(woT[pl.ds(i * (D3 // 2) + r, 8), j * TC:(j + 1) * TC]))
            for k, t in enumerate(ops):
                wo2[pl.ds(r, 8), _lt(k)] = t
        lo = lax.broadcasted_iota(jnp.int32, (16, 128), 1) < KY
        for r in range(0, hh, 8):
            a3, a4, b3, b4 = [_up(woT[pl.ds(r0 + r, 8), c0:c0 + 128]).astype(f32)
                              for r0 in (0, hh) for c0 in (384, 512)]
            wo2[pl.ds(r, 8), _lt(15)] = _pk(jnp.where(lo, a3, a3 - b3))
            wo2[pl.ds(r, 8), _lt(16)] = _pk(jnp.where(lo, b3, b4 - a4))
            wo2[pl.ds(r, 8), _lt(17)] = _pk(jnp.where(lo, a4, b3))

    def normalize(blk, mean, rstd, link):
        if not link:
            return (xres[blk] - mean) * rstd
        rs = jnp.broadcast_to(rstd, (8, TB))
        mb = jnp.broadcast_to(mean, (8, TB))
        outs = []
        for i in range(D // 8):
            if i and i % link == 0:
                rs = tie(rs, outs[-1])
            outs.append((xres[blk, pl.ds(i * 8, 8), :] - mb) * rs)
        return jnp.concatenate(outs, axis=0)

    def left_ops(src, put, plain=False, which=None, dep=None):
        k1, k2, k3 = 3 * TC, 3 * TC + KY, 3 * TC + 2 * KY
        for n in (list(range(6 if plain else 15)) + [15, 16, 17]) if which is None else which:
            def X(t, r0, rows):
                return src[t, pl.ds((zero8 if plain else zero(n)) + r0, rows), :]
            if n == 15:
                v = jnp.concatenate([X(0, k1, KY), X(0, k2, KY) - X(1, k2, KY)], axis=0)
            elif n == 16:
                v = jnp.concatenate([X(1, k1, KY), X(1, k3, KY) - X(0, k3, KY)], axis=0)
            elif n == 17:
                v = jnp.concatenate([X(0, k3, KY), X(1, k2, KY)], axis=0)
            elif plain:
                v = X(n // 3, (n % 3) * TC, TC)
            else:
                v = _ssum([(X(t, i * TC, TC), sg) for (i, t), lst in _HK_C.items() for k, sg in lst if k == n])
            if dep is not None:
                v = jnp.concatenate([tie(v[0:8], dep), v[8:]], axis=0)
            put(n, pltpu.bitcast(v.astype(bf16).T, u32))

    def ln1(pr, par, src, ln, dep=None):
        blk = 2 * pr + par
        if src == 'res':
            x = xres[blk]
        else:
            x = xin[pr, :, par * TB:(par + 1) * TB].astype(f32)
            xres[blk] = x
        mean, rstd = _ln_stats(x, ln[0], None if dep is None else (lambda v: tie(v, dep)))
        if src == 'res':
            xn_g[par, pl.ds(0, 8), :] = jnp.zeros((8, TB), f32)
        xn_g[par, pl.ds(zero8, D), :] = normalize(blk, mean, rstd, ln[1])

    def add_ln(clock, t0, cfg, blk, dst, par, inp=None):
        np1, np2, step, gap, delay = cfg
        st = dict(s1=[], s2=[], left=np2)
        nv = D // 16

        def load(i):
            if inp is None:
                return xres[blk, pl.ds(zero8 + i * 16, 16), :]
            x = inp(i).astype(f32)
            xres[blk, pl.ds(i * 16, 16), :] = x
            return x

        def stats(k, dep):
            xs = []
            for i in range(k * nv // np1, (k + 1) * nv // np1):
                x = load(i)
                xs += [x[0:8], x[8:16]]
            if k == 0:
                st['c'] = jnp.broadcast_to(xs[0][0:1], (8, TB))
            c = tie(st['c'], dep)
            ds = [x - c for x in xs]
            st['s1'].append(_tree(jnp.add, ds))
            st['s2'].append(_tree(jnp.add, [d * d for d in ds]))
            return pltpu.bitcast(st['s1'][-1], u32) | pltpu.bitcast(st['s2'][-1], u32)

        def norm(k, dep):
            if k == 0:
                m = jnp.sum(_tree(jnp.add, st['s1']), axis=0, keepdims=True) * (1.0 / D)
                v = jnp.sum(_tree(jnp.add, st['s2']), axis=0, keepdims=True) * (1.0 / D) - m * m
                st['mean'] = st['c'] + m
                st['rstd'] = jnp.broadcast_to(lax.rsqrt(jnp.maximum(v, 0.0) + EPS), (8, TB))
            mean = tie(st['mean'], dep)
            off = 0 if inp is None else zero8
            for i in range(k * 2 * nv // np2, (k + 1) * 2 * nv // np2):
                dst[par, pl.ds(i * 8, 8), :] = (xres[blk, pl.ds(off + i * 8, 8), :] - mean) * st['rstd']
            st['left'] -= 1
            return pltpu.bitcast(dst[par, pl.ds(zero8, 8), :], u32)
        for k in range(np1):
            clock.add_due(t0 + k * step, functools.partial(stats, k), delay)
        for k in range(np2):
            clock.add_due(t0 + np1 * step + gap + k * step, functools.partial(norm, k), delay)
        return st

    def q_left(plain, which=None, dep=None):
        def put(i, v):
            sq_scr[i] = v
        left_ops(xn_g, put, plain, which, dep)

    def hk_outputs(P, T, PT, tk, emit, two_cols=False):
        p8 = P(8)
        t7 = P(7) + p8
        tk(2, t7)
        s1 = PT(3, 1, 2) + t7
        tk(2, s1)
        p6 = P(6)
        p14 = P(14)
        tk(2, p14)
        emit(1, 1, T(1, 1) + (p6 + p14 + s1), 1)
        p13 = P(13)
        if two_cols:
            emit(1, 0, PT(2, 1, 0) + (p13 + s1), 3)
        else:
            p12 = P(12)
            tk(2, p12)
            emit(1, 0, PT(2, 1, 0) + (p12 + p13 + s1), 2)
        p11 = P(11)
        t10 = P(10) + p11
        tk(2, t10)
        if not two_cols:
            s2 = PT(5, 2, 2) + t10
            tk(2, s2)
            p9 = P(9)
            emit(2, 0, T(2, 0) + (p9 + p12 + s2), 2)
            emit(2, 1, PT(4, 2, 1) + (p14 - p13 + s2), 2)
        w0 = T(0, 2)
        emit(0, 0, PT(0, 0, 0) + ((p8 + t10 + w0) if two_cols else (p8 + p9 + t10 + w0)), 3)
        emit(0, 1, PT(1, 0, 1) + (p6 + p11 + t7 + w0), 2)

    QT = (0, 1, 2, 3)
    KT = (4, 5, 6, 7, 13)
    VT = (8, 9, 10, 11, 12)
    c2e = DH ** -0.5 * math.log2(math.e)
    neg = -1e9 * math.log2(math.e)

    def q_step(pr, chunk, src, cfg, rows=False, sums=False):
        clock = _Timeline()
        if sums:
            base, nx = 0, 1
            for k in range(40):
                clock.add(200 + k * 90, functools.partial(wq_sums, 8 * k))
        elif rows:
            base, nx = pr * (2 * TB), pr + 1
            for k in range(2):
                clock.add_due(QA_T[k], functools.partial(row_chain, k, QA_T[2]), QA_T[3] - QA_T[k])
        else:
            base = pl.multiple_of(pr * (2 * TB), 2 * TB)
            nx = jnp.minimum(pr + 1, NP - 1)
        pieces = []
        if chunk is not None:
            for m in range(3):
                pieces += prep_pieces(jnp.maximum(chunk - LAGS[m], 0) if LAGS[m] else chunk, m)

        def paced(piece, dep):
            pw[0, pl.ds(R_END, 8), 0:128] = pltpu.bitcast(dep, u32)
            piece()
        for k, piece in enumerate(pieces):
            clock.add(QP0 + k * (QP1 - QP0) // len(pieces), functools.partial(paced, piece))
        if src == 'in':
            for par in range(2):
                add_ln(clock, cfg[par], cfg[2:], 2 * nx + par, xn_g, par,
                       functools.partial(lambda par_, i: xin[nx, pl.ds(i * 16, 16), par_ * TB:(par_ + 1) * TB], par))
        for r0, nt, tiles in ((0, 2, (0, 4, 8)), (TC, 2, (2, 6, 10)), (2 * TC, 1, (12, 13))):
            def R(k):
                return wq[pl.ds(r0, nt * 64), _lt(k)]

            def P(k):
                return _dot_nt(_up(sq_scr[k]), _up(R(k)))

            def T(j, kind):
                rhs = _up(R(15 + 3 * j + kind))
                if nt == 1 and (j, kind) in (QSPL if src == 'res' else QSPL0):
                    nq = 4 if src == 'res' else 2
                    return jnp.concatenate([_dot_nt(_up(sq_scr[15 + kind, pl.ds(k * (64 // nq), 64 // nq), :]), rhs)
                                            for k in range(nq)], axis=0)
                return _dot_nt(_up(sq_scr[15 + kind]), rhs)

            def PT(k, j, kind):
                return _dot_nt(_up(jnp.concatenate([sq_scr[k], sq_scr[15 + kind]], axis=1)),
                               _up(jnp.concatenate([R(k), R(15 + 3 * j + kind)], axis=1)))

            def tk(np_, v):
                clock.tick(32 * nt * np_, v, 4)

            def emit(col, half, v, np_):
                for k in range(nt):
                    qall[tiles[col] + k, pl.ds(base + (HALO + half * TB), TB), :] = v[:, k * 128:(k + 1) * 128]
                tk(np_, v)
            if src == 'res':
                hk_outputs(P, T, PT, tk, emit, two_cols=(nt == 1))
                continue
            for j in range(len(tiles)):
                both = T(j, 2)
                clock.t += 32 * nt
                for t in range(2):
                    for k in range(nt):
                        lhs = [sq_scr[3 * t + i] for i in range(3)] + [sq_scr[15 + t]]
                        lhs[0] = gate(lhs[0], clock)
                        rhs = [wq[pl.ds(r0 + k * 64, 64), _lt(n)]
                               for n in [wq_slot(i, j) for i in range(3)] + [15 + 3 * j + t]]
                        v = _dot_nt(_up(jnp.concatenate(lhs, axis=1)), _up(jnp.concatenate(rhs, axis=1))) + both[:, _lt(k)]
                        qall[tiles[j] + k, pl.ds(base + (HALO + t * TB), TB), :] = v
                        clock.tick(128, v, QTK)
        assert not clock.pending()
        if src == 'in':
            q_left(True)

    def row_group(blk, par, r, nw, nv, mids=None):
        base = _al(blk * TB, TB)
        lo = lax.broadcasted_iota(jnp.int32, (RB, 128), 1) < KY
        r0 = r * RB

        def ld(t, w):
            return qall[t, pl.ds(base + (HALO + r0 - DIL * w), RB), :]
        dep = yield
        cs = tie(jnp.full((RB, 128), c2e, f32), dep)
        q = [ld(t, 0) * cs for t in QT] + [jnp.where(lo, pltpu.roll(ld(13, 0), KY, 1), 0.0) * cs]
        sc = []
        for w in range(W):
            if w and w % nw == 0:
                dep = yield
                q = [tie(q[0], dep)] + q[1:]
            acc = None
            for j, t in enumerate(KT):
                p = q[j] * ld(t, w)
                acc = p if acc is None else acc + p
            acc = acc + pltpu.roll(acc, 64, 1)
            if mids is not None:
                mids[r] = pltpu.bitcast(acc, u32)
            acc = acc + pltpu.roll(acc, 32, 1)
            if r0 - DIL * w < 0:
                pos = blk * TB + r0 + lax.broadcasted_iota(jnp.int32, (RB, 128), 0)
                acc = jnp.where(pos >= DIL * w, acc, neg)
            sc.append(acc)
        m = _tree(jnp.maximum, sc)
        e = [jnp.exp2(sc[w] - m) for w in range(W)]
        l = _tree(jnp.add, e)
        rinv = pl.reciprocal(l, approx=True)
        rinv = rinv * (2.0 - l * rinv)
        outs = []
        for j, t in enumerate(VT):
            if j and j % nv == 0:
                dep = yield _tree(jnp.bitwise_or, [pltpu.bitcast(v, u32) for v in outs])
                outs = []
                e = [tie(e[0], dep)] + e[1:]
            acc = None
            for w in range(W):
                p = e[w] * ld(t, w)
                acc = p if acc is None else acc + p
            o = acc * rinv
            o_s[par * 5 + j, pl.ds(r0, RB), :] = o
            outs.append(o)
        yield _tree(jnp.bitwise_or, [pltpu.bitcast(v, u32) for v in outs])

    def add_rows(clock, t0, blk, par, r, cfg):
        nw, nv, step, gap, d1, d2 = cfg
        gen = row_group(blk, par, r, nw, nv)
        next(gen)
        n1, n2 = -(-W // nw), -(-5 // nv)
        for k in range(n1):
            clock.add_due(t0 + k * step, gen.send, d1)
        for k in range(n2 - 1):
            clock.add_due(t0 + (n1 - 1) * step + gap + k * step, gen.send, d2)

    def row_chain(blk, lag, dep):
        mids, fins = {}, {}
        for r in range(nr):
            gen = row_group(blk, blk, r, W, 5, mids)
            next(gen)
            if r:
                dep = pltpu.bitcast(mids[r - 1] | fins[r - lag] if r >= lag else mids[r - 1], f32)
            fins[r] = gen.send(dep)
        return _tree(jnp.bitwise_or, [fins[r] for r in range(nr - lag, nr)])

    wo_seq = []
    for pos, k in enumerate(WORD):
        if pos in (0, 2):
            wo_seq += [('r', pos // 2, k_) for k_ in range(3)]
        wo_seq.append(('p', k))

    def wo_rhs(off):
        lo = lax.broadcasted_iota(jnp.int32, (TB, 128), 1) < KY

        rhs = {}
        for it in wo_seq:
            z = zero(wo_seq.index(it)) if off is None else off

            def O(t, j):
                return o_s[t * 5 + j, pl.ds(z, TB), :]
            if it[0] == 'p':
                v = _ssum([(O(t, j), sg) for j, t, sg in _HK_B[it[1]]])
            elif it[2] == 0:
                v = O(it[1], 3)
            else:
                v = jnp.where(lo, O(it[1], 2 + it[2]), O(it[1], 5 - it[2]))
            rhs[it] = v.astype(bf16)
        return rhs

    def wo_mm(blk0, rhs):
        res = {}
        for it in wo_seq:
            if it[0] == 'p':
                lhs = wo2[pl.ds(0, D3 // 2), _lt(it[1])]
            else:
                lhs = wo2[:, _lt(15 + it[2])]
            res[it] = _dot_nt(_up(lhs), rhs[it])
        for t in range(2):
            both = res['r', t, 2]
            rem = xres[blk0 + t] + jnp.concatenate([res['r', t, 0] + both, res['r', t, 1] + both], axis=0)
            y = jnp.concatenate([_ssum([(res['p', k], sg) for k, sg in _HK_C[i, t]]) for i in range(3)], axis=0)
            xres[blk0 + t] = y + rem

    def a_left(which=range(15), dep=None, cb=None):
        for n in which:
            v = _ssum([(xn_f[t, pl.ds(zero(n) + i * D3, D3), :], sg)
                       for (i, t), lst in _HK_C.items() for k, sg in lst if k == n])
            if dep is not None:
                v = jnp.concatenate([tie(v[0:8], dep), v[8:2 * KY], tie(v[2 * KY:2 * KY + 8], dep), v[2 * KY + 8:]],
                                    axis=0)
            t1 = pltpu.bitcast(v[:2 * KY].astype(bf16).T, u32)
            t2 = pltpu.bitcast(jnp.concatenate([v[2 * KY:], v[2 * KY:]], axis=0).astype(bf16).T, u32)
            if dep is None:
                arrange(n, t1, t2)
                cb(t1[0:8])
            else:
                st_s[2 * n] = t1
                st_s[2 * n + 1] = t2

    def arrange(n, t1, t2):
        lo = lax.broadcasted_iota(jnp.int32, (TB // 2, 128), 1) < KY
        s_scr[3 * n] = t1
        s_scr[3 * n + 1] = jnp.where(lo, t1, t2)
        s_scr[3 * n + 2] = jnp.where(lo, t2, t1)

    def a_arrange(n, dep):
        st_s[30, pl.ds(0, 8), :] = pltpu.bitcast(dep, u32)
        arrange(n, st_s[2 * n, pl.ds(zero8, TB // 2), :], st_s[2 * n + 1, pl.ds(zero8, TB // 2), :])

    k0 = math.sqrt(2.0 / math.pi)
    k1 = k0 * 0.044715

    def ffn(j, c0, script):
        clock = _Timeline()
        b0 = (2 * j) % NB
        an = (2 * j + 2) % NB
        acc = [None] * 15
        hs = {}
        lns, lq, staged, nrows = [], [], set(), 0

        pend = []

        def advance(keep):
            while len(pend) > keep:
                pend.pop(0)()

        def written(k):
            clock.due.append(lambda: pltpu.bitcast(p_s[k][pl.ds(zero8, 8), 0:128], u32))

        def gu(p):
            c, second = c0 + p // 2, p % 2
            m = 1 - second if UFIRST else second
            h = hs.setdefault(p // 2, [[None, None] for _ in range(3)])

            def mm(n, kind):
                lhs = gate(s_scr[3 * n + kind], clock)
                return _dot(_up(lhs), _up(pw[c, pl.ds((3 * n + kind) * (TC // 2), TC // 2), m * TC:(m + 1) * TC]))

            def get(name):
                return p_s[PSLOT[name]][pl.ds(zero8, TB), :]

            def post(n, v):
                adds, keep, emits = GU_POST[n]
                if keep[0] is not None:
                    p_s[PSLOT[keep[0]]][...] = v
                    written(PSLOT[keep[0]])
                w_ = v
                for name, sg in adds:
                    w_ = w_ + get(name) if sg == 1 else w_ - get(name)
                if keep[1] is not None:
                    p_s[PSLOT[keep[1]]][...] = w_
                    written(PSLOT[keep[1]])
                if emits is not None:
                    col, half = emits
                    if m == 0:
                        w_ = w_ + w_ * jnp.tanh(w_ * (k0 + k1 * (w_ * w_)))
                    if second:
                        k_ = 17 + 6 * ((p // 2) % 2) + 2 * col + half
                        p_s[k_][...] = w_ * p_s[11 + 2 * col + half][pl.ds(zero8, TB), :]
                        written(k_)
                        h[col][half] = k_
                    else:
                        p_s[11 + 2 * col + half][...] = w_
                        written(11 + 2 * col + half)
            for n in GU_ORD:
                both = mm(n, 2)
                v = jnp.concatenate([mm(n, 0) + both, mm(n, 1) + both], axis=1)
                pend.append(functools.partial(post, n, v))
                advance(PLAG)
                clock.tick(96, both, GTK)

        def down(ps):
            cs = ps[::2]
            hsl = [hs.pop(p // 2) for p in cs]
            for pos, i in enumerate(DORD_F if last else DORD):
                while any(h_[j_][t_] is None for h_ in hsl for j_, t_, _ in _HK_B[i]):
                    advance(len(pend) - 1)
                au = []
                for p in cs:
                    au += [pw[c0 + p // 2, pl.ds(R_SD + i * (D3 // 2), D3 // 2), k * TC:(k + 1) * TC] for k in range(2)]
                au[0] = gate(au[0], clock)
                r = _dot_nt(jnp.concatenate([_up(v) for v in au], axis=1),
                            jnp.concatenate([_ssum([(p_s[h_[j_][t_]][pl.ds(zero(i), TB), :], sg) for j_, t_, sg in _HK_B[i]])
                                             for h_ in hsl], axis=1).astype(bf16))
                acc[i] = r if acc[i] is None else r + acc[i]
                advance(max(len(pend) - DADV, 0))
                clock.tick(48 * len(ps), acc[i], DTK)

        pg = pd = 0
        for tok in script:
            if tok == 'G':
                gu(pg)
                pg += 1
            elif tok[0] == 'D':
                down(list(range(pd, pd + int(tok[1:]))))
                pd += int(tok[1:])
            elif tok == 'W':
                assert not clock.pending() and nrows == 2 * nr
                advance(0)
                wo_mm(an, wo_rhs(None))
                clock.t += 1152
            elif tok[0] == 'n':
                lns.append(add_ln(clock, clock.t + int(tok[3:]), LNJ + (JDL,), an + int(tok[1]), xn_f, int(tok[1])))
            elif tok[0] == 'm':
                lq.append(add_ln(clock, clock.t + int(tok[3:]), LNJ + (JDL,), (2 * j + 4) % NB + int(tok[1]), xn_g,
                                 int(tok[1])))
            elif tok[0] == 'k':
                _, t0, dt = tok.split('+')

                def qleft(which, dep):
                    assert len(lq) == 2 and not any(st['left'] for st in lq)
                    q_left(False, which, dep)
                    return sq_scr[which[0], pl.ds(zero8, 8), :]
                for k in range(NQL):
                    clock.add_due(clock.t + int(t0) + k * int(dt),
                                  functools.partial(qleft, range(k * 18 // NQL, (k + 1) * 18 // NQL)), LDL)
            elif tok[0] == 'l':
                _, t0, dt = tok.split('+')

                def left(which, dep):
                    assert len(lns) == 2 and not any(st['left'] for st in lns)
                    staged.update(which)
                    a_left(which, dep)
                    return st_s[0, pl.ds(zero8, 8), :]
                for k in range(NLEFT):
                    clock.add_due(clock.t + int(t0) + k * int(dt),
                                  functools.partial(left, range(k * 15 // NLEFT, (k + 1) * 15 // NLEFT)), LDL)
            elif tok[0] == 'c':
                _, t0, dt = tok.split('+')
                assert pg == 2 * NCH

                def place(k, dep):
                    assert k in staged
                    a_arrange(k, dep)
                for k in range(15):
                    clock.add(clock.t + int(t0) + k * int(dt), functools.partial(place, k))
            else:
                n, t0, dt = tok[1:].split('+')
                for k in range(int(n)):
                    add_rows(clock, clock.t + int(t0) + k * int(dt), an + nrows // nr, nrows // nr, nrows % nr,
                             RG + (RDL, JDL))
                    nrows += 1
        assert pg == pd and not clock.pending()
        for t in range(2):
            y = jnp.concatenate([_ssum([(acc[k], sg) for k, sg in _HK_C[i, t]]) for i in range(3)], axis=0)
            x2 = xres[b0 + t] + 0.5 * y
            xres[b0 + t] = x2
            xin[j % NP, :, t * TB:(t + 1) * TB] = x2.astype(bf16)

    if last:
        if ONLY in ('', 'f'):
            ffn(2 * NP - 1, g * NPC, SCRIPT_F)
        return
    assert NCH == NP - 2

    late = [(c, m) for c in range(NCH) for m in range(3) if c >= NCH - LAGS[m]]

    def prologue():
        cp_x(0).start()
        for sec in range(3):
            for cp in cp_qkv(sec):
                cp.start()
        qall[:, pl.ds(0, HALO), :] = jnp.zeros((16, HALO, 128), f32)
        cp_x(0).wait()
        ln1(0, 0, 'in', (4, 0))
        ln1(0, 1, 'in', (4, 0))
        q_left(True)
        for sec in range(3):
            for cp in cp_qkv(sec):
                cp.wait()
            if sec == 0:
                cp_x(1).start()
                cp_x(2).start()
                cp_wo().start()
                for c in range(NCH):
                    if 3 + c < NP:
                        cp_x(3 + c).start()
                    for m in range(3):
                        if c == 0 or c > LAGS[m]:
                            cp_unit(max(c - LAGS[m], 0), m).start()
                for c, m in late:
                    cp_unit(c, m).start()
            transpose_qkv(sec)
            build_wq(sec)

    def first_attention():
        cp_x(2).wait()
        q_step(1, None, 'in', CFG_QA, rows=True)
        cp_wo().wait()
        build_wo()
        wo_mm(0, wo_rhs(None if W0DYN else 0))

    def startup_step(c, carry):
        @pl.when(c + 3 < NP)
        def _():
            cp_x(c + 3).wait()
        for m in range(3):
            if LAGS[m]:
                @pl.when(jnp.logical_or(c == 0, c > LAGS[m]))
                def _():
                    cp_unit(jnp.maximum(c - LAGS[m], 0), m).wait()
            else:
                cp_unit(c, m).wait()
        q_step(c + 2, c, 'in', CFG_Q1)
        return carry

    @pl.when(g == 0)
    def _():
        if ONLY in ('', 'pro'):
            prologue()
            cp_x(1).wait()
            q_step(0, None, 'in', CFG_Q0, sums=True)
        if ONLY in ('', 'a'):
            first_attention()
        if ONLY in ('', 'q'):
            lax.fori_loop(0, NCH, startup_step, 0)
        if ONLY in ('', 'a'):
            pieces = []
            for c, m in late:
                cp_unit(c, m).wait()
                pieces += prep_pieces(c, m)
            npt = 15 + 2 * TLN

            def pace(v):
                pw[0, pl.ds(R_END + zero8, 8), 0:128] = v
                pace.k += 1
                for piece in pieces[(pace.k - 1) * len(pieces) // npt:pace.k * len(pieces) // npt]:
                    piece()
            pace.k = 0
            for t in range(2):
                mean, rstd = _ln_stats(xres[t], 4)
                xn = (xres[t, pl.ds(zero8, D), :] - mean) * rstd
                xn_f[t] = xn
                for k in range(TLN):
                    pace(pltpu.bitcast(xn[k * 64:k * 64 + 8], u32))
            a_left(cb=pace)

    @pl.when(g >= NP - 1)
    def _():
        if ONLY in ('', 'q', 'p'):
            q_step(g - (NP - 1), None, 'res', None)

    if ONLY in ('q', 'a', 'pro'):
        @pl.when(g == 2 * NP - 2)
        def _():
            xin[0, 0:16, 0:128] = (qall[g % 16, pl.ds(zero8, 16), :] + xres[g % 16, pl.ds(zero8, 16), :]
                                  + pltpu.bitcast(pw[g % 4, pl.ds(zero8, 16), 0:128] | s_scr[g % 8, pl.ds(zero8, 16), :]
                                                  | wo2[pl.ds(zero8, 16), 0:128] | wq[pl.ds(zero8, 16), 0:128] | sq_scr[g % 8, pl.ds(zero8, 16), :], f32)).astype(bf16)

    if ONLY in ('', 'p'):
        ffn(g, 0, SCRIPT)

    @pl.when(g >= NP)
    def _():
        _cp_out(g - NP, o_hbm, xin, sems).start()


def _cp_out(k, o_hbm, xin, sems):
    return pltpu.make_async_copy(xin.at[k], o_hbm.at[:, pl.ds(_al(k * 2 * TB, 128), 2 * TB)], sems.at[4 + k])


def _kernel(*refs, D, DF, S):
    def body(last, g, carry):
        _step(g, last, *refs, D=D, DF=DF, S=S)
        return carry
    NP = S // (2 * TB)
    lax.fori_loop(0, 2 * NP - 1, functools.partial(body, False), 0)
    lax.fori_loop(0, 2, functools.partial(body, True), 0)
    o_hbm, xin, sems = refs[6], refs[7], refs[24]
    _cp_out(NP - 1, o_hbm, xin, sems).start()
    for k in range(NP):
        _cp_out(k, o_hbm, xin, sems).wait()


@jax.jit
def pallas_interleave_layers__sliding_local_dilated__glu_gated_geglu__prompt_kernel(
    A_x, A_wqkv, A_wo, B_x, B_w_gate, B_w_up, B_w_down):
    B, S, D = A_x.shape
    DF = B_w_gate.shape[1]
    NB = S // TB
    NP = NB // 2
    NCH = DF // CW
    xT = A_x.reshape(S, D).T
    wdT = B_w_down.T
    hbm = pl.BlockSpec(memory_space=pltpu.HBM)
    outT = pl.pallas_call(
        functools.partial(_kernel, D=D, DF=DF, S=S),
        in_specs=[hbm] * 6,
        out_specs=hbm,
        out_shape=jax.ShapeDtypeStruct((D, S), A_x.dtype),
        scratch_shapes=[
            pltpu.VMEM((NP, D, 2 * TB), bf16),
            pltpu.VMEM((D, 3 * D), bf16),
            pltpu.VMEM((D, D), bf16),
            pltpu.VMEM((5, 14 * 128, 128), f32),
            pltpu.VMEM((WQR, 27 * 128), u32),
            pltpu.VMEM((D // 2, 640), u32),
            pltpu.VMEM((D // 4, 18 * 128), u32),
            pltpu.VMEM((NCH, 3, D, CW), bf16),
            pltpu.VMEM((NCH, 45 * (TC // 2) + 15 * (D // 6) + 16, 2 * TC), u32),
            pltpu.VMEM((16, S + QPAD, 128), f32),
            pltpu.VMEM((11, TB, 128), f32),
            pltpu.VMEM((NB, D, TB), f32),
            pltpu.VMEM((2, D, TB), f32),
            pltpu.VMEM((2, D, TB), f32),
            pltpu.VMEM((45, TB // 2, TC), u32),
            pltpu.VMEM((31, TB // 2, TC), u32),
            pltpu.VMEM((18, TB // 2, TC), u32),
            pltpu.SemaphoreType.DMA((4 + NP + 3 * NCH,)),
        ] + [pltpu.VMEM((TB, 2 * TC), f32)] * 29,
        compiler_params=pltpu.CompilerParams(
            vmem_limit_bytes=110 * 1024 * 1024,
            disable_bounds_checks=bool(NOCHK),
            disable_semaphore_checks=bool(NOCHK),
        ),
    )(xT, A_wqkv, A_wo, B_w_gate, B_w_up, wdT)
    return outT.T.reshape(B, S, D)
```

```python
import functools
import math
import jax
import jax.numpy as jnp
from jax import lax
import jax.experimental.pallas as pl
import jax.experimental.pallas.tpu as pltpu

DH = 18
W = 8
DIL = 2
HALO = 16
EPS = 1e-5
TB = 128
RB = 8
TC = 128
CW = 6 * TC
WQR = 320
KY = 64
QPAD = 40

SCRIPT = ('m0+50,m1+2900,k+8700+100,G,R6+50+240,G,G,R10+50+350,G,D4,G,R6+50+240,G,G,R10+50+280,'
          'G,D4,W,n0+1600,n1+2152,l+4300+180,G,G,G,G,c+400+96,D4').split(',')
SCRIPT_F = 'G,G,G,G,D2,G,G,D2,D2'.split(',')
GU_ORD = (8, 6, 7, 11, 3, 1, 10, 14, 9, 5, 0, 13, 12, 4, 2)
DORD = (1, 6, 0, 9, 10, 11, 4, 14, 5, 7, 8, 12, 13, 2, 3)
DORD_F = (1, 6, 0, 9, 10, 4, 11, 5, 14, 7, 2, 8, 3, 12, 13)
WORD = (0, 1, 2, 6, 7, 8, 9, 10, 11, 12, 13, 14, 3, 4, 5)
PLAG, DADV, GTK, DTK, QTK = 5, 2, 4, 4, 8
LNJ = (12, 9, 48, 48)
RG = (1, 1, 48, 460)
RDL, JDL, LDL = 650, 250, 500
NLEFT, NQL, TLN = 5, 9, 3
CFG_Q0 = (40, 1816, 18, 18, 48, 48, 350)
CFG_QA = (300, 748, 6, 6, 32, 64, 350)
CFG_Q1 = (40, 1456, 9, 9, 64, 64, 300)
QA_T = (300, 1000, 4, 3850)
QP0, QP1 = 100, 3850
LAGS = (0, 0, 2)

f32 = jnp.float32
bf16 = jnp.bfloat16
u32 = jnp.uint32
NT = (((1,), (1,)), ((), ()))


def _al(i, n):
    return i if isinstance(i, int) else pl.multiple_of(i, n)


def _lt(k):
    return slice(k * 128, (k + 1) * 128)


def _pk(x):
    return pltpu.bitcast(x.astype(bf16), u32)


def _up(x):
    return pltpu.bitcast(x, bf16)


def _dot(a, b):
    return jnp.dot(a, b, preferred_element_type=f32)


def _dot_nt(a, b):
    return lax.dot_general(a, b, NT, preferred_element_type=f32)


def _tree(fn, xs):
    xs = list(xs)
    while len(xs) > 1:
        xs = [fn(xs[i], xs[i + 1]) for i in range(0, len(xs) - 1, 2)] + ([xs[-1]] if len(xs) % 2 else [])
    return xs[0]


def _ln_stats(x, nacc=4):
    n = x.shape[0]
    c = x[0:1]
    s1 = [None] * nacc
    s2 = [None] * nacc
    for i in range(n // 8):
        d = x[i * 8:(i + 1) * 8] - c
        k = i % nacc
        s1[k] = d if s1[k] is None else s1[k] + d
        dd = d * d
        s2[k] = dd if s2[k] is None else s2[k] + dd
    m = jnp.sum(_tree(jnp.add, s1), axis=0, keepdims=True) * (1.0 / n)
    v = jnp.sum(_tree(jnp.add, s2), axis=0, keepdims=True) * (1.0 / n) - m * m
    v = jnp.maximum(v, 0.0)
    return c + m, lax.rsqrt(v + EPS)


_HK_A = (
    ((0, 0, 1), (0, 2, -1), (1, 0, -1)), ((0, 0, 1), (0, 1, -1), (2, 0, -1)), ((1, 1, 1), (0, 1, -1), (1, 2, -1)),
    ((1, 1, 1), (1, 0, -1), (2, 1, -1)), ((2, 2, 1), (0, 2, -1), (2, 1, -1)), ((2, 2, 1), (1, 2, -1), (2, 0, -1)),
    ((0, 1, 1),), ((0, 1, 1), (1, 0, -1)), ((1, 0, 1),),
    ((0, 2, 1),), ((0, 2, 1), (2, 0, -1)), ((2, 0, 1),),
    ((1, 2, 1),), ((2, 1, 1), (1, 2, -1)), ((2, 1, 1),),
)
_HK_C = {
    (0, 0): ((0, 1), (7, 1), (8, 1), (9, 1), (6, -1)),
    (0, 1): ((1, 1), (6, 1), (10, 1), (11, 1), (9, -1)),
    (1, 0): ((2, 1), (7, 1), (8, 1), (12, 1), (6, -1)),
    (1, 1): ((3, 1), (6, 1), (13, 1), (14, 1), (2, -1), (7, -1)),
    (2, 0): ((5, 1), (9, 1), (12, 1), (13, 1), (4, -1), (10, -1)),
    (2, 1): ((4, 1), (10, 1), (11, 1), (14, 1), (9, -1)),
}
_HK_B = (((0, 0, 1),), ((0, 1, 1),), ((1, 0, 1),), ((1, 0, 1), (1, 1, 1)), ((2, 1, 1),), ((2, 0, 1), (2, 1, 1)),
         ((0, 1, 1), (1, 1, 1)), ((0, 1, 1), (1, 0, 1), (1, 1, 1)), ((0, 0, 1), (0, 1, 1), (1, 0, 1), (1, 1, 1)),
         ((0, 0, 1), (2, 0, 1)), ((0, 0, 1), (2, 0, 1), (2, 1, 1)), ((0, 0, 1), (0, 1, 1), (2, 0, 1), (2, 1, 1)),
         ((1, 0, 1), (2, 0, 1)), ((1, 0, 1), (2, 1, -1)), ((1, 1, 1), (2, 1, 1)))


def _ssum(terms):
    terms = sorted(terms, key=lambda z: -z[1])
    acc = terms[0][0] if terms[0][1] == 1 else -terms[0][0]
    for v, sg in terms[1:]:
        acc = acc + v if sg == 1 else acc - v
    return acc


GU_POST = {
    8: ((), ('p8', None), None),
    7: ((('p8', 1),), (None, 't7'), None),
    3: ((('t7', 1),), (None, 's1'), None),
    6: ((), ('p6', None), None),
    14: ((('p6', 1), ('s1', 1)), ('p14', None), (1, 1)),
    12: ((('p9', 1), ('s2', 1)), ('p12', None), (2, 0)),
    13: ((), ('p13', None), None),
    2: ((('p12', 1), ('p13', 1), ('s1', 1)), (None, None), (1, 0)),
    11: ((), ('p11', None), None),
    10: ((('p11', 1),), (None, 't10'), None),
    5: ((('t10', 1),), (None, 's2'), None),
    9: ((), ('p9', None), None),
    4: ((('p14', 1), ('s2', 1), ('p13', -1)), (None, None), (2, 1)),
    0: ((('p8', 1), ('p9', 1), ('t10', 1)), (None, None), (0, 0)),
    1: ((('p6', 1), ('p11', 1), ('t7', 1)), (None, None), (0, 1)),
}
PSLOT = {k: i for i, k in enumerate(('p8', 't7', 's1', 'p6', 'p14', 'p12', 'p13', 'p11', 't10', 's2', 'p9'))}


class _Timeline:
    def __init__(self):
        self.t = 0
        self.jobs = []
        self.due = []

    def add(self, when, fn):
        self.jobs.append((when, len(self.jobs), fn))
        self.jobs.sort(key=lambda z: z[:2])

    def add_due(self, when, job, delay):
        def run(dep):
            val = job(dep)
            if val is not None:
                self.add(self.t + delay, lambda _: self.due.append(lambda: val))
        self.add(when, run)

    def pending(self):
        return [j for j in self.jobs if getattr(j[2], '__name__', '') != '<lambda>']

    def tick(self, dur, v, n):
        for k in range(n):
            self.t += dur // n
            r = k * (v.shape[0] // n)
            while self.jobs and self.jobs[0][0] <= self.t:
                self.jobs.pop(0)[2](v[r:r + 8, 0:128])


def _step(g, last, x_hbm, wqkv_hbm, wo_hbm, wg_hbm, wu_hbm, wd_hbm, o_hbm,
          xin, wqkv_raw, wo_raw, tmp, wq, woT, wo2, raw, pw, qall, o_s, xres, xn_f, xn_g, s_scr, st_s, sq_scr,
          sems, *p_s, D, DF, S):
    NB = S // TB
    NP = NB // 2
    NCH = DF // CW
    NPC = NCH // 2
    D3 = D // 3
    nr = TB // RB
    hh = D // 4
    zero8 = pl.multiple_of((g >> 20) * 8, 8)
    zvec = jnp.full((8, 128), (g >> 20).astype(u32), u32)

    def zero(k):
        return pl.multiple_of((g >> (8 + k)) * 8, 8)

    def tie(x, dep):
        return pltpu.bitcast(pltpu.bitcast(x, u32) | (pltpu.bitcast(dep, u32) & zvec), f32)

    def gate(lhs, clock):
        if not clock.due:
            return lhs
        pr = _tree(jnp.bitwise_or, [k() for k in clock.due]) & zvec
        del clock.due[:]
        return jnp.concatenate([lhs[0:8] | pr, lhs[8:]], axis=0)

    QSEC = ((0, 5), (5, 9), (9, 14))

    def cp_qkv(sec):
        out = []
        for j in range(*QSEC[sec]):
            n = min(128, 3 * D - j * 128)
            out.append(pltpu.make_async_copy(wqkv_hbm.at[:, pl.ds(j * 128, n)], wqkv_raw.at[:, pl.ds(j * 128, n)],
                                             sems.at[sec]))
        return out

    def cp_wo():
        return pltpu.make_async_copy(wo_hbm, wo_raw, sems.at[3])

    def cp_x(k):
        return pltpu.make_async_copy(x_hbm.at[:, pl.ds(_al(k * 2 * TB, 128), 2 * TB)], xin.at[k], sems.at[4 + k])

    def cp_unit(c, m):
        return pltpu.make_async_copy((wg_hbm, wu_hbm, wd_hbm)[m].at[:, pl.ds(_al(c * CW, 128), CW)], raw.at[c, m],
                                     sems.at[4 + NP + 3 * c + m])

    R_SD = 45 * (TC // 2)
    R_END = R_SD + 15 * (D3 // 2)

    def hk_a_ops(load, minus=None):
        blk = {}
        for i in range(3):
            for j in range(3):
                blk[i, j] = load(i, j).astype(f32)
                if minus is not None:
                    blk[i, j] = blk[i, j] - minus(i, j).astype(f32)
        return [_pk(_ssum([(blk[i, j], sg) for i, j, sg in terms])) for terms in _HK_A]

    def prep_pieces(c, m):
        def ld(r, cs):
            return lambda i, j: raw[c, m, pl.ds(i * D3 + r, 16), pl.ds((3 * cs + j) * TC, TC)]

        def gu_piece(q, r, cs, neg, kind, half):
            ops = hk_a_ops(ld(q * KY + r, cs), None if neg is None else ld(q * KY + r, neg))
            for k, t in enumerate(ops):
                pw.at[c][pl.ds((3 * k + kind) * (TC // 2) + (half * KY + r) // 2, 8), m * TC:(m + 1) * TC] = t

        def d_piece(r, cs):
            for k, t in enumerate(hk_a_ops(ld(r, cs))):
                pw.at[c][pl.ds(R_SD + k * (D3 // 2) + r // 2, 8), cs * TC:(cs + 1) * TC] = t
        if m == 2:
            return [functools.partial(d_piece, r, cs) for r in range(0, D3, 16) for cs in range(2)]
        spec = ((0, 0, None, 0, 0), (1, 0, 1, 0, 1), (0, 1, None, 1, 0), (2, 1, 0, 1, 1),
                (2, 0, None, 2, 0), (1, 1, None, 2, 1))
        return [functools.partial(gu_piece, q, r, cs, neg, kind, half)
                for r in range(0, KY, 16) for q, cs, neg, kind, half in spec]

    def transpose_qkv(sec):
        for j in range(*QSEC[sec]):
            wd_ = min(128, 3 * D - j * 128)
            blk = wqkv_raw[:, j * 128:j * 128 + wd_].astype(f32)
            if wd_ < 128:
                blk = jnp.concatenate([blk, jnp.zeros((D, 128 - wd_), f32)], axis=1)
            bt = jnp.concatenate([blk, blk[D - KY:]], axis=0).T
            for t in range(5):
                tmp[t, pl.ds(j * 128, 128), :] = bt[:, t * 128:(t + 1) * 128]

    def wq_slot(i, j):
        return 24 + i if i == j else [n for n, t in enumerate(_HK_A) if t == ((i, j, 1),)][0]

    def build_wq(sec):
        lo = lax.broadcasted_iota(jnp.int32, (32, 128), 1) < KY
        for d in range(DH):
            tt = [tmp[t, pl.ds(sec * D + d, 32, stride=DH), :] for t in range(5)]
            ops = tt[:4] + [jnp.where(lo, tt[3], tt[4]), jnp.where(lo, tt[4], tt[3])]
            if d < 16:
                dst = [(sec, d * 16)]
            else:
                dst = ([(1, (d + 2) * 16)], [(1, d * 16)], [(0, d * 16), (0, (d + 2) * 16)])[sec]
            for j, row in dst:
                for k, v in enumerate(ops):
                    wq[pl.ds(row, 16), _lt(wq_slot(k, j) if k < 3 else 12 + 3 * j + k)] = _pk(v)

    def wq_sums(r, dep):
        ncol = 3 if r < 256 else 2
        pin = pltpu.bitcast(dep, u32) & zvec
        blk = {(i, j): _up(wq[pl.ds(r, 8), _lt(wq_slot(i, j))] | pin).astype(f32) for i in range(3) for j in range(ncol)}
        for n, terms in enumerate(_HK_A):
            if len(terms) > 1 and not (ncol == 2 and n in (4, 5)):
                wq[pl.ds(r, 8), _lt(n)] = _pk(_ssum([(blk[i, j], sg) for i, j, sg in terms if j < ncol]))

    def build_wo():
        for t in range(5):
            wd_ = min(128, D - t * 128)
            blk = wo_raw[:, t * 128:t * 128 + wd_].astype(f32)
            if wd_ < 128:
                blk = jnp.concatenate([blk, jnp.zeros((D, 128 - wd_), f32)], axis=1)
            tmp[t, pl.ds(0, D), :] = blk
        for t in range(5):
            rows = [tmp[t, pl.ds(d, 32, stride=DH), :] for d in range(DH)]
            ft = jnp.concatenate(rows + rows[16:], axis=0).T
            n = min(128, D - t * 128)
            woT[pl.ds(t * 64, n // 2), :] = _pk(ft[:n])
        for r in range(0, D3 // 2, 8):
            ops = hk_a_ops(lambda i, j: _up(woT[pl.ds(i * (D3 // 2) + r, 8), j * TC:(j + 1) * TC]))
            for k, t in enumerate(ops):
                wo2[pl.ds(r, 8), _lt(k)] = t
        lo = lax.broadcasted_iota(jnp.int32, (16, 128), 1) < KY
        for r in range(0, hh, 8):
            a3, a4, b3, b4 = [_up(woT[pl.ds(r0 + r, 8), c0:c0 + 128]).astype(f32)
                              for r0 in (0, hh) for c0 in (384, 512)]
            wo2[pl.ds(r, 8), _lt(15)] = _pk(jnp.where(lo, a3, a3 - b3))
            wo2[pl.ds(r, 8), _lt(16)] = _pk(jnp.where(lo, b3, b4 - a4))
            wo2[pl.ds(r, 8), _lt(17)] = _pk(jnp.where(lo, a4, b3))

    def q_left(plain, which=None, dep=None):
        k1, k2, k3 = 3 * TC, 3 * TC + KY, 3 * TC + 2 * KY
        for n in (list(range(6 if plain else 15)) + [15, 16, 17]) if which is None else which:
            def X(t, r0, rows):
                return xn_g[t, pl.ds((zero8 if plain else zero(n)) + r0, rows), :]
            if n == 15:
                v = jnp.concatenate([X(0, k1, KY), X(0, k2, KY) - X(1, k2, KY)], axis=0)
            elif n == 16:
                v = jnp.concatenate([X(1, k1, KY), X(1, k3, KY) - X(0, k3, KY)], axis=0)
            elif n == 17:
                v = jnp.concatenate([X(0, k3, KY), X(1, k2, KY)], axis=0)
            elif plain:
                v = X(n // 3, (n % 3) * TC, TC)
            else:
                v = _ssum([(X(t, i * TC, TC), sg) for (i, t), lst in _HK_C.items() for k, sg in lst if k == n])
            if dep is not None:
                v = jnp.concatenate([tie(v[0:8], dep), v[8:]], axis=0)
            sq_scr[n] = pltpu.bitcast(v.astype(bf16).T, u32)

    def add_ln(clock, t0, cfg, blk, dst, par, inp=None):
        np1, np2, step, gap, delay = cfg
        st = dict(s1=[], s2=[], left=np2)
        nv = D // 16

        def load(i):
            if inp is None:
                return xres[blk, pl.ds(zero8 + i * 16, 16), :]
            x = inp(i).astype(f32)
            xres[blk, pl.ds(i * 16, 16), :] = x
            return x

        def stats(k, dep):
            xs = []
            for i in range(k * nv // np1, (k + 1) * nv // np1):
                x = load(i)
                xs += [x[0:8], x[8:16]]
            if k == 0:
                st['c'] = jnp.broadcast_to(xs[0][0:1], (8, TB))
            c = tie(st['c'], dep)
            ds = [x - c for x in xs]
            st['s1'].append(_tree(jnp.add, ds))
            st['s2'].append(_tree(jnp.add, [d * d for d in ds]))
            return pltpu.bitcast(st['s1'][-1], u32) | pltpu.bitcast(st['s2'][-1], u32)

        def norm(k, dep):
            if k == 0:
                m = jnp.sum(_tree(jnp.add, st['s1']), axis=0, keepdims=True) * (1.0 / D)
                v = jnp.sum(_tree(jnp.add, st['s2']), axis=0, keepdims=True) * (1.0 / D) - m * m
                st['mean'] = st['c'] + m
                st['rstd'] = jnp.broadcast_to(lax.rsqrt(jnp.maximum(v, 0.0) + EPS), (8, TB))
            mean = tie(st['mean'], dep)
            off = 0 if inp is None else zero8
            for i in range(k * 2 * nv // np2, (k + 1) * 2 * nv // np2):
                dst[par, pl.ds(i * 8, 8), :] = (xres[blk, pl.ds(off + i * 8, 8), :] - mean) * st['rstd']
            st['left'] -= 1
            return pltpu.bitcast(dst[par, pl.ds(zero8, 8), :], u32)
        for k in range(np1):
            clock.add_due(t0 + k * step, functools.partial(stats, k), delay)
        for k in range(np2):
            clock.add_due(t0 + np1 * step + gap + k * step, functools.partial(norm, k), delay)
        return st

    def hk_outputs(P, T, PT, emit, two_cols):
        p8 = P(8)
        t7 = P(7) + p8
        s1 = PT(3, 1, 2) + t7
        p6 = P(6)
        p14 = P(14)
        emit(1, 1, T(1, 1) + (p6 + p14 + s1))
        p13 = P(13)
        if two_cols:
            emit(1, 0, PT(2, 1, 0) + (p13 + s1))
        else:
            p12 = P(12)
            emit(1, 0, PT(2, 1, 0) + (p12 + p13 + s1))
        p11 = P(11)
        t10 = P(10) + p11
        if not two_cols:
            s2 = PT(5, 2, 2) + t10
            p9 = P(9)
            emit(2, 0, T(2, 0) + (p9 + p12 + s2))
            emit(2, 1, PT(4, 2, 1) + (p14 - p13 + s2))
        w0 = T(0, 2)
        emit(0, 0, PT(0, 0, 0) + ((p8 + t10 + w0) if two_cols else (p8 + p9 + t10 + w0)))
        emit(0, 1, PT(1, 0, 1) + (p6 + p11 + t7 + w0))

    QT = (0, 1, 2, 3)
    KT = (4, 5, 6, 7, 13)
    VT = (8, 9, 10, 11, 12)
    c2e = DH ** -0.5 * math.log2(math.e)
    neg = -1e9 * math.log2(math.e)

    def q_step(pr, cfg=None, chunk=None, rows=False, sums=False):
        first = cfg is not None
        clock = _Timeline()
        if sums:
            base, nx = 0, 1
            for k in range(40):
                clock.add(200 + k * 90, functools.partial(wq_sums, 8 * k))
        elif rows:
            base, nx = pr * (2 * TB), pr + 1
            for k in range(2):
                clock.add_due(QA_T[k], functools.partial(row_chain, k, QA_T[2]), QA_T[3] - QA_T[k])
        else:
            base = pl.multiple_of(pr * (2 * TB), 2 * TB)
            nx = jnp.minimum(pr + 1, NP - 1)
        pieces = []
        if chunk is not None:
            for m in range(3):
                pieces += prep_pieces(jnp.maximum(chunk - LAGS[m], 0) if LAGS[m] else chunk, m)

        def paced(piece, dep):
            pw[0, pl.ds(R_END, 8), 0:128] = pltpu.bitcast(dep, u32)
            piece()
        for k, piece in enumerate(pieces):
            clock.add(QP0 + k * (QP1 - QP0) // len(pieces), functools.partial(paced, piece))
        if first:
            for par in range(2):
                add_ln(clock, cfg[par], cfg[2:], 2 * nx + par, xn_g, par,
                       functools.partial(lambda par_, i: xin[nx, pl.ds(i * 16, 16), par_ * TB:(par_ + 1) * TB], par))
        for r0, nt, tiles in ((0, 2, (0, 4, 8)), (TC, 2, (2, 6, 10)), (2 * TC, 1, (12, 13))):
            def R(k):
                return wq[pl.ds(r0, nt * 64), _lt(k)]

            def P(k):
                return _dot_nt(_up(sq_scr[k]), _up(R(k)))

            def T(j, kind):
                rhs = _up(R(15 + 3 * j + kind))
                if nt == 1 and kind == 2:
                    nq = 2 if first else 4
                    return jnp.concatenate([_dot_nt(_up(sq_scr[15 + kind, pl.ds(k * (64 // nq), 64 // nq), :]), rhs)
                                            for k in range(nq)], axis=0)
                return _dot_nt(_up(sq_scr[15 + kind]), rhs)

            def PT(k, j, kind):
                return _dot_nt(_up(jnp.concatenate([sq_scr[k], sq_scr[15 + kind]], axis=1)),
                               _up(jnp.concatenate([R(k), R(15 + 3 * j + kind)], axis=1)))

            def emit(col, half, v):
                for k in range(nt):
                    qall[tiles[col] + k, pl.ds(base + (HALO + half * TB), TB), :] = v[:, k * 128:(k + 1) * 128]
            if not first:
                hk_outputs(P, T, PT, emit, nt == 1)
                continue
            for j in range(len(tiles)):
                both = T(j, 2)
                clock.t += 32 * nt
                for t in range(2):
                    for k in range(nt):
                        lhs = [sq_scr[3 * t + i] for i in range(3)] + [sq_scr[15 + t]]
                        lhs[0] = gate(lhs[0], clock)
                        rhs = [wq[pl.ds(r0 + k * 64, 64), _lt(n)]
                               for n in [wq_slot(i, j) for i in range(3)] + [15 + 3 * j + t]]
                        v = _dot_nt(_up(jnp.concatenate(lhs, axis=1)), _up(jnp.concatenate(rhs, axis=1))) + both[:, _lt(k)]
                        qall[tiles[j] + k, pl.ds(base + (HALO + t * TB), TB), :] = v
                        clock.tick(128, v, QTK)
        assert not clock.pending()
        if first:
            q_left(True)

    def row_group(blk, par, r, nw, nv, mids=None):
        base = _al(blk * TB, TB)
        lo = lax.broadcasted_iota(jnp.int32, (RB, 128), 1) < KY
        r0 = r * RB

        def ld(t, w):
            return qall[t, pl.ds(base + (HALO + r0 - DIL * w), RB), :]
        dep = yield
        cs = tie(jnp.full((RB, 128), c2e, f32), dep)
        q = [ld(t, 0) * cs for t in QT] + [jnp.where(lo, pltpu.roll(ld(13, 0), KY, 1), 0.0) * cs]
        sc = []
        for w in range(W):
            if w and w % nw == 0:
                dep = yield
                q = [tie(q[0], dep)] + q[1:]
            acc = None
            for j, t in enumerate(KT):
                p = q[j] * ld(t, w)
                acc = p if acc is None else acc + p
            acc = acc + pltpu.roll(acc, 64, 1)
            if mids is not None:
                mids[r] = pltpu.bitcast(acc, u32)
            acc = acc + pltpu.roll(acc, 32, 1)
            if r0 - DIL * w < 0:
                pos = blk * TB + r0 + lax.broadcasted_iota(jnp.int32, (RB, 128), 0)
                acc = jnp.where(pos >= DIL * w, acc, neg)
            sc.append(acc)
        m = _tree(jnp.maximum, sc)
        e = [jnp.exp2(sc[w] - m) for w in range(W)]
        l = _tree(jnp.add, e)
        rinv = pl.reciprocal(l, approx=True)
        rinv = rinv * (2.0 - l * rinv)
        outs = []
        for j, t in enumerate(VT):
            if j and j % nv == 0:
                dep = yield _tree(jnp.bitwise_or, [pltpu.bitcast(v, u32) for v in outs])
                outs = []
                e = [tie(e[0], dep)] + e[1:]
            acc = None
            for w in range(W):
                p = e[w] * ld(t, w)
                acc = p if acc is None else acc + p
            o = acc * rinv
            o_s[par * 5 + j, pl.ds(r0, RB), :] = o
            outs.append(o)
        yield _tree(jnp.bitwise_or, [pltpu.bitcast(v, u32) for v in outs])

    def add_rows(clock, t0, blk, par, r, cfg):
        nw, nv, step, gap, d1, d2 = cfg
        gen = row_group(blk, par, r, nw, nv)
        next(gen)
        n1, n2 = -(-W // nw), -(-5 // nv)
        for k in range(n1):
            clock.add_due(t0 + k * step, gen.send, d1)
        for k in range(n2 - 1):
            clock.add_due(t0 + (n1 - 1) * step + gap + k * step, gen.send, d2)

    def row_chain(blk, lag, dep):
        mids, fins = {}, {}
        for r in range(nr):
            gen = row_group(blk, blk, r, W, 5, mids)
            next(gen)
            if r:
                dep = pltpu.bitcast(mids[r - 1] | fins[r - lag] if r >= lag else mids[r - 1], f32)
            fins[r] = gen.send(dep)
        return _tree(jnp.bitwise_or, [fins[r] for r in range(nr - lag, nr)])

    wo_seq = []
    for pos, k in enumerate(WORD):
        if pos in (0, 2):
            wo_seq += [('r', pos // 2, k_) for k_ in range(3)]
        wo_seq.append(('p', k))

    def wo_rhs(off):
        lo = lax.broadcasted_iota(jnp.int32, (TB, 128), 1) < KY

        rhs = {}
        for it in wo_seq:
            z = zero(wo_seq.index(it)) if off is None else off

            def O(t, j):
                return o_s[t * 5 + j, pl.ds(z, TB), :]
            if it[0] == 'p':
                v = _ssum([(O(t, j), sg) for j, t, sg in _HK_B[it[1]]])
            elif it[2] == 0:
                v = O(it[1], 3)
            else:
                v = jnp.where(lo, O(it[1], 2 + it[2]), O(it[1], 5 - it[2]))
            rhs[it] = v.astype(bf16)
        return rhs

    def wo_mm(blk0, rhs):
        res = {}
        for it in wo_seq:
            if it[0] == 'p':
                lhs = wo2[pl.ds(0, D3 // 2), _lt(it[1])]
            else:
                lhs = wo2[:, _lt(15 + it[2])]
            res[it] = _dot_nt(_up(lhs), rhs[it])
        for t in range(2):
            both = res['r', t, 2]
            rem = xres[blk0 + t] + jnp.concatenate([res['r', t, 0] + both, res['r', t, 1] + both], axis=0)
            y = jnp.concatenate([_ssum([(res['p', k], sg) for k, sg in _HK_C[i, t]]) for i in range(3)], axis=0)
            xres[blk0 + t] = y + rem

    def a_left(which=range(15), dep=None, cb=None):
        for n in which:
            v = _ssum([(xn_f[t, pl.ds(zero(n) + i * D3, D3), :], sg)
                       for (i, t), lst in _HK_C.items() for k, sg in lst if k == n])
            if dep is not None:
                v = jnp.concatenate([tie(v[0:8], dep), v[8:2 * KY], tie(v[2 * KY:2 * KY + 8], dep), v[2 * KY + 8:]],
                                    axis=0)
            t1 = pltpu.bitcast(v[:2 * KY].astype(bf16).T, u32)
            t2 = pltpu.bitcast(jnp.concatenate([v[2 * KY:], v[2 * KY:]], axis=0).astype(bf16).T, u32)
            if dep is None:
                arrange(n, t1, t2)
                cb(t1[0:8])
            else:
                st_s[2 * n] = t1
                st_s[2 * n + 1] = t2

    def arrange(n, t1, t2):
        lo = lax.broadcasted_iota(jnp.int32, (TB // 2, 128), 1) < KY
        s_scr[3 * n] = t1
        s_scr[3 * n + 1] = jnp.where(lo, t1, t2)
        s_scr[3 * n + 2] = jnp.where(lo, t2, t1)

    def a_arrange(n, dep):
        st_s[30, pl.ds(0, 8), :] = pltpu.bitcast(dep, u32)
        arrange(n, st_s[2 * n, pl.ds(zero8, TB // 2), :], st_s[2 * n + 1, pl.ds(zero8, TB // 2), :])

    k0 = math.sqrt(2.0 / math.pi)
    k1 = k0 * 0.044715

    def ffn(j, c0, script):
        clock = _Timeline()
        b0 = (2 * j) % NB
        an = (2 * j + 2) % NB
        acc = [None] * 15
        hs = {}
        lns, lq, staged, nrows = [], [], set(), 0

        pend = []

        def advance(keep):
            while len(pend) > keep:
                pend.pop(0)()

        def written(k):
            clock.due.append(lambda: pltpu.bitcast(p_s[k][pl.ds(zero8, 8), 0:128], u32))

        def gu(p):
            c, m = c0 + p // 2, p % 2
            h = hs.setdefault(p // 2, [[None, None] for _ in range(3)])

            def mm(n, kind):
                lhs = gate(s_scr[3 * n + kind], clock)
                return _dot(_up(lhs), _up(pw[c, pl.ds((3 * n + kind) * (TC // 2), TC // 2), m * TC:(m + 1) * TC]))

            def get(name):
                return p_s[PSLOT[name]][pl.ds(zero8, TB), :]

            def post(n, v):
                adds, keep, emits = GU_POST[n]
                if keep[0] is not None:
                    p_s[PSLOT[keep[0]]][...] = v
                    written(PSLOT[keep[0]])
                w_ = v
                for name, sg in adds:
                    w_ = w_ + get(name) if sg == 1 else w_ - get(name)
                if keep[1] is not None:
                    p_s[PSLOT[keep[1]]][...] = w_
                    written(PSLOT[keep[1]])
                if emits is not None:
                    col, half = emits
                    if m == 1:
                        k_ = 17 + 6 * ((p // 2) % 2) + 2 * col + half
                        p_s[k_][...] = w_ * p_s[11 + 2 * col + half][pl.ds(zero8, TB), :]
                        written(k_)
                        h[col][half] = k_
                    else:
                        p_s[11 + 2 * col + half][...] = w_ + w_ * jnp.tanh(w_ * (k0 + k1 * (w_ * w_)))
                        written(11 + 2 * col + half)
            for n in GU_ORD:
                both = mm(n, 2)
                v = jnp.concatenate([mm(n, 0) + both, mm(n, 1) + both], axis=1)
                pend.append(functools.partial(post, n, v))
                advance(PLAG)
                clock.tick(96, both, GTK)

        def down(ps):
            cs = ps[::2]
            hsl = [hs.pop(p // 2) for p in cs]
            for i in (DORD_F if last else DORD):
                while any(h_[j_][t_] is None for h_ in hsl for j_, t_, _ in _HK_B[i]):
                    advance(len(pend) - 1)
                au = []
                for p in cs:
                    au += [pw[c0 + p // 2, pl.ds(R_SD + i * (D3 // 2), D3 // 2), k * TC:(k + 1) * TC] for k in range(2)]
                au[0] = gate(au[0], clock)
                r = _dot_nt(jnp.concatenate([_up(v) for v in au], axis=1),
                            jnp.concatenate([_ssum([(p_s[h_[j_][t_]][pl.ds(zero(i), TB), :], sg) for j_, t_, sg in _HK_B[i]])
                                             for h_ in hsl], axis=1).astype(bf16))
                acc[i] = r if acc[i] is None else r + acc[i]
                advance(max(len(pend) - DADV, 0))
                clock.tick(48 * len(ps), acc[i], DTK)

        pg = pd = 0
        for tok in script:
            if tok == 'G':
                gu(pg)
                pg += 1
            elif tok[0] == 'D':
                down(list(range(pd, pd + int(tok[1:]))))
                pd += int(tok[1:])
            elif tok == 'W':
                assert not clock.pending() and nrows == 2 * nr
                advance(0)
                wo_mm(an, wo_rhs(None))
                clock.t += 1152
            elif tok[0] == 'n':
                lns.append(add_ln(clock, clock.t + int(tok[3:]), LNJ + (JDL,), an + int(tok[1]), xn_f, int(tok[1])))
            elif tok[0] == 'm':
                lq.append(add_ln(clock, clock.t + int(tok[3:]), LNJ + (JDL,), (2 * j + 4) % NB + int(tok[1]), xn_g,
                                 int(tok[1])))
            elif tok[0] == 'k':
                _, t0, dt = tok.split('+')

                def qleft(which, dep):
                    assert len(lq) == 2 and not any(st['left'] for st in lq)
                    q_left(False, which, dep)
                    return sq_scr[which[0], pl.ds(zero8, 8), :]
                for k in range(NQL):
                    clock.add_due(clock.t + int(t0) + k * int(dt),
                                  functools.partial(qleft, range(k * 18 // NQL, (k + 1) * 18 // NQL)), LDL)
            elif tok[0] == 'l':
                _, t0, dt = tok.split('+')

                def left(which, dep):
                    assert len(lns) == 2 and not any(st['left'] for st in lns)
                    staged.update(which)
                    a_left(which, dep)
                    return st_s[0, pl.ds(zero8, 8), :]
                for k in range(NLEFT):
                    clock.add_due(clock.t + int(t0) + k * int(dt),
                                  functools.partial(left, range(k * 15 // NLEFT, (k + 1) * 15 // NLEFT)), LDL)
            elif tok[0] == 'c':
                _, t0, dt = tok.split('+')
                assert pg == 2 * NCH

                def place(k, dep):
                    assert k in staged
                    a_arrange(k, dep)
                for k in range(15):
                    clock.add(clock.t + int(t0) + k * int(dt), functools.partial(place, k))
            else:
                n, t0, dt = tok[1:].split('+')
                for k in range(int(n)):
                    add_rows(clock, clock.t + int(t0) + k * int(dt), an + nrows // nr, nrows // nr, nrows % nr,
                             RG + (RDL, JDL))
                    nrows += 1
        assert pg == pd and not clock.pending()
        for t in range(2):
            y = jnp.concatenate([_ssum([(acc[k], sg) for k, sg in _HK_C[i, t]]) for i in range(3)], axis=0)
            x2 = xres[b0 + t] + 0.5 * y
            xres[b0 + t] = x2
            xin[j % NP, :, t * TB:(t + 1) * TB] = x2.astype(bf16)

    if last:
        ffn(2 * NP - 1, g * NPC, SCRIPT_F)
        return
    assert NCH == NP - 2

    late = [(c, m) for c in range(NCH) for m in range(3) if c >= NCH - LAGS[m]]

    def prologue():
        cp_x(0).start()
        for sec in range(3):
            for cp in cp_qkv(sec):
                cp.start()
        qall[:, pl.ds(0, HALO), :] = jnp.zeros((16, HALO, 128), f32)
        cp_x(0).wait()
        for t in range(2):
            x = xin[0, :, t * TB:(t + 1) * TB].astype(f32)
            xres[t] = x
            mean, rstd = _ln_stats(x)
            xn_g[t, pl.ds(zero8, D), :] = (xres[t] - mean) * rstd
        q_left(True)
        for sec in range(3):
            for cp in cp_qkv(sec):
                cp.wait()
            if sec == 0:
                cp_x(1).start()
                cp_x(2).start()
                cp_wo().start()
                for c in range(NCH):
                    if 3 + c < NP:
                        cp_x(3 + c).start()
                    for m in range(3):
                        if c == 0 or c > LAGS[m]:
                            cp_unit(max(c - LAGS[m], 0), m).start()
                for c, m in late:
                    cp_unit(c, m).start()
            transpose_qkv(sec)
            build_wq(sec)

    def first_attention():
        cp_x(2).wait()
        q_step(1, CFG_QA, rows=True)
        cp_wo().wait()
        build_wo()
        wo_mm(0, wo_rhs(0))

    def startup_step(c, carry):
        @pl.when(c + 3 < NP)
        def _():
            cp_x(c + 3).wait()
        for m in range(3):
            if LAGS[m]:
                @pl.when(jnp.logical_or(c == 0, c > LAGS[m]))
                def _():
                    cp_unit(jnp.maximum(c - LAGS[m], 0), m).wait()
            else:
                cp_unit(c, m).wait()
        q_step(c + 2, CFG_Q1, chunk=c)
        return carry

    def startup_tail():
        pieces = []
        for c, m in late:
            cp_unit(c, m).wait()
            pieces += prep_pieces(c, m)
        npt = 15 + 2 * TLN
        done = []

        def pace(v):
            pw[0, pl.ds(R_END + zero8, 8), 0:128] = v
            done.append(v)
            for piece in pieces[(len(done) - 1) * len(pieces) // npt:len(done) * len(pieces) // npt]:
                piece()
        for t in range(2):
            mean, rstd = _ln_stats(xres[t])
            xn = (xres[t, pl.ds(zero8, D), :] - mean) * rstd
            xn_f[t] = xn
            for k in range(TLN):
                pace(pltpu.bitcast(xn[k * 64:k * 64 + 8], u32))
        a_left(cb=pace)
        assert len(done) == npt

    @pl.when(g == 0)
    def _():
        prologue()
        cp_x(1).wait()
        q_step(0, CFG_Q0, sums=True)
        first_attention()
        lax.fori_loop(0, NCH, startup_step, 0)
        startup_tail()

    @pl.when(g >= NP - 1)
    def _():
        q_step(g - (NP - 1))

    ffn(g, 0, SCRIPT)

    @pl.when(g >= NP)
    def _():
        _cp_out(g - NP, o_hbm, xin, sems).start()


def _cp_out(k, o_hbm, xin, sems):
    return pltpu.make_async_copy(xin.at[k], o_hbm.at[:, pl.ds(_al(k * 2 * TB, 128), 2 * TB)], sems.at[4 + k])


def _kernel(*refs, D, DF, S):
    def body(last, g, carry):
        _step(g, last, *refs, D=D, DF=DF, S=S)
        return carry
    NP = S // (2 * TB)
    lax.fori_loop(0, 2 * NP - 1, functools.partial(body, False), 0)
    lax.fori_loop(0, 2, functools.partial(body, True), 0)
    o_hbm, xin, sems = refs[6], refs[7], refs[24]
    _cp_out(NP - 1, o_hbm, xin, sems).start()
    for k in range(NP):
        _cp_out(k, o_hbm, xin, sems).wait()


@jax.jit
def pallas_interleave_layers__sliding_local_dilated__glu_gated_geglu__prompt_kernel(
    A_x, A_wqkv, A_wo, B_x, B_w_gate, B_w_up, B_w_down):
    B, S, D = A_x.shape
    DF = B_w_gate.shape[1]
    NB = S // TB
    NP = NB // 2
    NCH = DF // CW
    xT = A_x.reshape(S, D).T
    wdT = B_w_down.T
    hbm = pl.BlockSpec(memory_space=pltpu.HBM)
    outT = pl.pallas_call(
        functools.partial(_kernel, D=D, DF=DF, S=S),
        in_specs=[hbm] * 6,
        out_specs=hbm,
        out_shape=jax.ShapeDtypeStruct((D, S), A_x.dtype),
        scratch_shapes=[
            pltpu.VMEM((NP, D, 2 * TB), bf16),
            pltpu.VMEM((D, 3 * D), bf16),
            pltpu.VMEM((D, D), bf16),
            pltpu.VMEM((5, 14 * 128, 128), f32),
            pltpu.VMEM((WQR, 27 * 128), u32),
            pltpu.VMEM((D // 2, 640), u32),
            pltpu.VMEM((D // 4, 18 * 128), u32),
            pltpu.VMEM((NCH, 3, D, CW), bf16),
            pltpu.VMEM((NCH, 45 * (TC // 2) + 15 * (D // 6) + 16, 2 * TC), u32),
            pltpu.VMEM((16, S + QPAD, 128), f32),
            pltpu.VMEM((11, TB, 128), f32),
            pltpu.VMEM((NB, D, TB), f32),
            pltpu.VMEM((2, D, TB), f32),
            pltpu.VMEM((2, D, TB), f32),
            pltpu.VMEM((45, TB // 2, TC), u32),
            pltpu.VMEM((31, TB // 2, TC), u32),
            pltpu.VMEM((18, TB // 2, TC), u32),
            pltpu.SemaphoreType.DMA((4 + NP + 3 * NCH,)),
        ] + [pltpu.VMEM((TB, 2 * TC), f32)] * 29,
        compiler_params=pltpu.CompilerParams(
            vmem_limit_bytes=110 * 1024 * 1024,
            disable_bounds_checks=True,
            disable_semaphore_checks=True,
        ),
    )(xT, A_wqkv, A_wo, B_w_gate, B_w_up, wdT)
    return outT.T.reshape(B, S, D)
```

```python
import functools
import math
import jax
import jax.numpy as jnp
from jax import lax
import jax.experimental.pallas as pl
import jax.experimental.pallas.tpu as pltpu

DH = 18
W = 8
DIL = 2
HALO = 16
EPS = 1e-5
TB = 128
RB = 8
TC = 128
CW = 6 * TC
WQR = 320
KY = 64
QPAD = 40

SCRIPT = ('m0+50,m1+2804,k+8550+68,G,R7+74+200,G,G,R2+96+200,G,R9+300+260,D4,'
          'G,R7+74+200,G,G,R7+74+200,G,G,W,n0+300,n1+876,l+2900+80,G,G,G,c+600+192,D8').split(',')
SCRIPT_F = 'G,G,G,G,G,G,D6'.split(',')
GU_ORD = (8, 6, 7, 11, 3, 1, 10, 14, 9, 5, 0, 13, 12, 4, 2)
ORD6 = (0, 4, 3, 1, 5, 2)
WORD = (0, 1, 2, 6, 7, 8, 9, 10, 11, 12, 13, 14, 3, 4, 5)
PLAG, DADV, GTK, DTK, QTK = 6, 2, 2, 2, 8
LNJ = (12, 9, 48, 48)
RG = (2, 1, 24, 420)
RDL, JDL, LDL = 600, 300, 500
NLEFT, NQL, TLN, NHS = 15, 18, 8, 4
CFG_Q0 = (40, 1816, 18, 18, 48, 48, 350)
CFG_QA = (300, 748, 6, 6, 32, 64, 350)
CFG_Q1 = (40, 1456, 9, 9, 64, 64, 300)
QA_T = (300, 1000, 4, 3850)
QP0, QP1, QFR = 100, 3850, 0.6
DCUT = (0, 2, 4, 6, 8, 10, 12, 21, 30, 39, 48, 57)
LAGS = (1, 1, 0)

f32 = jnp.float32
bf16 = jnp.bfloat16
u32 = jnp.uint32
NT = (((1,), (1,)), ((), ()))


def _al(i, n):
    return i if isinstance(i, int) else pl.multiple_of(i, n)


def _lt(k):
    return slice(k * 128, (k + 1) * 128)


def _pk(x):
    return pltpu.bitcast(x.astype(bf16), u32)


def _up(x):
    return pltpu.bitcast(x, bf16)


def _dot(a, b):
    return jnp.dot(a, b, preferred_element_type=f32)


def _dot_nt(a, b):
    return lax.dot_general(a, b, NT, preferred_element_type=f32)


def _tree(fn, xs):
    xs = list(xs)
    while len(xs) > 1:
        xs = [fn(xs[i], xs[i + 1]) for i in range(0, len(xs) - 1, 2)] + ([xs[-1]] if len(xs) % 2 else [])
    return xs[0]


def _ln_stats(x, nacc=4):
    n = x.shape[0]
    c = x[0:1]
    s1 = [None] * nacc
    s2 = [None] * nacc
    for i in range(n // 8):
        d = x[i * 8:(i + 1) * 8] - c
        k = i % nacc
        s1[k] = d if s1[k] is None else s1[k] + d
        dd = d * d
        s2[k] = dd if s2[k] is None else s2[k] + dd
    m = jnp.sum(_tree(jnp.add, s1), axis=0, keepdims=True) * (1.0 / n)
    v = jnp.sum(_tree(jnp.add, s2), axis=0, keepdims=True) * (1.0 / n) - m * m
    v = jnp.maximum(v, 0.0)
    return c + m, lax.rsqrt(v + EPS)


_HK_A = (
    ((0, 0, 1), (0, 2, -1), (1, 0, -1)), ((0, 0, 1), (0, 1, -1), (2, 0, -1)), ((1, 1, 1), (0, 1, -1), (1, 2, -1)),
    ((1, 1, 1), (1, 0, -1), (2, 1, -1)), ((2, 2, 1), (0, 2, -1), (2, 1, -1)), ((2, 2, 1), (1, 2, -1), (2, 0, -1)),
    ((0, 1, 1),), ((0, 1, 1), (1, 0, -1)), ((1, 0, 1),),
    ((0, 2, 1),), ((0, 2, 1), (2, 0, -1)), ((2, 0, 1),),
    ((1, 2, 1),), ((2, 1, 1), (1, 2, -1)), ((2, 1, 1),),
)
_HK_C = {
    (0, 0): ((0, 1), (7, 1), (8, 1), (9, 1), (6, -1)),
    (0, 1): ((1, 1), (6, 1), (10, 1), (11, 1), (9, -1)),
    (1, 0): ((2, 1), (7, 1), (8, 1), (12, 1), (6, -1)),
    (1, 1): ((3, 1), (6, 1), (13, 1), (14, 1), (2, -1), (7, -1)),
    (2, 0): ((5, 1), (9, 1), (12, 1), (13, 1), (4, -1), (10, -1)),
    (2, 1): ((4, 1), (10, 1), (11, 1), (14, 1), (9, -1)),
}
_HK_B = (((0, 0, 1),), ((0, 1, 1),), ((1, 0, 1),), ((1, 0, 1), (1, 1, 1)), ((2, 1, 1),), ((2, 0, 1), (2, 1, 1)),
         ((0, 1, 1), (1, 1, 1)), ((0, 1, 1), (1, 0, 1), (1, 1, 1)), ((0, 0, 1), (0, 1, 1), (1, 0, 1), (1, 1, 1)),
         ((0, 0, 1), (2, 0, 1)), ((0, 0, 1), (2, 0, 1), (2, 1, 1)), ((0, 0, 1), (0, 1, 1), (2, 0, 1), (2, 1, 1)),
         ((1, 0, 1), (2, 0, 1)), ((1, 0, 1), (2, 1, -1)), ((1, 1, 1), (2, 1, 1)))


_HK6 = (
    '+00-01-02-30-50 +00 +00;+00-03+05-10-20 +01 +01;-01+11+13-15-40+41 +11 -10+11;-04-10+11+14+31+51 +12 +10;'
    '-02-12+21+22-23-25+35-42 +21 -20+21;-12-20+21+22+24-32-52+53 +22 +20;-03+31-32+33+43 +30 +30-31;'
    '+13-23-30+33-34 +32 +31;-04+34-40+41+42+44+54 +40 +40;-04+14-24-40-43+44-45 +41 +41;'
    '-05-12+35+45-51-52+53+55 +50 +50-51;+15+21-25+35+50-53-54+55 +52 +51;+01-40 +00+10 +00-01+10-11;'
    '+01-10 +00+12 +01-10+11;-04+10 +02+12 +01+11;+02 +00+20 +00-01+20-21;+02-20 +00+22 +01-20+21;'
    '+20 +02+22 +01+21;+03 +01+31 -00+01-30+31;+03-30 +01+32 +00+30-31;+30 +02+32 +00+30;+05 +01-51 +00-01+50-51;'
    '+05+50 +01-52 -00-50+51;+50 +02-52 +00+50;+31 +10-30 -10+30;+13-31 +11+30 +10-31;+13 +11-31 -11+31;'
    '+40-41 +10-40 +10-11-40+41;+04-14-40+41 +12-40 +10-11+41;+04-14 +12-42 +11-41;+12-51 +10+50 +10-50;'
    '+15+51 +11-50 -10+51;+15-21 +11+51 +11-51;+32+53 +20+30 +20+30;-23+32 +21-30 +20+31;+23-35 +21+31 +21+31;'
    '+42 +20-40 +20-21+40-41;+24+42 +22-40 -20+21+41;+24 +22-42 -21-41;+12+52-53 +20+50 +20+50;'
    '+12+21-25+35+52-53 +21-50 +20+51;-21+25-35 +21+51 +21+51;+43 +31+41 +30-31-40+41;+34+43 +32+41 -30+31+40;'
    '+34 +32+42 +30-40;+45 +41+51 -40+41+50-51;+45+54 +41+52 +40-50+51;+54 +42+52 -40+50;'
    '+40 +01+11+41 -00+01-10+11-40+41;-04+40 +02+12+41 +00-01+10-11+40;+04 +02+12+42 +00+10+40;'
    '+12 +10-20+50 -10+11-20+21+50-51;+12+21 +10-22+50 -11+20-21+51;+21 +12-22+52 +11+21-51;'
    '+35 +21+31+51 -20+21-30+31+50-51;+35+53 +21+31+52 +20+30-50+51;+53 +22+32+52 -20-30+50'
)


def _terms(txt):
    return tuple((int(txt[i + 1]), int(txt[i + 2]), 1 if txt[i] == '+' else -1) for i in range(0, len(txt), 3))


_A6, _B6, _Z6 = zip(*[[_terms(f) for f in row.split(' ')] for row in _HK6.split(';')])
_C6 = {(i, t): [(n, sg) for n, z in enumerate(_Z6) for i_, t_, sg in z if (i_, t_) == (i, t)]
       for i in range(6) for t in range(2)}


def _order6():
    early = [n for n, b in enumerate(_B6) if all(j % 3 == 0 or (j % 3 == 1 and d == 1) for j, d, _ in b)]
    early.sort(key=lambda n: max(d != 1 for _, d, _ in _B6[n]))
    out = list(early)
    for i in ORD6:
        out += [n for n, z in enumerate(_Z6) if n not in out and any(i_ == i for i_, _, _ in z)]
    return out


def _ssum(terms):
    terms = sorted(terms, key=lambda z: -z[1])
    acc = terms[0][0] if terms[0][1] == 1 else -terms[0][0]
    for v, sg in terms[1:]:
        acc = acc + v if sg == 1 else acc - v
    return acc


GU_POST = {
    8: ((), ('p8', None), None),
    7: ((('p8', 1),), (None, 't7'), None),
    3: ((('t7', 1),), (None, 's1'), None),
    6: ((), ('p6', None), None),
    14: ((('p6', 1), ('s1', 1)), ('p14', None), (1, 1)),
    12: ((('p9', 1), ('s2', 1)), ('p12', None), (2, 0)),
    13: ((), ('p13', None), None),
    2: ((('p12', 1), ('p13', 1), ('s1', 1)), (None, None), (1, 0)),
    11: ((), ('p11', None), None),
    10: ((('p11', 1),), (None, 't10'), None),
    5: ((('t10', 1),), (None, 's2'), None),
    9: ((), ('p9', None), None),
    4: ((('p14', 1), ('s2', 1), ('p13', -1)), (None, None), (2, 1)),
    0: ((('p8', 1), ('p9', 1), ('t10', 1)), (None, None), (0, 0)),
    1: ((('p6', 1), ('p11', 1), ('t7', 1)), (None, None), (0, 1)),
}
PSLOT = {k: i for i, k in enumerate(('p8', 't7', 's1', 'p6', 'p14', 'p12', 'p13', 'p11', 't10', 's2', 'p9'))}


class _Timeline:
    def __init__(self):
        self.t = 0
        self.jobs = []
        self.due = []

    def add(self, when, fn):
        self.jobs.append((when, len(self.jobs), fn))
        self.jobs.sort(key=lambda z: z[:2])

    def add_due(self, when, job, delay):
        def run(dep):
            val = job(dep)
            if val is not None:
                self.add(self.t + delay, lambda _: self.due.append(lambda: val))
        self.add(when, run)

    def pending(self):
        return [j for j in self.jobs if getattr(j[2], '__name__', '') != '<lambda>']

    def tick(self, dur, v, n):
        for k in range(n):
            self.t += dur // n
            r = k * (v.shape[0] // n)
            while self.jobs and self.jobs[0][0] <= self.t:
                self.jobs.pop(0)[2](v[r:r + 8, 0:128])


def _step(g, last, x_hbm, wqkv_hbm, wo_hbm, wg_hbm, wu_hbm, wd_hbm, o_hbm,
          xin, wqkv_raw, wo_raw, tmp, wq, woT, wo2, raw, pw, qall, o_s, xres, xn_f, xn_g, s_scr, st_s, sq_scr,
          sems, *p_s, D, DF, S):
    NB = S // TB
    NP = NB // 2
    NCH = DF // CW
    NPC = NCH // 2
    D3 = D // 3
    D6 = D // 6
    nr = TB // RB
    hh = D // 4
    zero8 = pl.multiple_of((g >> 20) * 8, 8)
    zvec = jnp.full((8, 128), (g >> 20).astype(u32), u32)

    def zero(k):
        return pl.multiple_of((g >> (8 + k)) * 8, 8)

    def tie(x, dep):
        return pltpu.bitcast(pltpu.bitcast(x, u32) | (pltpu.bitcast(dep, u32) & zvec), f32)

    def gate(lhs, clock):
        if not clock.due:
            return lhs
        pr = _tree(jnp.bitwise_or, [k() for k in clock.due]) & zvec
        del clock.due[:]
        return jnp.concatenate([lhs[0:8] | pr, lhs[8:]], axis=0)

    QSEC = ((0, 5), (5, 9), (9, 14))

    def cp_qkv(sec):
        out = []
        for j in range(*QSEC[sec]):
            n = min(128, 3 * D - j * 128)
            out.append(pltpu.make_async_copy(wqkv_hbm.at[:, pl.ds(j * 128, n)], wqkv_raw.at[:, pl.ds(j * 128, n)],
                                             sems.at[sec]))
        return out

    def cp_wo():
        return pltpu.make_async_copy(wo_hbm, wo_raw, sems.at[3])

    def cp_x(k):
        return pltpu.make_async_copy(x_hbm.at[:, pl.ds(_al(k * 2 * TB, 128), 2 * TB)], xin.at[k], sems.at[4 + k])

    def cp_unit(c, m):
        return pltpu.make_async_copy((wg_hbm, wu_hbm, wd_hbm)[m].at[:, pl.ds(_al(c * CW, 128), CW)], raw.at[c, m],
                                     sems.at[4 + NP + 3 * c + m])

    R_SD = 45 * (TC // 2)
    R_END = R_SD + 15 * (D3 // 2)

    def hk_a_ops(load, minus=None):
        blk = {}
        for i in range(3):
            for j in range(3):
                blk[i, j] = load(i, j).astype(f32)
                if minus is not None:
                    blk[i, j] = blk[i, j] - minus(i, j).astype(f32)
        return [_pk(_ssum([(blk[i, j], sg) for i, j, sg in terms])) for terms in _HK_A]

    def prep_pieces(c, m):
        def ld(r, cs):
            return lambda i, j: raw[c, m, pl.ds(i * D3 + r, 16), pl.ds((3 * cs + j) * TC, TC)]

        def gu_piece(q, r, cs, neg, kind, half):
            ops = hk_a_ops(ld(q * KY + r, cs), None if neg is None else ld(q * KY + r, neg))
            for k, t in enumerate(ops):
                pw.at[c][pl.ds((3 * k + kind) * (TC // 2) + (half * KY + r) // 2, 8), m * TC:(m + 1) * TC] = t

        def d_piece(r, q, ks):
            blk = {}
            z = pl.multiple_of(zero(q) * 2, 16)
            for k in ks:
                for i, j, _ in _A6[k]:
                    if (i, j) not in blk:
                        blk[i, j] = raw[c, m, pl.ds(z + i * D6 + r, 16), pl.ds(j * TC, TC)].astype(f32)
                pw.at[c][pl.ds(R_SD + (k // 2) * (D6 // 2) + r // 2, 8), _lt(k % 2)] = _pk(
                    _ssum([(blk[i, j], sg) for i, j, sg in _A6[k]]))
        if m == 2:
            return [functools.partial(d_piece, r, q, range(DCUT[q], DCUT[q + 1]))
                    for r in range(0, D6, 16) for q in range(len(DCUT) - 1)]
        spec = ((0, 0, None, 0, 0), (1, 0, 1, 0, 1), (0, 1, None, 1, 0), (2, 1, 0, 1, 1),
                (2, 0, None, 2, 0), (1, 1, None, 2, 1))
        return [functools.partial(gu_piece, q, r, cs, neg, kind, half)
                for r in range(0, KY, 16) for q, cs, neg, kind, half in spec]

    def transpose_qkv(sec):
        for j in range(*QSEC[sec]):
            wd_ = min(128, 3 * D - j * 128)
            blk = wqkv_raw[:, j * 128:j * 128 + wd_].astype(f32)
            if wd_ < 128:
                blk = jnp.concatenate([blk, jnp.zeros((D, 128 - wd_), f32)], axis=1)
            bt = jnp.concatenate([blk, blk[D - KY:]], axis=0).T
            for t in range(5):
                tmp[t, pl.ds(j * 128, 128), :] = bt[:, t * 128:(t + 1) * 128]

    def wq_slot(i, j):
        return 24 + i if i == j else [n for n, t in enumerate(_HK_A) if t == ((i, j, 1),)][0]

    def build_wq(sec):
        lo = lax.broadcasted_iota(jnp.int32, (32, 128), 1) < KY
        for d in range(DH):
            tt = [tmp[t, pl.ds(sec * D + d, 32, stride=DH), :] for t in range(5)]
            ops = tt[:4] + [jnp.where(lo, tt[3], tt[4]), jnp.where(lo, tt[4], tt[3])]
            if d < 16:
                dst = [(sec, d * 16)]
            else:
                dst = ([(1, (d + 2) * 16)], [(1, d * 16)], [(0, d * 16), (0, (d + 2) * 16)])[sec]
            for j, row in dst:
                for k, v in enumerate(ops):
                    wq[pl.ds(row, 16), _lt(wq_slot(k, j) if k < 3 else 12 + 3 * j + k)] = _pk(v)

    def wq_sums(r, dep):
        ncol = 3 if r < 256 else 2
        pin = pltpu.bitcast(dep, u32) & zvec
        blk = {(i, j): _up(wq[pl.ds(r, 8), _lt(wq_slot(i, j))] | pin).astype(f32) for i in range(3) for j in range(ncol)}
        for n, terms in enumerate(_HK_A):
            if len(terms) > 1 and not (ncol == 2 and n in (4, 5)):
                wq[pl.ds(r, 8), _lt(n)] = _pk(_ssum([(blk[i, j], sg) for i, j, sg in terms if j < ncol]))

    def build_wo():
        for t in range(5):
            wd_ = min(128, D - t * 128)
            blk = wo_raw[:, t * 128:t * 128 + wd_].astype(f32)
            if wd_ < 128:
                blk = jnp.concatenate([blk, jnp.zeros((D, 128 - wd_), f32)], axis=1)
            tmp[t, pl.ds(0, D), :] = blk
        for t in range(5):
            rows = [tmp[t, pl.ds(d, 32, stride=DH), :] for d in range(DH)]
            ft = jnp.concatenate(rows + rows[16:], axis=0).T
            n = min(128, D - t * 128)
            woT[pl.ds(t * 64, n // 2), :] = _pk(ft[:n])
        for r in range(0, D3 // 2, 8):
            ops = hk_a_ops(lambda i, j: _up(woT[pl.ds(i * (D3 // 2) + r, 8), j * TC:(j + 1) * TC]))
            for k, t in enumerate(ops):
                wo2[pl.ds(r, 8), _lt(k)] = t
        lo = lax.broadcasted_iota(jnp.int32, (16, 128), 1) < KY
        for r in range(0, hh, 8):
            a3, a4, b3, b4 = [_up(woT[pl.ds(r0 + r, 8), c0:c0 + 128]).astype(f32)
                              for r0 in (0, hh) for c0 in (384, 512)]
            wo2[pl.ds(r, 8), _lt(15)] = _pk(jnp.where(lo, a3, a3 - b3))
            wo2[pl.ds(r, 8), _lt(16)] = _pk(jnp.where(lo, b3, b4 - a4))
            wo2[pl.ds(r, 8), _lt(17)] = _pk(jnp.where(lo, a4, b3))

    def q_left(plain, which=None, dep=None):
        k1, k2, k3 = 3 * TC, 3 * TC + KY, 3 * TC + 2 * KY
        for n in (list(range(6 if plain else 15)) + [15, 16, 17]) if which is None else which:
            def X(t, r0, rows):
                return xn_g[t, pl.ds((zero8 if plain else zero(n)) + r0, rows), :]
            if n == 15:
                v = jnp.concatenate([X(0, k1, KY), X(0, k2, KY) - X(1, k2, KY)], axis=0)
            elif n == 16:
                v = jnp.concatenate([X(1, k1, KY), X(1, k3, KY) - X(0, k3, KY)], axis=0)
            elif n == 17:
                v = jnp.concatenate([X(0, k3, KY), X(1, k2, KY)], axis=0)
            elif plain:
                v = X(n // 3, (n % 3) * TC, TC)
            else:
                v = _ssum([(X(t, i * TC, TC), sg) for (i, t), lst in _HK_C.items() for k, sg in lst if k == n])
            if dep is not None:
                v = jnp.concatenate([tie(v[0:8], dep), v[8:]], axis=0)
            sq_scr[n] = pltpu.bitcast(v.astype(bf16).T, u32)

    def add_ln(clock, t0, cfg, blk, dst, par, inp=None):
        np1, np2, step, gap, delay = cfg
        st = dict(s1=[], s2=[], left=np2)
        nv = D // 16

        def load(i):
            if inp is None:
                return xres[blk, pl.ds(zero8 + i * 16, 16), :]
            x = inp(i).astype(f32)
            xres[blk, pl.ds(i * 16, 16), :] = x
            return x

        def stats(k, dep):
            xs = []
            for i in range(k * nv // np1, (k + 1) * nv // np1):
                x = load(i)
                xs += [x[0:8], x[8:16]]
            if k == 0:
                st['c'] = jnp.broadcast_to(xs[0][0:1], (8, TB))
            c = tie(st['c'], dep)
            ds = [x - c for x in xs]
            st['s1'].append(_tree(jnp.add, ds))
            st['s2'].append(_tree(jnp.add, [d * d for d in ds]))
            return pltpu.bitcast(st['s1'][-1], u32) | pltpu.bitcast(st['s2'][-1], u32)

        def norm(k, dep):
            if k == 0:
                m = jnp.sum(_tree(jnp.add, st['s1']), axis=0, keepdims=True) * (1.0 / D)
                v = jnp.sum(_tree(jnp.add, st['s2']), axis=0, keepdims=True) * (1.0 / D) - m * m
                st['mean'] = st['c'] + m
                st['rstd'] = jnp.broadcast_to(lax.rsqrt(jnp.maximum(v, 0.0) + EPS), (8, TB))
            mean = tie(st['mean'], dep)
            off = 0 if inp is None else zero8
            for i in range(k * 2 * nv // np2, (k + 1) * 2 * nv // np2):
                dst[par, pl.ds(i * 8, 8), :] = (xres[blk, pl.ds(off + i * 8, 8), :] - mean) * st['rstd']
            st['left'] -= 1
            return pltpu.bitcast(dst[par, pl.ds(zero8, 8), :], u32)
        for k in range(np1):
            clock.add_due(t0 + k * step, functools.partial(stats, k), delay)
        for k in range(np2):
            clock.add_due(t0 + np1 * step + gap + k * step, functools.partial(norm, k), delay)
        return st

    def hk_outputs(P, T, PT, emit, two_cols):
        p8 = P(8)
        t7 = P(7) + p8
        s1 = PT(3, 1, 2) + t7
        p6 = P(6)
        p14 = P(14)
        emit(1, 1, T(1, 1) + (p6 + p14 + s1))
        p13 = P(13)
        if two_cols:
            emit(1, 0, PT(2, 1, 0) + (p13 + s1))
        else:
            p12 = P(12)
            emit(1, 0, PT(2, 1, 0) + (p12 + p13 + s1))
        p11 = P(11)
        t10 = P(10) + p11
        if not two_cols:
            s2 = PT(5, 2, 2) + t10
            p9 = P(9)
            emit(2, 0, T(2, 0) + (p9 + p12 + s2))
            emit(2, 1, PT(4, 2, 1) + (p14 - p13 + s2))
        w0 = T(0, 2)
        emit(0, 0, PT(0, 0, 0) + ((p8 + t10 + w0) if two_cols else (p8 + p9 + t10 + w0)))
        emit(0, 1, PT(1, 0, 1) + (p6 + p11 + t7 + w0))

    QT = (0, 1, 2, 3)
    KT = (4, 5, 6, 7, 13)
    VT = (8, 9, 10, 11, 12)
    c2e = DH ** -0.5 * math.log2(math.e)
    neg = -1e9 * math.log2(math.e)

    def q_step(pr, cfg=None, chunk=None, rows=False, sums=False):
        first = cfg is not None
        clock = _Timeline()
        if sums:
            base, nx = 0, 1
            for k in range(40):
                clock.add(200 + k * 90, functools.partial(wq_sums, 8 * k))
        elif rows:
            base, nx = pr * (2 * TB), pr + 1
            for k in range(2):
                clock.add_due(QA_T[k], functools.partial(row_chain, k, QA_T[2]), QA_T[3] - QA_T[k])
        else:
            base = pl.multiple_of(pr * (2 * TB), 2 * TB)
            nx = jnp.minimum(pr + 1, NP - 1)
        pieces = []
        if chunk is not None:
            for m in range(3):
                pieces += prep_pieces(jnp.maximum(chunk - LAGS[m], 0) if LAGS[m] else chunk, m)

        def paced(piece, dep):
            pw[0, pl.ds(R_END, 8), 0:128] = pltpu.bitcast(dep, u32)
            piece()
        for k, piece in enumerate(pieces):
            frac = k / 48 * QFR if k < 48 else QFR + (k - 48) / (len(pieces) - 48) * (1 - QFR)
            clock.add(QP0 + int(frac * (QP1 - QP0)), functools.partial(paced, piece))
        if first:
            for par in range(2):
                add_ln(clock, cfg[par], cfg[2:], 2 * nx + par, xn_g, par,
                       functools.partial(lambda par_, i: xin[nx, pl.ds(i * 16, 16), par_ * TB:(par_ + 1) * TB], par))
        for r0, nt, tiles in ((0, 2, (0, 4, 8)), (TC, 2, (2, 6, 10)), (2 * TC, 1, (12, 13))):
            def R(k):
                return wq[pl.ds(r0, nt * 64), _lt(k)]

            def P(k):
                return _dot_nt(_up(sq_scr[k]), _up(R(k)))

            def T(j, kind):
                rhs = _up(R(15 + 3 * j + kind))
                if nt == 1 and kind == 2:
                    nq = 2 if first else 4
                    return jnp.concatenate([_dot_nt(_up(sq_scr[15 + kind, pl.ds(k * (64 // nq), 64 // nq), :]), rhs)
                                            for k in range(nq)], axis=0)
                return _dot_nt(_up(sq_scr[15 + kind]), rhs)

            def PT(k, j, kind):
                return _dot_nt(_up(jnp.concatenate([sq_scr[k], sq_scr[15 + kind]], axis=1)),
                               _up(jnp.concatenate([R(k), R(15 + 3 * j + kind)], axis=1)))

            def emit(col, half, v):
                for k in range(nt):
                    qall[tiles[col] + k, pl.ds(base + (HALO + half * TB), TB), :] = v[:, k * 128:(k + 1) * 128]
            if not first:
                hk_outputs(P, T, PT, emit, nt == 1)
                continue
            for j in range(len(tiles)):
                both = T(j, 2)
                clock.t += 32 * nt
                for t in range(2):
                    for k in range(nt):
                        lhs = [sq_scr[3 * t + i] for i in range(3)] + [sq_scr[15 + t]]
                        lhs[0] = gate(lhs[0], clock)
                        rhs = [wq[pl.ds(r0 + k * 64, 64), _lt(n)]
                               for n in [wq_slot(i, j) for i in range(3)] + [15 + 3 * j + t]]
                        v = _dot_nt(_up(jnp.concatenate(lhs, axis=1)), _up(jnp.concatenate(rhs, axis=1))) + both[:, _lt(k)]
                        qall[tiles[j] + k, pl.ds(base + (HALO + t * TB), TB), :] = v
                        clock.tick(128, v, QTK)
        assert not clock.pending()
        if first:
            q_left(True)

    def row_group(blk, par, r, nw, nv, mids=None):
        base = _al(blk * TB, TB)
        lo = lax.broadcasted_iota(jnp.int32, (RB, 128), 1) < KY
        r0 = r * RB

        def ld(t, w):
            return qall[t, pl.ds(base + (HALO + r0 - DIL * w), RB), :]
        dep = yield
        cs = tie(jnp.full((RB, 128), c2e, f32), dep)
        q = [ld(t, 0) * cs for t in QT] + [jnp.where(lo, pltpu.roll(ld(13, 0), KY, 1), 0.0) * cs]
        sc = []
        for w in range(W):
            if w and w % nw == 0:
                dep = yield
                q = [tie(q[0], dep)] + q[1:]
            acc = None
            for j, t in enumerate(KT):
                p = q[j] * ld(t, w)
                acc = p if acc is None else acc + p
            acc = acc + pltpu.roll(acc, 64, 1)
            if mids is not None:
                mids[r] = pltpu.bitcast(acc, u32)
            acc = acc + pltpu.roll(acc, 32, 1)
            if r0 - DIL * w < 0:
                pos = blk * TB + r0 + lax.broadcasted_iota(jnp.int32, (RB, 128), 0)
                acc = jnp.where(pos >= DIL * w, acc, neg)
            sc.append(acc)
        m = _tree(jnp.maximum, sc)
        e = [jnp.exp2(sc[w] - m) for w in range(W)]
        l = _tree(jnp.add, e)
        rinv = pl.reciprocal(l, approx=True)
        rinv = rinv * (2.0 - l * rinv)
        outs = []
        for j, t in enumerate(VT):
            if j and j % nv == 0:
                dep = yield _tree(jnp.bitwise_or, [pltpu.bitcast(v, u32) for v in outs])
                outs = []
                e = [tie(e[0], dep)] + e[1:]
            acc = None
            for w in range(W):
                p = e[w] * ld(t, w)
                acc = p if acc is None else acc + p
            o = acc * rinv
            o_s[par * 5 + j, pl.ds(r0, RB), :] = o
            outs.append(o)
        yield _tree(jnp.bitwise_or, [pltpu.bitcast(v, u32) for v in outs])

    def add_rows(clock, t0, blk, par, r, cfg):
        nw, nv, step, gap, d1, d2 = cfg
        gen = row_group(blk, par, r, nw, nv)
        next(gen)
        n1, n2 = -(-W // nw), -(-5 // nv)
        for k in range(n1):
            clock.add_due(t0 + k * step, gen.send, d1)
        for k in range(n2 - 1):
            clock.add_due(t0 + (n1 - 1) * step + gap + k * step, gen.send, d2)

    def row_chain(blk, lag, dep):
        mids, fins = {}, {}
        for r in range(nr):
            gen = row_group(blk, blk, r, W, 5, mids)
            next(gen)
            if r:
                dep = pltpu.bitcast(mids[r - 1] | fins[r - lag] if r >= lag else mids[r - 1], f32)
            fins[r] = gen.send(dep)
        return _tree(jnp.bitwise_or, [fins[r] for r in range(nr - lag, nr)])

    wo_seq = []
    for pos, k in enumerate(WORD):
        if pos in (0, 2):
            wo_seq += [('r', pos // 2, k_) for k_ in range(3)]
        wo_seq.append(('p', k))

    def wo_rhs(off):
        lo = lax.broadcasted_iota(jnp.int32, (TB, 128), 1) < KY

        rhs = {}
        for it in wo_seq:
            z = zero(wo_seq.index(it)) if off is None else off

            def O(t, j):
                return o_s[t * 5 + j, pl.ds(z, TB), :]
            if it[0] == 'p':
                v = _ssum([(O(t, j), sg) for j, t, sg in _HK_B[it[1]]])
            elif it[2] == 0:
                v = O(it[1], 3)
            else:
                v = jnp.where(lo, O(it[1], 2 + it[2]), O(it[1], 5 - it[2]))
            rhs[it] = v.astype(bf16)
        return rhs

    def wo_mm(blk0, rhs):
        res = {}
        for it in wo_seq:
            if it[0] == 'p':
                lhs = wo2[pl.ds(0, D3 // 2), _lt(it[1])]
            else:
                lhs = wo2[:, _lt(15 + it[2])]
            res[it] = _dot_nt(_up(lhs), rhs[it])
        for t in range(2):
            both = res['r', t, 2]
            rem = xres[blk0 + t] + jnp.concatenate([res['r', t, 0] + both, res['r', t, 1] + both], axis=0)
            y = jnp.concatenate([_ssum([(res['p', k], sg) for k, sg in _HK_C[i, t]]) for i in range(3)], axis=0)
            xres[blk0 + t] = y + rem

    def a_left(which=range(15), dep=None, cb=None):
        for n in which:
            v = _ssum([(xn_f[t, pl.ds(zero(n) + i * D3, D3), :], sg)
                       for (i, t), lst in _HK_C.items() for k, sg in lst if k == n])
            if dep is not None:
                v = jnp.concatenate([tie(v[0:8], dep), v[8:2 * KY], tie(v[2 * KY:2 * KY + 8], dep), v[2 * KY + 8:]],
                                    axis=0)
            t1 = pltpu.bitcast(v[:2 * KY].astype(bf16).T, u32)
            t2 = pltpu.bitcast(jnp.concatenate([v[2 * KY:], v[2 * KY:]], axis=0).astype(bf16).T, u32)
            if dep is None:
                arrange(n, t1, t2)
                cb(t1[0:8])
            else:
                st_s[2 * n] = t1
                st_s[2 * n + 1] = t2

    def arrange(n, t1, t2):
        lo = lax.broadcasted_iota(jnp.int32, (TB // 2, 128), 1) < KY
        s_scr[3 * n] = t1
        s_scr[3 * n + 1] = jnp.where(lo, t1, t2)
        s_scr[3 * n + 2] = jnp.where(lo, t2, t1)

    def a_arrange(n, dep):
        st_s[30, pl.ds(0, 8), :] = pltpu.bitcast(dep, u32)
        arrange(n, st_s[2 * n, pl.ds(zero8, TB // 2), :], st_s[2 * n + 1, pl.ds(zero8, TB // 2), :])

    k0 = math.sqrt(2.0 / math.pi)
    k1 = k0 * 0.044715

    def ffn(j, c0, script):
        clock = _Timeline()
        b0 = (2 * j) % NB
        an = (2 * j + 2) % NB
        acc = [None] * 57
        hs = {}
        lns, lq, staged, nrows = [], [], set(), 0

        pend = []

        def advance(keep):
            while len(pend) > keep:
                pend.pop(0)()

        def written(k):
            clock.due.append(lambda: pltpu.bitcast(p_s[k][pl.ds(zero8, 8), 0:128], u32))

        def gu(p):
            c, m = c0 + p // 2, p % 2
            h = hs.setdefault(p // 2, [[None, None, None] for _ in range(3)])

            def mm(n, kind):
                lhs = gate(s_scr[3 * n + kind], clock)
                return _dot(_up(lhs), _up(pw[c, pl.ds((3 * n + kind) * (TC // 2), TC // 2), m * TC:(m + 1) * TC]))

            def get(name):
                return p_s[PSLOT[name]][pl.ds(zero8, TB), :]

            def post(n, v):
                adds, keep, emits = GU_POST[n]
                if keep[0] is not None:
                    p_s[PSLOT[keep[0]]][...] = v
                    written(PSLOT[keep[0]])
                w_ = v
                for name, sg in adds:
                    w_ = w_ + get(name) if sg == 1 else w_ - get(name)
                if keep[1] is not None:
                    p_s[PSLOT[keep[1]]][...] = w_
                    written(PSLOT[keep[1]])
                if emits is not None:
                    col, half = emits
                    if m == 1:
                        k_ = 17 + 9 * ((p // 2) % NHS) + 3 * col
                        hv = w_ * p_s[11 + 2 * col + half][pl.ds(zero8, TB), :]
                        p_s[k_ + half][...] = hv
                        written(k_ + half)
                        h[col][half] = k_ + half
                        if h[col][1 - half] is not None:
                            p_s[k_ + 2][...] = hv + p_s[k_ + 1 - half][pl.ds(zero8, TB), :]
                            written(k_ + 2)
                            h[col][2] = k_ + 2
                    else:
                        p_s[11 + 2 * col + half][...] = w_ + w_ * jnp.tanh(w_ * (k0 + k1 * (w_ * w_)))
                        written(11 + 2 * col + half)
            for n in GU_ORD:
                both = mm(n, 2)
                v = jnp.concatenate([mm(n, 0) + both, mm(n, 1) + both], axis=1)
                pend.append(functools.partial(post, n, v))
                advance(PLAG)
                clock.tick(96, both, GTK)

        todo = [sum(any(i_ == i for i_, _, _ in z) for z in _Z6) for i in range(6)]

        def gather(i):
            if last:
                ys = [_ssum([(acc[n], sg) for n, sg in sorted(_C6[i, t], key=lambda z: _order6().index(z[0]))])
                      for t in range(2)]
            else:
                t0, t1 = dict(_C6[i, 0]), dict(_C6[i, 1])
                both = _ssum([(acc[n], sg) for n, sg in t0.items() if n in t1])
                ys = (_ssum([(acc[n], sg) for n, sg in t0.items() if n not in t1]) + both,
                      _ssum([(acc[n], sg) for n, sg in t1.items() if n not in t0]) - both)
            for t in range(2):
                x2 = xres[b0 + t, pl.ds(i * D6, D6), :] + 0.5 * ys[t]
                xres[b0 + t, pl.ds(i * D6, D6), :] = x2
                xin[j % NP, pl.ds(i * D6, D6), t * TB:(t + 1) * TB] = x2.astype(bf16)

        def down(ps, final):
            cs = ps[::2]
            hsl = [hs.pop(p // 2) for p in cs]
            for pos, i in enumerate(_order6()):
                while any(h_[j_ % 3][d_] is None for h_ in hsl for j_, d_, _ in _B6[i]):
                    advance(len(pend) - 1)
                au = [pw[c0 + p // 2, pl.ds(R_SD + (i // 2) * (D6 // 2), D6 // 2), _lt(i % 2)] for p in cs]
                au[0] = gate(au[0], clock)
                lhs = jnp.concatenate(au, axis=1)
                rhs = jnp.concatenate([_ssum([(p_s[h_[j_ % 3][d_]][pl.ds(zero(pos % 21), TB), _lt(j_ // 3)], sg)
                                              for j_, d_, sg in _B6[i]]) for h_ in hsl], axis=1).astype(bf16)
                r = _dot_nt(_up(lhs), rhs)
                acc[i] = r if acc[i] is None else r + acc[i]
                if final:
                    for i_ in sorted({i_ for i_, _, _ in _Z6[i]}):
                        todo[i_] -= 1
                        if not todo[i_]:
                            gather(i_)
                if pos % DADV == 0:
                    advance(max(len(pend) - 1, 0))
                clock.tick(24 * len(cs), acc[i], DTK)

        pg = pd = 0
        for tok in script:
            if tok == 'G':
                gu(pg)
                pg += 1
            elif tok[0] == 'D':
                down(list(range(pd, pd + int(tok[1:]))), pd + int(tok[1:]) == script.count('G'))
                pd += int(tok[1:])
            elif tok == 'W':
                assert not clock.pending() and nrows == 2 * nr
                advance(0)
                wo_mm(an, wo_rhs(None))
                clock.t += 1152
            elif tok[0] == 'n':
                lns.append(add_ln(clock, clock.t + int(tok[3:]), LNJ + (JDL,), an + int(tok[1]), xn_f, int(tok[1])))
            elif tok[0] == 'm':
                lq.append(add_ln(clock, clock.t + int(tok[3:]), LNJ + (JDL,), (2 * j + 4) % NB + int(tok[1]), xn_g,
                                 int(tok[1])))
            elif tok[0] == 'k':
                _, t0, dt = tok.split('+')

                def qleft(which, dep):
                    assert len(lq) == 2 and not any(st['left'] for st in lq)
                    q_left(False, which, dep)
                    return sq_scr[which[0], pl.ds(zero8, 8), :]
                for k in range(NQL):
                    clock.add_due(clock.t + int(t0) + k * int(dt),
                                  functools.partial(qleft, range(k * 18 // NQL, (k + 1) * 18 // NQL)), LDL)
            elif tok[0] == 'l':
                _, t0, dt = tok.split('+')

                def left(which, dep):
                    assert len(lns) == 2 and not any(st['left'] for st in lns)
                    staged.update(which)
                    a_left(which, dep)
                    return st_s[0, pl.ds(zero8, 8), :]
                for k in range(NLEFT):
                    clock.add_due(clock.t + int(t0) + k * int(dt),
                                  functools.partial(left, range(k * 15 // NLEFT, (k + 1) * 15 // NLEFT)), LDL)
            elif tok[0] == 'c':
                _, t0, dt = tok.split('+')
                assert pg == 2 * NCH

                def place(k, dep):
                    assert k in staged
                    a_arrange(k, dep)
                for k in range(15):
                    clock.add(clock.t + int(t0) + k * int(dt), functools.partial(place, k))
            else:
                n, t0, dt = tok[1:].split('+')
                for k in range(int(n)):
                    add_rows(clock, clock.t + int(t0) + k * int(dt), an + nrows // nr, nrows // nr, nrows % nr,
                             RG + (RDL, JDL))
                    nrows += 1
        assert pg == pd and not clock.pending()

    if last:
        ffn(2 * NP - 1, g * NPC, SCRIPT_F)
        return
    assert NCH == NP - 2

    late = [(c, m) for c in range(NCH) for m in range(3) if c >= NCH - LAGS[m]]

    def prologue():
        cp_x(0).start()
        for sec in range(3):
            for cp in cp_qkv(sec):
                cp.start()
        qall[:, pl.ds(0, HALO), :] = jnp.zeros((16, HALO, 128), f32)
        cp_x(0).wait()
        for t in range(2):
            x = xin[0, :, t * TB:(t + 1) * TB].astype(f32)
            xres[t] = x
            mean, rstd = _ln_stats(x)
            xn_g[t, pl.ds(zero8, D), :] = (xres[t] - mean) * rstd
        q_left(True)
        for sec in range(3):
            for cp in cp_qkv(sec):
                cp.wait()
            if sec == 0:
                cp_x(1).start()
                cp_x(2).start()
                cp_wo().start()
                for c in range(NCH):
                    if 3 + c < NP:
                        cp_x(3 + c).start()
                    for m in range(3):
                        if c == 0 or c > LAGS[m]:
                            cp_unit(max(c - LAGS[m], 0), m).start()
                for c, m in late:
                    cp_unit(c, m).start()
            transpose_qkv(sec)
            build_wq(sec)

    def first_attention():
        cp_x(2).wait()
        q_step(1, CFG_QA, rows=True)
        cp_wo().wait()
        build_wo()
        wo_mm(0, wo_rhs(0))

    def startup_step(c, carry):
        @pl.when(c + 3 < NP)
        def _():
            cp_x(c + 3).wait()
        for m in range(3):
            if LAGS[m]:
                @pl.when(jnp.logical_or(c == 0, c > LAGS[m]))
                def _():
                    cp_unit(jnp.maximum(c - LAGS[m], 0), m).wait()
            else:
                cp_unit(c, m).wait()
        q_step(c + 2, CFG_Q1, chunk=c)
        return carry

    def startup_tail():
        pieces = []
        for c, m in late:
            cp_unit(c, m).wait()
            pieces += prep_pieces(c, m)
        npt = 15 + 2 * TLN
        done = []

        def pace(v):
            pw[0, pl.ds(R_END + zero8, 8), 0:128] = v
            done.append(v)
            for piece in pieces[(len(done) - 1) * len(pieces) // npt:len(done) * len(pieces) // npt]:
                piece()
        for t in range(2):
            mean, rstd = _ln_stats(xres[t])
            xn = (xres[t, pl.ds(zero8, D), :] - mean) * rstd
            xn_f[t] = xn
            for k in range(TLN):
                pace(pltpu.bitcast(xn[k * 64:k * 64 + 8], u32))
        a_left(cb=pace)
        assert len(done) == npt

    @pl.when(g == 0)
    def _():
        prologue()
        cp_x(1).wait()
        q_step(0, CFG_Q0, sums=True)
        first_attention()
        lax.fori_loop(0, NCH, startup_step, 0)
        startup_tail()

    @pl.when(g >= NP - 1)
    def _():
        q_step(g - (NP - 1))

    ffn(g, 0, SCRIPT)

    @pl.when(g >= NP)
    def _():
        _cp_out(g - NP, o_hbm, xin, sems).start()


def _cp_out(k, o_hbm, xin, sems):
    return pltpu.make_async_copy(xin.at[k], o_hbm.at[:, pl.ds(_al(k * 2 * TB, 128), 2 * TB)], sems.at[4 + k])


def _kernel(*refs, D, DF, S):
    def body(last, g, carry):
        _step(g, last, *refs, D=D, DF=DF, S=S)
        return carry
    NP = S // (2 * TB)
    lax.fori_loop(0, 2 * NP - 1, functools.partial(body, False), 0)
    lax.fori_loop(0, 2, functools.partial(body, True), 0)
    o_hbm, xin, sems = refs[6], refs[7], refs[24]
    _cp_out(NP - 1, o_hbm, xin, sems).start()
    for k in range(NP):
        _cp_out(k, o_hbm, xin, sems).wait()


@jax.jit
def pallas_interleave_layers__sliding_local_dilated__glu_gated_geglu__prompt_kernel(
    A_x, A_wqkv, A_wo, B_x, B_w_gate, B_w_up, B_w_down):
    B, S, D = A_x.shape
    DF = B_w_gate.shape[1]
    NB = S // TB
    NP = NB // 2
    NCH = DF // CW
    xT = A_x.reshape(S, D).T
    wdT = B_w_down.T
    hbm = pl.BlockSpec(memory_space=pltpu.HBM)
    outT = pl.pallas_call(
        functools.partial(_kernel, D=D, DF=DF, S=S),
        in_specs=[hbm] * 6,
        out_specs=hbm,
        out_shape=jax.ShapeDtypeStruct((D, S), A_x.dtype),
        scratch_shapes=[
            pltpu.VMEM((NP, D, 2 * TB), bf16),
            pltpu.VMEM((D, 3 * D), bf16),
            pltpu.VMEM((D, D), bf16),
            pltpu.VMEM((5, 14 * 128, 128), f32),
            pltpu.VMEM((WQR, 27 * 128), u32),
            pltpu.VMEM((D // 2, 640), u32),
            pltpu.VMEM((D // 4, 18 * 128), u32),
            pltpu.VMEM((NCH, 3, D, CW), bf16),
            pltpu.VMEM((NCH, 45 * (TC // 2) + 15 * (D // 6) + 16, 2 * TC), u32),
            pltpu.VMEM((16, S + QPAD, 128), f32),
            pltpu.VMEM((11, TB, 128), f32),
            pltpu.VMEM((NB, D, TB), f32),
            pltpu.VMEM((2, D, TB), f32),
            pltpu.VMEM((2, D, TB), f32),
            pltpu.VMEM((45, TB // 2, TC), u32),
            pltpu.VMEM((31, TB // 2, TC), u32),
            pltpu.VMEM((18, TB // 2, TC), u32),
            pltpu.SemaphoreType.DMA((4 + NP + 3 * NCH,)),
        ] + [pltpu.VMEM((TB, 2 * TC), f32)] * (17 + 9 * NHS),
        compiler_params=pltpu.CompilerParams(
            vmem_limit_bytes=110 * 1024 * 1024,
            disable_bounds_checks=True,
            disable_semaphore_checks=True,
        ),
    )(xT, A_wqkv, A_wo, B_w_gate, B_w_up, wdT)
    return outT.T.reshape(B, S, D)
```

```python
import functools
import math
import jax
import jax.numpy as jnp
from jax import lax
import jax.experimental.pallas as pl
import jax.experimental.pallas.tpu as pltpu

DH = 18
W = 8
DIL = 2
HALO = 16
EPS = 1e-5
TB = 128
RB = 8
TC = 128
CW = 6 * TC
WQR = 320
KY = 64
QPAD = 40

SCRIPT = ('m0+50,m1+2804,k+8550+68,G,R7+74+200,G,G,R2+96+200,G,R9+300+260,D4,'
          'G,R7+74+200,G,G,R7+74+200,G,G,W,n0+300,n1+876,l+2900+80,G,G,G,c+600+192,D8').split(',')
SCRIPT_F = 'G,G,G,G,G,G,D6'.split(',')
GU_ORD = (8, 6, 7, 11, 3, 1, 10, 14, 9, 5, 0, 13, 12, 4, 2)
ORD6 = (0, 4, 3, 1, 5, 2)
WORD = (0, 1, 2, 6, 7, 8, 9, 10, 11, 12, 13, 14, 3, 4, 5)
PLAG, DADV, GTK, DTK, QTK = 6, 2, 2, 2, 8
LNJ = (12, 9, 48, 48)
RG = (2, 1, 24, 420)
RDL, JDL, LDL = 600, 300, 500
NLEFT, NQL, TLN, NHS, OSPL = 15, 18, 9, 4, 4
CFG_Q0 = (40, 1816, 18, 18, 48, 48, 350)
CFG_QA = (300, 748, 6, 6, 32, 64, 350)
CFG_Q1 = (40, 1456, 9, 9, 64, 64, 300)
QA_T = (300, 1000, 4, 3850)
QP0, QP1, QFR = 100, 3850, 0.6
DCUT = (0, 2, 4, 6, 8, 10, 12, 21, 30, 39, 48, 57)
LAGS = (1, 1, 0)

f32 = jnp.float32
bf16 = jnp.bfloat16
u32 = jnp.uint32
NT = (((1,), (1,)), ((), ()))


def _al(i, n):
    return i if isinstance(i, int) else pl.multiple_of(i, n)


def _lt(k):
    return slice(k * 128, (k + 1) * 128)


def _pk(x):
    return pltpu.bitcast(x.astype(bf16), u32)


def _up(x):
    return pltpu.bitcast(x, bf16)


def _dot(a, b):
    return jnp.dot(a, b, preferred_element_type=f32)


def _dot_nt(a, b):
    return lax.dot_general(a, b, NT, preferred_element_type=f32)


def _tree(fn, xs):
    xs = list(xs)
    while len(xs) > 1:
        xs = [fn(xs[i], xs[i + 1]) for i in range(0, len(xs) - 1, 2)] + ([xs[-1]] if len(xs) % 2 else [])
    return xs[0]


def _ln_stats(x, nacc=4):
    n = x.shape[0]
    c = x[0:1]
    s1 = [None] * nacc
    s2 = [None] * nacc
    for i in range(n // 8):
        d = x[i * 8:(i + 1) * 8] - c
        k = i % nacc
        s1[k] = d if s1[k] is None else s1[k] + d
        dd = d * d
        s2[k] = dd if s2[k] is None else s2[k] + dd
    m = jnp.sum(_tree(jnp.add, s1), axis=0, keepdims=True) * (1.0 / n)
    v = jnp.sum(_tree(jnp.add, s2), axis=0, keepdims=True) * (1.0 / n) - m * m
    v = jnp.maximum(v, 0.0)
    return c + m, lax.rsqrt(v + EPS)


_HK_A = (
    ((0, 0, 1), (0, 2, -1), (1, 0, -1)), ((0, 0, 1), (0, 1, -1), (2, 0, -1)), ((1, 1, 1), (0, 1, -1), (1, 2, -1)),
    ((1, 1, 1), (1, 0, -1), (2, 1, -1)), ((2, 2, 1), (0, 2, -1), (2, 1, -1)), ((2, 2, 1), (1, 2, -1), (2, 0, -1)),
    ((0, 1, 1),), ((0, 1, 1), (1, 0, -1)), ((1, 0, 1),),
    ((0, 2, 1),), ((0, 2, 1), (2, 0, -1)), ((2, 0, 1),),
    ((1, 2, 1),), ((2, 1, 1), (1, 2, -1)), ((2, 1, 1),),
)
_HK_C = {
    (0, 0): ((0, 1), (7, 1), (8, 1), (9, 1), (6, -1)),
    (0, 1): ((1, 1), (6, 1), (10, 1), (11, 1), (9, -1)),
    (1, 0): ((2, 1), (7, 1), (8, 1), (12, 1), (6, -1)),
    (1, 1): ((3, 1), (6, 1), (13, 1), (14, 1), (2, -1), (7, -1)),
    (2, 0): ((5, 1), (9, 1), (12, 1), (13, 1), (4, -1), (10, -1)),
    (2, 1): ((4, 1), (10, 1), (11, 1), (14, 1), (9, -1)),
}
_HK_B = (((0, 0, 1),), ((0, 1, 1),), ((1, 0, 1),), ((1, 0, 1), (1, 1, 1)), ((2, 1, 1),), ((2, 0, 1), (2, 1, 1)),
         ((0, 1, 1), (1, 1, 1)), ((0, 1, 1), (1, 0, 1), (1, 1, 1)), ((0, 0, 1), (0, 1, 1), (1, 0, 1), (1, 1, 1)),
         ((0, 0, 1), (2, 0, 1)), ((0, 0, 1), (2, 0, 1), (2, 1, 1)), ((0, 0, 1), (0, 1, 1), (2, 0, 1), (2, 1, 1)),
         ((1, 0, 1), (2, 0, 1)), ((1, 0, 1), (2, 1, -1)), ((1, 1, 1), (2, 1, 1)))


_HK6 = (
    '+00-01-02-30-50 +00 +00;+00-03+05-10-20 +01 +01;-01+11+13-15-40+41 +11 -10+11;-04-10+11+14+31+51 +12 +10;'
    '-02-12+21+22-23-25+35-42 +21 -20+21;-12-20+21+22+24-32-52+53 +22 +20;-03+31-32+33+43 +30 +30-31;'
    '+13-23-30+33-34 +32 +31;-04+34-40+41+42+44+54 +40 +40;-04+14-24-40-43+44-45 +41 +41;'
    '-05-12+35+45-51-52+53+55 +50 +50-51;+15+21-25+35+50-53-54+55 +52 +51;+01-40 +00+10 +00-01+10-11;'
    '+01-10 +00+12 +01-10+11;-04+10 +02+12 +01+11;+02 +00+20 +00-01+20-21;+02-20 +00+22 +01-20+21;'
    '+20 +02+22 +01+21;+03 +01+31 -00+01-30+31;+03-30 +01+32 +00+30-31;+30 +02+32 +00+30;+05 +01-51 +00-01+50-51;'
    '+05+50 +01-52 -00-50+51;+50 +02-52 +00+50;+31 +10-30 -10+30;+13-31 +11+30 +10-31;+13 +11-31 -11+31;'
    '+40-41 +10-40 +10-11-40+41;+04-14-40+41 +12-40 +10-11+41;+04-14 +12-42 +11-41;+12-51 +10+50 +10-50;'
    '+15+51 +11-50 -10+51;+15-21 +11+51 +11-51;+32+53 +20+30 +20+30;-23+32 +21-30 +20+31;+23-35 +21+31 +21+31;'
    '+42 +20-40 +20-21+40-41;+24+42 +22-40 -20+21+41;+24 +22-42 -21-41;+12+52-53 +20+50 +20+50;'
    '+12+21-25+35+52-53 +21-50 +20+51;-21+25-35 +21+51 +21+51;+43 +31+41 +30-31-40+41;+34+43 +32+41 -30+31+40;'
    '+34 +32+42 +30-40;+45 +41+51 -40+41+50-51;+45+54 +41+52 +40-50+51;+54 +42+52 -40+50;'
    '+40 +01+11+41 -00+01-10+11-40+41;-04+40 +02+12+41 +00-01+10-11+40;+04 +02+12+42 +00+10+40;'
    '+12 +10-20+50 -10+11-20+21+50-51;+12+21 +10-22+50 -11+20-21+51;+21 +12-22+52 +11+21-51;'
    '+35 +21+31+51 -20+21-30+31+50-51;+35+53 +21+31+52 +20+30-50+51;+53 +22+32+52 -20-30+50'
)


def _terms(txt):
    return tuple((int(txt[i + 1]), int(txt[i + 2]), 1 if txt[i] == '+' else -1) for i in range(0, len(txt), 3))


_A6, _B6, _Z6 = zip(*[[_terms(f) for f in row.split(' ')] for row in _HK6.split(';')])
_C6 = {(i, t): [(n, sg) for n, z in enumerate(_Z6) for i_, t_, sg in z if (i_, t_) == (i, t)]
       for i in range(6) for t in range(2)}


def _order6():
    early = [n for n, b in enumerate(_B6) if all(j % 3 == 0 or (j % 3 == 1 and d == 1) for j, d, _ in b)]
    early.sort(key=lambda n: max(d != 1 for _, d, _ in _B6[n]))
    out = list(early)
    for i in ORD6:
        out += [n for n, z in enumerate(_Z6) if n not in out and any(i_ == i for i_, _, _ in z)]
    return out


def _ssum(terms):
    terms = sorted(terms, key=lambda z: -z[1])
    acc = terms[0][0] if terms[0][1] == 1 else -terms[0][0]
    for v, sg in terms[1:]:
        acc = acc + v if sg == 1 else acc - v
    return acc


GU_POST = {
    8: ((), ('p8', None), None),
    7: ((('p8', 1),), (None, 't7'), None),
    3: ((('t7', 1),), (None, 's1'), None),
    6: ((), ('p6', None), None),
    14: ((('p6', 1), ('s1', 1)), ('p14', None), (1, 1)),
    12: ((('p9', 1), ('s2', 1)), ('p12', None), (2, 0)),
    13: ((), ('p13', None), None),
    2: ((('p12', 1), ('p13', 1), ('s1', 1)), (None, None), (1, 0)),
    11: ((), ('p11', None), None),
    10: ((('p11', 1),), (None, 't10'), None),
    5: ((('t10', 1),), (None, 's2'), None),
    9: ((), ('p9', None), None),
    4: ((('p14', 1), ('s2', 1), ('p13', -1)), (None, None), (2, 1)),
    0: ((('p8', 1), ('p9', 1), ('t10', 1)), (None, None), (0, 0)),
    1: ((('p6', 1), ('p11', 1), ('t7', 1)), (None, None), (0, 1)),
}
PSLOT = {k: i for i, k in enumerate(('p8', 't7', 's1', 'p6', 'p14', 'p12', 'p13', 'p11', 't10', 's2', 'p9'))}


class _Timeline:
    def __init__(self):
        self.t = 0
        self.jobs = []
        self.due = []

    def add(self, when, fn):
        self.jobs.append((when, len(self.jobs), fn))
        self.jobs.sort(key=lambda z: z[:2])

    def add_due(self, when, job, delay):
        def run(dep):
            val = job(dep)
            if val is not None:
                self.add(self.t + delay, lambda _: self.due.append(lambda: val))
        self.add(when, run)

    def pending(self):
        return [j for j in self.jobs if getattr(j[2], '__name__', '') != '<lambda>']

    def tick(self, dur, v, n):
        for k in range(n):
            self.t += dur // n
            r = k * (v.shape[0] // n)
            while self.jobs and self.jobs[0][0] <= self.t:
                self.jobs.pop(0)[2](v[r:r + 8, 0:128])


def _step(g, last, x_hbm, wqkv_hbm, wo_hbm, wg_hbm, wu_hbm, wd_hbm, o_hbm,
          xin, wqkv_raw, wo_raw, tmp, wq, woT, wo2, raw, pw, qall, o_s, xres, xn_f, xn_g, s_scr, st_s, sq_scr,
          sems, *p_s, D, DF, S):
    NB = S // TB
    NP = NB // 2
    NCH = DF // CW
    NPC = NCH // 2
    D3 = D // 3
    D6 = D // 6
    nr = TB // RB
    hh = D // 4
    zero8 = pl.multiple_of((g >> 20) * 8, 8)
    zvec = jnp.full((8, 128), (g >> 20).astype(u32), u32)

    def zero(k):
        return pl.multiple_of((g >> (8 + k)) * 8, 8)

    def tie(x, dep):
        return pltpu.bitcast(pltpu.bitcast(x, u32) | (pltpu.bitcast(dep, u32) & zvec), f32)

    def gate(lhs, clock):
        if not clock.due:
            return lhs
        pr = _tree(jnp.bitwise_or, [k() for k in clock.due]) & zvec
        del clock.due[:]
        return jnp.concatenate([lhs[0:8] | pr, lhs[8:]], axis=0)

    QSEC = ((0, 5), (5, 9), (9, 14))

    def cp_qkv(sec):
        out = []
        for j in range(*QSEC[sec]):
            n = min(128, 3 * D - j * 128)
            out.append(pltpu.make_async_copy(wqkv_hbm.at[:, pl.ds(j * 128, n)], wqkv_raw.at[:, pl.ds(j * 128, n)],
                                             sems.at[sec]))
        return out

    def cp_wo():
        return pltpu.make_async_copy(wo_hbm, wo_raw, sems.at[3])

    def cp_x(k):
        return pltpu.make_async_copy(x_hbm.at[:, pl.ds(_al(k * 2 * TB, 128), 2 * TB)], xin.at[k], sems.at[4 + k])

    def cp_unit(c, m):
        return pltpu.make_async_copy((wg_hbm, wu_hbm, wd_hbm)[m].at[:, pl.ds(_al(c * CW, 128), CW)], raw.at[c, m],
                                     sems.at[4 + NP + 3 * c + m])

    R_SD = 45 * (TC // 2)
    R_END = R_SD + 15 * (D3 // 2)

    def hk_a_ops(load, minus=None):
        blk = {}
        for i in range(3):
            for j in range(3):
                blk[i, j] = load(i, j).astype(f32)
                if minus is not None:
                    blk[i, j] = blk[i, j] - minus(i, j).astype(f32)
        return [_pk(_ssum([(blk[i, j], sg) for i, j, sg in terms])) for terms in _HK_A]

    def prep_pieces(c, m):
        def ld(r, cs):
            return lambda i, j: raw[c, m, pl.ds(i * D3 + r, 16), pl.ds((3 * cs + j) * TC, TC)]

        def gu_piece(q, r, cs, neg, kind, half):
            ops = hk_a_ops(ld(q * KY + r, cs), None if neg is None else ld(q * KY + r, neg))
            for k, t in enumerate(ops):
                pw.at[c][pl.ds((3 * k + kind) * (TC // 2) + (half * KY + r) // 2, 8), m * TC:(m + 1) * TC] = t

        def d_piece(r, q, ks):
            blk = {}
            z = pl.multiple_of(zero(q) * 2, 16)
            for k in ks:
                for i, j, _ in _A6[k]:
                    if (i, j) not in blk:
                        blk[i, j] = raw[c, m, pl.ds(z + i * D6 + r, 16), pl.ds(j * TC, TC)].astype(f32)
                pw.at[c][pl.ds(R_SD + (k // 2) * (D6 // 2) + r // 2, 8), _lt(k % 2)] = _pk(
                    _ssum([(blk[i, j], sg) for i, j, sg in _A6[k]]))
        if m == 2:
            return [functools.partial(d_piece, r, q, range(DCUT[q], DCUT[q + 1]))
                    for r in range(0, D6, 16) for q in range(len(DCUT) - 1)]
        spec = ((0, 0, None, 0, 0), (1, 0, 1, 0, 1), (0, 1, None, 1, 0), (2, 1, 0, 1, 1),
                (2, 0, None, 2, 0), (1, 1, None, 2, 1))
        return [functools.partial(gu_piece, q, r, cs, neg, kind, half)
                for r in range(0, KY, 16) for q, cs, neg, kind, half in spec]

    def transpose_qkv(sec):
        for j in range(*QSEC[sec]):
            wd_ = min(128, 3 * D - j * 128)
            blk = wqkv_raw[:, j * 128:j * 128 + wd_].astype(f32)
            if wd_ < 128:
                blk = jnp.concatenate([blk, jnp.zeros((D, 128 - wd_), f32)], axis=1)
            bt = jnp.concatenate([blk, blk[D - KY:]], axis=0).T
            for t in range(5):
                tmp[t, pl.ds(j * 128, 128), :] = bt[:, t * 128:(t + 1) * 128]

    def wq_slot(i, j):
        return 24 + i if i == j else [n for n, t in enumerate(_HK_A) if t == ((i, j, 1),)][0]

    def build_wq(sec):
        lo = lax.broadcasted_iota(jnp.int32, (32, 128), 1) < KY
        for d in range(DH):
            tt = [tmp[t, pl.ds(sec * D + d, 32, stride=DH), :] for t in range(5)]
            ops = tt[:4] + [jnp.where(lo, tt[3], tt[4]), jnp.where(lo, tt[4], tt[3])]
            if d < 16:
                dst = [(sec, d * 16)]
            else:
                dst = ([(1, (d + 2) * 16)], [(1, d * 16)], [(0, d * 16), (0, (d + 2) * 16)])[sec]
            for j, row in dst:
                for k, v in enumerate(ops):
                    wq[pl.ds(row, 16), _lt(wq_slot(k, j) if k < 3 else 12 + 3 * j + k)] = _pk(v)

    def wq_sums(r, dep):
        ncol = 3 if r < 256 else 2
        pin = pltpu.bitcast(dep, u32) & zvec
        blk = {(i, j): _up(wq[pl.ds(r, 8), _lt(wq_slot(i, j))] | pin).astype(f32) for i in range(3) for j in range(ncol)}
        for n, terms in enumerate(_HK_A):
            if len(terms) > 1 and not (ncol == 2 and n in (4, 5)):
                wq[pl.ds(r, 8), _lt(n)] = _pk(_ssum([(blk[i, j], sg) for i, j, sg in terms if j < ncol]))

    def build_wo():
        for t in range(5):
            wd_ = min(128, D - t * 128)
            blk = wo_raw[:, t * 128:t * 128 + wd_].astype(f32)
            if wd_ < 128:
                blk = jnp.concatenate([blk, jnp.zeros((D, 128 - wd_), f32)], axis=1)
            tmp[t, pl.ds(0, D), :] = blk
        for t in range(5):
            rows = [tmp[t, pl.ds(d, 32, stride=DH), :] for d in range(DH)]
            ft = jnp.concatenate(rows + rows[16:], axis=0).T
            n = min(128, D - t * 128)
            woT[pl.ds(t * 64, n // 2), :] = _pk(ft[:n])
        for r in range(0, D3 // 2, 8):
            ops = hk_a_ops(lambda i, j: _up(woT[pl.ds(i * (D3 // 2) + r, 8), j * TC:(j + 1) * TC]))
            for k, t in enumerate(ops):
                wo2[pl.ds(r, 8), _lt(k)] = t
        lo = lax.broadcasted_iota(jnp.int32, (16, 128), 1) < KY
        for r in range(0, hh, 8):
            a3, a4, b3, b4 = [_up(woT[pl.ds(r0 + r, 8), c0:c0 + 128]).astype(f32)
                              for r0 in (0, hh) for c0 in (384, 512)]
            wo2[pl.ds(r, 8), _lt(15)] = _pk(jnp.where(lo, a3, a3 - b3))
            wo2[pl.ds(r, 8), _lt(16)] = _pk(jnp.where(lo, b3, b4 - a4))
            wo2[pl.ds(r, 8), _lt(17)] = _pk(jnp.where(lo, a4, b3))

    def q_left(plain, which=None, dep=None):
        k1, k2, k3 = 3 * TC, 3 * TC + KY, 3 * TC + 2 * KY
        for n in (list(range(6 if plain else 15)) + [15, 16, 17]) if which is None else which:
            def X(t, r0, rows):
                return xn_g[t, pl.ds((zero8 if plain else zero(n)) + r0, rows), :]
            if n == 15:
                v = jnp.concatenate([X(0, k1, KY), X(0, k2, KY) - X(1, k2, KY)], axis=0)
            elif n == 16:
                v = jnp.concatenate([X(1, k1, KY), X(1, k3, KY) - X(0, k3, KY)], axis=0)
            elif n == 17:
                v = jnp.concatenate([X(0, k3, KY), X(1, k2, KY)], axis=0)
            elif plain:
                v = X(n // 3, (n % 3) * TC, TC)
            else:
                v = _ssum([(X(t, i * TC, TC), sg) for (i, t), lst in _HK_C.items() for k, sg in lst if k == n])
            if dep is not None:
                v = jnp.concatenate([tie(v[0:8], dep), v[8:]], axis=0)
            sq_scr[n] = pltpu.bitcast(v.astype(bf16).T, u32)

    def add_ln(clock, t0, cfg, blk, dst, par, inp=None):
        np1, np2, step, gap, delay = cfg
        st = dict(s1=[], s2=[], left=np2)
        nv = D // 16

        def load(i):
            if inp is None:
                return xres[blk, pl.ds(zero8 + i * 16, 16), :]
            x = inp(i).astype(f32)
            xres[blk, pl.ds(i * 16, 16), :] = x
            return x

        def stats(k, dep):
            xs = []
            for i in range(k * nv // np1, (k + 1) * nv // np1):
                x = load(i)
                xs += [x[0:8], x[8:16]]
            if k == 0:
                st['c'] = jnp.broadcast_to(xs[0][0:1], (8, TB))
            c = tie(st['c'], dep)
            ds = [x - c for x in xs]
            st['s1'].append(_tree(jnp.add, ds))
            st['s2'].append(_tree(jnp.add, [d * d for d in ds]))
            return pltpu.bitcast(st['s1'][-1], u32) | pltpu.bitcast(st['s2'][-1], u32)

        def norm(k, dep):
            if k == 0:
                m = jnp.sum(_tree(jnp.add, st['s1']), axis=0, keepdims=True) * (1.0 / D)
                v = jnp.sum(_tree(jnp.add, st['s2']), axis=0, keepdims=True) * (1.0 / D) - m * m
                st['mean'] = st['c'] + m
                st['rstd'] = jnp.broadcast_to(lax.rsqrt(jnp.maximum(v, 0.0) + EPS), (8, TB))
            mean = tie(st['mean'], dep)
            off = 0 if inp is None else zero8
            for i in range(k * 2 * nv // np2, (k + 1) * 2 * nv // np2):
                dst[par, pl.ds(i * 8, 8), :] = (xres[blk, pl.ds(off + i * 8, 8), :] - mean) * st['rstd']
            st['left'] -= 1
            return pltpu.bitcast(dst[par, pl.ds(zero8, 8), :], u32)
        for k in range(np1):
            clock.add_due(t0 + k * step, functools.partial(stats, k), delay)
        for k in range(np2):
            clock.add_due(t0 + np1 * step + gap + k * step, functools.partial(norm, k), delay)
        return st

    def hk_outputs(P, T, PT, emit, two_cols):
        p8 = P(8)
        t7 = P(7) + p8
        s1 = PT(3, 1, 2) + t7
        p6 = P(6)
        p14 = P(14)
        emit(1, 1, T(1, 1) + (p6 + p14 + s1))
        p13 = P(13)
        if two_cols:
            emit(1, 0, PT(2, 1, 0) + (p13 + s1))
        else:
            p12 = P(12)
            emit(1, 0, PT(2, 1, 0) + (p12 + p13 + s1))
        p11 = P(11)
        t10 = P(10) + p11
        if not two_cols:
            s2 = PT(5, 2, 2) + t10
            p9 = P(9)
            emit(2, 0, T(2, 0) + (p9 + p12 + s2))
            emit(2, 1, PT(4, 2, 1) + (p14 - p13 + s2))
        w0 = T(0, 2)
        emit(0, 0, PT(0, 0, 0) + ((p8 + t10 + w0) if two_cols else (p8 + p9 + t10 + w0)))
        emit(0, 1, PT(1, 0, 1) + (p6 + p11 + t7 + w0))

    QT = (0, 1, 2, 3)
    KT = (4, 5, 6, 7, 13)
    VT = (8, 9, 10, 11, 12)
    c2e = DH ** -0.5 * math.log2(math.e)
    neg = -1e9 * math.log2(math.e)

    def q_step(pr, cfg=None, chunk=None, rows=False, sums=False):
        first = cfg is not None
        clock = _Timeline()
        if sums:
            base, nx = 0, 1
            for k in range(40):
                clock.add(200 + k * 90, functools.partial(wq_sums, 8 * k))
        elif rows:
            base, nx = pr * (2 * TB), pr + 1
            for k in range(2):
                clock.add_due(QA_T[k], functools.partial(row_chain, k, QA_T[2]), QA_T[3] - QA_T[k])
        else:
            base = pl.multiple_of(pr * (2 * TB), 2 * TB)
            nx = jnp.minimum(pr + 1, NP - 1)
        pieces = []
        if chunk is not None:
            for m in range(3):
                pieces += prep_pieces(jnp.maximum(chunk - LAGS[m], 0) if LAGS[m] else chunk, m)

        def paced(piece, dep):
            pw[0, pl.ds(R_END, 8), 0:128] = pltpu.bitcast(dep, u32)
            piece()
        for k, piece in enumerate(pieces):
            frac = k / 48 * QFR if k < 48 else QFR + (k - 48) / (len(pieces) - 48) * (1 - QFR)
            clock.add(QP0 + int(frac * (QP1 - QP0)), functools.partial(paced, piece))
        if first:
            for par in range(2):
                add_ln(clock, cfg[par], cfg[2:], 2 * nx + par, xn_g, par,
                       functools.partial(lambda par_, i: xin[nx, pl.ds(i * 16, 16), par_ * TB:(par_ + 1) * TB], par))
        for r0, nt, tiles in ((0, 2, (0, 4, 8)), (TC, 2, (2, 6, 10)), (2 * TC, 1, (12, 13))):
            def R(k):
                return wq[pl.ds(r0, nt * 64), _lt(k)]

            def P(k):
                return _dot_nt(_up(sq_scr[k]), _up(R(k)))

            def T(j, kind):
                rhs = _up(R(15 + 3 * j + kind))
                if nt == 1 and kind == 2:
                    nq = 2 if first else 4
                    return jnp.concatenate([_dot_nt(_up(sq_scr[15 + kind, pl.ds(k * (64 // nq), 64 // nq), :]), rhs)
                                            for k in range(nq)], axis=0)
                return _dot_nt(_up(sq_scr[15 + kind]), rhs)

            def PT(k, j, kind):
                return _dot_nt(_up(jnp.concatenate([sq_scr[k], sq_scr[15 + kind]], axis=1)),
                               _up(jnp.concatenate([R(k), R(15 + 3 * j + kind)], axis=1)))

            def emit(col, half, v):
                for k in range(nt):
                    qall[tiles[col] + k, pl.ds(base + (HALO + half * TB), TB), :] = v[:, k * 128:(k + 1) * 128]
            if not first:
                hk_outputs(P, T, PT, emit, nt == 1)
                continue
            for j in range(len(tiles)):
                both = T(j, 2)
                clock.t += 32 * nt
                for t in range(2):
                    for k in range(nt):
                        lhs = [sq_scr[3 * t + i] for i in range(3)] + [sq_scr[15 + t]]
                        lhs[0] = gate(lhs[0], clock)
                        rhs = [wq[pl.ds(r0 + k * 64, 64), _lt(n)]
                               for n in [wq_slot(i, j) for i in range(3)] + [15 + 3 * j + t]]
                        v = _dot_nt(_up(jnp.concatenate(lhs, axis=1)), _up(jnp.concatenate(rhs, axis=1))) + both[:, _lt(k)]
                        qall[tiles[j] + k, pl.ds(base + (HALO + t * TB), TB), :] = v
                        clock.tick(128, v, QTK)
        assert not clock.pending()
        if first:
            q_left(True)

    def row_group(blk, par, r, nw, nv, mids=None):
        base = _al(blk * TB, TB)
        lo = lax.broadcasted_iota(jnp.int32, (RB, 128), 1) < KY
        r0 = r * RB

        def ld(t, w):
            return qall[t, pl.ds(base + (HALO + r0 - DIL * w), RB), :]
        dep = yield
        cs = tie(jnp.full((RB, 128), c2e, f32), dep)
        q = [ld(t, 0) * cs for t in QT] + [jnp.where(lo, pltpu.roll(ld(13, 0), KY, 1), 0.0) * cs]
        sc = []
        for w in range(W):
            if w and w % nw == 0:
                dep = yield
                q = [tie(q[0], dep)] + q[1:]
            acc = None
            for j, t in enumerate(KT):
                p = q[j] * ld(t, w)
                acc = p if acc is None else acc + p
            acc = acc + pltpu.roll(acc, 64, 1)
            if mids is not None:
                mids[r] = pltpu.bitcast(acc, u32)
            acc = acc + pltpu.roll(acc, 32, 1)
            if r0 - DIL * w < 0:
                pos = blk * TB + r0 + lax.broadcasted_iota(jnp.int32, (RB, 128), 0)
                acc = jnp.where(pos >= DIL * w, acc, neg)
            sc.append(acc)
        m = _tree(jnp.maximum, sc)
        e = [jnp.exp2(sc[w] - m) for w in range(W)]
        l = _tree(jnp.add, e)
        rinv = pl.reciprocal(l, approx=True)
        rinv = rinv * (2.0 - l * rinv)
        outs = []
        for j, t in enumerate(VT):
            if j and j % nv == 0:
                dep = yield _tree(jnp.bitwise_or, [pltpu.bitcast(v, u32) for v in outs])
                outs = []
                e = [tie(e[0], dep)] + e[1:]
            acc = None
            for w in range(W):
                p = e[w] * ld(t, w)
                acc = p if acc is None else acc + p
            o = acc * rinv
            o_s[par * 5 + j, pl.ds(r0, RB), :] = o
            outs.append(o)
        yield _tree(jnp.bitwise_or, [pltpu.bitcast(v, u32) for v in outs])

    def add_rows(clock, t0, blk, par, r, cfg):
        nw, nv, step, gap, d1, d2 = cfg
        gen = row_group(blk, par, r, nw, nv)
        next(gen)
        n1, n2 = -(-W // nw), -(-5 // nv)
        for k in range(n1):
            clock.add_due(t0 + k * step, gen.send, d1)
        for k in range(n2 - 1):
            clock.add_due(t0 + (n1 - 1) * step + gap + k * step, gen.send, d2)

    def row_chain(blk, lag, dep):
        mids, fins = {}, {}
        for r in range(nr):
            gen = row_group(blk, blk, r, W, 5, mids)
            next(gen)
            if r:
                dep = pltpu.bitcast(mids[r - 1] | fins[r - lag] if r >= lag else mids[r - 1], f32)
            fins[r] = gen.send(dep)
        return _tree(jnp.bitwise_or, [fins[r] for r in range(nr - lag, nr)])

    wo_seq = []
    for pos, k in enumerate(WORD):
        if pos in (0, 2):
            wo_seq += [('r', pos // 2, k_) for k_ in range(3)]
        wo_seq.append(('p', k))

    def wo_rhs(off):
        lo = lax.broadcasted_iota(jnp.int32, (TB, 128), 1) < KY

        rhs = {}
        for it in wo_seq:
            z = zero(wo_seq.index(it)) if off is None else off

            def O(t, j):
                return o_s[t * 5 + j, pl.ds(z, TB), :]
            if it[0] == 'p':
                v = _ssum([(O(t, j), sg) for j, t, sg in _HK_B[it[1]]])
            elif it[2] == 0:
                v = O(it[1], 3)
            else:
                v = jnp.where(lo, O(it[1], 2 + it[2]), O(it[1], 5 - it[2]))
            rhs[it] = v.astype(bf16)
        return rhs

    def wo_mm(blk0, rhs):
        res = {}
        for it in wo_seq:
            if it[0] == 'p':
                lhs = wo2[pl.ds(0, D3 // 2), _lt(it[1])]
            else:
                lhs = wo2[:, _lt(15 + it[2])]
            res[it] = _dot_nt(_up(lhs), rhs[it])
        for t in range(2):
            both = res['r', t, 2]
            rem = xres[blk0 + t] + jnp.concatenate([res['r', t, 0] + both, res['r', t, 1] + both], axis=0)
            y = jnp.concatenate([_ssum([(res['p', k], sg) for k, sg in _HK_C[i, t]]) for i in range(3)], axis=0)
            xres[blk0 + t] = y + rem

    def a_left(which=range(15), dep=None, cb=None):
        for n in which:
            v = _ssum([(xn_f[t, pl.ds(zero(n) + i * D3, D3), :], sg)
                       for (i, t), lst in _HK_C.items() for k, sg in lst if k == n])
            if dep is not None:
                v = jnp.concatenate([tie(v[0:8], dep), v[8:2 * KY], tie(v[2 * KY:2 * KY + 8], dep), v[2 * KY + 8:]],
                                    axis=0)
            t1 = pltpu.bitcast(v[:2 * KY].astype(bf16).T, u32)
            t2 = pltpu.bitcast(jnp.concatenate([v[2 * KY:], v[2 * KY:]], axis=0).astype(bf16).T, u32)
            if dep is None:
                arrange(n, t1, t2)
                cb(t1[0:8])
                cb(t2[0:8])
            else:
                st_s[2 * n] = t1
                st_s[2 * n + 1] = t2

    def arrange(n, t1, t2):
        lo = lax.broadcasted_iota(jnp.int32, (TB // 2, 128), 1) < KY
        s_scr[3 * n] = t1
        s_scr[3 * n + 1] = jnp.where(lo, t1, t2)
        s_scr[3 * n + 2] = jnp.where(lo, t2, t1)

    def a_arrange(n, dep):
        st_s[30, pl.ds(0, 8), :] = pltpu.bitcast(dep, u32)
        arrange(n, st_s[2 * n, pl.ds(zero8, TB // 2), :], st_s[2 * n + 1, pl.ds(zero8, TB // 2), :])

    k0 = math.sqrt(2.0 / math.pi)
    k1 = k0 * 0.044715

    def ffn(j, c0, script):
        clock = _Timeline()
        b0 = (2 * j) % NB
        an = (2 * j + 2) % NB
        acc = [None] * 57
        hs = {}
        lns, lq, staged, nrows = [], [], set(), 0

        pend = []

        def advance(keep):
            while len(pend) > keep:
                pend.pop(0)()

        def written(k):
            clock.due.append(lambda: pltpu.bitcast(p_s[k][pl.ds(zero8, 8), 0:128], u32))

        def gu(p):
            c, m = c0 + p // 2, p % 2
            h = hs.setdefault(p // 2, [[None, None, None] for _ in range(3)])

            def mm(n, kind):
                lhs = gate(s_scr[3 * n + kind], clock)
                return _dot(_up(lhs), _up(pw[c, pl.ds((3 * n + kind) * (TC // 2), TC // 2), m * TC:(m + 1) * TC]))

            def get(name):
                return p_s[PSLOT[name]][pl.ds(zero8, TB), :]

            def post(n, v):
                adds, keep, emits = GU_POST[n]
                if keep[0] is not None:
                    p_s[PSLOT[keep[0]]][...] = v
                    written(PSLOT[keep[0]])
                w_ = v
                for name, sg in adds:
                    w_ = w_ + get(name) if sg == 1 else w_ - get(name)
                if keep[1] is not None:
                    p_s[PSLOT[keep[1]]][...] = w_
                    written(PSLOT[keep[1]])
                if emits is not None:
                    col, half = emits
                    if m == 1:
                        k_ = 17 + 9 * ((p // 2) % NHS) + 3 * col
                        hv = w_ * p_s[11 + 2 * col + half][pl.ds(zero8, TB), :]
                        p_s[k_ + half][...] = hv
                        written(k_ + half)
                        h[col][half] = k_ + half
                        if h[col][1 - half] is not None:
                            p_s[k_ + 2][...] = hv + p_s[k_ + 1 - half][pl.ds(zero8, TB), :]
                            written(k_ + 2)
                            h[col][2] = k_ + 2
                    else:
                        p_s[11 + 2 * col + half][...] = w_ + w_ * jnp.tanh(w_ * (k0 + k1 * (w_ * w_)))
                        written(11 + 2 * col + half)
            for n in GU_ORD:
                both = mm(n, 2)
                v = jnp.concatenate([mm(n, 0) + both, mm(n, 1) + both], axis=1)
                pend.append(functools.partial(post, n, v))
                advance(PLAG)
                clock.tick(96, both, GTK)

        todo = [sum(any(i_ == i for i_, _, _ in z) for z in _Z6) for i in range(6)]

        def gather(i):
            if last:
                ys = [_ssum([(acc[n], sg) for n, sg in sorted(_C6[i, t], key=lambda z: _order6().index(z[0]))])
                      for t in range(2)]
            else:
                t0, t1 = dict(_C6[i, 0]), dict(_C6[i, 1])
                both = _ssum([(acc[n], sg) for n, sg in t0.items() if n in t1])
                ys = (_ssum([(acc[n], sg) for n, sg in t0.items() if n not in t1]) + both,
                      _ssum([(acc[n], sg) for n, sg in t1.items() if n not in t0]) - both)
            for t in range(2):
                x2 = xres[b0 + t, pl.ds(i * D6, D6), :] + 0.5 * ys[t]
                xres[b0 + t, pl.ds(i * D6, D6), :] = x2
                xin[j % NP, pl.ds(i * D6, D6), t * TB:(t + 1) * TB] = x2.astype(bf16)
            if last and i in ORD6[:OSPL]:
                @pl.when(g == 1)
                def _():
                    _cp_rows(i, o_hbm, xin, sems).start()

        def down(ps, final):
            cs = ps[::2]
            hsl = [hs.pop(p // 2) for p in cs]
            for pos, i in enumerate(_order6()):
                while any(h_[j_ % 3][d_] is None for h_ in hsl for j_, d_, _ in _B6[i]):
                    advance(len(pend) - 1)
                au = [pw[c0 + p // 2, pl.ds(R_SD + (i // 2) * (D6 // 2), D6 // 2), _lt(i % 2)] for p in cs]
                au[0] = gate(au[0], clock)
                lhs = jnp.concatenate(au, axis=1)
                rhs = jnp.concatenate([_ssum([(p_s[h_[j_ % 3][d_]][pl.ds(zero(pos % 21), TB), _lt(j_ // 3)], sg)
                                              for j_, d_, sg in _B6[i]]) for h_ in hsl], axis=1).astype(bf16)
                r = _dot_nt(_up(lhs), rhs)
                acc[i] = r if acc[i] is None else r + acc[i]
                if final:
                    for i_ in sorted({i_ for i_, _, _ in _Z6[i]}):
                        todo[i_] -= 1
                        if not todo[i_]:
                            gather(i_)
                if pos % DADV == 0:
                    advance(max(len(pend) - 1, 0))
                clock.tick(24 * len(cs), acc[i], DTK)

        pg = pd = 0
        for tok in script:
            if tok == 'G':
                gu(pg)
                pg += 1
            elif tok[0] == 'D':
                down(list(range(pd, pd + int(tok[1:]))), pd + int(tok[1:]) == script.count('G'))
                pd += int(tok[1:])
            elif tok == 'W':
                assert not clock.pending() and nrows == 2 * nr
                advance(0)
                wo_mm(an, wo_rhs(None))
                clock.t += 1152
            elif tok[0] == 'n':
                lns.append(add_ln(clock, clock.t + int(tok[3:]), LNJ + (JDL,), an + int(tok[1]), xn_f, int(tok[1])))
            elif tok[0] == 'm':
                lq.append(add_ln(clock, clock.t + int(tok[3:]), LNJ + (JDL,), (2 * j + 4) % NB + int(tok[1]), xn_g,
                                 int(tok[1])))
            elif tok[0] == 'k':
                _, t0, dt = tok.split('+')

                def qleft(which, dep):
                    assert len(lq) == 2 and not any(st['left'] for st in lq)
                    q_left(False, which, dep)
                    return sq_scr[which[0], pl.ds(zero8, 8), :]
                for k in range(NQL):
                    clock.add_due(clock.t + int(t0) + k * int(dt),
                                  functools.partial(qleft, range(k * 18 // NQL, (k + 1) * 18 // NQL)), LDL)
            elif tok[0] == 'l':
                _, t0, dt = tok.split('+')

                def left(which, dep):
                    assert len(lns) == 2 and not any(st['left'] for st in lns)
                    staged.update(which)
                    a_left(which, dep)
                    return st_s[0, pl.ds(zero8, 8), :]
                for k in range(NLEFT):
                    clock.add_due(clock.t + int(t0) + k * int(dt),
                                  functools.partial(left, range(k * 15 // NLEFT, (k + 1) * 15 // NLEFT)), LDL)
            elif tok[0] == 'c':
                _, t0, dt = tok.split('+')
                assert pg == 2 * NCH

                def place(k, dep):
                    assert k in staged
                    a_arrange(k, dep)
                for k in range(15):
                    clock.add(clock.t + int(t0) + k * int(dt), functools.partial(place, k))
            else:
                n, t0, dt = tok[1:].split('+')
                for k in range(int(n)):
                    add_rows(clock, clock.t + int(t0) + k * int(dt), an + nrows // nr, nrows // nr, nrows % nr,
                             RG + (RDL, JDL))
                    nrows += 1
        assert pg == pd and not clock.pending()

    if last:
        ffn(2 * NP - 1, g * NPC, SCRIPT_F)
        return
    assert NCH == NP - 2

    late = [(c, m) for c in range(NCH) for m in range(3) if c >= NCH - LAGS[m]]

    def prologue():
        cp_x(0).start()
        for sec in range(3):
            for cp in cp_qkv(sec):
                cp.start()
        qall[:, pl.ds(0, HALO), :] = jnp.zeros((16, HALO, 128), f32)
        cp_x(0).wait()
        for t in range(2):
            x = xin[0, :, t * TB:(t + 1) * TB].astype(f32)
            xres[t] = x
            mean, rstd = _ln_stats(x)
            xn_g[t, pl.ds(zero8, D), :] = (xres[t] - mean) * rstd
        q_left(True)
        for sec in range(3):
            for cp in cp_qkv(sec):
                cp.wait()
            if sec == 0:
                cp_x(1).start()
                cp_x(2).start()
                cp_wo().start()
                for c in range(NCH):
                    if 3 + c < NP:
                        cp_x(3 + c).start()
                    for m in range(3):
                        if c == 0 or c > LAGS[m]:
                            cp_unit(max(c - LAGS[m], 0), m).start()
                for c, m in late:
                    cp_unit(c, m).start()
            transpose_qkv(sec)
            build_wq(sec)

    def first_attention():
        cp_x(2).wait()
        q_step(1, CFG_QA, rows=True)
        cp_wo().wait()
        build_wo()
        wo_mm(0, wo_rhs(0))

    def startup_step(c, carry):
        @pl.when(c + 3 < NP)
        def _():
            cp_x(c + 3).wait()
        for m in range(3):
            if LAGS[m]:
                @pl.when(jnp.logical_or(c == 0, c > LAGS[m]))
                def _():
                    cp_unit(jnp.maximum(c - LAGS[m], 0), m).wait()
            else:
                cp_unit(c, m).wait()
        q_step(c + 2, CFG_Q1, chunk=c)
        return carry

    def startup_tail():
        pieces = []
        for c, m in late:
            cp_unit(c, m).wait()
            pieces += prep_pieces(c, m)
        npt = 30 + 2 * TLN
        done = []

        def pace(v):
            pw[0, pl.ds(R_END + zero8, 8), 0:128] = v
            done.append(v)
            for piece in pieces[(len(done) - 1) * len(pieces) // npt:len(done) * len(pieces) // npt]:
                piece()
        for t in range(2):
            mean, rstd = _ln_stats(xres[t])
            xn = (xres[t, pl.ds(zero8, D), :] - mean) * rstd
            xn_f[t] = xn
            for k in range(TLN):
                pace(pltpu.bitcast(xn[k * 64:k * 64 + 8], u32))
        a_left(cb=pace)
        assert len(done) == npt

    @pl.when(g == 0)
    def _():
        prologue()
        cp_x(1).wait()
        q_step(0, CFG_Q0, sums=True)
        first_attention()
        lax.fori_loop(0, NCH, startup_step, 0)
        startup_tail()

    @pl.when(g >= NP - 1)
    def _():
        q_step(g - (NP - 1))

    ffn(g, 0, SCRIPT)

    @pl.when(g >= NP)
    def _():
        _cp_out(g - NP, o_hbm, xin, sems).start()


def _cp_out(k, o_hbm, xin, sems):
    return pltpu.make_async_copy(xin.at[k], o_hbm.at[:, pl.ds(_al(k * 2 * TB, 128), 2 * TB)], sems.at[4 + k])


def _cp_rows(i, o_hbm, xin, sems):
    k, n = xin.shape[0] - 1, xin.shape[1] // 6
    return pltpu.make_async_copy(xin.at[k, pl.ds(i * n, n), :], o_hbm.at[pl.ds(i * n, n), pl.ds(k * 2 * TB, 2 * TB)],
                                 sems.at[4 + k])


def _kernel(*refs, D, DF, S):
    def body(last, g, carry):
        _step(g, last, *refs, D=D, DF=DF, S=S)
        return carry
    NP = S // (2 * TB)
    lax.fori_loop(0, 2 * NP - 1, functools.partial(body, False), 0)
    lax.fori_loop(0, 2, functools.partial(body, True), 0)
    o_hbm, xin, sems = refs[6], refs[7], refs[24]
    for i in ORD6[OSPL:]:
        _cp_rows(i, o_hbm, xin, sems).start()
    for k in range(NP - 1):
        _cp_out(k, o_hbm, xin, sems).wait()
    for i in range(6):
        _cp_rows(i, o_hbm, xin, sems).wait()


@jax.jit
def pallas_interleave_layers__sliding_local_dilated__glu_gated_geglu__prompt_kernel(
    A_x, A_wqkv, A_wo, B_x, B_w_gate, B_w_up, B_w_down):
    B, S, D = A_x.shape
    DF = B_w_gate.shape[1]
    NB = S // TB
    NP = NB // 2
    NCH = DF // CW
    xT = A_x.reshape(S, D).T
    wdT = B_w_down.T
    hbm = pl.BlockSpec(memory_space=pltpu.HBM)
    outT = pl.pallas_call(
        functools.partial(_kernel, D=D, DF=DF, S=S),
        in_specs=[hbm] * 6,
        out_specs=hbm,
        out_shape=jax.ShapeDtypeStruct((D, S), A_x.dtype),
        scratch_shapes=[
            pltpu.VMEM((NP, D, 2 * TB), bf16),
            pltpu.VMEM((D, 3 * D), bf16),
            pltpu.VMEM((D, D), bf16),
            pltpu.VMEM((5, 14 * 128, 128), f32),
            pltpu.VMEM((WQR, 27 * 128), u32),
            pltpu.VMEM((D // 2, 640), u32),
            pltpu.VMEM((D // 4, 18 * 128), u32),
            pltpu.VMEM((NCH, 3, D, CW), bf16),
            pltpu.VMEM((NCH, 45 * (TC // 2) + 15 * (D // 6) + 16, 2 * TC), u32),
            pltpu.VMEM((16, S + QPAD, 128), f32),
            pltpu.VMEM((11, TB, 128), f32),
            pltpu.VMEM((NB, D, TB), f32),
            pltpu.VMEM((2, D, TB), f32),
            pltpu.VMEM((2, D, TB), f32),
            pltpu.VMEM((45, TB // 2, TC), u32),
            pltpu.VMEM((31, TB // 2, TC), u32),
            pltpu.VMEM((18, TB // 2, TC), u32),
            pltpu.SemaphoreType.DMA((4 + NP + 3 * NCH,)),
        ] + [pltpu.VMEM((TB, 2 * TC), f32)] * (17 + 9 * NHS),
        compiler_params=pltpu.CompilerParams(
            vmem_limit_bytes=110 * 1024 * 1024,
            disable_bounds_checks=True,
            disable_semaphore_checks=True,
        ),
    )(xT, A_wqkv, A_wo, B_w_gate, B_w_up, wdT)
    return outT.T.reshape(B, S, D)
```

```python
import functools
import math
import jax
import jax.numpy as jnp
from jax import lax
import jax.experimental.pallas as pl
import jax.experimental.pallas.tpu as pltpu

DH = 18
W = 8
DIL = 2
HALO = 16
EPS = 1e-5
TB = 128
RB = 8
TC = 128
CW = 6 * TC
WQR = 320
KY = 64
QPAD = 40

SCRIPT = ('m0+50,m1+2804,k+8550+68,G,R7+74+200,G,G,R2+96+200,G,R9+300+260,D4,'
          'G,R7+74+200,G,G,R7+74+200,G,G,W,n0+300,n1+876,l+2900+80,G,G,G,c+600+192,D8').split(',')
SCRIPT_F = 'G,G,G,G,G,G,D6'.split(',')
GU_ORD = (8, 6, 7, 11, 3, 1, 10, 14, 9, 5, 0, 13, 12, 4, 2)
ORD6 = (0, 4, 3, 1, 5, 2)
WORD = (0, 1, 2, 6, 7, 8, 9, 10, 11, 12, 13, 14, 3, 4, 5)
PLAG, DADV, GTK, DTK, QTK = 6, 2, 2, 2, 8
LNJ = (12, 9, 48, 48)
RG = (2, 1, 24, 420)
RDL, JDL, LDL = 600, 300, 500
NLEFT, NQL, TLN, NHS, OSPL = 15, 18, 9, 4, 4
CFG_Q0 = (40, 1816, 18, 18, 48, 48, 350)
CFG_QA = (300, 748, 6, 6, 32, 64, 350)
CFG_Q1 = (40, 1456, 9, 9, 64, 64, 300)
QA_T = (300, 1000, 4, 3850)
QP0, QP1, QFR = 100, 3850, 0.6
DCUT = (0, 2, 4, 6, 8, 10, 12, 21, 30, 39, 48, 57)
LAGS = (1, 1, 0)

f32 = jnp.float32
bf16 = jnp.bfloat16
u32 = jnp.uint32
NT = (((1,), (1,)), ((), ()))


def _al(i, n):
    return i if isinstance(i, int) else pl.multiple_of(i, n)


def _lt(k):
    return slice(k * 128, (k + 1) * 128)


def _pk(x):
    return pltpu.bitcast(x.astype(bf16), u32)


def _up(x):
    return pltpu.bitcast(x, bf16)


def _dot(a, b):
    return jnp.dot(a, b, preferred_element_type=f32)


def _dot_nt(a, b):
    return lax.dot_general(a, b, NT, preferred_element_type=f32)


def _tree(fn, xs):
    xs = list(xs)
    while len(xs) > 1:
        xs = [fn(xs[i], xs[i + 1]) for i in range(0, len(xs) - 1, 2)] + ([xs[-1]] if len(xs) % 2 else [])
    return xs[0]


def _ln_stats(x, nacc=4):
    n = x.shape[0]
    c = x[0:1]
    s1 = [None] * nacc
    s2 = [None] * nacc
    for i in range(n // 8):
        d = x[i * 8:(i + 1) * 8] - c
        k = i % nacc
        s1[k] = d if s1[k] is None else s1[k] + d
        dd = d * d
        s2[k] = dd if s2[k] is None else s2[k] + dd
    m = jnp.sum(_tree(jnp.add, s1), axis=0, keepdims=True) * (1.0 / n)
    v = jnp.sum(_tree(jnp.add, s2), axis=0, keepdims=True) * (1.0 / n) - m * m
    v = jnp.maximum(v, 0.0)
    return c + m, lax.rsqrt(v + EPS)


_HK_A = (
    ((0, 0, 1), (0, 2, -1), (1, 0, -1)), ((0, 0, 1), (0, 1, -1), (2, 0, -1)), ((1, 1, 1), (0, 1, -1), (1, 2, -1)),
    ((1, 1, 1), (1, 0, -1), (2, 1, -1)), ((2, 2, 1), (0, 2, -1), (2, 1, -1)), ((2, 2, 1), (1, 2, -1), (2, 0, -1)),
    ((0, 1, 1),), ((0, 1, 1), (1, 0, -1)), ((1, 0, 1),),
    ((0, 2, 1),), ((0, 2, 1), (2, 0, -1)), ((2, 0, 1),),
    ((1, 2, 1),), ((2, 1, 1), (1, 2, -1)), ((2, 1, 1),),
)
_HK_C = {
    (0, 0): ((0, 1), (7, 1), (8, 1), (9, 1), (6, -1)),
    (0, 1): ((1, 1), (6, 1), (10, 1), (11, 1), (9, -1)),
    (1, 0): ((2, 1), (7, 1), (8, 1), (12, 1), (6, -1)),
    (1, 1): ((3, 1), (6, 1), (13, 1), (14, 1), (2, -1), (7, -1)),
    (2, 0): ((5, 1), (9, 1), (12, 1), (13, 1), (4, -1), (10, -1)),
    (2, 1): ((4, 1), (10, 1), (11, 1), (14, 1), (9, -1)),
}
_HK_B = (((0, 0, 1),), ((0, 1, 1),), ((1, 0, 1),), ((1, 0, 1), (1, 1, 1)), ((2, 1, 1),), ((2, 0, 1), (2, 1, 1)),
         ((0, 1, 1), (1, 1, 1)), ((0, 1, 1), (1, 0, 1), (1, 1, 1)), ((0, 0, 1), (0, 1, 1), (1, 0, 1), (1, 1, 1)),
         ((0, 0, 1), (2, 0, 1)), ((0, 0, 1), (2, 0, 1), (2, 1, 1)), ((0, 0, 1), (0, 1, 1), (2, 0, 1), (2, 1, 1)),
         ((1, 0, 1), (2, 0, 1)), ((1, 0, 1), (2, 1, -1)), ((1, 1, 1), (2, 1, 1)))


_HK6 = (
    '+00-01-02-30-50 +00 +00;+00-03+05-10-20 +01 +01;-01+11+13-15-40+41 +11 -10+11;-04-10+11+14+31+51 +12 +10;'
    '-02-12+21+22-23-25+35-42 +21 -20+21;-12-20+21+22+24-32-52+53 +22 +20;-03+31-32+33+43 +30 +30-31;'
    '+13-23-30+33-34 +32 +31;-04+34-40+41+42+44+54 +40 +40;-04+14-24-40-43+44-45 +41 +41;'
    '-05-12+35+45-51-52+53+55 +50 +50-51;+15+21-25+35+50-53-54+55 +52 +51;+01-40 +00+10 +00-01+10-11;'
    '+01-10 +00+12 +01-10+11;-04+10 +02+12 +01+11;+02 +00+20 +00-01+20-21;+02-20 +00+22 +01-20+21;'
    '+20 +02+22 +01+21;+03 +01+31 -00+01-30+31;+03-30 +01+32 +00+30-31;+30 +02+32 +00+30;+05 +01-51 +00-01+50-51;'
    '+05+50 +01-52 -00-50+51;+50 +02-52 +00+50;+31 +10-30 -10+30;+13-31 +11+30 +10-31;+13 +11-31 -11+31;'
    '+40-41 +10-40 +10-11-40+41;+04-14-40+41 +12-40 +10-11+41;+04-14 +12-42 +11-41;+12-51 +10+50 +10-50;'
    '+15+51 +11-50 -10+51;+15-21 +11+51 +11-51;+32+53 +20+30 +20+30;-23+32 +21-30 +20+31;+23-35 +21+31 +21+31;'
    '+42 +20-40 +20-21+40-41;+24+42 +22-40 -20+21+41;+24 +22-42 -21-41;+12+52-53 +20+50 +20+50;'
    '+12+21-25+35+52-53 +21-50 +20+51;-21+25-35 +21+51 +21+51;+43 +31+41 +30-31-40+41;+34+43 +32+41 -30+31+40;'
    '+34 +32+42 +30-40;+45 +41+51 -40+41+50-51;+45+54 +41+52 +40-50+51;+54 +42+52 -40+50;'
    '+40 +01+11+41 -00+01-10+11-40+41;-04+40 +02+12+41 +00-01+10-11+40;+04 +02+12+42 +00+10+40;'
    '+12 +10-20+50 -10+11-20+21+50-51;+12+21 +10-22+50 -11+20-21+51;+21 +12-22+52 +11+21-51;'
    '+35 +21+31+51 -20+21-30+31+50-51;+35+53 +21+31+52 +20+30-50+51;+53 +22+32+52 -20-30+50'
)


def _terms(txt):
    return tuple((int(txt[i + 1]), int(txt[i + 2]), 1 if txt[i] == '+' else -1) for i in range(0, len(txt), 3))


_A6, _B6, _Z6 = zip(*[[_terms(f) for f in row.split(' ')] for row in _HK6.split(';')])
_C6 = {(i, t): [(n, sg) for n, z in enumerate(_Z6) for i_, t_, sg in z if (i_, t_) == (i, t)]
       for i in range(6) for t in range(2)}


def _order6():
    early = [n for n, b in enumerate(_B6) if all(j % 3 == 0 or (j % 3 == 1 and d == 1) for j, d, _ in b)]
    early.sort(key=lambda n: max(d != 1 for _, d, _ in _B6[n]))
    out = list(early)
    for i in ORD6:
        out += [n for n, z in enumerate(_Z6) if n not in out and any(i_ == i for i_, _, _ in z)]
    return out


def _ssum(terms):
    terms = sorted(terms, key=lambda z: -z[1])
    acc = terms[0][0] if terms[0][1] == 1 else -terms[0][0]
    for v, sg in terms[1:]:
        acc = acc + v if sg == 1 else acc - v
    return acc


GU_POST = {
    8: ((), ('p8', None), None),
    7: ((('p8', 1),), (None, 't7'), None),
    3: ((('t7', 1),), (None, 's1'), None),
    6: ((), ('p6', None), None),
    14: ((('p6', 1), ('s1', 1)), ('p14', None), (1, 1)),
    12: ((('p9', 1), ('s2', 1)), ('p12', None), (2, 0)),
    13: ((), ('p13', None), None),
    2: ((('p12', 1), ('p13', 1), ('s1', 1)), (None, None), (1, 0)),
    11: ((), ('p11', None), None),
    10: ((('p11', 1),), (None, 't10'), None),
    5: ((('t10', 1),), (None, 's2'), None),
    9: ((), ('p9', None), None),
    4: ((('p14', 1), ('s2', 1), ('p13', -1)), (None, None), (2, 1)),
    0: ((('p8', 1), ('p9', 1), ('t10', 1)), (None, None), (0, 0)),
    1: ((('p6', 1), ('p11', 1), ('t7', 1)), (None, None), (0, 1)),
}
PSLOT = {k: i for i, k in enumerate(('p8', 't7', 's1', 'p6', 'p14', 'p12', 'p13', 'p11', 't10', 's2', 'p9'))}


class _Timeline:
    def __init__(self):
        self.t = 0
        self.jobs = []
        self.due = []

    def add(self, when, fn):
        self.jobs.append((when, len(self.jobs), fn))
        self.jobs.sort(key=lambda z: z[:2])

    def add_due(self, when, job, delay):
        def run(dep):
            val = job(dep)
            if val is not None:
                self.add(self.t + delay, lambda _: self.due.append(lambda: val))
        self.add(when, run)

    def pending(self):
        return [j for j in self.jobs if getattr(j[2], '__name__', '') != '<lambda>']

    def tick(self, dur, v, n):
        for k in range(n):
            self.t += dur // n
            r = k * (v.shape[0] // n)
            while self.jobs and self.jobs[0][0] <= self.t:
                self.jobs.pop(0)[2](v[r:r + 8, 0:128])


def _step(g, last, x_hbm, wqkv_hbm, wo_hbm, wg_hbm, wu_hbm, wd_hbm, o_hbm,
          xin, wqkv_raw, wo_raw, tmp, wq, woT, wo2, raw, pw, qall, o_s, xres, xn_f, xn_g, s_scr, st_s, sq_scr,
          sems, *p_s, D, DF, S):
    NB = S // TB
    NP = NB // 2
    NCH = DF // CW
    NPC = NCH // 2
    D3 = D // 3
    D6 = D // 6
    nr = TB // RB
    hh = D // 4
    zero8 = pl.multiple_of((g >> 20) * 8, 8)
    zvec = jnp.full((8, 128), (g >> 20).astype(u32), u32)

    def zero(k):
        return pl.multiple_of((g >> (8 + k)) * 8, 8)

    def tie(x, dep):
        return pltpu.bitcast(pltpu.bitcast(x, u32) | (pltpu.bitcast(dep, u32) & zvec), f32)

    def gate(lhs, clock):
        if not clock.due:
            return lhs
        pr = _tree(jnp.bitwise_or, [k() for k in clock.due]) & zvec
        del clock.due[:]
        return jnp.concatenate([lhs[0:8] | pr, lhs[8:]], axis=0)

    QSEC = ((0, 5), (5, 9), (9, 14))

    def cp_qkv(sec):
        out = []
        for j in range(*QSEC[sec]):
            n = min(128, 3 * D - j * 128)
            out.append(pltpu.make_async_copy(wqkv_hbm.at[:, pl.ds(j * 128, n)], wqkv_raw.at[:, pl.ds(j * 128, n)],
                                             sems.at[sec]))
        return out

    def cp_wo():
        return pltpu.make_async_copy(wo_hbm, wo_raw, sems.at[3])

    def cp_x(k):
        return pltpu.make_async_copy(x_hbm.at[:, pl.ds(_al(k * 2 * TB, 128), 2 * TB)], xin.at[k], sems.at[4 + k])

    def cp_unit(c, m):
        return pltpu.make_async_copy((wg_hbm, wu_hbm, wd_hbm)[m].at[:, pl.ds(_al(c * CW, 128), CW)], raw.at[c, m],
                                     sems.at[4 + NP + 3 * c + m])

    R_SD = 45 * (TC // 2)
    R_END = R_SD + 15 * (D3 // 2)

    def hk_a_ops(load, minus=None):
        blk = {}
        for i in range(3):
            for j in range(3):
                blk[i, j] = load(i, j).astype(f32)
                if minus is not None:
                    blk[i, j] = blk[i, j] - minus(i, j).astype(f32)
        return [_pk(_ssum([(blk[i, j], sg) for i, j, sg in terms])) for terms in _HK_A]

    def prep_pieces(c, m):
        def ld(r, cs):
            return lambda i, j: raw[c, m, pl.ds(i * D3 + r, 16), pl.ds((3 * cs + j) * TC, TC)]

        def gu_piece(q, r, cs, neg, kind, half):
            ops = hk_a_ops(ld(q * KY + r, cs), None if neg is None else ld(q * KY + r, neg))
            for k, t in enumerate(ops):
                pw.at[c][pl.ds((3 * k + kind) * (TC // 2) + (half * KY + r) // 2, 8), m * TC:(m + 1) * TC] = t

        def d_piece(r, q, ks):
            blk = {}
            cz = c + (g >> (8 + q))
            for k in ks:
                for i, j, _ in _A6[k]:
                    if (i, j) not in blk:
                        blk[i, j] = raw[cz, m, pl.ds(i * D6 + r, 16), pl.ds(j * TC, TC)].astype(f32)
                pw.at[c][pl.ds(R_SD + (k // 2) * (D6 // 2) + r // 2, 8), _lt(k % 2)] = _pk(
                    _ssum([(blk[i, j], sg) for i, j, sg in _A6[k]]))
        if m == 2:
            return [functools.partial(d_piece, r, q, range(DCUT[q], DCUT[q + 1]))
                    for r in range(0, D6, 16) for q in range(len(DCUT) - 1)]
        spec = ((0, 0, None, 0, 0), (1, 0, 1, 0, 1), (0, 1, None, 1, 0), (2, 1, 0, 1, 1),
                (2, 0, None, 2, 0), (1, 1, None, 2, 1))
        return [functools.partial(gu_piece, q, r, cs, neg, kind, half)
                for r in range(0, KY, 16) for q, cs, neg, kind, half in spec]

    def transpose_qkv(sec):
        for j in range(*QSEC[sec]):
            wd_ = min(128, 3 * D - j * 128)
            blk = wqkv_raw[:, j * 128:j * 128 + wd_].astype(f32)
            if wd_ < 128:
                blk = jnp.concatenate([blk, jnp.zeros((D, 128 - wd_), f32)], axis=1)
            bt = jnp.concatenate([blk, blk[D - KY:]], axis=0).T
            for t in range(5):
                tmp[t, pl.ds(j * 128, 128), :] = bt[:, t * 128:(t + 1) * 128]

    def wq_slot(i, j):
        return 24 + i if i == j else [n for n, t in enumerate(_HK_A) if t == ((i, j, 1),)][0]

    def build_wq(sec):
        lo = lax.broadcasted_iota(jnp.int32, (32, 128), 1) < KY
        for d in range(DH):
            tt = [tmp[t, pl.ds(sec * D + d, 32, stride=DH), :] for t in range(5)]
            ops = tt[:4] + [jnp.where(lo, tt[3], tt[4]), jnp.where(lo, tt[4], tt[3])]
            if d < 16:
                dst = [(sec, d * 16)]
            else:
                dst = ([(1, (d + 2) * 16)], [(1, d * 16)], [(0, d * 16), (0, (d + 2) * 16)])[sec]
            for j, row in dst:
                for k, v in enumerate(ops):
                    wq[pl.ds(row, 16), _lt(wq_slot(k, j) if k < 3 else 12 + 3 * j + k)] = _pk(v)

    def wq_sums(r, dep):
        ncol = 3 if r < 256 else 2
        pin = pltpu.bitcast(dep, u32) & zvec
        blk = {(i, j): _up(wq[pl.ds(r, 8), _lt(wq_slot(i, j))] | pin).astype(f32) for i in range(3) for j in range(ncol)}
        for n, terms in enumerate(_HK_A):
            if len(terms) > 1 and not (ncol == 2 and n in (4, 5)):
                wq[pl.ds(r, 8), _lt(n)] = _pk(_ssum([(blk[i, j], sg) for i, j, sg in terms if j < ncol]))

    def build_wo():
        for t in range(5):
            wd_ = min(128, D - t * 128)
            blk = wo_raw[:, t * 128:t * 128 + wd_].astype(f32)
            if wd_ < 128:
                blk = jnp.concatenate([blk, jnp.zeros((D, 128 - wd_), f32)], axis=1)
            tmp[t, pl.ds(0, D), :] = blk
        for t in range(5):
            rows = [tmp[t, pl.ds(d, 32, stride=DH), :] for d in range(DH)]
            ft = jnp.concatenate(rows + rows[16:], axis=0).T
            n = min(128, D - t * 128)
            woT[pl.ds(t * 64, n // 2), :] = _pk(ft[:n])
        for r in range(0, D3 // 2, 8):
            ops = hk_a_ops(lambda i, j: _up(woT[pl.ds(i * (D3 // 2) + r, 8), j * TC:(j + 1) * TC]))
            for k, t in enumerate(ops):
                wo2[pl.ds(r, 8), _lt(k)] = t
        lo = lax.broadcasted_iota(jnp.int32, (16, 128), 1) < KY
        for r in range(0, hh, 8):
            a3, a4, b3, b4 = [_up(woT[pl.ds(r0 + r, 8), c0:c0 + 128]).astype(f32)
                              for r0 in (0, hh) for c0 in (384, 512)]
            wo2[pl.ds(r, 8), _lt(15)] = _pk(jnp.where(lo, a3, a3 - b3))
            wo2[pl.ds(r, 8), _lt(16)] = _pk(jnp.where(lo, b3, b4 - a4))
            wo2[pl.ds(r, 8), _lt(17)] = _pk(jnp.where(lo, a4, b3))

    def q_left(plain, which=None, dep=None, slot=0):
        k1, k2, k3 = 3 * TC, 3 * TC + KY, 3 * TC + 2 * KY
        for n in (list(range(6 if plain else 15)) + [15, 16, 17]) if which is None else which:
            def X(t, r0, rows):
                return xn_g[t, pl.ds((zero8 if plain else zero(n)) + r0, rows), :]
            if n == 15:
                v = jnp.concatenate([X(0, k1, KY), X(0, k2, KY) - X(1, k2, KY)], axis=0)
            elif n == 16:
                v = jnp.concatenate([X(1, k1, KY), X(1, k3, KY) - X(0, k3, KY)], axis=0)
            elif n == 17:
                v = jnp.concatenate([X(0, k3, KY), X(1, k2, KY)], axis=0)
            elif plain:
                v = X(n // 3, (n % 3) * TC, TC)
            else:
                v = _ssum([(X(t, i * TC, TC), sg) for (i, t), lst in _HK_C.items() for k, sg in lst if k == n])
            if dep is not None:
                v = jnp.concatenate([tie(v[0:8], dep), v[8:]], axis=0)
            sq_scr[n, slot] = pltpu.bitcast(v.astype(bf16).T, u32)

    def add_ln(clock, t0, cfg, blk, dst, par, inp=None):
        np1, np2, step, gap, delay = cfg
        st = dict(s1=[], s2=[], left=np2)
        nv = D // 16

        def load(i):
            if inp is None:
                return xres[blk, pl.ds(zero8 + i * 16, 16), :]
            x = inp(i).astype(f32)
            xres[blk, pl.ds(i * 16, 16), :] = x
            return x

        def stats(k, dep):
            xs = []
            for i in range(k * nv // np1, (k + 1) * nv // np1):
                x = load(i)
                xs += [x[0:8], x[8:16]]
            if k == 0:
                st['c'] = jnp.broadcast_to(xs[0][0:1], (8, TB))
            c = tie(st['c'], dep)
            ds = [x - c for x in xs]
            st['s1'].append(_tree(jnp.add, ds))
            st['s2'].append(_tree(jnp.add, [d * d for d in ds]))
            return pltpu.bitcast(st['s1'][-1], u32) | pltpu.bitcast(st['s2'][-1], u32)

        def norm(k, dep):
            if k == 0:
                m = jnp.sum(_tree(jnp.add, st['s1']), axis=0, keepdims=True) * (1.0 / D)
                v = jnp.sum(_tree(jnp.add, st['s2']), axis=0, keepdims=True) * (1.0 / D) - m * m
                st['mean'] = st['c'] + m
                st['rstd'] = jnp.broadcast_to(lax.rsqrt(jnp.maximum(v, 0.0) + EPS), (8, TB))
            mean = tie(st['mean'], dep)
            off = 0 if inp is None else zero8
            for i in range(k * 2 * nv // np2, (k + 1) * 2 * nv // np2):
                dst[par, pl.ds(i * 8, 8), :] = (xres[blk, pl.ds(off + i * 8, 8), :] - mean) * st['rstd']
            st['left'] -= 1
            return pltpu.bitcast(dst[par, pl.ds(zero8, 8), :], u32)
        for k in range(np1):
            clock.add_due(t0 + k * step, functools.partial(stats, k), delay)
        for k in range(np2):
            clock.add_due(t0 + np1 * step + gap + k * step, functools.partial(norm, k), delay)
        return st

    def hk_outputs(P, T, PT, emit, two_cols):
        p8 = P(8)
        t7 = P(7) + p8
        s1 = PT(3, 1, 2) + t7
        p6 = P(6)
        p14 = P(14)
        emit(1, 1, T(1, 1) + (p6 + p14 + s1))
        p13 = P(13)
        if two_cols:
            emit(1, 0, PT(2, 1, 0) + (p13 + s1))
        else:
            p12 = P(12)
            emit(1, 0, PT(2, 1, 0) + (p12 + p13 + s1))
        p11 = P(11)
        t10 = P(10) + p11
        if not two_cols:
            s2 = PT(5, 2, 2) + t10
            p9 = P(9)
            emit(2, 0, T(2, 0) + (p9 + p12 + s2))
            emit(2, 1, PT(4, 2, 1) + (p14 - p13 + s2))
        w0 = T(0, 2)
        emit(0, 0, PT(0, 0, 0) + ((p8 + t10 + w0) if two_cols else (p8 + p9 + t10 + w0)))
        emit(0, 1, PT(1, 0, 1) + (p6 + p11 + t7 + w0))

    QT = (0, 1, 2, 3)
    KT = (4, 5, 6, 7, 13)
    VT = (8, 9, 10, 11, 12)
    c2e = DH ** -0.5 * math.log2(math.e)
    neg = -1e9 * math.log2(math.e)

    def q_step(pr, cfg=None, chunk=None, rows=False, sums=False):
        first = cfg is not None
        clock = _Timeline()
        if sums:
            base, nx = 0, 1
            for k in range(40):
                clock.add(200 + k * 90, functools.partial(wq_sums, 8 * k))
        elif rows:
            base, nx = pr * (2 * TB), pr + 1
            for k in range(2):
                clock.add_due(QA_T[k], functools.partial(row_chain, k, QA_T[2]), QA_T[3] - QA_T[k])
        else:
            base = pl.multiple_of(pr * (2 * TB), 2 * TB)
            nx = jnp.minimum(pr + 1, NP - 1)
        pieces = []
        if chunk is not None:
            for m in range(3):
                pieces += prep_pieces(jnp.maximum(chunk - LAGS[m], 0) if LAGS[m] else chunk, m)

        def paced(piece, dep):
            pw[0, pl.ds(R_END, 8), 0:128] = pltpu.bitcast(dep, u32)
            piece()
        for k, piece in enumerate(pieces):
            frac = k / 48 * QFR if k < 48 else QFR + (k - 48) / (len(pieces) - 48) * (1 - QFR)
            clock.add(QP0 + int(frac * (QP1 - QP0)), functools.partial(paced, piece))
        if first:
            for par in range(2):
                add_ln(clock, cfg[par], cfg[2:], 2 * nx + par, xn_g, par,
                       functools.partial(lambda par_, i: xin[nx, pl.ds(i * 16, 16), par_ * TB:(par_ + 1) * TB], par))
        for r0, nt, tiles in ((0, 2, (0, 4, 8)), (TC, 2, (2, 6, 10)), (2 * TC, 1, (12, 13))):
            def R(k):
                return wq[pl.ds(r0, nt * 64), _lt(k)]

            def L(k):
                return sq_scr[k, 0] if first else jnp.concatenate([sq_scr[k, 0], sq_scr[k, 1]], axis=0)

            def P(k):
                return _dot_nt(_up(L(k)), _up(R(k)))

            def T(j, kind):
                rhs = _up(R(15 + 3 * j + kind))
                if nt == 1 and kind == 2:
                    lhs = L(15 + kind)
                    return jnp.concatenate([_dot_nt(_up(lhs[k:k + 32]), rhs) for k in range(0, lhs.shape[0], 32)],
                                           axis=0)
                return _dot_nt(_up(L(15 + kind)), rhs)

            def PT(k, j, kind):
                return _dot_nt(_up(jnp.concatenate([L(k), L(15 + kind)], axis=1)),
                               _up(jnp.concatenate([R(k), R(15 + 3 * j + kind)], axis=1)))

            def emit(col, half, v):
                for k in range(nt):
                    for q_ in range(2):
                        rows_ = pl.ds(base + (HALO + (2 * q_ + half) * TB), TB)
                        qall[tiles[col] + k, rows_, :] = v[q_ * TB:(q_ + 1) * TB, _lt(k)]
            if not first:
                hk_outputs(P, T, PT, emit, nt == 1)
                continue
            for j in range(len(tiles)):
                both = T(j, 2)
                clock.t += 32 * nt
                for t in range(2):
                    for k in range(nt):
                        lhs = [L(3 * t + i) for i in range(3)] + [L(15 + t)]
                        lhs[0] = gate(lhs[0], clock)
                        rhs = [wq[pl.ds(r0 + k * 64, 64), _lt(n)]
                               for n in [wq_slot(i, j) for i in range(3)] + [15 + 3 * j + t]]
                        v = _dot_nt(_up(jnp.concatenate(lhs, axis=1)), _up(jnp.concatenate(rhs, axis=1))) + both[:, _lt(k)]
                        qall[tiles[j] + k, pl.ds(base + (HALO + t * TB), TB), :] = v
                        clock.tick(128, v, QTK)
        assert not clock.pending()
        if first:
            q_left(True)

    def row_group(blk, par, r, nw, nv, mids=None):
        base = _al(blk * TB, TB)
        lo = lax.broadcasted_iota(jnp.int32, (RB, 128), 1) < KY
        r0 = r * RB

        def ld(t, w):
            return qall[t, pl.ds(base + (HALO + r0 - DIL * w), RB), :]
        dep = yield
        cs = tie(jnp.full((RB, 128), c2e, f32), dep)
        q = [ld(t, 0) * cs for t in QT] + [jnp.where(lo, pltpu.roll(ld(13, 0), KY, 1), 0.0) * cs]
        sc = []
        for w in range(W):
            if w and w % nw == 0:
                dep = yield
                q = [tie(q[0], dep)] + q[1:]
            acc = None
            for j, t in enumerate(KT):
                p = q[j] * ld(t, w)
                acc = p if acc is None else acc + p
            acc = acc + pltpu.roll(acc, 64, 1)
            if mids is not None:
                mids[r] = pltpu.bitcast(acc, u32)
            acc = acc + pltpu.roll(acc, 32, 1)
            if r0 - DIL * w < 0:
                pos = blk * TB + r0 + lax.broadcasted_iota(jnp.int32, (RB, 128), 0)
                acc = jnp.where(pos >= DIL * w, acc, neg)
            sc.append(acc)
        m = _tree(jnp.maximum, sc)
        e = [jnp.exp2(sc[w] - m) for w in range(W)]
        l = _tree(jnp.add, e)
        rinv = pl.reciprocal(l, approx=True)
        rinv = rinv * (2.0 - l * rinv)
        outs = []
        for j, t in enumerate(VT):
            if j and j % nv == 0:
                dep = yield _tree(jnp.bitwise_or, [pltpu.bitcast(v, u32) for v in outs])
                outs = []
                e = [tie(e[0], dep)] + e[1:]
            acc = None
            for w in range(W):
                p = e[w] * ld(t, w)
                acc = p if acc is None else acc + p
            o = acc * rinv
            o_s[par * 5 + j, pl.ds(r0, RB), :] = o
            outs.append(o)
        yield _tree(jnp.bitwise_or, [pltpu.bitcast(v, u32) for v in outs])

    def add_rows(clock, t0, blk, par, r, cfg):
        nw, nv, step, gap, d1, d2 = cfg
        gen = row_group(blk, par, r, nw, nv)
        next(gen)
        n1, n2 = -(-W // nw), -(-5 // nv)
        for k in range(n1):
            clock.add_due(t0 + k * step, gen.send, d1)
        for k in range(n2 - 1):
            clock.add_due(t0 + (n1 - 1) * step + gap + k * step, gen.send, d2)

    def row_chain(blk, lag, dep):
        mids, fins = {}, {}
        for r in range(nr):
            gen = row_group(blk, blk, r, W, 5, mids)
            next(gen)
            if r:
                dep = pltpu.bitcast(mids[r - 1] | fins[r - lag] if r >= lag else mids[r - 1], f32)
            fins[r] = gen.send(dep)
        return _tree(jnp.bitwise_or, [fins[r] for r in range(nr - lag, nr)])

    wo_seq = []
    for pos, k in enumerate(WORD):
        if pos in (0, 2):
            wo_seq += [('r', pos // 2, k_) for k_ in range(3)]
        wo_seq.append(('p', k))

    def wo_rhs(off):
        lo = lax.broadcasted_iota(jnp.int32, (TB, 128), 1) < KY

        rhs = {}
        for it in wo_seq:
            z = zero(wo_seq.index(it)) if off is None else off

            def O(t, j):
                return o_s[t * 5 + j, pl.ds(z, TB), :]
            if it[0] == 'p':
                v = _ssum([(O(t, j), sg) for j, t, sg in _HK_B[it[1]]])
            elif it[2] == 0:
                v = O(it[1], 3)
            else:
                v = jnp.where(lo, O(it[1], 2 + it[2]), O(it[1], 5 - it[2]))
            rhs[it] = v.astype(bf16)
        return rhs

    def wo_mm(blk0, rhs):
        res = {}
        for it in wo_seq:
            if it[0] == 'p':
                lhs = wo2[pl.ds(0, D3 // 2), _lt(it[1])]
            else:
                lhs = wo2[:, _lt(15 + it[2])]
            res[it] = _dot_nt(_up(lhs), rhs[it])
        for t in range(2):
            both = res['r', t, 2]
            rem = xres[blk0 + t] + jnp.concatenate([res['r', t, 0] + both, res['r', t, 1] + both], axis=0)
            y = jnp.concatenate([_ssum([(res['p', k], sg) for k, sg in _HK_C[i, t]]) for i in range(3)], axis=0)
            xres[blk0 + t] = y + rem

    def a_left(which=range(15), dep=None, cb=None):
        for n in which:
            v = _ssum([(xn_f[t, pl.ds(zero(n) + i * D3, D3), :], sg)
                       for (i, t), lst in _HK_C.items() for k, sg in lst if k == n])
            if dep is not None:
                v = jnp.concatenate([tie(v[0:8], dep), v[8:2 * KY], tie(v[2 * KY:2 * KY + 8], dep), v[2 * KY + 8:]],
                                    axis=0)
            t1 = pltpu.bitcast(v[:2 * KY].astype(bf16).T, u32)
            t2 = pltpu.bitcast(jnp.concatenate([v[2 * KY:], v[2 * KY:]], axis=0).astype(bf16).T, u32)
            if dep is None:
                arrange(n, t1, t2)
                cb(t1[0:8])
                cb(t2[0:8])
            else:
                st_s[2 * n] = t1
                st_s[2 * n + 1] = t2

    def arrange(n, t1, t2):
        lo = lax.broadcasted_iota(jnp.int32, (TB // 2, 128), 1) < KY
        s_scr[3 * n] = t1
        s_scr[3 * n + 1] = jnp.where(lo, t1, t2)
        s_scr[3 * n + 2] = jnp.where(lo, t2, t1)

    def a_arrange(n, dep):
        st_s[30, pl.ds(0, 8), :] = pltpu.bitcast(dep, u32)
        arrange(n, st_s[2 * n, pl.ds(zero8, TB // 2), :], st_s[2 * n + 1, pl.ds(zero8, TB // 2), :])

    k0 = math.sqrt(2.0 / math.pi)
    k1 = k0 * 0.044715

    def ffn(j, c0, script):
        clock = _Timeline()
        b0 = (2 * j) % NB
        an = (2 * j + 2) % NB
        acc = [None] * 57
        hs = {}
        lns, lq, staged, nrows = [], [], set(), 0

        pend = []

        def advance(keep):
            while len(pend) > keep:
                pend.pop(0)()

        def written(k):
            clock.due.append(lambda: pltpu.bitcast(p_s[k][pl.ds(zero8, 8), 0:128], u32))

        def gu(p):
            c, m = c0 + p // 2, p % 2
            h = hs.setdefault(p // 2, [[None, None, None] for _ in range(3)])

            def mm(n, kind):
                lhs = gate(s_scr[3 * n + kind], clock)
                return _dot(_up(lhs), _up(pw[c, pl.ds((3 * n + kind) * (TC // 2), TC // 2), m * TC:(m + 1) * TC]))

            def get(name):
                return p_s[PSLOT[name]][pl.ds(zero8, TB), :]

            def post(n, v):
                adds, keep, emits = GU_POST[n]
                if keep[0] is not None:
                    p_s[PSLOT[keep[0]]][...] = v
                    written(PSLOT[keep[0]])
                w_ = v
                for name, sg in adds:
                    w_ = w_ + get(name) if sg == 1 else w_ - get(name)
                if keep[1] is not None:
                    p_s[PSLOT[keep[1]]][...] = w_
                    written(PSLOT[keep[1]])
                if emits is not None:
                    col, half = emits
                    if m == 1:
                        k_ = 17 + 9 * ((p // 2) % NHS) + 3 * col
                        hv = w_ * p_s[11 + 2 * col + half][pl.ds(zero8, TB), :]
                        p_s[k_ + half][...] = hv
                        written(k_ + half)
                        h[col][half] = k_ + half
                        if h[col][1 - half] is not None:
                            p_s[k_ + 2][...] = hv + p_s[k_ + 1 - half][pl.ds(zero8, TB), :]
                            written(k_ + 2)
                            h[col][2] = k_ + 2
                    else:
                        p_s[11 + 2 * col + half][...] = w_ + w_ * jnp.tanh(w_ * (k0 + k1 * (w_ * w_)))
                        written(11 + 2 * col + half)
            for n in GU_ORD:
                both = mm(n, 2)
                v = jnp.concatenate([mm(n, 0) + both, mm(n, 1) + both], axis=1)
                pend.append(functools.partial(post, n, v))
                advance(PLAG)
                clock.tick(96, both, GTK)

        todo = [sum(any(i_ == i for i_, _, _ in z) for z in _Z6) for i in range(6)]

        def gather(i):
            if last:
                ys = [_ssum([(acc[n], sg) for n, sg in sorted(_C6[i, t], key=lambda z: _order6().index(z[0]))])
                      for t in range(2)]
            else:
                t0, t1 = dict(_C6[i, 0]), dict(_C6[i, 1])
                both = _ssum([(acc[n], sg) for n, sg in t0.items() if n in t1])
                ys = (_ssum([(acc[n], sg) for n, sg in t0.items() if n not in t1]) + both,
                      _ssum([(acc[n], sg) for n, sg in t1.items() if n not in t0]) - both)
            for t in range(2):
                x2 = xres[b0 + t, pl.ds(i * D6, D6), :] + 0.5 * ys[t]
                xres[b0 + t, pl.ds(i * D6, D6), :] = x2
                xin[j % NP, pl.ds(i * D6, D6), t * TB:(t + 1) * TB] = x2.astype(bf16)
            if last and i in ORD6[:OSPL]:
                @pl.when(g == 1)
                def _():
                    _cp_rows(i, o_hbm, xin, sems).start()

        def down(ps, final):
            cs = ps[::2]
            hsl = [hs.pop(p // 2) for p in cs]
            for pos, i in enumerate(_order6()):
                while any(h_[j_ % 3][d_] is None for h_ in hsl for j_, d_, _ in _B6[i]):
                    advance(len(pend) - 1)
                au = [pw[c0 + p // 2, pl.ds(R_SD + (i // 2) * (D6 // 2), D6 // 2), _lt(i % 2)] for p in cs]
                au[0] = gate(au[0], clock)
                lhs = jnp.concatenate(au, axis=1)
                rhs = jnp.concatenate([_ssum([(p_s[h_[j_ % 3][d_]][pl.ds(zero(pos % 21), TB), _lt(j_ // 3)], sg)
                                              for j_, d_, sg in _B6[i]]) for h_ in hsl], axis=1).astype(bf16)
                r = _dot_nt(_up(lhs), rhs)
                acc[i] = r if acc[i] is None else r + acc[i]
                if final:
                    for i_ in sorted({i_ for i_, _, _ in _Z6[i]}):
                        todo[i_] -= 1
                        if not todo[i_]:
                            gather(i_)
                if pos % DADV == 0:
                    advance(max(len(pend) - 1, 0))
                clock.tick(24 * len(cs), acc[i], DTK)

        pg = pd = 0
        for tok in script:
            if tok == 'G':
                gu(pg)
                pg += 1
            elif tok[0] == 'D':
                down(list(range(pd, pd + int(tok[1:]))), pd + int(tok[1:]) == script.count('G'))
                pd += int(tok[1:])
            elif tok == 'W':
                assert not clock.pending() and nrows == 2 * nr
                advance(0)
                wo_mm(an, wo_rhs(None))
                clock.t += 1152
            elif tok[0] == 'n':
                lns.append(add_ln(clock, clock.t + int(tok[3:]), LNJ + (JDL,), an + int(tok[1]), xn_f, int(tok[1])))
            elif tok[0] == 'm':
                lq.append(add_ln(clock, clock.t + int(tok[3:]), LNJ + (JDL,), (2 * j + 6) % NB + int(tok[1]), xn_g,
                                 int(tok[1])))
            elif tok[0] == 'k':
                _, t0, dt = tok.split('+')

                def qleft(which, dep):
                    assert len(lq) == 2 and not any(st['left'] for st in lq)
                    q_left(False, which, dep, (j + 1) % 2)
                    return sq_scr[which[0], (j + 1) % 2, pl.ds(zero8, 8), :]
                for k in range(NQL):
                    clock.add_due(clock.t + int(t0) + k * int(dt),
                                  functools.partial(qleft, range(k * 18 // NQL, (k + 1) * 18 // NQL)), LDL)
            elif tok[0] == 'l':
                _, t0, dt = tok.split('+')

                def left(which, dep):
                    assert len(lns) == 2 and not any(st['left'] for st in lns)
                    staged.update(which)
                    a_left(which, dep)
                    return st_s[0, pl.ds(zero8, 8), :]
                for k in range(NLEFT):
                    clock.add_due(clock.t + int(t0) + k * int(dt),
                                  functools.partial(left, range(k * 15 // NLEFT, (k + 1) * 15 // NLEFT)), LDL)
            elif tok[0] == 'c':
                _, t0, dt = tok.split('+')
                assert pg == 2 * NCH

                def place(k, dep):
                    assert k in staged
                    a_arrange(k, dep)
                for k in range(15):
                    clock.add(clock.t + int(t0) + k * int(dt), functools.partial(place, k))
            else:
                n, t0, dt = tok[1:].split('+')
                for k in range(int(n)):
                    add_rows(clock, clock.t + int(t0) + k * int(dt), an + nrows // nr, nrows // nr, nrows % nr,
                             RG + (RDL, JDL))
                    nrows += 1
        assert pg == pd and not clock.pending()

    if last:
        ffn(2 * NP - 1, g * NPC, SCRIPT_F)
        return
    assert NCH == NP - 2

    late = [(c, m) for c in range(NCH) for m in range(3) if c >= NCH - LAGS[m]]

    def prologue():
        cp_x(0).start()
        for sec in range(3):
            for cp in cp_qkv(sec):
                cp.start()
        qall[:, pl.ds(0, HALO), :] = jnp.zeros((16, HALO, 128), f32)
        cp_x(0).wait()
        for t in range(2):
            x = xin[0, :, t * TB:(t + 1) * TB].astype(f32)
            xres[t] = x
            mean, rstd = _ln_stats(x)
            xn_g[t, pl.ds(zero8, D), :] = (xres[t] - mean) * rstd
        q_left(True)
        for sec in range(3):
            for cp in cp_qkv(sec):
                cp.wait()
            if sec == 0:
                cp_x(1).start()
                cp_x(2).start()
                cp_wo().start()
                for c in range(NCH):
                    if 3 + c < NP:
                        cp_x(3 + c).start()
                    for m in range(3):
                        if c == 0 or c > LAGS[m]:
                            cp_unit(max(c - LAGS[m], 0), m).start()
                for c, m in late:
                    cp_unit(c, m).start()
            transpose_qkv(sec)
            build_wq(sec)

    def first_attention():
        cp_x(2).wait()
        q_step(1, CFG_QA, rows=True)
        cp_wo().wait()
        build_wo()
        wo_mm(0, wo_rhs(0))

    def startup_step(c, carry):
        @pl.when(c + 3 < NP)
        def _():
            cp_x(c + 3).wait()
        for m in range(3):
            if LAGS[m]:
                @pl.when(jnp.logical_or(c == 0, c > LAGS[m]))
                def _():
                    cp_unit(jnp.maximum(c - LAGS[m], 0), m).wait()
            else:
                cp_unit(c, m).wait()
        q_step(c + 2, CFG_Q1, chunk=c)
        return carry

    def startup_tail():
        pieces = []
        for c, m in late:
            cp_unit(c, m).wait()
            pieces += prep_pieces(c, m)
        npt = 30 + 2 * TLN
        done = []

        def pace(v):
            pw[g >> 20, pl.ds(R_END, 8), 0:128] = v
            done.append(v)
            for piece in pieces[(len(done) - 1) * len(pieces) // npt:len(done) * len(pieces) // npt]:
                piece()
        for t in range(2):
            mean, rstd = _ln_stats(xres[t])
            xn = (xres[t, pl.ds(zero8, D), :] - mean) * rstd
            xn_f[t] = xn
            for k in range(TLN):
                pace(pltpu.bitcast(xn[k * 64:k * 64 + 8], u32))
        a_left(cb=pace)
        assert len(done) == npt

    @pl.when(g == 0)
    def _():
        prologue()
        cp_x(1).wait()
        q_step(0, CFG_Q0, sums=True)
        first_attention()
        lax.fori_loop(0, NCH, startup_step, 0)
        startup_tail()

    @pl.when(jnp.logical_and(g >= NP - 1, g % 2 == 1))
    def _():
        q_step(g - (NP - 1))

    ffn(g, 0, SCRIPT)

    @pl.when(g >= NP)
    def _():
        _cp_out(g - NP, o_hbm, xin, sems).start()


def _cp_out(k, o_hbm, xin, sems):
    return pltpu.make_async_copy(xin.at[k], o_hbm.at[:, pl.ds(_al(k * 2 * TB, 128), 2 * TB)], sems.at[4 + k])


def _cp_rows(i, o_hbm, xin, sems):
    k, n = xin.shape[0] - 1, xin.shape[1] // 6
    return pltpu.make_async_copy(xin.at[k, pl.ds(i * n, n), :], o_hbm.at[pl.ds(i * n, n), pl.ds(k * 2 * TB, 2 * TB)],
                                 sems.at[4 + k])


def _kernel(*refs, D, DF, S):
    def body(last, g, carry):
        _step(g, last, *refs, D=D, DF=DF, S=S)
        return carry
    NP = S // (2 * TB)
    lax.fori_loop(0, 2 * NP - 1, functools.partial(body, False), 0)
    lax.fori_loop(0, 2, functools.partial(body, True), 0)
    o_hbm, xin, sems = refs[6], refs[7], refs[24]
    for i in ORD6[OSPL:]:
        _cp_rows(i, o_hbm, xin, sems).start()
    for k in range(NP - 1):
        _cp_out(k, o_hbm, xin, sems).wait()
    for i in range(6):
        _cp_rows(i, o_hbm, xin, sems).wait()


@jax.jit
def pallas_interleave_layers__sliding_local_dilated__glu_gated_geglu__prompt_kernel(
    A_x, A_wqkv, A_wo, B_x, B_w_gate, B_w_up, B_w_down):
    B, S, D = A_x.shape
    DF = B_w_gate.shape[1]
    NB = S // TB
    NP = NB // 2
    NCH = DF // CW
    xT = A_x.reshape(S, D).T
    wdT = B_w_down.T
    hbm = pl.BlockSpec(memory_space=pltpu.HBM)
    outT = pl.pallas_call(
        functools.partial(_kernel, D=D, DF=DF, S=S),
        in_specs=[hbm] * 6,
        out_specs=hbm,
        out_shape=jax.ShapeDtypeStruct((D, S), A_x.dtype),
        scratch_shapes=[
            pltpu.VMEM((NP, D, 2 * TB), bf16),
            pltpu.VMEM((D, 3 * D), bf16),
            pltpu.VMEM((D, D), bf16),
            pltpu.VMEM((5, 14 * 128, 128), f32),
            pltpu.VMEM((WQR, 27 * 128), u32),
            pltpu.VMEM((D // 2, 640), u32),
            pltpu.VMEM((D // 4, 18 * 128), u32),
            pltpu.VMEM((NCH, 3, D, CW), bf16),
            pltpu.VMEM((NCH, 45 * (TC // 2) + 15 * (D // 6) + 16, 2 * TC), u32),
            pltpu.VMEM((16, S + QPAD, 128), f32),
            pltpu.VMEM((11, TB, 128), f32),
            pltpu.VMEM((NB, D, TB), f32),
            pltpu.VMEM((2, D, TB), f32),
            pltpu.VMEM((2, D, TB), f32),
            pltpu.VMEM((45, TB // 2, TC), u32),
            pltpu.VMEM((31, TB // 2, TC), u32),
            pltpu.VMEM((18, 2, TB // 2, TC), u32),
            pltpu.SemaphoreType.DMA((4 + NP + 3 * NCH,)),
        ] + [pltpu.VMEM((TB, 2 * TC), f32)] * (17 + 9 * NHS),
        compiler_params=pltpu.CompilerParams(
            vmem_limit_bytes=110 * 1024 * 1024,
            disable_bounds_checks=True,
            disable_semaphore_checks=True,
        ),
    )(xT, A_wqkv, A_wo, B_w_gate, B_w_up, wdT)
    return outT.T.reshape(B, S, D)
```

```python
import functools
import math
import jax
import jax.numpy as jnp
from jax import lax
import jax.experimental.pallas as pl
import jax.experimental.pallas.tpu as pltpu

DH = 18
W = 8
DIL = 2
HALO = 16
EPS = 1e-5
TB = 128
RB = 8
TC = 128
CW = 6 * TC
WQR = 320
KY = 64
QPAD = 40

SCRIPT = ('m0+50,m1+2804,k+8550+68,G,R7+74+200,G,G,R2+96+200,G,R9+300+260,D4,'
          'G,R7+74+200,G,G,R7+74+200,G,G,W,n0+300,n1+876,l+2900+80,G,G,G,c+600+192,D8').split(',')
SCRIPT_F = 'G,G,G,G,G,G,D6'.split(',')
GU_ORD = (8, 6, 7, 11, 3, 1, 10, 14, 9, 5, 0, 13, 12, 4, 2)
ORD6 = (0, 4, 3, 1, 5, 2)
WORD = (0, 1, 2, 6, 7, 8, 9, 10, 11, 12, 13, 14, 3, 4, 5)
PLAG, DADV, GTK, DTK, QTK = 6, 2, 2, 2, 8
LNJ = (12, 9, 48, 48)
RG = (2, 1, 24, 420)
RDL, JDL, LDL = 600, 300, 500
NLEFT, NQL, TLN, NHS, OSPL = 15, 18, 9, 4, 4
CFG_Q0 = (40, 1816, 18, 18, 48, 48, 350)
CFG_QA = (300, 748, 6, 6, 32, 64, 350)
CFG_Q1 = (40, 1456, 9, 9, 64, 64, 300)
QA_T = (300, 1000, 4, 3850)
QP0, QP1, QFR = 100, 3850, 0.6
DCUT = (0, 2, 4, 6, 8, 10, 12, 21, 30, 39, 48, 57)
LAGS = (1, 1, 0)

f32 = jnp.float32
bf16 = jnp.bfloat16
u32 = jnp.uint32
NT = (((1,), (1,)), ((), ()))


def _al(i, n):
    return i if isinstance(i, int) else pl.multiple_of(i, n)


def _lt(k):
    return slice(k * 128, (k + 1) * 128)


def _pk(x):
    return pltpu.bitcast(x.astype(bf16), u32)


def _up(x):
    return pltpu.bitcast(x, bf16)


def _dot(a, b):
    return jnp.dot(a, b, preferred_element_type=f32)


def _dot_nt(a, b):
    return lax.dot_general(a, b, NT, preferred_element_type=f32)


def _tree(fn, xs):
    xs = list(xs)
    while len(xs) > 1:
        xs = [fn(xs[i], xs[i + 1]) for i in range(0, len(xs) - 1, 2)] + ([xs[-1]] if len(xs) % 2 else [])
    return xs[0]


def _ln_stats(x, nacc=4):
    n = x.shape[0]
    c = x[0:1]
    s1 = [None] * nacc
    s2 = [None] * nacc
    for i in range(n // 8):
        d = x[i * 8:(i + 1) * 8] - c
        k = i % nacc
        s1[k] = d if s1[k] is None else s1[k] + d
        dd = d * d
        s2[k] = dd if s2[k] is None else s2[k] + dd
    m = jnp.sum(_tree(jnp.add, s1), axis=0, keepdims=True) * (1.0 / n)
    v = jnp.sum(_tree(jnp.add, s2), axis=0, keepdims=True) * (1.0 / n) - m * m
    v = jnp.maximum(v, 0.0)
    return c + m, lax.rsqrt(v + EPS)


_HK_A = (
    ((0, 0, 1), (0, 2, -1), (1, 0, -1)), ((0, 0, 1), (0, 1, -1), (2, 0, -1)), ((1, 1, 1), (0, 1, -1), (1, 2, -1)),
    ((1, 1, 1), (1, 0, -1), (2, 1, -1)), ((2, 2, 1), (0, 2, -1), (2, 1, -1)), ((2, 2, 1), (1, 2, -1), (2, 0, -1)),
    ((0, 1, 1),), ((0, 1, 1), (1, 0, -1)), ((1, 0, 1),),
    ((0, 2, 1),), ((0, 2, 1), (2, 0, -1)), ((2, 0, 1),),
    ((1, 2, 1),), ((2, 1, 1), (1, 2, -1)), ((2, 1, 1),),
)
_HK_C = {
    (0, 0): ((0, 1), (7, 1), (8, 1), (9, 1), (6, -1)),
    (0, 1): ((1, 1), (6, 1), (10, 1), (11, 1), (9, -1)),
    (1, 0): ((2, 1), (7, 1), (8, 1), (12, 1), (6, -1)),
    (1, 1): ((3, 1), (6, 1), (13, 1), (14, 1), (2, -1), (7, -1)),
    (2, 0): ((5, 1), (9, 1), (12, 1), (13, 1), (4, -1), (10, -1)),
    (2, 1): ((4, 1), (10, 1), (11, 1), (14, 1), (9, -1)),
}
_HK_B = (((0, 0, 1),), ((0, 1, 1),), ((1, 0, 1),), ((1, 0, 1), (1, 1, 1)), ((2, 1, 1),), ((2, 0, 1), (2, 1, 1)),
         ((0, 1, 1), (1, 1, 1)), ((0, 1, 1), (1, 0, 1), (1, 1, 1)), ((0, 0, 1), (0, 1, 1), (1, 0, 1), (1, 1, 1)),
         ((0, 0, 1), (2, 0, 1)), ((0, 0, 1), (2, 0, 1), (2, 1, 1)), ((0, 0, 1), (0, 1, 1), (2, 0, 1), (2, 1, 1)),
         ((1, 0, 1), (2, 0, 1)), ((1, 0, 1), (2, 1, -1)), ((1, 1, 1), (2, 1, 1)))


_HK6 = (
    '+00-01-02-30-50 +00 +00;+00-03+05-10-20 +01 +01;-01+11+13-15-40+41 +11 -10+11;-04-10+11+14+31+51 +12 +10;'
    '-02-12+21+22-23-25+35-42 +21 -20+21;-12-20+21+22+24-32-52+53 +22 +20;-03+31-32+33+43 +30 +30-31;'
    '+13-23-30+33-34 +32 +31;-04+34-40+41+42+44+54 +40 +40;-04+14-24-40-43+44-45 +41 +41;'
    '-05-12+35+45-51-52+53+55 +50 +50-51;+15+21-25+35+50-53-54+55 +52 +51;+01-40 +00+10 +00-01+10-11;'
    '+01-10 +00+12 +01-10+11;-04+10 +02+12 +01+11;+02 +00+20 +00-01+20-21;+02-20 +00+22 +01-20+21;'
    '+20 +02+22 +01+21;+03 +01+31 -00+01-30+31;+03-30 +01+32 +00+30-31;+30 +02+32 +00+30;+05 +01-51 +00-01+50-51;'
    '+05+50 +01-52 -00-50+51;+50 +02-52 +00+50;+31 +10-30 -10+30;+13-31 +11+30 +10-31;+13 +11-31 -11+31;'
    '+40-41 +10-40 +10-11-40+41;+04-14-40+41 +12-40 +10-11+41;+04-14 +12-42 +11-41;+12-51 +10+50 +10-50;'
    '+15+51 +11-50 -10+51;+15-21 +11+51 +11-51;+32+53 +20+30 +20+30;-23+32 +21-30 +20+31;+23-35 +21+31 +21+31;'
    '+42 +20-40 +20-21+40-41;+24+42 +22-40 -20+21+41;+24 +22-42 -21-41;+12+52-53 +20+50 +20+50;'
    '+12+21-25+35+52-53 +21-50 +20+51;-21+25-35 +21+51 +21+51;+43 +31+41 +30-31-40+41;+34+43 +32+41 -30+31+40;'
    '+34 +32+42 +30-40;+45 +41+51 -40+41+50-51;+45+54 +41+52 +40-50+51;+54 +42+52 -40+50;'
    '+40 +01+11+41 -00+01-10+11-40+41;-04+40 +02+12+41 +00-01+10-11+40;+04 +02+12+42 +00+10+40;'
    '+12 +10-20+50 -10+11-20+21+50-51;+12+21 +10-22+50 -11+20-21+51;+21 +12-22+52 +11+21-51;'
    '+35 +21+31+51 -20+21-30+31+50-51;+35+53 +21+31+52 +20+30-50+51;+53 +22+32+52 -20-30+50'
)


def _terms(txt):
    return tuple((int(txt[i + 1]), int(txt[i + 2]), 1 if txt[i] == '+' else -1) for i in range(0, len(txt), 3))


_A6, _B6, _Z6 = zip(*[[_terms(f) for f in row.split(' ')] for row in _HK6.split(';')])
_C6 = {(i, t): [(n, sg) for n, z in enumerate(_Z6) for i_, t_, sg in z if (i_, t_) == (i, t)]
       for i in range(6) for t in range(2)}


def _order6():
    early = [n for n, b in enumerate(_B6) if all(j % 3 == 0 or (j % 3 == 1 and d == 1) for j, d, _ in b)]
    early.sort(key=lambda n: max(d != 1 for _, d, _ in _B6[n]))
    out = list(early)
    for i in ORD6:
        out += [n for n, z in enumerate(_Z6) if n not in out and any(i_ == i for i_, _, _ in z)]
    return out


def _ssum(terms):
    terms = sorted(terms, key=lambda z: -z[1])
    acc = terms[0][0] if terms[0][1] == 1 else -terms[0][0]
    for v, sg in terms[1:]:
        acc = acc + v if sg == 1 else acc - v
    return acc


GU_POST = {
    8: ((), ('p8', None), None),
    7: ((('p8', 1),), (None, 't7'), None),
    3: ((('t7', 1),), (None, 's1'), None),
    6: ((), ('p6', None), None),
    14: ((('p6', 1), ('s1', 1)), ('p14', None), (1, 1)),
    12: ((('p9', 1), ('s2', 1)), ('p12', None), (2, 0)),
    13: ((), ('p13', None), None),
    2: ((('p12', 1), ('p13', 1), ('s1', 1)), (None, None), (1, 0)),
    11: ((), ('p11', None), None),
    10: ((('p11', 1),), (None, 't10'), None),
    5: ((('t10', 1),), (None, 's2'), None),
    9: ((), ('p9', None), None),
    4: ((('p14', 1), ('s2', 1), ('p13', -1)), (None, None), (2, 1)),
    0: ((('p8', 1), ('p9', 1), ('t10', 1)), (None, None), (0, 0)),
    1: ((('p6', 1), ('p11', 1), ('t7', 1)), (None, None), (0, 1)),
}
PSLOT = {k: i for i, k in enumerate(('p8', 't7', 's1', 'p6', 'p14', 'p12', 'p13', 'p11', 't10', 's2', 'p9'))}


class _Timeline:
    def __init__(self):
        self.t = 0
        self.jobs = []
        self.due = []

    def add(self, when, fn):
        self.jobs.append((when, len(self.jobs), fn))
        self.jobs.sort(key=lambda z: z[:2])

    def add_due(self, when, job, delay):
        def run(dep):
            val = job(dep)
            if val is not None:
                self.add(self.t + delay, lambda _: self.due.append(lambda: val))
        self.add(when, run)

    def pending(self):
        return [j for j in self.jobs if getattr(j[2], '__name__', '') != '<lambda>']

    def tick(self, dur, v, n):
        for k in range(n):
            self.t += dur // n
            r = k * (v.shape[0] // n)
            while self.jobs and self.jobs[0][0] <= self.t:
                self.jobs.pop(0)[2](v[r:r + 8, 0:128])


def _step(g, phase, x_hbm, wqkv_hbm, wo_hbm, wg_hbm, wu_hbm, wd_hbm, o_hbm,
          xin, wqkv_raw, wo_raw, tmp, wq, woT, wo2, raw, pw, qall, o_s, xres, xn_f, xn_g, s_scr, st_s, sq_scr,
          sems, *p_s, D, DF, S):
    last = phase == 'last'
    NB = S // TB
    NP = NB // 2
    NCH = DF // CW
    NPC = NCH // 2
    D3 = D // 3
    D6 = D // 6
    nr = TB // RB
    hh = D // 4
    zero8 = pl.multiple_of((g >> 20) * 8, 8)
    zvec = jnp.full((8, 128), (g >> 20).astype(u32), u32)

    def zero(k):
        return pl.multiple_of((g >> (8 + k)) * 8, 8)

    def tie(x, dep):
        return pltpu.bitcast(pltpu.bitcast(x, u32) | (pltpu.bitcast(dep, u32) & zvec), f32)

    def gate(lhs, clock):
        if not clock.due:
            return lhs
        pr = _tree(jnp.bitwise_or, [k() for k in clock.due]) & zvec
        del clock.due[:]
        return jnp.concatenate([lhs[0:8] | pr, lhs[8:]], axis=0)

    QSEC = ((0, 5), (5, 9), (9, 14))

    def cp_qkv(sec):
        out = []
        for j in range(*QSEC[sec]):
            n = min(128, 3 * D - j * 128)
            out.append(pltpu.make_async_copy(wqkv_hbm.at[:, pl.ds(j * 128, n)], wqkv_raw.at[:, pl.ds(j * 128, n)],
                                             sems.at[sec]))
        return out

    def cp_wo():
        return pltpu.make_async_copy(wo_hbm, wo_raw, sems.at[3])

    def cp_x(k):
        return pltpu.make_async_copy(x_hbm.at[:, pl.ds(_al(k * 2 * TB, 128), 2 * TB)], xin.at[k], sems.at[4 + k])

    def cp_unit(c, m):
        return pltpu.make_async_copy((wg_hbm, wu_hbm, wd_hbm)[m].at[:, pl.ds(_al(c * CW, 128), CW)], raw.at[c, m],
                                     sems.at[4 + NP + 3 * c + m])

    R_SD = 45 * (TC // 2)
    R_END = R_SD + 15 * (D3 // 2)

    def hk_a_ops(load, minus=None):
        blk = {}
        for i in range(3):
            for j in range(3):
                blk[i, j] = load(i, j).astype(f32)
                if minus is not None:
                    blk[i, j] = blk[i, j] - minus(i, j).astype(f32)
        return [_pk(_ssum([(blk[i, j], sg) for i, j, sg in terms])) for terms in _HK_A]

    def prep_pieces(c, m):
        def ld(r, cs):
            return lambda i, j: raw[c, m, pl.ds(i * D3 + r, 16), pl.ds((3 * cs + j) * TC, TC)]

        def gu_piece(q, r, cs, neg, kind, half):
            ops = hk_a_ops(ld(q * KY + r, cs), None if neg is None else ld(q * KY + r, neg))
            for k, t in enumerate(ops):
                pw.at[c][pl.ds((3 * k + kind) * (TC // 2) + (half * KY + r) // 2, 8), m * TC:(m + 1) * TC] = t

        def d_piece(r, q, ks):
            blk = {}
            cz = c + (g >> (8 + q))
            for k in ks:
                for i, j, _ in _A6[k]:
                    if (i, j) not in blk:
                        blk[i, j] = raw[cz, m, pl.ds(i * D6 + r, 16), pl.ds(j * TC, TC)].astype(f32)
                pw.at[c][pl.ds(R_SD + (k // 2) * (D6 // 2) + r // 2, 8), _lt(k % 2)] = _pk(
                    _ssum([(blk[i, j], sg) for i, j, sg in _A6[k]]))
        if m == 2:
            return [functools.partial(d_piece, r, q, range(DCUT[q], DCUT[q + 1]))
                    for r in range(0, D6, 16) for q in range(len(DCUT) - 1)]
        spec = ((0, 0, None, 0, 0), (1, 0, 1, 0, 1), (0, 1, None, 1, 0), (2, 1, 0, 1, 1),
                (2, 0, None, 2, 0), (1, 1, None, 2, 1))
        return [functools.partial(gu_piece, q, r, cs, neg, kind, half)
                for r in range(0, KY, 16) for q, cs, neg, kind, half in spec]

    def transpose_qkv(sec):
        for j in range(*QSEC[sec]):
            wd_ = min(128, 3 * D - j * 128)
            blk = wqkv_raw[:, j * 128:j * 128 + wd_].astype(f32)
            if wd_ < 128:
                blk = jnp.concatenate([blk, jnp.zeros((D, 128 - wd_), f32)], axis=1)
            bt = jnp.concatenate([blk, blk[D - KY:]], axis=0).T
            for t in range(5):
                tmp[t, pl.ds(j * 128, 128), :] = bt[:, t * 128:(t + 1) * 128]

    def wq_slot(i, j):
        return 24 + i if i == j else [n for n, t in enumerate(_HK_A) if t == ((i, j, 1),)][0]

    def build_wq(sec):
        lo = lax.broadcasted_iota(jnp.int32, (32, 128), 1) < KY
        for d in range(DH):
            tt = [tmp[t, pl.ds(sec * D + d, 32, stride=DH), :] for t in range(5)]
            ops = tt[:4] + [jnp.where(lo, tt[3], tt[4]), jnp.where(lo, tt[4], tt[3])]
            if d < 16:
                dst = [(sec, d * 16)]
            else:
                dst = ([(1, (d + 2) * 16)], [(1, d * 16)], [(0, d * 16), (0, (d + 2) * 16)])[sec]
            for j, row in dst:
                for k, v in enumerate(ops):
                    wq[pl.ds(row, 16), _lt(wq_slot(k, j) if k < 3 else 12 + 3 * j + k)] = _pk(v)

    def wq_sums(r, dep):
        ncol = 3 if r < 256 else 2
        pin = pltpu.bitcast(dep, u32) & zvec
        blk = {(i, j): _up(wq[pl.ds(r, 8), _lt(wq_slot(i, j))] | pin).astype(f32) for i in range(3) for j in range(ncol)}
        for n, terms in enumerate(_HK_A):
            if len(terms) > 1 and not (ncol == 2 and n in (4, 5)):
                wq[pl.ds(r, 8), _lt(n)] = _pk(_ssum([(blk[i, j], sg) for i, j, sg in terms if j < ncol]))

    def build_wo():
        for t in range(5):
            wd_ = min(128, D - t * 128)
            blk = wo_raw[:, t * 128:t * 128 + wd_].astype(f32)
            if wd_ < 128:
                blk = jnp.concatenate([blk, jnp.zeros((D, 128 - wd_), f32)], axis=1)
            tmp[t, pl.ds(0, D), :] = blk
        for t in range(5):
            rows = [tmp[t, pl.ds(d, 32, stride=DH), :] for d in range(DH)]
            ft = jnp.concatenate(rows + rows[16:], axis=0).T
            n = min(128, D - t * 128)
            woT[pl.ds(t * 64, n // 2), :] = _pk(ft[:n])
        for r in range(0, D3 // 2, 8):
            ops = hk_a_ops(lambda i, j: _up(woT[pl.ds(i * (D3 // 2) + r, 8), j * TC:(j + 1) * TC]))
            for k, t in enumerate(ops):
                wo2[pl.ds(r, 8), _lt(k)] = t
        lo = lax.broadcasted_iota(jnp.int32, (16, 128), 1) < KY
        for r in range(0, hh, 8):
            a3, a4, b3, b4 = [_up(woT[pl.ds(r0 + r, 8), c0:c0 + 128]).astype(f32)
                              for r0 in (0, hh) for c0 in (384, 512)]
            wo2[pl.ds(r, 8), _lt(15)] = _pk(jnp.where(lo, a3, a3 - b3))
            wo2[pl.ds(r, 8), _lt(16)] = _pk(jnp.where(lo, b3, b4 - a4))
            wo2[pl.ds(r, 8), _lt(17)] = _pk(jnp.where(lo, a4, b3))

    def q_left(plain, which=None, dep=None, slot=0):
        k1, k2, k3 = 3 * TC, 3 * TC + KY, 3 * TC + 2 * KY
        for n in (list(range(6 if plain else 15)) + [15, 16, 17]) if which is None else which:
            def X(t, r0, rows):
                return xn_g[t, pl.ds((zero8 if plain else zero(n)) + r0, rows), :]
            if n == 15:
                v = jnp.concatenate([X(0, k1, KY), X(0, k2, KY) - X(1, k2, KY)], axis=0)
            elif n == 16:
                v = jnp.concatenate([X(1, k1, KY), X(1, k3, KY) - X(0, k3, KY)], axis=0)
            elif n == 17:
                v = jnp.concatenate([X(0, k3, KY), X(1, k2, KY)], axis=0)
            elif plain:
                v = X(n // 3, (n % 3) * TC, TC)
            else:
                v = _ssum([(X(t, i * TC, TC), sg) for (i, t), lst in _HK_C.items() for k, sg in lst if k == n])
            if dep is not None:
                v = jnp.concatenate([tie(v[0:8], dep), v[8:]], axis=0)
            sq_scr[n, slot] = pltpu.bitcast(v.astype(bf16).T, u32)

    def add_ln(clock, t0, cfg, blk, dst, par, inp=None):
        np1, np2, step, gap, delay = cfg
        st = dict(s1=[], s2=[], left=np2)
        nv = D // 16

        def load(i):
            if inp is None:
                return xres[blk, pl.ds(zero8 + i * 16, 16), :]
            x = inp(i).astype(f32)
            xres[blk, pl.ds(i * 16, 16), :] = x
            return x

        def stats(k, dep):
            xs = []
            for i in range(k * nv // np1, (k + 1) * nv // np1):
                x = load(i)
                xs += [x[0:8], x[8:16]]
            if k == 0:
                st['c'] = jnp.broadcast_to(xs[0][0:1], (8, TB))
            c = tie(st['c'], dep)
            ds = [x - c for x in xs]
            st['s1'].append(_tree(jnp.add, ds))
            st['s2'].append(_tree(jnp.add, [d * d for d in ds]))
            return pltpu.bitcast(st['s1'][-1], u32) | pltpu.bitcast(st['s2'][-1], u32)

        def norm(k, dep):
            if k == 0:
                m = jnp.sum(_tree(jnp.add, st['s1']), axis=0, keepdims=True) * (1.0 / D)
                v = jnp.sum(_tree(jnp.add, st['s2']), axis=0, keepdims=True) * (1.0 / D) - m * m
                st['mean'] = st['c'] + m
                st['rstd'] = jnp.broadcast_to(lax.rsqrt(jnp.maximum(v, 0.0) + EPS), (8, TB))
            mean = tie(st['mean'], dep)
            off = 0 if inp is None else zero8
            for i in range(k * 2 * nv // np2, (k + 1) * 2 * nv // np2):
                dst[par, pl.ds(i * 8, 8), :] = (xres[blk, pl.ds(off + i * 8, 8), :] - mean) * st['rstd']
            st['left'] -= 1
            return pltpu.bitcast(dst[par, pl.ds(zero8, 8), :], u32)
        for k in range(np1):
            clock.add_due(t0 + k * step, functools.partial(stats, k), delay)
        for k in range(np2):
            clock.add_due(t0 + np1 * step + gap + k * step, functools.partial(norm, k), delay)
        return st

    def hk_outputs(P, T, PT, emit, two_cols):
        p8 = P(8)
        t7 = P(7) + p8
        s1 = PT(3, 1, 2) + t7
        p6 = P(6)
        p14 = P(14)
        emit(1, 1, T(1, 1) + (p6 + p14 + s1))
        p13 = P(13)
        if two_cols:
            emit(1, 0, PT(2, 1, 0) + (p13 + s1))
        else:
            p12 = P(12)
            emit(1, 0, PT(2, 1, 0) + (p12 + p13 + s1))
        p11 = P(11)
        t10 = P(10) + p11
        if not two_cols:
            s2 = PT(5, 2, 2) + t10
            p9 = P(9)
            emit(2, 0, T(2, 0) + (p9 + p12 + s2))
            emit(2, 1, PT(4, 2, 1) + (p14 - p13 + s2))
        w0 = T(0, 2)
        emit(0, 0, PT(0, 0, 0) + ((p8 + t10 + w0) if two_cols else (p8 + p9 + t10 + w0)))
        emit(0, 1, PT(1, 0, 1) + (p6 + p11 + t7 + w0))

    QT = (0, 1, 2, 3)
    KT = (4, 5, 6, 7, 13)
    VT = (8, 9, 10, 11, 12)
    c2e = DH ** -0.5 * math.log2(math.e)
    neg = -1e9 * math.log2(math.e)

    def q_step(pr, cfg=None, chunk=None, rows=False, sums=False):
        first = cfg is not None
        clock = _Timeline()
        if sums:
            base, nx = 0, 1
            for k in range(40):
                clock.add(200 + k * 90, functools.partial(wq_sums, 8 * k))
        elif rows:
            base, nx = pr * (2 * TB), pr + 1
            for k in range(2):
                clock.add_due(QA_T[k], functools.partial(row_chain, k, QA_T[2]), QA_T[3] - QA_T[k])
        else:
            base = pl.multiple_of(pr * (2 * TB), 2 * TB)
            nx = jnp.minimum(pr + 1, NP - 1)
        pieces = []
        if chunk is not None:
            for m in range(3):
                pieces += prep_pieces(jnp.maximum(chunk - LAGS[m], 0) if LAGS[m] else chunk, m)

        def paced(piece, dep):
            pw[0, pl.ds(R_END, 8), 0:128] = pltpu.bitcast(dep, u32)
            piece()
        for k, piece in enumerate(pieces):
            frac = k / 48 * QFR if k < 48 else QFR + (k - 48) / (len(pieces) - 48) * (1 - QFR)
            clock.add(QP0 + int(frac * (QP1 - QP0)), functools.partial(paced, piece))
        if first:
            for par in range(2):
                add_ln(clock, cfg[par], cfg[2:], 2 * nx + par, xn_g, par,
                       functools.partial(lambda par_, i: xin[nx, pl.ds(i * 16, 16), par_ * TB:(par_ + 1) * TB], par))
        for r0, nt, tiles in ((0, 2, (0, 4, 8)), (TC, 2, (2, 6, 10)), (2 * TC, 1, (12, 13))):
            def R(k):
                return wq[pl.ds(r0, nt * 64), _lt(k)]

            def L(k):
                return sq_scr[k, 0] if first else jnp.concatenate([sq_scr[k, 0], sq_scr[k, 1]], axis=0)

            def P(k):
                return _dot_nt(_up(L(k)), _up(R(k)))

            def T(j, kind):
                rhs = _up(R(15 + 3 * j + kind))
                if nt == 1 and kind == 2:
                    lhs = L(15 + kind)
                    return jnp.concatenate([_dot_nt(_up(lhs[k:k + 32]), rhs) for k in range(0, lhs.shape[0], 32)],
                                           axis=0)
                return _dot_nt(_up(L(15 + kind)), rhs)

            def PT(k, j, kind):
                return _dot_nt(_up(jnp.concatenate([L(k), L(15 + kind)], axis=1)),
                               _up(jnp.concatenate([R(k), R(15 + 3 * j + kind)], axis=1)))

            def emit(col, half, v):
                for k in range(nt):
                    for q_ in range(2):
                        rows_ = pl.ds(base + (HALO + (2 * q_ + half) * TB), TB)
                        qall[tiles[col] + k, rows_, :] = v[q_ * TB:(q_ + 1) * TB, _lt(k)]
            if not first:
                hk_outputs(P, T, PT, emit, nt == 1)
                continue
            for j in range(len(tiles)):
                both = T(j, 2)
                clock.t += 32 * nt
                for t in range(2):
                    for k in range(nt):
                        lhs = [L(3 * t + i) for i in range(3)] + [L(15 + t)]
                        lhs[0] = gate(lhs[0], clock)
                        rhs = [wq[pl.ds(r0 + k * 64, 64), _lt(n)]
                               for n in [wq_slot(i, j) for i in range(3)] + [15 + 3 * j + t]]
                        v = _dot_nt(_up(jnp.concatenate(lhs, axis=1)), _up(jnp.concatenate(rhs, axis=1))) + both[:, _lt(k)]
                        qall[tiles[j] + k, pl.ds(base + (HALO + t * TB), TB), :] = v
                        clock.tick(128, v, QTK)
        assert not clock.pending()
        if first:
            q_left(True)

    def row_group(blk, par, r, nw, nv, mids=None):
        base = _al(blk * TB, TB)
        lo = lax.broadcasted_iota(jnp.int32, (RB, 128), 1) < KY
        r0 = r * RB

        def ld(t, w):
            return qall[t, pl.ds(base + (HALO + r0 - DIL * w), RB), :]
        dep = yield
        cs = tie(jnp.full((RB, 128), c2e, f32), dep)
        q = [ld(t, 0) * cs for t in QT] + [jnp.where(lo, pltpu.roll(ld(13, 0), KY, 1), 0.0) * cs]
        sc = []
        for w in range(W):
            if w and w % nw == 0:
                dep = yield
                q = [tie(q[0], dep)] + q[1:]
            acc = None
            for j, t in enumerate(KT):
                p = q[j] * ld(t, w)
                acc = p if acc is None else acc + p
            acc = acc + pltpu.roll(acc, 64, 1)
            if mids is not None:
                mids[r] = pltpu.bitcast(acc, u32)
            acc = acc + pltpu.roll(acc, 32, 1)
            if r0 - DIL * w < 0:
                pos = blk * TB + r0 + lax.broadcasted_iota(jnp.int32, (RB, 128), 0)
                acc = jnp.where(pos >= DIL * w, acc, neg)
            sc.append(acc)
        m = _tree(jnp.maximum, sc)
        e = [jnp.exp2(sc[w] - m) for w in range(W)]
        l = _tree(jnp.add, e)
        rinv = pl.reciprocal(l, approx=True)
        rinv = rinv * (2.0 - l * rinv)
        outs = []
        for j, t in enumerate(VT):
            if j and j % nv == 0:
                dep = yield _tree(jnp.bitwise_or, [pltpu.bitcast(v, u32) for v in outs])
                outs = []
                e = [tie(e[0], dep)] + e[1:]
            acc = None
            for w in range(W):
                p = e[w] * ld(t, w)
                acc = p if acc is None else acc + p
            o = acc * rinv
            o_s[par * 5 + j, pl.ds(r0, RB), :] = o
            outs.append(o)
        yield _tree(jnp.bitwise_or, [pltpu.bitcast(v, u32) for v in outs])

    def add_rows(clock, t0, blk, par, r, cfg):
        nw, nv, step, gap, d1, d2 = cfg
        gen = row_group(blk, par, r, nw, nv)
        next(gen)
        n1, n2 = -(-W // nw), -(-5 // nv)
        for k in range(n1):
            clock.add_due(t0 + k * step, gen.send, d1)
        for k in range(n2 - 1):
            clock.add_due(t0 + (n1 - 1) * step + gap + k * step, gen.send, d2)

    def row_chain(blk, lag, dep):
        mids, fins = {}, {}
        for r in range(nr):
            gen = row_group(blk, blk, r, W, 5, mids)
            next(gen)
            if r:
                dep = pltpu.bitcast(mids[r - 1] | fins[r - lag] if r >= lag else mids[r - 1], f32)
            fins[r] = gen.send(dep)
        return _tree(jnp.bitwise_or, [fins[r] for r in range(nr - lag, nr)])

    wo_seq = []
    for pos, k in enumerate(WORD):
        if pos in (0, 2):
            wo_seq += [('r', pos // 2, k_) for k_ in range(3)]
        wo_seq.append(('p', k))

    def wo_rhs(off):
        lo = lax.broadcasted_iota(jnp.int32, (TB, 128), 1) < KY

        rhs = {}
        for it in wo_seq:
            z = zero(wo_seq.index(it)) if off is None else off

            def O(t, j):
                return o_s[t * 5 + j, pl.ds(z, TB), :]
            if it[0] == 'p':
                v = _ssum([(O(t, j), sg) for j, t, sg in _HK_B[it[1]]])
            elif it[2] == 0:
                v = O(it[1], 3)
            else:
                v = jnp.where(lo, O(it[1], 2 + it[2]), O(it[1], 5 - it[2]))
            rhs[it] = v.astype(bf16)
        return rhs

    def wo_mm(blk0, rhs):
        res = {}
        for it in wo_seq:
            if it[0] == 'p':
                lhs = wo2[pl.ds(0, D3 // 2), _lt(it[1])]
            else:
                lhs = wo2[:, _lt(15 + it[2])]
            res[it] = _dot_nt(_up(lhs), rhs[it])
        for t in range(2):
            both = res['r', t, 2]
            rem = xres[blk0 + t] + jnp.concatenate([res['r', t, 0] + both, res['r', t, 1] + both], axis=0)
            y = jnp.concatenate([_ssum([(res['p', k], sg) for k, sg in _HK_C[i, t]]) for i in range(3)], axis=0)
            xres[blk0 + t] = y + rem

    def a_left(which=range(15), dep=None, cb=None):
        for n in which:
            v = _ssum([(xn_f[t, pl.ds(zero(n) + i * D3, D3), :], sg)
                       for (i, t), lst in _HK_C.items() for k, sg in lst if k == n])
            if dep is not None:
                v = jnp.concatenate([tie(v[0:8], dep), v[8:2 * KY], tie(v[2 * KY:2 * KY + 8], dep), v[2 * KY + 8:]],
                                    axis=0)
            t1 = pltpu.bitcast(v[:2 * KY].astype(bf16).T, u32)
            t2 = pltpu.bitcast(jnp.concatenate([v[2 * KY:], v[2 * KY:]], axis=0).astype(bf16).T, u32)
            if dep is None:
                arrange(n, t1, t2)
                cb(t1[0:8])
                cb(t2[0:8])
            else:
                st_s[2 * n] = t1
                st_s[2 * n + 1] = t2

    def arrange(n, t1, t2):
        lo = lax.broadcasted_iota(jnp.int32, (TB // 2, 128), 1) < KY
        s_scr[3 * n] = t1
        s_scr[3 * n + 1] = jnp.where(lo, t1, t2)
        s_scr[3 * n + 2] = jnp.where(lo, t2, t1)

    def a_arrange(n, dep):
        st_s[30, pl.ds(0, 8), :] = pltpu.bitcast(dep, u32)
        arrange(n, st_s[2 * n, pl.ds(zero8, TB // 2), :], st_s[2 * n + 1, pl.ds(zero8, TB // 2), :])

    k0 = math.sqrt(2.0 / math.pi)
    k1 = k0 * 0.044715

    def ffn(j, c0, script):
        clock = _Timeline()
        b0 = (2 * j) % NB
        an = (2 * j + 2) % NB
        acc = [None] * 57
        hs = {}
        lns, lq, staged, nrows = [], [], set(), 0

        pend = []

        def advance(keep):
            while len(pend) > keep:
                pend.pop(0)()

        def written(k):
            clock.due.append(lambda: pltpu.bitcast(p_s[k][pl.ds(zero8, 8), 0:128], u32))

        def gu(p):
            c, m = c0 + p // 2, p % 2
            h = hs.setdefault(p // 2, [[None, None, None] for _ in range(3)])

            def mm(n, kind):
                lhs = gate(s_scr[3 * n + kind], clock)
                return _dot(_up(lhs), _up(pw[c, pl.ds((3 * n + kind) * (TC // 2), TC // 2), m * TC:(m + 1) * TC]))

            def get(name):
                return p_s[PSLOT[name]][pl.ds(zero8, TB), :]

            def post(n, v):
                adds, keep, emits = GU_POST[n]
                if keep[0] is not None:
                    p_s[PSLOT[keep[0]]][...] = v
                    written(PSLOT[keep[0]])
                w_ = v
                for name, sg in adds:
                    w_ = w_ + get(name) if sg == 1 else w_ - get(name)
                if keep[1] is not None:
                    p_s[PSLOT[keep[1]]][...] = w_
                    written(PSLOT[keep[1]])
                if emits is not None:
                    col, half = emits
                    if m == 1:
                        k_ = 17 + 9 * ((p // 2) % NHS) + 3 * col
                        hv = w_ * p_s[11 + 2 * col + half][pl.ds(zero8, TB), :]
                        p_s[k_ + half][...] = hv
                        written(k_ + half)
                        h[col][half] = k_ + half
                        if h[col][1 - half] is not None:
                            p_s[k_ + 2][...] = hv + p_s[k_ + 1 - half][pl.ds(zero8, TB), :]
                            written(k_ + 2)
                            h[col][2] = k_ + 2
                    else:
                        p_s[11 + 2 * col + half][...] = w_ + w_ * jnp.tanh(w_ * (k0 + k1 * (w_ * w_)))
                        written(11 + 2 * col + half)
            for n in GU_ORD:
                both = mm(n, 2)
                v = jnp.concatenate([mm(n, 0) + both, mm(n, 1) + both], axis=1)
                pend.append(functools.partial(post, n, v))
                advance(PLAG)
                clock.tick(96, both, GTK)

        todo = [sum(any(i_ == i for i_, _, _ in z) for z in _Z6) for i in range(6)]

        def gather(i):
            if last:
                ys = [_ssum([(acc[n], sg) for n, sg in sorted(_C6[i, t], key=lambda z: _order6().index(z[0]))])
                      for t in range(2)]
            else:
                t0, t1 = dict(_C6[i, 0]), dict(_C6[i, 1])
                both = _ssum([(acc[n], sg) for n, sg in t0.items() if n in t1])
                ys = (_ssum([(acc[n], sg) for n, sg in t0.items() if n not in t1]) + both,
                      _ssum([(acc[n], sg) for n, sg in t1.items() if n not in t0]) - both)
            for t in range(2):
                x2 = xres[b0 + t, pl.ds(i * D6, D6), :] + 0.5 * ys[t]
                xres[b0 + t, pl.ds(i * D6, D6), :] = x2
                xin[j % NP, pl.ds(i * D6, D6), t * TB:(t + 1) * TB] = x2.astype(bf16)
            if last and i in ORD6[:OSPL]:
                @pl.when(g == 1)
                def _():
                    _cp_rows(i, o_hbm, xin, sems).start()

        def down(ps, final):
            cs = ps[::2]
            hsl = [hs.pop(p // 2) for p in cs]
            for pos, i in enumerate(_order6()):
                while any(h_[j_ % 3][d_] is None for h_ in hsl for j_, d_, _ in _B6[i]):
                    advance(len(pend) - 1)
                au = [pw[c0 + p // 2, pl.ds(R_SD + (i // 2) * (D6 // 2), D6 // 2), _lt(i % 2)] for p in cs]
                au[0] = gate(au[0], clock)
                lhs = jnp.concatenate(au, axis=1)
                rhs = jnp.concatenate([_ssum([(p_s[h_[j_ % 3][d_]][pl.ds(zero(pos % 21), TB), _lt(j_ // 3)], sg)
                                              for j_, d_, sg in _B6[i]]) for h_ in hsl], axis=1).astype(bf16)
                r = _dot_nt(_up(lhs), rhs)
                acc[i] = r if acc[i] is None else r + acc[i]
                if final:
                    for i_ in sorted({i_ for i_, _, _ in _Z6[i]}):
                        todo[i_] -= 1
                        if not todo[i_]:
                            gather(i_)
                if pos % DADV == 0:
                    advance(max(len(pend) - 1, 0))
                clock.tick(24 * len(cs), acc[i], DTK)

        pg = pd = 0
        for tok in script:
            if tok == 'G':
                gu(pg)
                pg += 1
            elif tok[0] == 'D':
                down(list(range(pd, pd + int(tok[1:]))), pd + int(tok[1:]) == script.count('G'))
                pd += int(tok[1:])
            elif tok == 'W':
                assert not clock.pending() and nrows == 2 * nr
                advance(0)
                wo_mm(an, wo_rhs(None))
                clock.t += 1152
            elif tok[0] == 'n':
                lns.append(add_ln(clock, clock.t + int(tok[3:]), LNJ + (JDL,), an + int(tok[1]), xn_f, int(tok[1])))
            elif tok[0] == 'm':
                lq.append(add_ln(clock, clock.t + int(tok[3:]), LNJ + (JDL,), (2 * j + 6) % NB + int(tok[1]), xn_g,
                                 int(tok[1])))
            elif tok[0] == 'k':
                _, t0, dt = tok.split('+')

                def qleft(which, dep):
                    assert len(lq) == 2 and not any(st['left'] for st in lq)
                    q_left(False, which, dep, (j + 1) % 2)
                    return sq_scr[which[0], (j + 1) % 2, pl.ds(zero8, 8), :]
                for k in range(NQL):
                    clock.add_due(clock.t + int(t0) + k * int(dt),
                                  functools.partial(qleft, range(k * 18 // NQL, (k + 1) * 18 // NQL)), LDL)
            elif tok[0] == 'l':
                _, t0, dt = tok.split('+')

                def left(which, dep):
                    assert len(lns) == 2 and not any(st['left'] for st in lns)
                    staged.update(which)
                    a_left(which, dep)
                    return st_s[0, pl.ds(zero8, 8), :]
                for k in range(NLEFT):
                    clock.add_due(clock.t + int(t0) + k * int(dt),
                                  functools.partial(left, range(k * 15 // NLEFT, (k + 1) * 15 // NLEFT)), LDL)
            elif tok[0] == 'c':
                _, t0, dt = tok.split('+')
                assert pg == 2 * NCH

                def place(k, dep):
                    assert k in staged
                    a_arrange(k, dep)
                for k in range(15):
                    clock.add(clock.t + int(t0) + k * int(dt), functools.partial(place, k))
            else:
                n, t0, dt = tok[1:].split('+')
                for k in range(int(n)):
                    add_rows(clock, clock.t + int(t0) + k * int(dt), an + nrows // nr, nrows // nr, nrows % nr,
                             RG + (RDL, JDL))
                    nrows += 1
        assert pg == pd and not clock.pending()

    if last:
        ffn(2 * NP - 1, g * NPC, SCRIPT_F)
        return
    if phase == 'main':
        @pl.when(jnp.logical_and(g >= NP - 1, (g & 1) == 1))
        def _():
            q_step(g - (NP - 1))

        ffn(g, 0, SCRIPT)

        @pl.when(g >= NP)
        def _():
            _cp_out(g - NP, o_hbm, xin, sems).start()
        return
    assert NCH == NP - 2

    late = [(c, m) for c in range(NCH) for m in range(3) if c >= NCH - LAGS[m]]

    def prologue():
        cp_x(0).start()
        for sec in range(3):
            for cp in cp_qkv(sec):
                cp.start()
        qall[:, pl.ds(0, HALO), :] = jnp.zeros((16, HALO, 128), f32)
        cp_x(0).wait()
        for t in range(2):
            x = xin[0, :, t * TB:(t + 1) * TB].astype(f32)
            xres[t] = x
            mean, rstd = _ln_stats(x)
            xn_g[t, pl.ds(zero8, D), :] = (xres[t] - mean) * rstd
        q_left(True)
        for sec in range(3):
            for cp in cp_qkv(sec):
                cp.wait()
            if sec == 0:
                cp_x(1).start()
                cp_x(2).start()
                cp_wo().start()
                for c in range(NCH):
                    if 3 + c < NP:
                        cp_x(3 + c).start()
                    for m in range(3):
                        if c == 0 or c > LAGS[m]:
                            cp_unit(max(c - LAGS[m], 0), m).start()
                for c, m in late:
                    cp_unit(c, m).start()
            transpose_qkv(sec)
            build_wq(sec)

    def first_attention():
        cp_x(2).wait()
        q_step(1, CFG_QA, rows=True)
        cp_wo().wait()
        build_wo()
        wo_mm(0, wo_rhs(0))

    def startup_step(c, carry):
        @pl.when(c + 3 < NP)
        def _():
            cp_x(c + 3).wait()
        for m in range(3):
            if LAGS[m]:
                @pl.when(jnp.logical_or(c == 0, c > LAGS[m]))
                def _():
                    cp_unit(jnp.maximum(c - LAGS[m], 0), m).wait()
            else:
                cp_unit(c, m).wait()
        q_step(c + 2, CFG_Q1, chunk=c)
        return carry

    def startup_tail():
        pieces = []
        for c, m in late:
            cp_unit(c, m).wait()
            pieces += prep_pieces(c, m)
        npt = 30 + 2 * TLN
        done = []

        def pace(v):
            pw[g >> 20, pl.ds(R_END, 8), 0:128] = v
            done.append(v)
            for piece in pieces[(len(done) - 1) * len(pieces) // npt:len(done) * len(pieces) // npt]:
                piece()
        for t in range(2):
            mean, rstd = _ln_stats(xres[t])
            xn = (xres[t, pl.ds(zero8, D), :] - mean) * rstd
            xn_f[t] = xn
            for k in range(TLN):
                pace(pltpu.bitcast(xn[k * 64:k * 64 + 8], u32))
        a_left(cb=pace)
        assert len(done) == npt

    @pl.when(g == 0)
    def _():
        prologue()
        cp_x(1).wait()
        q_step(0, CFG_Q0, sums=True)
        first_attention()
        lax.fori_loop(0, NCH, startup_step, 0)
        startup_tail()


def _cp_out(k, o_hbm, xin, sems):
    return pltpu.make_async_copy(xin.at[k], o_hbm.at[:, pl.ds(_al(k * 2 * TB, 128), 2 * TB)], sems.at[4 + k])


def _cp_rows(i, o_hbm, xin, sems):
    k, n = xin.shape[0] - 1, xin.shape[1] // 6
    return pltpu.make_async_copy(xin.at[k, pl.ds(i * n, n), :], o_hbm.at[pl.ds(i * n, n), pl.ds(k * 2 * TB, 2 * TB)],
                                 sems.at[4 + k])


def _kernel(*refs, D, DF, S):
    def body(phase, g, carry):
        _step(g, phase, *refs, D=D, DF=DF, S=S)
        return carry
    NP = S // (2 * TB)
    lax.fori_loop(0, 2, functools.partial(body, 'start'), 0)
    lax.fori_loop(0, 2 * NP - 1, functools.partial(body, 'main'), 0)
    lax.fori_loop(0, 2, functools.partial(body, 'last'), 0)
    o_hbm, xin, sems = refs[6], refs[7], refs[24]
    for i in ORD6[OSPL:]:
        _cp_rows(i, o_hbm, xin, sems).start()
    for k in range(NP - 1):
        _cp_out(k, o_hbm, xin, sems).wait()
    for i in range(6):
        _cp_rows(i, o_hbm, xin, sems).wait()


@jax.jit
def pallas_interleave_layers__sliding_local_dilated__glu_gated_geglu__prompt_kernel(
    A_x, A_wqkv, A_wo, B_x, B_w_gate, B_w_up, B_w_down):
    B, S, D = A_x.shape
    DF = B_w_gate.shape[1]
    NB = S // TB
    NP = NB // 2
    NCH = DF // CW
    xT = A_x.reshape(S, D).T
    wdT = B_w_down.T
    hbm = pl.BlockSpec(memory_space=pltpu.HBM)
    outT = pl.pallas_call(
        functools.partial(_kernel, D=D, DF=DF, S=S),
        in_specs=[hbm] * 6,
        out_specs=hbm,
        out_shape=jax.ShapeDtypeStruct((D, S), A_x.dtype),
        scratch_shapes=[
            pltpu.VMEM((NP, D, 2 * TB), bf16),
            pltpu.VMEM((D, 3 * D), bf16),
            pltpu.VMEM((D, D), bf16),
            pltpu.VMEM((5, 14 * 128, 128), f32),
            pltpu.VMEM((WQR, 27 * 128), u32),
            pltpu.VMEM((D // 2, 640), u32),
            pltpu.VMEM((D // 4, 18 * 128), u32),
            pltpu.VMEM((NCH, 3, D, CW), bf16),
            pltpu.VMEM((NCH, 45 * (TC // 2) + 15 * (D // 6) + 16, 2 * TC), u32),
            pltpu.VMEM((16, S + QPAD, 128), f32),
            pltpu.VMEM((11, TB, 128), f32),
            pltpu.VMEM((NB, D, TB), f32),
            pltpu.VMEM((2, D, TB), f32),
            pltpu.VMEM((2, D, TB), f32),
            pltpu.VMEM((45, TB // 2, TC), u32),
            pltpu.VMEM((31, TB // 2, TC), u32),
            pltpu.VMEM((18, 2, TB // 2, TC), u32),
            pltpu.SemaphoreType.DMA((4 + NP + 3 * NCH,)),
        ] + [pltpu.VMEM((TB, 2 * TC), f32)] * (17 + 9 * NHS),
        compiler_params=pltpu.CompilerParams(
            vmem_limit_bytes=110 * 1024 * 1024,
            disable_bounds_checks=True,
            disable_semaphore_checks=True,
        ),
    )(xT, A_wqkv, A_wo, B_w_gate, B_w_up, wdT)
    return outT.T.reshape(B, S, D)
```

```python
import functools
import math
import jax
import jax.numpy as jnp
from jax import lax
import jax.experimental.pallas as pl
import jax.experimental.pallas.tpu as pltpu

DH = 18
W = 8
DIL = 2
HALO = 16
EPS = 1e-5
TB = 128
RB = 8
TC = 128
CW = 6 * TC
WQR = 320
KY = 64
QPAD = 40

SCRIPT = ('m0+50,m1+2804,k+8550+68,G,R7+74+200,G,G,R2+96+200,G,R9+300+260,D4,'
          'G,R7+74+200,G,G,R7+74+200,G,G,W,n0+300,n1+876,l+2900+80,G,G,G,c+600+192,D8').split(',')
SCRIPT_F = 'G,G,G,G,G,G,D6'.split(',')
GU_ORD = (8, 6, 7, 11, 3, 1, 10, 14, 9, 5, 0, 13, 12, 4, 2)
ORD6 = (0, 4, 3, 1, 5, 2)
WORD = (0, 1, 2, 6, 7, 8, 9, 10, 11, 12, 13, 14, 3, 4, 5)
PLAG, DADV, GTK, DTK, QTK = 6, 2, 2, 2, 8
LNJ = (12, 9, 48, 48)
RG = (2, 1, 24, 420)
RDL, JDL, LDL = 600, 300, 500
NLEFT, NQL, NHS, OSPL = 15, 18, 4, 4
CFG_Q0 = (40, 400, 9, 9, 32, 64, 300)
CFG_QA = (300, 748, 6, 6, 32, 64, 350)
CFG_Q1 = (40, 1456, 9, 9, 64, 64, 300)
BT, SUMT = (640, 560, 30), (60, 40)
QA_T = (300, 1000, 4, 3850)
QP0, QP1, QFR = 100, 3850, 0.6
DCUT = (0, 2, 4, 6, 8, 10, 12, 21, 30, 39, 48, 57)
LAGS = (1, 1, 0)

f32 = jnp.float32
bf16 = jnp.bfloat16
u32 = jnp.uint32
NT = (((1,), (1,)), ((), ()))


def _al(i, n):
    return i if isinstance(i, int) else pl.multiple_of(i, n)


def _lt(k):
    return slice(k * 128, (k + 1) * 128)


def _pk(x):
    return pltpu.bitcast(x.astype(bf16), u32)


def _up(x):
    return pltpu.bitcast(x, bf16)


def _dot(a, b):
    return jnp.dot(a, b, preferred_element_type=f32)


def _dot_nt(a, b):
    return lax.dot_general(a, b, NT, preferred_element_type=f32)


def _tree(fn, xs):
    xs = list(xs)
    while len(xs) > 1:
        xs = [fn(xs[i], xs[i + 1]) for i in range(0, len(xs) - 1, 2)] + ([xs[-1]] if len(xs) % 2 else [])
    return xs[0]


def _ln_stats(x, nacc=4):
    n = x.shape[0]
    c = x[0:1]
    s1 = [None] * nacc
    s2 = [None] * nacc
    for i in range(n // 8):
        d = x[i * 8:(i + 1) * 8] - c
        k = i % nacc
        s1[k] = d if s1[k] is None else s1[k] + d
        dd = d * d
        s2[k] = dd if s2[k] is None else s2[k] + dd
    m = jnp.sum(_tree(jnp.add, s1), axis=0, keepdims=True) * (1.0 / n)
    v = jnp.sum(_tree(jnp.add, s2), axis=0, keepdims=True) * (1.0 / n) - m * m
    v = jnp.maximum(v, 0.0)
    return c + m, lax.rsqrt(v + EPS)


_HK_A = (
    ((0, 0, 1), (0, 2, -1), (1, 0, -1)), ((0, 0, 1), (0, 1, -1), (2, 0, -1)), ((1, 1, 1), (0, 1, -1), (1, 2, -1)),
    ((1, 1, 1), (1, 0, -1), (2, 1, -1)), ((2, 2, 1), (0, 2, -1), (2, 1, -1)), ((2, 2, 1), (1, 2, -1), (2, 0, -1)),
    ((0, 1, 1),), ((0, 1, 1), (1, 0, -1)), ((1, 0, 1),),
    ((0, 2, 1),), ((0, 2, 1), (2, 0, -1)), ((2, 0, 1),),
    ((1, 2, 1),), ((2, 1, 1), (1, 2, -1)), ((2, 1, 1),),
)
_HK_C = {
    (0, 0): ((0, 1), (7, 1), (8, 1), (9, 1), (6, -1)),
    (0, 1): ((1, 1), (6, 1), (10, 1), (11, 1), (9, -1)),
    (1, 0): ((2, 1), (7, 1), (8, 1), (12, 1), (6, -1)),
    (1, 1): ((3, 1), (6, 1), (13, 1), (14, 1), (2, -1), (7, -1)),
    (2, 0): ((5, 1), (9, 1), (12, 1), (13, 1), (4, -1), (10, -1)),
    (2, 1): ((4, 1), (10, 1), (11, 1), (14, 1), (9, -1)),
}
_HK_B = (((0, 0, 1),), ((0, 1, 1),), ((1, 0, 1),), ((1, 0, 1), (1, 1, 1)), ((2, 1, 1),), ((2, 0, 1), (2, 1, 1)),
         ((0, 1, 1), (1, 1, 1)), ((0, 1, 1), (1, 0, 1), (1, 1, 1)), ((0, 0, 1), (0, 1, 1), (1, 0, 1), (1, 1, 1)),
         ((0, 0, 1), (2, 0, 1)), ((0, 0, 1), (2, 0, 1), (2, 1, 1)), ((0, 0, 1), (0, 1, 1), (2, 0, 1), (2, 1, 1)),
         ((1, 0, 1), (2, 0, 1)), ((1, 0, 1), (2, 1, -1)), ((1, 1, 1), (2, 1, 1)))


_HK6 = (
    '+00-01-02-30-50 +00 +00;+00-03+05-10-20 +01 +01;-01+11+13-15-40+41 +11 -10+11;-04-10+11+14+31+51 +12 +10;'
    '-02-12+21+22-23-25+35-42 +21 -20+21;-12-20+21+22+24-32-52+53 +22 +20;-03+31-32+33+43 +30 +30-31;'
    '+13-23-30+33-34 +32 +31;-04+34-40+41+42+44+54 +40 +40;-04+14-24-40-43+44-45 +41 +41;'
    '-05-12+35+45-51-52+53+55 +50 +50-51;+15+21-25+35+50-53-54+55 +52 +51;+01-40 +00+10 +00-01+10-11;'
    '+01-10 +00+12 +01-10+11;-04+10 +02+12 +01+11;+02 +00+20 +00-01+20-21;+02-20 +00+22 +01-20+21;'
    '+20 +02+22 +01+21;+03 +01+31 -00+01-30+31;+03-30 +01+32 +00+30-31;+30 +02+32 +00+30;+05 +01-51 +00-01+50-51;'
    '+05+50 +01-52 -00-50+51;+50 +02-52 +00+50;+31 +10-30 -10+30;+13-31 +11+30 +10-31;+13 +11-31 -11+31;'
    '+40-41 +10-40 +10-11-40+41;+04-14-40+41 +12-40 +10-11+41;+04-14 +12-42 +11-41;+12-51 +10+50 +10-50;'
    '+15+51 +11-50 -10+51;+15-21 +11+51 +11-51;+32+53 +20+30 +20+30;-23+32 +21-30 +20+31;+23-35 +21+31 +21+31;'
    '+42 +20-40 +20-21+40-41;+24+42 +22-40 -20+21+41;+24 +22-42 -21-41;+12+52-53 +20+50 +20+50;'
    '+12+21-25+35+52-53 +21-50 +20+51;-21+25-35 +21+51 +21+51;+43 +31+41 +30-31-40+41;+34+43 +32+41 -30+31+40;'
    '+34 +32+42 +30-40;+45 +41+51 -40+41+50-51;+45+54 +41+52 +40-50+51;+54 +42+52 -40+50;'
    '+40 +01+11+41 -00+01-10+11-40+41;-04+40 +02+12+41 +00-01+10-11+40;+04 +02+12+42 +00+10+40;'
    '+12 +10-20+50 -10+11-20+21+50-51;+12+21 +10-22+50 -11+20-21+51;+21 +12-22+52 +11+21-51;'
    '+35 +21+31+51 -20+21-30+31+50-51;+35+53 +21+31+52 +20+30-50+51;+53 +22+32+52 -20-30+50'
)


def _terms(txt):
    return tuple((int(txt[i + 1]), int(txt[i + 2]), 1 if txt[i] == '+' else -1) for i in range(0, len(txt), 3))


_A6, _B6, _Z6 = zip(*[[_terms(f) for f in row.split(' ')] for row in _HK6.split(';')])
_C6 = {(i, t): [(n, sg) for n, z in enumerate(_Z6) for i_, t_, sg in z if (i_, t_) == (i, t)]
       for i in range(6) for t in range(2)}


def _order6():
    early = [n for n, b in enumerate(_B6) if all(j % 3 == 0 or (j % 3 == 1 and d == 1) for j, d, _ in b)]
    early.sort(key=lambda n: max(d != 1 for _, d, _ in _B6[n]))
    out = list(early)
    for i in ORD6:
        out += [n for n, z in enumerate(_Z6) if n not in out and any(i_ == i for i_, _, _ in z)]
    return out


def _ssum(terms):
    terms = sorted(terms, key=lambda z: -z[1])
    acc = terms[0][0] if terms[0][1] == 1 else -terms[0][0]
    for v, sg in terms[1:]:
        acc = acc + v if sg == 1 else acc - v
    return acc


GU_POST = {
    8: ((), ('p8', None), None),
    7: ((('p8', 1),), (None, 't7'), None),
    3: ((('t7', 1),), (None, 's1'), None),
    6: ((), ('p6', None), None),
    14: ((('p6', 1), ('s1', 1)), ('p14', None), (1, 1)),
    12: ((('p9', 1), ('s2', 1)), ('p12', None), (2, 0)),
    13: ((), ('p13', None), None),
    2: ((('p12', 1), ('p13', 1), ('s1', 1)), (None, None), (1, 0)),
    11: ((), ('p11', None), None),
    10: ((('p11', 1),), (None, 't10'), None),
    5: ((('t10', 1),), (None, 's2'), None),
    9: ((), ('p9', None), None),
    4: ((('p14', 1), ('s2', 1), ('p13', -1)), (None, None), (2, 1)),
    0: ((('p8', 1), ('p9', 1), ('t10', 1)), (None, None), (0, 0)),
    1: ((('p6', 1), ('p11', 1), ('t7', 1)), (None, None), (0, 1)),
}
PSLOT = {k: i for i, k in enumerate(('p8', 't7', 's1', 'p6', 'p14', 'p12', 'p13', 'p11', 't10', 's2', 'p9'))}


class _Timeline:
    def __init__(self):
        self.t = 0
        self.jobs = []
        self.due = []

    def add(self, when, fn):
        self.jobs.append((when, len(self.jobs), fn))
        self.jobs.sort(key=lambda z: z[:2])

    def add_due(self, when, job, delay):
        def run(dep):
            val = job(dep)
            if val is not None:
                self.add(self.t + delay, lambda _: self.due.append(lambda: val))
        self.add(when, run)

    def pending(self):
        return [j for j in self.jobs if getattr(j[2], '__name__', '') != '<lambda>']

    def tick(self, dur, v, n):
        for k in range(n):
            self.t += dur // n
            r = k * (v.shape[0] // n)
            while self.jobs and self.jobs[0][0] <= self.t:
                self.jobs.pop(0)[2](v[r:r + 8, 0:128])


def _step(g, phase, x_hbm, wqkv_hbm, wo_hbm, wg_hbm, wu_hbm, wd_hbm, o_hbm,
          xin, wqkv_raw, wo_raw, tmp, wq, woT, wo2, raw, pw, qall, o_s, xres, xn_f, xn_g, s_scr, st_s, sq_scr,
          sems, *p_s, D, DF, S):
    last = phase == 'last'
    NB = S // TB
    NP = NB // 2
    NCH = DF // CW
    NPC = NCH // 2
    D3 = D // 3
    D6 = D // 6
    nr = TB // RB
    hh = D // 4
    zero8 = pl.multiple_of((g >> 20) * 8, 8)
    zvec = jnp.full((8, 128), (g >> 20).astype(u32), u32)

    def zero(k):
        return pl.multiple_of((g >> (8 + k)) * 8, 8)

    def tie(x, dep):
        return pltpu.bitcast(pltpu.bitcast(x, u32) | (pltpu.bitcast(dep, u32) & zvec), f32)

    def gate(lhs, clock):
        if not clock.due:
            return lhs
        pr = _tree(jnp.bitwise_or, [k() for k in clock.due]) & zvec
        del clock.due[:]
        return jnp.concatenate([lhs[0:8] | pr, lhs[8:]], axis=0)

    QSEC = ((0, 5), (5, 9), (9, 14))

    def cp_qkv(sec):
        out = []
        for j in range(*QSEC[sec]):
            n = min(128, 3 * D - j * 128)
            out.append(pltpu.make_async_copy(wqkv_hbm.at[:, pl.ds(j * 128, n)], wqkv_raw.at[:, pl.ds(j * 128, n)],
                                             sems.at[sec]))
        return out

    def cp_wo():
        return pltpu.make_async_copy(wo_hbm, wo_raw, sems.at[3])

    def cp_x(k):
        return pltpu.make_async_copy(x_hbm.at[:, pl.ds(_al(k * 2 * TB, 128), 2 * TB)], xin.at[k], sems.at[4 + k])

    def cp_unit(c, m):
        return pltpu.make_async_copy((wg_hbm, wu_hbm, wd_hbm)[m].at[:, pl.ds(_al(c * CW, 128), CW)], raw.at[c, m],
                                     sems.at[4 + NP + 3 * c + m])

    R_SD = 45 * (TC // 2)
    R_END = R_SD + 15 * (D3 // 2)

    def hk_a_ops(load, minus=None):
        blk = {}
        for i in range(3):
            for j in range(3):
                blk[i, j] = load(i, j).astype(f32)
                if minus is not None:
                    blk[i, j] = blk[i, j] - minus(i, j).astype(f32)
        return [_pk(_ssum([(blk[i, j], sg) for i, j, sg in terms])) for terms in _HK_A]

    def prep_pieces(c, m):
        def ld(r, cs):
            return lambda i, j: raw[c, m, pl.ds(i * D3 + r, 16), pl.ds((3 * cs + j) * TC, TC)]

        def gu_piece(q, r, cs, neg, kind, half):
            ops = hk_a_ops(ld(q * KY + r, cs), None if neg is None else ld(q * KY + r, neg))
            for k, t in enumerate(ops):
                pw.at[c][pl.ds((3 * k + kind) * (TC // 2) + (half * KY + r) // 2, 8), m * TC:(m + 1) * TC] = t

        def d_piece(r, q, ks):
            blk = {}
            cz = c + (g >> (8 + q))
            for k in ks:
                for i, j, _ in _A6[k]:
                    if (i, j) not in blk:
                        blk[i, j] = raw[cz, m, pl.ds(i * D6 + r, 16), pl.ds(j * TC, TC)].astype(f32)
                pw.at[c][pl.ds(R_SD + (k // 2) * (D6 // 2) + r // 2, 8), _lt(k % 2)] = _pk(
                    _ssum([(blk[i, j], sg) for i, j, sg in _A6[k]]))
        if m == 2:
            return [functools.partial(d_piece, r, q, range(DCUT[q], DCUT[q + 1]))
                    for r in range(0, D6, 16) for q in range(len(DCUT) - 1)]
        spec = ((0, 0, None, 0, 0), (1, 0, 1, 0, 1), (0, 1, None, 1, 0), (2, 1, 0, 1, 1),
                (2, 0, None, 2, 0), (1, 1, None, 2, 1))
        return [functools.partial(gu_piece, q, r, cs, neg, kind, half)
                for r in range(0, KY, 16) for q, cs, neg, kind, half in spec]

    def transpose_qkv(sec):
        for j in range(*QSEC[sec]):
            wd_ = min(128, 3 * D - j * 128)
            blk = wqkv_raw[:, j * 128:j * 128 + wd_].astype(f32)
            if wd_ < 128:
                blk = jnp.concatenate([blk, jnp.zeros((D, 128 - wd_), f32)], axis=1)
            bt = jnp.concatenate([blk, blk[D - KY:]], axis=0).T
            for t in range(5):
                tmp[t, pl.ds(j * 128, 128), :] = bt[:, t * 128:(t + 1) * 128]

    def wq_slot(i, j):
        return 24 + i if i == j else [n for n, t in enumerate(_HK_A) if t == ((i, j, 1),)][0]

    def build_wq(sec, ds=range(DH), dep=None):
        lo = lax.broadcasted_iota(jnp.int32, (32, 128), 1) < KY
        if dep is not None:
            tmp[0, pl.ds(zero8 + 3 * D + 32, 8), :] = dep
        for d in ds:
            tt = [tmp[t, pl.ds(sec * D + d, 32, stride=DH), :] for t in range(5)]
            ops = tt[:4] + [jnp.where(lo, tt[3], tt[4]), jnp.where(lo, tt[4], tt[3])]
            if d < 16:
                dst = [(sec, d * 16)]
            else:
                dst = ([(1, (d + 2) * 16)], [(1, d * 16)], [(0, d * 16), (0, (d + 2) * 16)])[sec]
            for j, row in dst:
                for k, v in enumerate(ops):
                    wq[pl.ds(row, 16), _lt(wq_slot(k, j) if k < 3 else 12 + 3 * j + k)] = _pk(v)

    def wq_sums(r, dep):
        ncol = 3 if r < 256 else 2
        pin = pltpu.bitcast(dep, u32) & zvec
        blk = {(i, j): _up(wq[pl.ds(r, 8), _lt(wq_slot(i, j))] | pin).astype(f32) for i in range(3) for j in range(ncol)}
        for n, terms in enumerate(_HK_A):
            if len(terms) > 1 and not (ncol == 2 and n in (4, 5)):
                wq[pl.ds(r, 8), _lt(n)] = _pk(_ssum([(blk[i, j], sg) for i, j, sg in terms if j < ncol]))

    def build_wo():
        for t in range(5):
            wd_ = min(128, D - t * 128)
            blk = wo_raw[:, t * 128:t * 128 + wd_].astype(f32)
            if wd_ < 128:
                blk = jnp.concatenate([blk, jnp.zeros((D, 128 - wd_), f32)], axis=1)
            tmp[t, pl.ds(0, D), :] = blk
        for t in range(5):
            rows = [tmp[t, pl.ds(d, 32, stride=DH), :] for d in range(DH)]
            ft = jnp.concatenate(rows + rows[16:], axis=0).T
            n = min(128, D - t * 128)
            woT[pl.ds(t * 64, n // 2), :] = _pk(ft[:n])
        for r in range(0, D3 // 2, 8):
            ops = hk_a_ops(lambda i, j: _up(woT[pl.ds(i * (D3 // 2) + r, 8), j * TC:(j + 1) * TC]))
            for k, t in enumerate(ops):
                wo2[pl.ds(r, 8), _lt(k)] = t
        lo = lax.broadcasted_iota(jnp.int32, (16, 128), 1) < KY
        for r in range(0, hh, 8):
            a3, a4, b3, b4 = [_up(woT[pl.ds(r0 + r, 8), c0:c0 + 128]).astype(f32)
                              for r0 in (0, hh) for c0 in (384, 512)]
            wo2[pl.ds(r, 8), _lt(15)] = _pk(jnp.where(lo, a3, a3 - b3))
            wo2[pl.ds(r, 8), _lt(16)] = _pk(jnp.where(lo, b3, b4 - a4))
            wo2[pl.ds(r, 8), _lt(17)] = _pk(jnp.where(lo, a4, b3))

    def q_left(plain, which=None, dep=None, slot=0):
        k1, k2, k3 = 3 * TC, 3 * TC + KY, 3 * TC + 2 * KY
        for n in (list(range(6 if plain else 15)) + [15, 16, 17]) if which is None else which:
            def X(t, r0, rows):
                return xn_g[t, pl.ds((zero8 if plain else zero(n)) + r0, rows), :]
            if n == 15:
                v = jnp.concatenate([X(0, k1, KY), X(0, k2, KY) - X(1, k2, KY)], axis=0)
            elif n == 16:
                v = jnp.concatenate([X(1, k1, KY), X(1, k3, KY) - X(0, k3, KY)], axis=0)
            elif n == 17:
                v = jnp.concatenate([X(0, k3, KY), X(1, k2, KY)], axis=0)
            elif plain:
                v = X(n // 3, (n % 3) * TC, TC)
            else:
                v = _ssum([(X(t, i * TC, TC), sg) for (i, t), lst in _HK_C.items() for k, sg in lst if k == n])
            if dep is not None:
                v = jnp.concatenate([tie(v[0:8], dep), v[8:]], axis=0)
            sq_scr[n, slot] = pltpu.bitcast(v.astype(bf16).T, u32)

    def add_ln(clock, t0, cfg, blk, dst, par, inp=None):
        np1, np2, step, gap, delay = cfg
        st = dict(s1=[], s2=[], left=np2)
        nv = D // 16

        def load(i):
            if inp is None:
                return xres[blk, pl.ds(zero8 + i * 16, 16), :]
            x = inp(i).astype(f32)
            xres[blk, pl.ds(i * 16, 16), :] = x
            return x

        def stats(k, dep):
            xs = []
            for i in range(k * nv // np1, (k + 1) * nv // np1):
                x = load(i)
                xs += [x[0:8], x[8:16]]
            if k == 0:
                st['c'] = jnp.broadcast_to(xs[0][0:1], (8, TB))
            c = tie(st['c'], dep)
            ds = [x - c for x in xs]
            st['s1'].append(_tree(jnp.add, ds))
            st['s2'].append(_tree(jnp.add, [d * d for d in ds]))
            return pltpu.bitcast(st['s1'][-1], u32) | pltpu.bitcast(st['s2'][-1], u32)

        def norm(k, dep):
            if k == 0:
                m = jnp.sum(_tree(jnp.add, st['s1']), axis=0, keepdims=True) * (1.0 / D)
                v = jnp.sum(_tree(jnp.add, st['s2']), axis=0, keepdims=True) * (1.0 / D) - m * m
                st['mean'] = st['c'] + m
                st['rstd'] = jnp.broadcast_to(lax.rsqrt(jnp.maximum(v, 0.0) + EPS), (8, TB))
            mean = tie(st['mean'], dep)
            off = 0 if inp is None else zero8
            for i in range(k * 2 * nv // np2, (k + 1) * 2 * nv // np2):
                dst[par, pl.ds(i * 8, 8), :] = (xres[blk, pl.ds(off + i * 8, 8), :] - mean) * st['rstd']
            st['left'] -= 1
            return pltpu.bitcast(dst[par, pl.ds(zero8, 8), :], u32)
        for k in range(np1):
            clock.add_due(t0 + k * step, functools.partial(stats, k), delay)
        for k in range(np2):
            clock.add_due(t0 + np1 * step + gap + k * step, functools.partial(norm, k), delay)
        return st

    def hk_outputs(P, T, PT, emit, two_cols):
        p8 = P(8)
        t7 = P(7) + p8
        s1 = PT(3, 1, 2) + t7
        p6 = P(6)
        p14 = P(14)
        emit(1, 1, T(1, 1) + (p6 + p14 + s1))
        p13 = P(13)
        if two_cols:
            emit(1, 0, PT(2, 1, 0) + (p13 + s1))
        else:
            p12 = P(12)
            emit(1, 0, PT(2, 1, 0) + (p12 + p13 + s1))
        p11 = P(11)
        t10 = P(10) + p11
        if not two_cols:
            s2 = PT(5, 2, 2) + t10
            p9 = P(9)
            emit(2, 0, T(2, 0) + (p9 + p12 + s2))
            emit(2, 1, PT(4, 2, 1) + (p14 - p13 + s2))
        w0 = T(0, 2)
        emit(0, 0, PT(0, 0, 0) + ((p8 + t10 + w0) if two_cols else (p8 + p9 + t10 + w0)))
        emit(0, 1, PT(1, 0, 1) + (p6 + p11 + t7 + w0))

    QT = (0, 1, 2, 3)
    KT = (4, 5, 6, 7, 13)
    VT = (8, 9, 10, 11, 12)
    c2e = DH ** -0.5 * math.log2(math.e)
    neg = -1e9 * math.log2(math.e)

    def q_step(pr, cfg=None, chunk=None, rows=False, part=None):
        first = cfg is not None
        clock = _Timeline()
        if part is not None:
            base, nx = 0, 1
            if part < 2:
                transpose_qkv(part + 1)
                probe = pltpu.bitcast(tmp[0, pl.ds(zero8, 8), :], u32)
                clock.add(BT[0], lambda _: clock.due.append(lambda: probe))
                for d in range(DH):
                    clock.add(BT[1] + d * BT[2], functools.partial(build_wq, part + 1, [d]))
            else:
                for k in range(40):
                    clock.add(SUMT[0] + k * SUMT[1], functools.partial(wq_sums, 8 * k))
        elif rows:
            base, nx = pr * (2 * TB), pr + 1
            for k in range(2):
                clock.add_due(QA_T[k], functools.partial(row_chain, k, QA_T[2]), QA_T[3] - QA_T[k])
        else:
            base = pl.multiple_of(pr * (2 * TB), 2 * TB)
            nx = jnp.minimum(pr + 1, NP - 1)
        pieces = []
        if chunk is not None:
            for m in range(3):
                pieces += prep_pieces(jnp.maximum(chunk - LAGS[m], 0) if LAGS[m] else chunk, m)

        def paced(piece, dep):
            pw[0, pl.ds(R_END, 8), 0:128] = pltpu.bitcast(dep, u32)
            piece()
        for k, piece in enumerate(pieces):
            frac = k / 48 * QFR if k < 48 else QFR + (k - 48) / (len(pieces) - 48) * (1 - QFR)
            clock.add(QP0 + int(frac * (QP1 - QP0)), functools.partial(paced, piece))
        if first and part in (None, 2):
            for par in range(2):
                add_ln(clock, cfg[par], cfg[2:], 2 * nx + par, xn_g, par,
                       functools.partial(lambda par_, i: xin[nx, pl.ds(i * 16, 16), par_ * TB:(par_ + 1) * TB], par))
        for r0, nt, tiles in ((0, 2, (0, 4, 8)), (TC, 2, (2, 6, 10)), (2 * TC, 1, (12, 13))):
            def R(k):
                return wq[pl.ds(r0, nt * 64), _lt(k)]

            def L(k):
                return sq_scr[k, 0] if first else jnp.concatenate([sq_scr[k, 0], sq_scr[k, 1]], axis=0)

            def P(k):
                return _dot_nt(_up(L(k)), _up(R(k)))

            def T(j, kind):
                rhs = _up(R(15 + 3 * j + kind))
                if nt == 1 and kind == 2:
                    lhs = L(15 + kind)
                    return jnp.concatenate([_dot_nt(_up(lhs[k:k + 32]), rhs) for k in range(0, lhs.shape[0], 32)],
                                           axis=0)
                return _dot_nt(_up(L(15 + kind)), rhs)

            def PT(k, j, kind):
                return _dot_nt(_up(jnp.concatenate([L(k), L(15 + kind)], axis=1)),
                               _up(jnp.concatenate([R(k), R(15 + 3 * j + kind)], axis=1)))

            def emit(col, half, v):
                for k in range(nt):
                    for q_ in range(2):
                        rows_ = pl.ds(base + (HALO + (2 * q_ + half) * TB), TB)
                        qall[tiles[col] + k, rows_, :] = v[q_ * TB:(q_ + 1) * TB, _lt(k)]
            if not first:
                hk_outputs(P, T, PT, emit, nt == 1)
                continue
            for j in range(len(tiles)):
                if part is not None and (j if nt == 2 else 2) != part:
                    continue
                both = T(j, 2)
                clock.t += 32 * nt
                for t in range(2):
                    for k in range(nt):
                        lhs = [L(3 * t + i) for i in range(3)] + [L(15 + t)]
                        lhs[0] = gate(lhs[0], clock)
                        rhs = [wq[pl.ds(r0 + k * 64, 64), _lt(n)]
                               for n in [wq_slot(i, j) for i in range(3)] + [15 + 3 * j + t]]
                        v = _dot_nt(_up(jnp.concatenate(lhs, axis=1)), _up(jnp.concatenate(rhs, axis=1))) + both[:, _lt(k)]
                        qall[tiles[j] + k, pl.ds(base + (HALO + t * TB), TB), :] = v
                        clock.tick(128, v, QTK)
        assert not clock.pending()
        if first and part in (None, 2):
            q_left(True)

    def row_group(blk, par, r, nw, nv, mids=None):
        base = _al(blk * TB, TB)
        lo = lax.broadcasted_iota(jnp.int32, (RB, 128), 1) < KY
        r0 = r * RB

        def ld(t, w):
            return qall[t, pl.ds(base + (HALO + r0 - DIL * w), RB), :]
        dep = yield
        cs = tie(jnp.full((RB, 128), c2e, f32), dep)
        q = [ld(t, 0) * cs for t in QT] + [jnp.where(lo, pltpu.roll(ld(13, 0), KY, 1), 0.0) * cs]
        sc = []
        for w in range(W):
            if w and w % nw == 0:
                dep = yield
                q = [tie(q[0], dep)] + q[1:]
            acc = None
            for j, t in enumerate(KT):
                p = q[j] * ld(t, w)
                acc = p if acc is None else acc + p
            acc = acc + pltpu.roll(acc, 64, 1)
            if mids is not None:
                mids[r] = pltpu.bitcast(acc, u32)
            acc = acc + pltpu.roll(acc, 32, 1)
            if r0 - DIL * w < 0:
                pos = blk * TB + r0 + lax.broadcasted_iota(jnp.int32, (RB, 128), 0)
                acc = jnp.where(pos >= DIL * w, acc, neg)
            sc.append(acc)
        m = _tree(jnp.maximum, sc)
        e = [jnp.exp2(sc[w] - m) for w in range(W)]
        l = _tree(jnp.add, e)
        rinv = pl.reciprocal(l, approx=True)
        rinv = rinv * (2.0 - l * rinv)
        outs = []
        for j, t in enumerate(VT):
            if j and j % nv == 0:
                dep = yield _tree(jnp.bitwise_or, [pltpu.bitcast(v, u32) for v in outs])
                outs = []
                e = [tie(e[0], dep)] + e[1:]
            acc = None
            for w in range(W):
                p = e[w] * ld(t, w)
                acc = p if acc is None else acc + p
            o = acc * rinv
            o_s[par * 5 + j, pl.ds(r0, RB), :] = o
            outs.append(o)
        yield _tree(jnp.bitwise_or, [pltpu.bitcast(v, u32) for v in outs])

    def add_rows(clock, t0, blk, par, r, cfg):
        nw, nv, step, gap, d1, d2 = cfg
        gen = row_group(blk, par, r, nw, nv)
        next(gen)
        n1, n2 = -(-W // nw), -(-5 // nv)
        for k in range(n1):
            clock.add_due(t0 + k * step, gen.send, d1)
        for k in range(n2 - 1):
            clock.add_due(t0 + (n1 - 1) * step + gap + k * step, gen.send, d2)

    def row_chain(blk, lag, dep):
        mids, fins = {}, {}
        for r in range(nr):
            gen = row_group(blk, blk, r, W, 5, mids)
            next(gen)
            if r:
                dep = pltpu.bitcast(mids[r - 1] | fins[r - lag] if r >= lag else mids[r - 1], f32)
            fins[r] = gen.send(dep)
        return _tree(jnp.bitwise_or, [fins[r] for r in range(nr - lag, nr)])

    wo_seq = []
    for pos, k in enumerate(WORD):
        if pos in (0, 2):
            wo_seq += [('r', pos // 2, k_) for k_ in range(3)]
        wo_seq.append(('p', k))

    def wo_rhs(off):
        lo = lax.broadcasted_iota(jnp.int32, (TB, 128), 1) < KY

        rhs = {}
        for it in wo_seq:
            z = zero(wo_seq.index(it)) if off is None else off

            def O(t, j):
                return o_s[t * 5 + j, pl.ds(z, TB), :]
            if it[0] == 'p':
                v = _ssum([(O(t, j), sg) for j, t, sg in _HK_B[it[1]]])
            elif it[2] == 0:
                v = O(it[1], 3)
            else:
                v = jnp.where(lo, O(it[1], 2 + it[2]), O(it[1], 5 - it[2]))
            rhs[it] = v.astype(bf16)
        return rhs

    def wo_mm(blk0, rhs):
        res = {}
        for it in wo_seq:
            if it[0] == 'p':
                lhs = wo2[pl.ds(0, D3 // 2), _lt(it[1])]
            else:
                lhs = wo2[:, _lt(15 + it[2])]
            res[it] = _dot_nt(_up(lhs), rhs[it])
        for t in range(2):
            both = res['r', t, 2]
            rem = xres[blk0 + t] + jnp.concatenate([res['r', t, 0] + both, res['r', t, 1] + both], axis=0)
            y = jnp.concatenate([_ssum([(res['p', k], sg) for k, sg in _HK_C[i, t]]) for i in range(3)], axis=0)
            xres[blk0 + t] = y + rem

    def a_left(which=range(15), dep=None):
        for n in which:
            v = _ssum([(xn_f[t, pl.ds(zero(n) + i * D3, D3), :], sg)
                       for (i, t), lst in _HK_C.items() for k, sg in lst if k == n])
            if dep is not None:
                v = jnp.concatenate([tie(v[0:8], dep), v[8:2 * KY], tie(v[2 * KY:2 * KY + 8], dep), v[2 * KY + 8:]],
                                    axis=0)
            t1 = pltpu.bitcast(v[:2 * KY].astype(bf16).T, u32)
            t2 = pltpu.bitcast(jnp.concatenate([v[2 * KY:], v[2 * KY:]], axis=0).astype(bf16).T, u32)
            if dep is None:
                arrange(n, t1, t2)
            else:
                st_s[2 * n] = t1
                st_s[2 * n + 1] = t2

    def arrange(n, t1, t2):
        lo = lax.broadcasted_iota(jnp.int32, (TB // 2, 128), 1) < KY
        s_scr[3 * n] = t1
        s_scr[3 * n + 1] = jnp.where(lo, t1, t2)
        s_scr[3 * n + 2] = jnp.where(lo, t2, t1)

    def a_arrange(n, dep):
        st_s[30, pl.ds(0, 8), :] = pltpu.bitcast(dep, u32)
        arrange(n, st_s[2 * n, pl.ds(zero8, TB // 2), :], st_s[2 * n + 1, pl.ds(zero8, TB // 2), :])

    k0 = math.sqrt(2.0 / math.pi)
    k1 = k0 * 0.044715

    def ffn(j, c0, script):
        clock = _Timeline()
        b0 = (2 * j) % NB
        an = (2 * j + 2) % NB
        acc = [None] * 57
        hs = {}
        lns, lq, staged, nrows = [], [], set(), 0

        pend = []

        def advance(keep):
            while len(pend) > keep:
                pend.pop(0)()

        def written(k):
            clock.due.append(lambda: pltpu.bitcast(p_s[k][pl.ds(zero8, 8), 0:128], u32))

        def gu(p):
            c, m = c0 + p // 2, p % 2
            h = hs.setdefault(p // 2, [[None, None, None] for _ in range(3)])

            def mm(n, kind):
                lhs = gate(s_scr[3 * n + kind], clock)
                return _dot(_up(lhs), _up(pw[c, pl.ds((3 * n + kind) * (TC // 2), TC // 2), m * TC:(m + 1) * TC]))

            def get(name):
                return p_s[PSLOT[name]][pl.ds(zero8, TB), :]

            def post(n, v):
                adds, keep, emits = GU_POST[n]
                if keep[0] is not None:
                    p_s[PSLOT[keep[0]]][...] = v
                    written(PSLOT[keep[0]])
                w_ = v
                for name, sg in adds:
                    w_ = w_ + get(name) if sg == 1 else w_ - get(name)
                if keep[1] is not None:
                    p_s[PSLOT[keep[1]]][...] = w_
                    written(PSLOT[keep[1]])
                if emits is not None:
                    col, half = emits
                    if m == 1:
                        k_ = 17 + 9 * ((p // 2) % NHS) + 3 * col
                        hv = w_ * p_s[11 + 2 * col + half][pl.ds(zero8, TB), :]
                        p_s[k_ + half][...] = hv
                        written(k_ + half)
                        h[col][half] = k_ + half
                        if h[col][1 - half] is not None:
                            p_s[k_ + 2][...] = hv + p_s[k_ + 1 - half][pl.ds(zero8, TB), :]
                            written(k_ + 2)
                            h[col][2] = k_ + 2
                    else:
                        p_s[11 + 2 * col + half][...] = w_ + w_ * jnp.tanh(w_ * (k0 + k1 * (w_ * w_)))
                        written(11 + 2 * col + half)
            for n in GU_ORD:
                both = mm(n, 2)
                v = jnp.concatenate([mm(n, 0) + both, mm(n, 1) + both], axis=1)
                pend.append(functools.partial(post, n, v))
                advance(PLAG)
                clock.tick(96, both, GTK)

        todo = [sum(any(i_ == i for i_, _, _ in z) for z in _Z6) for i in range(6)]

        def gather(i):
            if last:
                ys = [_ssum([(acc[n], sg) for n, sg in sorted(_C6[i, t], key=lambda z: _order6().index(z[0]))])
                      for t in range(2)]
            else:
                t0, t1 = dict(_C6[i, 0]), dict(_C6[i, 1])
                both = _ssum([(acc[n], sg) for n, sg in t0.items() if n in t1])
                ys = (_ssum([(acc[n], sg) for n, sg in t0.items() if n not in t1]) + both,
                      _ssum([(acc[n], sg) for n, sg in t1.items() if n not in t0]) - both)
            for t in range(2):
                x2 = xres[b0 + t, pl.ds(i * D6, D6), :] + 0.5 * ys[t]
                xres[b0 + t, pl.ds(i * D6, D6), :] = x2
                xin[j % NP, pl.ds(i * D6, D6), t * TB:(t + 1) * TB] = x2.astype(bf16)
            if last and i in ORD6[:OSPL]:
                @pl.when(g == 1)
                def _():
                    _cp_rows(i, o_hbm, xin, sems).start()

        def down(ps, final):
            cs = ps[::2]
            hsl = [hs.pop(p // 2) for p in cs]
            for pos, i in enumerate(_order6()):
                while any(h_[j_ % 3][d_] is None for h_ in hsl for j_, d_, _ in _B6[i]):
                    advance(len(pend) - 1)
                au = [pw[c0 + p // 2, pl.ds(R_SD + (i // 2) * (D6 // 2), D6 // 2), _lt(i % 2)] for p in cs]
                au[0] = gate(au[0], clock)
                lhs = jnp.concatenate(au, axis=1)
                rhs = jnp.concatenate([_ssum([(p_s[h_[j_ % 3][d_]][pl.ds(zero(pos % 21), TB), _lt(j_ // 3)], sg)
                                              for j_, d_, sg in _B6[i]]) for h_ in hsl], axis=1).astype(bf16)
                r = _dot_nt(_up(lhs), rhs)
                acc[i] = r if acc[i] is None else r + acc[i]
                if final:
                    for i_ in sorted({i_ for i_, _, _ in _Z6[i]}):
                        todo[i_] -= 1
                        if not todo[i_]:
                            gather(i_)
                if pos % DADV == 0:
                    advance(max(len(pend) - 1, 0))
                clock.tick(24 * len(cs), acc[i], DTK)

        pg = pd = 0
        for tok in script:
            if tok == 'G':
                gu(pg)
                pg += 1
            elif tok[0] == 'D':
                down(list(range(pd, pd + int(tok[1:]))), pd + int(tok[1:]) == script.count('G'))
                pd += int(tok[1:])
            elif tok == 'W':
                assert not clock.pending() and nrows == 2 * nr
                advance(0)
                wo_mm(an, wo_rhs(None))
                clock.t += 1152
            elif tok[0] == 'n':
                lns.append(add_ln(clock, clock.t + int(tok[3:]), LNJ + (JDL,), an + int(tok[1]), xn_f, int(tok[1])))
            elif tok[0] == 'm':
                lq.append(add_ln(clock, clock.t + int(tok[3:]), LNJ + (JDL,), (2 * j + 6) % NB + int(tok[1]), xn_g,
                                 int(tok[1])))
            elif tok[0] == 'k':
                _, t0, dt = tok.split('+')

                def qleft(which, dep):
                    assert len(lq) == 2 and not any(st['left'] for st in lq)
                    q_left(False, which, dep, (j + 1) % 2)
                    return sq_scr[which[0], (j + 1) % 2, pl.ds(zero8, 8), :]
                for k in range(NQL):
                    clock.add_due(clock.t + int(t0) + k * int(dt),
                                  functools.partial(qleft, range(k * 18 // NQL, (k + 1) * 18 // NQL)), LDL)
            elif tok[0] == 'l':
                _, t0, dt = tok.split('+')

                def left(which, dep):
                    assert len(lns) == 2 and not any(st['left'] for st in lns)
                    staged.update(which)
                    a_left(which, dep)
                    return st_s[0, pl.ds(zero8, 8), :]
                for k in range(NLEFT):
                    clock.add_due(clock.t + int(t0) + k * int(dt),
                                  functools.partial(left, range(k * 15 // NLEFT, (k + 1) * 15 // NLEFT)), LDL)
            elif tok[0] == 'c':
                _, t0, dt = tok.split('+')
                assert pg == 2 * NCH

                def place(k, dep):
                    assert k in staged
                    a_arrange(k, dep)
                for k in range(15):
                    clock.add(clock.t + int(t0) + k * int(dt), functools.partial(place, k))
            else:
                n, t0, dt = tok[1:].split('+')
                for k in range(int(n)):
                    add_rows(clock, clock.t + int(t0) + k * int(dt), an + nrows // nr, nrows // nr, nrows % nr,
                             RG + (RDL, JDL))
                    nrows += 1
        assert pg == pd and not clock.pending()

    if last:
        ffn(2 * NP - 1, g * NPC, SCRIPT_F)
        return
    if phase == 'main':
        @pl.when(jnp.logical_and(g >= NP - 1, (g & 1) == 1))
        def _():
            q_step(g - (NP - 1))

        ffn(g, 0, SCRIPT)

        @pl.when(g >= NP)
        def _():
            _cp_out(g - NP, o_hbm, xin, sems).start()
        return
    assert NCH == NP - 2

    late = [(c, m) for c in range(NCH) for m in range(3) if c >= NCH - LAGS[m]]

    def prologue():
        cp_x(0).start()
        for sec in range(3):
            for cp in cp_qkv(sec):
                cp.start()
        qall[:, pl.ds(0, HALO), :] = jnp.zeros((16, HALO, 128), f32)
        cp_x(0).wait()
        for t in range(2):
            x = xin[0, :, t * TB:(t + 1) * TB].astype(f32)
            xres[t] = x
            mean, rstd = _ln_stats(x)
            xn_g[t, pl.ds(zero8, D), :] = (xres[t] - mean) * rstd
        q_left(True)
        for sec in range(3):
            for cp in cp_qkv(sec):
                cp.wait()
            if sec == 0:
                cp_x(1).start()
                cp_x(2).start()
                cp_wo().start()
                for c in range(NCH):
                    if 3 + c < NP:
                        cp_x(3 + c).start()
                    for m in range(3):
                        if c == 0 or c > LAGS[m]:
                            cp_unit(max(c - LAGS[m], 0), m).start()
                for c, m in late:
                    cp_unit(c, m).start()
            if sec == 0:
                transpose_qkv(sec)
                build_wq(sec)
            else:
                q_step(0, CFG_Q0, part=sec - 1)

    def first_attention():
        cp_x(2).wait()
        q_step(1, CFG_QA, rows=True)
        cp_wo().wait()
        build_wo()
        wo_mm(0, wo_rhs(0))
        for t in range(2):
            mean, rstd = _ln_stats(xres[t])
            xn_f[t] = (xres[t] - mean) * rstd
        a_left()

    def startup_step(c, carry):
        @pl.when(c + 3 < NP)
        def _():
            cp_x(c + 3).wait()
        for m in range(3):
            if LAGS[m]:
                @pl.when(jnp.logical_or(c == 0, c > LAGS[m]))
                def _():
                    cp_unit(jnp.maximum(c - LAGS[m], 0), m).wait()
            else:
                cp_unit(c, m).wait()
        q_step(c + 2, CFG_Q1, chunk=c)
        return carry

    @pl.when(g == 0)
    def _():
        prologue()
        cp_x(1).wait()
        q_step(0, CFG_Q0, part=2)
        first_attention()
        lax.fori_loop(0, NCH, startup_step, 0)
        for c, m in late:
            cp_unit(c, m).wait()
        for c, m in late:
            for piece in prep_pieces(c, m):
                piece()


def _cp_out(k, o_hbm, xin, sems):
    return pltpu.make_async_copy(xin.at[k], o_hbm.at[:, pl.ds(_al(k * 2 * TB, 128), 2 * TB)], sems.at[4 + k])


def _cp_rows(i, o_hbm, xin, sems):
    k, n = xin.shape[0] - 1, xin.shape[1] // 6
    return pltpu.make_async_copy(xin.at[k, pl.ds(i * n, n), :], o_hbm.at[pl.ds(i * n, n), pl.ds(k * 2 * TB, 2 * TB)],
                                 sems.at[4 + k])


def _kernel(*refs, D, DF, S):
    def body(phase, g, carry):
        _step(g, phase, *refs, D=D, DF=DF, S=S)
        return carry
    NP = S // (2 * TB)
    lax.fori_loop(0, 2, functools.partial(body, 'start'), 0)
    lax.fori_loop(0, 2 * NP - 1, functools.partial(body, 'main'), 0)
    lax.fori_loop(0, 2, functools.partial(body, 'last'), 0)
    o_hbm, xin, sems = refs[6], refs[7], refs[24]
    for i in ORD6[OSPL:]:
        _cp_rows(i, o_hbm, xin, sems).start()
    for k in range(NP - 1):
        _cp_out(k, o_hbm, xin, sems).wait()
    for i in range(6):
        _cp_rows(i, o_hbm, xin, sems).wait()


@jax.jit
def pallas_interleave_layers__sliding_local_dilated__glu_gated_geglu__prompt_kernel(
    A_x, A_wqkv, A_wo, B_x, B_w_gate, B_w_up, B_w_down):
    B, S, D = A_x.shape
    DF = B_w_gate.shape[1]
    NB = S // TB
    NP = NB // 2
    NCH = DF // CW
    xT = A_x.reshape(S, D).T
    wdT = B_w_down.T
    hbm = pl.BlockSpec(memory_space=pltpu.HBM)
    outT = pl.pallas_call(
        functools.partial(_kernel, D=D, DF=DF, S=S),
        in_specs=[hbm] * 6,
        out_specs=hbm,
        out_shape=jax.ShapeDtypeStruct((D, S), A_x.dtype),
        scratch_shapes=[
            pltpu.VMEM((NP, D, 2 * TB), bf16),
            pltpu.VMEM((D, 3 * D), bf16),
            pltpu.VMEM((D, D), bf16),
            pltpu.VMEM((5, 14 * 128, 128), f32),
            pltpu.VMEM((WQR, 27 * 128), u32),
            pltpu.VMEM((D // 2, 640), u32),
            pltpu.VMEM((D // 4, 18 * 128), u32),
            pltpu.VMEM((NCH, 3, D, CW), bf16),
            pltpu.VMEM((NCH, 45 * (TC // 2) + 15 * (D // 6) + 16, 2 * TC), u32),
            pltpu.VMEM((16, S + QPAD, 128), f32),
            pltpu.VMEM((11, TB, 128), f32),
            pltpu.VMEM((NB, D, TB), f32),
            pltpu.VMEM((2, D, TB), f32),
            pltpu.VMEM((2, D, TB), f32),
            pltpu.VMEM((45, TB // 2, TC), u32),
            pltpu.VMEM((31, TB // 2, TC), u32),
            pltpu.VMEM((18, 2, TB // 2, TC), u32),
            pltpu.SemaphoreType.DMA((4 + NP + 3 * NCH,)),
        ] + [pltpu.VMEM((TB, 2 * TC), f32)] * (17 + 9 * NHS),
        compiler_params=pltpu.CompilerParams(
            vmem_limit_bytes=110 * 1024 * 1024,
            disable_bounds_checks=True,
            disable_semaphore_checks=True,
        ),
    )(xT, A_wqkv, A_wo, B_w_gate, B_w_up, wdT)
    return outT.T.reshape(B, S, D)
```

```python
import functools
import math
import jax
import jax.numpy as jnp
from jax import lax
import jax.experimental.pallas as pl
import jax.experimental.pallas.tpu as pltpu

DH = 18
W = 8
DIL = 2
HALO = 16
EPS = 1e-5
TB = 128
RB = 8
TC = 128
CW = 6 * TC
WQR = 320
KY = 64
QPAD = 40

SCRIPT = ('m0+50,m1+2804,k+5848+80,G,R6+74+200,G,G,R5+74+200,G,G,R6+74+224,G,G,R3+96+200,G,R12+204+330,D8,'
          'W,n0+1476,n1+2028,l+4204+80,G,G,G,G,c+304+96,D4').split(',')
SCRIPT_F = 'G,G,G,G,G,G,D6'.split(',')
GU_ORD = (8, 6, 7, 11, 3, 1, 10, 14, 9, 5, 0, 13, 12, 4, 2)
ORD6 = (0, 4, 3, 1, 5, 2)
WORD = (0, 1, 2, 6, 7, 8, 9, 10, 11, 12, 13, 14, 3, 4, 5)
PLAG, DADV, GTK, DTK, QTK = 6, 2, 2, 2, 8
LNJ = (12, 9, 48, 48)
RG = (2, 1, 24, 400)
RDL, JDL, LDL = 600, 300, 700
NLEFT, NQL, NHS, OSPL = 15, 18, 4, 4
CFG_Q0 = (40, 400, 9, 9, 32, 64, 300)
CFG_QA = (300, 748, 6, 6, 32, 64, 350)
CFG_Q1 = (40, 1456, 9, 9, 64, 64, 300)
BT, SUMT = (640, 560, 30), (60, 40)
QA_T = (300, 1000, 4, 3850)
QP0, QP1, QFR = 100, 3850, 0.6
DCUT = (0, 2, 4, 6, 8, 10, 12, 21, 30, 39, 48, 57)
LAGS = (1, 1, 0)

f32 = jnp.float32
bf16 = jnp.bfloat16
u32 = jnp.uint32
NT = (((1,), (1,)), ((), ()))


def _al(i, n):
    return i if isinstance(i, int) else pl.multiple_of(i, n)


def _lt(k):
    return slice(k * 128, (k + 1) * 128)


def _pk(x):
    return pltpu.bitcast(x.astype(bf16), u32)


def _up(x):
    return pltpu.bitcast(x, bf16)


def _dot(a, b):
    return jnp.dot(a, b, preferred_element_type=f32)


def _dot_nt(a, b):
    return lax.dot_general(a, b, NT, preferred_element_type=f32)


def _tree(fn, xs):
    xs = list(xs)
    while len(xs) > 1:
        xs = [fn(xs[i], xs[i + 1]) for i in range(0, len(xs) - 1, 2)] + ([xs[-1]] if len(xs) % 2 else [])
    return xs[0]


def _ln_stats(x, nacc=4):
    n = x.shape[0]
    c = x[0:1]
    s1 = [None] * nacc
    s2 = [None] * nacc
    for i in range(n // 8):
        d = x[i * 8:(i + 1) * 8] - c
        k = i % nacc
        s1[k] = d if s1[k] is None else s1[k] + d
        dd = d * d
        s2[k] = dd if s2[k] is None else s2[k] + dd
    m = jnp.sum(_tree(jnp.add, s1), axis=0, keepdims=True) * (1.0 / n)
    v = jnp.sum(_tree(jnp.add, s2), axis=0, keepdims=True) * (1.0 / n) - m * m
    v = jnp.maximum(v, 0.0)
    return c + m, lax.rsqrt(v + EPS)


_HK_A = (
    ((0, 0, 1), (0, 2, -1), (1, 0, -1)), ((0, 0, 1), (0, 1, -1), (2, 0, -1)), ((1, 1, 1), (0, 1, -1), (1, 2, -1)),
    ((1, 1, 1), (1, 0, -1), (2, 1, -1)), ((2, 2, 1), (0, 2, -1), (2, 1, -1)), ((2, 2, 1), (1, 2, -1), (2, 0, -1)),
    ((0, 1, 1),), ((0, 1, 1), (1, 0, -1)), ((1, 0, 1),),
    ((0, 2, 1),), ((0, 2, 1), (2, 0, -1)), ((2, 0, 1),),
    ((1, 2, 1),), ((2, 1, 1), (1, 2, -1)), ((2, 1, 1),),
)
_HK_C = {
    (0, 0): ((0, 1), (7, 1), (8, 1), (9, 1), (6, -1)),
    (0, 1): ((1, 1), (6, 1), (10, 1), (11, 1), (9, -1)),
    (1, 0): ((2, 1), (7, 1), (8, 1), (12, 1), (6, -1)),
    (1, 1): ((3, 1), (6, 1), (13, 1), (14, 1), (2, -1), (7, -1)),
    (2, 0): ((5, 1), (9, 1), (12, 1), (13, 1), (4, -1), (10, -1)),
    (2, 1): ((4, 1), (10, 1), (11, 1), (14, 1), (9, -1)),
}
_HK_B = (((0, 0, 1),), ((0, 1, 1),), ((1, 0, 1),), ((1, 0, 1), (1, 1, 1)), ((2, 1, 1),), ((2, 0, 1), (2, 1, 1)),
         ((0, 1, 1), (1, 1, 1)), ((0, 1, 1), (1, 0, 1), (1, 1, 1)), ((0, 0, 1), (0, 1, 1), (1, 0, 1), (1, 1, 1)),
         ((0, 0, 1), (2, 0, 1)), ((0, 0, 1), (2, 0, 1), (2, 1, 1)), ((0, 0, 1), (0, 1, 1), (2, 0, 1), (2, 1, 1)),
         ((1, 0, 1), (2, 0, 1)), ((1, 0, 1), (2, 1, -1)), ((1, 1, 1), (2, 1, 1)))


_HK6 = (
    '+00-01-02-30-50 +00 +00;+00-03+05-10-20 +01 +01;-01+11+13-15-40+41 +11 -10+11;-04-10+11+14+31+51 +12 +10;'
    '-02-12+21+22-23-25+35-42 +21 -20+21;-12-20+21+22+24-32-52+53 +22 +20;-03+31-32+33+43 +30 +30-31;'
    '+13-23-30+33-34 +32 +31;-04+34-40+41+42+44+54 +40 +40;-04+14-24-40-43+44-45 +41 +41;'
    '-05-12+35+45-51-52+53+55 +50 +50-51;+15+21-25+35+50-53-54+55 +52 +51;+01-40 +00+10 +00-01+10-11;'
    '+01-10 +00+12 +01-10+11;-04+10 +02+12 +01+11;+02 +00+20 +00-01+20-21;+02-20 +00+22 +01-20+21;'
    '+20 +02+22 +01+21;+03 +01+31 -00+01-30+31;+03-30 +01+32 +00+30-31;+30 +02+32 +00+30;+05 +01-51 +00-01+50-51;'
    '+05+50 +01-52 -00-50+51;+50 +02-52 +00+50;+31 +10-30 -10+30;+13-31 +11+30 +10-31;+13 +11-31 -11+31;'
    '+40-41 +10-40 +10-11-40+41;+04-14-40+41 +12-40 +10-11+41;+04-14 +12-42 +11-41;+12-51 +10+50 +10-50;'
    '+15+51 +11-50 -10+51;+15-21 +11+51 +11-51;+32+53 +20+30 +20+30;-23+32 +21-30 +20+31;+23-35 +21+31 +21+31;'
    '+42 +20-40 +20-21+40-41;+24+42 +22-40 -20+21+41;+24 +22-42 -21-41;+12+52-53 +20+50 +20+50;'
    '+12+21-25+35+52-53 +21-50 +20+51;-21+25-35 +21+51 +21+51;+43 +31+41 +30-31-40+41;+34+43 +32+41 -30+31+40;'
    '+34 +32+42 +30-40;+45 +41+51 -40+41+50-51;+45+54 +41+52 +40-50+51;+54 +42+52 -40+50;'
    '+40 +01+11+41 -00+01-10+11-40+41;-04+40 +02+12+41 +00-01+10-11+40;+04 +02+12+42 +00+10+40;'
    '+12 +10-20+50 -10+11-20+21+50-51;+12+21 +10-22+50 -11+20-21+51;+21 +12-22+52 +11+21-51;'
    '+35 +21+31+51 -20+21-30+31+50-51;+35+53 +21+31+52 +20+30-50+51;+53 +22+32+52 -20-30+50'
)


def _terms(txt):
    return tuple((int(txt[i + 1]), int(txt[i + 2]), 1 if txt[i] == '+' else -1) for i in range(0, len(txt), 3))


_A6, _B6, _Z6 = zip(*[[_terms(f) for f in row.split(' ')] for row in _HK6.split(';')])
_C6 = {(i, t): [(n, sg) for n, z in enumerate(_Z6) for i_, t_, sg in z if (i_, t_) == (i, t)]
       for i in range(6) for t in range(2)}


def _order6():
    early = [n for n, b in enumerate(_B6) if all(j % 3 == 0 or (j % 3 == 1 and d == 1) for j, d, _ in b)]
    early.sort(key=lambda n: max(d != 1 for _, d, _ in _B6[n]))
    out = list(early)
    for i in ORD6:
        out += [n for n, z in enumerate(_Z6) if n not in out and any(i_ == i for i_, _, _ in z)]
    return out


def _ssum(terms):
    terms = sorted(terms, key=lambda z: -z[1])
    acc = terms[0][0] if terms[0][1] == 1 else -terms[0][0]
    for v, sg in terms[1:]:
        acc = acc + v if sg == 1 else acc - v
    return acc


GU_POST = {
    8: ((), ('p8', None), None),
    7: ((('p8', 1),), (None, 't7'), None),
    3: ((('t7', 1),), (None, 's1'), None),
    6: ((), ('p6', None), None),
    14: ((('p6', 1), ('s1', 1)), ('p14', None), (1, 1)),
    12: ((('p9', 1), ('s2', 1)), ('p12', None), (2, 0)),
    13: ((), ('p13', None), None),
    2: ((('p12', 1), ('p13', 1), ('s1', 1)), (None, None), (1, 0)),
    11: ((), ('p11', None), None),
    10: ((('p11', 1),), (None, 't10'), None),
    5: ((('t10', 1),), (None, 's2'), None),
    9: ((), ('p9', None), None),
    4: ((('p14', 1), ('s2', 1), ('p13', -1)), (None, None), (2, 1)),
    0: ((('p8', 1), ('p9', 1), ('t10', 1)), (None, None), (0, 0)),
    1: ((('p6', 1), ('p11', 1), ('t7', 1)), (None, None), (0, 1)),
}
PSLOT = {k: i for i, k in enumerate(('p8', 't7', 's1', 'p6', 'p14', 'p12', 'p13', 'p11', 't10', 's2', 'p9'))}


class _Timeline:
    def __init__(self):
        self.t = 0
        self.jobs = []
        self.due = []

    def add(self, when, fn):
        self.jobs.append((when, len(self.jobs), fn))
        self.jobs.sort(key=lambda z: z[:2])

    def add_due(self, when, job, delay):
        def run(dep):
            val = job(dep)
            if val is not None:
                self.add(self.t + delay, lambda _: self.due.append(lambda: val))
        self.add(when, run)

    def pending(self):
        return [j for j in self.jobs if getattr(j[2], '__name__', '') != '<lambda>']

    def tick(self, dur, v, n):
        for k in range(n):
            self.t += dur // n
            r = k * (v.shape[0] // n)
            while self.jobs and self.jobs[0][0] <= self.t:
                self.jobs.pop(0)[2](v[r:r + 8, 0:128])


def _step(g, phase, x_hbm, wqkv_hbm, wo_hbm, wg_hbm, wu_hbm, wd_hbm, o_hbm,
          xin, wqkv_raw, wo_raw, tmp, wq, woT, wo2, raw, pw, qall, o_s, xres, xn_f, xn_g, s_scr, st_s, sq_scr,
          sems, *p_s, D, DF, S):
    last = phase == 'last'
    NB = S // TB
    NP = NB // 2
    NCH = DF // CW
    NPC = NCH // 2
    D3 = D // 3
    D6 = D // 6
    nr = TB // RB
    hh = D // 4
    zero8 = pl.multiple_of((g >> 20) * 8, 8)
    zvec = jnp.full((8, 128), (g >> 20).astype(u32), u32)

    def zero(k):
        return pl.multiple_of((g >> (8 + k)) * 8, 8)

    def tie(x, dep):
        return pltpu.bitcast(pltpu.bitcast(x, u32) | (pltpu.bitcast(dep, u32) & zvec), f32)

    def gate(lhs, clock):
        if not clock.due:
            return lhs
        pr = _tree(jnp.bitwise_or, [k() for k in clock.due]) & zvec
        del clock.due[:]
        return jnp.concatenate([lhs[0:8] | pr, lhs[8:]], axis=0)

    QSEC = ((0, 5), (5, 9), (9, 14))

    def cp_qkv(sec):
        out = []
        for j in range(*QSEC[sec]):
            n = min(128, 3 * D - j * 128)
            out.append(pltpu.make_async_copy(wqkv_hbm.at[:, pl.ds(j * 128, n)], wqkv_raw.at[:, pl.ds(j * 128, n)],
                                             sems.at[sec]))
        return out

    def cp_wo():
        return pltpu.make_async_copy(wo_hbm, wo_raw, sems.at[3])

    def cp_x(k):
        return pltpu.make_async_copy(x_hbm.at[:, pl.ds(_al(k * 2 * TB, 128), 2 * TB)], xin.at[k], sems.at[4 + k])

    def cp_unit(c, m):
        return pltpu.make_async_copy((wg_hbm, wu_hbm, wd_hbm)[m].at[:, pl.ds(_al(c * CW, 128), CW)], raw.at[c, m],
                                     sems.at[4 + NP + 3 * c + m])

    R_SD = 45 * (TC // 2)
    R_END = R_SD + 15 * (D3 // 2)

    def hk_a_ops(load, minus=None):
        blk = {}
        for i in range(3):
            for j in range(3):
                blk[i, j] = load(i, j).astype(f32)
                if minus is not None:
                    blk[i, j] = blk[i, j] - minus(i, j).astype(f32)
        return [_pk(_ssum([(blk[i, j], sg) for i, j, sg in terms])) for terms in _HK_A]

    def prep_pieces(c, m):
        def ld(r, cs):
            return lambda i, j: raw[c, m, pl.ds(i * D3 + r, 16), pl.ds((3 * cs + j) * TC, TC)]

        def gu_piece(q, r, cs, neg, kind, half):
            ops = hk_a_ops(ld(q * KY + r, cs), None if neg is None else ld(q * KY + r, neg))
            for k, t in enumerate(ops):
                pw.at[c][pl.ds((3 * k + kind) * (TC // 2) + (half * KY + r) // 2, 8), m * TC:(m + 1) * TC] = t

        def d_piece(r, q, ks):
            blk = {}
            cz = c + (g >> (8 + q))
            for k in ks:
                for i, j, _ in _A6[k]:
                    if (i, j) not in blk:
                        blk[i, j] = raw[cz, m, pl.ds(i * D6 + r, 16), pl.ds(j * TC, TC)].astype(f32)
                pw.at[c][pl.ds(R_SD + (k // 2) * (D6 // 2) + r // 2, 8), _lt(k % 2)] = _pk(
                    _ssum([(blk[i, j], sg) for i, j, sg in _A6[k]]))
        if m == 2:
            return [functools.partial(d_piece, r, q, range(DCUT[q], DCUT[q + 1]))
                    for r in range(0, D6, 16) for q in range(len(DCUT) - 1)]
        spec = ((0, 0, None, 0, 0), (1, 0, 1, 0, 1), (0, 1, None, 1, 0), (2, 1, 0, 1, 1),
                (2, 0, None, 2, 0), (1, 1, None, 2, 1))
        return [functools.partial(gu_piece, q, r, cs, neg, kind, half)
                for r in range(0, KY, 16) for q, cs, neg, kind, half in spec]

    def transpose_qkv(sec):
        for j in range(*QSEC[sec]):
            wd_ = min(128, 3 * D - j * 128)
            blk = wqkv_raw[:, j * 128:j * 128 + wd_].astype(f32)
            if wd_ < 128:
                blk = jnp.concatenate([blk, jnp.zeros((D, 128 - wd_), f32)], axis=1)
            bt = jnp.concatenate([blk, blk[D - KY:]], axis=0).T
            for t in range(5):
                tmp[t, pl.ds(j * 128, 128), :] = bt[:, t * 128:(t + 1) * 128]

    def wq_slot(i, j):
        return 24 + i if i == j else [n for n, t in enumerate(_HK_A) if t == ((i, j, 1),)][0]

    def build_wq(sec, ds=range(DH), dep=None):
        lo = lax.broadcasted_iota(jnp.int32, (32, 128), 1) < KY
        if dep is not None:
            tmp[0, pl.ds(zero8 + 3 * D + 32, 8), :] = dep
        for d in ds:
            tt = [tmp[t, pl.ds(sec * D + d, 32, stride=DH), :] for t in range(5)]
            ops = tt[:4] + [jnp.where(lo, tt[3], tt[4]), jnp.where(lo, tt[4], tt[3])]
            if d < 16:
                dst = [(sec, d * 16)]
            else:
                dst = ([(1, (d + 2) * 16)], [(1, d * 16)], [(0, d * 16), (0, (d + 2) * 16)])[sec]
            for j, row in dst:
                for k, v in enumerate(ops):
                    wq[pl.ds(row, 16), _lt(wq_slot(k, j) if k < 3 else 12 + 3 * j + k)] = _pk(v)

    def wq_sums(r, dep):
        ncol = 3 if r < 256 else 2
        pin = pltpu.bitcast(dep, u32) & zvec
        blk = {(i, j): _up(wq[pl.ds(r, 8), _lt(wq_slot(i, j))] | pin).astype(f32) for i in range(3) for j in range(ncol)}
        for n, terms in enumerate(_HK_A):
            if len(terms) > 1 and not (ncol == 2 and n in (4, 5)):
                wq[pl.ds(r, 8), _lt(n)] = _pk(_ssum([(blk[i, j], sg) for i, j, sg in terms if j < ncol]))

    def build_wo():
        for t in range(5):
            wd_ = min(128, D - t * 128)
            blk = wo_raw[:, t * 128:t * 128 + wd_].astype(f32)
            if wd_ < 128:
                blk = jnp.concatenate([blk, jnp.zeros((D, 128 - wd_), f32)], axis=1)
            tmp[t, pl.ds(0, D), :] = blk
        for t in range(5):
            rows = [tmp[t, pl.ds(d, 32, stride=DH), :] for d in range(DH)]
            ft = jnp.concatenate(rows + rows[16:], axis=0).T
            n = min(128, D - t * 128)
            woT[pl.ds(t * 64, n // 2), :] = _pk(ft[:n])
        for r in range(0, D3 // 2, 8):
            ops = hk_a_ops(lambda i, j: _up(woT[pl.ds(i * (D3 // 2) + r, 8), j * TC:(j + 1) * TC]))
            for k, t in enumerate(ops):
                wo2[pl.ds(r, 8), _lt(k)] = t
        lo = lax.broadcasted_iota(jnp.int32, (16, 128), 1) < KY
        for r in range(0, hh, 8):
            a3, a4, b3, b4 = [_up(woT[pl.ds(r0 + r, 8), c0:c0 + 128]).astype(f32)
                              for r0 in (0, hh) for c0 in (384, 512)]
            wo2[pl.ds(r, 8), _lt(15)] = _pk(jnp.where(lo, a3, a3 - b3))
            wo2[pl.ds(r, 8), _lt(16)] = _pk(jnp.where(lo, b3, b4 - a4))
            wo2[pl.ds(r, 8), _lt(17)] = _pk(jnp.where(lo, a4, b3))

    def q_left(plain, which=None, dep=None, slot=0):
        k1, k2, k3 = 3 * TC, 3 * TC + KY, 3 * TC + 2 * KY
        for n in (list(range(6 if plain else 15)) + [15, 16, 17]) if which is None else which:
            def X(t, r0, rows):
                return xn_g[t, pl.ds((zero8 if plain else zero(n)) + r0, rows), :]
            if n == 15:
                v = jnp.concatenate([X(0, k1, KY), X(0, k2, KY) - X(1, k2, KY)], axis=0)
            elif n == 16:
                v = jnp.concatenate([X(1, k1, KY), X(1, k3, KY) - X(0, k3, KY)], axis=0)
            elif n == 17:
                v = jnp.concatenate([X(0, k3, KY), X(1, k2, KY)], axis=0)
            elif plain:
                v = X(n // 3, (n % 3) * TC, TC)
            else:
                v = _ssum([(X(t, i * TC, TC), sg) for (i, t), lst in _HK_C.items() for k, sg in lst if k == n])
            if dep is not None:
                v = jnp.concatenate([tie(v[0:8], dep), v[8:]], axis=0)
            sq_scr[n, slot] = pltpu.bitcast(v.astype(bf16).T, u32)

    def add_ln(clock, t0, cfg, blk, dst, par, inp=None):
        np1, np2, step, gap, delay = cfg
        st = dict(s1=[], s2=[], left=np2)
        nv = D // 16

        def load(i):
            if inp is None:
                return xres[blk, pl.ds(zero8 + i * 16, 16), :]
            x = inp(i).astype(f32)
            xres[blk, pl.ds(i * 16, 16), :] = x
            return x

        def stats(k, dep):
            xs = []
            for i in range(k * nv // np1, (k + 1) * nv // np1):
                x = load(i)
                xs += [x[0:8], x[8:16]]
            if k == 0:
                st['c'] = jnp.broadcast_to(xs[0][0:1], (8, TB))
            c = tie(st['c'], dep)
            ds = [x - c for x in xs]
            st['s1'].append(_tree(jnp.add, ds))
            st['s2'].append(_tree(jnp.add, [d * d for d in ds]))
            return pltpu.bitcast(st['s1'][-1], u32) | pltpu.bitcast(st['s2'][-1], u32)

        def norm(k, dep):
            if k == 0:
                m = jnp.sum(_tree(jnp.add, st['s1']), axis=0, keepdims=True) * (1.0 / D)
                v = jnp.sum(_tree(jnp.add, st['s2']), axis=0, keepdims=True) * (1.0 / D) - m * m
                st['mean'] = st['c'] + m
                st['rstd'] = jnp.broadcast_to(lax.rsqrt(jnp.maximum(v, 0.0) + EPS), (8, TB))
            mean = tie(st['mean'], dep)
            off = 0 if inp is None else zero8
            for i in range(k * 2 * nv // np2, (k + 1) * 2 * nv // np2):
                dst[par, pl.ds(i * 8, 8), :] = (xres[blk, pl.ds(off + i * 8, 8), :] - mean) * st['rstd']
            st['left'] -= 1
            return pltpu.bitcast(dst[par, pl.ds(zero8, 8), :], u32)
        for k in range(np1):
            clock.add_due(t0 + k * step, functools.partial(stats, k), delay)
        for k in range(np2):
            clock.add_due(t0 + np1 * step + gap + k * step, functools.partial(norm, k), delay)
        return st

    def hk_outputs(P, T, PT, emit, two_cols):
        p8 = P(8)
        t7 = P(7) + p8
        s1 = PT(3, 1, 2) + t7
        p6 = P(6)
        p14 = P(14)
        emit(1, 1, T(1, 1) + (p6 + p14 + s1))
        p13 = P(13)
        if two_cols:
            emit(1, 0, PT(2, 1, 0) + (p13 + s1))
        else:
            p12 = P(12)
            emit(1, 0, PT(2, 1, 0) + (p12 + p13 + s1))
        p11 = P(11)
        t10 = P(10) + p11
        if not two_cols:
            s2 = PT(5, 2, 2) + t10
            p9 = P(9)
            emit(2, 0, T(2, 0) + (p9 + p12 + s2))
            emit(2, 1, PT(4, 2, 1) + (p14 - p13 + s2))
        w0 = T(0, 2)
        emit(0, 0, PT(0, 0, 0) + ((p8 + t10 + w0) if two_cols else (p8 + p9 + t10 + w0)))
        emit(0, 1, PT(1, 0, 1) + (p6 + p11 + t7 + w0))

    QT = (0, 1, 2, 3)
    KT = (4, 5, 6, 7, 13)
    VT = (8, 9, 10, 11, 12)
    c2e = DH ** -0.5 * math.log2(math.e)
    neg = -1e9 * math.log2(math.e)

    def q_step(pr, cfg=None, chunk=None, rows=False, part=None):
        first = cfg is not None
        clock = _Timeline()
        if part is not None:
            base, nx = 0, 1
            if part < 2:
                transpose_qkv(part + 1)
                probe = pltpu.bitcast(tmp[0, pl.ds(zero8, 8), :], u32)
                clock.add(BT[0], lambda _: clock.due.append(lambda: probe))
                for d in range(DH):
                    clock.add(BT[1] + d * BT[2], functools.partial(build_wq, part + 1, [d]))
            else:
                for k in range(40):
                    clock.add(SUMT[0] + k * SUMT[1], functools.partial(wq_sums, 8 * k))
        elif rows:
            base, nx = pr * (2 * TB), pr + 1
            for k in range(2):
                clock.add_due(QA_T[k], functools.partial(row_chain, k, QA_T[2]), QA_T[3] - QA_T[k])
        else:
            base = pl.multiple_of(pr * (2 * TB), 2 * TB)
            nx = jnp.minimum(pr + 1, NP - 1)
        pieces = []
        if chunk is not None:
            for m in range(3):
                pieces += prep_pieces(jnp.maximum(chunk - LAGS[m], 0) if LAGS[m] else chunk, m)

        def paced(piece, dep):
            pw[0, pl.ds(R_END, 8), 0:128] = pltpu.bitcast(dep, u32)
            piece()
        for k, piece in enumerate(pieces):
            frac = k / 48 * QFR if k < 48 else QFR + (k - 48) / (len(pieces) - 48) * (1 - QFR)
            clock.add(QP0 + int(frac * (QP1 - QP0)), functools.partial(paced, piece))
        if first and part in (None, 2):
            for par in range(2):
                add_ln(clock, cfg[par], cfg[2:], 2 * nx + par, xn_g, par,
                       functools.partial(lambda par_, i: xin[nx, pl.ds(i * 16, 16), par_ * TB:(par_ + 1) * TB], par))
        for r0, nt, tiles in ((0, 2, (0, 4, 8)), (TC, 2, (2, 6, 10)), (2 * TC, 1, (12, 13))):
            def R(k):
                return wq[pl.ds(r0, nt * 64), _lt(k)]

            def L(k):
                return sq_scr[k, 0] if first else jnp.concatenate([sq_scr[k, 0], sq_scr[k, 1]], axis=0)

            def P(k):
                return _dot_nt(_up(L(k)), _up(R(k)))

            def T(j, kind):
                rhs = _up(R(15 + 3 * j + kind))
                if nt == 1 and kind == 2:
                    lhs = L(15 + kind)
                    return jnp.concatenate([_dot_nt(_up(lhs[k:k + 32]), rhs) for k in range(0, lhs.shape[0], 32)],
                                           axis=0)
                return _dot_nt(_up(L(15 + kind)), rhs)

            def PT(k, j, kind):
                return _dot_nt(_up(jnp.concatenate([L(k), L(15 + kind)], axis=1)),
                               _up(jnp.concatenate([R(k), R(15 + 3 * j + kind)], axis=1)))

            def emit(col, half, v):
                for k in range(nt):
                    for q_ in range(2):
                        rows_ = pl.ds(base + (HALO + (2 * q_ + half) * TB), TB)
                        qall[tiles[col] + k, rows_, :] = v[q_ * TB:(q_ + 1) * TB, _lt(k)]
            if not first:
                hk_outputs(P, T, PT, emit, nt == 1)
                continue
            for j in range(len(tiles)):
                if part is not None and (j if nt == 2 else 2) != part:
                    continue
                both = T(j, 2)
                clock.t += 32 * nt
                for t in range(2):
                    for k in range(nt):
                        lhs = [L(3 * t + i) for i in range(3)] + [L(15 + t)]
                        lhs[0] = gate(lhs[0], clock)
                        rhs = [wq[pl.ds(r0 + k * 64, 64), _lt(n)]
                               for n in [wq_slot(i, j) for i in range(3)] + [15 + 3 * j + t]]
                        v = _dot_nt(_up(jnp.concatenate(lhs, axis=1)), _up(jnp.concatenate(rhs, axis=1))) + both[:, _lt(k)]
                        qall[tiles[j] + k, pl.ds(base + (HALO + t * TB), TB), :] = v
                        clock.tick(128, v, QTK)
        assert not clock.pending()
        if first and part in (None, 2):
            q_left(True)

    def row_group(blk, par, r, nw, nv, mids=None):
        base = _al(blk * TB, TB)
        lo = lax.broadcasted_iota(jnp.int32, (RB, 128), 1) < KY
        r0 = r * RB

        def ld(t, w):
            return qall[t, pl.ds(base + (HALO + r0 - DIL * w), RB), :]
        dep = yield
        cs = tie(jnp.full((RB, 128), c2e, f32), dep)
        q = [ld(t, 0) * cs for t in QT] + [jnp.where(lo, pltpu.roll(ld(13, 0), KY, 1), 0.0) * cs]
        sc = []
        for w in range(W):
            if w and w % nw == 0:
                dep = yield
                q = [tie(q[0], dep)] + q[1:]
            acc = None
            for j, t in enumerate(KT):
                p = q[j] * ld(t, w)
                acc = p if acc is None else acc + p
            acc = acc + pltpu.roll(acc, 64, 1)
            if mids is not None:
                mids[r] = pltpu.bitcast(acc, u32)
            acc = acc + pltpu.roll(acc, 32, 1)
            if r0 - DIL * w < 0:
                pos = blk * TB + r0 + lax.broadcasted_iota(jnp.int32, (RB, 128), 0)
                acc = jnp.where(pos >= DIL * w, acc, neg)
            sc.append(acc)
        m = _tree(jnp.maximum, sc)
        e = [jnp.exp2(sc[w] - m) for w in range(W)]
        l = _tree(jnp.add, e)
        rinv = pl.reciprocal(l, approx=True)
        rinv = rinv * (2.0 - l * rinv)
        outs = []
        for j, t in enumerate(VT):
            if j and j % nv == 0:
                dep = yield _tree(jnp.bitwise_or, [pltpu.bitcast(v, u32) for v in outs])
                outs = []
                e = [tie(e[0], dep)] + e[1:]
            acc = None
            for w in range(W):
                p = e[w] * ld(t, w)
                acc = p if acc is None else acc + p
            o = acc * rinv
            o_s[par * 5 + j, pl.ds(r0, RB), :] = o
            outs.append(o)
        yield _tree(jnp.bitwise_or, [pltpu.bitcast(v, u32) for v in outs])

    def add_rows(clock, t0, blk, par, r, cfg):
        nw, nv, step, gap, d1, d2 = cfg
        gen = row_group(blk, par, r, nw, nv)
        next(gen)
        n1, n2 = -(-W // nw), -(-5 // nv)
        for k in range(n1):
            clock.add_due(t0 + k * step, gen.send, d1)
        for k in range(n2 - 1):
            clock.add_due(t0 + (n1 - 1) * step + gap + k * step, gen.send, d2)

    def row_chain(blk, lag, dep):
        mids, fins = {}, {}
        for r in range(nr):
            gen = row_group(blk, blk, r, W, 5, mids)
            next(gen)
            if r:
                dep = pltpu.bitcast(mids[r - 1] | fins[r - lag] if r >= lag else mids[r - 1], f32)
            fins[r] = gen.send(dep)
        return _tree(jnp.bitwise_or, [fins[r] for r in range(nr - lag, nr)])

    wo_seq = []
    for pos, k in enumerate(WORD):
        if pos in (0, 2):
            wo_seq += [('r', pos // 2, k_) for k_ in range(3)]
        wo_seq.append(('p', k))

    def wo_rhs(off):
        lo = lax.broadcasted_iota(jnp.int32, (TB, 128), 1) < KY

        rhs = {}
        for it in wo_seq:
            z = zero(wo_seq.index(it)) if off is None else off

            def O(t, j):
                return o_s[t * 5 + j, pl.ds(z, TB), :]
            if it[0] == 'p':
                v = _ssum([(O(t, j), sg) for j, t, sg in _HK_B[it[1]]])
            elif it[2] == 0:
                v = O(it[1], 3)
            else:
                v = jnp.where(lo, O(it[1], 2 + it[2]), O(it[1], 5 - it[2]))
            rhs[it] = v.astype(bf16)
        return rhs

    def wo_mm(blk0, rhs):
        res = {}
        for it in wo_seq:
            if it[0] == 'p':
                lhs = wo2[pl.ds(0, D3 // 2), _lt(it[1])]
            else:
                lhs = wo2[:, _lt(15 + it[2])]
            res[it] = _dot_nt(_up(lhs), rhs[it])
        for t in range(2):
            both = res['r', t, 2]
            rem = xres[blk0 + t] + jnp.concatenate([res['r', t, 0] + both, res['r', t, 1] + both], axis=0)
            y = jnp.concatenate([_ssum([(res['p', k], sg) for k, sg in _HK_C[i, t]]) for i in range(3)], axis=0)
            xres[blk0 + t] = y + rem

    def a_left(which=range(15), dep=None):
        for n in which:
            v = _ssum([(xn_f[t, pl.ds(zero(n) + i * D3, D3), :], sg)
                       for (i, t), lst in _HK_C.items() for k, sg in lst if k == n])
            if dep is not None:
                v = jnp.concatenate([tie(v[0:8], dep), v[8:2 * KY], tie(v[2 * KY:2 * KY + 8], dep), v[2 * KY + 8:]],
                                    axis=0)
            t1 = pltpu.bitcast(v[:2 * KY].astype(bf16).T, u32)
            t2 = pltpu.bitcast(jnp.concatenate([v[2 * KY:], v[2 * KY:]], axis=0).astype(bf16).T, u32)
            if dep is None:
                arrange(n, t1, t2)
            else:
                st_s[2 * n] = t1
                st_s[2 * n + 1] = t2

    def arrange(n, t1, t2):
        lo = lax.broadcasted_iota(jnp.int32, (TB // 2, 128), 1) < KY
        s_scr[3 * n] = t1
        s_scr[3 * n + 1] = jnp.where(lo, t1, t2)
        s_scr[3 * n + 2] = jnp.where(lo, t2, t1)

    def a_arrange(n, dep):
        st_s[30, pl.ds(0, 8), :] = pltpu.bitcast(dep, u32)
        arrange(n, st_s[2 * n, pl.ds(zero8, TB // 2), :], st_s[2 * n + 1, pl.ds(zero8, TB // 2), :])

    k0 = math.sqrt(2.0 / math.pi)
    k1 = k0 * 0.044715

    def ffn(j, c0, script):
        clock = _Timeline()
        b0 = (2 * j) % NB
        an = (2 * j + 2) % NB
        acc = [None] * 57
        hs = {}
        lns, lq, staged, nrows = [], [], set(), 0

        pend = []

        def advance(keep):
            while len(pend) > keep:
                pend.pop(0)()

        def written(k):
            clock.due.append(lambda: pltpu.bitcast(p_s[k][pl.ds(zero8, 8), 0:128], u32))

        def gu(p):
            c, m = c0 + p // 2, p % 2
            h = hs.setdefault(p // 2, [[None, None, None] for _ in range(3)])

            def mm(n, kind):
                lhs = gate(s_scr[3 * n + kind], clock)
                return _dot(_up(lhs), _up(pw[c, pl.ds((3 * n + kind) * (TC // 2), TC // 2), m * TC:(m + 1) * TC]))

            def get(name):
                return p_s[PSLOT[name]][pl.ds(zero8, TB), :]

            def post(n, v):
                adds, keep, emits = GU_POST[n]
                if keep[0] is not None:
                    p_s[PSLOT[keep[0]]][...] = v
                    written(PSLOT[keep[0]])
                w_ = v
                for name, sg in adds:
                    w_ = w_ + get(name) if sg == 1 else w_ - get(name)
                if keep[1] is not None:
                    p_s[PSLOT[keep[1]]][...] = w_
                    written(PSLOT[keep[1]])
                if emits is not None:
                    col, half = emits
                    if m == 1:
                        k_ = 17 + 9 * ((p // 2) % NHS) + 3 * col
                        hv = w_ * p_s[11 + 2 * col + half][pl.ds(zero8, TB), :]
                        p_s[k_ + half][...] = hv
                        written(k_ + half)
                        h[col][half] = k_ + half
                        if h[col][1 - half] is not None:
                            p_s[k_ + 2][...] = hv + p_s[k_ + 1 - half][pl.ds(zero8, TB), :]
                            written(k_ + 2)
                            h[col][2] = k_ + 2
                    else:
                        p_s[11 + 2 * col + half][...] = w_ + w_ * jnp.tanh(w_ * (k0 + k1 * (w_ * w_)))
                        written(11 + 2 * col + half)
            for n in GU_ORD:
                both = mm(n, 2)
                v = jnp.concatenate([mm(n, 0) + both, mm(n, 1) + both], axis=1)
                pend.append(functools.partial(post, n, v))
                advance(PLAG)
                clock.tick(96, both, GTK)

        todo = [sum(any(i_ == i for i_, _, _ in z) for z in _Z6) for i in range(6)]

        def gather(i):
            ys = [_ssum([(acc[n], sg) for n, sg in sorted(_C6[i, t], key=lambda z: _order6().index(z[0]))])
                  for t in range(2)]
            for t in range(2):
                x2 = xres[b0 + t, pl.ds(i * D6, D6), :] + 0.5 * ys[t]
                xres[b0 + t, pl.ds(i * D6, D6), :] = x2
                xin[j % NP, pl.ds(i * D6, D6), t * TB:(t + 1) * TB] = x2.astype(bf16)
            if last and i in ORD6[:OSPL]:
                @pl.when(g == 1)
                def _():
                    _cp_rows(i, o_hbm, xin, sems).start()

        def down(ps, final):
            cs = ps[::2]
            hsl = [hs.pop(p // 2) for p in cs]
            for pos, i in enumerate(_order6()):
                while any(h_[j_ % 3][d_] is None for h_ in hsl for j_, d_, _ in _B6[i]):
                    advance(len(pend) - 1)
                au = [pw[c0 + p // 2, pl.ds(R_SD + (i // 2) * (D6 // 2), D6 // 2), _lt(i % 2)] for p in cs]
                au[0] = gate(au[0], clock)
                lhs = jnp.concatenate(au, axis=1)
                rhs = jnp.concatenate([_ssum([(p_s[h_[j_ % 3][d_]][pl.ds(zero(pos % 21), TB), _lt(j_ // 3)], sg)
                                              for j_, d_, sg in _B6[i]]) for h_ in hsl], axis=1).astype(bf16)
                r = _dot_nt(_up(lhs), rhs)
                acc[i] = r if acc[i] is None else r + acc[i]
                if final:
                    for i_ in sorted({i_ for i_, _, _ in _Z6[i]}):
                        todo[i_] -= 1
                        if not todo[i_]:
                            gather(i_)
                if pos % DADV == 0:
                    advance(max(len(pend) - 1, 0))
                clock.tick(24 * len(cs), acc[i], DTK)

        pg = pd = 0
        for tok in script:
            if tok == 'G':
                gu(pg)
                pg += 1
            elif tok[0] == 'D':
                down(list(range(pd, pd + int(tok[1:]))), pd + int(tok[1:]) == script.count('G'))
                pd += int(tok[1:])
            elif tok == 'W':
                assert not clock.pending() and nrows == 2 * nr
                advance(0)
                wo_mm(an, wo_rhs(None))
                clock.t += 1152
            elif tok[0] == 'n':
                lns.append(add_ln(clock, clock.t + int(tok[3:]), LNJ + (JDL,), an + int(tok[1]), xn_f, int(tok[1])))
            elif tok[0] == 'm':
                lq.append(add_ln(clock, clock.t + int(tok[3:]), LNJ + (JDL,), (2 * j + 6) % NB + int(tok[1]), xn_g,
                                 int(tok[1])))
            elif tok[0] == 'k':
                _, t0, dt = tok.split('+')

                def qleft(which, dep):
                    assert len(lq) == 2 and not any(st['left'] for st in lq)
                    q_left(False, which, dep, (j + 1) % 2)
                    return sq_scr[which[0], (j + 1) % 2, pl.ds(zero8, 8), :]
                for k in range(NQL):
                    clock.add_due(clock.t + int(t0) + k * int(dt),
                                  functools.partial(qleft, range(k * 18 // NQL, (k + 1) * 18 // NQL)), LDL)
            elif tok[0] == 'l':
                _, t0, dt = tok.split('+')

                def left(which, dep):
                    assert len(lns) == 2 and not any(st['left'] for st in lns)
                    staged.update(which)
                    a_left(which, dep)
                    return st_s[0, pl.ds(zero8, 8), :]
                for k in range(NLEFT):
                    clock.add_due(clock.t + int(t0) + k * int(dt),
                                  functools.partial(left, range(k * 15 // NLEFT, (k + 1) * 15 // NLEFT)), LDL)
            elif tok[0] == 'c':
                _, t0, dt = tok.split('+')
                assert pg == 2 * NCH

                def place(k, dep):
                    assert k in staged
                    a_arrange(k, dep)
                for k in range(15):
                    clock.add(clock.t + int(t0) + k * int(dt), functools.partial(place, k))
            else:
                n, t0, dt = tok[1:].split('+')
                for k in range(int(n)):
                    add_rows(clock, clock.t + int(t0) + k * int(dt), an + nrows // nr, nrows // nr, nrows % nr,
                             RG + (RDL, JDL))
                    nrows += 1
        assert pg == pd and not clock.pending()

    if last:
        ffn(2 * NP - 1, g * NPC, SCRIPT_F)
        return
    if phase == 'main':
        @pl.when(jnp.logical_and(g >= NP - 1, (g & 1) == 1))
        def _():
            q_step(g - (NP - 1))

        ffn(g, 0, SCRIPT)

        @pl.when(g >= NP)
        def _():
            _cp_out(g - NP, o_hbm, xin, sems).start()
        return
    assert NCH == NP - 2

    late = [(c, m) for c in range(NCH) for m in range(3) if c >= NCH - LAGS[m]]

    def prologue():
        cp_x(0).start()
        for sec in range(3):
            for cp in cp_qkv(sec):
                cp.start()
        qall[:, pl.ds(0, HALO), :] = jnp.zeros((16, HALO, 128), f32)
        cp_x(0).wait()
        for t in range(2):
            x = xin[0, :, t * TB:(t + 1) * TB].astype(f32)
            xres[t] = x
            mean, rstd = _ln_stats(x)
            xn_g[t, pl.ds(zero8, D), :] = (xres[t] - mean) * rstd
        q_left(True)
        for sec in range(3):
            for cp in cp_qkv(sec):
                cp.wait()
            if sec == 0:
                cp_x(1).start()
                cp_x(2).start()
                cp_wo().start()
                for c in range(NCH):
                    if 3 + c < NP:
                        cp_x(3 + c).start()
                    for m in range(3):
                        if c == 0 or c > LAGS[m]:
                            cp_unit(max(c - LAGS[m], 0), m).start()
                for c, m in late:
                    cp_unit(c, m).start()
            if sec == 0:
                transpose_qkv(sec)
                build_wq(sec)
            else:
                q_step(0, CFG_Q0, part=sec - 1)

    def first_attention():
        cp_x(2).wait()
        q_step(1, CFG_QA, rows=True)
        cp_wo().wait()
        build_wo()
        wo_mm(0, wo_rhs(0))
        for t in range(2):
            mean, rstd = _ln_stats(xres[t])
            xn_f[t] = (xres[t] - mean) * rstd
        a_left()

    def startup_step(c, carry):
        @pl.when(c + 3 < NP)
        def _():
            cp_x(c + 3).wait()
        for m in range(3):
            if LAGS[m]:
                @pl.when(jnp.logical_or(c == 0, c > LAGS[m]))
                def _():
                    cp_unit(jnp.maximum(c - LAGS[m], 0), m).wait()
            else:
                cp_unit(c, m).wait()
        q_step(c + 2, CFG_Q1, chunk=c)
        return carry

    @pl.when(g == 0)
    def _():
        prologue()
        cp_x(1).wait()
        q_step(0, CFG_Q0, part=2)
        first_attention()
        lax.fori_loop(0, NCH, startup_step, 0)
        for c, m in late:
            cp_unit(c, m).wait()
        for c, m in late:
            for piece in prep_pieces(c, m):
                piece()


def _cp_out(k, o_hbm, xin, sems):
    return pltpu.make_async_copy(xin.at[k], o_hbm.at[:, pl.ds(_al(k * 2 * TB, 128), 2 * TB)], sems.at[4 + k])


def _cp_rows(i, o_hbm, xin, sems):
    k, n = xin.shape[0] - 1, xin.shape[1] // 6
    return pltpu.make_async_copy(xin.at[k, pl.ds(i * n, n), :], o_hbm.at[pl.ds(i * n, n), pl.ds(k * 2 * TB, 2 * TB)],
                                 sems.at[4 + k])


def _kernel(*refs, D, DF, S):
    def body(phase, g, carry):
        _step(g, phase, *refs, D=D, DF=DF, S=S)
        return carry
    NP = S // (2 * TB)
    lax.fori_loop(0, 2, functools.partial(body, 'start'), 0)
    lax.fori_loop(0, 2 * NP - 1, functools.partial(body, 'main'), 0)
    lax.fori_loop(0, 2, functools.partial(body, 'last'), 0)
    o_hbm, xin, sems = refs[6], refs[7], refs[24]
    for i in ORD6[OSPL:]:
        _cp_rows(i, o_hbm, xin, sems).start()
    for k in range(NP - 1):
        _cp_out(k, o_hbm, xin, sems).wait()
    for i in range(6):
        _cp_rows(i, o_hbm, xin, sems).wait()


@jax.jit
def pallas_interleave_layers__sliding_local_dilated__glu_gated_geglu__prompt_kernel(
    A_x, A_wqkv, A_wo, B_x, B_w_gate, B_w_up, B_w_down):
    B, S, D = A_x.shape
    DF = B_w_gate.shape[1]
    NB = S // TB
    NP = NB // 2
    NCH = DF // CW
    xT = A_x.reshape(S, D).T
    wdT = B_w_down.T
    hbm = pl.BlockSpec(memory_space=pltpu.HBM)
    outT = pl.pallas_call(
        functools.partial(_kernel, D=D, DF=DF, S=S),
        in_specs=[hbm] * 6,
        out_specs=hbm,
        out_shape=jax.ShapeDtypeStruct((D, S), A_x.dtype),
        scratch_shapes=[
            pltpu.VMEM((NP, D, 2 * TB), bf16),
            pltpu.VMEM((D, 3 * D), bf16),
            pltpu.VMEM((D, D), bf16),
            pltpu.VMEM((5, 14 * 128, 128), f32),
            pltpu.VMEM((WQR, 27 * 128), u32),
            pltpu.VMEM((D // 2, 640), u32),
            pltpu.VMEM((D // 4, 18 * 128), u32),
            pltpu.VMEM((NCH, 3, D, CW), bf16),
            pltpu.VMEM((NCH, 45 * (TC // 2) + 15 * (D // 6) + 16, 2 * TC), u32),
            pltpu.VMEM((16, S + QPAD, 128), f32),
            pltpu.VMEM((11, TB, 128), f32),
            pltpu.VMEM((NB, D, TB), f32),
            pltpu.VMEM((2, D, TB), f32),
            pltpu.VMEM((2, D, TB), f32),
            pltpu.VMEM((45, TB // 2, TC), u32),
            pltpu.VMEM((31, TB // 2, TC), u32),
            pltpu.VMEM((18, 2, TB // 2, TC), u32),
            pltpu.SemaphoreType.DMA((4 + NP + 3 * NCH,)),
        ] + [pltpu.VMEM((TB, 2 * TC), f32)] * (17 + 9 * NHS),
        compiler_params=pltpu.CompilerParams(
            vmem_limit_bytes=110 * 1024 * 1024,
            disable_bounds_checks=True,
            disable_semaphore_checks=True,
        ),
    )(xT, A_wqkv, A_wo, B_w_gate, B_w_up, wdT)
    return outT.T.reshape(B, S, D)
```

```python
import functools
import math
import jax
import jax.numpy as jnp
from jax import lax
import jax.experimental.pallas as pl
import jax.experimental.pallas.tpu as pltpu

DH = 18
W = 8
DIL = 2
HALO = 16
EPS = 1e-5
TB = 128
RB = 8
TC = 128
CW = 6 * TC
WQR = 320
KY = 64
QPAD = 40

SCRIPT = ('m0+0,m1+2804,k+5848+80,G,R6+74+200,G,G,R5+74+200,G,G,R6+74+224,G,G,R3+144+200,G,R12+204+330,D8,'
          'W,n0+1476,n1+2028,l+4204+80,G,G,G,G,c+256+96,D4').split(',')
SCRIPT_F = 'G,G,G,G,G,G,D6'.split(',')
GU_ORD = (8, 6, 7, 11, 3, 1, 10, 14, 9, 5, 0, 13, 12, 4, 2)
D_ORD = (1, 2, 9, 18, 26, 42, 7, 0, 48, 6, 19, 20, 25, 43, 12, 15, 13, 14, 16, 21, 17, 22, 23, 49, 8, 37, 28, 29, 27, 36,
         50, 38, 45, 24, 46, 44, 47, 33, 34, 54, 35, 55, 56, 3, 30, 31, 51, 32, 52, 53, 10, 11, 39, 40, 41, 4, 5)
ORD6 = (0, 4, 3, 1, 5, 2)
WORD = (0, 1, 2, 6, 7, 8, 9, 10, 11, 12, 13, 14, 3, 4, 5)
PLAG, DADV, GTK, DTK, QTK = 6, 3, 2, 2, 8
LNJ = (12, 9, 48, 48)
RG = (2, 1, 24, 400)
RDL, JDL, LDL = 600, 300, 700
NLEFT, NQL, NHS, OSPL = 15, 18, 4, 4
CFG_Q0 = (40, 400, 9, 9, 32, 64, 300)
CFG_QA = (300, 748, 6, 6, 32, 64, 350)
CFG_Q1 = (40, 1456, 9, 9, 64, 64, 300)
BT, SUMT = (640, 560, 30), (60, 40)
QA_T = (300, 1000, 4, 3850)
QP0, QP1, QFR = 100, 3850, 0.6
DCUT = (0, 2, 4, 6, 8, 10, 12, 21, 30, 39, 48, 57)
LAGS = (1, 1, 0)

f32 = jnp.float32
bf16 = jnp.bfloat16
u32 = jnp.uint32
NT = (((1,), (1,)), ((), ()))


def _al(i, n):
    return i if isinstance(i, int) else pl.multiple_of(i, n)


def _lt(k):
    return slice(k * 128, (k + 1) * 128)


def _pk(x):
    return pltpu.bitcast(x.astype(bf16), u32)


def _up(x):
    return pltpu.bitcast(x, bf16)


def _dot(a, b):
    return jnp.dot(a, b, preferred_element_type=f32)


def _dot_nt(a, b):
    return lax.dot_general(a, b, NT, preferred_element_type=f32)


def _tree(fn, xs):
    xs = list(xs)
    while len(xs) > 1:
        xs = [fn(xs[i], xs[i + 1]) for i in range(0, len(xs) - 1, 2)] + ([xs[-1]] if len(xs) % 2 else [])
    return xs[0]


def _ln_stats(x, nacc=4):
    n = x.shape[0]
    c = x[0:1]
    s1 = [None] * nacc
    s2 = [None] * nacc
    for i in range(n // 8):
        d = x[i * 8:(i + 1) * 8] - c
        k = i % nacc
        s1[k] = d if s1[k] is None else s1[k] + d
        dd = d * d
        s2[k] = dd if s2[k] is None else s2[k] + dd
    m = jnp.sum(_tree(jnp.add, s1), axis=0, keepdims=True) * (1.0 / n)
    v = jnp.sum(_tree(jnp.add, s2), axis=0, keepdims=True) * (1.0 / n) - m * m
    v = jnp.maximum(v, 0.0)
    return c + m, lax.rsqrt(v + EPS)


_HK_A = (
    ((0, 0, 1), (0, 2, -1), (1, 0, -1)), ((0, 0, 1), (0, 1, -1), (2, 0, -1)), ((1, 1, 1), (0, 1, -1), (1, 2, -1)),
    ((1, 1, 1), (1, 0, -1), (2, 1, -1)), ((2, 2, 1), (0, 2, -1), (2, 1, -1)), ((2, 2, 1), (1, 2, -1), (2, 0, -1)),
    ((0, 1, 1),), ((0, 1, 1), (1, 0, -1)), ((1, 0, 1),),
    ((0, 2, 1),), ((0, 2, 1), (2, 0, -1)), ((2, 0, 1),),
    ((1, 2, 1),), ((2, 1, 1), (1, 2, -1)), ((2, 1, 1),),
)
_HK_C = {
    (0, 0): ((0, 1), (7, 1), (8, 1), (9, 1), (6, -1)),
    (0, 1): ((1, 1), (6, 1), (10, 1), (11, 1), (9, -1)),
    (1, 0): ((2, 1), (7, 1), (8, 1), (12, 1), (6, -1)),
    (1, 1): ((3, 1), (6, 1), (13, 1), (14, 1), (2, -1), (7, -1)),
    (2, 0): ((5, 1), (9, 1), (12, 1), (13, 1), (4, -1), (10, -1)),
    (2, 1): ((4, 1), (10, 1), (11, 1), (14, 1), (9, -1)),
}
_HK_B = (((0, 0, 1),), ((0, 1, 1),), ((1, 0, 1),), ((1, 0, 1), (1, 1, 1)), ((2, 1, 1),), ((2, 0, 1), (2, 1, 1)),
         ((0, 1, 1), (1, 1, 1)), ((0, 1, 1), (1, 0, 1), (1, 1, 1)), ((0, 0, 1), (0, 1, 1), (1, 0, 1), (1, 1, 1)),
         ((0, 0, 1), (2, 0, 1)), ((0, 0, 1), (2, 0, 1), (2, 1, 1)), ((0, 0, 1), (0, 1, 1), (2, 0, 1), (2, 1, 1)),
         ((1, 0, 1), (2, 0, 1)), ((1, 0, 1), (2, 1, -1)), ((1, 1, 1), (2, 1, 1)))


_HK6 = (
    '+00-01-02-30-50 +00 +00;+00-03+05-10-20 +01 +01;-01+11+13-15-40+41 +11 -10+11;-04-10+11+14+31+51 +12 +10;'
    '-02-12+21+22-23-25+35-42 +21 -20+21;-12-20+21+22+24-32-52+53 +22 +20;-03+31-32+33+43 +30 +30-31;'
    '+13-23-30+33-34 +32 +31;-04+34-40+41+42+44+54 +40 +40;-04+14-24-40-43+44-45 +41 +41;'
    '-05-12+35+45-51-52+53+55 +50 +50-51;+15+21-25+35+50-53-54+55 +52 +51;+01-40 +00+10 +00-01+10-11;'
    '+01-10 +00+12 +01-10+11;-04+10 +02+12 +01+11;+02 +00+20 +00-01+20-21;+02-20 +00+22 +01-20+21;'
    '+20 +02+22 +01+21;+03 +01+31 -00+01-30+31;+03-30 +01+32 +00+30-31;+30 +02+32 +00+30;+05 +01-51 +00-01+50-51;'
    '+05+50 +01-52 -00-50+51;+50 +02-52 +00+50;+31 +10-30 -10+30;+13-31 +11+30 +10-31;+13 +11-31 -11+31;'
    '+40-41 +10-40 +10-11-40+41;+04-14-40+41 +12-40 +10-11+41;+04-14 +12-42 +11-41;+12-51 +10+50 +10-50;'
    '+15+51 +11-50 -10+51;+15-21 +11+51 +11-51;+32+53 +20+30 +20+30;-23+32 +21-30 +20+31;+23-35 +21+31 +21+31;'
    '+42 +20-40 +20-21+40-41;+24+42 +22-40 -20+21+41;+24 +22-42 -21-41;+12+52-53 +20+50 +20+50;'
    '+12+21-25+35+52-53 +21-50 +20+51;-21+25-35 +21+51 +21+51;+43 +31+41 +30-31-40+41;+34+43 +32+41 -30+31+40;'
    '+34 +32+42 +30-40;+45 +41+51 -40+41+50-51;+45+54 +41+52 +40-50+51;+54 +42+52 -40+50;'
    '+40 +01+11+41 -00+01-10+11-40+41;-04+40 +02+12+41 +00-01+10-11+40;+04 +02+12+42 +00+10+40;'
    '+12 +10-20+50 -10+11-20+21+50-51;+12+21 +10-22+50 -11+20-21+51;+21 +12-22+52 +11+21-51;'
    '+35 +21+31+51 -20+21-30+31+50-51;+35+53 +21+31+52 +20+30-50+51;+53 +22+32+52 -20-30+50'
)


def _terms(txt):
    return tuple((int(txt[i + 1]), int(txt[i + 2]), 1 if txt[i] == '+' else -1) for i in range(0, len(txt), 3))


_A6, _B6, _Z6 = zip(*[[_terms(f) for f in row.split(' ')] for row in _HK6.split(';')])
_C6 = {(i, t): [(n, sg) for n, z in enumerate(_Z6) for i_, t_, sg in z if (i_, t_) == (i, t)]
       for i in range(6) for t in range(2)}


def _ssum(terms):
    terms = sorted(terms, key=lambda z: -z[1])
    acc = terms[0][0] if terms[0][1] == 1 else -terms[0][0]
    for v, sg in terms[1:]:
        acc = acc + v if sg == 1 else acc - v
    return acc


GU_POST = {
    8: ((), ('p8', None), None),
    7: ((('p8', 1),), (None, 't7'), None),
    3: ((('t7', 1),), (None, 's1'), None),
    6: ((), ('p6', None), None),
    14: ((('p6', 1), ('s1', 1)), ('p14', None), (1, 1)),
    12: ((('p9', 1), ('s2', 1)), ('p12', None), (2, 0)),
    13: ((), ('p13', None), None),
    2: ((('p12', 1), ('p13', 1), ('s1', 1)), (None, None), (1, 0)),
    11: ((), ('p11', None), None),
    10: ((('p11', 1),), (None, 't10'), None),
    5: ((('t10', 1),), (None, 's2'), None),
    9: ((), ('p9', None), None),
    4: ((('p14', 1), ('s2', 1), ('p13', -1)), (None, None), (2, 1)),
    0: ((('p8', 1), ('p9', 1), ('t10', 1)), (None, None), (0, 0)),
    1: ((('p6', 1), ('p11', 1), ('t7', 1)), (None, None), (0, 1)),
}
PSLOT = {k: i for i, k in enumerate(('p8', 't7', 's1', 'p6', 'p14', 'p12', 'p13', 'p11', 't10', 's2', 'p9'))}


class _Timeline:
    def __init__(self):
        self.t = 0
        self.jobs = []
        self.due = []

    def add(self, when, fn):
        self.jobs.append((when, len(self.jobs), fn))
        self.jobs.sort(key=lambda z: z[:2])

    def add_due(self, when, job, delay):
        def run(dep):
            val = job(dep)
            if val is not None:
                self.add(self.t + delay, lambda _: self.due.append(lambda: val))
        self.add(when, run)

    def pending(self):
        return [j for j in self.jobs if getattr(j[2], '__name__', '') != '<lambda>']

    def tick(self, dur, v, n):
        for k in range(n):
            self.t += dur // n
            r = k * (v.shape[0] // n)
            while self.jobs and self.jobs[0][0] <= self.t:
                self.jobs.pop(0)[2](v[r:r + 8, 0:128])


def _step(g, phase, x_hbm, wqkv_hbm, wo_hbm, wg_hbm, wu_hbm, wd_hbm, o_hbm,
          xin, wqkv_raw, wo_raw, tmp, wq, woT, wo2, raw, pw, qall, o_s, xres, xn_f, xn_g, s_scr, st_s, sq_scr,
          sems, *p_s, D, DF, S):
    last = phase == 'last'
    NB = S // TB
    NP = NB // 2
    NCH = DF // CW
    NPC = NCH // 2
    D3 = D // 3
    D6 = D // 6
    nr = TB // RB
    hh = D // 4
    zero8 = pl.multiple_of((g >> 20) * 8, 8)
    zvec = jnp.full((8, 128), (g >> 20).astype(u32), u32)

    def zero(k):
        return pl.multiple_of((g >> (8 + k)) * 8, 8)

    def tie(x, dep):
        return pltpu.bitcast(pltpu.bitcast(x, u32) | (pltpu.bitcast(dep, u32) & zvec), f32)

    def gate(lhs, clock):
        if not clock.due:
            return lhs
        pr = _tree(jnp.bitwise_or, [k() for k in clock.due]) & zvec
        del clock.due[:]
        return jnp.concatenate([lhs[0:8] | pr, lhs[8:]], axis=0)

    QSEC = ((0, 5), (5, 9), (9, 14))

    def cp_qkv(sec):
        out = []
        for j in range(*QSEC[sec]):
            n = min(128, 3 * D - j * 128)
            out.append(pltpu.make_async_copy(wqkv_hbm.at[:, pl.ds(j * 128, n)], wqkv_raw.at[:, pl.ds(j * 128, n)],
                                             sems.at[sec]))
        return out

    def cp_wo():
        return pltpu.make_async_copy(wo_hbm, wo_raw, sems.at[3])

    def cp_x(k):
        return pltpu.make_async_copy(x_hbm.at[:, pl.ds(_al(k * 2 * TB, 128), 2 * TB)], xin.at[k], sems.at[4 + k])

    def cp_unit(c, m):
        return pltpu.make_async_copy((wg_hbm, wu_hbm, wd_hbm)[m].at[:, pl.ds(_al(c * CW, 128), CW)], raw.at[c, m],
                                     sems.at[4 + NP + 3 * c + m])

    R_SD = 45 * (TC // 2)
    R_END = R_SD + 15 * (D3 // 2)

    def hk_a_ops(load, minus=None):
        blk = {}
        for i in range(3):
            for j in range(3):
                blk[i, j] = load(i, j).astype(f32)
                if minus is not None:
                    blk[i, j] = blk[i, j] - minus(i, j).astype(f32)
        return [_pk(_ssum([(blk[i, j], sg) for i, j, sg in terms])) for terms in _HK_A]

    def prep_pieces(c, m):
        def ld(r, cs):
            return lambda i, j: raw[c, m, pl.ds(i * D3 + r, 16), pl.ds((3 * cs + j) * TC, TC)]

        def gu_piece(q, r, cs, neg, kind, half):
            ops = hk_a_ops(ld(q * KY + r, cs), None if neg is None else ld(q * KY + r, neg))
            for k, t in enumerate(ops):
                pw.at[c][pl.ds((3 * k + kind) * (TC // 2) + (half * KY + r) // 2, 8), m * TC:(m + 1) * TC] = t

        def d_piece(r, q, ks):
            blk = {}
            cz = c + (g >> (8 + q))
            for k in ks:
                for i, j, _ in _A6[k]:
                    if (i, j) not in blk:
                        blk[i, j] = raw[cz, m, pl.ds(i * D6 + r, 16), pl.ds(j * TC, TC)].astype(f32)
                pw.at[c][pl.ds(R_SD + (k // 2) * (D6 // 2) + r // 2, 8), _lt(k % 2)] = _pk(
                    _ssum([(blk[i, j], sg) for i, j, sg in _A6[k]]))
        if m == 2:
            return [functools.partial(d_piece, r, q, range(DCUT[q], DCUT[q + 1]))
                    for r in range(0, D6, 16) for q in range(len(DCUT) - 1)]
        spec = ((0, 0, None, 0, 0), (1, 0, 1, 0, 1), (0, 1, None, 1, 0), (2, 1, 0, 1, 1),
                (2, 0, None, 2, 0), (1, 1, None, 2, 1))
        return [functools.partial(gu_piece, q, r, cs, neg, kind, half)
                for r in range(0, KY, 16) for q, cs, neg, kind, half in spec]

    def transpose_qkv(sec):
        for j in range(*QSEC[sec]):
            wd_ = min(128, 3 * D - j * 128)
            blk = wqkv_raw[:, j * 128:j * 128 + wd_].astype(f32)
            if wd_ < 128:
                blk = jnp.concatenate([blk, jnp.zeros((D, 128 - wd_), f32)], axis=1)
            bt = jnp.concatenate([blk, blk[D - KY:]], axis=0).T
            for t in range(5):
                tmp[t, pl.ds(j * 128, 128), :] = bt[:, t * 128:(t + 1) * 128]

    def wq_slot(i, j):
        return 24 + i if i == j else [n for n, t in enumerate(_HK_A) if t == ((i, j, 1),)][0]

    def build_wq(sec, ds=range(DH), dep=None):
        lo = lax.broadcasted_iota(jnp.int32, (32, 128), 1) < KY
        if dep is not None:
            tmp[0, pl.ds(zero8 + 3 * D + 32, 8), :] = dep
        for d in ds:
            tt = [tmp[t, pl.ds(sec * D + d, 32, stride=DH), :] for t in range(5)]
            ops = tt[:4] + [jnp.where(lo, tt[3], tt[4]), jnp.where(lo, tt[4], tt[3])]
            if d < 16:
                dst = [(sec, d * 16)]
            else:
                dst = ([(1, (d + 2) * 16)], [(1, d * 16)], [(0, d * 16), (0, (d + 2) * 16)])[sec]
            for j, row in dst:
                for k, v in enumerate(ops):
                    wq[pl.ds(row, 16), _lt(wq_slot(k, j) if k < 3 else 12 + 3 * j + k)] = _pk(v)

    def wq_sums(r, dep):
        ncol = 3 if r < 256 else 2
        pin = pltpu.bitcast(dep, u32) & zvec
        blk = {(i, j): _up(wq[pl.ds(r, 8), _lt(wq_slot(i, j))] | pin).astype(f32) for i in range(3) for j in range(ncol)}
        for n, terms in enumerate(_HK_A):
            if len(terms) > 1 and not (ncol == 2 and n in (4, 5)):
                wq[pl.ds(r, 8), _lt(n)] = _pk(_ssum([(blk[i, j], sg) for i, j, sg in terms if j < ncol]))

    def build_wo():
        for t in range(5):
            wd_ = min(128, D - t * 128)
            blk = wo_raw[:, t * 128:t * 128 + wd_].astype(f32)
            if wd_ < 128:
                blk = jnp.concatenate([blk, jnp.zeros((D, 128 - wd_), f32)], axis=1)
            tmp[t, pl.ds(0, D), :] = blk
        for t in range(5):
            rows = [tmp[t, pl.ds(d, 32, stride=DH), :] for d in range(DH)]
            ft = jnp.concatenate(rows + rows[16:], axis=0).T
            n = min(128, D - t * 128)
            woT[pl.ds(t * 64, n // 2), :] = _pk(ft[:n])
        for r in range(0, D3 // 2, 8):
            ops = hk_a_ops(lambda i, j: _up(woT[pl.ds(i * (D3 // 2) + r, 8), j * TC:(j + 1) * TC]))
            for k, t in enumerate(ops):
                wo2[pl.ds(r, 8), _lt(k)] = t
        lo = lax.broadcasted_iota(jnp.int32, (16, 128), 1) < KY
        for r in range(0, hh, 8):
            a3, a4, b3, b4 = [_up(woT[pl.ds(r0 + r, 8), c0:c0 + 128]).astype(f32)
                              for r0 in (0, hh) for c0 in (384, 512)]
            wo2[pl.ds(r, 8), _lt(15)] = _pk(jnp.where(lo, a3, a3 - b3))
            wo2[pl.ds(r, 8), _lt(16)] = _pk(jnp.where(lo, b3, b4 - a4))
            wo2[pl.ds(r, 8), _lt(17)] = _pk(jnp.where(lo, a4, b3))

    def q_left(plain, which=None, dep=None, slot=0):
        k1, k2, k3 = 3 * TC, 3 * TC + KY, 3 * TC + 2 * KY
        for n in (list(range(6 if plain else 15)) + [15, 16, 17]) if which is None else which:
            def X(t, r0, rows):
                return xn_g[t, pl.ds((zero8 if plain else zero(n)) + r0, rows), :]
            if n == 15:
                v = jnp.concatenate([X(0, k1, KY), X(0, k2, KY) - X(1, k2, KY)], axis=0)
            elif n == 16:
                v = jnp.concatenate([X(1, k1, KY), X(1, k3, KY) - X(0, k3, KY)], axis=0)
            elif n == 17:
                v = jnp.concatenate([X(0, k3, KY), X(1, k2, KY)], axis=0)
            elif plain:
                v = X(n // 3, (n % 3) * TC, TC)
            else:
                v = _ssum([(X(t, i * TC, TC), sg) for (i, t), lst in _HK_C.items() for k, sg in lst if k == n])
            if dep is not None:
                v = jnp.concatenate([tie(v[0:8], dep), v[8:]], axis=0)
            sq_scr[n, slot] = pltpu.bitcast(v.astype(bf16).T, u32)

    def add_ln(clock, t0, cfg, blk, dst, par, inp=None):
        np1, np2, step, gap, delay = cfg
        st = dict(s1=[], s2=[], left=np2)
        nv = D // 16

        def load(i):
            if inp is None:
                return xres[blk, pl.ds(zero8 + i * 16, 16), :]
            x = inp(i).astype(f32)
            xres[blk, pl.ds(i * 16, 16), :] = x
            return x

        def stats(k, dep):
            xs = []
            for i in range(k * nv // np1, (k + 1) * nv // np1):
                x = load(i)
                xs += [x[0:8], x[8:16]]
            if k == 0:
                st['c'] = jnp.broadcast_to(xs[0][0:1], (8, TB))
            c = tie(st['c'], dep)
            ds = [x - c for x in xs]
            st['s1'].append(_tree(jnp.add, ds))
            st['s2'].append(_tree(jnp.add, [d * d for d in ds]))
            return pltpu.bitcast(st['s1'][-1], u32) | pltpu.bitcast(st['s2'][-1], u32)

        def norm(k, dep):
            if k == 0:
                m = jnp.sum(_tree(jnp.add, st['s1']), axis=0, keepdims=True) * (1.0 / D)
                v = jnp.sum(_tree(jnp.add, st['s2']), axis=0, keepdims=True) * (1.0 / D) - m * m
                st['mean'] = st['c'] + m
                st['rstd'] = jnp.broadcast_to(lax.rsqrt(jnp.maximum(v, 0.0) + EPS), (8, TB))
            mean = tie(st['mean'], dep)
            off = 0 if inp is None else zero8
            for i in range(k * 2 * nv // np2, (k + 1) * 2 * nv // np2):
                dst[par, pl.ds(i * 8, 8), :] = (xres[blk, pl.ds(off + i * 8, 8), :] - mean) * st['rstd']
            st['left'] -= 1
            return pltpu.bitcast(dst[par, pl.ds(zero8, 8), :], u32)
        for k in range(np1):
            clock.add_due(t0 + k * step, functools.partial(stats, k), delay)
        for k in range(np2):
            clock.add_due(t0 + np1 * step + gap + k * step, functools.partial(norm, k), delay)
        return st

    def hk_outputs(P, T, PT, emit, two_cols):
        p8 = P(8)
        t7 = P(7) + p8
        s1 = PT(3, 1, 2) + t7
        p6 = P(6)
        p14 = P(14)
        emit(1, 1, T(1, 1) + (p6 + p14 + s1))
        p13 = P(13)
        if two_cols:
            emit(1, 0, PT(2, 1, 0) + (p13 + s1))
        else:
            p12 = P(12)
            emit(1, 0, PT(2, 1, 0) + (p12 + p13 + s1))
        p11 = P(11)
        t10 = P(10) + p11
        if not two_cols:
            s2 = PT(5, 2, 2) + t10
            p9 = P(9)
            emit(2, 0, T(2, 0) + (p9 + p12 + s2))
            emit(2, 1, PT(4, 2, 1) + (p14 - p13 + s2))
        w0 = T(0, 2)
        emit(0, 0, PT(0, 0, 0) + ((p8 + t10 + w0) if two_cols else (p8 + p9 + t10 + w0)))
        emit(0, 1, PT(1, 0, 1) + (p6 + p11 + t7 + w0))

    QT = (0, 1, 2, 3)
    KT = (4, 5, 6, 7, 13)
    VT = (8, 9, 10, 11, 12)
    c2e = DH ** -0.5 * math.log2(math.e)
    neg = -1e9 * math.log2(math.e)

    def q_step(pr, cfg=None, chunk=None, rows=False, part=None):
        first = cfg is not None
        clock = _Timeline()
        if part is not None:
            base, nx = 0, 1
            if part < 2:
                transpose_qkv(part + 1)
                probe = pltpu.bitcast(tmp[0, pl.ds(zero8, 8), :], u32)
                clock.add(BT[0], lambda _: clock.due.append(lambda: probe))
                for d in range(DH):
                    clock.add(BT[1] + d * BT[2], functools.partial(build_wq, part + 1, [d]))
            else:
                for k in range(40):
                    clock.add(SUMT[0] + k * SUMT[1], functools.partial(wq_sums, 8 * k))
        elif rows:
            base, nx = pr * (2 * TB), pr + 1
            for k in range(2):
                clock.add_due(QA_T[k], functools.partial(row_chain, k, QA_T[2]), QA_T[3] - QA_T[k])
        else:
            base = pl.multiple_of(pr * (2 * TB), 2 * TB)
            nx = jnp.minimum(pr + 1, NP - 1)
        pieces = []
        if chunk is not None:
            for m in range(3):
                pieces += prep_pieces(jnp.maximum(chunk - LAGS[m], 0) if LAGS[m] else chunk, m)

        def paced(piece, dep):
            pw[0, pl.ds(R_END, 8), 0:128] = pltpu.bitcast(dep, u32)
            piece()
        for k, piece in enumerate(pieces):
            frac = k / 48 * QFR if k < 48 else QFR + (k - 48) / (len(pieces) - 48) * (1 - QFR)
            clock.add(QP0 + int(frac * (QP1 - QP0)), functools.partial(paced, piece))
        if first and part in (None, 2):
            for par in range(2):
                add_ln(clock, cfg[par], cfg[2:], 2 * nx + par, xn_g, par,
                       functools.partial(lambda par_, i: xin[nx, pl.ds(i * 16, 16), par_ * TB:(par_ + 1) * TB], par))
        for r0, nt, tiles in ((0, 2, (0, 4, 8)), (TC, 2, (2, 6, 10)), (2 * TC, 1, (12, 13))):
            def R(k):
                return wq[pl.ds(r0, nt * 64), _lt(k)]

            def L(k):
                return sq_scr[k, 0] if first else jnp.concatenate([sq_scr[k, 0], sq_scr[k, 1]], axis=0)

            def P(k):
                return _dot_nt(_up(L(k)), _up(R(k)))

            def T(j, kind):
                rhs = _up(R(15 + 3 * j + kind))
                if nt == 1 and kind == 2:
                    lhs = L(15 + kind)
                    return jnp.concatenate([_dot_nt(_up(lhs[k:k + 32]), rhs) for k in range(0, lhs.shape[0], 32)],
                                           axis=0)
                return _dot_nt(_up(L(15 + kind)), rhs)

            def PT(k, j, kind):
                return _dot_nt(_up(jnp.concatenate([L(k), L(15 + kind)], axis=1)),
                               _up(jnp.concatenate([R(k), R(15 + 3 * j + kind)], axis=1)))

            def emit(col, half, v):
                for k in range(nt):
                    for q_ in range(2):
                        rows_ = pl.ds(base + (HALO + (2 * q_ + half) * TB), TB)
                        qall[tiles[col] + k, rows_, :] = v[q_ * TB:(q_ + 1) * TB, _lt(k)]
            if not first:
                hk_outputs(P, T, PT, emit, nt == 1)
                continue
            for j in range(len(tiles)):
                if part is not None and (j if nt == 2 else 2) != part:
                    continue
                both = T(j, 2)
                clock.t += 32 * nt
                for t in range(2):
                    for k in range(nt):
                        lhs = [L(3 * t + i) for i in range(3)] + [L(15 + t)]
                        lhs[0] = gate(lhs[0], clock)
                        rhs = [wq[pl.ds(r0 + k * 64, 64), _lt(n)]
                               for n in [wq_slot(i, j) for i in range(3)] + [15 + 3 * j + t]]
                        v = _dot_nt(_up(jnp.concatenate(lhs, axis=1)), _up(jnp.concatenate(rhs, axis=1))) + both[:, _lt(k)]
                        qall[tiles[j] + k, pl.ds(base + (HALO + t * TB), TB), :] = v
                        clock.tick(128, v, QTK)
        assert not clock.pending()
        if first and part in (None, 2):
            q_left(True)

    def row_group(blk, par, r, nw, nv, mids=None):
        base = _al(blk * TB, TB)
        lo = lax.broadcasted_iota(jnp.int32, (RB, 128), 1) < KY
        r0 = r * RB

        def ld(t, w):
            return qall[t, pl.ds(base + (HALO + r0 - DIL * w), RB), :]
        dep = yield
        cs = tie(jnp.full((RB, 128), c2e, f32), dep)
        q = [ld(t, 0) * cs for t in QT] + [jnp.where(lo, pltpu.roll(ld(13, 0), KY, 1), 0.0) * cs]
        sc = []
        for w in range(W):
            if w and w % nw == 0:
                dep = yield
                q = [tie(q[0], dep)] + q[1:]
            acc = None
            for j, t in enumerate(KT):
                p = q[j] * ld(t, w)
                acc = p if acc is None else acc + p
            acc = acc + pltpu.roll(acc, 64, 1)
            if mids is not None:
                mids[r] = pltpu.bitcast(acc, u32)
            acc = acc + pltpu.roll(acc, 32, 1)
            if r0 - DIL * w < 0:
                pos = blk * TB + r0 + lax.broadcasted_iota(jnp.int32, (RB, 128), 0)
                acc = jnp.where(pos >= DIL * w, acc, neg)
            sc.append(acc)
        m = _tree(jnp.maximum, sc)
        e = [jnp.exp2(sc[w] - m) for w in range(W)]
        l = _tree(jnp.add, e)
        rinv = pl.reciprocal(l, approx=True)
        rinv = rinv * (2.0 - l * rinv)
        outs = []
        for j, t in enumerate(VT):
            if j and j % nv == 0:
                dep = yield _tree(jnp.bitwise_or, [pltpu.bitcast(v, u32) for v in outs])
                outs = []
                e = [tie(e[0], dep)] + e[1:]
            acc = None
            for w in range(W):
                p = e[w] * ld(t, w)
                acc = p if acc is None else acc + p
            o = acc * rinv
            o_s[par * 5 + j, pl.ds(r0, RB), :] = o
            outs.append(o)
        yield _tree(jnp.bitwise_or, [pltpu.bitcast(v, u32) for v in outs])

    def add_rows(clock, t0, blk, par, r, cfg):
        nw, nv, step, gap, d1, d2 = cfg
        gen = row_group(blk, par, r, nw, nv)
        next(gen)
        n1, n2 = -(-W // nw), -(-5 // nv)
        for k in range(n1):
            clock.add_due(t0 + k * step, gen.send, d1)
        for k in range(n2 - 1):
            clock.add_due(t0 + (n1 - 1) * step + gap + k * step, gen.send, d2)

    def row_chain(blk, lag, dep):
        mids, fins = {}, {}
        for r in range(nr):
            gen = row_group(blk, blk, r, W, 5, mids)
            next(gen)
            if r:
                dep = pltpu.bitcast(mids[r - 1] | fins[r - lag] if r >= lag else mids[r - 1], f32)
            fins[r] = gen.send(dep)
        return _tree(jnp.bitwise_or, [fins[r] for r in range(nr - lag, nr)])

    wo_seq = []
    for pos, k in enumerate(WORD):
        if pos in (0, 2):
            wo_seq += [('r', pos // 2, k_) for k_ in range(3)]
        wo_seq.append(('p', k))

    def wo_rhs(off):
        lo = lax.broadcasted_iota(jnp.int32, (TB, 128), 1) < KY

        rhs = {}
        for it in wo_seq:
            z = zero(wo_seq.index(it)) if off is None else off

            def O(t, j):
                return o_s[t * 5 + j, pl.ds(z, TB), :]
            if it[0] == 'p':
                v = _ssum([(O(t, j), sg) for j, t, sg in _HK_B[it[1]]])
            elif it[2] == 0:
                v = O(it[1], 3)
            else:
                v = jnp.where(lo, O(it[1], 2 + it[2]), O(it[1], 5 - it[2]))
            rhs[it] = v.astype(bf16)
        return rhs

    def wo_mm(blk0, rhs):
        res = {}
        for it in wo_seq:
            if it[0] == 'p':
                lhs = wo2[pl.ds(0, D3 // 2), _lt(it[1])]
            else:
                lhs = wo2[:, _lt(15 + it[2])]
            res[it] = _dot_nt(_up(lhs), rhs[it])
        for t in range(2):
            both = res['r', t, 2]
            rem = xres[blk0 + t] + jnp.concatenate([res['r', t, 0] + both, res['r', t, 1] + both], axis=0)
            y = jnp.concatenate([_ssum([(res['p', k], sg) for k, sg in _HK_C[i, t]]) for i in range(3)], axis=0)
            xres[blk0 + t] = y + rem

    def a_left(which=range(15), dep=None):
        for n in which:
            v = _ssum([(xn_f[t, pl.ds(zero(n) + i * D3, D3), :], sg)
                       for (i, t), lst in _HK_C.items() for k, sg in lst if k == n])
            if dep is not None:
                v = jnp.concatenate([tie(v[0:8], dep), v[8:2 * KY], tie(v[2 * KY:2 * KY + 8], dep), v[2 * KY + 8:]],
                                    axis=0)
            t1 = pltpu.bitcast(v[:2 * KY].astype(bf16).T, u32)
            t2 = pltpu.bitcast(jnp.concatenate([v[2 * KY:], v[2 * KY:]], axis=0).astype(bf16).T, u32)
            if dep is None:
                arrange(n, t1, t2)
            else:
                st_s[2 * n] = t1
                st_s[2 * n + 1] = t2

    def arrange(n, t1, t2):
        lo = lax.broadcasted_iota(jnp.int32, (TB // 2, 128), 1) < KY
        s_scr[3 * n] = t1
        s_scr[3 * n + 1] = jnp.where(lo, t1, t2)
        s_scr[3 * n + 2] = jnp.where(lo, t2, t1)

    def a_arrange(n, dep):
        st_s[30, pl.ds(0, 8), :] = pltpu.bitcast(dep, u32)
        arrange(n, st_s[2 * n, pl.ds(zero8, TB // 2), :], st_s[2 * n + 1, pl.ds(zero8, TB // 2), :])

    k0 = math.sqrt(2.0 / math.pi)
    k1 = k0 * 0.044715

    def ffn(j, c0, script):
        clock = _Timeline()
        b0 = (2 * j) % NB
        an = (2 * j + 2) % NB
        acc = [None] * 57
        hs = {}
        lns, lq, staged, nrows = [], [], set(), 0

        pend = []

        def advance(keep):
            while len(pend) > keep:
                pend.pop(0)()

        def written(k):
            clock.due.append(lambda: pltpu.bitcast(p_s[k][pl.ds(zero8, 8), 0:128], u32))

        def gu(p):
            c, m = c0 + p // 2, p % 2
            h = hs.setdefault(p // 2, [[None, None, None] for _ in range(3)])

            def mm(n, kind):
                lhs = gate(s_scr[3 * n + kind], clock)
                return _dot(_up(lhs), _up(pw[c, pl.ds((3 * n + kind) * (TC // 2), TC // 2), m * TC:(m + 1) * TC]))

            def get(name):
                return p_s[PSLOT[name]][pl.ds(zero8, TB), :]

            def post(n, v):
                adds, keep, emits = GU_POST[n]
                if keep[0] is not None:
                    p_s[PSLOT[keep[0]]][...] = v
                    written(PSLOT[keep[0]])
                w_ = v
                for name, sg in adds:
                    w_ = w_ + get(name) if sg == 1 else w_ - get(name)
                if keep[1] is not None:
                    p_s[PSLOT[keep[1]]][...] = w_
                    written(PSLOT[keep[1]])
                if emits is not None:
                    col, half = emits
                    if m == 1:
                        k_ = 17 + 9 * ((p // 2) % NHS) + 3 * col
                        hv = w_ * p_s[11 + 2 * col + half][pl.ds(zero8, TB), :]
                        p_s[k_ + half][...] = hv
                        written(k_ + half)
                        h[col][half] = k_ + half
                        if h[col][1 - half] is not None:
                            p_s[k_ + 2][...] = hv + p_s[k_ + 1 - half][pl.ds(zero8, TB), :]
                            written(k_ + 2)
                            h[col][2] = k_ + 2
                    else:
                        p_s[11 + 2 * col + half][...] = w_ + w_ * jnp.tanh(w_ * (k0 + k1 * (w_ * w_)))
                        written(11 + 2 * col + half)
            for n in GU_ORD:
                both = mm(n, 2)
                v = jnp.concatenate([mm(n, 0) + both, mm(n, 1) + both], axis=1)
                pend.append(functools.partial(post, n, v))
                advance(PLAG)
                clock.tick(96, both, GTK)

        todo = [sum(any(i_ == i for i_, _, _ in z) for z in _Z6) for i in range(6)]

        def gather(i):
            ys = [_ssum([(acc[n], sg) for n, sg in sorted(_C6[i, t], key=lambda z: D_ORD.index(z[0]))])
                  for t in range(2)]
            for t in range(2):
                x2 = xres[b0 + t, pl.ds(i * D6, D6), :] + 0.5 * ys[t]
                xres[b0 + t, pl.ds(i * D6, D6), :] = x2
                xin[j % NP, pl.ds(i * D6, D6), t * TB:(t + 1) * TB] = x2.astype(bf16)
            if last and i in ORD6[:OSPL]:
                @pl.when(g == 1)
                def _():
                    _cp_rows(i, o_hbm, xin, sems).start()

        def down(ps, final):
            cs = ps[::2]
            hsl = [hs.pop(p // 2) for p in cs]
            for pos, i in enumerate(D_ORD):
                while any(h_[j_ % 3][d_] is None for h_ in hsl for j_, d_, _ in _B6[i]):
                    advance(len(pend) - 1)
                au = [pw[c0 + p // 2, pl.ds(R_SD + (i // 2) * (D6 // 2), D6 // 2), _lt(i % 2)] for p in cs]
                au[0] = gate(au[0], clock)
                lhs = jnp.concatenate(au, axis=1)
                rhs = jnp.concatenate([_ssum([(p_s[h_[j_ % 3][d_]][pl.ds(zero(pos % 21), TB), _lt(j_ // 3)], sg)
                                              for j_, d_, sg in _B6[i]]) for h_ in hsl], axis=1).astype(bf16)
                r = _dot_nt(_up(lhs), rhs)
                acc[i] = r if acc[i] is None else r + acc[i]
                if final:
                    for i_ in sorted({i_ for i_, _, _ in _Z6[i]}):
                        todo[i_] -= 1
                        if not todo[i_]:
                            gather(i_)
                if pos % DADV == 0:
                    advance(max(len(pend) - 1, 0))
                clock.tick(24 * len(cs), acc[i], DTK)

        pg = pd = 0
        for tok in script:
            if tok == 'G':
                gu(pg)
                pg += 1
            elif tok[0] == 'D':
                down(list(range(pd, pd + int(tok[1:]))), pd + int(tok[1:]) == script.count('G'))
                pd += int(tok[1:])
            elif tok == 'W':
                assert not clock.pending() and nrows == 2 * nr
                advance(0)
                wo_mm(an, wo_rhs(None))
                clock.t += 1152
            elif tok[0] == 'n':
                lns.append(add_ln(clock, clock.t + int(tok[3:]), LNJ + (JDL,), an + int(tok[1]), xn_f, int(tok[1])))
            elif tok[0] == 'm':
                lq.append(add_ln(clock, clock.t + int(tok[3:]), LNJ + (JDL,), (2 * j + 6) % NB + int(tok[1]), xn_g,
                                 int(tok[1])))
            elif tok[0] == 'k':
                _, t0, dt = tok.split('+')

                def qleft(which, dep):
                    assert len(lq) == 2 and not any(st['left'] for st in lq)
                    q_left(False, which, dep, (j + 1) % 2)
                    return sq_scr[which[0], (j + 1) % 2, pl.ds(zero8, 8), :]
                for k in range(NQL):
                    clock.add_due(clock.t + int(t0) + k * int(dt),
                                  functools.partial(qleft, range(k * 18 // NQL, (k + 1) * 18 // NQL)), LDL)
            elif tok[0] == 'l':
                _, t0, dt = tok.split('+')

                def left(which, dep):
                    assert len(lns) == 2 and not any(st['left'] for st in lns)
                    staged.update(which)
                    a_left(which, dep)
                    return st_s[0, pl.ds(zero8, 8), :]
                for k in range(NLEFT):
                    clock.add_due(clock.t + int(t0) + k * int(dt),
                                  functools.partial(left, range(k * 15 // NLEFT, (k + 1) * 15 // NLEFT)), LDL)
            elif tok[0] == 'c':
                _, t0, dt = tok.split('+')
                assert pg == 2 * NCH

                def place(k, dep):
                    assert k in staged
                    a_arrange(k, dep)
                for k in range(15):
                    clock.add(clock.t + int(t0) + k * int(dt), functools.partial(place, k))
            else:
                n, t0, dt = tok[1:].split('+')
                for k in range(int(n)):
                    add_rows(clock, clock.t + int(t0) + k * int(dt), an + nrows // nr, nrows // nr, nrows % nr,
                             RG + (RDL, JDL))
                    nrows += 1
        assert pg == pd and not clock.pending()

    if last:
        ffn(2 * NP - 1, g * NPC, SCRIPT_F)
        return
    if phase == 'main':
        @pl.when(jnp.logical_and(g >= NP - 1, (g & 1) == 1))
        def _():
            q_step(g - (NP - 1))

        ffn(g, 0, SCRIPT)

        @pl.when(g >= NP)
        def _():
            _cp_out(g - NP, o_hbm, xin, sems).start()
        return
    assert NCH == NP - 2

    late = [(c, m) for c in range(NCH) for m in range(3) if c >= NCH - LAGS[m]]

    def prologue():
        cp_x(0).start()
        for sec in range(3):
            for cp in cp_qkv(sec):
                cp.start()
        qall[:, pl.ds(0, HALO), :] = jnp.zeros((16, HALO, 128), f32)
        cp_x(0).wait()
        for t in range(2):
            x = xin[0, :, t * TB:(t + 1) * TB].astype(f32)
            xres[t] = x
            mean, rstd = _ln_stats(x)
            xn_g[t, pl.ds(zero8, D), :] = (xres[t] - mean) * rstd
        q_left(True)
        for sec in range(3):
            for cp in cp_qkv(sec):
                cp.wait()
            if sec == 0:
                cp_x(1).start()
                cp_x(2).start()
                cp_wo().start()
                for c in range(NCH):
                    if 3 + c < NP:
                        cp_x(3 + c).start()
                    for m in range(3):
                        if c == 0 or c > LAGS[m]:
                            cp_unit(max(c - LAGS[m], 0), m).start()
                for c, m in late:
                    cp_unit(c, m).start()
            if sec == 0:
                transpose_qkv(sec)
                build_wq(sec)
            else:
                q_step(0, CFG_Q0, part=sec - 1)

    def first_attention():
        cp_x(2).wait()
        q_step(1, CFG_QA, rows=True)
        cp_wo().wait()
        build_wo()
        wo_mm(0, wo_rhs(0))
        for t in range(2):
            mean, rstd = _ln_stats(xres[t])
            xn_f[t] = (xres[t] - mean) * rstd
        a_left()

    def startup_step(c, carry):
        @pl.when(c + 3 < NP)
        def _():
            cp_x(c + 3).wait()
        for m in range(3):
            if LAGS[m]:
                @pl.when(jnp.logical_or(c == 0, c > LAGS[m]))
                def _():
                    cp_unit(jnp.maximum(c - LAGS[m], 0), m).wait()
            else:
                cp_unit(c, m).wait()
        q_step(c + 2, CFG_Q1, chunk=c)
        return carry

    @pl.when(g == 0)
    def _():
        prologue()
        cp_x(1).wait()
        q_step(0, CFG_Q0, part=2)
        first_attention()
        lax.fori_loop(0, NCH, startup_step, 0)
        for c, m in late:
            cp_unit(c, m).wait()
        for c, m in late:
            for piece in prep_pieces(c, m):
                piece()


def _cp_out(k, o_hbm, xin, sems):
    return pltpu.make_async_copy(xin.at[k], o_hbm.at[:, pl.ds(_al(k * 2 * TB, 128), 2 * TB)], sems.at[4 + k])


def _cp_rows(i, o_hbm, xin, sems):
    k, n = xin.shape[0] - 1, xin.shape[1] // 6
    return pltpu.make_async_copy(xin.at[k, pl.ds(i * n, n), :], o_hbm.at[pl.ds(i * n, n), pl.ds(k * 2 * TB, 2 * TB)],
                                 sems.at[4 + k])


def _kernel(*refs, D, DF, S):
    def body(phase, g, carry):
        _step(g, phase, *refs, D=D, DF=DF, S=S)
        return carry
    NP = S // (2 * TB)
    lax.fori_loop(0, 2, functools.partial(body, 'start'), 0)
    lax.fori_loop(0, 2 * NP - 1, functools.partial(body, 'main'), 0)
    lax.fori_loop(0, 2, functools.partial(body, 'last'), 0)
    o_hbm, xin, sems = refs[6], refs[7], refs[24]
    for i in ORD6[OSPL:]:
        _cp_rows(i, o_hbm, xin, sems).start()
    for k in range(NP - 1):
        _cp_out(k, o_hbm, xin, sems).wait()
    for i in range(6):
        _cp_rows(i, o_hbm, xin, sems).wait()


@jax.jit
def pallas_interleave_layers__sliding_local_dilated__glu_gated_geglu__prompt_kernel(
    A_x, A_wqkv, A_wo, B_x, B_w_gate, B_w_up, B_w_down):
    B, S, D = A_x.shape
    DF = B_w_gate.shape[1]
    NB = S // TB
    NP = NB // 2
    NCH = DF // CW
    xT = A_x.reshape(S, D).T
    wdT = B_w_down.T
    hbm = pl.BlockSpec(memory_space=pltpu.HBM)
    outT = pl.pallas_call(
        functools.partial(_kernel, D=D, DF=DF, S=S),
        in_specs=[hbm] * 6,
        out_specs=hbm,
        out_shape=jax.ShapeDtypeStruct((D, S), A_x.dtype),
        scratch_shapes=[
            pltpu.VMEM((NP, D, 2 * TB), bf16),
            pltpu.VMEM((D, 3 * D), bf16),
            pltpu.VMEM((D, D), bf16),
            pltpu.VMEM((5, 14 * 128, 128), f32),
            pltpu.VMEM((WQR, 27 * 128), u32),
            pltpu.VMEM((D // 2, 640), u32),
            pltpu.VMEM((D // 4, 18 * 128), u32),
            pltpu.VMEM((NCH, 3, D, CW), bf16),
            pltpu.VMEM((NCH, 45 * (TC // 2) + 15 * (D // 6) + 16, 2 * TC), u32),
            pltpu.VMEM((16, S + QPAD, 128), f32),
            pltpu.VMEM((11, TB, 128), f32),
            pltpu.VMEM((NB, D, TB), f32),
            pltpu.VMEM((2, D, TB), f32),
            pltpu.VMEM((2, D, TB), f32),
            pltpu.VMEM((45, TB // 2, TC), u32),
            pltpu.VMEM((31, TB // 2, TC), u32),
            pltpu.VMEM((18, 2, TB // 2, TC), u32),
            pltpu.SemaphoreType.DMA((4 + NP + 3 * NCH,)),
        ] + [pltpu.VMEM((TB, 2 * TC), f32)] * (17 + 9 * NHS),
        compiler_params=pltpu.CompilerParams(
            vmem_limit_bytes=110 * 1024 * 1024,
            disable_bounds_checks=True,
            disable_semaphore_checks=True,
        ),
    )(xT, A_wqkv, A_wo, B_w_gate, B_w_up, wdT)
    return outT.T.reshape(B, S, D)
```
